```python
import jax
import jax.numpy as jnp

def _softmax(x, axis=-1):
    return jax.nn.softmax(x, axis=axis)

def _gelu(x):
    return jax.nn.gelu(x, approximate=True)

def _silu(x):
    return jax.nn.silu(x)

def _sigmoid(x):
    return jax.nn.sigmoid(x)

def _layernorm(x, axis=-1, eps=1e-05):
    m = jnp.mean(x, axis=axis, keepdims=True)
    v = jnp.var(x, axis=axis, keepdims=True)
    return (x - m) / jnp.sqrt(v + eps)

def _scatter_add(tgt, idx, src, axis=0):
    return tgt.at[idx].add(src)

def _segment_sum(src, seg, n):
    return jax.ops.segment_sum(src, seg, n)

class _Rng:

    def __init__(self, key):
        self._k = key

    def _next(self):
        self._k, sub = jax.random.split(self._k)
        return sub

    def normal(self, shape):
        return jax.random.normal(self._next(), shape, dtype=jnp.bfloat16)

    def randint(self, lo, hi, shape):
        return jax.random.randint(self._next(), shape, lo, hi, dtype=jnp.int32)

    def uniform(self, shape, lo=0.0, hi=1.0):
        return jax.random.uniform(self._next(), shape, jnp.bfloat16, lo, hi)

    def permutation(self, n):
        return jax.random.permutation(self._next(), n)
kernel_name = 'interleave_layers__memory_aug_recurrent_mem_tr__ssm_conv_h3__prompt'

def setup_inputs():
    _rng = _Rng(jax.random.key(int.from_bytes(__import__("os").urandom(4), "little")))
    _w = lambda a: (lambda t: t.astype(jnp.bfloat16) if jnp.issubdtype(t.dtype, jnp.floating) else t)(jnp.asarray(a))

    def _A_setup():
        B, S, Dm = (1, 2048, 640)
        H, Dh = (32, 128)
        M, seg = (8, 32)
        seg = min(seg, S)
        S = S // seg * seg
        return {'x': _w((lambda *s: _rng.normal(s) * 0.05)(B, S, Dm)), 'mem0': _w((lambda *s: _rng.normal(s) * 0.05)(B, M, Dm)), 'Wq': _w((lambda *s: _rng.normal(s) * 0.05)(Dm, H, Dh) * Dm ** (-0.5)), 'Wk': _w((lambda *s: _rng.normal(s) * 0.05)(Dm, H, Dh) * Dm ** (-0.5)), 'Wv': _w((lambda *s: _rng.normal(s) * 0.05)(Dm, H, Dh) * Dm ** (-0.5)), 'Wo': _w((lambda *s: _rng.normal(s) * 0.05)(H, Dh, Dm) * (H * Dh) ** (-0.5)), 'seg_len': seg}
    _A_in = _A_setup()

    def _B_setup():
        B, S, D = (1, 2048, 640)
        ks = 4
        return {'q': _w((lambda *s: _rng.normal(s) * 0.05)(B, S, D)), 'k': _w((lambda *s: _rng.normal(s) * 0.05)(B, S, D)), 'v': _w((lambda *s: _rng.normal(s) * 0.05)(B, S, D)), 'shift_k': _w((lambda *s: _rng.normal(s) * 0.05)(D, ks) * 0.5), 'ssm_k': _w((lambda *s: _rng.normal(s) * 0.05)(D, S) * (1.0 / S ** 0.5)), 'ssm_D': _w((lambda *s: _rng.normal(s) * 0.05)(D))}
    _B_in = _B_setup()
    return {'A_x': _A_in['x'], 'A_mem0': _A_in['mem0'], 'A_Wq': _A_in['Wq'], 'A_Wk': _A_in['Wk'], 'A_Wv': _A_in['Wv'], 'A_Wo': _A_in['Wo'], 'A_seg_len': _A_in['seg_len'], 'B_q': _B_in['q'], 'B_k': _B_in['k'], 'B_v': _B_in['v'], 'B_shift_k': _B_in['shift_k'], 'B_ssm_k': _B_in['ssm_k'], 'B_ssm_D': _B_in['ssm_D']}

def reference(A_x, A_mem0, A_Wq, A_Wk, A_Wv, A_Wo, A_seg_len, B_q, B_k, B_v, B_shift_k, B_ssm_k, B_ssm_D):

    def _A_ref(x, mem0, Wq, Wk, Wv, Wo, seg_len):
        B, S, Dm = x.shape
        H, Dh = (Wq.shape[1], Wq.shape[2])
        M = mem0.shape[1]
        scale = Dh ** (-0.5)
        n_seg = S // seg_len
        L = M + seg_len
        idx = jnp.arange(L)
        mask = (idx[:, None] < M) | (idx[:, None] >= idx[None, :])
        mem = mem0
        outs = []
        for s in range(n_seg):
            xs = x[:, s * seg_len:(s + 1) * seg_len, :].copy()
            h = jnp.concatenate([mem, xs], axis=1)
            q = jnp.einsum('btd,dhe->bhte', h, Wq)
            k = jnp.einsum('btd,dhe->bhte', h, Wk)
            v = jnp.einsum('btd,dhe->bhte', h, Wv)
            scores = jnp.einsum('bhqe,bhke->bhqk', q, k) * scale
            scores = jnp.where(mask[None, None], scores, -1000000000.0)
            p = _softmax(scores, axis=-1)
            o = jnp.einsum('bhqk,bhke->bhqe', p, v)
            o = jnp.einsum('bhte,hed->btd', o, Wo)
            mem = o[:, :M, :].copy()
            outs.append(o[:, M:, :])
        return jnp.concatenate(outs, axis=1)

    def _B_ref(q, k, v, shift_k, ssm_k, ssm_D):
        B, S, D = q.shape
        ks = shift_k.shape[-1]
        k_pad = jnp.pad(k, ((0, 0), (ks - 1, 0), (0, 0)))
        k_shift = jnp.zeros_like(k)
        for t in range(ks):
            k_shift = k_shift + k_pad[:, t:t + S, :] * shift_k[:, ks - 1 - t][None, None, :]
        kv = k_shift * v
        L = 2 * S
        kv_pad = jnp.pad(kv, ((0, 0), (0, S), (0, 0)))
        kf_pad = jnp.pad(ssm_k, ((0, 0), (0, S)))
        kv_f = (lambda x, axes=(-2, -1): jnp.fft.rfft2(x.astype(jnp.float32), axes=axes))(kv_pad[:, None, :, :], axes=(1, 2))
        kf_f = (lambda x, axes=(-2, -1): jnp.fft.rfft2(x.astype(jnp.float32), axes=axes))(kf_pad[:, None, :], axes=(1, 2))
        kf_f = (lambda x, *d: x.transpose(*d))(kf_f, 1, 2, 0)
        y_f = kv_f * kf_f[None, :, :, :]
        y = (lambda x, s, axes=(-2, -1): jnp.fft.irfft2(x, s=s, axes=axes).astype(jnp.bfloat16))(y_f, (1, L), axes=(1, 2))[:, 0, :S, :]
        y = y + kv * ssm_D[None, None, :]
        return q * y
    x = A_x
    x = x + _A_ref(_layernorm(x, axis=-1), A_mem0, A_Wq, A_Wk, A_Wv, A_Wo, A_seg_len)
    x = x + _B_ref(_layernorm(x, axis=-1), B_k, B_v, B_shift_k, B_ssm_k, B_ssm_D)
    x = x + _A_ref(_layernorm(x, axis=-1), A_mem0, A_Wq, A_Wk, A_Wv, A_Wo, A_seg_len)
    x = x + _B_ref(_layernorm(x, axis=-1), B_k, B_v, B_shift_k, B_ssm_k, B_ssm_D)
    return x
```

```python
import functools
import math

import jax
import jax.numpy as jnp
from jax import lax
import jax.experimental.pallas as pl
import jax.experimental.pallas.tpu as pltpu

F32 = jnp.float32
BF16 = jnp.bfloat16
U32 = jnp.uint32

S = 2048
D = 640
H = 32
DH = 128
M = 8
SEG = 32
NSEG = S // SEG
KS = 4
LAG = 2
ROWS = 2 * M + 2 * SEG
HG = 4
NG = H // HG
NLB = D // 128
TB = 128
NB = S // TB
WP = 324


def _ln(x):
    m = jnp.mean(x, axis=-1, keepdims=True)
    c = x - m
    v = jnp.mean(c * c, axis=-1, keepdims=True)
    return c * lax.rsqrt(v + 1e-5)


def _r(x):
    return x.astype(BF16).astype(F32)


def _split(x):
    hi = x.astype(BF16)
    lo = (x - hi.astype(F32)).astype(BF16)
    return hi, lo


def _dft_tables(f_axis):
    fi = lax.broadcasted_iota(jnp.int32, (TB, TB), f_axis)
    t = lax.broadcasted_iota(jnp.int32, (TB, TB), 1 - f_axis)
    f = jnp.where(fi < TB // 2, 2 * fi, 2 * fi - (TB - 1))
    n = ((2 * f + 1) * t) & (4 * TB - 1)
    n = jnp.where(n >= 2 * TB, n - 4 * TB, n)
    ang = n.astype(F32) * (2.0 * math.pi / (4 * TB))
    return jnp.cos(ang), jnp.sin(ang)


def _kernel(x_hbm, mem0_ref, wq_hbm, wk_hbm, wv_hbm, wo_hbm,
            k_hbm, v_hbm, shk_ref, ssmk_hbm, ssmd_ref,
            out_ref,
            x_s, k_s, v_s, ssmk_s, wraw, wt, wo_s,
            fwd_s, inv_s, kpad, kv_s, u_s, kf_s, c_s, y_s,
            hbuf, obuf, x2_s,
            sem_c, sem_w, sem_o, sem_x):
    def conv_copies(j):
        r0 = j * TB if isinstance(j, int) else pl.multiple_of(j * TB, TB)
        return (
            pltpu.make_async_copy(k_hbm.at[pl.ds(r0, TB), :], k_s.at[pl.ds(r0, TB), :], sem_c.at[j]),
            pltpu.make_async_copy(v_hbm.at[pl.ds(r0, TB), :], v_s.at[pl.ds(r0, TB), :], sem_c.at[NB + j]),
            pltpu.make_async_copy(ssmk_hbm.at[:, pl.ds(r0, TB)], ssmk_s.at[j], sem_c.at[2 * NB + j]),
        )
    for j in range(NB):
        for c in conv_copies(j):
            c.start()
    w_copies = [pltpu.make_async_copy(w, wraw.at[t], sem_w.at[t])
                for t, w in enumerate((wq_hbm, wk_hbm, wv_hbm))]
    x_copy = pltpu.make_async_copy(x_hbm, x_s, sem_x.at[0])
    wo_copies = [pltpu.make_async_copy(wo_hbm.at[:, pl.ds(n * 128, 128)], wo_s.at[n], sem_o.at[n])
                 for n in range(NLB)]
    for c in w_copies:
        c.start()
    x_copy.start()
    for c in wo_copies:
        c.start()

    cf, sf = _dft_tables(0)
    fh, fl = _split(jnp.concatenate([cf, sf], axis=0))
    fwd_s[...] = jnp.concatenate([fh, fl], axis=1)
    cg, sg = _dft_tables(1)
    gh, gl = _split(jnp.concatenate([cg, sg], axis=1) * (1.0 / TB))
    inv_s[...] = jnp.concatenate([gh, gl, gh], axis=1)

    shk = shk_ref[...].astype(F32)
    taps = []
    for j in range(KS):
        parts = []
        for g in range(NLB):
            col = jnp.broadcast_to(shk[g * 128:(g + 1) * 128, j:j + 1], (128, 128))
            parts.append(col.T[0:1, :])
        taps.append(parts)
    dvec = ssmd_ref[...].astype(F32)
    for g in range(NLB):
        kpad[g, 0:8, :] = jnp.zeros((8, 128), F32)
    c_s[0] = jnp.zeros(c_s.shape[1:], F32)

    def fwd_stage(j):
        for c in conv_copies(j):
            c.wait()
        r0 = pl.multiple_of(j * TB, TB)
        parts = []
        for g in range(NLB):
            lb = slice(g * 128, (g + 1) * 128)
            kb = k_s[pl.ds(r0, TB), lb].astype(F32)
            kpad[g, pl.ds(r0 + 8, TB), :] = kb
            acc = kb * taps[0][g]
            for t in range(1, KS):
                acc = acc + kpad[g, pl.ds(r0 + 8 - t, TB), :] * taps[t][g]
            parts.append((_r(acc) * v_s[pl.ds(r0, TB), lb].astype(F32)).astype(BF16))
        u = jnp.concatenate(parts, axis=1)
        kv_s[pl.ds(r0, TB), :] = u
        f2 = fwd_s[...]
        uf = jnp.dot(f2, jnp.concatenate([u, u], axis=0), preferred_element_type=F32)
        u_s[j, 0] = uf[0:TB]
        u_s[j, 1] = uf[TB:]
        kb = ssmk_s[j]
        kf = lax.dot_general(f2, jnp.concatenate([kb, kb], axis=1),
                             (((1,), (1,)), ((), ())), preferred_element_type=F32)
        kr, ki = kf[0:TB], kf[TB:]
        kf_s[j, 0] = kr
        kf_s[j, 1] = ki - kr
        kf_s[j, 2] = kr + ki

    HB = NB // 2

    def mac_stage(jj, second):
        for rg in range(2):
            rs = pl.ds(pl.multiple_of((2 * jj + rg) * 8, 8), 8)
            for g in range(NLB):
                lb = slice(g * 128, (g + 1) * 128)
                outs = range(HB, NB) if second else range(0, NB - 1)
                sums = []
                for p in range(3):
                    def uu(i):
                        if p == 0:
                            return u_s[i, 0, rs, lb] + u_s[i, 1, rs, lb]
                        return u_s[i, p - 1, rs, lb]
                    if second:
                        pairs = [(a, b) for a in range(NB) for b in range(NB)
                                 if a + b < NB and (a >= HB or b >= HB)]
                    else:
                        pairs = [(a, b) for a in range(HB) for b in range(HB)]
                    ua = {a: uu(a) for a in sorted({a for a, _ in pairs})}
                    kb = {b: kf_s[b, p, rs, lb] for b in sorted({b for _, b in pairs})}
                    acc = {}
                    for a, b in pairs:
                        t = ua[a] * kb[b]
                        acc[a + b] = t if a + b not in acc else acc[a + b] + t
                    sums.append(acc)
                for i in outs:
                    re = sums[0][i] - sums[2][i]
                    im = sums[0][i] + sums[1][i]
                    if second and i < NB - 1:
                        re = re + c_s[i + 1, 0, rs, lb]
                        im = im + c_s[i + 1, 1, rs, lb]
                    c_s[i + 1, 0, rs, lb] = re
                    c_s[i + 1, 1, rs, lb] = im

    def inv_stage(i):
        hb = TB // 2
        cr, ci = c_s[i + 1, 0], c_s[i + 1, 1]
        pr, pi = c_s[i, 0], c_s[i, 1]
        c = jnp.concatenate([cr[:hb] + pi[:hb], cr[hb:] - pi[hb:],
                             ci[:hb] - pr[:hb], ci[hb:] + pr[hb:]], axis=0)
        ch, cl = _split(c)
        y = jnp.dot(inv_s[...], jnp.concatenate([ch, ch, cl], axis=0),
                    preferred_element_type=F32)
        r0 = pl.multiple_of(i * TB, TB)
        kv = kv_s[pl.ds(r0, TB), :].astype(F32)
        y_s[pl.ds(r0, TB), :] = (_r(y) + _r(kv * dvec)).astype(BF16)

    def relayout(t):
        w_copies[t].wait()

        def body(i, _):
            for dd in range(8):
                dp = i * 8 + dd
                a = pltpu.bitcast(wraw[t, 2 * dp], U32)
                b = pltpu.bitcast(wraw[t, 2 * dp + 1], U32)
                lo = (a & jnp.uint32(0xFFFF)) | (b << 16)
                hi = (a >> 16) | (b & jnp.uint32(0xFFFF0000))
                wt[pl.ds(t * H * WP + dp, 16, stride=WP), :] = lo
                wt[pl.ds((t * H + 16) * WP + dp, 16, stride=WP), :] = hi
            return 0
        lax.fori_loop(0, D // 16, body, 0)

    def wslab(t, h):
        s0 = (t * H + (h % 2) * 16 + h // 2) * WP
        return pltpu.bitcast(wt[s0:s0 + D // 2, :], BF16)

    def loop(n, fn):
        def body(j, _):
            fn(j)
            return 0
        lax.fori_loop(0, n, body, 0)

    with jax.named_scope("conv_a"):
        loop(HB, fwd_stage)
    with jax.named_scope("conv_b"):
        loop(HB, lambda j: (fwd_stage(j + HB), mac_stage(j, False)))
    with jax.named_scope("rel0"):
        relayout(0)
    with jax.named_scope("conv_c"):
        loop(HB, lambda j: (inv_stage(j), mac_stage(j, True)))
    with jax.named_scope("rel1"):
        relayout(1)
    with jax.named_scope("conv_d"):
        loop(HB, lambda j: inv_stage(j + HB))
    with jax.named_scope("rel2"):
        relayout(2)
    with jax.named_scope("waitx"):
        x_copy.wait()
        for c in wo_copies:
            c.wait()

    qi = lax.broadcasted_iota(jnp.int32, (ROWS, ROWS), 0)
    kj = lax.broadcasted_iota(jnp.int32, (ROWS, ROWS), 1)

    def layer_of(i):
        return jnp.where(i < 2 * M, i // M, (i - 2 * M) // SEG)
    same = layer_of(qi) == layer_of(kj)
    vis = same & ((qi < 2 * M) | (qi >= kj))
    fill = jnp.where(same, -1e9, -jnp.inf).astype(F32)
    scale = DH ** -0.5

    mem0 = mem0_ref[...].astype(F32)
    hbuf[0:16, :] = jnp.concatenate([mem0, mem0], axis=0).astype(BF16)
    hbuf[16:48, :] = _ln(x_s[0:SEG, :].astype(F32)).astype(BF16)
    hbuf[48:80, :] = jnp.zeros((SEG, D), BF16)
    obuf[...] = jnp.zeros((2 * SEG, D), F32)
    x2_s[...] = jnp.zeros(x2_s.shape, F32)

    def gate(xa, r0):
        return xa + _r(_r(_ln(xa)) * y_s[pl.ds(r0, SEG), :].astype(F32))

    def step(s):
        h = hbuf[...]
        r1 = pl.multiple_of(jnp.clip(s - 1, 0, NSEG - 1) * SEG, SEG)
        xb2 = _r(gate(_r(x_s[pl.ds(r1, SEG), :].astype(F32) + obuf[0:SEG, :]), r1))
        h2n = _ln(xb2).astype(BF16)
        r3 = pl.multiple_of(jnp.clip(s - 1 - LAG, 0, NSEG - 1) * SEG, SEG)
        xo = gate(_r(x2_s[(s + 4 - 1 - LAG) % 4] + obuf[SEG:2 * SEG, :]), r3)
        out_ref[pl.ds(r3, SEG), :] = xo.astype(BF16)
        x2_s[(s + 4 - 1) % 4] = xb2
        rn = pl.multiple_of(jnp.clip(s + 1, 0, NSEG - 1) * SEG, SEG)
        h1n = _ln(x_s[pl.ds(rn, SEG), :].astype(F32)).astype(BF16)

        def proj(g):
            return [[jnp.dot(h, wslab(t, g * HG + j), preferred_element_type=F32).astype(BF16)
                     for j in range(HG)] for t in range(3)]

        def probs(qkv):
            scs = [lax.dot_general(qkv[0][j], qkv[1][j], (((1,), (1,)), ((), ())),
                                   preferred_element_type=F32) for j in range(HG)]
            ps = []
            for sc in scs:
                sc = jnp.where(vis, sc * scale, fill)
                e = jnp.exp(sc - jnp.max(sc, axis=-1, keepdims=True))
                den = jnp.sum(e, axis=-1, keepdims=True)
                r = pl.reciprocal(den, approx=True)
                r = r * (2.0 - den * r)
                ps.append((e * r).astype(BF16))
            return ps

        def oproj(os_, h0):
            oc = jnp.concatenate(os_, axis=1)
            k0, k1 = h0 * DH, (h0 + len(os_)) * DH
            return [jnp.dot(oc, wo_s[n, k0:k1, :], preferred_element_type=F32)
                    for n in range(NLB)]

        heads = []
        qkv = proj(0)
        oa = None
        for g in range(NG):
            ps = probs(qkv)
            vs = qkv[2]
            if g + 1 < NG:
                qkv = proj(g + 1)
            else:
                oa = oproj(heads[:H // 2], 0)
            heads += [jnp.dot(ps[j], vs[j], preferred_element_type=F32).astype(BF16)
                      for j in range(HG)]
        ob = oproj(heads[H // 2:], H // 2)
        o = jnp.concatenate([a + b for a, b in zip(oa, ob)], axis=1)

        mem2 = jnp.where(s == LAG - 1, mem0, o[M:2 * M])
        hbuf[0:16, :] = jnp.concatenate([o[0:M], mem2], axis=0).astype(BF16)
        hbuf[16:48, :] = h1n
        hbuf[48:80, :] = h2n
        obuf[...] = _r(o[2 * M:])

    with jax.named_scope("main"):
        loop(NSEG + LAG, step)

    r3 = (NSEG - 1) * SEG
    xo = gate(_r(x2_s[(NSEG - 1) % 4] + obuf[SEG:2 * SEG, :]), r3)
    out_ref[r3:r3 + SEG, :] = xo.astype(BF16)


@functools.partial(jax.jit, static_argnames=("A_seg_len",))
def pallas_interleave_layers__memory_aug_recurrent_mem_tr__ssm_conv_h3__prompt_kernel(
    A_x, A_mem0, A_Wq, A_Wk, A_Wv, A_Wo, A_seg_len,
    B_q, B_k, B_v, B_shift_k, B_ssm_k, B_ssm_D,
):
    assert A_seg_len == SEG and A_x.shape == (1, S, D)
    vm = pl.BlockSpec(memory_space=pltpu.VMEM)
    hbm = pl.BlockSpec(memory_space=pl.ANY)
    out = pl.pallas_call(
        _kernel,
        out_shape=jax.ShapeDtypeStruct((S, D), BF16),
        in_specs=[hbm, vm, hbm, hbm, hbm, hbm, hbm, hbm, vm, hbm, vm],
        out_specs=vm,
        scratch_shapes=[
            pltpu.VMEM((S, D), BF16),
            pltpu.VMEM((S, D), BF16),
            pltpu.VMEM((S, D), BF16),
            pltpu.VMEM((NB, D, TB), BF16),
            pltpu.VMEM((3, D, H, DH), BF16),
            pltpu.VMEM((3 * H * WP, 128), U32),
            pltpu.VMEM((NLB, H * DH, 128), BF16),
            pltpu.VMEM((2 * TB, 2 * TB), BF16),
            pltpu.VMEM((TB, 6 * TB), BF16),
            pltpu.VMEM((NLB, S + 8, 128), F32),
            pltpu.VMEM((S, D), BF16),
            pltpu.VMEM((NB, 2, TB, D), F32),
            pltpu.VMEM((NB, 3, TB, D), F32),
            pltpu.VMEM((NB + 1, 2, TB, D), F32),
            pltpu.VMEM((S, D), BF16),
            pltpu.VMEM((ROWS, D), BF16),
            pltpu.VMEM((2 * SEG, D), F32),
            pltpu.VMEM((4, SEG, D), F32),
            pltpu.SemaphoreType.DMA((3 * NB,)),
            pltpu.SemaphoreType.DMA((3,)),
            pltpu.SemaphoreType.DMA((NLB,)),
            pltpu.SemaphoreType.DMA((1,)),
        ],
        compiler_params=pltpu.CompilerParams(vmem_limit_bytes=120 * 1024 * 1024),
    )(A_x.reshape(S, D), A_mem0.reshape(M, D), A_Wq, A_Wk, A_Wv,
      A_Wo.reshape(H * DH, D), B_k.reshape(S, D), B_v.reshape(S, D),
      B_shift_k, B_ssm_k, B_ssm_D.reshape(1, D))
    return out.reshape(1, S, D)
```

```python
import functools
import math

import jax
import jax.numpy as jnp
from jax import lax
import jax.experimental.pallas as pl
import jax.experimental.pallas.tpu as pltpu

F32 = jnp.float32
BF16 = jnp.bfloat16
U32 = jnp.uint32

S = 2048
D = 640
H = 32
DH = 128
M = 8
SEG = 32
NSEG = S // SEG
KS = 4
LAG = 2
ROWS = 2 * M + 2 * SEG
HG = 4
NG = H // HG
NLB = D // 128
TB = 128
NB = S // TB
WP = 324


def _ln(x):
    m = jnp.mean(x, axis=-1, keepdims=True)
    c = x - m
    v = jnp.mean(c * c, axis=-1, keepdims=True)
    return c * lax.rsqrt(v + 1e-5)


def _r(x):
    return x.astype(BF16).astype(F32)


def _split(x):
    hi = x.astype(BF16)
    lo = (x - hi.astype(F32)).astype(BF16)
    return hi, lo


def _dft_tables(f_axis):
    fi = lax.broadcasted_iota(jnp.int32, (TB, TB), f_axis)
    t = lax.broadcasted_iota(jnp.int32, (TB, TB), 1 - f_axis)
    f = jnp.where(fi < TB // 2, 2 * fi, 2 * fi - (TB - 1))
    n = ((2 * f + 1) * t) & (4 * TB - 1)
    n = jnp.where(n >= 2 * TB, n - 4 * TB, n)
    ang = n.astype(F32) * (2.0 * math.pi / (4 * TB))
    return jnp.cos(ang), jnp.sin(ang)


def _kernel(x_hbm, mem0_ref, wq_hbm, wk_hbm, wv_hbm, wo_hbm,
            k_hbm, v_hbm, shk_ref, ssmk_hbm, ssmd_ref,
            out_ref,
            x_s, k_s, v_s, ssmk_s, wraw, wt, wo_s,
            fwd_s, inv_s, kpad, kv_s, u_a, u_b, kf_a, kf_b, c_a, c_b, y_s,
            hbuf, obuf, x2_s,
            sem_c, sem_w, sem_o, sem_x):
    def conv_copies(j):
        r0 = j * TB if isinstance(j, int) else pl.multiple_of(j * TB, TB)
        return (
            pltpu.make_async_copy(k_hbm.at[pl.ds(r0, TB), :], k_s.at[pl.ds(r0, TB), :], sem_c.at[j]),
            pltpu.make_async_copy(v_hbm.at[pl.ds(r0, TB), :], v_s.at[pl.ds(r0, TB), :], sem_c.at[NB + j]),
            pltpu.make_async_copy(ssmk_hbm.at[:, pl.ds(r0, TB)], ssmk_s.at[j], sem_c.at[2 * NB + j]),
        )
    for j in range(NB):
        for c in conv_copies(j):
            c.start()
    w_copies = [pltpu.make_async_copy(w, wraw.at[t], sem_w.at[t])
                for t, w in enumerate((wq_hbm, wk_hbm, wv_hbm))]
    x_copy = pltpu.make_async_copy(x_hbm, x_s, sem_x.at[0])
    wo_copies = [pltpu.make_async_copy(wo_hbm.at[:, pl.ds(n * 128, 128)], wo_s.at[n], sem_o.at[n])
                 for n in range(NLB)]
    for c in w_copies:
        c.start(priority=1)
    x_copy.start(priority=1)
    for c in wo_copies:
        c.start(priority=1)

    cf, sf = _dft_tables(0)
    fh, fl = _split(jnp.concatenate([cf, sf], axis=0))
    fwd_s[...] = jnp.concatenate([fh, fl], axis=1)
    cg, sg = _dft_tables(1)
    gh, gl = _split(jnp.concatenate([cg, sg], axis=1) * (1.0 / TB))
    inv_s[...] = jnp.concatenate([gh, gl, gh], axis=1)

    shk = shk_ref[...].astype(F32)
    taps = []
    for j in range(KS):
        parts = []
        for g in range(NLB):
            col = jnp.broadcast_to(shk[g * 128:(g + 1) * 128, j:j + 1], (128, 128))
            parts.append(col.T[0:1, :])
        taps.append(parts)
    dvec = ssmd_ref[...].astype(F32)
    for g in range(NLB):
        kpad[g, 0:8, :] = jnp.zeros((8, 128), F32)
    c_a[0] = jnp.zeros(c_a.shape[1:], F32)
    HB = NB // 2

    def fwd_stage(jl, half):
        j = jl + half * HB
        u_s, kf_s = ((u_a, kf_a), (u_b, kf_b))[half]
        for c in conv_copies(j):
            c.wait()
        r0 = pl.multiple_of(j * TB, TB)
        parts = []
        for g in range(NLB):
            lb = slice(g * 128, (g + 1) * 128)
            kb = k_s[pl.ds(r0, TB), lb].astype(F32)
            kpad[g, pl.ds(r0 + 8, TB), :] = kb
            acc = kb * taps[0][g]
            for t in range(1, KS):
                acc = acc + kpad[g, pl.ds(r0 + 8 - t, TB), :] * taps[t][g]
            parts.append((_r(acc) * v_s[pl.ds(r0, TB), lb].astype(F32)).astype(BF16))
        u = jnp.concatenate(parts, axis=1)
        kv_s[pl.ds(r0, TB), :] = u
        f2 = fwd_s[...]
        uf = jnp.dot(f2, jnp.concatenate([u, u], axis=0), preferred_element_type=F32)
        u_s[jl, 0] = uf[0:TB]
        u_s[jl, 1] = uf[TB:]
        kb = ssmk_s[j]
        kf = lax.dot_general(f2, jnp.concatenate([kb, kb], axis=1),
                             (((1,), (1,)), ((), ())), preferred_element_type=F32)
        kr, ki = kf[0:TB], kf[TB:]
        kf_s[jl, 0] = kr
        kf_s[jl, 1] = ki - kr
        kf_s[jl, 2] = kr + ki

    def mac_stage(jj, second):
        for rg in range(2):
            rs = pl.ds(pl.multiple_of((2 * jj + rg) * 8, 8), 8)
            for g in range(NLB):
                lb = slice(g * 128, (g + 1) * 128)
                outs = range(HB, NB) if second else range(0, NB - 1)
                sums = []
                for p in range(3):
                    def uu(i):
                        u_s = u_a if i < HB else u_b
                        if p == 0:
                            return u_s[i % HB, 0, rs, lb] + u_s[i % HB, 1, rs, lb]
                        return u_s[i % HB, p - 1, rs, lb]
                    if second:
                        pairs = [(a, b) for a in range(NB) for b in range(NB)
                                 if a + b < NB and (a >= HB or b >= HB)]
                    else:
                        pairs = [(a, b) for a in range(HB) for b in range(HB)]
                    ua = {a: uu(a) for a in sorted({a for a, _ in pairs})}
                    kb = {b: (kf_a if b < HB else kf_b)[b % HB, p, rs, lb]
                          for b in sorted({b for _, b in pairs})}
                    acc = {}
                    for a, b in pairs:
                        t = ua[a] * kb[b]
                        acc[a + b] = t if a + b not in acc else acc[a + b] + t
                    sums.append(acc)
                for i in outs:
                    re = sums[0][i] - sums[2][i]
                    im = sums[0][i] + sums[1][i]
                    c_s = c_a if i < HB else c_b
                    if second and i < NB - 1:
                        re = re + c_s[i % HB + 1, 0, rs, lb]
                        im = im + c_s[i % HB + 1, 1, rs, lb]
                    c_s[i % HB + 1, 0, rs, lb] = re
                    c_s[i % HB + 1, 1, rs, lb] = im
                    if i == HB - 1:
                        c_b[0, 0, rs, lb] = re
                        c_b[0, 1, rs, lb] = im

    def inv_stage(il, half):
        i = il + half * HB
        c_s = (c_a, c_b)[half]
        hb = TB // 2
        cr, ci = c_s[il + 1, 0], c_s[il + 1, 1]
        pr, pi = c_s[il, 0], c_s[il, 1]
        c = jnp.concatenate([cr[:hb] + pi[:hb], cr[hb:] - pi[hb:],
                             ci[:hb] - pr[:hb], ci[hb:] + pr[hb:]], axis=0)
        ch, cl = _split(c)
        y = jnp.dot(inv_s[...], jnp.concatenate([ch, ch, cl], axis=0),
                    preferred_element_type=F32)
        r0 = pl.multiple_of(i * TB, TB)
        kv = kv_s[pl.ds(r0, TB), :].astype(F32)
        y_s[pl.ds(r0, TB), :] = (_r(y) + _r(kv * dvec)).astype(BF16)

    def relayout(t):
        w_copies[t].wait()

        def body(i, _):
            for dd in range(8):
                dp = i * 8 + dd
                a = pltpu.bitcast(wraw[t, 2 * dp], U32)
                b = pltpu.bitcast(wraw[t, 2 * dp + 1], U32)
                lo = (a & jnp.uint32(0xFFFF)) | (b << 16)
                hi = (a >> 16) | (b & jnp.uint32(0xFFFF0000))
                wt[pl.ds(t * H * WP + dp, 16, stride=WP), :] = lo
                wt[pl.ds((t * H + 16) * WP + dp, 16, stride=WP), :] = hi
            return 0
        lax.fori_loop(0, D // 16, body, 0)

    def wslab(t, h):
        s0 = (t * H + (h % 2) * 16 + h // 2) * WP
        return pltpu.bitcast(wt[s0:s0 + D // 2, :], BF16)

    def loop(n, fn):
        def body(j, _):
            fn(j)
            return 0
        lax.fori_loop(0, n, body, 0)

    with jax.named_scope("conv_a"):
        loop(HB, lambda j: fwd_stage(j, 0))
    with jax.named_scope("conv_b"):
        loop(HB, lambda j: (fwd_stage(j, 1), mac_stage(j, False)))
    with jax.named_scope("rel0"):
        relayout(0)
    with jax.named_scope("conv_c"):
        loop(HB, lambda j: (inv_stage(j, 0), mac_stage(j, True)))
    with jax.named_scope("rel1"):
        relayout(1)
    with jax.named_scope("conv_d"):
        loop(HB, lambda j: inv_stage(j, 1))
    with jax.named_scope("rel2"):
        relayout(2)
    with jax.named_scope("waitx"):
        x_copy.wait()
        for c in wo_copies:
            c.wait()

    qi = lax.broadcasted_iota(jnp.int32, (ROWS, ROWS), 0)
    kj = lax.broadcasted_iota(jnp.int32, (ROWS, ROWS), 1)

    def layer_of(i):
        return jnp.where(i < 2 * M, i // M, (i - 2 * M) // SEG)
    same = layer_of(qi) == layer_of(kj)
    vis = same & ((qi < 2 * M) | (qi >= kj))
    fill = jnp.where(same, -1e9, -jnp.inf).astype(F32)
    scale = DH ** -0.5

    mem0 = mem0_ref[...].astype(F32)
    hbuf[0:16, :] = jnp.concatenate([mem0, mem0], axis=0).astype(BF16)
    hbuf[16:48, :] = _ln(x_s[0:SEG, :].astype(F32)).astype(BF16)
    hbuf[48:80, :] = jnp.zeros((SEG, D), BF16)
    obuf[...] = jnp.zeros((2 * SEG, D), F32)
    x2_s[...] = jnp.zeros(x2_s.shape, F32)

    def gate(xa, r0):
        return xa + _r(_r(_ln(xa)) * y_s[pl.ds(r0, SEG), :].astype(F32))

    def step(s):
        h = hbuf[...]
        r1 = pl.multiple_of(jnp.clip(s - 1, 0, NSEG - 1) * SEG, SEG)
        xb2 = _r(gate(_r(x_s[pl.ds(r1, SEG), :].astype(F32) + obuf[0:SEG, :]), r1))
        h2n = _ln(xb2).astype(BF16)
        r3 = pl.multiple_of(jnp.clip(s - 1 - LAG, 0, NSEG - 1) * SEG, SEG)
        xo = gate(_r(x2_s[(s + 4 - 1 - LAG) % 4] + obuf[SEG:2 * SEG, :]), r3)
        out_ref[pl.ds(r3, SEG), :] = xo.astype(BF16)
        x2_s[(s + 4 - 1) % 4] = xb2
        rn = pl.multiple_of(jnp.clip(s + 1, 0, NSEG - 1) * SEG, SEG)
        h1n = _ln(x_s[pl.ds(rn, SEG), :].astype(F32)).astype(BF16)

        def proj(g):
            return [[jnp.dot(h, wslab(t, g * HG + j), preferred_element_type=F32).astype(BF16)
                     for j in range(HG)] for t in range(3)]

        def probs(qkv):
            scs = [lax.dot_general(qkv[0][j], qkv[1][j], (((1,), (1,)), ((), ())),
                                   preferred_element_type=F32) for j in range(HG)]
            ps = []
            for sc in scs:
                sc = jnp.where(vis, sc * scale, fill)
                e = jnp.exp(sc - jnp.max(sc, axis=-1, keepdims=True))
                den = jnp.sum(e, axis=-1, keepdims=True)
                r = pl.reciprocal(den, approx=True)
                r = r * (2.0 - den * r)
                ps.append((e * r).astype(BF16))
            return ps

        def oproj(os_, h0):
            oc = jnp.concatenate(os_, axis=1)
            k0, k1 = h0 * DH, (h0 + len(os_)) * DH
            return [jnp.dot(oc, wo_s[n, k0:k1, :], preferred_element_type=F32)
                    for n in range(NLB)]

        heads = []
        qkv = proj(0)
        oa = None
        for g in range(NG):
            ps = probs(qkv)
            vs = qkv[2]
            if g + 1 < NG:
                qkv = proj(g + 1)
            else:
                oa = oproj(heads[:H // 2], 0)
            heads += [jnp.dot(ps[j], vs[j], preferred_element_type=F32).astype(BF16)
                      for j in range(HG)]
        ob = oproj(heads[H // 2:], H // 2)
        o = jnp.concatenate([b + a for a, b in zip(oa, ob)], axis=1)

        mem2 = jnp.where(s == LAG - 1, mem0, o[M:2 * M])
        hbuf[0:16, :] = jnp.concatenate([o[0:M], mem2], axis=0).astype(BF16)
        hbuf[16:48, :] = h1n
        hbuf[48:80, :] = h2n
        obuf[...] = _r(o[2 * M:])

    with jax.named_scope("main"):
        loop(NSEG + LAG, step)

    r3 = (NSEG - 1) * SEG
    xo = gate(_r(x2_s[(NSEG - 1) % 4] + obuf[SEG:2 * SEG, :]), r3)
    out_ref[r3:r3 + SEG, :] = xo.astype(BF16)


@functools.partial(jax.jit, static_argnames=("A_seg_len",))
def pallas_interleave_layers__memory_aug_recurrent_mem_tr__ssm_conv_h3__prompt_kernel(
    A_x, A_mem0, A_Wq, A_Wk, A_Wv, A_Wo, A_seg_len,
    B_q, B_k, B_v, B_shift_k, B_ssm_k, B_ssm_D,
):
    assert A_seg_len == SEG and A_x.shape == (1, S, D)
    vm = pl.BlockSpec(memory_space=pltpu.VMEM)
    hbm = pl.BlockSpec(memory_space=pl.ANY)
    out = pl.pallas_call(
        _kernel,
        out_shape=jax.ShapeDtypeStruct((S, D), BF16),
        in_specs=[hbm, vm, hbm, hbm, hbm, hbm, hbm, hbm, vm, hbm, vm],
        out_specs=vm,
        scratch_shapes=[
            pltpu.VMEM((S, D), BF16),
            pltpu.VMEM((S, D), BF16),
            pltpu.VMEM((S, D), BF16),
            pltpu.VMEM((NB, D, TB), BF16),
            pltpu.VMEM((3, D, H, DH), BF16),
            pltpu.VMEM((3 * H * WP, 128), U32),
            pltpu.VMEM((NLB, H * DH, 128), BF16),
            pltpu.VMEM((2 * TB, 2 * TB), BF16),
            pltpu.VMEM((TB, 6 * TB), BF16),
            pltpu.VMEM((NLB, S + 8, 128), F32),
            pltpu.VMEM((S, D), BF16),
            pltpu.VMEM((NB // 2, 2, TB, D), F32),
            pltpu.VMEM((NB // 2, 2, TB, D), F32),
            pltpu.VMEM((NB // 2, 3, TB, D), F32),
            pltpu.VMEM((NB // 2, 3, TB, D), F32),
            pltpu.VMEM((NB // 2 + 1, 2, TB, D), F32),
            pltpu.VMEM((NB // 2 + 1, 2, TB, D), F32),
            pltpu.VMEM((S, D), BF16),
            pltpu.VMEM((ROWS, D), BF16),
            pltpu.VMEM((2 * SEG, D), F32),
            pltpu.VMEM((4, SEG, D), F32),
            pltpu.SemaphoreType.DMA((3 * NB,)),
            pltpu.SemaphoreType.DMA((3,)),
            pltpu.SemaphoreType.DMA((NLB,)),
            pltpu.SemaphoreType.DMA((1,)),
        ],
        compiler_params=pltpu.CompilerParams(vmem_limit_bytes=120 * 1024 * 1024),
    )(A_x.reshape(S, D), A_mem0.reshape(M, D), A_Wq, A_Wk, A_Wv,
      A_Wo.reshape(H * DH, D), B_k.reshape(S, D), B_v.reshape(S, D),
      B_shift_k, B_ssm_k, B_ssm_D.reshape(1, D))
    return out.reshape(1, S, D)
```

```python
import functools
import math

import jax
import jax.numpy as jnp
from jax import lax
import jax.experimental.pallas as pl
import jax.experimental.pallas.tpu as pltpu

F32 = jnp.float32
BF16 = jnp.bfloat16
U32 = jnp.uint32

S = 2048
D = 640
H = 32
DH = 128
M = 8
SEG = 32
NSEG = S // SEG
KS = 4
LAG = 2
ROWS = 2 * M + 2 * SEG
HG = 4
NG = H // HG
NLB = D // 128
TB = 128
NB = S // TB
WP = 324


def _ln(x):
    m = jnp.mean(x, axis=-1, keepdims=True)
    c = x - m
    v = jnp.mean(c * c, axis=-1, keepdims=True)
    return c * lax.rsqrt(v + 1e-5)


def _r(x):
    return x.astype(BF16).astype(F32)


def _split(x):
    hi = x.astype(BF16)
    lo = (x - hi.astype(F32)).astype(BF16)
    return hi, lo


def _dft_tables(f_axis):
    fi = lax.broadcasted_iota(jnp.int32, (TB, TB), f_axis)
    t = lax.broadcasted_iota(jnp.int32, (TB, TB), 1 - f_axis)
    f = jnp.where(fi < TB // 2, 2 * fi, 2 * fi - (TB - 1))
    n = ((2 * f + 1) * t) & (4 * TB - 1)
    n = jnp.where(n >= 2 * TB, n - 4 * TB, n)
    ang = n.astype(F32) * (2.0 * math.pi / (4 * TB))
    return jnp.cos(ang), jnp.sin(ang)


def _kernel(x_hbm, mem0_ref, wq_hbm, wk_hbm, wv_hbm, wo_hbm,
            k_hbm, v_hbm, shk_ref, ssmk_hbm, ssmd_ref,
            out_hbm,
            x_s, k_s, v_s, ssmk_s, wraw, wt, wo_s,
            fwd_s, inv_s, kpad, kv_s, u_a, u_b, kf_a, kf_b, c_a, c_b, y_s,
            hbuf, obuf, x2_s, out_s,
            sem_c, sem_w, sem_o, sem_x):
    def conv_copies(j):
        r0 = j * TB if isinstance(j, int) else pl.multiple_of(j * TB, TB)
        return (
            pltpu.make_async_copy(k_hbm.at[pl.ds(r0, TB), :], k_s.at[pl.ds(r0, TB), :], sem_c.at[j]),
            pltpu.make_async_copy(v_hbm.at[pl.ds(r0, TB), :], v_s.at[pl.ds(r0, TB), :], sem_c.at[NB + j]),
            pltpu.make_async_copy(ssmk_hbm.at[:, pl.ds(r0, TB)], ssmk_s.at[j], sem_c.at[2 * NB + j]),
        )
    for j in range(NB):
        for c in conv_copies(j):
            c.start()
    w_copies = [pltpu.make_async_copy(w, wraw.at[t], sem_w.at[t])
                for t, w in enumerate((wq_hbm, wk_hbm, wv_hbm))]
    x_copy = pltpu.make_async_copy(x_hbm, x_s, sem_x.at[0])
    wo_copies = [pltpu.make_async_copy(wo_hbm.at[:, pl.ds(n * 128, 128)], wo_s.at[n], sem_o.at[n])
                 for n in range(NLB)]
    for c in w_copies:
        c.start(priority=1)
    x_copy.start(priority=1)
    for c in wo_copies:
        c.start(priority=1)

    cf, sf = _dft_tables(0)
    fh, fl = _split(jnp.concatenate([cf, sf], axis=0))
    fwd_s[...] = jnp.concatenate([fh, fl], axis=1)
    cg, sg = _dft_tables(1)
    gh, gl = _split(jnp.concatenate([cg, sg], axis=1) * (1.0 / TB))
    inv_s[...] = jnp.concatenate([gh, gl, gh], axis=1)

    shk = shk_ref[...].astype(F32)
    taps = []
    for j in range(KS):
        parts = []
        for g in range(NLB):
            col = jnp.broadcast_to(shk[g * 128:(g + 1) * 128, j:j + 1], (128, 128))
            parts.append(col.T[0:1, :])
        taps.append(parts)
    dvec = ssmd_ref[...].astype(F32)
    for g in range(NLB):
        kpad[g, 0:8, :] = jnp.zeros((8, 128), F32)
    c_a[0] = jnp.zeros(c_a.shape[1:], F32)
    HB = NB // 2

    def fwd_stage(jl, half):
        j = jl + half * HB
        u_s, kf_s = ((u_a, kf_a), (u_b, kf_b))[half]
        for c in conv_copies(j):
            c.wait()
        r0 = pl.multiple_of(j * TB, TB)
        parts = []
        for g in range(NLB):
            lb = slice(g * 128, (g + 1) * 128)
            kb = k_s[pl.ds(r0, TB), lb].astype(F32)
            kpad[g, pl.ds(r0 + 8, TB), :] = kb
            acc = kb * taps[0][g]
            for t in range(1, KS):
                acc = acc + kpad[g, pl.ds(r0 + 8 - t, TB), :] * taps[t][g]
            parts.append((_r(acc) * v_s[pl.ds(r0, TB), lb].astype(F32)).astype(BF16))
        u = jnp.concatenate(parts, axis=1)
        kv_s[pl.ds(r0, TB), :] = u
        f2 = fwd_s[...]
        uf = jnp.dot(f2, jnp.concatenate([u, u], axis=0), preferred_element_type=F32)
        u_s[jl, 0] = uf[0:TB]
        u_s[jl, 1] = uf[TB:]
        kb = ssmk_s[j]
        kf = lax.dot_general(f2, jnp.concatenate([kb, kb], axis=1),
                             (((1,), (1,)), ((), ())), preferred_element_type=F32)
        kr, ki = kf[0:TB], kf[TB:]
        kf_s[jl, 0] = kr
        kf_s[jl, 1] = ki - kr
        kf_s[jl, 2] = kr + ki

    def mac_stage(jj, second):
        for rg in range(2):
            rs = pl.ds(pl.multiple_of((2 * jj + rg) * 8, 8), 8)
            for g in range(NLB):
                lb = slice(g * 128, (g + 1) * 128)
                outs = range(HB, NB) if second else range(0, NB - 1)
                sums = []
                for p in range(3):
                    def uu(i):
                        u_s = u_a if i < HB else u_b
                        if p == 0:
                            return u_s[i % HB, 0, rs, lb] + u_s[i % HB, 1, rs, lb]
                        return u_s[i % HB, p - 1, rs, lb]
                    if second:
                        pairs = [(a, b) for a in range(NB) for b in range(NB)
                                 if a + b < NB and (a >= HB or b >= HB)]
                    else:
                        pairs = [(a, b) for a in range(HB) for b in range(HB)]
                    ua = {a: uu(a) for a in sorted({a for a, _ in pairs})}
                    kb = {b: (kf_a if b < HB else kf_b)[b % HB, p, rs, lb]
                          for b in sorted({b for _, b in pairs})}
                    acc = {}
                    for a, b in pairs:
                        t = ua[a] * kb[b]
                        acc[a + b] = t if a + b not in acc else acc[a + b] + t
                    sums.append(acc)
                for i in outs:
                    re = sums[0][i] - sums[2][i]
                    im = sums[0][i] + sums[1][i]
                    c_s = c_a if i < HB else c_b
                    if second and i < NB - 1:
                        re = re + c_s[i % HB + 1, 0, rs, lb]
                        im = im + c_s[i % HB + 1, 1, rs, lb]
                    c_s[i % HB + 1, 0, rs, lb] = re
                    c_s[i % HB + 1, 1, rs, lb] = im
                    if i == HB - 1:
                        c_b[0, 0, rs, lb] = re
                        c_b[0, 1, rs, lb] = im

    def inv_stage(il, half):
        i = il + half * HB
        c_s = (c_a, c_b)[half]
        hb = TB // 2
        cr, ci = c_s[il + 1, 0], c_s[il + 1, 1]
        pr, pi = c_s[il, 0], c_s[il, 1]
        c = jnp.concatenate([cr[:hb] + pi[:hb], cr[hb:] - pi[hb:],
                             ci[:hb] - pr[:hb], ci[hb:] + pr[hb:]], axis=0)
        ch, cl = _split(c)
        y = jnp.dot(inv_s[...], jnp.concatenate([ch, ch, cl], axis=0),
                    preferred_element_type=F32)
        r0 = pl.multiple_of(i * TB, TB)
        kv = kv_s[pl.ds(r0, TB), :].astype(F32)
        y_s[pl.ds(r0, TB), :] = (_r(y) + _r(kv * dvec)).astype(BF16)

    def relayout(t):
        w_copies[t].wait()

        def body(i, _):
            for dd in range(8):
                dp = i * 8 + dd
                a = pltpu.bitcast(wraw[t, 2 * dp], U32)
                b = pltpu.bitcast(wraw[t, 2 * dp + 1], U32)
                lo = (a & jnp.uint32(0xFFFF)) | (b << 16)
                hi = (a >> 16) | (b & jnp.uint32(0xFFFF0000))
                wt[pl.ds(t * H * WP + dp, 16, stride=WP), :] = lo
                wt[pl.ds((t * H + 16) * WP + dp, 16, stride=WP), :] = hi
            return 0
        lax.fori_loop(0, D // 16, body, 0)

    def wslab(t, h):
        s0 = (t * H + (h % 2) * 16 + h // 2) * WP
        return pltpu.bitcast(wt[s0:s0 + D // 2, :], BF16)

    def loop(n, fn):
        def body(j, _):
            fn(j)
            return 0
        lax.fori_loop(0, n, body, 0)

    with jax.named_scope("conv_a"):
        loop(HB, lambda j: fwd_stage(j, 0))
    with jax.named_scope("conv_b"):
        loop(HB, lambda j: (fwd_stage(j, 1), mac_stage(j, False)))
    with jax.named_scope("rel0"):
        relayout(0)
    with jax.named_scope("conv_c"):
        loop(HB, lambda j: (inv_stage(j, 0), mac_stage(j, True)))
    with jax.named_scope("rel1"):
        relayout(1)
    with jax.named_scope("conv_d"):
        loop(HB, lambda j: inv_stage(j, 1))
    with jax.named_scope("rel2"):
        relayout(2)
    with jax.named_scope("waitx"):
        x_copy.wait()
        for c in wo_copies:
            c.wait()

    scale = DH ** -0.5

    def masks(mode):
        rows = ROWS if mode == 0 else ROWS - SEG
        qi = lax.broadcasted_iota(jnp.int32, (rows, rows), 0)
        kj = lax.broadcasted_iota(jnp.int32, (rows, rows), 1)

        def layer_of(i):
            xl = (i - 2 * M) // SEG if mode == 0 else mode - 1
            return jnp.where(i < 2 * M, i // M, xl)
        same = layer_of(qi) == layer_of(kj)
        vis = same & ((qi < 2 * M) | (qi >= kj))
        fill = jnp.where(same, -1e9, -jnp.inf).astype(F32)
        return vis, fill

    mem0 = mem0_ref[...].astype(F32)
    hbuf[0:16, :] = jnp.concatenate([mem0, mem0], axis=0).astype(BF16)
    hbuf[16:48, :] = _ln(x_s[0:SEG, :].astype(F32)).astype(BF16)
    obuf[...] = jnp.zeros((2 * SEG, D), F32)
    x2_s[...] = jnp.zeros(x2_s.shape, F32)

    def seg_row(seg):
        return pl.multiple_of(jnp.clip(seg, 0, NSEG - 1) * SEG, SEG)

    def gate(xa, r0):
        return xa + _r(_r(_ln(xa)) * y_s[pl.ds(r0, SEG), :].astype(F32))

    def attention(h, vis, fill):
        def proj(g):
            return [[jnp.dot(h, wslab(t, g * HG + j), preferred_element_type=F32).astype(BF16)
                     for j in range(HG)] for t in range(3)]

        def probs(qkv):
            scs = [lax.dot_general(qkv[0][j], qkv[1][j], (((1,), (1,)), ((), ())),
                                   preferred_element_type=F32) for j in range(HG)]
            ps = []
            for sc in scs:
                sc = jnp.where(vis, sc * scale, fill)
                e = jnp.exp(sc - jnp.max(sc, axis=-1, keepdims=True))
                den = jnp.sum(e, axis=-1, keepdims=True)
                r = pl.reciprocal(den, approx=True)
                r = r * (2.0 - den * r)
                ps.append((e * r).astype(BF16))
            return ps

        def oproj(os_, h0):
            oc = jnp.concatenate(os_, axis=1)
            k0, k1 = h0 * DH, (h0 + len(os_)) * DH
            return [jnp.dot(oc, wo_s[n, k0:k1, :], preferred_element_type=F32)
                    for n in range(NLB)]

        heads = []
        qkv = proj(0)
        oa = None
        for g in range(NG):
            ps = probs(qkv)
            vs = qkv[2]
            if g + 1 < NG:
                qkv = proj(g + 1)
            else:
                oa = oproj(heads[:H // 2], 0)
            heads += [jnp.dot(ps[j], vs[j], preferred_element_type=F32).astype(BF16)
                      for j in range(HG)]
        ob = oproj(heads[H // 2:], H // 2)
        return jnp.concatenate([b + a for a, b in zip(oa, ob)], axis=1)

    def post2(s):
        r3 = seg_row(s - 1 - LAG)
        xo = gate(_r(x2_s[(s + 4 - 1 - LAG) % 4] + obuf[SEG:2 * SEG, :]), r3)
        out_s[pl.ds(r3, SEG), :] = xo.astype(BF16)

    def step(s, mode, vis, fill):
        if mode == 0:
            h = hbuf[...]
        elif mode == 1:
            h = hbuf[0:48, :]
        else:
            h = jnp.concatenate([hbuf[0:16, :], hbuf[48:80, :]], axis=0)
        r1 = seg_row(s - 1)
        xb2 = _r(gate(_r(x_s[pl.ds(r1, SEG), :].astype(F32) + obuf[0:SEG, :]), r1))
        h2n = _ln(xb2).astype(BF16)
        if mode != 1:
            post2(s)
        x2_s[(s + 4 - 1) % 4] = xb2
        if mode != 2:
            h1n = _ln(x_s[pl.ds(seg_row(s + 1), SEG), :].astype(F32)).astype(BF16)

        o = attention(h, vis, fill)

        mem2 = mem0 if mode == 1 else o[M:2 * M]
        hbuf[0:16, :] = jnp.concatenate([o[0:M], mem2], axis=0).astype(BF16)
        if mode != 2:
            hbuf[16:48, :] = h1n
        hbuf[48:80, :] = h2n
        if mode == 0:
            obuf[...] = _r(o[2 * M:])
        elif mode == 1:
            obuf[0:SEG, :] = _r(o[2 * M:])
        else:
            obuf[SEG:2 * SEG, :] = _r(o[2 * M:])

    with jax.named_scope("pro"):
        vis, fill = masks(1)
        loop(LAG, lambda s: step(s, 1, vis, fill))
    with jax.named_scope("main"):
        vis, fill = masks(0)
        loop(NSEG - LAG, lambda s: step(s + LAG, 0, vis, fill))
    done = (NSEG - 1 - LAG) * SEG
    out_a = pltpu.make_async_copy(out_s.at[0:done, :], out_hbm.at[0:done, :], sem_x.at[1])
    out_a.start()
    with jax.named_scope("epi"):
        vis, fill = masks(2)
        loop(LAG, lambda s: step(s + NSEG, 2, vis, fill))
    post2(NSEG + LAG)
    out_b = pltpu.make_async_copy(out_s.at[done:S, :], out_hbm.at[done:S, :], sem_x.at[2])
    out_b.start()
    out_a.wait()
    out_b.wait()


@functools.partial(jax.jit, static_argnames=("A_seg_len",))
def pallas_interleave_layers__memory_aug_recurrent_mem_tr__ssm_conv_h3__prompt_kernel(
    A_x, A_mem0, A_Wq, A_Wk, A_Wv, A_Wo, A_seg_len,
    B_q, B_k, B_v, B_shift_k, B_ssm_k, B_ssm_D,
):
    assert A_seg_len == SEG and A_x.shape == (1, S, D)
    vm = pl.BlockSpec(memory_space=pltpu.VMEM)
    hbm = pl.BlockSpec(memory_space=pl.ANY)
    out = pl.pallas_call(
        _kernel,
        out_shape=jax.ShapeDtypeStruct((S, D), BF16),
        in_specs=[hbm, vm, hbm, hbm, hbm, hbm, hbm, hbm, vm, hbm, vm],
        out_specs=hbm,
        scratch_shapes=[
            pltpu.VMEM((S, D), BF16),
            pltpu.VMEM((S, D), BF16),
            pltpu.VMEM((S, D), BF16),
            pltpu.VMEM((NB, D, TB), BF16),
            pltpu.VMEM((3, D, H, DH), BF16),
            pltpu.VMEM((3 * H * WP, 128), U32),
            pltpu.VMEM((NLB, H * DH, 128), BF16),
            pltpu.VMEM((2 * TB, 2 * TB), BF16),
            pltpu.VMEM((TB, 6 * TB), BF16),
            pltpu.VMEM((NLB, S + 8, 128), F32),
            pltpu.VMEM((S, D), BF16),
            pltpu.VMEM((NB // 2, 2, TB, D), F32),
            pltpu.VMEM((NB // 2, 2, TB, D), F32),
            pltpu.VMEM((NB // 2, 3, TB, D), F32),
            pltpu.VMEM((NB // 2, 3, TB, D), F32),
            pltpu.VMEM((NB // 2 + 1, 2, TB, D), F32),
            pltpu.VMEM((NB // 2 + 1, 2, TB, D), F32),
            pltpu.VMEM((S, D), BF16),
            pltpu.VMEM((ROWS, D), BF16),
            pltpu.VMEM((2 * SEG, D), F32),
            pltpu.VMEM((4, SEG, D), F32),
            pltpu.VMEM((S, D), BF16),
            pltpu.SemaphoreType.DMA((3 * NB,)),
            pltpu.SemaphoreType.DMA((3,)),
            pltpu.SemaphoreType.DMA((NLB,)),
            pltpu.SemaphoreType.DMA((3,)),
        ],
        compiler_params=pltpu.CompilerParams(vmem_limit_bytes=120 * 1024 * 1024),
    )(A_x.reshape(S, D), A_mem0.reshape(M, D), A_Wq, A_Wk, A_Wv,
      A_Wo.reshape(H * DH, D), B_k.reshape(S, D), B_v.reshape(S, D),
      B_shift_k, B_ssm_k, B_ssm_D.reshape(1, D))
    return out.reshape(1, S, D)
```

```python
import functools
import math

import jax
import jax.numpy as jnp
from jax import lax
import jax.experimental.pallas as pl
import jax.experimental.pallas.tpu as pltpu

F32 = jnp.float32
BF16 = jnp.bfloat16
U32 = jnp.uint32

S = 2048
D = 640
H = 32
DH = 128
M = 8
SEG = 32
NSEG = S // SEG
KS = 4
LAG = 2
ROWS = 2 * M + 2 * SEG
HG = 4
NG = H // HG
NLB = D // 128
TB = 128
NB = S // TB
WP = 324


def _ln(x):
    m = jnp.mean(x, axis=-1, keepdims=True)
    c = x - m
    v = jnp.mean(c * c, axis=-1, keepdims=True)
    return c * lax.rsqrt(v + 1e-5)


def _r(x):
    return x.astype(BF16).astype(F32)


def _split(x):
    hi = x.astype(BF16)
    lo = (x - hi.astype(F32)).astype(BF16)
    return hi, lo


def _basis(r, t):
    b = r & 63
    f = jnp.where(b < 32, 2 * b, 2 * b - 63)
    n = ((2 * f + 1) * t - jnp.where(r >= 64, TB, 0)) & (4 * TB - 1)
    n = jnp.where(n >= 2 * TB, n - 4 * TB, n)
    return jnp.cos(n.astype(F32) * (2.0 * math.pi / (4 * TB)))


def _halves(x):
    w = pltpu.bitcast(x, U32)
    return (pltpu.bitcast(w << 16, F32),
            pltpu.bitcast(w & jnp.uint32(0xFFFF0000), F32))


def _kernel(x_hbm, mem0_ref, wq_hbm, wk_hbm, wv_hbm, wo_hbm,
            k_hbm, v_hbm, shk_ref, ssmk_hbm, ssmd_ref,
            out_hbm,
            x_s, k_s, v_s, ssmk_s, wraw, wt, wo_s,
            fk_s, fu_s, inv_s, kpad, u_a, u_b, kf_a, kf_b, c_a, c_b, y_s,
            hbuf, obuf, x2_s, out_s,
            sem_c, sem_w, sem_o, sem_x):
    def conv_copies(j):
        r0 = j * TB if isinstance(j, int) else pl.multiple_of(j * TB, TB)
        return (
            pltpu.make_async_copy(k_hbm.at[pl.ds(r0, TB), :], k_s.at[pl.ds(r0, TB), :], sem_c.at[j]),
            pltpu.make_async_copy(v_hbm.at[pl.ds(r0, TB), :], v_s.at[pl.ds(r0, TB), :], sem_c.at[NB + j]),
            pltpu.make_async_copy(ssmk_hbm.at[:, pl.ds(r0, TB)], ssmk_s.at[j], sem_c.at[2 * NB + j]),
        )
    for j in range(NB):
        for c in conv_copies(j):
            c.start()
    w_copies = [pltpu.make_async_copy(w, wraw.at[t], sem_w.at[t])
                for t, w in enumerate((wq_hbm, wk_hbm, wv_hbm))]
    x_copy = pltpu.make_async_copy(x_hbm, x_s, sem_x.at[0])
    wo_copies = [pltpu.make_async_copy(wo_hbm.at[:, pl.ds(n * 128, 128)], wo_s.at[n], sem_o.at[n])
                 for n in range(NLB)]
    for c in w_copies:
        c.start(priority=1)
    x_copy.start(priority=1)
    for c in wo_copies:
        c.start(priority=1)

    hb = TB // 2
    HB = NB // 2
    ri = lax.broadcasted_iota(jnp.int32, (TB, TB), 0)
    ci = lax.broadcasted_iota(jnp.int32, (TB, TB), 1)
    full = _basis(ri, ci)
    alt = jnp.where((ci & 1) == 0, full, -full)
    fk = jnp.concatenate([full[:hb], alt[:hb], full[hb:], -alt[hb:]], axis=0)
    fh, fl = _split(fk)
    fk_s[...] = jnp.concatenate([fh, fl], axis=1)
    for par in range(2):
        tab = _basis(ri, 2 * (ci & 63) + par)
        hi = _r(tab)
        fu_s[par] = jnp.where(ci < hb, hi, tab - hi).astype(BF16)
        gh, gl = _split(_basis(lax.broadcasted_iota(jnp.int32, (hb, TB), 1),
                               2 * lax.broadcasted_iota(jnp.int32, (hb, TB), 0) + par) * (1.0 / TB))
        inv_s[par] = jnp.concatenate([gh, gl, gh], axis=1)

    shk = shk_ref[...].astype(F32)
    taps = []
    for j in range(KS):
        parts = []
        for g in range(NLB):
            col = jnp.broadcast_to(shk[g * 128:(g + 1) * 128, j:j + 1], (128, 128))
            parts.append(col.T[0:1, :])
        taps.append(parts)
    dvec = ssmd_ref[...].astype(F32)
    for g in range(NLB):
        kpad[0, g, 0:8, :] = jnp.zeros((8, 128), F32)
        kpad[1, g, 0:8, :] = jnp.zeros((8, 128), F32)
    c_a[0] = jnp.zeros(c_a.shape[1:], F32)

    def fwd_stage(jl, half):
        j = jl + half * HB
        u_s, kf_s = ((u_a, kf_a), (u_b, kf_b))[half]
        for c in conv_copies(j):
            c.wait()
        r0 = pl.multiple_of(j * TB, TB)
        q0 = pl.multiple_of(j * hb, hb) + 8
        es, os_ = [], []
        for g in range(NLB):
            lb = slice(g * 128, (g + 1) * 128)
            ke, ko = _halves(k_s[pl.ds(r0, TB), lb])
            ve, vo = _halves(v_s[pl.ds(r0, TB), lb])
            kpad[0, g, pl.ds(q0, hb), :] = ke
            kpad[1, g, pl.ds(q0, hb), :] = ko
            ke1 = kpad[0, g, pl.ds(q0 - 1, hb), :]
            ko1 = kpad[1, g, pl.ds(q0 - 1, hb), :]
            ko2 = kpad[1, g, pl.ds(q0 - 2, hb), :]
            t0, t1, t2, t3 = (taps[t][g] for t in range(KS))
            es.append(((ke * t0 + ko1 * t1 + ke1 * t2 + ko2 * t3) * ve).astype(BF16))
            os_.append(((ko * t0 + ke * t1 + ko1 * t2 + ke1 * t3) * vo).astype(BF16))
        e = jnp.concatenate(es, axis=1)
        o = jnp.concatenate(os_, axis=1)
        fe = jnp.dot(fu_s[0], jnp.concatenate([e, e], axis=0), preferred_element_type=F32)
        fo = jnp.dot(fu_s[1], jnp.concatenate([o, o], axis=0), preferred_element_type=F32)
        u_s[jl, 0, 0:hb] = fe[:hb] + fo[:hb]
        u_s[jl, 0, hb:TB] = fe[:hb] - fo[:hb]
        u_s[jl, 1, 0:hb] = fe[hb:] + fo[hb:]
        u_s[jl, 1, hb:TB] = fo[hb:] - fe[hb:]
        kb = ssmk_s[j]
        kf = lax.dot_general(fk_s[...], jnp.concatenate([kb, kb], axis=1),
                             (((1,), (1,)), ((), ())), preferred_element_type=F32)
        kr, ki = kf[0:TB], kf[TB:]
        if half == 0:
            kr = kr + jnp.where(jl == 0, dvec, 0.0)
        kf_s[jl, 0] = kr
        kf_s[jl, 1] = ki - kr
        kf_s[jl, 2] = kr + ki

    def mac_stage(jj, second):
        for rg in range(2):
            rs = pl.ds(pl.multiple_of((2 * jj + rg) * 8, 8), 8)
            for g in range(NLB):
                lb = slice(g * 128, (g + 1) * 128)

                def uu(i, p):
                    u_s = u_a if i < HB else u_b
                    if p == 0:
                        return u_s[i % HB, 0, rs, lb] + u_s[i % HB, 1, rs, lb]
                    return u_s[i % HB, p - 1, rs, lb]

                def kk(i, p):
                    return (kf_a if i < HB else kf_b)[i % HB, p, rs, lb]

                def poly(p, acc):
                    acc = dict(acc)
                    for a0, b0 in (((0, HB), (HB, 0)) if second else ((0, 0),)):
                        ua = [uu(a0 + a, p) for a in range(HB)]
                        kb = [kk(b0 + b, p) for b in range(HB)]
                        for i in range(min(2 * HB - 1, NB - a0 - b0)):
                            for a in range(max(0, i - HB + 1), min(i, HB - 1) + 1):
                                t = ua[a] * kb[i - a]
                                io = i + a0 + b0
                                if io not in acc:
                                    acc[io] = t
                                elif p == 2:
                                    acc[io] = acc[io] - t
                                else:
                                    acc[io] = acc[io] + t
                    return acc

                s1 = poly(0, {})
                for p, comp in ((1, 1), (2, 0)):
                    init = s1
                    if second:
                        init = {i: (v + c_b[i - HB + 1, comp, rs, lb] if i < NB - 1 else v)
                                for i, v in s1.items()}
                    for i, v in poly(p, init).items():
                        (c_a if i < HB else c_b)[i % HB + 1, comp, rs, lb] = v
                        if i == HB - 1:
                            c_b[0, comp, rs, lb] = v

    def inv_stage(il, half):
        i = il + half * HB
        c_s = (c_a, c_b)[half]
        q = TB // 4
        re, im = [], []
        for b in range(4):
            rows = slice(b * q, (b + 1) * q)
            cr, ci_ = c_s[il + 1, 0, rows], c_s[il + 1, 1, rows]
            pr, pi = c_s[il, 0, rows], c_s[il, 1, rows]
            re.append(cr + pi if b in (0, 3) else cr - pi)
            im.append(ci_ - pr if b in (0, 3) else ci_ + pr)
        pe = jnp.concatenate([re[0] + re[2], re[1] + re[3], im[0] - im[2], im[1] - im[3]], axis=0)
        po = jnp.concatenate([re[0] - re[2], re[1] - re[3], im[0] + im[2], im[1] + im[3]], axis=0)
        for par, pp in enumerate((pe, po)):
            ph, plo = _split(pp)
            y = jnp.dot(inv_s[par], jnp.concatenate([ph, ph, plo], axis=0),
                        preferred_element_type=F32)
            for g in range(NLB):
                y_s[g, pl.ds(i * TB + par, hb, stride=2), :] = y[:, g * 128:(g + 1) * 128]

    def relayout(t):
        w_copies[t].wait()

        def body(i, _):
            for dd in range(8):
                dp = i * 8 + dd
                a = pltpu.bitcast(wraw[t, 2 * dp], U32)
                b = pltpu.bitcast(wraw[t, 2 * dp + 1], U32)
                lo = (a & jnp.uint32(0xFFFF)) | (b << 16)
                hi = (a >> 16) | (b & jnp.uint32(0xFFFF0000))
                wt[pl.ds(t * H * WP + dp, 16, stride=WP), :] = lo
                wt[pl.ds((t * H + 16) * WP + dp, 16, stride=WP), :] = hi
            return 0
        lax.fori_loop(0, D // 16, body, 0)

    def wslab(t, h):
        s0 = (t * H + (h % 2) * 16 + h // 2) * WP
        return pltpu.bitcast(wt[s0:s0 + D // 2, :], BF16)

    def loop(n, fn):
        def body(j, _):
            fn(j)
            return 0
        lax.fori_loop(0, n, body, 0)

    with jax.named_scope("conv_a"):
        loop(HB, lambda j: fwd_stage(j, 0))
    with jax.named_scope("conv_b"):
        loop(HB, lambda j: (fwd_stage(j, 1), mac_stage(j, False)))
    with jax.named_scope("rel0"):
        relayout(0)
    with jax.named_scope("conv_c"):
        loop(HB, lambda j: (inv_stage(j, 0), mac_stage(j, True)))
    with jax.named_scope("rel1"):
        relayout(1)
    with jax.named_scope("conv_d"):
        loop(HB, lambda j: inv_stage(j, 1))
    with jax.named_scope("rel2"):
        relayout(2)
    with jax.named_scope("waitx"):
        x_copy.wait()
        for c in wo_copies:
            c.wait()

    scale = DH ** -0.5

    def masks(mode):
        rows = ROWS if mode == 0 else ROWS - SEG
        qi = lax.broadcasted_iota(jnp.int32, (rows, rows), 0)
        kj = lax.broadcasted_iota(jnp.int32, (rows, rows), 1)

        def layer_of(i):
            xl = (i - 2 * M) // SEG if mode == 0 else mode - 1
            return jnp.where(i < 2 * M, i // M, xl)
        same = layer_of(qi) == layer_of(kj)
        vis = same & ((qi < 2 * M) | (qi >= kj))
        fill = jnp.where(same, -1e9, -jnp.inf).astype(F32)
        return vis, fill

    mem0 = mem0_ref[...].astype(F32)
    hbuf[0:16, :] = jnp.concatenate([mem0, mem0], axis=0).astype(BF16)
    hbuf[16:48, :] = _ln(x_s[0:SEG, :].astype(F32)).astype(BF16)
    obuf[...] = jnp.zeros((2 * SEG, D), F32)
    x2_s[...] = jnp.zeros(x2_s.shape, F32)

    def seg_row(seg):
        return pl.multiple_of(jnp.clip(seg, 0, NSEG - 1) * SEG, SEG)

    def gate(xa, r0):
        y = jnp.concatenate([y_s[g, pl.ds(r0, SEG), :] for g in range(NLB)], axis=1)
        return xa + _r(_r(_ln(xa)) * y)

    def attention(h, vis, fill):
        def proj(g):
            return [[jnp.dot(h, wslab(t, g * HG + j), preferred_element_type=F32).astype(BF16)
                     for j in range(HG)] for t in range(3)]

        def probs(qkv):
            scs = [lax.dot_general(qkv[0][j], qkv[1][j], (((1,), (1,)), ((), ())),
                                   preferred_element_type=F32) for j in range(HG)]
            ps = []
            for sc in scs:
                sc = jnp.where(vis, sc * scale, fill)
                e = jnp.exp(sc - jnp.max(sc, axis=-1, keepdims=True))
                den = jnp.sum(e, axis=-1, keepdims=True)
                r = pl.reciprocal(den, approx=True)
                r = r * (2.0 - den * r)
                ps.append((e * r).astype(BF16))
            return ps

        def oproj(os_, h0):
            oc = jnp.concatenate(os_, axis=1)
            k0, k1 = h0 * DH, (h0 + len(os_)) * DH
            return [jnp.dot(oc, wo_s[n, k0:k1, :], preferred_element_type=F32)
                    for n in range(NLB)]

        heads = []
        qkv = proj(0)
        oa = None
        for g in range(NG):
            ps = probs(qkv)
            vs = qkv[2]
            if g + 1 < NG:
                qkv = proj(g + 1)
            else:
                oa = oproj(heads[:H // 2], 0)
            heads += [jnp.dot(ps[j], vs[j], preferred_element_type=F32).astype(BF16)
                      for j in range(HG)]
        ob = oproj(heads[H // 2:], H // 2)
        return jnp.concatenate([b + a for a, b in zip(oa, ob)], axis=1)

    def post2(s):
        r3 = seg_row(s - 1 - LAG)
        xo = gate(_r(x2_s[(s + 4 - 1 - LAG) % 4] + obuf[SEG:2 * SEG, :]), r3)
        out_s[pl.ds(r3, SEG), :] = xo.astype(BF16)

    def step(s, mode, vis, fill):
        if mode == 0:
            h = hbuf[...]
        elif mode == 1:
            h = hbuf[0:48, :]
        else:
            h = jnp.concatenate([hbuf[0:16, :], hbuf[48:80, :]], axis=0)
        r1 = seg_row(s - 1)
        xb2 = _r(gate(_r(x_s[pl.ds(r1, SEG), :].astype(F32) + obuf[0:SEG, :]), r1))
        h2n = _ln(xb2).astype(BF16)
        if mode != 1:
            post2(s)
        x2_s[(s + 4 - 1) % 4] = xb2
        if mode != 2:
            h1n = _ln(x_s[pl.ds(seg_row(s + 1), SEG), :].astype(F32)).astype(BF16)

        o = attention(h, vis, fill)

        mem2 = mem0 if mode == 1 else o[M:2 * M]
        hbuf[0:16, :] = jnp.concatenate([o[0:M], mem2], axis=0).astype(BF16)
        if mode != 2:
            hbuf[16:48, :] = h1n
        hbuf[48:80, :] = h2n
        if mode == 0:
            obuf[...] = _r(o[2 * M:])
        elif mode == 1:
            obuf[0:SEG, :] = _r(o[2 * M:])
        else:
            obuf[SEG:2 * SEG, :] = _r(o[2 * M:])

    with jax.named_scope("pro"):
        vis, fill = masks(1)
        loop(LAG, lambda s: step(s, 1, vis, fill))
    with jax.named_scope("main"):
        vis, fill = masks(0)
        loop(NSEG - LAG, lambda s: step(s + LAG, 0, vis, fill))
    done = (NSEG - 1 - LAG) * SEG
    out_a = pltpu.make_async_copy(out_s.at[0:done, :], out_hbm.at[0:done, :], sem_x.at[1])
    out_a.start()
    with jax.named_scope("epi"):
        vis, fill = masks(2)
        loop(LAG, lambda s: step(s + NSEG, 2, vis, fill))
    post2(NSEG + LAG)
    out_b = pltpu.make_async_copy(out_s.at[done:S, :], out_hbm.at[done:S, :], sem_x.at[2])
    out_b.start()
    out_a.wait()
    out_b.wait()


@functools.partial(jax.jit, static_argnames=("A_seg_len",))
def pallas_interleave_layers__memory_aug_recurrent_mem_tr__ssm_conv_h3__prompt_kernel(
    A_x, A_mem0, A_Wq, A_Wk, A_Wv, A_Wo, A_seg_len,
    B_q, B_k, B_v, B_shift_k, B_ssm_k, B_ssm_D,
):
    assert A_seg_len == SEG and A_x.shape == (1, S, D)
    vm = pl.BlockSpec(memory_space=pltpu.VMEM)
    hbm = pl.BlockSpec(memory_space=pl.ANY)
    out = pl.pallas_call(
        _kernel,
        out_shape=jax.ShapeDtypeStruct((S, D), BF16),
        in_specs=[hbm, vm, hbm, hbm, hbm, hbm, hbm, hbm, vm, hbm, vm],
        out_specs=hbm,
        scratch_shapes=[
            pltpu.VMEM((S, D), BF16),
            pltpu.VMEM((S, D), BF16),
            pltpu.VMEM((S, D), BF16),
            pltpu.VMEM((NB, D, TB), BF16),
            pltpu.VMEM((3, D, H, DH), BF16),
            pltpu.VMEM((3 * H * WP, 128), U32),
            pltpu.VMEM((NLB, H * DH, 128), BF16),
            pltpu.VMEM((2 * TB, 2 * TB), BF16),
            pltpu.VMEM((2, TB, TB), BF16),
            pltpu.VMEM((2, TB // 2, 3 * TB), BF16),
            pltpu.VMEM((2, NLB, S // 2 + 8, 128), F32),
            pltpu.VMEM((NB // 2, 2, TB, D), F32),
            pltpu.VMEM((NB // 2, 2, TB, D), F32),
            pltpu.VMEM((NB // 2, 3, TB, D), F32),
            pltpu.VMEM((NB // 2, 3, TB, D), F32),
            pltpu.VMEM((NB // 2 + 1, 2, TB, D), F32),
            pltpu.VMEM((NB // 2 + 1, 2, TB, D), F32),
            pltpu.VMEM((NLB, S, 128), F32),
            pltpu.VMEM((ROWS, D), BF16),
            pltpu.VMEM((2 * SEG, D), F32),
            pltpu.VMEM((4, SEG, D), F32),
            pltpu.VMEM((S, D), BF16),
            pltpu.SemaphoreType.DMA((3 * NB,)),
            pltpu.SemaphoreType.DMA((3,)),
            pltpu.SemaphoreType.DMA((NLB,)),
            pltpu.SemaphoreType.DMA((3,)),
        ],
        compiler_params=pltpu.CompilerParams(vmem_limit_bytes=120 * 1024 * 1024),
    )(A_x.reshape(S, D), A_mem0.reshape(M, D), A_Wq, A_Wk, A_Wv,
      A_Wo.reshape(H * DH, D), B_k.reshape(S, D), B_v.reshape(S, D),
      B_shift_k, B_ssm_k, B_ssm_D.reshape(1, D))
    return out.reshape(1, S, D)
```

```python
import functools
import math

import jax
import jax.numpy as jnp
from jax import lax
import jax.experimental.pallas as pl
import jax.experimental.pallas.tpu as pltpu

F32 = jnp.float32
BF16 = jnp.bfloat16
U32 = jnp.uint32

S = 2048
D = 640
H = 32
DH = 128
M = 8
SEG = 32
NSEG = S // SEG
KS = 4
LAG = 2
ROWS = 2 * M + 2 * SEG
HG = 4
NG = H // HG
NLB = D // 128
TB = 128
NB = S // TB
WP = 324


def _ln(x):
    m = jnp.mean(x, axis=-1, keepdims=True)
    c = x - m
    v = jnp.mean(c * c, axis=-1, keepdims=True)
    return c * lax.rsqrt(v + 1e-5)


def _r(x):
    return x.astype(BF16).astype(F32)


def _split(x):
    hi = x.astype(BF16)
    lo = (x - hi.astype(F32)).astype(BF16)
    return hi, lo


def _basis(r, t):
    b = r & 63
    f = jnp.where(b < 32, 2 * b, 2 * b - 63)
    n = ((2 * f + 1) * t - jnp.where(r >= 64, TB, 0)) & (4 * TB - 1)
    n = jnp.where(n >= 2 * TB, n - 4 * TB, n)
    return jnp.cos(n.astype(F32) * (2.0 * math.pi / (4 * TB)))


def _halves(x):
    w = pltpu.bitcast(x, U32)
    return (pltpu.bitcast(w << 16, F32),
            pltpu.bitcast(w & jnp.uint32(0xFFFF0000), F32))


def _kernel(x_hbm, mem0_ref, wq_hbm, wk_hbm, wv_hbm, wo_hbm,
            k_hbm, v_hbm, shk_ref, ssmk_hbm, ssmd_ref,
            out_hbm,
            x_s, k_s, v_s, ssmk_s, wraw, wt, wo_s,
            fk_s, fu_s, inv_s, kpad, u_a, u_b, kf_a, kf_b, c_a, c_b, c_p, y_s,
            hbuf, obuf, x2_s, out_s,
            sem_c, sem_w, sem_x):
    HB = NB // 2
    XH = 4 * SEG

    def conv_copies(j):
        r0 = j * TB if isinstance(j, int) else pl.multiple_of(j * TB, TB)
        return (
            pltpu.make_async_copy(ssmk_hbm.at[:, pl.ds(r0, TB)], ssmk_s.at[j], sem_c.at[j]),
            pltpu.make_async_copy(k_hbm.at[pl.ds(r0, TB), :], k_s.at[pl.ds(r0, TB), :], sem_c.at[HB + j]),
            pltpu.make_async_copy(v_hbm.at[pl.ds(r0, TB), :], v_s.at[pl.ds(r0, TB), :], sem_c.at[NB + j]),
        )
    late_copies = [pltpu.make_async_copy(ssmk_hbm.at[:, pl.ds(j * TB, TB)], ssmk_s.at[j], sem_c.at[3 * HB])
                   for j in range(HB, NB)]
    late_copies += [pltpu.make_async_copy(src.at[S // 2:, :], dst.at[S // 2:, :], sem_c.at[3 * HB])
                    for src, dst in ((k_hbm, k_s), (v_hbm, v_s))]
    w_copies = [pltpu.make_async_copy(w, wraw.at[t], sem_w.at[t])
                for t, w in enumerate((wq_hbm, wk_hbm, wv_hbm))]
    wo_copy = pltpu.make_async_copy(wo_hbm, wo_s, sem_w.at[3])
    xa_copy = pltpu.make_async_copy(x_hbm.at[0:XH, :], x_s.at[0:XH, :], sem_x.at[0])
    xb_copy = pltpu.make_async_copy(x_hbm.at[XH:, :], x_s.at[XH:, :], sem_x.at[3])
    for j in range(HB):
        for c in conv_copies(j):
            c.start()
    for c in late_copies:
        c.start()
    xa_copy.start()
    wo_copy.start(priority=1)
    xb_copy.start(priority=1)

    hb = TB // 2
    ri = lax.broadcasted_iota(jnp.int32, (TB, TB), 0)
    ci = lax.broadcasted_iota(jnp.int32, (TB, TB), 1)
    full = _basis(ri, ci)
    alt = jnp.where((ci & 1) == 0, full, -full)
    fk = jnp.concatenate([full[:hb], alt[:hb], full[hb:], -alt[hb:]], axis=0)
    fh, fl = _split(fk)
    fk_s[...] = jnp.concatenate([fh, fl], axis=1)
    for par in range(2):
        tab = _basis(ri, 2 * (ci & 63) + par)
        hi = _r(tab)
        fu_s[par] = jnp.where(ci < hb, hi, tab - hi).astype(BF16)
        gh, gl = _split(_basis(lax.broadcasted_iota(jnp.int32, (hb, TB), 1),
                               2 * lax.broadcasted_iota(jnp.int32, (hb, TB), 0) + par) * (1.0 / TB))
        inv_s[par] = jnp.concatenate([gh, gl, gh], axis=1)

    eye = (lax.broadcasted_iota(jnp.int32, (8, KS), 0)
           == lax.broadcasted_iota(jnp.int32, (8, KS), 1)).astype(F32).astype(BF16)
    shk_t = lax.dot_general(eye, shk_ref[...], (((1,), (1,)), ((), ())),
                            preferred_element_type=F32)
    taps = [[shk_t[j:j + 1, g * 128:(g + 1) * 128] for g in range(NLB)] for j in range(KS)]
    dvec = ssmd_ref[...].astype(F32)
    for g in range(NLB):
        kpad[0, g, 0:8, :] = jnp.zeros((8, 128), F32)
        kpad[1, g, 0:8, :] = jnp.zeros((8, 128), F32)
    c_a[0] = jnp.zeros(c_a.shape[1:], F32)

    def fwd_stage(jl, half):
        j = jl + half * HB
        u_s, kf_s = ((u_a, kf_a), (u_b, kf_b))[half]
        if half == 0:
            for c in conv_copies(j):
                c.wait()
        kb = ssmk_s[j]
        kf = lax.dot_general(fk_s[...], jnp.concatenate([kb, kb], axis=1),
                             (((1,), (1,)), ((), ())), preferred_element_type=F32)
        kr, ki = kf[0:TB], kf[TB:]
        if half == 0:
            kr = kr + jnp.where(jl == 0, dvec, 0.0)
        kf_s[jl, 0] = kr
        kf_s[jl, 1] = ki - kr
        kf_s[jl, 2] = kr + ki
        r0 = pl.multiple_of(j * TB, TB)
        q0 = pl.multiple_of(j * hb, hb) + 8
        es, os_ = [], []
        for g in range(NLB):
            lb = slice(g * 128, (g + 1) * 128)
            ke, ko = _halves(k_s[pl.ds(r0, TB), lb])
            ve, vo = _halves(v_s[pl.ds(r0, TB), lb])
            kpad[0, g, pl.ds(q0, hb), :] = ke
            kpad[1, g, pl.ds(q0, hb), :] = ko
            ke1 = kpad[0, g, pl.ds(q0 - 1, hb), :]
            ko1 = kpad[1, g, pl.ds(q0 - 1, hb), :]
            ko2 = kpad[1, g, pl.ds(q0 - 2, hb), :]
            t0, t1, t2, t3 = (taps[t][g] for t in range(KS))
            es.append(((ke * t0 + ko1 * t1 + ke1 * t2 + ko2 * t3) * ve).astype(BF16))
            os_.append(((ko * t0 + ke * t1 + ko1 * t2 + ke1 * t3) * vo).astype(BF16))
        e = jnp.concatenate(es, axis=1)
        o = jnp.concatenate(os_, axis=1)
        fe = jnp.dot(fu_s[0], jnp.concatenate([e, e], axis=0), preferred_element_type=F32)
        fo = jnp.dot(fu_s[1], jnp.concatenate([o, o], axis=0), preferred_element_type=F32)
        u_s[jl, 0, 0:hb] = fe[:hb] + fo[:hb]
        u_s[jl, 0, hb:TB] = fe[:hb] - fo[:hb]
        u_s[jl, 1, 0:hb] = fe[hb:] + fo[hb:]
        u_s[jl, 1, hb:TB] = fo[hb:] - fe[hb:]

    def mac_stage(jj, second):
        for rg in range(2):
            rs = pl.ds(pl.multiple_of((2 * jj + rg) * 8, 8), 8)
            for g in range(NLB):
                lb = slice(g * 128, (g + 1) * 128)

                def uu(i, p):
                    u_s = u_a if i < HB else u_b
                    if p == 0:
                        return u_s[i % HB, 0, rs, lb] + u_s[i % HB, 1, rs, lb]
                    return u_s[i % HB, p - 1, rs, lb]

                def kk(i, p):
                    return (kf_a if i < HB else kf_b)[i % HB, p, rs, lb]

                def poly(p, acc):
                    acc = dict(acc)
                    for a0, b0 in (((0, HB), (HB, 0)) if second else ((0, 0),)):
                        ua = [uu(a0 + a, p) for a in range(HB)]
                        kb = [kk(b0 + b, p) for b in range(HB)]
                        for i in range(min(2 * HB - 1, NB - a0 - b0)):
                            for a in range(max(0, i - HB + 1), min(i, HB - 1) + 1):
                                t = ua[a] * kb[i - a]
                                io = i + a0 + b0
                                if io not in acc:
                                    acc[io] = t
                                elif p == 2:
                                    acc[io] = acc[io] - t
                                else:
                                    acc[io] = acc[io] + t
                    return acc

                s1 = poly(0, {})
                for p, comp in ((1, 1), (2, 0)):
                    init = s1
                    if second:
                        init = {i: (v + c_p[i - HB, comp, rs, lb] if i < NB - 1 else v)
                                for i, v in s1.items()}
                    for i, v in poly(p, init).items():
                        if i < HB:
                            c_a[i + 1, comp, rs, lb] = v
                        elif second:
                            c_b[i - HB + 1, comp, rs, lb] = v
                        else:
                            c_p[i - HB, comp, rs, lb] = v
                        if i == HB - 1:
                            c_b[0, comp, rs, lb] = v

    def inv_stage(il, half):
        i = il + half * HB
        c_s = (c_a, c_b)[half]
        q = TB // 4
        re, im = [], []
        for b in range(4):
            rows = slice(b * q, (b + 1) * q)
            cr, ci_ = c_s[il + 1, 0, rows], c_s[il + 1, 1, rows]
            pr, pi = c_s[il, 0, rows], c_s[il, 1, rows]
            re.append(cr + pi if b in (0, 3) else cr - pi)
            im.append(ci_ - pr if b in (0, 3) else ci_ + pr)
        pe = jnp.concatenate([re[0] + re[2], re[1] + re[3], im[0] - im[2], im[1] - im[3]], axis=0)
        po = jnp.concatenate([re[0] - re[2], re[1] - re[3], im[0] + im[2], im[1] + im[3]], axis=0)
        for par, pp in enumerate((pe, po)):
            ph, plo = _split(pp)
            y = jnp.dot(inv_s[par], jnp.concatenate([ph, ph, plo], axis=0),
                        preferred_element_type=F32)
            for g in range(NLB):
                y_s[g, pl.ds(i * TB + par, hb, stride=2), :] = y[:, g * 128:(g + 1) * 128]

    def relayout(t):
        w_copies[t].wait()

        def body(i, _):
            for dd in range(8):
                dp = i * 8 + dd
                a = pltpu.bitcast(wraw[t, 2 * dp], U32)
                b = pltpu.bitcast(wraw[t, 2 * dp + 1], U32)
                lo = (a & jnp.uint32(0xFFFF)) | (b << 16)
                hi = (a >> 16) | (b & jnp.uint32(0xFFFF0000))
                wt[pl.ds(t * H * WP + dp, 16, stride=WP), :] = lo
                wt[pl.ds((t * H + 16) * WP + dp, 16, stride=WP), :] = hi
            return 0
        lax.fori_loop(0, D // 16, body, 0)

    def wslab(t, h):
        s0 = (t * H + (h % 2) * 16 + h // 2) * WP
        return pltpu.bitcast(wt[s0:s0 + D // 2, :], BF16)

    def loop(n, fn):
        def body(j, _):
            fn(j)
            return 0
        lax.fori_loop(0, n, body, 0)

    with jax.named_scope("conv_a"):
        loop(HB, lambda j: fwd_stage(j, 0))
    with jax.named_scope("conv_b"):
        for c in w_copies:
            c.start()
        for c in late_copies:
            c.wait()
        loop(HB, lambda j: (fwd_stage(j, 1), mac_stage(j, False)))
    with jax.named_scope("rel0"):
        relayout(0)
    with jax.named_scope("conv_c"):
        loop(HB, lambda j: (inv_stage(j, 0), mac_stage(j, True)))
    with jax.named_scope("rel1"):
        relayout(1)
    with jax.named_scope("conv_d"):
        loop(HB, lambda j: inv_stage(j, 1))
    with jax.named_scope("rel2"):
        relayout(2)
    with jax.named_scope("waitx"):
        xa_copy.wait()
        wo_copy.wait()

    scale = DH ** -0.5

    def masks(mode):
        rows = ROWS if mode == 0 else ROWS - SEG
        qi = lax.broadcasted_iota(jnp.int32, (rows, rows), 0)
        kj = lax.broadcasted_iota(jnp.int32, (rows, rows), 1)

        def layer_of(i):
            xl = (i - 2 * M) // SEG if mode == 0 else mode - 1
            return jnp.where(i < 2 * M, i // M, xl)
        same = layer_of(qi) == layer_of(kj)
        vis = same & ((qi < 2 * M) | (qi >= kj))
        fill = jnp.where(same, -1e9, -jnp.inf).astype(F32)
        return vis, fill

    mem0 = mem0_ref[...].astype(F32)
    hbuf[0:16, :] = jnp.concatenate([mem0, mem0], axis=0).astype(BF16)
    hbuf[16:48, :] = _ln(x_s[0:SEG, :].astype(F32)).astype(BF16)
    obuf[...] = jnp.zeros((2 * SEG, D), F32)
    x2_s[...] = jnp.zeros(x2_s.shape, F32)

    def seg_row(seg):
        return pl.multiple_of(jnp.clip(seg, 0, NSEG - 1) * SEG, SEG)

    def gate(xa, r0):
        y = jnp.concatenate([y_s[g, pl.ds(r0, SEG), :] for g in range(NLB)], axis=1)
        return xa + _r(_r(_ln(xa)) * y)

    def attention(h, vis, fill):
        def proj(g):
            return [[jnp.dot(h, wslab(t, g * HG + j), preferred_element_type=F32).astype(BF16)
                     for j in range(HG)] for t in range(3)]

        def probs(qkv):
            scs = [lax.dot_general(qkv[0][j], qkv[1][j], (((1,), (1,)), ((), ())),
                                   preferred_element_type=F32) for j in range(HG)]
            ps = []
            for sc in scs:
                sc = jnp.where(vis, sc * scale, fill)
                e = jnp.exp(sc - jnp.max(sc, axis=-1, keepdims=True))
                den = jnp.sum(e, axis=-1, keepdims=True)
                r = pl.reciprocal(den, approx=True)
                r = r * (2.0 - den * r)
                ps.append((e * r).astype(BF16))
            return ps

        def oproj(os_, h0):
            oc = jnp.concatenate(os_, axis=1)
            k0, k1 = h0 * DH, (h0 + len(os_)) * DH
            return [jnp.dot(oc, wo_s[k0:k1, n * 128:(n + 1) * 128], preferred_element_type=F32)
                    for n in range(NLB)]

        heads = []
        qkv = proj(0)
        oa = None
        for g in range(NG):
            ps = probs(qkv)
            vs = qkv[2]
            if g + 1 < NG:
                qkv = proj(g + 1)
            else:
                oa = oproj(heads[:H // 2], 0)
            heads += [jnp.dot(ps[j], vs[j], preferred_element_type=F32).astype(BF16)
                      for j in range(HG)]
        ob = oproj(heads[H // 2:], H // 2)
        return jnp.concatenate([b + a for a, b in zip(oa, ob)], axis=1)

    def post2(s):
        r3 = seg_row(s - 1 - LAG)
        xo = gate(_r(x2_s[(s + 4 - 1 - LAG) % 4] + obuf[SEG:2 * SEG, :]), r3)
        out_s[pl.ds(r3, SEG), :] = xo.astype(BF16)

    def step(s, mode, vis, fill):
        if mode == 0:
            h = hbuf[...]
        elif mode == 1:
            h = hbuf[0:48, :]
        else:
            h = jnp.concatenate([hbuf[0:16, :], hbuf[48:80, :]], axis=0)
        r1 = seg_row(s - 1)
        xb2 = _r(gate(_r(x_s[pl.ds(r1, SEG), :].astype(F32) + obuf[0:SEG, :]), r1))
        h2n = _ln(xb2).astype(BF16)
        if mode != 1:
            post2(s)
        x2_s[(s + 4 - 1) % 4] = xb2
        if mode != 2:
            h1n = _ln(x_s[pl.ds(seg_row(s + 1), SEG), :].astype(F32)).astype(BF16)

        o = attention(h, vis, fill)

        mem2 = mem0 if mode == 1 else o[M:2 * M]
        hbuf[0:16, :] = jnp.concatenate([o[0:M], mem2], axis=0).astype(BF16)
        if mode != 2:
            hbuf[16:48, :] = h1n
        hbuf[48:80, :] = h2n
        if mode == 0:
            obuf[...] = _r(o[2 * M:])
        elif mode == 1:
            obuf[0:SEG, :] = _r(o[2 * M:])
        else:
            obuf[SEG:2 * SEG, :] = _r(o[2 * M:])

    with jax.named_scope("pro"):
        vis, fill = masks(1)
        loop(LAG, lambda s: step(s, 1, vis, fill))
    xb_copy.wait()
    with jax.named_scope("main"):
        vis, fill = masks(0)
        loop(NSEG - LAG, lambda s: step(s + LAG, 0, vis, fill))
    done = (NSEG - 1 - LAG) * SEG
    out_a = pltpu.make_async_copy(out_s.at[0:done, :], out_hbm.at[0:done, :], sem_x.at[1])
    out_a.start()
    with jax.named_scope("epi"):
        vis, fill = masks(2)
        loop(LAG, lambda s: step(s + NSEG, 2, vis, fill))
    post2(NSEG + LAG)
    out_b = pltpu.make_async_copy(out_s.at[done:S, :], out_hbm.at[done:S, :], sem_x.at[2])
    out_b.start()
    out_a.wait()
    out_b.wait()


@functools.partial(jax.jit, static_argnames=("A_seg_len",))
def pallas_interleave_layers__memory_aug_recurrent_mem_tr__ssm_conv_h3__prompt_kernel(
    A_x, A_mem0, A_Wq, A_Wk, A_Wv, A_Wo, A_seg_len,
    B_q, B_k, B_v, B_shift_k, B_ssm_k, B_ssm_D,
):
    assert A_seg_len == SEG and A_x.shape == (1, S, D)
    vm = pl.BlockSpec(memory_space=pltpu.VMEM)
    hbm = pl.BlockSpec(memory_space=pl.ANY)
    out = pl.pallas_call(
        _kernel,
        out_shape=jax.ShapeDtypeStruct((S, D), BF16),
        in_specs=[hbm, vm, hbm, hbm, hbm, hbm, hbm, hbm, vm, hbm, vm],
        out_specs=hbm,
        scratch_shapes=[
            pltpu.VMEM((S, D), BF16),
            pltpu.VMEM((S, D), BF16),
            pltpu.VMEM((S, D), BF16),
            pltpu.VMEM((NB, D, TB), BF16),
            pltpu.VMEM((3, D, H, DH), BF16),
            pltpu.VMEM((3 * H * WP, 128), U32),
            pltpu.VMEM((H * DH, D), BF16),
            pltpu.VMEM((2 * TB, 2 * TB), BF16),
            pltpu.VMEM((2, TB, TB), BF16),
            pltpu.VMEM((2, TB // 2, 3 * TB), BF16),
            pltpu.VMEM((2, NLB, S // 2 + 8, 128), F32),
            pltpu.VMEM((NB // 2, 2, TB, D), F32),
            pltpu.VMEM((NB // 2, 2, TB, D), F32),
            pltpu.VMEM((NB // 2, 3, TB, D), F32),
            pltpu.VMEM((NB // 2, 3, TB, D), F32),
            pltpu.VMEM((NB // 2 + 1, 2, TB, D), F32),
            pltpu.VMEM((NB // 2 + 1, 2, TB, D), F32),
            pltpu.VMEM((NB // 2 - 1, 2, TB, D), F32),
            pltpu.VMEM((NLB, S, 128), F32),
            pltpu.VMEM((ROWS, D), BF16),
            pltpu.VMEM((2 * SEG, D), F32),
            pltpu.VMEM((4, SEG, D), F32),
            pltpu.VMEM((S, D), BF16),
            pltpu.SemaphoreType.DMA((3 * (NB // 2) + 1,)),
            pltpu.SemaphoreType.DMA((4,)),
            pltpu.SemaphoreType.DMA((4,)),
        ],
        compiler_params=pltpu.CompilerParams(vmem_limit_bytes=120 * 1024 * 1024),
    )(A_x.reshape(S, D), A_mem0.reshape(M, D), A_Wq, A_Wk, A_Wv,
      A_Wo.reshape(H * DH, D), B_k.reshape(S, D), B_v.reshape(S, D),
      B_shift_k, B_ssm_k, B_ssm_D.reshape(1, D))
    return out.reshape(1, S, D)
```

```python
import functools
import math

import jax
import jax.numpy as jnp
from jax import lax
import jax.experimental.pallas as pl
import jax.experimental.pallas.tpu as pltpu

F32 = jnp.float32
BF16 = jnp.bfloat16
U32 = jnp.uint32

S = 2048
D = 640
H = 32
DH = 128
M = 8
SEG = 32
NSEG = S // SEG
KS = 4
LAG = 2
ROWS = 2 * M + 2 * SEG
HG = 4
NG = H // HG
NLB = D // 128
TB = 128
NB = S // TB
WP = 324


def _ln(x):
    m = jnp.mean(x, axis=-1, keepdims=True)
    c = x - m
    v = jnp.mean(c * c, axis=-1, keepdims=True)
    return c * lax.rsqrt(v + 1e-5)


def _r(x):
    return x.astype(BF16).astype(F32)


def _split(x):
    hi = pltpu.bitcast(pltpu.bitcast(x, U32) & jnp.uint32(0xFFFF0000), F32)
    return hi, x - hi


def _bf(x):
    return jnp.concatenate([x[:, g:g + 128].astype(BF16)
                            for g in range(0, x.shape[1], 128)], axis=1)


def _basis(r, t):
    b = r & 63
    f = jnp.where(b < 32, 2 * b, 2 * b - 63)
    n = ((2 * f + 1) * t - jnp.where(r >= 64, TB, 0)) & (4 * TB - 1)
    n = jnp.where(n >= 2 * TB, n - 4 * TB, n)
    return jnp.cos(n.astype(F32) * (2.0 * math.pi / (4 * TB)))


def _halves(x):
    w = pltpu.bitcast(x, U32)
    return (pltpu.bitcast(w << 16, F32),
            pltpu.bitcast(w & jnp.uint32(0xFFFF0000), F32))


def _kernel(x_hbm, mem0_ref, wq_hbm, wk_hbm, wv_hbm, wo_hbm,
            k_hbm, v_hbm, shk_ref, ssmk_hbm, ssmd_ref,
            out_hbm,
            x_s, k_s, v_s, ssmk_s, wraw, wt, wo_s,
            fk_s, fu_s, inv_s, kpad, u_a, u_b, kf_a, kf_b, c_a, c_b, c_p, y_s,
            hbuf, obuf, x2_s, out_s,
            sem_c, sem_w, sem_x):
    HB = NB // 2
    XH = 4 * SEG

    def conv_copies(j):
        r0 = j * TB if isinstance(j, int) else pl.multiple_of(j * TB, TB)
        return (
            pltpu.make_async_copy(ssmk_hbm.at[:, pl.ds(r0, TB)], ssmk_s.at[j], sem_c.at[j]),
            pltpu.make_async_copy(k_hbm.at[pl.ds(r0, TB), :], k_s.at[pl.ds(r0, TB), :], sem_c.at[HB + j]),
            pltpu.make_async_copy(v_hbm.at[pl.ds(r0, TB), :], v_s.at[pl.ds(r0, TB), :], sem_c.at[NB + j]),
        )
    late_copies = [pltpu.make_async_copy(ssmk_hbm.at[:, pl.ds(j * TB, TB)], ssmk_s.at[j], sem_c.at[3 * HB])
                   for j in range(HB, NB)]
    late_copies += [pltpu.make_async_copy(src.at[S // 2:, :], dst.at[S // 2:, :], sem_c.at[3 * HB])
                    for src, dst in ((k_hbm, k_s), (v_hbm, v_s))]
    w_copies = [pltpu.make_async_copy(w, wraw.at[t], sem_w.at[t])
                for t, w in enumerate((wq_hbm, wk_hbm, wv_hbm))]
    wo_copy = pltpu.make_async_copy(wo_hbm, wo_s, sem_w.at[3])
    xa_copy = pltpu.make_async_copy(x_hbm.at[0:XH, :], x_s.at[0:XH, :], sem_x.at[0])
    xb_copy = pltpu.make_async_copy(x_hbm.at[XH:, :], x_s.at[XH:, :], sem_x.at[3])
    for j in range(HB):
        for c in conv_copies(j):
            c.start()
    for c in late_copies:
        c.start()
    xa_copy.start()
    wo_copy.start(priority=1)
    xb_copy.start(priority=1)

    hb = TB // 2
    ri = lax.broadcasted_iota(jnp.int32, (TB, TB), 0)
    ci = lax.broadcasted_iota(jnp.int32, (TB, TB), 1)
    full = _basis(ri, ci)
    alt = jnp.where((ci & 1) == 0, full, -full)
    fk = jnp.concatenate([full[:hb], alt[:hb], full[hb:], -alt[hb:]], axis=0)
    fk_s[...] = _bf(jnp.concatenate(_split(fk), axis=1))
    tab = _basis(ri, 2 * (ci & 63) + (ci >> 6))
    hi, lo = _split(tab)
    fu_s[0] = jnp.where(ci < hb, hi, pltpu.roll(lo, hb, 1)).astype(BF16)
    fu_s[1] = jnp.where(ci < hb, pltpu.roll(hi, hb, 1), lo).astype(BF16)
    gh, gl = _split(tab.T * (1.0 / TB))
    ginv = _bf(jnp.concatenate([gh, gl, gh], axis=1))
    inv_s[0] = ginv[:hb]
    inv_s[1] = ginv[hb:]

    eye = (lax.broadcasted_iota(jnp.int32, (8, KS), 0)
           == lax.broadcasted_iota(jnp.int32, (8, KS), 1)).astype(F32).astype(BF16)
    shk_t = lax.dot_general(eye, shk_ref[...], (((1,), (1,)), ((), ())),
                            preferred_element_type=F32)
    taps = [[shk_t[j:j + 1, g * 128:(g + 1) * 128] for g in range(NLB)] for j in range(KS)]
    dvec = ssmd_ref[...].astype(F32)
    for g in range(NLB):
        kpad[0, g, 0:8, :] = jnp.zeros((8, 128), F32)
        kpad[1, g, 0:8, :] = jnp.zeros((8, 128), F32)
    c_a[0] = jnp.zeros(c_a.shape[1:], F32)

    def fwd_stage(jl, half):
        j = jl + half * HB
        u_s, kf_s = ((u_a, kf_a), (u_b, kf_b))[half]
        if half == 0:
            for c in conv_copies(j):
                c.wait()
        kb = ssmk_s[j]
        kf = lax.dot_general(fk_s[...], jnp.concatenate([kb, kb], axis=1),
                             (((1,), (1,)), ((), ())), preferred_element_type=F32)
        kr, ki = kf[0:TB], kf[TB:]
        if half == 0:
            kr = kr + jnp.where(jl == 0, dvec, 0.0)
        kf_s[jl, 0] = kr
        kf_s[jl, 1] = ki - kr
        kf_s[jl, 2] = kr + ki
        r0 = pl.multiple_of(j * TB, TB)
        q0 = pl.multiple_of(j * hb, hb) + 8
        es, os_ = [], []
        for g in range(NLB):
            lb = slice(g * 128, (g + 1) * 128)
            ke, ko = _halves(k_s[pl.ds(r0, TB), lb])
            ve, vo = _halves(v_s[pl.ds(r0, TB), lb])
            kpad[0, g, pl.ds(q0, hb), :] = ke
            kpad[1, g, pl.ds(q0, hb), :] = ko
            ke1 = kpad[0, g, pl.ds(q0 - 1, hb), :]
            ko1 = kpad[1, g, pl.ds(q0 - 1, hb), :]
            ko2 = kpad[1, g, pl.ds(q0 - 2, hb), :]
            t0, t1, t2, t3 = (taps[t][g] for t in range(KS))
            es.append(((ke * t0 + ko1 * t1 + ke1 * t2 + ko2 * t3) * ve).astype(BF16))
            os_.append(((ko * t0 + ke * t1 + ko1 * t2 + ke1 * t3) * vo).astype(BF16))
        e = jnp.concatenate(es, axis=1)
        o = jnp.concatenate(os_, axis=1)
        fe = jnp.dot(fu_s[0], jnp.concatenate([e, e], axis=0), preferred_element_type=F32)
        fo = jnp.dot(fu_s[1], jnp.concatenate([o, o], axis=0), preferred_element_type=F32)
        u_s[jl, 0, 0:hb] = fe[:hb] + fo[:hb]
        u_s[jl, 0, hb:TB] = fe[:hb] - fo[:hb]
        u_s[jl, 1, 0:hb] = fe[hb:] + fo[hb:]
        u_s[jl, 1, hb:TB] = fo[hb:] - fe[hb:]

    def mac_stage(jj, second):
        for rg in range(2):
            rs = pl.ds(pl.multiple_of((2 * jj + rg) * 8, 8), 8)
            for g in range(NLB):
                lb = slice(g * 128, (g + 1) * 128)

                def uu(i, p):
                    u_s = u_a if i < HB else u_b
                    if p == 0:
                        return u_s[i % HB, 0, rs, lb] + u_s[i % HB, 1, rs, lb]
                    return u_s[i % HB, p - 1, rs, lb]

                def kk(i, p):
                    return (kf_a if i < HB else kf_b)[i % HB, p, rs, lb]

                def poly(p, acc):
                    acc = dict(acc)
                    for a0, b0 in (((0, HB), (HB, 0)) if second else ((0, 0),)):
                        ua = [uu(a0 + a, p) for a in range(HB)]
                        kb = [kk(b0 + b, p) for b in range(HB)]
                        for i in range(min(2 * HB - 1, NB - a0 - b0)):
                            for a in range(max(0, i - HB + 1), min(i, HB - 1) + 1):
                                t = ua[a] * kb[i - a]
                                io = i + a0 + b0
                                if io not in acc:
                                    acc[io] = t
                                elif p == 2:
                                    acc[io] = acc[io] - t
                                else:
                                    acc[io] = acc[io] + t
                    return acc

                s1 = poly(0, {})
                for p, comp in ((1, 1), (2, 0)):
                    init = s1
                    if second:
                        init = {i: (v + c_p[i - HB, comp, rs, lb] if i < NB - 1 else v)
                                for i, v in s1.items()}
                    for i, v in poly(p, init).items():
                        if i < HB:
                            c_a[i + 1, comp, rs, lb] = v
                        elif second:
                            c_b[i - HB + 1, comp, rs, lb] = v
                        else:
                            c_p[i - HB, comp, rs, lb] = v
                        if i == HB - 1:
                            c_b[0, comp, rs, lb] = v

    def inv_stage(il, half):
        i = il + half * HB
        c_s = (c_a, c_b)[half]
        q = TB // 4
        re, im = [], []
        for b in range(4):
            rows = slice(b * q, (b + 1) * q)
            cr, ci_ = c_s[il + 1, 0, rows], c_s[il + 1, 1, rows]
            pr, pi = c_s[il, 0, rows], c_s[il, 1, rows]
            re.append(cr + pi if b in (0, 3) else cr - pi)
            im.append(ci_ - pr if b in (0, 3) else ci_ + pr)
        pe = jnp.concatenate([re[0] + re[2], re[1] + re[3], im[0] - im[2], im[1] - im[3]], axis=0)
        po = jnp.concatenate([re[0] - re[2], re[1] - re[3], im[0] + im[2], im[1] + im[3]], axis=0)
        for par, pp in enumerate((pe, po)):
            ph, plo = (_bf(t) for t in _split(pp))
            y = jnp.dot(inv_s[par], jnp.concatenate([ph, ph, plo], axis=0),
                        preferred_element_type=F32)
            for g in range(NLB):
                y_s[g, pl.ds(i * TB + par, hb, stride=2), :] = y[:, g * 128:(g + 1) * 128]

    def relayout(t):
        w_copies[t].wait()

        def body(i, _):
            for dd in range(32):
                dp = i * 32 + dd
                a = pltpu.bitcast(wraw[t, 2 * dp], U32)
                b = pltpu.bitcast(wraw[t, 2 * dp + 1], U32)
                lo = (a & jnp.uint32(0xFFFF)) | (b << 16)
                hi = (a >> 16) | (b & jnp.uint32(0xFFFF0000))
                wt[pl.ds(t * H * WP + dp, 16, stride=WP), :] = lo
                wt[pl.ds((t * H + 16) * WP + dp, 16, stride=WP), :] = hi
            return 0
        lax.fori_loop(0, D // 64, body, 0)

    def wslab(t, h):
        s0 = (t * H + (h % 2) * 16 + h // 2) * WP
        return pltpu.bitcast(wt[s0:s0 + D // 2, :], BF16)

    def loop(n, fn):
        def body(j, _):
            fn(j)
            return 0
        lax.fori_loop(0, n, body, 0)

    with jax.named_scope("conv_a"):
        loop(HB, lambda j: fwd_stage(j, 0))
    with jax.named_scope("conv_b"):
        for c in w_copies:
            c.start()
        loop(HB, lambda j: mac_stage(j, False))
        for c in late_copies:
            c.wait()
        loop(HB // 2, lambda j: (fwd_stage(2 * j, 1), fwd_stage(2 * j + 1, 1)))
    with jax.named_scope("rel0"):
        relayout(0)
    with jax.named_scope("conv_c"):
        loop(HB, lambda j: (inv_stage(j, 0), mac_stage(j, True)))
    with jax.named_scope("rel1"):
        relayout(1)
    with jax.named_scope("conv_d"):
        loop(HB // 2, lambda j: (inv_stage(2 * j, 1), inv_stage(2 * j + 1, 1)))
    with jax.named_scope("rel2"):
        relayout(2)
    with jax.named_scope("waitx"):
        xa_copy.wait()

    scale = DH ** -0.5

    def masks(mode):
        rows = ROWS if mode == 0 else ROWS - SEG
        qi = lax.broadcasted_iota(jnp.int32, (rows, rows), 0)
        kj = lax.broadcasted_iota(jnp.int32, (rows, rows), 1)

        def layer_of(i):
            xl = (i - 2 * M) // SEG if mode == 0 else mode - 1
            return jnp.where(i < 2 * M, i // M, xl)
        same = layer_of(qi) == layer_of(kj)
        vis = same & ((qi < 2 * M) | (qi >= kj))
        fill = jnp.where(same, -1e9, -jnp.inf).astype(F32)
        return vis, fill

    mem0 = mem0_ref[...].astype(F32)
    hbuf[0:16, :] = jnp.concatenate([mem0, mem0], axis=0).astype(BF16)
    hbuf[16:48, :] = _ln(x_s[0:SEG, :].astype(F32)).astype(BF16)
    obuf[...] = jnp.zeros((2 * SEG, D), F32)
    x2_s[...] = jnp.zeros(x2_s.shape, F32)

    def seg_row(seg):
        if isinstance(seg, int):
            return min(max(seg, 0), NSEG - 1) * SEG
        return pl.multiple_of(jnp.clip(seg, 0, NSEG - 1) * SEG, SEG)

    def gate(xa, r0):
        y = jnp.concatenate([y_s[g, pl.ds(r0, SEG), :] for g in range(NLB)], axis=1)
        return xa + _r(_r(_ln(xa)) * y)

    def attention(h, vis, fill, before_oproj=None):
        def proj(g):
            return [[jnp.dot(h, wslab(t, g * HG + j), preferred_element_type=F32).astype(BF16)
                     for j in range(HG)] for t in range(3)]

        def probs(qkv):
            scs = [lax.dot_general(qkv[0][j], qkv[1][j], (((1,), (1,)), ((), ())),
                                   preferred_element_type=F32) for j in range(HG)]
            ps = []
            for sc in scs:
                sc = jnp.where(vis, sc * scale, fill)
                e = jnp.exp(sc - jnp.max(sc, axis=-1, keepdims=True))
                den = jnp.sum(e, axis=-1, keepdims=True)
                r = pl.reciprocal(den, approx=True)
                r = r * (2.0 - den * r)
                ps.append((e * r).astype(BF16))
            return ps

        def oproj(os_, h0):
            oc = jnp.concatenate(os_, axis=1)
            k0, k1 = h0 * DH, (h0 + len(os_)) * DH
            return [jnp.dot(oc, wo_s[k0:k1, n * 128:(n + 1) * 128], preferred_element_type=F32)
                    for n in range(NLB)]

        heads = []
        qkv = proj(0)
        oa = None
        for g in range(NG):
            ps = probs(qkv)
            vs = qkv[2]
            if g + 1 < NG:
                qkv = proj(g + 1)
            else:
                if before_oproj is not None:
                    before_oproj()
                oa = oproj(heads[:H // 2], 0)
            heads += [jnp.dot(ps[j], vs[j], preferred_element_type=F32).astype(BF16)
                      for j in range(HG)]
        ob = oproj(heads[H // 2:], H // 2)
        return jnp.concatenate([b + a for a, b in zip(oa, ob)], axis=1)

    def post2(s):
        r3 = seg_row(s - 1 - LAG)
        xo = gate(_r(x2_s[(s + 4 - 1 - LAG) % 4] + obuf[SEG:2 * SEG, :]), r3)
        out_s[pl.ds(r3, SEG), :] = xo.astype(BF16)

    def step(s, mode, vis, fill, before_oproj=None):
        if mode == 0:
            h = hbuf[...]
        elif mode == 1:
            h = hbuf[0:48, :]
        else:
            h = jnp.concatenate([hbuf[0:16, :], hbuf[48:80, :]], axis=0)
        r1 = seg_row(s - 1)
        xb2 = _r(gate(_r(x_s[pl.ds(r1, SEG), :].astype(F32) + obuf[0:SEG, :]), r1))
        h2n = _ln(xb2).astype(BF16)
        if mode != 1:
            post2(s)
        x2_s[(s + 4 - 1) % 4] = xb2
        if mode != 2:
            h1n = _ln(x_s[pl.ds(seg_row(s + 1), SEG), :].astype(F32)).astype(BF16)

        o = attention(h, vis, fill, before_oproj)

        mem2 = mem0 if mode == 1 else o[M:2 * M]
        hbuf[0:16, :] = jnp.concatenate([o[0:M], mem2], axis=0).astype(BF16)
        if mode != 2:
            hbuf[16:48, :] = h1n
        hbuf[48:80, :] = h2n
        if mode == 0:
            obuf[...] = _r(o[2 * M:])
        elif mode == 1:
            obuf[0:SEG, :] = _r(o[2 * M:])
        else:
            obuf[SEG:2 * SEG, :] = _r(o[2 * M:])

    with jax.named_scope("pro"):
        vis, fill = masks(1)
        step(0, 1, vis, fill, wo_copy.wait)
        step(1, 1, vis, fill)
    xb_copy.wait()
    with jax.named_scope("main"):
        vis, fill = masks(0)
        loop(NSEG - LAG, lambda s: step(s + LAG, 0, vis, fill))
    done = (NSEG - 1 - LAG) * SEG
    out_a = pltpu.make_async_copy(out_s.at[0:done, :], out_hbm.at[0:done, :], sem_x.at[1])
    out_a.start()
    with jax.named_scope("epi"):
        vis, fill = masks(2)
        loop(LAG, lambda s: step(s + NSEG, 2, vis, fill))
    post2(NSEG + LAG)
    out_b = pltpu.make_async_copy(out_s.at[done:S, :], out_hbm.at[done:S, :], sem_x.at[2])
    out_b.start()
    out_a.wait()
    out_b.wait()


@functools.partial(jax.jit, static_argnames=("A_seg_len",))
def pallas_interleave_layers__memory_aug_recurrent_mem_tr__ssm_conv_h3__prompt_kernel(
    A_x, A_mem0, A_Wq, A_Wk, A_Wv, A_Wo, A_seg_len,
    B_q, B_k, B_v, B_shift_k, B_ssm_k, B_ssm_D,
):
    assert A_seg_len == SEG and A_x.shape == (1, S, D)
    vm = pl.BlockSpec(memory_space=pltpu.VMEM)
    hbm = pl.BlockSpec(memory_space=pl.ANY)
    out = pl.pallas_call(
        _kernel,
        out_shape=jax.ShapeDtypeStruct((S, D), BF16),
        in_specs=[hbm, vm, hbm, hbm, hbm, hbm, hbm, hbm, vm, hbm, vm],
        out_specs=hbm,
        scratch_shapes=[
            pltpu.VMEM((S, D), BF16),
            pltpu.VMEM((S, D), BF16),
            pltpu.VMEM((S, D), BF16),
            pltpu.VMEM((NB, D, TB), BF16),
            pltpu.VMEM((3, D, H, DH), BF16),
            pltpu.VMEM((3 * H * WP, 128), U32),
            pltpu.VMEM((H * DH, D), BF16),
            pltpu.VMEM((2 * TB, 2 * TB), BF16),
            pltpu.VMEM((2, TB, TB), BF16),
            pltpu.VMEM((2, TB // 2, 3 * TB), BF16),
            pltpu.VMEM((2, NLB, S // 2 + 8, 128), F32),
            pltpu.VMEM((NB // 2, 2, TB, D), F32),
            pltpu.VMEM((NB // 2, 2, TB, D), F32),
            pltpu.VMEM((NB // 2, 3, TB, D), F32),
            pltpu.VMEM((NB // 2, 3, TB, D), F32),
            pltpu.VMEM((NB // 2 + 1, 2, TB, D), F32),
            pltpu.VMEM((NB // 2 + 1, 2, TB, D), F32),
            pltpu.VMEM((NB // 2 - 1, 2, TB, D), F32),
            pltpu.VMEM((NLB, S, 128), F32),
            pltpu.VMEM((ROWS, D), BF16),
            pltpu.VMEM((2 * SEG, D), F32),
            pltpu.VMEM((4, SEG, D), F32),
            pltpu.VMEM((S, D), BF16),
            pltpu.SemaphoreType.DMA((3 * (NB // 2) + 1,)),
            pltpu.SemaphoreType.DMA((4,)),
            pltpu.SemaphoreType.DMA((4,)),
        ],
        compiler_params=pltpu.CompilerParams(vmem_limit_bytes=120 * 1024 * 1024),
    )(A_x.reshape(S, D), A_mem0.reshape(M, D), A_Wq, A_Wk, A_Wv,
      A_Wo.reshape(H * DH, D), B_k.reshape(S, D), B_v.reshape(S, D),
      B_shift_k, B_ssm_k, B_ssm_D.reshape(1, D))
    return out.reshape(1, S, D)
```

```python
import functools
import math

import jax
import jax.numpy as jnp
from jax import lax
import jax.experimental.pallas as pl
import jax.experimental.pallas.tpu as pltpu

F32 = jnp.float32
BF16 = jnp.bfloat16
U32 = jnp.uint32

S = 2048
D = 640
H = 32
DH = 128
M = 8
SEG = 32
NSEG = S // SEG
KS = 4
LAG = 2
ROWS = 2 * M + 2 * SEG
HG = 4
NG = H // HG
NLB = D // 128
TB = 128
NB = S // TB
WP = 324


def _ln(x):
    m = jnp.mean(x, axis=-1, keepdims=True)
    c = x - m
    v = jnp.mean(c * c, axis=-1, keepdims=True)
    return c * lax.rsqrt(v + 1e-5)


def _r(x):
    return x.astype(BF16).astype(F32)


def _split(x):
    hi = pltpu.bitcast(pltpu.bitcast(x, U32) & jnp.uint32(0xFFFF0000), F32)
    return hi, x - hi


def _bf(x):
    return jnp.concatenate([x[:, g:g + 128].astype(BF16)
                            for g in range(0, x.shape[1], 128)], axis=1)


def _basis(r, t):
    b = r & 63
    f = jnp.where(b < 32, 2 * b, 2 * b - 63)
    n = ((2 * f + 1) * t - jnp.where(r >= 64, TB, 0)) & (4 * TB - 1)
    n = jnp.where(n >= 2 * TB, n - 4 * TB, n)
    return jnp.cos(n.astype(F32) * (2.0 * math.pi / (4 * TB)))


def _halves(x):
    w = pltpu.bitcast(x, U32)
    return (pltpu.bitcast(w << 16, F32),
            pltpu.bitcast(w & jnp.uint32(0xFFFF0000), F32))


def _kernel(x_hbm, mem0_ref, wq_hbm, wk_hbm, wv_hbm, wo_hbm,
            k_hbm, v_hbm, shk_ref, ssmk_hbm, ssmd_ref,
            out_hbm,
            x_s, k_s, v_s, ssmk_s, wraw, wt, wo_s,
            fk_s, fu_s, inv_s, kpad, u_a, u_b, kf_a, kf_b, c_a, c_b, c_p, y_s,
            hbuf, obuf, x2_s, out_s,
            sem_c, sem_w, sem_x):
    HB = NB // 2
    XH = 4 * SEG

    def conv_copies(j):
        r0 = j * TB if isinstance(j, int) else pl.multiple_of(j * TB, TB)
        return (
            pltpu.make_async_copy(ssmk_hbm.at[:, pl.ds(r0, TB)], ssmk_s.at[j], sem_c.at[j]),
            pltpu.make_async_copy(k_hbm.at[pl.ds(r0, TB), :], k_s.at[pl.ds(r0, TB), :], sem_c.at[HB + j]),
            pltpu.make_async_copy(v_hbm.at[pl.ds(r0, TB), :], v_s.at[pl.ds(r0, TB), :], sem_c.at[NB + j]),
        )
    late_copies = [pltpu.make_async_copy(ssmk_hbm.at[:, pl.ds(j * TB, TB)], ssmk_s.at[j], sem_c.at[3 * HB])
                   for j in range(HB, NB)]
    late_copies += [pltpu.make_async_copy(src.at[S // 2:, :], dst.at[S // 2:, :], sem_c.at[3 * HB])
                    for src, dst in ((k_hbm, k_s), (v_hbm, v_s))]
    w_copies = [pltpu.make_async_copy(w, wraw.at[t], sem_w.at[t])
                for t, w in enumerate((wq_hbm, wk_hbm, wv_hbm))]
    wo_copy = pltpu.make_async_copy(wo_hbm, wo_s, sem_w.at[3])
    xa_copy = pltpu.make_async_copy(x_hbm.at[0:XH, :], x_s.at[0:XH, :], sem_x.at[0])
    xb_copy = pltpu.make_async_copy(x_hbm.at[XH:, :], x_s.at[XH:, :], sem_x.at[3])
    for j in range(HB):
        for c in conv_copies(j):
            c.start()
    for c in late_copies:
        c.start()
    xa_copy.start()
    wo_copy.start(priority=1)
    xb_copy.start(priority=1)

    hb = TB // 2
    ri = lax.broadcasted_iota(jnp.int32, (TB, TB), 0)
    ci = lax.broadcasted_iota(jnp.int32, (TB, TB), 1)
    full = _basis(ri, ci)
    alt = jnp.where((ci & 1) == 0, full, -full)
    fk = jnp.concatenate([full[:hb], alt[:hb], full[hb:], -alt[hb:]], axis=0)
    fk_s[...] = _bf(jnp.concatenate(_split(fk), axis=1))
    tab = _basis(ri, 2 * (ci & 63) + (ci >> 6))
    hi, lo = _split(tab)
    fu_s[0] = jnp.where(ci < hb, hi, pltpu.roll(lo, hb, 1)).astype(BF16)
    fu_s[1] = jnp.where(ci < hb, pltpu.roll(hi, hb, 1), lo).astype(BF16)
    gh, gl = _split(tab.T * (1.0 / TB))
    ginv = _bf(jnp.concatenate([gh, gl, gh], axis=1))
    inv_s[0] = ginv[:hb]
    inv_s[1] = ginv[hb:]

    eye = (lax.broadcasted_iota(jnp.int32, (8, KS), 0)
           == lax.broadcasted_iota(jnp.int32, (8, KS), 1)).astype(F32).astype(BF16)
    shk_t = lax.dot_general(eye, shk_ref[...], (((1,), (1,)), ((), ())),
                            preferred_element_type=F32)
    taps = [[shk_t[j:j + 1, g * 128:(g + 1) * 128] for g in range(NLB)] for j in range(KS)]
    dvec = ssmd_ref[...].astype(F32)
    for g in range(NLB):
        kpad[0, g, 0:8, :] = jnp.zeros((8, 128), F32)
        kpad[1, g, 0:8, :] = jnp.zeros((8, 128), F32)
    c_a[0] = jnp.zeros(c_a.shape[1:], F32)

    def fwd_stage(jl, half):
        j = jl + half * HB
        u_s, kf_s = ((u_a, kf_a), (u_b, kf_b))[half]
        if half == 0:
            for c in conv_copies(j):
                c.wait()
        kb = ssmk_s[j]
        kf = lax.dot_general(fk_s[...], jnp.concatenate([kb, kb], axis=1),
                             (((1,), (1,)), ((), ())), preferred_element_type=F32)
        kr, ki = kf[0:TB], kf[TB:]
        if half == 0:
            kr = kr + jnp.where(jl == 0, dvec, 0.0)
        kf_s[jl, 0] = kr
        kf_s[jl, 1] = ki - kr
        kf_s[jl, 2] = kr + ki
        r0 = pl.multiple_of(j * TB, TB)
        q0 = pl.multiple_of(j * hb, hb) + 8
        es, os_ = [], []
        for g in range(NLB):
            lb = slice(g * 128, (g + 1) * 128)
            ke, ko = _halves(k_s[pl.ds(r0, TB), lb])
            ve, vo = _halves(v_s[pl.ds(r0, TB), lb])
            kpad[0, g, pl.ds(q0, hb), :] = ke
            kpad[1, g, pl.ds(q0, hb), :] = ko
            ke1 = kpad[0, g, pl.ds(q0 - 1, hb), :]
            ko1 = kpad[1, g, pl.ds(q0 - 1, hb), :]
            ko2 = kpad[1, g, pl.ds(q0 - 2, hb), :]
            t0, t1, t2, t3 = (taps[t][g] for t in range(KS))
            es.append(((ke * t0 + ko1 * t1 + ke1 * t2 + ko2 * t3) * ve))
            os_.append(((ko * t0 + ke * t1 + ko1 * t2 + ke1 * t3) * vo))
        e = jnp.concatenate(es, axis=1)
        o = jnp.concatenate(os_, axis=1)
        fe = jnp.dot(fu_s[0], jnp.concatenate([e, e], axis=0).astype(BF16), preferred_element_type=F32)
        fo = jnp.dot(fu_s[1], jnp.concatenate([o, o], axis=0).astype(BF16), preferred_element_type=F32)
        u_s[jl, 0, 0:hb] = fe[:hb] + fo[:hb]
        u_s[jl, 0, hb:TB] = fe[:hb] - fo[:hb]
        u_s[jl, 1, 0:hb] = fe[hb:] + fo[hb:]
        u_s[jl, 1, hb:TB] = fo[hb:] - fe[hb:]

    def mac_stage(jj, second):
        for rg in range(2):
            rs = pl.ds(pl.multiple_of((2 * jj + rg) * 8, 8), 8)
            for g in range(NLB):
                lb = slice(g * 128, (g + 1) * 128)

                def uu(i, p):
                    u_s = u_a if i < HB else u_b
                    if p == 0:
                        return u_s[i % HB, 0, rs, lb] + u_s[i % HB, 1, rs, lb]
                    return u_s[i % HB, p - 1, rs, lb]

                def kk(i, p):
                    return (kf_a if i < HB else kf_b)[i % HB, p, rs, lb]

                def poly(p, acc):
                    acc = dict(acc)
                    for a0, b0 in (((0, HB), (HB, 0)) if second else ((0, 0),)):
                        ua = [uu(a0 + a, p) for a in range(HB)]
                        kb = [kk(b0 + b, p) for b in range(HB)]
                        for i in range(min(2 * HB - 1, NB - a0 - b0)):
                            for a in range(max(0, i - HB + 1), min(i, HB - 1) + 1):
                                t = ua[a] * kb[i - a]
                                io = i + a0 + b0
                                if io not in acc:
                                    acc[io] = t
                                elif p == 2:
                                    acc[io] = acc[io] - t
                                else:
                                    acc[io] = acc[io] + t
                    return acc

                s1 = poly(0, {})
                for p, comp in ((1, 1), (2, 0)):
                    init = s1
                    if second:
                        init = {i: (v + c_p[i - HB, comp, rs, lb] if i < NB - 1 else v)
                                for i, v in s1.items()}
                    for i, v in poly(p, init).items():
                        if i < HB:
                            c_a[i + 1, comp, rs, lb] = v
                        elif second:
                            c_b[i - HB + 1, comp, rs, lb] = v
                        else:
                            c_p[i - HB, comp, rs, lb] = v
                        if i == HB - 1:
                            c_b[0, comp, rs, lb] = v

    def inv_stage(il, half):
        i = il + half * HB
        c_s = (c_a, c_b)[half]
        q = TB // 4
        re, im = [], []
        for b in range(4):
            rows = slice(b * q, (b + 1) * q)
            cr, ci_ = c_s[il + 1, 0, rows], c_s[il + 1, 1, rows]
            pr, pi = c_s[il, 0, rows], c_s[il, 1, rows]
            re.append(cr + pi if b in (0, 3) else cr - pi)
            im.append(ci_ - pr if b in (0, 3) else ci_ + pr)
        pe = jnp.concatenate([re[0] + re[2], re[1] + re[3], im[0] - im[2], im[1] - im[3]], axis=0)
        po = jnp.concatenate([re[0] - re[2], re[1] - re[3], im[0] + im[2], im[1] + im[3]], axis=0)
        for par, pp in enumerate((pe, po)):
            ph, plo = _split(pp)
            y = jnp.dot(inv_s[par], jnp.concatenate([ph, ph, plo], axis=0).astype(BF16),
                        preferred_element_type=F32)
            for g in range(NLB):
                y_s[g, pl.ds(i * TB + par, hb, stride=2), :] = y[:, g * 128:(g + 1) * 128]

    def relayout(t):
        w_copies[t].wait()

        def body(i, _):
            for dd in range(32):
                dp = i * 32 + dd
                a = pltpu.bitcast(wraw[t, 2 * dp], U32)
                b = pltpu.bitcast(wraw[t, 2 * dp + 1], U32)
                lo = (a & jnp.uint32(0xFFFF)) | (b << 16)
                hi = (a >> 16) | (b & jnp.uint32(0xFFFF0000))
                wt[pl.ds(t * H * WP + dp, 16, stride=WP), :] = lo
                wt[pl.ds((t * H + 16) * WP + dp, 16, stride=WP), :] = hi
            return 0
        lax.fori_loop(0, D // 64, body, 0)

    def wslab(t, h):
        s0 = (t * H + (h % 2) * 16 + h // 2) * WP
        return pltpu.bitcast(wt[s0:s0 + D // 2, :], BF16)

    def loop(n, fn):
        def body(j, _):
            fn(j)
            return 0
        lax.fori_loop(0, n, body, 0)

    with jax.named_scope("conv_a"):
        loop(HB, lambda j: fwd_stage(j, 0))
    with jax.named_scope("conv_b"):
        for c in w_copies:
            c.start()
        loop(HB, lambda j: mac_stage(j, False))
        for c in late_copies:
            c.wait()
        loop(HB // 2, lambda j: (fwd_stage(2 * j, 1), fwd_stage(2 * j + 1, 1)))
    with jax.named_scope("rel0"):
        relayout(0)
    with jax.named_scope("conv_c"):
        loop(HB, lambda j: (inv_stage(j, 0), mac_stage(j, True)))
    with jax.named_scope("rel1"):
        relayout(1)
    with jax.named_scope("conv_d"):
        loop(HB // 2, lambda j: (inv_stage(2 * j, 1), inv_stage(2 * j + 1, 1)))
    with jax.named_scope("rel2"):
        relayout(2)
    with jax.named_scope("waitx"):
        xa_copy.wait()

    scale = DH ** -0.5

    def masks(mode):
        rows = ROWS if mode == 0 else ROWS - SEG
        qi = lax.broadcasted_iota(jnp.int32, (rows, rows), 0)
        kj = lax.broadcasted_iota(jnp.int32, (rows, rows), 1)

        def layer_of(i):
            xl = (i - 2 * M) // SEG if mode == 0 else mode - 1
            return jnp.where(i < 2 * M, i // M, xl)
        same = layer_of(qi) == layer_of(kj)
        vis = same & ((qi < 2 * M) | (qi >= kj))
        fill = jnp.where(same, -1e9, -jnp.inf).astype(F32)
        return vis, fill

    mem0 = mem0_ref[...].astype(F32)
    hbuf[0:16, :] = jnp.concatenate([mem0, mem0], axis=0).astype(BF16)
    hbuf[16:48, :] = _ln(x_s[0:SEG, :].astype(F32)).astype(BF16)
    obuf[...] = jnp.zeros((2 * SEG, D), F32)
    x2_s[...] = jnp.zeros(x2_s.shape, F32)

    def seg_row(seg):
        if isinstance(seg, int):
            return min(max(seg, 0), NSEG - 1) * SEG
        return pl.multiple_of(jnp.clip(seg, 0, NSEG - 1) * SEG, SEG)

    def gate(xa, r0):
        y = jnp.concatenate([y_s[g, pl.ds(r0, SEG), :] for g in range(NLB)], axis=1)
        return xa + _r(_r(_ln(xa)) * y)

    def attention(h, vis, fill, before_oproj=None):
        def proj(g):
            return [[jnp.dot(h, wslab(t, g * HG + j), preferred_element_type=F32).astype(BF16)
                     for j in range(HG)] for t in range(3)]

        def probs(qkv):
            scs = [lax.dot_general(qkv[0][j], qkv[1][j], (((1,), (1,)), ((), ())),
                                   preferred_element_type=F32) for j in range(HG)]
            ps = []
            for sc in scs:
                sc = jnp.where(vis, sc * scale, fill)
                e = jnp.exp(sc - jnp.max(sc, axis=-1, keepdims=True))
                den = jnp.sum(e, axis=-1, keepdims=True)
                r = pl.reciprocal(den, approx=True)
                r = r * (2.0 - den * r)
                ps.append((e * r).astype(BF16))
            return ps

        def oproj(os_, h0):
            oc = jnp.concatenate(os_, axis=1)
            k0, k1 = h0 * DH, (h0 + len(os_)) * DH
            return [jnp.dot(oc, wo_s[k0:k1, n * 128:(n + 1) * 128], preferred_element_type=F32)
                    for n in range(NLB)]

        heads = []
        qkv = proj(0)
        oa = None
        for g in range(NG):
            ps = probs(qkv)
            vs = qkv[2]
            if g + 1 < NG:
                qkv = proj(g + 1)
            else:
                if before_oproj is not None:
                    before_oproj()
                oa = oproj(heads[:H // 2], 0)
            heads += [jnp.dot(ps[j], vs[j], preferred_element_type=F32).astype(BF16)
                      for j in range(HG)]
        ob = oproj(heads[H // 2:], H // 2)
        return jnp.concatenate([b + a for a, b in zip(oa, ob)], axis=1)

    def post2(s):
        r3 = seg_row(s - 1 - LAG)
        xo = gate(_r(x2_s[(s + 4 - 1 - LAG) % 4] + obuf[SEG:2 * SEG, :]), r3)
        out_s[pl.ds(r3, SEG), :] = xo.astype(BF16)

    def step(s, mode, vis, fill, before_oproj=None):
        if mode == 0:
            h = hbuf[...]
        elif mode == 1:
            h = hbuf[0:48, :]
        else:
            h = jnp.concatenate([hbuf[0:16, :], hbuf[48:80, :]], axis=0)
        r1 = seg_row(s - 1)
        xb2 = _r(gate(_r(x_s[pl.ds(r1, SEG), :].astype(F32) + obuf[0:SEG, :]), r1))
        h2n = _ln(xb2).astype(BF16)
        if mode != 1:
            post2(s)
        x2_s[(s + 4 - 1) % 4] = xb2
        if mode != 2:
            h1n = _ln(x_s[pl.ds(seg_row(s + 1), SEG), :].astype(F32)).astype(BF16)

        o = attention(h, vis, fill, before_oproj)

        mem2 = mem0 if mode == 1 else o[M:2 * M]
        hbuf[0:16, :] = jnp.concatenate([o[0:M], mem2], axis=0).astype(BF16)
        if mode != 2:
            hbuf[16:48, :] = h1n
        hbuf[48:80, :] = h2n
        if mode == 0:
            obuf[...] = _r(o[2 * M:])
        elif mode == 1:
            obuf[0:SEG, :] = _r(o[2 * M:])
        else:
            obuf[SEG:2 * SEG, :] = _r(o[2 * M:])

    with jax.named_scope("pro"):
        vis, fill = masks(1)
        step(0, 1, vis, fill, wo_copy.wait)
        step(1, 1, vis, fill)
    xb_copy.wait()
    with jax.named_scope("main"):
        vis, fill = masks(0)
        loop(NSEG - LAG, lambda s: step(s + LAG, 0, vis, fill))
    done = (NSEG - 1 - LAG) * SEG
    out_a = pltpu.make_async_copy(out_s.at[0:done, :], out_hbm.at[0:done, :], sem_x.at[1])
    out_a.start()
    with jax.named_scope("epi"):
        vis, fill = masks(2)
        loop(LAG, lambda s: step(s + NSEG, 2, vis, fill))
    post2(NSEG + LAG)
    out_b = pltpu.make_async_copy(out_s.at[done:S, :], out_hbm.at[done:S, :], sem_x.at[2])
    out_b.start()
    out_a.wait()
    out_b.wait()


@functools.partial(jax.jit, static_argnames=("A_seg_len",))
def pallas_interleave_layers__memory_aug_recurrent_mem_tr__ssm_conv_h3__prompt_kernel(
    A_x, A_mem0, A_Wq, A_Wk, A_Wv, A_Wo, A_seg_len,
    B_q, B_k, B_v, B_shift_k, B_ssm_k, B_ssm_D,
):
    assert A_seg_len == SEG and A_x.shape == (1, S, D)
    vm = pl.BlockSpec(memory_space=pltpu.VMEM)
    hbm = pl.BlockSpec(memory_space=pl.ANY)
    out = pl.pallas_call(
        _kernel,
        out_shape=jax.ShapeDtypeStruct((S, D), BF16),
        in_specs=[hbm, vm, hbm, hbm, hbm, hbm, hbm, hbm, vm, hbm, vm],
        out_specs=hbm,
        scratch_shapes=[
            pltpu.VMEM((S, D), BF16),
            pltpu.VMEM((S, D), BF16),
            pltpu.VMEM((S, D), BF16),
            pltpu.VMEM((NB, D, TB), BF16),
            pltpu.VMEM((3, D, H, DH), BF16),
            pltpu.VMEM((3 * H * WP, 128), U32),
            pltpu.VMEM((H * DH, D), BF16),
            pltpu.VMEM((2 * TB, 2 * TB), BF16),
            pltpu.VMEM((2, TB, TB), BF16),
            pltpu.VMEM((2, TB // 2, 3 * TB), BF16),
            pltpu.VMEM((2, NLB, S // 2 + 8, 128), F32),
            pltpu.VMEM((NB // 2, 2, TB, D), F32),
            pltpu.VMEM((NB // 2, 2, TB, D), F32),
            pltpu.VMEM((NB // 2, 3, TB, D), F32),
            pltpu.VMEM((NB // 2, 3, TB, D), F32),
            pltpu.VMEM((NB // 2 + 1, 2, TB, D), F32),
            pltpu.VMEM((NB // 2 + 1, 2, TB, D), F32),
            pltpu.VMEM((NB // 2 - 1, 2, TB, D), F32),
            pltpu.VMEM((NLB, S, 128), F32),
            pltpu.VMEM((ROWS, D), BF16),
            pltpu.VMEM((2 * SEG, D), F32),
            pltpu.VMEM((4, SEG, D), F32),
            pltpu.VMEM((S, D), BF16),
            pltpu.SemaphoreType.DMA((3 * (NB // 2) + 1,)),
            pltpu.SemaphoreType.DMA((4,)),
            pltpu.SemaphoreType.DMA((4,)),
        ],
        compiler_params=pltpu.CompilerParams(vmem_limit_bytes=120 * 1024 * 1024),
    )(A_x.reshape(S, D), A_mem0.reshape(M, D), A_Wq, A_Wk, A_Wv,
      A_Wo.reshape(H * DH, D), B_k.reshape(S, D), B_v.reshape(S, D),
      B_shift_k, B_ssm_k, B_ssm_D.reshape(1, D))
    return out.reshape(1, S, D)
```

```python
import functools
import math

import jax
import jax.numpy as jnp
from jax import lax
import jax.experimental.pallas as pl
import jax.experimental.pallas.tpu as pltpu

F32 = jnp.float32
BF16 = jnp.bfloat16
U32 = jnp.uint32

S = 2048
D = 640
H = 32
DH = 128
M = 8
SEG = 32
NSEG = S // SEG
KS = 4
LAG = 2
ROWS = 2 * M + 2 * SEG
HG = 4
NG = H // HG
NLB = D // 128
TB = 128
NB = S // TB
WP = 324


def _ln(x):
    m = jnp.mean(x, axis=-1, keepdims=True)
    c = x - m
    v = jnp.mean(c * c, axis=-1, keepdims=True)
    return c * lax.rsqrt(v + 1e-5)


def _r(x):
    return x.astype(BF16).astype(F32)


def _split(x):
    hi = pltpu.bitcast(pltpu.bitcast(x, U32) & jnp.uint32(0xFFFF0000), F32)
    return hi, x - hi


def _bf(x):
    return jnp.concatenate([x[:, g:g + 128].astype(BF16)
                            for g in range(0, x.shape[1], 128)], axis=1)


def _basis(r, t):
    b = r & 63
    f = jnp.where(b < 32, 2 * b, 2 * b - 63)
    n = ((2 * f + 1) * t - jnp.where(r >= 64, TB, 0)) & (4 * TB - 1)
    n = jnp.where(n >= 2 * TB, n - 4 * TB, n)
    return jnp.cos(n.astype(F32) * (2.0 * math.pi / (4 * TB)))


def _halves(x):
    w = pltpu.bitcast(x, U32)
    return (pltpu.bitcast(w << 16, F32),
            pltpu.bitcast(w & jnp.uint32(0xFFFF0000), F32))


def _kernel(x_hbm, mem0_ref, wq_hbm, wk_hbm, wv_hbm, wo_hbm,
            k_hbm, v_hbm, shk_ref, ssmk_hbm, ssmd_ref,
            out_hbm,
            x_s, k_s, v_s, ssmk_s, wraw, wt, wo_s,
            fk_s, fu_s, inv_s, kpad, u_a, u_b, kf_a, kf_b, c_a, c_b, c_p, y_s,
            hbuf, obuf, x2_s, out_s,
            sem_c, sem_w, sem_x):
    HB = NB // 2
    XH = 4 * SEG

    def conv_copies(j):
        r0 = j * TB if isinstance(j, int) else pl.multiple_of(j * TB, TB)
        return (
            pltpu.make_async_copy(ssmk_hbm.at[:, pl.ds(r0, TB)], ssmk_s.at[j], sem_c.at[j]),
            pltpu.make_async_copy(k_hbm.at[pl.ds(r0, TB), :], k_s.at[pl.ds(r0, TB), :], sem_c.at[HB + j]),
            pltpu.make_async_copy(v_hbm.at[pl.ds(r0, TB), :], v_s.at[pl.ds(r0, TB), :], sem_c.at[NB + j]),
        )
    late_copies = [pltpu.make_async_copy(ssmk_hbm.at[:, pl.ds(j * TB, TB)], ssmk_s.at[j], sem_c.at[3 * HB])
                   for j in range(HB, NB)]
    late_copies += [pltpu.make_async_copy(src.at[S // 2:, :], dst.at[S // 2:, :], sem_c.at[3 * HB])
                    for src, dst in ((k_hbm, k_s), (v_hbm, v_s))]
    w_copies = [pltpu.make_async_copy(w, wraw.at[t], sem_w.at[t])
                for t, w in enumerate((wq_hbm, wk_hbm, wv_hbm))]
    wo_copy = pltpu.make_async_copy(wo_hbm, wo_s, sem_w.at[3])
    xa_copy = pltpu.make_async_copy(x_hbm.at[0:XH, :], x_s.at[0:XH, :], sem_x.at[0])
    xb_copy = pltpu.make_async_copy(x_hbm.at[XH:, :], x_s.at[XH:, :], sem_x.at[3])
    for j in range(HB):
        for c in conv_copies(j):
            c.start()
    for c in late_copies:
        c.start()
    xa_copy.start()
    wo_copy.start(priority=1)
    xb_copy.start(priority=1)

    hb = TB // 2
    ri = lax.broadcasted_iota(jnp.int32, (TB, TB), 0)
    ci = lax.broadcasted_iota(jnp.int32, (TB, TB), 1)
    full = _basis(ri, ci)
    alt = jnp.where((ci & 1) == 0, full, -full)
    fk = jnp.concatenate([full[:hb], alt[:hb], full[hb:], -alt[hb:]], axis=0)
    fk_s[...] = _bf(jnp.concatenate(_split(fk), axis=1))
    tab = _basis(ri, 2 * (ci & 63) + (ci >> 6))
    hi, lo = _split(tab)
    fu_s[0] = jnp.where(ci < hb, hi, pltpu.roll(lo, hb, 1)).astype(BF16)
    fu_s[1] = jnp.where(ci < hb, pltpu.roll(hi, hb, 1), lo).astype(BF16)
    gh, gl = _split(tab.T * (1.0 / TB))
    ginv = _bf(jnp.concatenate([gh, gl, gh], axis=1))
    inv_s[0] = ginv[:hb]
    inv_s[1] = ginv[hb:]

    shk_t = shk_ref[...].astype(F32)
    taps = [[shk_t[j:j + 1, g * 128:(g + 1) * 128] for g in range(NLB)] for j in range(KS)]
    dvec = ssmd_ref[...].astype(F32).reshape(1, D)
    for g in range(NLB):
        kpad[0, g, 0:8, :] = jnp.zeros((8, 128), F32)
        kpad[1, g, 0:8, :] = jnp.zeros((8, 128), F32)
    c_a[0] = jnp.zeros(c_a.shape[1:], F32)

    def fwd_stage(jl, half):
        j = jl + half * HB
        u_s, kf_s = ((u_a, kf_a), (u_b, kf_b))[half]
        if half == 0:
            for c in conv_copies(j):
                c.wait()
        kb = ssmk_s[j]
        kf = lax.dot_general(fk_s[...], jnp.concatenate([kb, kb], axis=1),
                             (((1,), (1,)), ((), ())), preferred_element_type=F32)
        kr, ki = kf[0:TB], kf[TB:]
        if half == 0:
            kr = kr + jnp.where(jl == 0, dvec, 0.0)
        kf_s[jl, 0] = kr
        kf_s[jl, 1] = ki - kr
        kf_s[jl, 2] = kr + ki
        r0 = pl.multiple_of(j * TB, TB)
        q0 = pl.multiple_of(j * hb, hb) + 8
        es, os_ = [], []
        for g in range(NLB):
            lb = slice(g * 128, (g + 1) * 128)
            ke, ko = _halves(k_s[pl.ds(r0, TB), lb])
            ve, vo = _halves(v_s[pl.ds(r0, TB), lb])
            kpad[0, g, pl.ds(q0, hb), :] = ke
            kpad[1, g, pl.ds(q0, hb), :] = ko
            ke1 = kpad[0, g, pl.ds(q0 - 1, hb), :]
            ko1 = kpad[1, g, pl.ds(q0 - 1, hb), :]
            ko2 = kpad[1, g, pl.ds(q0 - 2, hb), :]
            t0, t1, t2, t3 = (taps[t][g] for t in range(KS))
            es.append(((ke * t0 + ko1 * t1 + ke1 * t2 + ko2 * t3) * ve))
            os_.append(((ko * t0 + ke * t1 + ko1 * t2 + ke1 * t3) * vo))
        e = jnp.concatenate(es, axis=1)
        o = jnp.concatenate(os_, axis=1)
        fe = jnp.dot(fu_s[0], jnp.concatenate([e, e], axis=0).astype(BF16), preferred_element_type=F32)
        fo = jnp.dot(fu_s[1], jnp.concatenate([o, o], axis=0).astype(BF16), preferred_element_type=F32)
        u_s[jl, 0, 0:hb] = fe[:hb] + fo[:hb]
        u_s[jl, 0, hb:TB] = fe[:hb] - fo[:hb]
        u_s[jl, 1, 0:hb] = fe[hb:] + fo[hb:]
        u_s[jl, 1, hb:TB] = fo[hb:] - fe[hb:]

    def mac_stage(jj, second):
        for rg in range(2):
            rs = pl.ds(pl.multiple_of((2 * jj + rg) * 8, 8), 8)
            for g in range(NLB):
                lb = slice(g * 128, (g + 1) * 128)

                def uu(i, p):
                    u_s = u_a if i < HB else u_b
                    if p == 0:
                        return u_s[i % HB, 0, rs, lb] + u_s[i % HB, 1, rs, lb]
                    return u_s[i % HB, p - 1, rs, lb]

                def kk(i, p):
                    return (kf_a if i < HB else kf_b)[i % HB, p, rs, lb]

                def poly(p, acc):
                    acc = dict(acc)
                    for a0, b0 in (((0, HB), (HB, 0)) if second else ((0, 0),)):
                        ua = [uu(a0 + a, p) for a in range(HB)]
                        kb = [kk(b0 + b, p) for b in range(HB)]
                        for i in range(min(2 * HB - 1, NB - a0 - b0)):
                            for a in range(max(0, i - HB + 1), min(i, HB - 1) + 1):
                                t = ua[a] * kb[i - a]
                                io = i + a0 + b0
                                if io not in acc:
                                    acc[io] = t
                                elif p == 2:
                                    acc[io] = acc[io] - t
                                else:
                                    acc[io] = acc[io] + t
                    return acc

                s1 = poly(0, {})
                for p, comp in ((1, 1), (2, 0)):
                    init = s1
                    if second:
                        init = {i: (v + c_p[i - HB, comp, rs, lb] if i < NB - 1 else v)
                                for i, v in s1.items()}
                    for i, v in poly(p, init).items():
                        if i < HB:
                            c_a[i + 1, comp, rs, lb] = v
                        elif second:
                            c_b[i - HB + 1, comp, rs, lb] = v
                        else:
                            c_p[i - HB, comp, rs, lb] = v
                        if i == HB - 1:
                            c_b[0, comp, rs, lb] = v

    def inv_stage(il, half):
        i = il + half * HB
        c_s = (c_a, c_b)[half]
        q = TB // 4
        re, im = [], []
        for b in range(4):
            rows = slice(b * q, (b + 1) * q)
            cr, ci_ = c_s[il + 1, 0, rows], c_s[il + 1, 1, rows]
            pr, pi = c_s[il, 0, rows], c_s[il, 1, rows]
            re.append(cr + pi if b in (0, 3) else cr - pi)
            im.append(ci_ - pr if b in (0, 3) else ci_ + pr)
        pe = jnp.concatenate([re[0] + re[2], re[1] + re[3], im[0] - im[2], im[1] - im[3]], axis=0)
        po = jnp.concatenate([re[0] - re[2], re[1] - re[3], im[0] + im[2], im[1] + im[3]], axis=0)
        for par, pp in enumerate((pe, po)):
            ph, plo = _split(pp)
            y = jnp.dot(inv_s[par], jnp.concatenate([ph, ph, plo], axis=0).astype(BF16),
                        preferred_element_type=F32)
            for g in range(NLB):
                y_s[g, pl.ds(i * TB + par, hb, stride=2), :] = y[:, g * 128:(g + 1) * 128]

    def relayout(t):
        w_copies[t].wait()

        def body(i, _):
            for dd in range(32):
                dp = i * 32 + dd
                a = pltpu.bitcast(wraw[t, 2 * dp], U32)
                b = pltpu.bitcast(wraw[t, 2 * dp + 1], U32)
                lo = (a & jnp.uint32(0xFFFF)) | (b << 16)
                hi = (a >> 16) | (b & jnp.uint32(0xFFFF0000))
                wt[pl.ds(t * H * WP + dp, 16, stride=WP), :] = lo
                wt[pl.ds((t * H + 16) * WP + dp, 16, stride=WP), :] = hi
            return 0
        lax.fori_loop(0, D // 64, body, 0)

    def wslab(t, h):
        s0 = (t * H + (h % 2) * 16 + h // 2) * WP
        return pltpu.bitcast(wt[s0:s0 + D // 2, :], BF16)

    def loop(n, fn):
        def body(j, _):
            fn(j)
            return 0
        lax.fori_loop(0, n, body, 0)

    with jax.named_scope("conv_a"):
        loop(HB, lambda j: fwd_stage(j, 0))
    with jax.named_scope("conv_b"):
        for c in w_copies:
            c.start()
        loop(HB, lambda j: mac_stage(j, False))
        for c in late_copies:
            c.wait()
        loop(HB // 2, lambda j: (fwd_stage(2 * j, 1), fwd_stage(2 * j + 1, 1)))
    with jax.named_scope("rel0"):
        relayout(0)
    with jax.named_scope("conv_c"):
        loop(HB, lambda j: (inv_stage(j, 0), mac_stage(j, True)))
    with jax.named_scope("rel1"):
        relayout(1)
    with jax.named_scope("conv_d"):
        loop(HB // 2, lambda j: (inv_stage(2 * j, 1), inv_stage(2 * j + 1, 1)))
    with jax.named_scope("rel2"):
        relayout(2)
    with jax.named_scope("waitx"):
        xa_copy.wait()

    scale = DH ** -0.5

    def masks(mode):
        rows = ROWS if mode == 0 else ROWS - SEG
        qi = lax.broadcasted_iota(jnp.int32, (rows, rows), 0)
        kj = lax.broadcasted_iota(jnp.int32, (rows, rows), 1)

        def layer_of(i):
            xl = (i - 2 * M) // SEG if mode == 0 else mode - 1
            return jnp.where(i < 2 * M, i // M, xl)
        same = layer_of(qi) == layer_of(kj)
        vis = same & ((qi < 2 * M) | (qi >= kj))
        fill = jnp.where(same, -1e9, -jnp.inf).astype(F32)
        return vis, fill

    mem0 = mem0_ref[...].astype(F32)
    hbuf[0:16, :] = jnp.concatenate([mem0, mem0], axis=0).astype(BF16)
    hbuf[16:48, :] = _ln(x_s[0:SEG, :].astype(F32)).astype(BF16)
    obuf[...] = jnp.zeros((2 * SEG, D), F32)
    x2_s[...] = jnp.zeros(x2_s.shape, F32)

    def seg_row(seg):
        if isinstance(seg, int):
            return min(max(seg, 0), NSEG - 1) * SEG
        return pl.multiple_of(jnp.clip(seg, 0, NSEG - 1) * SEG, SEG)

    def gate(xa, r0):
        y = jnp.concatenate([y_s[g, pl.ds(r0, SEG), :] for g in range(NLB)], axis=1)
        return xa + _r(_r(_ln(xa)) * y)

    def attention(h, vis, fill, before_oproj=None):
        def proj(g):
            return [[jnp.dot(h, wslab(t, g * HG + j), preferred_element_type=F32).astype(BF16)
                     for j in range(HG)] for t in range(3)]

        def probs(qkv):
            scs = [lax.dot_general(qkv[0][j], qkv[1][j], (((1,), (1,)), ((), ())),
                                   preferred_element_type=F32) for j in range(HG)]
            ps = []
            for sc in scs:
                sc = jnp.where(vis, sc * scale, fill)
                e = jnp.exp(sc - jnp.max(sc, axis=-1, keepdims=True))
                den = jnp.sum(e, axis=-1, keepdims=True)
                r = pl.reciprocal(den, approx=True)
                r = r * (2.0 - den * r)
                ps.append((e * r).astype(BF16))
            return ps

        def oproj(os_, h0):
            oc = jnp.concatenate(os_, axis=1)
            k0, k1 = h0 * DH, (h0 + len(os_)) * DH
            return [jnp.dot(oc, wo_s[k0:k1, n * 128:(n + 1) * 128], preferred_element_type=F32)
                    for n in range(NLB)]

        heads = []
        qkv = proj(0)
        oa = None
        for g in range(NG):
            ps = probs(qkv)
            vs = qkv[2]
            if g + 1 < NG:
                qkv = proj(g + 1)
            else:
                if before_oproj is not None:
                    before_oproj()
                oa = oproj(heads[:H // 2], 0)
            heads += [jnp.dot(ps[j], vs[j], preferred_element_type=F32).astype(BF16)
                      for j in range(HG)]
        ob = oproj(heads[H // 2:], H // 2)
        return jnp.concatenate([b + a for a, b in zip(oa, ob)], axis=1)

    def post2(s):
        r3 = seg_row(s - 1 - LAG)
        xo = gate(_r(x2_s[(s + 4 - 1 - LAG) % 4] + obuf[SEG:2 * SEG, :]), r3)
        out_s[pl.ds(r3, SEG), :] = xo.astype(BF16)

    def step(s, mode, vis, fill, before_oproj=None):
        if mode == 0:
            h = hbuf[...]
        elif mode == 1:
            h = hbuf[0:48, :]
        else:
            h = jnp.concatenate([hbuf[0:16, :], hbuf[48:80, :]], axis=0)
        r1 = seg_row(s - 1)
        xb2 = _r(gate(_r(x_s[pl.ds(r1, SEG), :].astype(F32) + obuf[0:SEG, :]), r1))
        h2n = _ln(xb2).astype(BF16)
        if mode != 1:
            post2(s)
        x2_s[(s + 4 - 1) % 4] = xb2
        if mode != 2:
            h1n = _ln(x_s[pl.ds(seg_row(s + 1), SEG), :].astype(F32)).astype(BF16)

        o = attention(h, vis, fill, before_oproj)

        mem2 = mem0 if mode == 1 else o[M:2 * M]
        hbuf[0:16, :] = jnp.concatenate([o[0:M], mem2], axis=0).astype(BF16)
        if mode != 2:
            hbuf[16:48, :] = h1n
        hbuf[48:80, :] = h2n
        if mode == 0:
            obuf[...] = _r(o[2 * M:])
        elif mode == 1:
            obuf[0:SEG, :] = _r(o[2 * M:])
        else:
            obuf[SEG:2 * SEG, :] = _r(o[2 * M:])

    with jax.named_scope("pro"):
        vis, fill = masks(1)
        step(0, 1, vis, fill, wo_copy.wait)
        step(1, 1, vis, fill)
    xb_copy.wait()
    with jax.named_scope("main"):
        vis, fill = masks(0)
        loop(NSEG - LAG, lambda s: step(s + LAG, 0, vis, fill))
    done = (NSEG - 1 - LAG) * SEG
    out_a = pltpu.make_async_copy(out_s.at[0:done, :], out_hbm.at[0:done, :], sem_x.at[1])
    out_a.start()
    with jax.named_scope("epi"):
        vis, fill = masks(2)
        loop(LAG, lambda s: step(s + NSEG, 2, vis, fill))
    post2(NSEG + LAG)
    out_b = pltpu.make_async_copy(out_s.at[done:S, :], out_hbm.at[done:S, :], sem_x.at[2])
    out_b.start()
    out_a.wait()
    out_b.wait()


@functools.partial(jax.jit, static_argnames=("A_seg_len",))
def pallas_interleave_layers__memory_aug_recurrent_mem_tr__ssm_conv_h3__prompt_kernel(
    A_x, A_mem0, A_Wq, A_Wk, A_Wv, A_Wo, A_seg_len,
    B_q, B_k, B_v, B_shift_k, B_ssm_k, B_ssm_D,
):
    assert A_seg_len == SEG and A_x.shape == (1, S, D)
    vm = pl.BlockSpec(memory_space=pltpu.VMEM)
    hbm = pl.BlockSpec(memory_space=pl.ANY)
    out = pl.pallas_call(
        _kernel,
        out_shape=jax.ShapeDtypeStruct((S, D), BF16),
        in_specs=[hbm, vm, hbm, hbm, hbm, hbm, hbm, hbm, vm, hbm, vm],
        out_specs=hbm,
        scratch_shapes=[
            pltpu.VMEM((S, D), BF16),
            pltpu.VMEM((S, D), BF16),
            pltpu.VMEM((S, D), BF16),
            pltpu.VMEM((NB, D, TB), BF16),
            pltpu.VMEM((3, D, H, DH), BF16),
            pltpu.VMEM((3 * H * WP, 128), U32),
            pltpu.VMEM((H * DH, D), BF16),
            pltpu.VMEM((2 * TB, 2 * TB), BF16),
            pltpu.VMEM((2, TB, TB), BF16),
            pltpu.VMEM((2, TB // 2, 3 * TB), BF16),
            pltpu.VMEM((2, NLB, S // 2 + 8, 128), F32),
            pltpu.VMEM((NB // 2, 2, TB, D), F32),
            pltpu.VMEM((NB // 2, 2, TB, D), F32),
            pltpu.VMEM((NB // 2, 3, TB, D), F32),
            pltpu.VMEM((NB // 2, 3, TB, D), F32),
            pltpu.VMEM((NB // 2 + 1, 2, TB, D), F32),
            pltpu.VMEM((NB // 2 + 1, 2, TB, D), F32),
            pltpu.VMEM((NB // 2 - 1, 2, TB, D), F32),
            pltpu.VMEM((NLB, S, 128), F32),
            pltpu.VMEM((ROWS, D), BF16),
            pltpu.VMEM((2 * SEG, D), F32),
            pltpu.VMEM((4, SEG, D), F32),
            pltpu.VMEM((S, D), BF16),
            pltpu.SemaphoreType.DMA((3 * (NB // 2) + 1,)),
            pltpu.SemaphoreType.DMA((4,)),
            pltpu.SemaphoreType.DMA((4,)),
        ],
        compiler_params=pltpu.CompilerParams(vmem_limit_bytes=120 * 1024 * 1024),
    )(A_x.reshape(S, D), A_mem0.reshape(M, D), A_Wq, A_Wk, A_Wv,
      A_Wo.reshape(H * DH, D), B_k.reshape(S, D), B_v.reshape(S, D),
      B_shift_k.T, B_ssm_k, B_ssm_D)
    return out.reshape(1, S, D)
```

```python
import functools
import math

import jax
import jax.numpy as jnp
from jax import lax
import jax.experimental.pallas as pl
import jax.experimental.pallas.tpu as pltpu

F32 = jnp.float32
BF16 = jnp.bfloat16
U32 = jnp.uint32

S = 2048
D = 640
H = 32
DH = 128
M = 8
SEG = 32
NSEG = S // SEG
KS = 4
LAG = 2
ROWS = 2 * M + 2 * SEG
HG = 4
NG = H // HG
NLB = D // 128
TB = 128
NB = S // TB
UNR = 1
WP = 324


def _ln(x):
    m = jnp.mean(x, axis=-1, keepdims=True)
    c = x - m
    v = jnp.mean(c * c, axis=-1, keepdims=True)
    return c * lax.rsqrt(v + 1e-5)


def _r(x):
    return x.astype(BF16).astype(F32)


def _split(x):
    hi = pltpu.bitcast(pltpu.bitcast(x, U32) & jnp.uint32(0xFFFF0000), F32)
    return hi, x - hi


def _bf(x):
    return jnp.concatenate([x[:, g:g + 128].astype(BF16)
                            for g in range(0, x.shape[1], 128)], axis=1)


def _basis(r, t):
    b = r & 63
    f = jnp.where(b < 32, 2 * b, 2 * b - 63)
    n = ((2 * f + 1) * t - jnp.where(r >= 64, TB, 0)) & (4 * TB - 1)
    n = jnp.where(n >= 2 * TB, n - 4 * TB, n)
    return jnp.cos(n.astype(F32) * (2.0 * math.pi / (4 * TB)))


def _halves(x):
    w = pltpu.bitcast(x, U32)
    return (pltpu.bitcast(w << 16, F32),
            pltpu.bitcast(w & jnp.uint32(0xFFFF0000), F32))


def _kernel(x_hbm, mem0_ref, wq_hbm, wk_hbm, wv_hbm, wo_hbm,
            k_hbm, v_hbm, shk_ref, ssmk_hbm, ssmd_ref,
            out_hbm,
            x_s, k_s, v_s, ssmk_s, wraw, wt, wo_s,
            fk_s, fu_s, inv_s, kpad, u_a, u_b, kf_a, kf_b, c_a, c_b, c_p, y_s,
            hbuf, obuf, x2_s, out_s,
            sem_c, sem_w, sem_x):
    HB = NB // 2
    XH = 4 * SEG

    def conv_copies(j):
        r0 = j * TB if isinstance(j, int) else pl.multiple_of(j * TB, TB)
        return (
            pltpu.make_async_copy(ssmk_hbm.at[:, pl.ds(r0, TB)], ssmk_s.at[j], sem_c.at[j]),
            pltpu.make_async_copy(k_hbm.at[pl.ds(r0, TB), :], k_s.at[pl.ds(r0, TB), :], sem_c.at[HB + j]),
            pltpu.make_async_copy(v_hbm.at[pl.ds(r0, TB), :], v_s.at[pl.ds(r0, TB), :], sem_c.at[NB + j]),
        )
    late_copies = [pltpu.make_async_copy(ssmk_hbm.at[:, pl.ds(j * TB, TB)], ssmk_s.at[j], sem_c.at[3 * HB])
                   for j in range(HB, NB)]
    late_copies += [pltpu.make_async_copy(src.at[S // 2:, :], dst.at[S // 2:, :], sem_c.at[3 * HB])
                    for src, dst in ((k_hbm, k_s), (v_hbm, v_s))]
    w_copies = [pltpu.make_async_copy(w, wraw.at[t], sem_w.at[t])
                for t, w in enumerate((wq_hbm, wk_hbm, wv_hbm))]
    wo_copy = pltpu.make_async_copy(wo_hbm, wo_s, sem_w.at[3])
    xa_copy = pltpu.make_async_copy(x_hbm.at[0:XH, :], x_s.at[0:XH, :], sem_x.at[0])
    xb_copy = pltpu.make_async_copy(x_hbm.at[XH:, :], x_s.at[XH:, :], sem_x.at[3])
    for j in range(HB):
        for c in conv_copies(j):
            c.start()
    for c in late_copies:
        c.start()
    xa_copy.start()
    wo_copy.start(priority=1)
    xb_copy.start(priority=1)

    hb = TB // 2
    ri = lax.broadcasted_iota(jnp.int32, (TB, TB), 0)
    ci = lax.broadcasted_iota(jnp.int32, (TB, TB), 1)
    full = _basis(ri, ci)
    alt = jnp.where((ci & 1) == 0, full, -full)
    fk = jnp.concatenate([full[:hb], alt[:hb], full[hb:], -alt[hb:]], axis=0)
    fk_s[...] = _bf(jnp.concatenate(_split(fk), axis=1))
    tab = _basis(ri, 2 * (ci & 63) + (ci >> 6))
    hi, lo = _split(tab)
    fu_s[0] = jnp.where(ci < hb, hi, pltpu.roll(lo, hb, 1)).astype(BF16)
    fu_s[1] = jnp.where(ci < hb, pltpu.roll(hi, hb, 1), lo).astype(BF16)
    gh, gl = _split(tab.T * (1.0 / TB))
    ginv = _bf(jnp.concatenate([gh, gl, gh], axis=1))
    inv_s[0] = ginv[:hb]
    inv_s[1] = ginv[hb:]

    shk_t = shk_ref[...].astype(F32)
    taps = [[shk_t[j:j + 1, g * 128:(g + 1) * 128] for g in range(NLB)] for j in range(KS)]
    dvec = ssmd_ref[...].astype(F32).reshape(1, D)
    for g in range(NLB):
        kpad[0, g, 0:8, :] = jnp.zeros((8, 128), F32)
        kpad[1, g, 0:8, :] = jnp.zeros((8, 128), F32)
    c_a[0] = jnp.zeros(c_a.shape[1:], F32)

    def fwd_stage(jl, half):
        j = jl + half * HB
        u_s, kf_s = ((u_a, kf_a), (u_b, kf_b))[half]
        if half == 0:
            for c in conv_copies(j):
                c.wait()
        kb = ssmk_s[j]
        kf = lax.dot_general(fk_s[...], jnp.concatenate([kb, kb], axis=1),
                             (((1,), (1,)), ((), ())), preferred_element_type=F32)
        kr, ki = kf[0:TB], kf[TB:]
        if half == 0:
            kr = kr + jnp.where(jl == 0, dvec, 0.0)
        kf_s[jl, 0] = kr
        kf_s[jl, 1] = ki - kr
        kf_s[jl, 2] = kr + ki
        r0 = pl.multiple_of(j * TB, TB)
        q0 = pl.multiple_of(j * hb, hb) + 8
        es, os_ = [], []
        for g in range(NLB):
            lb = slice(g * 128, (g + 1) * 128)
            ke, ko = _halves(k_s[pl.ds(r0, TB), lb])
            ve, vo = _halves(v_s[pl.ds(r0, TB), lb])
            kpad[0, g, pl.ds(q0, hb), :] = ke
            kpad[1, g, pl.ds(q0, hb), :] = ko
            ke1 = kpad[0, g, pl.ds(q0 - 1, hb), :]
            ko1 = kpad[1, g, pl.ds(q0 - 1, hb), :]
            ko2 = kpad[1, g, pl.ds(q0 - 2, hb), :]
            t0, t1, t2, t3 = (taps[t][g] for t in range(KS))
            es.append(((ke * t0 + ko1 * t1 + ke1 * t2 + ko2 * t3) * ve))
            os_.append(((ko * t0 + ke * t1 + ko1 * t2 + ke1 * t3) * vo))
        e = jnp.concatenate(es, axis=1)
        o = jnp.concatenate(os_, axis=1)
        fe = jnp.dot(fu_s[0], jnp.concatenate([e, e], axis=0).astype(BF16), preferred_element_type=F32)
        fo = jnp.dot(fu_s[1], jnp.concatenate([o, o], axis=0).astype(BF16), preferred_element_type=F32)
        u_s[jl, 0, 0:hb] = fe[:hb] + fo[:hb]
        u_s[jl, 0, hb:TB] = fe[:hb] - fo[:hb]
        u_s[jl, 1, 0:hb] = fe[hb:] + fo[hb:]
        u_s[jl, 1, hb:TB] = fo[hb:] - fe[hb:]

    def mac_stage(jj, second):
        for rg in range(2):
            rs = pl.ds(pl.multiple_of((2 * jj + rg) * 8, 8), 8)
            for g in range(NLB):
                lb = slice(g * 128, (g + 1) * 128)

                def uu(i, p):
                    u_s = u_a if i < HB else u_b
                    if p == 0:
                        return u_s[i % HB, 0, rs, lb] + u_s[i % HB, 1, rs, lb]
                    return u_s[i % HB, p - 1, rs, lb]

                def kk(i, p):
                    return (kf_a if i < HB else kf_b)[i % HB, p, rs, lb]

                def poly(p, acc):
                    acc = dict(acc)
                    for a0, b0 in (((0, HB), (HB, 0)) if second else ((0, 0),)):
                        ua = [uu(a0 + a, p) for a in range(HB)]
                        kb = [kk(b0 + b, p) for b in range(HB)]
                        for i in range(min(2 * HB - 1, NB - a0 - b0)):
                            for a in range(max(0, i - HB + 1), min(i, HB - 1) + 1):
                                t = ua[a] * kb[i - a]
                                io = i + a0 + b0
                                if io not in acc:
                                    acc[io] = t
                                elif p == 2:
                                    acc[io] = acc[io] - t
                                else:
                                    acc[io] = acc[io] + t
                    return acc

                s1 = poly(0, {})
                for p, comp in ((1, 1), (2, 0)):
                    init = s1
                    if second:
                        init = {i: (v + c_p[i - HB, comp, rs, lb] if i < NB - 1 else v)
                                for i, v in s1.items()}
                    for i, v in poly(p, init).items():
                        if i < HB:
                            c_a[i + 1, comp, rs, lb] = v
                        elif second:
                            c_b[i - HB + 1, comp, rs, lb] = v
                        else:
                            c_p[i - HB, comp, rs, lb] = v
                        if i == HB - 1:
                            c_b[0, comp, rs, lb] = v

    def inv_stage(il, half):
        i = il + half * HB
        c_s = (c_a, c_b)[half]
        q = TB // 4
        re, im = [], []
        for b in range(4):
            rows = slice(b * q, (b + 1) * q)
            cr, ci_ = c_s[il + 1, 0, rows], c_s[il + 1, 1, rows]
            pr, pi = c_s[il, 0, rows], c_s[il, 1, rows]
            re.append(cr + pi if b in (0, 3) else cr - pi)
            im.append(ci_ - pr if b in (0, 3) else ci_ + pr)
        pe = jnp.concatenate([re[0] + re[2], re[1] + re[3], im[0] - im[2], im[1] - im[3]], axis=0)
        po = jnp.concatenate([re[0] - re[2], re[1] - re[3], im[0] + im[2], im[1] + im[3]], axis=0)
        for par, pp in enumerate((pe, po)):
            ph, plo = _split(pp)
            y = jnp.dot(inv_s[par], jnp.concatenate([ph, ph, plo], axis=0).astype(BF16),
                        preferred_element_type=F32)
            for g in range(NLB):
                y_s[g, pl.ds(i * TB + par, hb, stride=2), :] = y[:, g * 128:(g + 1) * 128]

    def relayout(t):
        w_copies[t].wait()

        def body(i, _):
            for dd in range(32):
                dp = i * 32 + dd
                a = pltpu.bitcast(wraw[t, 2 * dp], U32)
                b = pltpu.bitcast(wraw[t, 2 * dp + 1], U32)
                lo = (a & jnp.uint32(0xFFFF)) | (b << 16)
                hi = (a >> 16) | (b & jnp.uint32(0xFFFF0000))
                wt[pl.ds(t * H * WP + dp, 16, stride=WP), :] = lo
                wt[pl.ds((t * H + 16) * WP + dp, 16, stride=WP), :] = hi
            return 0
        lax.fori_loop(0, D // 64, body, 0)

    def wslab(t, h):
        s0 = (t * H + (h % 2) * 16 + h // 2) * WP
        return pltpu.bitcast(wt[s0:s0 + D // 2, :], BF16)

    def loop(n, fn):
        def body(j, _):
            fn(j)
            return 0
        lax.fori_loop(0, n, body, 0)

    with jax.named_scope("conv_a"):
        loop(HB, lambda j: fwd_stage(j, 0))
    with jax.named_scope("conv_b"):
        for c in w_copies:
            c.start()
        loop(HB, lambda j: mac_stage(j, False))
        for c in late_copies:
            c.wait()
        loop(HB // 2, lambda j: (fwd_stage(2 * j, 1), fwd_stage(2 * j + 1, 1)))
    with jax.named_scope("rel0"):
        relayout(0)
    with jax.named_scope("conv_c"):
        loop(HB, lambda j: (inv_stage(j, 0), mac_stage(j, True)))
    with jax.named_scope("rel1"):
        relayout(1)
    with jax.named_scope("conv_d"):
        loop(HB // 2, lambda j: (inv_stage(2 * j, 1), inv_stage(2 * j + 1, 1)))
    with jax.named_scope("rel2"):
        relayout(2)
    with jax.named_scope("waitx"):
        xa_copy.wait()

    scale = DH ** -0.5

    def masks(mode):
        rows = ROWS if mode == 0 else ROWS - SEG
        qi = lax.broadcasted_iota(jnp.int32, (rows, rows), 0)
        kj = lax.broadcasted_iota(jnp.int32, (rows, rows), 1)

        def layer_of(i):
            xl = (i - 2 * M) // SEG if mode == 0 else mode - 1
            return jnp.where(i < 2 * M, i // M, xl)
        same = layer_of(qi) == layer_of(kj)
        vis = same & ((qi < 2 * M) | (qi >= kj))
        fill = jnp.where(same, -1e9, -jnp.inf).astype(F32)
        return vis, fill

    mem0 = mem0_ref[...].astype(F32)
    hbuf[0:16, :] = jnp.concatenate([mem0, mem0], axis=0).astype(BF16)
    hbuf[16:48, :] = _ln(x_s[0:SEG, :].astype(F32)).astype(BF16)
    obuf[...] = jnp.zeros((2 * SEG, D), F32)
    x2_s[...] = jnp.zeros(x2_s.shape, F32)

    def seg_row(seg):
        if isinstance(seg, int):
            return min(max(seg, 0), NSEG - 1) * SEG
        return pl.multiple_of(jnp.clip(seg, 0, NSEG - 1) * SEG, SEG)

    def gate(xa, r0):
        y = jnp.concatenate([y_s[g, pl.ds(r0, SEG), :] for g in range(NLB)], axis=1)
        return xa + _r(_r(_ln(xa)) * y)

    def attention(h, vis, fill, chained, before_oproj=None):
        def proj(g):
            if g == 0 and chained:
                kc = D - 128
                part = [jnp.dot(h[:, :kc], wslab(0, j)[:kc], preferred_element_type=F32)
                        for j in range(HG)]
                q = [(jnp.dot(h[:, kc:], wslab(0, j)[kc:], preferred_element_type=F32)
                      + part[j]).astype(BF16) for j in range(HG)]
                return [q] + [[jnp.dot(h, wslab(t, j), preferred_element_type=F32).astype(BF16)
                               for j in range(HG)] for t in range(1, 3)]
            return [[jnp.dot(h, wslab(t, g * HG + j), preferred_element_type=F32).astype(BF16)
                     for j in range(HG)] for t in range(3)]

        def probs(qkv):
            scs = [lax.dot_general(qkv[0][j], qkv[1][j], (((1,), (1,)), ((), ())),
                                   preferred_element_type=F32) for j in range(HG)]
            ps = []
            for sc in scs:
                sc = jnp.where(vis, sc * scale, fill)
                e = jnp.exp(sc - jnp.max(sc, axis=-1, keepdims=True))
                den = jnp.sum(e, axis=-1, keepdims=True)
                r = pl.reciprocal(den, approx=True)
                r = r * (2.0 - den * r)
                ps.append((e * r).astype(BF16))
            return ps

        def oproj(os_, h0):
            oc = jnp.concatenate(os_, axis=1)
            k0, k1 = h0 * DH, (h0 + len(os_)) * DH
            return [jnp.dot(oc, wo_s[k0:k1, n * 128:(n + 1) * 128], preferred_element_type=F32)
                    for n in range(NLB)]

        heads = []
        qkv = proj(0)
        oa = None
        for g in range(NG):
            ps = probs(qkv)
            vs = qkv[2]
            if g + 1 < NG:
                qkv = proj(g + 1)
            else:
                if before_oproj is not None:
                    before_oproj()
                oa = oproj(heads[:H // 2], 0)
            heads += [jnp.dot(ps[j], vs[j], preferred_element_type=F32).astype(BF16)
                      for j in range(HG)]
        ob = oproj(heads[H // 2:], H // 2)
        return jnp.concatenate([b + a for a, b in zip(oa, ob)], axis=1)

    def post2(s):
        r3 = seg_row(s - 1 - LAG)
        xo = gate(_r(x2_s[(s + 4 - 1 - LAG) % 4] + obuf[SEG:2 * SEG, :]), r3)
        out_s[pl.ds(r3, SEG), :] = xo.astype(BF16)

    def step(s, mode, vis, fill, chained=False, before_oproj=None):
        if mode == 0:
            h = hbuf[...]
        elif mode == 1:
            h = hbuf[0:48, :]
        else:
            h = jnp.concatenate([hbuf[0:16, :], hbuf[48:80, :]], axis=0)
        r1 = seg_row(s - 1)
        xb2 = _r(gate(_r(x_s[pl.ds(r1, SEG), :].astype(F32) + obuf[0:SEG, :]), r1))
        h2n = _ln(xb2).astype(BF16)
        if mode != 1:
            post2(s)
        x2_s[(s + 4 - 1) % 4] = xb2
        if mode != 2:
            h1n = _ln(x_s[pl.ds(seg_row(s + 1), SEG), :].astype(F32)).astype(BF16)

        o = attention(h, vis, fill, chained, before_oproj)

        mem2 = mem0 if mode == 1 else o[M:2 * M]
        hbuf[0:16, :] = jnp.concatenate([o[0:M], mem2], axis=0).astype(BF16)
        if mode != 2:
            hbuf[16:48, :] = h1n
        hbuf[48:80, :] = h2n
        if mode == 0:
            obuf[...] = _r(o[2 * M:])
        elif mode == 1:
            obuf[0:SEG, :] = _r(o[2 * M:])
        else:
            obuf[SEG:2 * SEG, :] = _r(o[2 * M:])

    with jax.named_scope("pro"):
        vis, fill = masks(1)
        step(0, 1, vis, fill, False, wo_copy.wait)
        step(1, 1, vis, fill, True)
    xb_copy.wait()
    with jax.named_scope("main"):
        vis, fill = masks(0)
        loop((NSEG - LAG) // UNR, lambda i: [step(UNR * i + u + LAG, 0, vis, fill, u > 0)
                                             for u in range(UNR)])
    done = (NSEG - 1 - LAG) * SEG
    out_a = pltpu.make_async_copy(out_s.at[0:done, :], out_hbm.at[0:done, :], sem_x.at[1])
    out_a.start()
    with jax.named_scope("epi"):
        vis, fill = masks(2)
        step(NSEG, 2, vis, fill)
        step(NSEG + 1, 2, vis, fill, True)
    post2(NSEG + LAG)
    out_b = pltpu.make_async_copy(out_s.at[done:S, :], out_hbm.at[done:S, :], sem_x.at[2])
    out_b.start()
    out_a.wait()
    out_b.wait()


@functools.partial(jax.jit, static_argnames=("A_seg_len",))
def pallas_interleave_layers__memory_aug_recurrent_mem_tr__ssm_conv_h3__prompt_kernel(
    A_x, A_mem0, A_Wq, A_Wk, A_Wv, A_Wo, A_seg_len,
    B_q, B_k, B_v, B_shift_k, B_ssm_k, B_ssm_D,
):
    assert A_seg_len == SEG and A_x.shape == (1, S, D)
    vm = pl.BlockSpec(memory_space=pltpu.VMEM)
    hbm = pl.BlockSpec(memory_space=pl.ANY)
    out = pl.pallas_call(
        _kernel,
        out_shape=jax.ShapeDtypeStruct((S, D), BF16),
        in_specs=[hbm, vm, hbm, hbm, hbm, hbm, hbm, hbm, vm, hbm, vm],
        out_specs=hbm,
        scratch_shapes=[
            pltpu.VMEM((S, D), BF16),
            pltpu.VMEM((S, D), BF16),
            pltpu.VMEM((S, D), BF16),
            pltpu.VMEM((NB, D, TB), BF16),
            pltpu.VMEM((3, D, H, DH), BF16),
            pltpu.VMEM((3 * H * WP, 128), U32),
            pltpu.VMEM((H * DH, D), BF16),
            pltpu.VMEM((2 * TB, 2 * TB), BF16),
            pltpu.VMEM((2, TB, TB), BF16),
            pltpu.VMEM((2, TB // 2, 3 * TB), BF16),
            pltpu.VMEM((2, NLB, S // 2 + 8, 128), F32),
            pltpu.VMEM((NB // 2, 2, TB, D), F32),
            pltpu.VMEM((NB // 2, 2, TB, D), F32),
            pltpu.VMEM((NB // 2, 3, TB, D), F32),
            pltpu.VMEM((NB // 2, 3, TB, D), F32),
            pltpu.VMEM((NB // 2 + 1, 2, TB, D), F32),
            pltpu.VMEM((NB // 2 + 1, 2, TB, D), F32),
            pltpu.VMEM((NB // 2 - 1, 2, TB, D), F32),
            pltpu.VMEM((NLB, S, 128), F32),
            pltpu.VMEM((ROWS, D), BF16),
            pltpu.VMEM((2 * SEG, D), F32),
            pltpu.VMEM((4, SEG, D), F32),
            pltpu.VMEM((S, D), BF16),
            pltpu.SemaphoreType.DMA((3 * (NB // 2) + 1,)),
            pltpu.SemaphoreType.DMA((4,)),
            pltpu.SemaphoreType.DMA((4,)),
        ],
        compiler_params=pltpu.CompilerParams(vmem_limit_bytes=120 * 1024 * 1024),
    )(A_x.reshape(S, D), A_mem0.reshape(M, D), A_Wq, A_Wk, A_Wv,
      A_Wo.reshape(H * DH, D), B_k.reshape(S, D), B_v.reshape(S, D),
      B_shift_k.T, B_ssm_k, B_ssm_D)
    return out.reshape(1, S, D)
```

```python
import math

import jax
import jax.numpy as jnp
from jax import lax
import jax.experimental.pallas as pl
import jax.experimental.pallas.tpu as pltpu

F32 = jnp.float32
BF16 = jnp.bfloat16
U32 = jnp.uint32

S = 2048
D = 640
H = 32
DH = 128
M = 8
SEG = 32
NSEG = S // SEG
KS = 4
LAG = 2
ROWS = 2 * M + 2 * SEG
HG = 4
NG = H // HG
NLB = D // 128
TB = 128
NB = S // TB
UNR = 1
WP = 324


def _ln(x):
    m = jnp.mean(x, axis=-1, keepdims=True)
    c = x - m
    v = jnp.mean(c * c, axis=-1, keepdims=True)
    return c * lax.rsqrt(v + 1e-5)


def _r(x):
    return x.astype(BF16).astype(F32)


def _split(x):
    hi = pltpu.bitcast(pltpu.bitcast(x, U32) & jnp.uint32(0xFFFF0000), F32)
    return hi, x - hi


def _bf(x):
    return jnp.concatenate([x[:, g:g + 128].astype(BF16)
                            for g in range(0, x.shape[1], 128)], axis=1)


def _basis(r, t):
    b = r & 63
    f = jnp.where(b < 32, 2 * b, 2 * b - 63)
    n = ((2 * f + 1) * t - jnp.where(r >= 64, TB, 0)) & (4 * TB - 1)
    n = jnp.where(n >= 2 * TB, n - 4 * TB, n)
    return jnp.cos(n.astype(F32) * (2.0 * math.pi / (4 * TB)))


def _halves(x):
    w = pltpu.bitcast(x, U32)
    return (pltpu.bitcast(w << 16, F32),
            pltpu.bitcast(w & jnp.uint32(0xFFFF0000), F32))


def _kernel(x_hbm, mem0_ref, wq_hbm, wk_hbm, wv_hbm, wo_hbm,
            k_hbm, v_hbm, shk_ref, ssmk_hbm, ssmd_ref,
            out_hbm,
            x_s, k_s, v_s, ssmk_s, wraw, wt, wo_s,
            fk_s, fu_s, inv_s, kpad, u_a, u_b, kf_a, kf_b, c_a, c_b, c_p, y_s,
            hbuf, obuf, x2_s, out_s,
            sem_c, sem_w, sem_x):
    HB = NB // 2
    XH = 4 * SEG

    def conv_copies(j):
        r0 = j * TB if isinstance(j, int) else pl.multiple_of(j * TB, TB)
        return (
            pltpu.make_async_copy(ssmk_hbm.at[:, pl.ds(r0, TB)], ssmk_s.at[j], sem_c.at[j]),
            pltpu.make_async_copy(k_hbm.at[pl.ds(r0, TB), :], k_s.at[pl.ds(r0, TB), :], sem_c.at[HB + j]),
            pltpu.make_async_copy(v_hbm.at[pl.ds(r0, TB), :], v_s.at[pl.ds(r0, TB), :], sem_c.at[NB + j]),
        )
    late_copies = [pltpu.make_async_copy(ssmk_hbm.at[:, pl.ds(j * TB, TB)], ssmk_s.at[j], sem_c.at[3 * HB])
                   for j in range(HB, NB)]
    late_copies += [pltpu.make_async_copy(src.at[S // 2:, :], dst.at[S // 2:, :], sem_c.at[3 * HB])
                    for src, dst in ((k_hbm, k_s), (v_hbm, v_s))]
    w_copies = [pltpu.make_async_copy(w, wraw.at[t], sem_w.at[t])
                for t, w in enumerate((wq_hbm, wk_hbm, wv_hbm))]
    wo_copy = pltpu.make_async_copy(wo_hbm, wo_s, sem_w.at[3])
    xa_copy = pltpu.make_async_copy(x_hbm.at[0:XH, :], x_s.at[0:XH, :], sem_x.at[0])
    xb_copy = pltpu.make_async_copy(x_hbm.at[XH:, :], x_s.at[XH:, :], sem_x.at[3])
    for j in range(HB):
        for c in conv_copies(j):
            c.start()
    for c in late_copies:
        c.start()
    xa_copy.start()
    wo_copy.start(priority=1)
    xb_copy.start(priority=1)

    hb = TB // 2
    ri = lax.broadcasted_iota(jnp.int32, (TB, TB), 0)
    ci = lax.broadcasted_iota(jnp.int32, (TB, TB), 1)
    full = _basis(ri, ci)
    alt = jnp.where((ci & 1) == 0, full, -full)
    fk = jnp.concatenate([full[:hb], alt[:hb], full[hb:], -alt[hb:]], axis=0)
    fk_s[...] = _bf(jnp.concatenate(_split(fk), axis=1))
    tab = _basis(ri, 2 * (ci & 63) + (ci >> 6))
    hi, lo = _split(tab)
    fu_s[0] = jnp.where(ci < hb, hi, pltpu.roll(lo, hb, 1)).astype(BF16)
    fu_s[1] = jnp.where(ci < hb, pltpu.roll(hi, hb, 1), lo).astype(BF16)
    gh, gl = _split(tab.T * (1.0 / TB))
    ginv = _bf(jnp.concatenate([gh, gl, gh], axis=1))
    inv_s[0] = ginv[:hb]
    inv_s[1] = ginv[hb:]

    shk_t = shk_ref[...].astype(F32)
    taps = [[shk_t[j:j + 1, g * 128:(g + 1) * 128] for g in range(NLB)] for j in range(KS)]
    dvec = ssmd_ref[...].astype(F32).reshape(1, D)
    for g in range(NLB):
        kpad[0, g, 0:8, :] = jnp.zeros((8, 128), F32)
        kpad[1, g, 0:8, :] = jnp.zeros((8, 128), F32)
    c_a[0] = jnp.zeros(c_a.shape[1:], F32)

    def fwd_stage(jl, half):
        j = jl + half * HB
        u_s, kf_s = ((u_a, kf_a), (u_b, kf_b))[half]
        if half == 0:
            for c in conv_copies(j):
                c.wait()
        kb = ssmk_s[j]
        kf = lax.dot_general(fk_s[...], jnp.concatenate([kb, kb], axis=1),
                             (((1,), (1,)), ((), ())), preferred_element_type=F32)
        kr, ki = kf[0:TB], kf[TB:]
        if half == 0:
            kr = kr + jnp.where(jl == 0, dvec, 0.0)
        kf_s[jl, 0] = kr
        kf_s[jl, 1] = ki - kr
        kf_s[jl, 2] = kr + ki
        r0 = pl.multiple_of(j * TB, TB)
        q0 = pl.multiple_of(j * hb, hb) + 8
        es, os_ = [], []
        for g in range(NLB):
            lb = slice(g * 128, (g + 1) * 128)
            ke, ko = _halves(k_s[pl.ds(r0, TB), lb])
            ve, vo = _halves(v_s[pl.ds(r0, TB), lb])
            kpad[0, g, pl.ds(q0, hb), :] = ke
            kpad[1, g, pl.ds(q0, hb), :] = ko
            ke1 = kpad[0, g, pl.ds(q0 - 1, hb), :]
            ko1 = kpad[1, g, pl.ds(q0 - 1, hb), :]
            ko2 = kpad[1, g, pl.ds(q0 - 2, hb), :]
            t0, t1, t2, t3 = (taps[t][g] for t in range(KS))
            es.append(((ke * t0 + ko1 * t1 + ke1 * t2 + ko2 * t3) * ve))
            os_.append(((ko * t0 + ke * t1 + ko1 * t2 + ke1 * t3) * vo))
        e = jnp.concatenate(es, axis=1)
        o = jnp.concatenate(os_, axis=1)
        fe = jnp.dot(fu_s[0], jnp.concatenate([e, e], axis=0).astype(BF16), preferred_element_type=F32)
        fo = jnp.dot(fu_s[1], jnp.concatenate([o, o], axis=0).astype(BF16), preferred_element_type=F32)
        u_s[jl, 0, 0:hb] = fe[:hb] + fo[:hb]
        u_s[jl, 0, hb:TB] = fe[:hb] - fo[:hb]
        u_s[jl, 1, 0:hb] = fe[hb:] + fo[hb:]
        u_s[jl, 1, hb:TB] = fo[hb:] - fe[hb:]

    def mac_stage(jj, second):
        for rg in range(2):
            rs = pl.ds(pl.multiple_of((2 * jj + rg) * 8, 8), 8)
            for g in range(NLB):
                lb = slice(g * 128, (g + 1) * 128)

                def uu(i, p):
                    u_s = u_a if i < HB else u_b
                    if p == 0:
                        return u_s[i % HB, 0, rs, lb] + u_s[i % HB, 1, rs, lb]
                    return u_s[i % HB, p - 1, rs, lb]

                def kk(i, p):
                    return (kf_a if i < HB else kf_b)[i % HB, p, rs, lb]

                def poly(p, acc):
                    acc = dict(acc)
                    for a0, b0 in (((0, HB), (HB, 0)) if second else ((0, 0),)):
                        ua = [uu(a0 + a, p) for a in range(HB)]
                        kb = [kk(b0 + b, p) for b in range(HB)]
                        for i in range(min(2 * HB - 1, NB - a0 - b0)):
                            for a in range(max(0, i - HB + 1), min(i, HB - 1) + 1):
                                t = ua[a] * kb[i - a]
                                io = i + a0 + b0
                                if io not in acc:
                                    acc[io] = t
                                elif p == 2:
                                    acc[io] = acc[io] - t
                                else:
                                    acc[io] = acc[io] + t
                    return acc

                s1 = poly(0, {})
                for p, comp in ((1, 1), (2, 0)):
                    init = s1
                    if second:
                        init = {i: (v + c_p[i - HB, comp, rs, lb] if i < NB - 1 else v)
                                for i, v in s1.items()}
                    for i, v in poly(p, init).items():
                        if i < HB:
                            c_a[i + 1, comp, rs, lb] = v
                        elif second:
                            c_b[i - HB + 1, comp, rs, lb] = v
                        else:
                            c_p[i - HB, comp, rs, lb] = v
                        if i == HB - 1:
                            c_b[0, comp, rs, lb] = v

    def inv_stage(il, half):
        i = il + half * HB
        c_s = (c_a, c_b)[half]
        q = TB // 4
        re, im = [], []
        for b in range(4):
            rows = slice(b * q, (b + 1) * q)
            cr, ci_ = c_s[il + 1, 0, rows], c_s[il + 1, 1, rows]
            pr, pi = c_s[il, 0, rows], c_s[il, 1, rows]
            re.append(cr + pi if b in (0, 3) else cr - pi)
            im.append(ci_ - pr if b in (0, 3) else ci_ + pr)
        pe = jnp.concatenate([re[0] + re[2], re[1] + re[3], im[0] - im[2], im[1] - im[3]], axis=0)
        po = jnp.concatenate([re[0] - re[2], re[1] - re[3], im[0] + im[2], im[1] + im[3]], axis=0)
        for par, pp in enumerate((pe, po)):
            ph, plo = _split(pp)
            y = jnp.dot(inv_s[par], jnp.concatenate([ph, ph, plo], axis=0).astype(BF16),
                        preferred_element_type=F32)
            for g in range(NLB):
                y_s[g, pl.ds(i * TB + par, hb, stride=2), :] = y[:, g * 128:(g + 1) * 128]

    def relayout(t):
        w_copies[t].wait()

        def body(i, _):
            for dd in range(32):
                dp = i * 32 + dd
                a = pltpu.bitcast(wraw[t, 2 * dp], U32)
                b = pltpu.bitcast(wraw[t, 2 * dp + 1], U32)
                lo = (a & jnp.uint32(0xFFFF)) | (b << 16)
                hi = (a >> 16) | (b & jnp.uint32(0xFFFF0000))
                wt[pl.ds(t * H * WP + dp, 16, stride=WP), :] = lo
                wt[pl.ds((t * H + 16) * WP + dp, 16, stride=WP), :] = hi
            return 0
        lax.fori_loop(0, D // 64, body, 0)

    def wslab(t, h):
        s0 = (t * H + (h % 2) * 16 + h // 2) * WP
        return pltpu.bitcast(wt[s0:s0 + D // 2, :], BF16)

    def loop(n, fn):
        def body(j, _):
            fn(j)
            return 0
        lax.fori_loop(0, n, body, 0)

    with jax.named_scope("conv_a"):
        loop(HB, lambda j: fwd_stage(j, 0))
    with jax.named_scope("conv_b"):
        for c in w_copies:
            c.start()
        loop(HB, lambda j: mac_stage(j, False))
        for c in late_copies:
            c.wait()
        loop(HB // 2, lambda j: (fwd_stage(2 * j, 1), fwd_stage(2 * j + 1, 1)))
    with jax.named_scope("rel0"):
        relayout(0)
    with jax.named_scope("conv_c"):
        loop(HB, lambda j: (inv_stage(j, 0), mac_stage(j, True)))
    with jax.named_scope("rel1"):
        relayout(1)
    with jax.named_scope("conv_d"):
        loop(HB // 2, lambda j: (inv_stage(2 * j, 1), inv_stage(2 * j + 1, 1)))
    with jax.named_scope("rel2"):
        relayout(2)
    with jax.named_scope("waitx"):
        xa_copy.wait()

    scale = DH ** -0.5

    def masks(mode):
        rows = ROWS if mode == 0 else ROWS - SEG
        qi = lax.broadcasted_iota(jnp.int32, (rows, rows), 0)
        kj = lax.broadcasted_iota(jnp.int32, (rows, rows), 1)

        def layer_of(i):
            xl = (i - 2 * M) // SEG if mode == 0 else mode - 1
            return jnp.where(i < 2 * M, i // M, xl)
        same = layer_of(qi) == layer_of(kj)
        vis = same & ((qi < 2 * M) | (qi >= kj))
        fill = jnp.where(same, -1e9, -jnp.inf).astype(F32)
        return vis, fill

    mem0 = mem0_ref[...].astype(F32)
    hbuf[0:16, :] = jnp.concatenate([mem0, mem0], axis=0).astype(BF16)
    hbuf[16:48, :] = _ln(x_s[0:SEG, :].astype(F32)).astype(BF16)
    obuf[...] = jnp.zeros((2 * SEG, D), F32)
    x2_s[...] = jnp.zeros(x2_s.shape, F32)

    def seg_row(seg):
        if isinstance(seg, int):
            return min(max(seg, 0), NSEG - 1) * SEG
        return pl.multiple_of(jnp.clip(seg, 0, NSEG - 1) * SEG, SEG)

    def gate(xa, r0):
        y = jnp.concatenate([y_s[g, pl.ds(r0, SEG), :] for g in range(NLB)], axis=1)
        return xa + _r(_r(_ln(xa)) * y)

    def attention(h, vis, fill, chained, before_oproj=None):
        def proj(g):
            if g == 0 and chained:
                kc = D - 128
                part = [jnp.dot(h[:, :kc], wslab(0, j)[:kc], preferred_element_type=F32)
                        for j in range(HG)]
                q = [(jnp.dot(h[:, kc:], wslab(0, j)[kc:], preferred_element_type=F32)
                      + part[j]).astype(BF16) for j in range(HG)]
                return [q] + [[jnp.dot(h, wslab(t, j), preferred_element_type=F32).astype(BF16)
                               for j in range(HG)] for t in range(1, 3)]
            return [[jnp.dot(h, wslab(t, g * HG + j), preferred_element_type=F32).astype(BF16)
                     for j in range(HG)] for t in range(3)]

        def probs(qkv):
            scs = [lax.dot_general(qkv[0][j], qkv[1][j], (((1,), (1,)), ((), ())),
                                   preferred_element_type=F32) for j in range(HG)]
            ps = []
            for sc in scs:
                sc = jnp.where(vis, sc * scale, fill)
                e = jnp.exp(sc - jnp.max(sc, axis=-1, keepdims=True))
                den = jnp.sum(e, axis=-1, keepdims=True)
                r = pl.reciprocal(den, approx=True)
                r = r * (2.0 - den * r)
                ps.append((e * r).astype(BF16))
            return ps

        def oproj(os_, h0):
            oc = jnp.concatenate(os_, axis=1)
            k0, k1 = h0 * DH, (h0 + len(os_)) * DH
            return [jnp.dot(oc, wo_s[k0:k1, n * 128:(n + 1) * 128], preferred_element_type=F32)
                    for n in range(NLB)]

        heads = []
        qkv = proj(0)
        oa = None
        for g in range(NG):
            ps = probs(qkv)
            vs = qkv[2]
            if g + 1 < NG:
                qkv = proj(g + 1)
            else:
                if before_oproj is not None:
                    before_oproj()
                oa = oproj(heads[:H // 2], 0)
            heads += [jnp.dot(ps[j], vs[j], preferred_element_type=F32).astype(BF16)
                      for j in range(HG)]
        ob = oproj(heads[H // 2:], H // 2)
        return jnp.concatenate([b + a for a, b in zip(oa, ob)], axis=1)

    def post2(s):
        r3 = seg_row(s - 1 - LAG)
        xo = gate(_r(x2_s[(s + 4 - 1 - LAG) % 4] + obuf[SEG:2 * SEG, :]), r3)
        out_s[pl.ds(r3, SEG), :] = xo.astype(BF16)

    def step(s, mode, vis, fill, chained=False, before_oproj=None):
        if mode == 0:
            h = hbuf[...]
        elif mode == 1:
            h = hbuf[0:48, :]
        else:
            h = jnp.concatenate([hbuf[0:16, :], hbuf[48:80, :]], axis=0)
        r1 = seg_row(s - 1)
        xb2 = _r(gate(_r(x_s[pl.ds(r1, SEG), :].astype(F32) + obuf[0:SEG, :]), r1))
        h2n = _ln(xb2).astype(BF16)
        if mode != 1:
            post2(s)
        x2_s[(s + 4 - 1) % 4] = xb2
        if mode != 2:
            h1n = _ln(x_s[pl.ds(seg_row(s + 1), SEG), :].astype(F32)).astype(BF16)

        o = attention(h, vis, fill, chained, before_oproj)

        mem2 = mem0 if mode == 1 else o[M:2 * M]
        hbuf[0:16, :] = jnp.concatenate([o[0:M], mem2], axis=0).astype(BF16)
        if mode != 2:
            hbuf[16:48, :] = h1n
        hbuf[48:80, :] = h2n
        if mode == 0:
            obuf[...] = _r(o[2 * M:])
        elif mode == 1:
            obuf[0:SEG, :] = _r(o[2 * M:])
        else:
            obuf[SEG:2 * SEG, :] = _r(o[2 * M:])

    with jax.named_scope("pro"):
        vis, fill = masks(1)
        step(0, 1, vis, fill, False, wo_copy.wait)
        step(1, 1, vis, fill, True)
    xb_copy.wait()
    with jax.named_scope("main"):
        vis, fill = masks(0)
        loop((NSEG - LAG) // UNR, lambda i: [step(UNR * i + u + LAG, 0, vis, fill, u > 0)
                                             for u in range(UNR)])
    done = (NSEG - 1 - LAG) * SEG
    out_a = pltpu.make_async_copy(out_s.at[0:done, :], out_hbm.at[0:done, :], sem_x.at[1])
    out_a.start()
    with jax.named_scope("epi"):
        vis, fill = masks(2)
        step(NSEG, 2, vis, fill)
        step(NSEG + 1, 2, vis, fill, True)
    post2(NSEG + LAG)
    out_b = pltpu.make_async_copy(out_s.at[done:S, :], out_hbm.at[done:S, :], sem_x.at[2])
    out_b.start()
    out_a.wait()
    out_b.wait()


@jax.jit
def pallas_interleave_layers__memory_aug_recurrent_mem_tr__ssm_conv_h3__prompt_kernel(
    A_x, A_mem0, A_Wq, A_Wk, A_Wv, A_Wo, A_seg_len,
    B_q, B_k, B_v, B_shift_k, B_ssm_k, B_ssm_D,
):
    del A_seg_len, B_q
    assert A_x.shape == (1, S, D) and A_Wq.shape == (D, H, DH)
    vm = pl.BlockSpec(memory_space=pltpu.VMEM)
    hbm = pl.BlockSpec(memory_space=pl.ANY)
    out = pl.pallas_call(
        _kernel,
        out_shape=jax.ShapeDtypeStruct((S, D), BF16),
        in_specs=[hbm, vm, hbm, hbm, hbm, hbm, hbm, hbm, vm, hbm, vm],
        out_specs=hbm,
        scratch_shapes=[
            pltpu.VMEM((S, D), BF16),
            pltpu.VMEM((S, D), BF16),
            pltpu.VMEM((S, D), BF16),
            pltpu.VMEM((NB, D, TB), BF16),
            pltpu.VMEM((3, D, H, DH), BF16),
            pltpu.VMEM(((3 * H + 1) * WP, 128), U32),
            pltpu.VMEM((H * DH, D), BF16),
            pltpu.VMEM((2 * TB, 2 * TB), BF16),
            pltpu.VMEM((2, TB, TB), BF16),
            pltpu.VMEM((2, TB // 2, 3 * TB), BF16),
            pltpu.VMEM((2, NLB, S // 2 + 8, 128), F32),
            pltpu.VMEM((NB // 2, 2, TB, D), F32),
            pltpu.VMEM((NB // 2, 2, TB, D), F32),
            pltpu.VMEM((NB // 2, 3, TB, D), F32),
            pltpu.VMEM((NB // 2, 3, TB, D), F32),
            pltpu.VMEM((NB // 2 + 1, 2, TB, D), F32),
            pltpu.VMEM((NB // 2 + 1, 2, TB, D), F32),
            pltpu.VMEM((NB // 2 - 1, 2, TB, D), F32),
            pltpu.VMEM((NLB, S + 8, 128), F32),
            pltpu.VMEM((ROWS, D), BF16),
            pltpu.VMEM((2 * SEG, D), F32),
            pltpu.VMEM((4, SEG, D), F32),
            pltpu.VMEM((S, D), BF16),
            pltpu.SemaphoreType.DMA((3 * (NB // 2) + 1,)),
            pltpu.SemaphoreType.DMA((4,)),
            pltpu.SemaphoreType.DMA((4,)),
        ],
        compiler_params=pltpu.CompilerParams(vmem_limit_bytes=120 * 1024 * 1024),
    )(A_x.reshape(S, D), A_mem0.reshape(M, D), A_Wq, A_Wk, A_Wv,
      A_Wo.reshape(H * DH, D), B_k.reshape(S, D), B_v.reshape(S, D),
      B_shift_k.T, B_ssm_k, B_ssm_D)
    return out.reshape(1, S, D)
```

```python
import math

import jax
import jax.numpy as jnp
from jax import lax
import jax.experimental.pallas as pl
import jax.experimental.pallas.tpu as pltpu

F32 = jnp.float32
BF16 = jnp.bfloat16
U32 = jnp.uint32

S = 2048
D = 640
H = 32
DH = 128
M = 8
SEG = 32
NSEG = S // SEG
KS = 4
LAG = 2
ROWS = 2 * M + 2 * SEG
HG = 4
NG = H // HG
NLB = D // 128
TB = 128
NB = S // TB
UNR = 1
WP = 324


def _ln(x):
    m = jnp.mean(x, axis=-1, keepdims=True)
    c = x - m
    v = jnp.mean(c * c, axis=-1, keepdims=True)
    return c * lax.rsqrt(v + 1e-5)


def _r(x):
    return x.astype(BF16).astype(F32)


def _split(x):
    hi = pltpu.bitcast(pltpu.bitcast(x, U32) & jnp.uint32(0xFFFF0000), F32)
    return hi, x - hi


def _bf(x):
    return jnp.concatenate([x[:, g:g + 128].astype(BF16)
                            for g in range(0, x.shape[1], 128)], axis=1)


def _basis(r, t):
    b = r & 63
    f = jnp.where(b < 32, 2 * b, 2 * b - 63)
    n = ((2 * f + 1) * t - jnp.where(r >= 64, TB, 0)) & (4 * TB - 1)
    n = jnp.where(n >= 2 * TB, n - 4 * TB, n)
    return jnp.cos(n.astype(F32) * (2.0 * math.pi / (4 * TB)))


def _halves(x):
    w = pltpu.bitcast(x, U32)
    return (pltpu.bitcast(w << 16, F32),
            pltpu.bitcast(w & jnp.uint32(0xFFFF0000), F32))


def _kernel(x_hbm, mem0_ref, wq_hbm, wk_hbm, wv_hbm, wo_hbm,
            k_hbm, v_hbm, shk_ref, ssmk_hbm, ssmd_ref,
            out_hbm,
            x_s, k_s, v_s, ssmk_s, wraw, wt, wo_s,
            perm_s, fu_s, inv_s, kpad, u_a, u_b, kf_a, kf_b, c_a, c_b, s1_s, y_s,
            hbuf, obuf, x2_s, out_s,
            sem_c, sem_w, sem_x):
    HB = NB // 2
    XH = 4 * SEG

    def conv_copies(j):
        r0 = j * TB if isinstance(j, int) else pl.multiple_of(j * TB, TB)
        return (
            pltpu.make_async_copy(ssmk_hbm.at[:, pl.ds(r0, TB)], ssmk_s.at[j], sem_c.at[j]),
            pltpu.make_async_copy(k_hbm.at[pl.ds(r0, TB), :], k_s.at[pl.ds(r0, TB), :], sem_c.at[HB + j]),
            pltpu.make_async_copy(v_hbm.at[pl.ds(r0, TB), :], v_s.at[pl.ds(r0, TB), :], sem_c.at[NB + j]),
        )
    late_copies = [pltpu.make_async_copy(ssmk_hbm.at[:, pl.ds(j * TB, TB)], ssmk_s.at[j], sem_c.at[3 * HB])
                   for j in range(HB, NB)]
    late_copies += [pltpu.make_async_copy(src.at[S // 2:, :], dst.at[S // 2:, :], sem_c.at[3 * HB])
                    for src, dst in ((k_hbm, k_s), (v_hbm, v_s))]
    w_copies = [pltpu.make_async_copy(w, wraw.at[t], sem_w.at[t])
                for t, w in enumerate((wq_hbm, wk_hbm, wv_hbm))]
    wo_copy = pltpu.make_async_copy(wo_hbm, wo_s, sem_w.at[3])
    xa_copy = pltpu.make_async_copy(x_hbm.at[0:XH, :], x_s.at[0:XH, :], sem_x.at[0])
    xb_copy = pltpu.make_async_copy(x_hbm.at[XH:, :], x_s.at[XH:, :], sem_x.at[3])
    for j in range(HB):
        for c in conv_copies(j):
            c.start()
    for c in late_copies:
        c.start()
    xa_copy.start()
    wo_copy.start(priority=1)
    xb_copy.start(priority=1)

    hb = TB // 2
    ri = lax.broadcasted_iota(jnp.int32, (TB, TB), 0)
    ci = lax.broadcasted_iota(jnp.int32, (TB, TB), 1)
    perm_s[...] = jnp.where(ci == 2 * (ri & 63) + (ri >> 6), 1.0, 0.0).astype(BF16)
    tab = _basis(ri, 2 * (ci & 63) + (ci >> 6))
    hi, lo = _split(tab)
    fu_s[0] = jnp.where(ci < hb, hi, pltpu.roll(lo, hb, 1)).astype(BF16)
    fu_s[1] = jnp.where(ci < hb, pltpu.roll(hi, hb, 1), lo).astype(BF16)
    gh, gl = _split(tab.T * (1.0 / TB))
    ginv = _bf(jnp.concatenate([gh, gl, gh], axis=1))
    inv_s[0] = ginv[:hb]
    inv_s[1] = ginv[hb:]

    shk_t = shk_ref[...].astype(F32)
    taps = [[shk_t[j:j + 1, g * 128:(g + 1) * 128] for g in range(NLB)] for j in range(KS)]
    dvec = ssmd_ref[...].astype(F32).reshape(1, D)
    for g in range(NLB):
        kpad[0, g, 0:8, :] = jnp.zeros((8, 128), F32)
        kpad[1, g, 0:8, :] = jnp.zeros((8, 128), F32)
    c_a[0] = jnp.zeros(c_a.shape[1:], F32)

    def spectrum(e, o):
        fe = jnp.dot(fu_s[0], jnp.concatenate([e, e], axis=0).astype(BF16), preferred_element_type=F32)
        fo = jnp.dot(fu_s[1], jnp.concatenate([o, o], axis=0).astype(BF16), preferred_element_type=F32)
        return ((fe[:hb] + fo[:hb], fe[hb:] + fo[hb:]), (fe[:hb] - fo[:hb], fo[hb:] - fe[hb:]))

    def fwd_stage(jls, half):
        u_s, kf_s = ((u_a, kf_a), (u_b, kf_b))[half]
        if half == 0:
            for jl in jls:
                for c in conv_copies(jl):
                    c.wait()
        kts = [lax.dot_general(perm_s[...], ssmk_s[jl + half * HB], (((1,), (1,)), ((), ())),
                               preferred_element_type=F32) for jl in jls]
        halves = (slice(0, hb), slice(hb, TB))
        for jl, kt in zip(jls, kts):
            j = jl + half * HB
            r0 = pl.multiple_of(j * TB, TB)
            q0 = pl.multiple_of(j * hb, hb) + 8
            for g in range(NLB):
                lb = slice(g * 128, (g + 1) * 128)
                for rows, (kr, ki) in zip(halves, spectrum(kt[:hb, lb], kt[hb:, lb])):
                    if half == 0:
                        kr = kr + jnp.where(jl == 0, dvec[:, lb], 0.0)
                    kf_s[jl, 0, rows, lb] = kr
                    kf_s[jl, 1, rows, lb] = ki - kr
                    kf_s[jl, 2, rows, lb] = kr + ki
                ke, ko = _halves(k_s[pl.ds(r0, TB), lb])
                ve, vo = _halves(v_s[pl.ds(r0, TB), lb])
                kpad[0, g, pl.ds(q0, hb), :] = ke
                kpad[1, g, pl.ds(q0, hb), :] = ko
                ke1 = kpad[0, g, pl.ds(q0 - 1, hb), :]
                ko1 = kpad[1, g, pl.ds(q0 - 1, hb), :]
                ko2 = kpad[1, g, pl.ds(q0 - 2, hb), :]
                t0, t1, t2, t3 = (taps[t][g] for t in range(KS))
                e = (ke * t0 + ko1 * t1 + ke1 * t2 + ko2 * t3) * ve
                o = (ko * t0 + ke * t1 + ko1 * t2 + ke1 * t3) * vo
                for rows, (ur, ui) in zip(halves, spectrum(e, o)):
                    u_s[jl, 0, rows, lb] = ur
                    u_s[jl, 1, rows, lb] = ui

    def mac_stage(jj, half, only=None):
        c_s = (c_a, c_b)[half]
        for rg in range(2):
            rs = pl.ds(pl.multiple_of((2 * jj + rg) * 8, 8), 8)
            for g in range(NLB):
                lb = slice(g * 128, (g + 1) * 128)

                def uu(i, p):
                    u_s = u_a if i < HB else u_b
                    if p == 0:
                        return u_s[i % HB, 0, rs, lb] + u_s[i % HB, 1, rs, lb]
                    return u_s[i % HB, p - 1, rs, lb]

                def kk(i, p):
                    return (kf_a if i < HB else kf_b)[i % HB, p, rs, lb]

                def poly(p, acc):
                    acc = dict(acc)
                    ua, kb = {}, {}
                    for a0, b0 in (((0, HB), (0, 0), (HB, 0)) if half else ((0, 0),)):
                        for a in range(a0, a0 + HB):
                            for i in range(half * HB, half * HB + HB):
                                b = i - a
                                if not b0 <= b < b0 + HB:
                                    continue
                                if a not in ua:
                                    ua[a] = uu(a, p)
                                if b not in kb:
                                    kb[b] = kk(b, p)
                                t = ua[a] * kb[b]
                                if i not in acc:
                                    acc[i] = t
                                elif p == 2:
                                    acc[i] = acc[i] - t
                                else:
                                    acc[i] = acc[i] + t
                    return acc

                if only in (None, 0):
                    s1 = poly(0, {})
                if only == 0:
                    for i, v in s1.items():
                        s1_s[i % HB, rs, lb] = v
                    continue
                if only is not None:
                    s1 = {i: s1_s[i % HB, rs, lb] for i in range(half * HB, half * HB + HB)}
                for p, comp in ((1, 1), (2, 0)):
                    if only not in (None, p):
                        continue
                    for i, v in poly(p, s1).items():
                        c_s[i % HB + 1, comp, rs, lb] = v
                        if i == HB - 1:
                            c_b[0, comp, rs, lb] = v

    def inv_stage(il, half):
        i = il + half * HB
        c_s = (c_a, c_b)[half]
        q = TB // 4
        re, im = [], []
        for b in range(4):
            rows = slice(b * q, (b + 1) * q)
            cr, ci_ = c_s[il + 1, 0, rows], c_s[il + 1, 1, rows]
            pr, pi = c_s[il, 0, rows], c_s[il, 1, rows]
            re.append(cr + pi if b in (0, 3) else cr - pi)
            im.append(ci_ - pr if b in (0, 3) else ci_ + pr)
        pe = jnp.concatenate([re[0] + re[2], re[1] + re[3], im[0] - im[2], im[1] - im[3]], axis=0)
        po = jnp.concatenate([re[0] - re[2], re[1] - re[3], im[0] + im[2], im[1] + im[3]], axis=0)
        for par, pp in enumerate((pe, po)):
            ph, plo = _split(pp)
            y = jnp.dot(inv_s[par], jnp.concatenate([ph, ph, plo], axis=0).astype(BF16),
                        preferred_element_type=F32)
            for g in range(NLB):
                y_s[g, pl.ds(i * TB + par, hb, stride=2), :] = y[:, g * 128:(g + 1) * 128]

    def relayout(t):
        w_copies[t].wait()

        def body(i, _):
            for dd in range(32):
                dp = i * 32 + dd
                a = pltpu.bitcast(wraw[t, 2 * dp], U32)
                b = pltpu.bitcast(wraw[t, 2 * dp + 1], U32)
                lo = (a & jnp.uint32(0xFFFF)) | (b << 16)
                hi = (a >> 16) | (b & jnp.uint32(0xFFFF0000))
                wt[pl.ds(t * H * WP + dp, 16, stride=WP), :] = lo
                wt[pl.ds((t * H + 16) * WP + dp, 16, stride=WP), :] = hi
            return 0
        lax.fori_loop(0, D // 64, body, 0)

    def wslab(t, h):
        s0 = (t * H + (h % 2) * 16 + h // 2) * WP
        return pltpu.bitcast(wt[s0:s0 + D // 2, :], BF16)

    def loop(n, fn):
        def body(j, _):
            fn(j)
            return 0
        lax.fori_loop(0, n, body, 0)

    with jax.named_scope("conv_a"):
        loop(HB // 2, lambda j: fwd_stage((2 * j, 2 * j + 1), 0))
    with jax.named_scope("conv_b"):
        for c in w_copies:
            c.start()
        loop(HB, lambda j: mac_stage(j, 0))
        loop(HB // 2, lambda j: (inv_stage(2 * j, 0), inv_stage(2 * j + 1, 0)))
    with jax.named_scope("conv_c"):
        for c in late_copies:
            c.wait()
        loop(HB // 2, lambda j: fwd_stage((2 * j, 2 * j + 1), 1))
    with jax.named_scope("rel0"):
        relayout(0)
    with jax.named_scope("conv_d"):
        for p in range(3):
            loop(HB // 2, lambda j: (mac_stage(2 * j, 1, p), mac_stage(2 * j + 1, 1, p)))
    with jax.named_scope("rel1"):
        relayout(1)
    with jax.named_scope("conv_e"):
        loop(HB // 2, lambda j: (inv_stage(2 * j, 1), inv_stage(2 * j + 1, 1)))
    with jax.named_scope("rel2"):
        relayout(2)
    with jax.named_scope("waitx"):
        xa_copy.wait()

    scale = DH ** -0.5

    def masks(mode):
        rows = ROWS if mode == 0 else ROWS - SEG
        qi = lax.broadcasted_iota(jnp.int32, (rows, rows), 0)
        kj = lax.broadcasted_iota(jnp.int32, (rows, rows), 1)

        def layer_of(i):
            xl = (i - 2 * M) // SEG if mode == 0 else mode - 1
            return jnp.where(i < 2 * M, i // M, xl)
        same = layer_of(qi) == layer_of(kj)
        vis = same & ((qi < 2 * M) | (qi >= kj))
        fill = jnp.where(same, -1e9, -jnp.inf).astype(F32)
        return vis, fill

    mem0 = mem0_ref[...].astype(F32)
    hbuf[0:16, :] = jnp.concatenate([mem0, mem0], axis=0).astype(BF16)
    hbuf[16:48, :] = _ln(x_s[0:SEG, :].astype(F32)).astype(BF16)
    obuf[...] = jnp.zeros((2 * SEG, D), F32)
    x2_s[...] = jnp.zeros(x2_s.shape, F32)

    def seg_row(seg):
        if isinstance(seg, int):
            return min(max(seg, 0), NSEG - 1) * SEG
        return pl.multiple_of(jnp.clip(seg, 0, NSEG - 1) * SEG, SEG)

    def gate(xa, r0):
        y = jnp.concatenate([y_s[g, pl.ds(r0, SEG), :] for g in range(NLB)], axis=1)
        return xa + _r(_r(_ln(xa)) * y)

    def attention(h, vis, fill, chained, before_oproj=None):
        def proj(g):
            if g == 0 and chained:
                kc = D - 128
                part = [jnp.dot(h[:, :kc], wslab(0, j)[:kc], preferred_element_type=F32)
                        for j in range(HG)]
                q = [(jnp.dot(h[:, kc:], wslab(0, j)[kc:], preferred_element_type=F32)
                      + part[j]).astype(BF16) for j in range(HG)]
                return [q] + [[jnp.dot(h, wslab(t, j), preferred_element_type=F32).astype(BF16)
                               for j in range(HG)] for t in range(1, 3)]
            return [[jnp.dot(h, wslab(t, g * HG + j), preferred_element_type=F32).astype(BF16)
                     for j in range(HG)] for t in range(3)]

        def probs(qkv):
            scs = [lax.dot_general(qkv[0][j], qkv[1][j], (((1,), (1,)), ((), ())),
                                   preferred_element_type=F32) for j in range(HG)]
            ps = []
            for sc in scs:
                sc = jnp.where(vis, sc * scale, fill)
                e = jnp.exp(sc - jnp.max(sc, axis=-1, keepdims=True))
                den = jnp.sum(e, axis=-1, keepdims=True)
                r = pl.reciprocal(den, approx=True)
                r = r * (2.0 - den * r)
                ps.append((e * r).astype(BF16))
            return ps

        def oproj(os_, h0):
            oc = jnp.concatenate(os_, axis=1)
            k0, k1 = h0 * DH, (h0 + len(os_)) * DH
            return [jnp.dot(oc, wo_s[k0:k1, n * 128:(n + 1) * 128], preferred_element_type=F32)
                    for n in range(NLB)]

        heads = []
        qkv = proj(0)
        oa = None
        for g in range(NG):
            ps = probs(qkv)
            vs = qkv[2]
            if g + 1 < NG:
                qkv = proj(g + 1)
            else:
                if before_oproj is not None:
                    before_oproj()
                oa = oproj(heads[:H // 2], 0)
            heads += [jnp.dot(ps[j], vs[j], preferred_element_type=F32).astype(BF16)
                      for j in range(HG)]
        ob = oproj(heads[H // 2:], H // 2)
        return jnp.concatenate([b + a for a, b in zip(oa, ob)], axis=1)

    def post2(s):
        r3 = seg_row(s - 1 - LAG)
        xo = gate(_r(x2_s[(s + 4 - 1 - LAG) % 4] + obuf[SEG:2 * SEG, :]), r3)
        out_s[pl.ds(r3, SEG), :] = xo.astype(BF16)

    def step(s, mode, vis, fill, chained=False, before_oproj=None):
        if mode == 0:
            h = hbuf[...]
        elif mode == 1:
            h = hbuf[0:48, :]
        else:
            h = jnp.concatenate([hbuf[0:16, :], hbuf[48:80, :]], axis=0)
        r1 = seg_row(s - 1)
        xb2 = _r(gate(_r(x_s[pl.ds(r1, SEG), :].astype(F32) + obuf[0:SEG, :]), r1))
        h2n = _ln(xb2).astype(BF16)
        if mode != 1:
            post2(s)
        x2_s[(s + 4 - 1) % 4] = xb2
        if mode != 2:
            h1n = _ln(x_s[pl.ds(seg_row(s + 1), SEG), :].astype(F32)).astype(BF16)

        o = attention(h, vis, fill, chained, before_oproj)

        mem2 = mem0 if mode == 1 else o[M:2 * M]
        hbuf[0:16, :] = jnp.concatenate([o[0:M], mem2], axis=0).astype(BF16)
        if mode != 2:
            hbuf[16:48, :] = h1n
        hbuf[48:80, :] = h2n
        if mode == 0:
            obuf[...] = _r(o[2 * M:])
        elif mode == 1:
            obuf[0:SEG, :] = _r(o[2 * M:])
        else:
            obuf[SEG:2 * SEG, :] = _r(o[2 * M:])

    with jax.named_scope("pro"):
        vis, fill = masks(1)
        step(0, 1, vis, fill, False, wo_copy.wait)
        step(1, 1, vis, fill, True)
    xb_copy.wait()
    with jax.named_scope("main"):
        vis, fill = masks(0)
        loop((NSEG - LAG) // UNR, lambda i: [step(UNR * i + u + LAG, 0, vis, fill, u > 0)
                                             for u in range(UNR)])
    done = (NSEG - 1 - LAG) * SEG
    out_a = pltpu.make_async_copy(out_s.at[0:done, :], out_hbm.at[0:done, :], sem_x.at[1])
    out_a.start()
    with jax.named_scope("epi"):
        vis, fill = masks(2)
        step(NSEG, 2, vis, fill)
        step(NSEG + 1, 2, vis, fill, True)
    post2(NSEG + LAG)
    out_b = pltpu.make_async_copy(out_s.at[done:S, :], out_hbm.at[done:S, :], sem_x.at[2])
    out_b.start()
    out_a.wait()
    out_b.wait()


@jax.jit
def pallas_interleave_layers__memory_aug_recurrent_mem_tr__ssm_conv_h3__prompt_kernel(
    A_x, A_mem0, A_Wq, A_Wk, A_Wv, A_Wo, A_seg_len,
    B_q, B_k, B_v, B_shift_k, B_ssm_k, B_ssm_D,
):
    del A_seg_len, B_q
    assert A_x.shape == (1, S, D) and A_Wq.shape == (D, H, DH)
    vm = pl.BlockSpec(memory_space=pltpu.VMEM)
    hbm = pl.BlockSpec(memory_space=pl.ANY)
    out = pl.pallas_call(
        _kernel,
        out_shape=jax.ShapeDtypeStruct((S, D), BF16),
        in_specs=[hbm, vm, hbm, hbm, hbm, hbm, hbm, hbm, vm, hbm, vm],
        out_specs=hbm,
        scratch_shapes=[
            pltpu.VMEM((S, D), BF16),
            pltpu.VMEM((S, D), BF16),
            pltpu.VMEM((S, D), BF16),
            pltpu.VMEM((NB, D, TB), BF16),
            pltpu.VMEM((3, D, H, DH), BF16),
            pltpu.VMEM(((3 * H + 1) * WP, 128), U32),
            pltpu.VMEM((H * DH, D), BF16),
            pltpu.VMEM((TB, TB), BF16),
            pltpu.VMEM((2, TB, TB), BF16),
            pltpu.VMEM((2, TB // 2, 3 * TB), BF16),
            pltpu.VMEM((2, NLB, S // 2 + 8, 128), F32),
            pltpu.VMEM((NB // 2, 2, TB, D), F32),
            pltpu.VMEM((NB // 2, 2, TB, D), F32),
            pltpu.VMEM((NB // 2, 3, TB, D), F32),
            pltpu.VMEM((NB // 2, 3, TB, D), F32),
            pltpu.VMEM((NB // 2 + 1, 2, TB, D), F32),
            pltpu.VMEM((NB // 2 + 1, 2, TB, D), F32),
            pltpu.VMEM((NB // 2, TB, D), F32),
            pltpu.VMEM((NLB, S + 8, 128), F32),
            pltpu.VMEM((ROWS, D), BF16),
            pltpu.VMEM((2 * SEG, D), F32),
            pltpu.VMEM((4, SEG, D), F32),
            pltpu.VMEM((S, D), BF16),
            pltpu.SemaphoreType.DMA((3 * (NB // 2) + 1,)),
            pltpu.SemaphoreType.DMA((4,)),
            pltpu.SemaphoreType.DMA((4,)),
        ],
        compiler_params=pltpu.CompilerParams(vmem_limit_bytes=120 * 1024 * 1024),
    )(A_x.reshape(S, D), A_mem0.reshape(M, D), A_Wq, A_Wk, A_Wv,
      A_Wo.reshape(H * DH, D), B_k.reshape(S, D), B_v.reshape(S, D),
      B_shift_k.T, B_ssm_k, B_ssm_D)
    return out.reshape(1, S, D)
```

```python
import math

import jax
import jax.numpy as jnp
from jax import lax
import jax.experimental.pallas as pl
import jax.experimental.pallas.tpu as pltpu

F32 = jnp.float32
BF16 = jnp.bfloat16
U32 = jnp.uint32

S = 2048
D = 640
H = 32
DH = 128
M = 8
SEG = 32
NSEG = S // SEG
KS = 4
LAG = 2
ROWS = 2 * M + 2 * SEG
HG = 4
NG = H // HG
NLB = D // 128
TB = 128
NB = S // TB
UNR = 1
WP = 324


def _ln(x):
    m = jnp.mean(x, axis=-1, keepdims=True)
    c = x - m
    v = jnp.mean(c * c, axis=-1, keepdims=True)
    return c * lax.rsqrt(v + 1e-5)


def _r(x):
    return x.astype(BF16).astype(F32)


def _split(x):
    hi = pltpu.bitcast(pltpu.bitcast(x, U32) & jnp.uint32(0xFFFF0000), F32)
    return hi, x - hi


def _bf(x):
    return jnp.concatenate([x[:, g:g + 128].astype(BF16)
                            for g in range(0, x.shape[1], 128)], axis=1)


def _basis(r, t):
    b = r & 63
    f = jnp.where(b < 32, 2 * b, 2 * b - 63)
    n = ((2 * f + 1) * t - jnp.where(r >= 64, TB, 0)) & (4 * TB - 1)
    n = jnp.where(n >= 2 * TB, n - 4 * TB, n)
    return jnp.cos(n.astype(F32) * (2.0 * math.pi / (4 * TB)))


def _halves(x):
    w = pltpu.bitcast(x, U32)
    return (pltpu.bitcast(w << 16, F32),
            pltpu.bitcast(w & jnp.uint32(0xFFFF0000), F32))


def _kernel(x_hbm, mem0_ref, wq_hbm, wk_hbm, wv_hbm, wo_hbm,
            k_hbm, v_hbm, shk_ref, ssmk_hbm, ssmd_ref,
            out_hbm,
            x_s, k_s, v_s, ssmk_s, wraw, wt, wo_s,
            perm_s, fu_s, inv_s, kpad, u_a, u_b, kf_a, kf_b, c_a, c_b, s1_s, y_s,
            hbuf, obuf, x2_s, out_s,
            sem_c, sem_w, sem_x):
    HB = NB // 2
    XH = 4 * SEG

    def conv_copies(j):
        r0 = j * TB if isinstance(j, int) else pl.multiple_of(j * TB, TB)
        return (
            pltpu.make_async_copy(ssmk_hbm.at[:, pl.ds(r0, TB)], ssmk_s.at[j], sem_c.at[j]),
            pltpu.make_async_copy(k_hbm.at[pl.ds(r0, TB), :], k_s.at[pl.ds(r0, TB), :], sem_c.at[HB + j]),
            pltpu.make_async_copy(v_hbm.at[pl.ds(r0, TB), :], v_s.at[pl.ds(r0, TB), :], sem_c.at[NB + j]),
        )
    late_copies = [pltpu.make_async_copy(ssmk_hbm.at[:, pl.ds(j * TB, TB)], ssmk_s.at[j], sem_c.at[3 * HB])
                   for j in range(HB, NB)]
    late_copies += [pltpu.make_async_copy(src.at[S // 2:, :], dst.at[S // 2:, :], sem_c.at[3 * HB])
                    for src, dst in ((k_hbm, k_s), (v_hbm, v_s))]
    w_copies = [pltpu.make_async_copy(w, wraw.at[t], sem_w.at[t])
                for t, w in enumerate((wq_hbm, wk_hbm, wv_hbm))]
    wo_copy = pltpu.make_async_copy(wo_hbm, wo_s, sem_w.at[3])
    xa_copy = pltpu.make_async_copy(x_hbm.at[0:XH, :], x_s.at[0:XH, :], sem_x.at[0])
    xb_copy = pltpu.make_async_copy(x_hbm.at[XH:, :], x_s.at[XH:, :], sem_x.at[3])
    for j in range(HB):
        for c in conv_copies(j):
            c.start()
    for c in late_copies:
        c.start()
    xa_copy.start()
    wo_copy.start(priority=1)
    xb_copy.start(priority=1)

    hb = TB // 2
    ri = lax.broadcasted_iota(jnp.int32, (TB, TB), 0)
    ci = lax.broadcasted_iota(jnp.int32, (TB, TB), 1)
    perm_s[...] = jnp.where(ci == 2 * (ri & 63) + (ri >> 6), 1.0, 0.0).astype(BF16)
    tab = _basis(ri, 2 * (ci & 63) + (ci >> 6))
    hi, lo = _split(tab)
    fu_s[0] = jnp.where(ci < hb, hi, pltpu.roll(lo, hb, 1)).astype(BF16)
    fu_s[1] = jnp.where(ci < hb, pltpu.roll(hi, hb, 1), lo).astype(BF16)
    gh, gl = _split(tab.T * (1.0 / TB))
    ginv = _bf(jnp.concatenate([gh, gl, gh], axis=1))
    inv_s[0] = ginv[:hb]
    inv_s[1] = ginv[hb:]

    shk_t = shk_ref[...].astype(F32)
    taps = [[shk_t[j:j + 1, g * 128:(g + 1) * 128] for g in range(NLB)] for j in range(KS)]
    dvec = ssmd_ref[...].astype(F32).reshape(1, D)
    for g in range(NLB):
        kpad[0, g, 0:8, :] = jnp.zeros((8, 128), F32)
        kpad[1, g, 0:8, :] = jnp.zeros((8, 128), F32)
    c_a[0] = jnp.zeros(c_a.shape[1:], F32)

    def spectrum(e, o):
        fe = jnp.dot(fu_s[0], jnp.concatenate([e, e], axis=0).astype(BF16), preferred_element_type=F32)
        fo = jnp.dot(fu_s[1], jnp.concatenate([o, o], axis=0).astype(BF16), preferred_element_type=F32)
        return ((fe[:hb] + fo[:hb], fe[hb:] + fo[hb:]), (fe[:hb] - fo[:hb], fo[hb:] - fe[hb:]))

    def fwd_stage(jls, half):
        u_s, kf_s = ((u_a, kf_a), (u_b, kf_b))[half]
        if half == 0:
            for jl in jls:
                for c in conv_copies(jl):
                    c.wait()
        kts = [lax.dot_general(perm_s[...], ssmk_s[jl + half * HB], (((1,), (1,)), ((), ())),
                               preferred_element_type=F32) for jl in jls]
        halves = (slice(0, hb), slice(hb, TB))
        for jl, kt in zip(jls, kts):
            j = jl + half * HB
            r0 = pl.multiple_of(j * TB, TB)
            q0 = pl.multiple_of(j * hb, hb) + 8
            for g in range(NLB):
                lb = slice(g * 128, (g + 1) * 128)
                for rows, (kr, ki) in zip(halves, spectrum(kt[:hb, lb], kt[hb:, lb])):
                    if half == 0:
                        kr = kr + jnp.where(jl == 0, dvec[:, lb], 0.0)
                    kf_s[jl, 0, rows, lb] = kr
                    kf_s[jl, 1, rows, lb] = ki - kr
                    kf_s[jl, 2, rows, lb] = kr + ki
                ke, ko = _halves(k_s[pl.ds(r0, TB), lb])
                ve, vo = _halves(v_s[pl.ds(r0, TB), lb])
                kpad[0, g, pl.ds(q0, hb), :] = ke
                kpad[1, g, pl.ds(q0, hb), :] = ko
                ke1 = kpad[0, g, pl.ds(q0 - 1, hb), :]
                ko1 = kpad[1, g, pl.ds(q0 - 1, hb), :]
                ko2 = kpad[1, g, pl.ds(q0 - 2, hb), :]
                t0, t1, t2, t3 = (taps[t][g] for t in range(KS))
                e = (ke * t0 + ko1 * t1 + ke1 * t2 + ko2 * t3) * ve
                o = (ko * t0 + ke * t1 + ko1 * t2 + ke1 * t3) * vo
                for rows, (ur, ui) in zip(halves, spectrum(e, o)):
                    u_s[jl, 0, rows, lb] = ur
                    u_s[jl, 1, rows, lb] = ui

    def mac_stage(jj, half, only=None):
        c_s = (c_a, c_b)[half]
        for rg in range(2):
            rs = pl.ds(pl.multiple_of((2 * jj + rg) * 8, 8), 8)
            for g in range(NLB):
                lb = slice(g * 128, (g + 1) * 128)

                def uu(i, p):
                    u_s = u_a if i < HB else u_b
                    if p == 0:
                        return u_s[i % HB, 0, rs, lb] + u_s[i % HB, 1, rs, lb]
                    return u_s[i % HB, p - 1, rs, lb]

                def kk(i, p):
                    return (kf_a if i < HB else kf_b)[i % HB, p, rs, lb]

                def poly(p, acc):
                    acc = dict(acc)
                    ua, kb = {}, {}
                    for a0, b0 in (((0, HB), (0, 0), (HB, 0)) if half else ((0, 0),)):
                        for a in range(a0, a0 + HB):
                            for i in range(half * HB, half * HB + HB):
                                b = i - a
                                if not b0 <= b < b0 + HB:
                                    continue
                                if a not in ua:
                                    ua[a] = uu(a, p)
                                if b not in kb:
                                    kb[b] = kk(b, p)
                                t = ua[a] * kb[b]
                                if i not in acc:
                                    acc[i] = t
                                elif p == 2:
                                    acc[i] = acc[i] - t
                                else:
                                    acc[i] = acc[i] + t
                    return acc

                if only in (None, 0):
                    s1 = poly(0, {})
                if only == 0:
                    for i, v in s1.items():
                        s1_s[i % HB, rs, lb] = v
                    continue
                if only is not None:
                    s1 = {i: s1_s[i % HB, rs, lb] for i in range(half * HB, half * HB + HB)}
                for p, comp in ((1, 1), (2, 0)):
                    if only not in (None, p):
                        continue
                    for i, v in poly(p, s1).items():
                        c_s[i % HB + 1, comp, rs, lb] = v
                        if i == HB - 1:
                            c_b[0, comp, rs, lb] = v

    def inv_stage(il, half):
        i = il + half * HB
        c_s = (c_a, c_b)[half]
        q = TB // 4
        re, im = [], []
        for b in range(4):
            rows = slice(b * q, (b + 1) * q)
            cr, ci_ = c_s[il + 1, 0, rows], c_s[il + 1, 1, rows]
            pr, pi = c_s[il, 0, rows], c_s[il, 1, rows]
            re.append(cr + pi if b in (0, 3) else cr - pi)
            im.append(ci_ - pr if b in (0, 3) else ci_ + pr)
        pe = jnp.concatenate([re[0] + re[2], re[1] + re[3], im[0] - im[2], im[1] - im[3]], axis=0)
        po = jnp.concatenate([re[0] - re[2], re[1] - re[3], im[0] + im[2], im[1] + im[3]], axis=0)
        for par, pp in enumerate((pe, po)):
            ph, plo = _split(pp)
            y = jnp.dot(inv_s[par], jnp.concatenate([ph, ph, plo], axis=0).astype(BF16),
                        preferred_element_type=F32)
            for g in range(NLB):
                y_s[g, pl.ds(i * TB + par, hb, stride=2), :] = y[:, g * 128:(g + 1) * 128]

    def relayout(t):
        w_copies[t].wait()

        def body(i, _):
            for dd in range(32):
                dp = i * 32 + dd
                a = pltpu.bitcast(wraw[t, 2 * dp], U32)
                b = pltpu.bitcast(wraw[t, 2 * dp + 1], U32)
                lo = (a & jnp.uint32(0xFFFF)) | (b << 16)
                hi = (a >> 16) | (b & jnp.uint32(0xFFFF0000))
                wt[pl.ds(t * H * WP + dp, 16, stride=WP), :] = lo
                wt[pl.ds((t * H + 16) * WP + dp, 16, stride=WP), :] = hi
            return 0
        lax.fori_loop(0, D // 64, body, 0)

    def wslab(t, h):
        s0 = (t * H + (h % 2) * 16 + h // 2) * WP
        return pltpu.bitcast(wt[s0:s0 + D // 2, :], BF16)

    def loop(n, fn):
        def body(j, _):
            fn(j)
            return 0
        lax.fori_loop(0, n, body, 0)

    with jax.named_scope("conv_a"):
        loop(HB // 2, lambda j: fwd_stage((2 * j, 2 * j + 1), 0))
    with jax.named_scope("conv_b"):
        for c in w_copies:
            c.start()
        loop(HB, lambda j: mac_stage(j, 0))
        loop(HB // 2, lambda j: (inv_stage(2 * j, 0), inv_stage(2 * j + 1, 0)))
    with jax.named_scope("conv_c"):
        for c in late_copies:
            c.wait()
        loop(HB // 2, lambda j: fwd_stage((2 * j, 2 * j + 1), 1))
    with jax.named_scope("rel0"):
        relayout(0)
    with jax.named_scope("conv_d"):
        for p in range(3):
            loop(HB // 2, lambda j: (mac_stage(2 * j, 1, p), mac_stage(2 * j + 1, 1, p)))
    with jax.named_scope("rel1"):
        relayout(1)
    with jax.named_scope("conv_e"):
        loop(HB // 2, lambda j: (inv_stage(2 * j, 1), inv_stage(2 * j + 1, 1)))
    with jax.named_scope("rel2"):
        relayout(2)
    with jax.named_scope("waitx"):
        xa_copy.wait()

    scale = DH ** -0.5

    def masks(mode, q0=0):
        rows = ROWS if mode == 0 else ROWS - SEG
        qi = lax.broadcasted_iota(jnp.int32, (rows - q0, rows), 0) + q0
        kj = lax.broadcasted_iota(jnp.int32, (rows - q0, rows), 1)

        def layer_of(i):
            xl = (i - 2 * M) // SEG if mode == 0 else mode - 1
            return jnp.where(i < 2 * M, i // M, xl)
        same = layer_of(qi) == layer_of(kj)
        vis = same & ((qi < 2 * M) | (qi >= kj))
        fill = jnp.where(same, -1e9, -jnp.inf).astype(F32)
        return vis, fill

    mem0 = mem0_ref[...].astype(F32)
    hbuf[0:16, :] = jnp.concatenate([mem0, mem0], axis=0).astype(BF16)
    hbuf[16:48, :] = _ln(x_s[0:SEG, :].astype(F32)).astype(BF16)
    obuf[...] = jnp.zeros((2 * SEG, D), F32)
    x2_s[...] = jnp.zeros(x2_s.shape, F32)

    def seg_row(seg):
        if isinstance(seg, int):
            return min(max(seg, 0), NSEG - 1) * SEG
        return pl.multiple_of(jnp.clip(seg, 0, NSEG - 1) * SEG, SEG)

    def gate(xa, r0):
        y = jnp.concatenate([y_s[g, pl.ds(r0, SEG), :] for g in range(NLB)], axis=1)
        return xa + _r(_r(_ln(xa)) * y)

    def attention(h, vis, fill, chained, before_oproj=None):
        q0 = h.shape[0] - vis.shape[0]

        def proj(g):
            if g == 0 and chained and q0 == 0:
                kc = D - 128
                part = [jnp.dot(h[:, :kc], wslab(0, j)[:kc], preferred_element_type=F32)
                        for j in range(HG)]
                q = [(jnp.dot(h[:, kc:], wslab(0, j)[kc:], preferred_element_type=F32)
                      + part[j]).astype(BF16) for j in range(HG)]
                return [q] + [[jnp.dot(h, wslab(t, j), preferred_element_type=F32).astype(BF16)
                               for j in range(HG)] for t in range(1, 3)]
            return [[jnp.dot(h if t else h[q0:], wslab(t, g * HG + j),
                             preferred_element_type=F32).astype(BF16)
                     for j in range(HG)] for t in range(3)]

        def probs(qkv):
            scs = [lax.dot_general(qkv[0][j], qkv[1][j], (((1,), (1,)), ((), ())),
                                   preferred_element_type=F32) for j in range(HG)]
            ps = []
            for sc in scs:
                sc = jnp.where(vis, sc * scale, fill)
                e = jnp.exp(sc - jnp.max(sc, axis=-1, keepdims=True))
                den = jnp.sum(e, axis=-1, keepdims=True)
                r = pl.reciprocal(den, approx=True)
                r = r * (2.0 - den * r)
                ps.append((e * r).astype(BF16))
            return ps

        def oproj(os_, h0):
            oc = jnp.concatenate(os_, axis=1)
            k0, k1 = h0 * DH, (h0 + len(os_)) * DH
            return [jnp.dot(oc, wo_s[k0:k1, n * 128:(n + 1) * 128], preferred_element_type=F32)
                    for n in range(NLB)]

        heads = []
        qkv = proj(0)
        oa = None
        for g in range(NG):
            ps = probs(qkv)
            vs = qkv[2]
            if g + 1 < NG:
                qkv = proj(g + 1)
            else:
                if before_oproj is not None:
                    before_oproj()
                oa = oproj(heads[:H // 2], 0)
            heads += [jnp.dot(ps[j], vs[j], preferred_element_type=F32).astype(BF16)
                      for j in range(HG)]
        ob = oproj(heads[H // 2:], H // 2)
        return jnp.concatenate([b + a for a, b in zip(oa, ob)], axis=1)

    def post2(s):
        r3 = seg_row(s - 1 - LAG)
        xo = gate(_r(x2_s[(s + 4 - 1 - LAG) % 4] + obuf[SEG:2 * SEG, :]), r3)
        out_s[pl.ds(r3, SEG), :] = xo.astype(BF16)

    def step(s, mode, vis, fill, chained=False, before_oproj=None):
        if mode == 0:
            h = hbuf[...]
        elif mode == 1:
            h = hbuf[0:48, :]
        else:
            h = jnp.concatenate([hbuf[0:16, :], hbuf[48:80, :]], axis=0)
        last = isinstance(s, int) and s == NSEG + LAG - 1
        if last:
            post2(s)
            obuf[SEG:2 * SEG, :] = _r(attention(h, vis, fill, chained))
            return
        r1 = seg_row(s - 1)
        xb2 = _r(gate(_r(x_s[pl.ds(r1, SEG), :].astype(F32) + obuf[0:SEG, :]), r1))
        h2n = _ln(xb2).astype(BF16)
        if mode != 1:
            post2(s)
        x2_s[(s + 4 - 1) % 4] = xb2
        if mode != 2:
            h1n = _ln(x_s[pl.ds(seg_row(s + 1), SEG), :].astype(F32)).astype(BF16)

        o = attention(h, vis, fill, chained, before_oproj)

        mem2 = mem0 if mode == 1 else o[M:2 * M]
        hbuf[0:16, :] = jnp.concatenate([o[0:M], mem2], axis=0).astype(BF16)
        if mode != 2:
            hbuf[16:48, :] = h1n
        hbuf[48:80, :] = h2n
        if mode == 0:
            obuf[...] = _r(o[2 * M:])
        elif mode == 1:
            obuf[0:SEG, :] = _r(o[2 * M:])
        else:
            obuf[SEG:2 * SEG, :] = _r(o[2 * M:])

    with jax.named_scope("pro"):
        vis, fill = masks(1)
        step(0, 1, vis, fill, False, wo_copy.wait)
        step(1, 1, vis, fill, True)
    xb_copy.wait()
    with jax.named_scope("main"):
        vis, fill = masks(0)
        loop((NSEG - LAG) // UNR, lambda i: [step(UNR * i + u + LAG, 0, vis, fill, u > 0)
                                             for u in range(UNR)])
    done = (NSEG - 1 - LAG) * SEG
    out_a = pltpu.make_async_copy(out_s.at[0:done, :], out_hbm.at[0:done, :], sem_x.at[1])
    out_a.start()
    with jax.named_scope("epi"):
        vis, fill = masks(2)
        step(NSEG, 2, vis, fill)
        step(NSEG + 1, 2, *masks(2, 2 * M), True)
    post2(NSEG + LAG)
    out_b = pltpu.make_async_copy(out_s.at[done:S, :], out_hbm.at[done:S, :], sem_x.at[2])
    out_b.start()
    out_a.wait()
    out_b.wait()


@jax.jit
def pallas_interleave_layers__memory_aug_recurrent_mem_tr__ssm_conv_h3__prompt_kernel(
    A_x, A_mem0, A_Wq, A_Wk, A_Wv, A_Wo, A_seg_len,
    B_q, B_k, B_v, B_shift_k, B_ssm_k, B_ssm_D,
):
    del A_seg_len, B_q
    assert A_x.shape == (1, S, D) and A_Wq.shape == (D, H, DH)
    vm = pl.BlockSpec(memory_space=pltpu.VMEM)
    hbm = pl.BlockSpec(memory_space=pl.ANY)
    out = pl.pallas_call(
        _kernel,
        out_shape=jax.ShapeDtypeStruct((S, D), BF16),
        in_specs=[hbm, vm, hbm, hbm, hbm, hbm, hbm, hbm, vm, hbm, vm],
        out_specs=hbm,
        scratch_shapes=[
            pltpu.VMEM((S, D), BF16),
            pltpu.VMEM((S, D), BF16),
            pltpu.VMEM((S, D), BF16),
            pltpu.VMEM((NB, D, TB), BF16),
            pltpu.VMEM((3, D, H, DH), BF16),
            pltpu.VMEM(((3 * H + 1) * WP, 128), U32),
            pltpu.VMEM((H * DH, D), BF16),
            pltpu.VMEM((TB, TB), BF16),
            pltpu.VMEM((2, TB, TB), BF16),
            pltpu.VMEM((2, TB // 2, 3 * TB), BF16),
            pltpu.VMEM((2, NLB, S // 2 + 8, 128), F32),
            pltpu.VMEM((NB // 2, 2, TB, D), F32),
            pltpu.VMEM((NB // 2, 2, TB, D), F32),
            pltpu.VMEM((NB // 2, 3, TB, D), F32),
            pltpu.VMEM((NB // 2, 3, TB, D), F32),
            pltpu.VMEM((NB // 2 + 1, 2, TB, D), F32),
            pltpu.VMEM((NB // 2 + 1, 2, TB, D), F32),
            pltpu.VMEM((NB // 2, TB, D), F32),
            pltpu.VMEM((NLB, S + 8, 128), F32),
            pltpu.VMEM((ROWS, D), BF16),
            pltpu.VMEM((2 * SEG, D), F32),
            pltpu.VMEM((4, SEG, D), F32),
            pltpu.VMEM((S, D), BF16),
            pltpu.SemaphoreType.DMA((3 * (NB // 2) + 1,)),
            pltpu.SemaphoreType.DMA((4,)),
            pltpu.SemaphoreType.DMA((4,)),
        ],
        compiler_params=pltpu.CompilerParams(vmem_limit_bytes=120 * 1024 * 1024),
    )(A_x.reshape(S, D), A_mem0.reshape(M, D), A_Wq, A_Wk, A_Wv,
      A_Wo.reshape(H * DH, D), B_k.reshape(S, D), B_v.reshape(S, D),
      B_shift_k.T, B_ssm_k, B_ssm_D)
    return out.reshape(1, S, D)
```

```python
import functools
import math

import jax
import jax.numpy as jnp
from jax import lax
import jax.experimental.pallas as pl
import jax.experimental.pallas.tpu as pltpu

F32 = jnp.float32
BF16 = jnp.bfloat16
U32 = jnp.uint32

S = 2048
D = 640
H = 32
DH = 128
M = 8
SEG = 32
NSEG = S // SEG
KS = 4
LAG = 2
ROWS = 2 * M + 2 * SEG
HG = 4
NG = H // HG
NLB = D // 128
TB = 128
NB = S // TB
HB = NB // 2
NPOS = NLB * TB // 8
NA = 28
PPS = 3
NQH = 16
WP = 324


def _ln(x):
    m = jnp.mean(x, axis=-1, keepdims=True)
    c = x - m
    v = jnp.mean(c * c, axis=-1, keepdims=True)
    return c * lax.rsqrt(v + 1e-5)


def _r(x):
    return x.astype(BF16).astype(F32)


def _split(x):
    hi = pltpu.bitcast(pltpu.bitcast(x, U32) & jnp.uint32(0xFFFF0000), F32)
    return hi, x - hi


def _bf(x):
    return jnp.concatenate([x[:, g:g + 128].astype(BF16)
                            for g in range(0, x.shape[1], 128)], axis=1)


def _basis(r, t):
    b = r & 63
    f = jnp.where(b < 32, 2 * b, 2 * b - 63)
    n = ((2 * f + 1) * t - jnp.where(r >= 64, TB, 0)) & (4 * TB - 1)
    n = jnp.where(n >= 2 * TB, n - 4 * TB, n)
    return jnp.cos(n.astype(F32) * (2.0 * math.pi / (4 * TB)))


def _halves(x):
    w = pltpu.bitcast(x, U32)
    return (pltpu.bitcast(w << 16, F32),
            pltpu.bitcast(w & jnp.uint32(0xFFFF0000), F32))


def _kernel(x_hbm, mem0_ref, wq_hbm, wk_hbm, wv_hbm, wo_hbm,
            k_hbm, v_hbm, shk_ref, ssmk_hbm, ssmd_ref,
            out_hbm,
            x_s, k_s, v_s, ssmk_s, wraw, wt, wo_s,
            perm_s, fu_s, inv_s, kpad, u_s, kf_s, c_s, y_s,
            hbuf, obuf, x2_s, out_s, hl_s, qh_s,
            sem_c, sem_w, sem_x):
    XH = (LAG + NA) * SEG

    def conv_copies(j):
        r0 = j * TB if isinstance(j, int) else pl.multiple_of(j * TB, TB)
        return (
            pltpu.make_async_copy(ssmk_hbm.at[:, pl.ds(r0, TB)], ssmk_s.at[j], sem_c.at[j]),
            pltpu.make_async_copy(k_hbm.at[pl.ds(r0, TB), :], k_s.at[pl.ds(r0, TB), :], sem_c.at[HB + j]),
            pltpu.make_async_copy(v_hbm.at[pl.ds(r0, TB), :], v_s.at[pl.ds(r0, TB), :], sem_c.at[NB + j]),
        )
    late_copies = [pltpu.make_async_copy(ssmk_hbm.at[:, pl.ds(j * TB, TB)], ssmk_s.at[j], sem_c.at[3 * HB])
                   for j in range(HB, NB)]
    late_copies += [pltpu.make_async_copy(src.at[S // 2:, :], dst.at[S // 2:, :], sem_c.at[3 * HB])
                    for src, dst in ((k_hbm, k_s), (v_hbm, v_s))]
    w_copies = [pltpu.make_async_copy(w, wraw.at[t], sem_w.at[t])
                for t, w in enumerate((wq_hbm, wk_hbm, wv_hbm))]
    wo_copy = pltpu.make_async_copy(wo_hbm, wo_s, sem_w.at[3])
    xa_copy = pltpu.make_async_copy(x_hbm.at[0:XH, :], x_s.at[0:XH, :], sem_x.at[0])
    xb_copy = pltpu.make_async_copy(x_hbm.at[XH:, :], x_s.at[XH:, :], sem_x.at[3])
    for j in range(HB):
        for c in conv_copies(j):
            c.start()
    for c in late_copies:
        c.start()
    xa_copy.start()
    wo_copy.start(priority=1)
    xb_copy.start(priority=1)

    hb = TB // 2
    ri = lax.broadcasted_iota(jnp.int32, (TB, TB), 0)
    ci = lax.broadcasted_iota(jnp.int32, (TB, TB), 1)
    perm_s[...] = jnp.where(ci == 2 * (ri & 63) + (ri >> 6), 1.0, 0.0).astype(BF16)
    tab = _basis(ri, 2 * (ci & 63) + (ci >> 6))
    hi, lo = _split(tab)
    fu_s[0] = jnp.where(ci < hb, hi, pltpu.roll(lo, hb, 1)).astype(BF16)
    fu_s[1] = jnp.where(ci < hb, pltpu.roll(hi, hb, 1), lo).astype(BF16)
    gh, gl = _split(tab.T * (1.0 / TB))
    ginv = _bf(jnp.concatenate([gh, gl, gh], axis=1))
    inv_s[0] = ginv[:hb]
    inv_s[1] = ginv[hb:]

    shk_t = shk_ref[...].astype(F32)
    taps = [[shk_t[j:j + 1, g * 128:(g + 1) * 128] for g in range(NLB)] for j in range(KS)]
    dvec = ssmd_ref[...].astype(F32).reshape(1, D)
    for g in range(NLB):
        kpad[0, g, 0:8, :] = jnp.zeros((8, 128), F32)
        kpad[1, g, 0:8, :] = jnp.zeros((8, 128), F32)
    c_s[0] = jnp.zeros(c_s.shape[1:], F32)

    def spectrum(e, o):
        fe = jnp.dot(fu_s[0], jnp.concatenate([e, e], axis=0).astype(BF16), preferred_element_type=F32)
        fo = jnp.dot(fu_s[1], jnp.concatenate([o, o], axis=0).astype(BF16), preferred_element_type=F32)
        return ((fe[:hb] + fo[:hb], fe[hb:] + fo[hb:]), (fe[:hb] - fo[:hb], fo[hb:] - fe[hb:]))

    def fwd_stage(js, first):
        if first:
            for j in js:
                for c in conv_copies(j):
                    c.wait()
        kts = [lax.dot_general(perm_s[...], ssmk_s[j], (((1,), (1,)), ((), ())),
                               preferred_element_type=F32) for j in js]
        for j, kt in zip(js, kts):
            r0 = pl.multiple_of(j * TB, TB)
            q0 = pl.multiple_of(j * hb, hb) + 8
            for g in range(NLB):
                lb = slice(g * 128, (g + 1) * 128)
                halves = (slice(g * TB, g * TB + hb), slice(g * TB + hb, (g + 1) * TB))
                for rows, (kr, ki) in zip(halves, spectrum(kt[:hb, lb], kt[hb:, lb])):
                    if first:
                        kr = kr + jnp.where(j == 0, dvec[:, lb], 0.0)
                    kf_s[j, 0, rows] = kr
                    kf_s[j, 1, rows] = ki - kr
                    kf_s[j, 2, rows] = kr + ki
                ke, ko = _halves(k_s[pl.ds(r0, TB), lb])
                ve, vo = _halves(v_s[pl.ds(r0, TB), lb])
                kpad[0, g, pl.ds(q0, hb), :] = ke
                kpad[1, g, pl.ds(q0, hb), :] = ko
                ke1 = kpad[0, g, pl.ds(q0 - 1, hb), :]
                ko1 = kpad[1, g, pl.ds(q0 - 1, hb), :]
                ko2 = kpad[1, g, pl.ds(q0 - 2, hb), :]
                t0, t1, t2, t3 = (taps[t][g] for t in range(KS))
                e = (ke * t0 + ko1 * t1 + ke1 * t2 + ko2 * t3) * ve
                o = (ko * t0 + ke * t1 + ko1 * t2 + ke1 * t3) * vo
                for rows, (ur, ui) in zip(halves, spectrum(e, o)):
                    u_s[j, 0, rows] = ur
                    u_s[j, 1, rows] = ui

    def mac_units(pos, half):
        rs = pl.ds(pl.multiple_of(pos * 8, 8), 8)
        state = {}

        def unit(p, a0, b0, final, tok=None):
            us = [u_s[a0 + a, 0, rs] + u_s[a0 + a, 1, rs] if p == 0 else u_s[a0 + a, p - 1, rs]
                  for a in range(HB)]
            ks = [kf_s[b0 + b, p, rs] for b in range(HB)]
            if tok is not None:
                ks = [k + tok for k in ks]
            acc = state.setdefault(p, dict(state.get(0, {})))
            for a in range(HB):
                for i in range(half * HB, half * HB + HB):
                    b = i - a0 - a - b0
                    if 0 <= b < HB:
                        t = us[a] * ks[b]
                        acc[i] = t if i not in acc else (acc[i] - t if p == 2 else acc[i] + t)
            if final and p:
                for i, v in acc.items():
                    c_s[i + 1, 2 - p, rs] = v

        subs = ((0, HB), (0, 0), (HB, 0)) if half else ((0, 0),)
        return [functools.partial(unit, p, a0, b0, n == len(subs) - 1)
                for p in range(3) for n, (a0, b0) in enumerate(subs)]

    def inv_stage(i):
        q = TB // 4
        for g in range(NLB):
            re, im = [], []
            for b in range(4):
                rows = slice(g * TB + b * q, g * TB + (b + 1) * q)
                cr, ci_ = c_s[i + 1, 0, rows], c_s[i + 1, 1, rows]
                pr, pi = c_s[i, 0, rows], c_s[i, 1, rows]
                re.append(cr + pi if b in (0, 3) else cr - pi)
                im.append(ci_ - pr if b in (0, 3) else ci_ + pr)
            pe = jnp.concatenate([re[0] + re[2], re[1] + re[3], im[0] - im[2], im[1] - im[3]], axis=0)
            po = jnp.concatenate([re[0] - re[2], re[1] - re[3], im[0] + im[2], im[1] + im[3]], axis=0)
            for par, pp in enumerate((pe, po)):
                ph, plo = _split(pp)
                y_s[g, pl.ds(i * TB + par, hb, stride=2), :] = jnp.dot(
                    inv_s[par], jnp.concatenate([ph, ph, plo], axis=0).astype(BF16),
                    preferred_element_type=F32)

    def relayout(t):
        w_copies[t].wait()

        def body(i, _):
            for dd in range(32):
                dp = i * 32 + dd
                a = pltpu.bitcast(wraw[t, 2 * dp], U32)
                b = pltpu.bitcast(wraw[t, 2 * dp + 1], U32)
                lo = (a & jnp.uint32(0xFFFF)) | (b << 16)
                hi = (a >> 16) | (b & jnp.uint32(0xFFFF0000))
                wt[pl.ds(t * H * WP + dp, 16, stride=WP), :] = lo
                wt[pl.ds((t * H + 16) * WP + dp, 16, stride=WP), :] = hi
            return 0
        lax.fori_loop(0, D // 64, body, 0)

    def wslab(t, h):
        s0 = (t * H + (h % 2) * 16 + h // 2) * WP
        return pltpu.bitcast(wt[s0:s0 + D // 2, :], BF16)

    def loop(n, fn):
        def body(j, _):
            fn(j)
            return 0
        lax.fori_loop(0, n, body, 0)

    def norm_rows(c):
        r0 = pl.multiple_of(c * TB, TB)
        hl_s[pl.ds(r0, TB), :] = _ln(x_s[pl.ds(r0 + LAG * SEG, TB), :].astype(F32)).astype(BF16)

    def pre_queries(c):
        r0 = pl.multiple_of(c * TB, TB)
        hl = hl_s[pl.ds(r0, TB), :]
        for hd in range(NQH):
            qh_s[hd, pl.ds(r0, TB), :] = jnp.dot(
                hl, wslab(0, hd), preferred_element_type=F32).astype(BF16)

    nch = NA * SEG // TB
    with jax.named_scope("conv_a"):
        loop(HB // 2, lambda j: fwd_stage((2 * j, 2 * j + 1), True))
    with jax.named_scope("conv_b"):
        for c in w_copies:
            c.start()
        loop(NPOS // 10, lambda j: [u() for n in range(10) for u in mac_units(10 * j + n, 0)])
        loop(HB // 2, lambda j: (inv_stage(2 * j), inv_stage(2 * j + 1)))
    with jax.named_scope("conv_c"):
        for c in late_copies:
            c.wait()
        loop(HB // 2, lambda j: fwd_stage((HB + 2 * j, HB + 2 * j + 1), False))
    with jax.named_scope("norm"):
        xa_copy.wait()
        loop(nch, norm_rows)
    with jax.named_scope("rel0"):
        relayout(0)
    with jax.named_scope("preq"):
        loop(nch, pre_queries)
    with jax.named_scope("rel1"):
        relayout(1)
    with jax.named_scope("rel2"):
        relayout(2)

    scale = DH ** -0.5

    def masks(mode, q0=0):
        rows = ROWS if mode == 0 else ROWS - SEG
        qi = lax.broadcasted_iota(jnp.int32, (rows - q0, rows), 0) + q0
        kj = lax.broadcasted_iota(jnp.int32, (rows - q0, rows), 1)

        def layer_of(i):
            xl = (i - 2 * M) // SEG if mode == 0 else mode - 1
            return jnp.where(i < 2 * M, i // M, xl)
        same = layer_of(qi) == layer_of(kj)
        vis = same & ((qi < 2 * M) | (qi >= kj))
        fill = jnp.where(same, -1e9, -jnp.inf).astype(F32)
        return vis, fill

    mem0 = mem0_ref[...].astype(F32)
    hbuf[0:16, :] = jnp.concatenate([mem0, mem0], axis=0).astype(BF16)
    hbuf[16:48, :] = _ln(x_s[0:SEG, :].astype(F32)).astype(BF16)
    obuf[...] = jnp.zeros((2 * SEG, D), F32)
    x2_s[...] = jnp.zeros(x2_s.shape, F32)

    def seg_row(seg):
        if isinstance(seg, int):
            return min(max(seg, 0), NSEG - 1) * SEG
        return pl.multiple_of(jnp.clip(seg, 0, NSEG - 1) * SEG, SEG)

    def gate(xa, r0):
        y = jnp.concatenate([y_s[g, pl.ds(r0, SEG), :] for g in range(NLB)], axis=1)
        return xa + _r(_r(_ln(xa)) * y)

    def attention(h, vis, fill, chained, before_oproj=None, early=None):
        q0 = h.shape[0] - vis.shape[0]
        if early is not None:
            hrest = jnp.concatenate([h[:2 * M], h[2 * M + SEG:]], axis=0)
            qrow = pl.multiple_of(early * SEG, SEG)
            units = [u for n in range(PPS)
                     for u in mac_units(jnp.minimum(early * PPS + n, NPOS - 1), 1)]

        def proj(g):
            if g == 0 and chained and q0 == 0:
                kc = D - 128
                part = [jnp.dot(h[:, :kc], wslab(0, j)[:kc], preferred_element_type=F32)
                        for j in range(HG)]
                q = [(jnp.dot(h[:, kc:], wslab(0, j)[kc:], preferred_element_type=F32)
                      + part[j]).astype(BF16) for j in range(HG)]
                return [q] + [[jnp.dot(h, wslab(t, j), preferred_element_type=F32).astype(BF16)
                               for j in range(HG)] for t in range(1, 3)]
            res = [[None] * HG for _ in range(3)]
            order = [(t, j) for j in range(HG) for t in range(2)] + [(2, j) for j in range(HG)]
            for n, (t, j) in enumerate(order):
                hd = g * HG + j
                pre = early is not None and t == 0 and hd < NQH
                lhs = hrest if pre else (h if t else h[q0:])
                r = jnp.dot(lhs, wslab(t, hd), preferred_element_type=F32)
                if early is not None and n % 3 == 1 and units:
                    units.pop(0)(jnp.minimum(jnp.abs(r[0:8]), 0.0))
                r = r.astype(BF16)
                if pre:
                    r = jnp.concatenate([r[:2 * M], qh_s[hd, pl.ds(qrow, SEG), :], r[2 * M:]], axis=0)
                res[t][j] = r
            return res

        def probs(qkv):
            scs = [lax.dot_general(qkv[0][j], qkv[1][j], (((1,), (1,)), ((), ())),
                                   preferred_element_type=F32) for j in range(HG)]
            ps = []
            for sc in scs:
                sc = jnp.where(vis, sc * scale, fill)
                e = jnp.exp(sc - jnp.max(sc, axis=-1, keepdims=True))
                den = jnp.sum(e, axis=-1, keepdims=True)
                r = pl.reciprocal(den, approx=True)
                r = r * (2.0 - den * r)
                ps.append((e * r).astype(BF16))
            return ps

        def oproj(os_, h0):
            oc = jnp.concatenate(os_, axis=1)
            k0, k1 = h0 * DH, (h0 + len(os_)) * DH
            return [jnp.dot(oc, wo_s[k0:k1, n * 128:(n + 1) * 128], preferred_element_type=F32)
                    for n in range(NLB)]

        heads = []
        qkv = proj(0)
        oa = None
        for g in range(NG):
            ps = probs(qkv)
            vs = qkv[2]
            if g + 1 < NG:
                qkv = proj(g + 1)
            else:
                if before_oproj is not None:
                    before_oproj()
                oa = oproj(heads[:H // 2], 0)
            heads += [jnp.dot(ps[j], vs[j], preferred_element_type=F32).astype(BF16)
                      for j in range(HG)]
        assert early is None or not units
        ob = oproj(heads[H // 2:], H // 2)
        return jnp.concatenate([b + a for a, b in zip(oa, ob)], axis=1)

    def post2(s):
        r3 = seg_row(s - 1 - LAG)
        xo = gate(_r(x2_s[(s + 4 - 1 - LAG) % 4] + obuf[SEG:2 * SEG, :]), r3)
        out_s[pl.ds(r3, SEG), :] = xo.astype(BF16)

    def step(s, mode, vis, fill, chained=False, before_oproj=None, early=None):
        if mode == 0:
            h = hbuf[...]
        elif mode == 1:
            h = hbuf[0:48, :]
        else:
            h = jnp.concatenate([hbuf[0:16, :], hbuf[48:80, :]], axis=0)
        last = isinstance(s, int) and s == NSEG + LAG - 1
        if last:
            post2(s)
            obuf[SEG:2 * SEG, :] = _r(attention(h, vis, fill, chained))
            return
        r1 = seg_row(s - 1)
        xb2 = _r(gate(_r(x_s[pl.ds(r1, SEG), :].astype(F32) + obuf[0:SEG, :]), r1))
        h2n = _ln(xb2).astype(BF16)
        if mode != 1:
            post2(s)
        x2_s[(s + 4 - 1) % 4] = xb2
        if mode != 2:
            h1n = _ln(x_s[pl.ds(seg_row(s + 1), SEG), :].astype(F32)).astype(BF16)

        o = attention(h, vis, fill, chained, before_oproj, early)

        mem2 = mem0 if mode == 1 else o[M:2 * M]
        hbuf[0:16, :] = jnp.concatenate([o[0:M], mem2], axis=0).astype(BF16)
        if mode != 2:
            hbuf[16:48, :] = h1n
        hbuf[48:80, :] = h2n
        if mode == 0:
            obuf[...] = _r(o[2 * M:])
        elif mode == 1:
            obuf[0:SEG, :] = _r(o[2 * M:])
        else:
            obuf[SEG:2 * SEG, :] = _r(o[2 * M:])

    with jax.named_scope("pro"):
        vis, fill = masks(1)
        step(0, 1, vis, fill, False, wo_copy.wait)
        step(1, 1, vis, fill, True)
    xb_copy.wait()
    vis, fill = masks(0)
    with jax.named_scope("main_a"):
        loop(NA, lambda i: step(i + LAG, 0, vis, fill, early=i))
    with jax.named_scope("conv_e"):
        loop(HB // 2, lambda j: (inv_stage(HB + 2 * j), inv_stage(HB + 2 * j + 1)))
    with jax.named_scope("main_b"):
        loop(NSEG - LAG - NA, lambda i: step(i + LAG + NA, 0, vis, fill))
    done = (NSEG - 1 - LAG) * SEG
    out_a = pltpu.make_async_copy(out_s.at[0:done, :], out_hbm.at[0:done, :], sem_x.at[1])
    out_a.start()
    with jax.named_scope("epi"):
        vis, fill = masks(2)
        step(NSEG, 2, vis, fill)
        step(NSEG + 1, 2, *masks(2, 2 * M), True)
    post2(NSEG + LAG)
    out_b = pltpu.make_async_copy(out_s.at[done:S, :], out_hbm.at[done:S, :], sem_x.at[2])
    out_b.start()
    out_a.wait()
    out_b.wait()


@jax.jit
def pallas_interleave_layers__memory_aug_recurrent_mem_tr__ssm_conv_h3__prompt_kernel(
    A_x, A_mem0, A_Wq, A_Wk, A_Wv, A_Wo, A_seg_len,
    B_q, B_k, B_v, B_shift_k, B_ssm_k, B_ssm_D,
):
    del A_seg_len, B_q
    assert A_x.shape == (1, S, D) and A_Wq.shape == (D, H, DH)
    vm = pl.BlockSpec(memory_space=pltpu.VMEM)
    hbm = pl.BlockSpec(memory_space=pl.ANY)
    out = pl.pallas_call(
        _kernel,
        out_shape=jax.ShapeDtypeStruct((S, D), BF16),
        in_specs=[hbm, vm, hbm, hbm, hbm, hbm, hbm, hbm, vm, hbm, vm],
        out_specs=hbm,
        scratch_shapes=[
            pltpu.VMEM((S, D), BF16),
            pltpu.VMEM((S, D), BF16),
            pltpu.VMEM((S, D), BF16),
            pltpu.VMEM((NB, D, TB), BF16),
            pltpu.VMEM((3, D, H, DH), BF16),
            pltpu.VMEM(((3 * H + 1) * WP, 128), U32),
            pltpu.VMEM((H * DH, D), BF16),
            pltpu.VMEM((TB, TB), BF16),
            pltpu.VMEM((2, TB, TB), BF16),
            pltpu.VMEM((2, TB // 2, 3 * TB), BF16),
            pltpu.VMEM((2, NLB, S // 2 + 8, 128), F32),
            pltpu.VMEM((NB, 2, NLB * TB, 128), F32),
            pltpu.VMEM((NB, 3, NLB * TB, 128), F32),
            pltpu.VMEM((NB + 1, 2, NLB * TB, 128), F32),
            pltpu.VMEM((NLB, S + 8, 128), F32),
            pltpu.VMEM((ROWS, D), BF16),
            pltpu.VMEM((2 * SEG, D), F32),
            pltpu.VMEM((4, SEG, D), F32),
            pltpu.VMEM((S, D), BF16),
            pltpu.VMEM((NA * SEG, D), BF16),
            pltpu.VMEM((NQH, NA * SEG, DH), BF16),
            pltpu.SemaphoreType.DMA((3 * (NB // 2) + 1,)),
            pltpu.SemaphoreType.DMA((4,)),
            pltpu.SemaphoreType.DMA((4,)),
        ],
        compiler_params=pltpu.CompilerParams(vmem_limit_bytes=120 * 1024 * 1024),
    )(A_x.reshape(S, D), A_mem0.reshape(M, D), A_Wq, A_Wk, A_Wv,
      A_Wo.reshape(H * DH, D), B_k.reshape(S, D), B_v.reshape(S, D),
      B_shift_k.T, B_ssm_k, B_ssm_D)
    return out.reshape(1, S, D)
```

```python
import functools
import math

import jax
import jax.numpy as jnp
from jax import lax
import jax.experimental.pallas as pl
import jax.experimental.pallas.tpu as pltpu

F32 = jnp.float32
BF16 = jnp.bfloat16
U32 = jnp.uint32

S = 2048
D = 640
H = 32
DH = 128
M = 8
SEG = 32
NSEG = S // SEG
KS = 4
LAG = 2
ROWS = 2 * M + 2 * SEG
HG = 4
NG = H // HG
NLB = D // 128
TB = 128
NB = S // TB
HB = NB // 2
NPOS = NLB * TB // 8
NA = 28
PPS = 3
UCUT = (range(0, 3), range(3, 6), range(6, 9), range(9, 16))
TOKP = (2, 1)
NQH = 16
WP = 324


def _ln(x):
    m = jnp.mean(x, axis=-1, keepdims=True)
    c = x - m
    v = jnp.mean(c * c, axis=-1, keepdims=True)
    return c * lax.rsqrt(v + 1e-5)


def _r(x):
    return x.astype(BF16).astype(F32)


def _split(x):
    hi = pltpu.bitcast(pltpu.bitcast(x, U32) & jnp.uint32(0xFFFF0000), F32)
    return hi, x - hi


def _bf(x):
    return jnp.concatenate([x[:, g:g + 128].astype(BF16)
                            for g in range(0, x.shape[1], 128)], axis=1)


def _basis(r, t):
    b = r & 63
    f = jnp.where(b < 32, 2 * b, 2 * b - 63)
    n = ((2 * f + 1) * t - jnp.where(r >= 64, TB, 0)) & (4 * TB - 1)
    n = jnp.where(n >= 2 * TB, n - 4 * TB, n)
    return jnp.cos(n.astype(F32) * (2.0 * math.pi / (4 * TB)))


def _halves(x):
    w = pltpu.bitcast(x, U32)
    return (pltpu.bitcast(w << 16, F32),
            pltpu.bitcast(w & jnp.uint32(0xFFFF0000), F32))


def _kernel(x_hbm, mem0_ref, wq_hbm, wk_hbm, wv_hbm, wo_hbm,
            k_hbm, v_hbm, shk_ref, ssmk_hbm, ssmd_ref,
            out_hbm,
            x_s, k_s, v_s, ssmk_s, wraw, wt, wo_s,
            perm_s, fu_s, inv_s, kpad, u_s, kf_s, c_s, y_s,
            hbuf, obuf, x2_s, out_s, hl_s, qh_s,
            sem_c, sem_w, sem_x):
    XH = (LAG + NA) * SEG

    def conv_copies(j):
        r0 = j * TB if isinstance(j, int) else pl.multiple_of(j * TB, TB)
        return (
            pltpu.make_async_copy(ssmk_hbm.at[:, pl.ds(r0, TB)], ssmk_s.at[j], sem_c.at[j]),
            pltpu.make_async_copy(k_hbm.at[pl.ds(r0, TB), :], k_s.at[pl.ds(r0, TB), :], sem_c.at[HB + j]),
            pltpu.make_async_copy(v_hbm.at[pl.ds(r0, TB), :], v_s.at[pl.ds(r0, TB), :], sem_c.at[NB + j]),
        )
    late_copies = [pltpu.make_async_copy(ssmk_hbm.at[:, pl.ds(j * TB, TB)], ssmk_s.at[j], sem_c.at[3 * HB])
                   for j in range(HB, NB)]
    late_copies += [pltpu.make_async_copy(src.at[S // 2:, :], dst.at[S // 2:, :], sem_c.at[3 * HB])
                    for src, dst in ((k_hbm, k_s), (v_hbm, v_s))]
    w_copies = [pltpu.make_async_copy(w, wraw.at[t], sem_w.at[t])
                for t, w in enumerate((wq_hbm, wk_hbm, wv_hbm))]
    wo_copy = pltpu.make_async_copy(wo_hbm, wo_s, sem_w.at[3])
    xa_copy = pltpu.make_async_copy(x_hbm.at[0:XH, :], x_s.at[0:XH, :], sem_x.at[0])
    xb_copy = pltpu.make_async_copy(x_hbm.at[XH:, :], x_s.at[XH:, :], sem_x.at[3])
    for j in range(HB):
        for c in conv_copies(j):
            c.start()
    for c in late_copies:
        c.start()
    xa_copy.start()
    wo_copy.start(priority=1)
    xb_copy.start(priority=1)

    hb = TB // 2
    ri = lax.broadcasted_iota(jnp.int32, (TB, TB), 0)
    ci = lax.broadcasted_iota(jnp.int32, (TB, TB), 1)
    perm_s[...] = jnp.where(ci == 2 * (ri & 63) + (ri >> 6), 1.0, 0.0).astype(BF16)
    tab = _basis(ri, 2 * (ci & 63) + (ci >> 6))
    hi, lo = _split(tab)
    fu_s[0] = jnp.where(ci < hb, hi, pltpu.roll(lo, hb, 1)).astype(BF16)
    fu_s[1] = jnp.where(ci < hb, pltpu.roll(hi, hb, 1), lo).astype(BF16)
    gh, gl = _split(tab.T * (1.0 / TB))
    ginv = _bf(jnp.concatenate([gh, gl, gh], axis=1))
    inv_s[0] = ginv[:hb]
    inv_s[1] = ginv[hb:]

    shk_t = shk_ref[...].astype(F32)
    taps = [[shk_t[j:j + 1, g * 128:(g + 1) * 128] for g in range(NLB)] for j in range(KS)]
    dvec = ssmd_ref[...].astype(F32).reshape(1, D)
    for g in range(NLB):
        kpad[0, g, 0:8, :] = jnp.zeros((8, 128), F32)
        kpad[1, g, 0:8, :] = jnp.zeros((8, 128), F32)
    c_s[0] = jnp.zeros(c_s.shape[1:], F32)

    def spectrum(e, o):
        fe = jnp.dot(fu_s[0], jnp.concatenate([e, e], axis=0).astype(BF16), preferred_element_type=F32)
        fo = jnp.dot(fu_s[1], jnp.concatenate([o, o], axis=0).astype(BF16), preferred_element_type=F32)
        return ((fe[:hb] + fo[:hb], fe[hb:] + fo[hb:]), (fe[:hb] - fo[:hb], fo[hb:] - fe[hb:]))

    def fwd_stage(js, first):
        if first:
            for j in js:
                for c in conv_copies(j):
                    c.wait()
        kts = [lax.dot_general(perm_s[...], ssmk_s[j], (((1,), (1,)), ((), ())),
                               preferred_element_type=F32) for j in js]
        for j, kt in zip(js, kts):
            r0 = pl.multiple_of(j * TB, TB)
            q0 = pl.multiple_of(j * hb, hb) + 8
            for g in range(NLB):
                lb = slice(g * 128, (g + 1) * 128)
                halves = (slice(g * TB, g * TB + hb), slice(g * TB + hb, (g + 1) * TB))
                for rows, (kr, ki) in zip(halves, spectrum(kt[:hb, lb], kt[hb:, lb])):
                    if first:
                        kr = kr + jnp.where(j == 0, dvec[:, lb], 0.0)
                    kf_s[j, 0, rows] = kr
                    kf_s[j, 1, rows] = ki - kr
                    kf_s[j, 2, rows] = kr + ki
                ke, ko = _halves(k_s[pl.ds(r0, TB), lb])
                ve, vo = _halves(v_s[pl.ds(r0, TB), lb])
                kpad[0, g, pl.ds(q0, hb), :] = ke
                kpad[1, g, pl.ds(q0, hb), :] = ko
                ke1 = kpad[0, g, pl.ds(q0 - 1, hb), :]
                ko1 = kpad[1, g, pl.ds(q0 - 1, hb), :]
                ko2 = kpad[1, g, pl.ds(q0 - 2, hb), :]
                t0, t1, t2, t3 = (taps[t][g] for t in range(KS))
                e = (ke * t0 + ko1 * t1 + ke1 * t2 + ko2 * t3) * ve
                o = (ko * t0 + ke * t1 + ko1 * t2 + ke1 * t3) * vo
                for rows, (ur, ui) in zip(halves, spectrum(e, o)):
                    u_s[j, 0, rows] = ur
                    u_s[j, 1, rows] = ui

    def mac_units(pos, half):
        rs = pl.ds(pl.multiple_of(pos * 8, 8), 8)
        state = {}

        def unit(p, avals, final, tok=None):
            acc = state.setdefault(p, dict(state.get(0, {})))
            for a in avals:
                u = u_s[a, 0, rs] + u_s[a, 1, rs] if p == 0 else u_s[a, p - 1, rs]
                if tok is not None:
                    u = u + tok
                for i in range(max(a, half * HB), half * HB + HB):
                    t = u * kf_s[i - a, p, rs]
                    acc[i] = t if i not in acc else (acc[i] - t if p == 2 else acc[i] + t)
            if final and p:
                for i, v in acc.items():
                    c_s[i + 1, 2 - p, rs] = v

        subs = UCUT if half else (range(HB),)
        return [functools.partial(unit, p, avals, n == len(subs) - 1)
                for p in range(3) for n, avals in enumerate(subs)]

    def inv_stage(i):
        q = TB // 4
        for g in range(NLB):
            re, im = [], []
            for b in range(4):
                rows = slice(g * TB + b * q, g * TB + (b + 1) * q)
                cr, ci_ = c_s[i + 1, 0, rows], c_s[i + 1, 1, rows]
                pr, pi = c_s[i, 0, rows], c_s[i, 1, rows]
                re.append(cr + pi if b in (0, 3) else cr - pi)
                im.append(ci_ - pr if b in (0, 3) else ci_ + pr)
            pe = jnp.concatenate([re[0] + re[2], re[1] + re[3], im[0] - im[2], im[1] - im[3]], axis=0)
            po = jnp.concatenate([re[0] - re[2], re[1] - re[3], im[0] + im[2], im[1] + im[3]], axis=0)
            for par, pp in enumerate((pe, po)):
                ph, plo = _split(pp)
                y_s[g, pl.ds(i * TB + par, hb, stride=2), :] = jnp.dot(
                    inv_s[par], jnp.concatenate([ph, ph, plo], axis=0).astype(BF16),
                    preferred_element_type=F32)

    def relayout(t):
        w_copies[t].wait()

        def body(i, _):
            for dd in range(32):
                dp = i * 32 + dd
                a = pltpu.bitcast(wraw[t, 2 * dp], U32)
                b = pltpu.bitcast(wraw[t, 2 * dp + 1], U32)
                lo = (a & jnp.uint32(0xFFFF)) | (b << 16)
                hi = (a >> 16) | (b & jnp.uint32(0xFFFF0000))
                wt[pl.ds(t * H * WP + dp, 16, stride=WP), :] = lo
                wt[pl.ds((t * H + 16) * WP + dp, 16, stride=WP), :] = hi
            return 0
        lax.fori_loop(0, D // 64, body, 0)

    def wslab(t, h):
        s0 = (t * H + (h % 2) * 16 + h // 2) * WP
        return pltpu.bitcast(wt[s0:s0 + D // 2, :], BF16)

    def loop(n, fn):
        def body(j, _):
            fn(j)
            return 0
        lax.fori_loop(0, n, body, 0)

    def norm_rows(c):
        r0 = c * TB if isinstance(c, int) else pl.multiple_of(c * TB, TB)
        hl_s[pl.ds(r0, TB), :] = _ln(x_s[pl.ds(r0 + LAG * SEG, TB), :].astype(F32)).astype(BF16)

    def pre_queries(c):
        for sub in range(2):
            r0 = pl.multiple_of((2 * c + sub) * QR, 16)
            hl = hl_s[pl.ds(r0, QR), :]
            for hd in range(NQH):
                qh_s[hd, pl.ds(r0, QR), :] = jnp.dot(
                    hl, wslab(0, hd), preferred_element_type=F32).astype(BF16)

    nch = NA * SEG // TB
    QR = NA * SEG // 8
    with jax.named_scope("conv_a"):
        loop(HB // 2, lambda j: fwd_stage((2 * j, 2 * j + 1), True))
    with jax.named_scope("conv_b"):
        for c in w_copies:
            c.start()
        loop(NPOS // 10, lambda j: [u() for n in range(10) for u in mac_units(10 * j + n, 0)])
        loop(HB // 2, lambda j: (inv_stage(2 * j), inv_stage(2 * j + 1)))
    with jax.named_scope("conv_c"):
        for c in late_copies:
            c.wait()
        loop(HB // 2, lambda j: fwd_stage((HB + 2 * j, HB + 2 * j + 1), False))
    with jax.named_scope("norm"):
        xa_copy.wait()
        norm_rows(0)
        loop(nch // 2, lambda c: (norm_rows(2 * c + 1), norm_rows(2 * c + 2)))
    with jax.named_scope("rel0"):
        relayout(0)
    with jax.named_scope("preq"):
        loop(4, pre_queries)
    with jax.named_scope("rel1"):
        relayout(1)
    with jax.named_scope("rel2"):
        relayout(2)

    scale = DH ** -0.5

    def masks(mode, q0=0):
        rows = ROWS if mode == 0 else ROWS - SEG
        qi = lax.broadcasted_iota(jnp.int32, (rows - q0, rows), 0) + q0
        kj = lax.broadcasted_iota(jnp.int32, (rows - q0, rows), 1)

        def layer_of(i):
            xl = (i - 2 * M) // SEG if mode == 0 else mode - 1
            return jnp.where(i < 2 * M, i // M, xl)
        same = layer_of(qi) == layer_of(kj)
        vis = same & ((qi < 2 * M) | (qi >= kj))
        fill = jnp.where(same, -1e9, -jnp.inf).astype(F32)
        return vis, fill

    mem0 = mem0_ref[...].astype(F32)
    hbuf[0:16, :] = jnp.concatenate([mem0, mem0], axis=0).astype(BF16)
    hbuf[16:48, :] = _ln(x_s[0:SEG, :].astype(F32)).astype(BF16)
    obuf[...] = jnp.zeros((2 * SEG, D), F32)
    x2_s[...] = jnp.zeros(x2_s.shape, F32)

    def seg_row(seg):
        if isinstance(seg, int):
            return min(max(seg, 0), NSEG - 1) * SEG
        return pl.multiple_of(jnp.clip(seg, 0, NSEG - 1) * SEG, SEG)

    def gate(xa, r0):
        y = jnp.concatenate([y_s[g, pl.ds(r0, SEG), :] for g in range(NLB)], axis=1)
        return xa + _r(_r(_ln(xa)) * y)

    def attention(h, vis, fill, chained, before_oproj=None, early=None):
        q0 = h.shape[0] - vis.shape[0]
        if early is not None:
            hrest = jnp.concatenate([h[:2 * M], h[2 * M + SEG:]], axis=0)
            qrow = pl.multiple_of(early * SEG, SEG)
            units = [u for n in range(PPS)
                     for u in mac_units(jnp.minimum(early * PPS + n, NPOS - 1), 1)]

        def proj(g):
            if g == 0 and chained and q0 == 0:
                kc = D - 128
                part = [jnp.dot(h[:, :kc], wslab(0, j)[:kc], preferred_element_type=F32)
                        for j in range(HG)]
                q = [(jnp.dot(h[:, kc:], wslab(0, j)[kc:], preferred_element_type=F32)
                      + part[j]).astype(BF16) for j in range(HG)]
                return [q] + [[jnp.dot(h, wslab(t, j), preferred_element_type=F32).astype(BF16)
                               for j in range(HG)] for t in range(1, 3)]
            res = [[None] * HG for _ in range(3)]
            order = [(t, j) for j in range(HG) for t in range(2)] + [(2, j) for j in range(HG)]
            for n, (t, j) in enumerate(order):
                hd = g * HG + j
                pre = early is not None and t == 0 and hd < NQH
                lhs = hrest if pre else (h if t else h[q0:])
                r = jnp.dot(lhs, wslab(t, hd), preferred_element_type=F32)
                if early is not None and n % TOKP[0] == TOKP[1] and units:
                    units.pop(0)(jnp.minimum(jnp.abs(r[0:8]), 0.0))
                r = r.astype(BF16)
                if pre:
                    r = jnp.concatenate([r[:2 * M], qh_s[hd, pl.ds(qrow, SEG), :], r[2 * M:]], axis=0)
                res[t][j] = r
            return res

        def probs(qkv):
            scs = [lax.dot_general(qkv[0][j], qkv[1][j], (((1,), (1,)), ((), ())),
                                   preferred_element_type=F32) for j in range(HG)]
            ps = []
            for sc in scs:
                sc = jnp.where(vis, sc * scale, fill)
                e = jnp.exp(sc - jnp.max(sc, axis=-1, keepdims=True))
                den = jnp.sum(e, axis=-1, keepdims=True)
                r = pl.reciprocal(den, approx=True)
                r = r * (2.0 - den * r)
                ps.append((e * r).astype(BF16))
            return ps

        def oproj(os_, h0):
            oc = jnp.concatenate(os_, axis=1)
            k0, k1 = h0 * DH, (h0 + len(os_)) * DH
            return [jnp.dot(oc, wo_s[k0:k1, n * 128:(n + 1) * 128], preferred_element_type=F32)
                    for n in range(NLB)]

        heads = []
        qkv = proj(0)
        oa = None
        for g in range(NG):
            ps = probs(qkv)
            vs = qkv[2]
            if g + 1 < NG:
                qkv = proj(g + 1)
            else:
                if before_oproj is not None:
                    before_oproj()
                oa = oproj(heads[:H // 2], 0)
            heads += [jnp.dot(ps[j], vs[j], preferred_element_type=F32).astype(BF16)
                      for j in range(HG)]
        assert early is None or not units
        ob = oproj(heads[H // 2:], H // 2)
        return jnp.concatenate([b + a for a, b in zip(oa, ob)], axis=1)

    def post2(s):
        r3 = seg_row(s - 1 - LAG)
        xo = gate(_r(x2_s[(s + 4 - 1 - LAG) % 4] + obuf[SEG:2 * SEG, :]), r3)
        out_s[pl.ds(r3, SEG), :] = xo.astype(BF16)

    def step(s, mode, vis, fill, chained=False, before_oproj=None, early=None):
        if mode == 0:
            h = hbuf[...]
        elif mode == 1:
            h = hbuf[0:48, :]
        else:
            h = jnp.concatenate([hbuf[0:16, :], hbuf[48:80, :]], axis=0)
        last = isinstance(s, int) and s == NSEG + LAG - 1
        if last:
            post2(s)
            obuf[SEG:2 * SEG, :] = _r(attention(h, vis, fill, chained))
            return
        r1 = seg_row(s - 1)
        xb2 = _r(gate(_r(x_s[pl.ds(r1, SEG), :].astype(F32) + obuf[0:SEG, :]), r1))
        h2n = _ln(xb2).astype(BF16)
        if mode != 1:
            post2(s)
        x2_s[(s + 4 - 1) % 4] = xb2
        if mode != 2:
            h1n = _ln(x_s[pl.ds(seg_row(s + 1), SEG), :].astype(F32)).astype(BF16)

        o = attention(h, vis, fill, chained, before_oproj, early)

        mem2 = mem0 if mode == 1 else o[M:2 * M]
        hbuf[0:16, :] = jnp.concatenate([o[0:M], mem2], axis=0).astype(BF16)
        if mode != 2:
            hbuf[16:48, :] = h1n
        hbuf[48:80, :] = h2n
        if mode == 0:
            obuf[...] = _r(o[2 * M:])
        elif mode == 1:
            obuf[0:SEG, :] = _r(o[2 * M:])
        else:
            obuf[SEG:2 * SEG, :] = _r(o[2 * M:])

    with jax.named_scope("pro"):
        vis, fill = masks(1)
        step(0, 1, vis, fill, False, wo_copy.wait)
        step(1, 1, vis, fill, True)
    xb_copy.wait()
    vis, fill = masks(0)
    with jax.named_scope("main_a"):
        loop(NA, lambda i: step(i + LAG, 0, vis, fill, early=i))
    with jax.named_scope("conv_e"):
        loop(HB // 2, lambda j: (inv_stage(HB + 2 * j), inv_stage(HB + 2 * j + 1)))
    with jax.named_scope("main_b"):
        loop(NSEG - LAG - NA, lambda i: step(i + LAG + NA, 0, vis, fill))
    done = (NSEG - 1 - LAG) * SEG
    out_a = pltpu.make_async_copy(out_s.at[0:done, :], out_hbm.at[0:done, :], sem_x.at[1])
    out_a.start()
    with jax.named_scope("epi"):
        vis, fill = masks(2)
        step(NSEG, 2, vis, fill)
        step(NSEG + 1, 2, *masks(2, 2 * M), True)
    post2(NSEG + LAG)
    out_b = pltpu.make_async_copy(out_s.at[done:S, :], out_hbm.at[done:S, :], sem_x.at[2])
    out_b.start()
    out_a.wait()
    out_b.wait()


@jax.jit
def pallas_interleave_layers__memory_aug_recurrent_mem_tr__ssm_conv_h3__prompt_kernel(
    A_x, A_mem0, A_Wq, A_Wk, A_Wv, A_Wo, A_seg_len,
    B_q, B_k, B_v, B_shift_k, B_ssm_k, B_ssm_D,
):
    del A_seg_len, B_q
    assert A_x.shape == (1, S, D) and A_Wq.shape == (D, H, DH)
    vm = pl.BlockSpec(memory_space=pltpu.VMEM)
    hbm = pl.BlockSpec(memory_space=pl.ANY)
    out = pl.pallas_call(
        _kernel,
        out_shape=jax.ShapeDtypeStruct((S, D), BF16),
        in_specs=[hbm, vm, hbm, hbm, hbm, hbm, hbm, hbm, vm, hbm, vm],
        out_specs=hbm,
        scratch_shapes=[
            pltpu.VMEM((S, D), BF16),
            pltpu.VMEM((S, D), BF16),
            pltpu.VMEM((S, D), BF16),
            pltpu.VMEM((NB, D, TB), BF16),
            pltpu.VMEM((3, D, H, DH), BF16),
            pltpu.VMEM(((3 * H + 1) * WP, 128), U32),
            pltpu.VMEM((H * DH, D), BF16),
            pltpu.VMEM((TB, TB), BF16),
            pltpu.VMEM((2, TB, TB), BF16),
            pltpu.VMEM((2, TB // 2, 3 * TB), BF16),
            pltpu.VMEM((2, NLB, S // 2 + 8, 128), F32),
            pltpu.VMEM((NB, 2, NLB * TB, 128), F32),
            pltpu.VMEM((NB, 3, NLB * TB, 128), F32),
            pltpu.VMEM((NB + 1, 2, NLB * TB, 128), F32),
            pltpu.VMEM((NLB, S + 8, 128), F32),
            pltpu.VMEM((ROWS, D), BF16),
            pltpu.VMEM((2 * SEG, D), F32),
            pltpu.VMEM((4, SEG, D), F32),
            pltpu.VMEM((S, D), BF16),
            pltpu.VMEM((NA * SEG, D), BF16),
            pltpu.VMEM((NQH, NA * SEG, DH), BF16),
            pltpu.SemaphoreType.DMA((3 * (NB // 2) + 1,)),
            pltpu.SemaphoreType.DMA((4,)),
            pltpu.SemaphoreType.DMA((4,)),
        ],
        compiler_params=pltpu.CompilerParams(vmem_limit_bytes=120 * 1024 * 1024),
    )(A_x.reshape(S, D), A_mem0.reshape(M, D), A_Wq, A_Wk, A_Wv,
      A_Wo.reshape(H * DH, D), B_k.reshape(S, D), B_v.reshape(S, D),
      B_shift_k.T, B_ssm_k, B_ssm_D)
    return out.reshape(1, S, D)
```

```python
import functools
import math

import jax
import jax.numpy as jnp
from jax import lax
import jax.experimental.pallas as pl
import jax.experimental.pallas.tpu as pltpu

F32 = jnp.float32
BF16 = jnp.bfloat16
U32 = jnp.uint32

S = 2048
D = 640
H = 32
DH = 128
M = 8
SEG = 32
NSEG = S // SEG
KS = 4
LAG = 2
ROWS = 2 * M + 2 * SEG
HG = 4
NG = H // HG
NLB = D // 128
TB = 128
NB = S // TB
HB = NB // 2
NPOS = NLB * TB // 8
NA = 20
PPS = 4
UCUT = (range(0, 3), range(3, 6), range(6, 9), range(9, 16))
TOKP = (2, 1)
NQH = 22
WP = 324


def _ln(x):
    m = jnp.mean(x, axis=-1, keepdims=True)
    c = x - m
    v = jnp.mean(c * c, axis=-1, keepdims=True)
    return c * lax.rsqrt(v + 1e-5)


def _r(x):
    return x.astype(BF16).astype(F32)


def _split(x):
    hi = pltpu.bitcast(pltpu.bitcast(x, U32) & jnp.uint32(0xFFFF0000), F32)
    return hi, x - hi


def _bf(x):
    return jnp.concatenate([x[:, g:g + 128].astype(BF16)
                            for g in range(0, x.shape[1], 128)], axis=1)


def _basis(r, t):
    b = r & 63
    f = jnp.where(b < 32, 2 * b, 2 * b - 63)
    n = ((2 * f + 1) * t - jnp.where(r >= 64, TB, 0)) & (4 * TB - 1)
    n = jnp.where(n >= 2 * TB, n - 4 * TB, n)
    return jnp.cos(n.astype(F32) * (2.0 * math.pi / (4 * TB)))


def _halves(x):
    w = pltpu.bitcast(x, U32)
    return (pltpu.bitcast(w << 16, F32),
            pltpu.bitcast(w & jnp.uint32(0xFFFF0000), F32))


def _kernel(x_hbm, mem0_ref, wq_hbm, wk_hbm, wv_hbm, wo_hbm,
            k_hbm, v_hbm, shk_ref, ssmk_hbm, ssmd_ref,
            out_hbm,
            x_s, k_s, v_s, ssmk_s, wraw, wt, wo_s,
            perm_s, fu_s, inv_s, kpad, u_s, kf_s, c_s, y_s,
            hbuf, obuf, x2_s, out_s, hl_s, qh_s,
            sem_c, sem_w, sem_x):
    XH = (LAG + NA) * SEG

    def conv_copies(j):
        r0 = j * TB if isinstance(j, int) else pl.multiple_of(j * TB, TB)
        return (
            pltpu.make_async_copy(ssmk_hbm.at[:, pl.ds(r0, TB)], ssmk_s.at[j], sem_c.at[j]),
            pltpu.make_async_copy(k_hbm.at[pl.ds(r0, TB), :], k_s.at[pl.ds(r0, TB), :], sem_c.at[HB + j]),
            pltpu.make_async_copy(v_hbm.at[pl.ds(r0, TB), :], v_s.at[pl.ds(r0, TB), :], sem_c.at[NB + j]),
        )
    late_copies = [pltpu.make_async_copy(ssmk_hbm.at[:, pl.ds(j * TB, TB)], ssmk_s.at[j], sem_c.at[3 * HB])
                   for j in range(HB, NB)]
    late_copies += [pltpu.make_async_copy(src.at[S // 2:, :], dst.at[S // 2:, :], sem_c.at[3 * HB])
                    for src, dst in ((k_hbm, k_s), (v_hbm, v_s))]
    w_copies = [pltpu.make_async_copy(w, wraw.at[t], sem_w.at[t])
                for t, w in enumerate((wq_hbm, wk_hbm, wv_hbm))]
    wo_copy = pltpu.make_async_copy(wo_hbm, wo_s, sem_w.at[3])
    xa_copy = pltpu.make_async_copy(x_hbm.at[0:XH, :], x_s.at[0:XH, :], sem_x.at[0])
    xb_copy = pltpu.make_async_copy(x_hbm.at[XH:, :], x_s.at[XH:, :], sem_x.at[3])
    for j in range(HB):
        for c in conv_copies(j):
            c.start()
    for c in late_copies:
        c.start()
    xa_copy.start()
    wo_copy.start(priority=1)
    xb_copy.start(priority=1)

    hb = TB // 2
    ri = lax.broadcasted_iota(jnp.int32, (TB, TB), 0)
    ci = lax.broadcasted_iota(jnp.int32, (TB, TB), 1)
    perm_s[...] = jnp.where(ci == 2 * (ri & 63) + (ri >> 6), 1.0, 0.0).astype(BF16)
    tab = _basis(ri, 2 * (ci & 63) + (ci >> 6))
    hi, lo = _split(tab)
    fu_s[0] = jnp.where(ci < hb, hi, pltpu.roll(lo, hb, 1)).astype(BF16)
    fu_s[1] = jnp.where(ci < hb, pltpu.roll(hi, hb, 1), lo).astype(BF16)
    gh, gl = _split(tab.T * (1.0 / TB))
    ginv = _bf(jnp.concatenate([gh, gl, gh], axis=1))
    inv_s[0] = ginv[:hb]
    inv_s[1] = ginv[hb:]

    shk_t = shk_ref[...].astype(F32)
    taps = [[shk_t[j:j + 1, g * 128:(g + 1) * 128] for g in range(NLB)] for j in range(KS)]
    dvec = ssmd_ref[...].astype(F32).reshape(1, D)
    for g in range(NLB):
        kpad[0, g, 0:8, :] = jnp.zeros((8, 128), F32)
        kpad[1, g, 0:8, :] = jnp.zeros((8, 128), F32)
    c_s[0] = jnp.zeros(c_s.shape[1:], F32)

    def spectrum(e, o):
        fe = jnp.dot(fu_s[0], jnp.concatenate([e, e], axis=0).astype(BF16), preferred_element_type=F32)
        fo = jnp.dot(fu_s[1], jnp.concatenate([o, o], axis=0).astype(BF16), preferred_element_type=F32)
        return ((fe[:hb] + fo[:hb], fe[hb:] + fo[hb:]), (fe[:hb] - fo[:hb], fo[hb:] - fe[hb:]))

    def fwd_stage(js, first):
        if first:
            for j in js:
                for c in conv_copies(j):
                    c.wait()
        kts = [lax.dot_general(perm_s[...], ssmk_s[j], (((1,), (1,)), ((), ())),
                               preferred_element_type=F32) for j in js]
        for j, kt in zip(js, kts):
            r0 = pl.multiple_of(j * TB, TB)
            q0 = pl.multiple_of(j * hb, hb) + 8
            for g in range(NLB):
                lb = slice(g * 128, (g + 1) * 128)
                halves = (slice(g * TB, g * TB + hb), slice(g * TB + hb, (g + 1) * TB))
                for rows, (kr, ki) in zip(halves, spectrum(kt[:hb, lb], kt[hb:, lb])):
                    if first:
                        kr = kr + jnp.where(j == 0, dvec[:, lb], 0.0)
                    kf_s[j, 0, rows] = kr
                    kf_s[j, 1, rows] = ki - kr
                    kf_s[j, 2, rows] = kr + ki
                ke, ko = _halves(k_s[pl.ds(r0, TB), lb])
                ve, vo = _halves(v_s[pl.ds(r0, TB), lb])
                kpad[0, g, pl.ds(q0, hb), :] = ke
                kpad[1, g, pl.ds(q0, hb), :] = ko
                ke1 = kpad[0, g, pl.ds(q0 - 1, hb), :]
                ko1 = kpad[1, g, pl.ds(q0 - 1, hb), :]
                ko2 = kpad[1, g, pl.ds(q0 - 2, hb), :]
                t0, t1, t2, t3 = (taps[t][g] for t in range(KS))
                e = (ke * t0 + ko1 * t1 + ke1 * t2 + ko2 * t3) * ve
                o = (ko * t0 + ke * t1 + ko1 * t2 + ke1 * t3) * vo
                for rows, (ur, ui) in zip(halves, spectrum(e, o)):
                    u_s[j, 0, rows] = ur
                    u_s[j, 1, rows] = ui

    def mac_units(row, half):
        rs = pl.ds(row, 8)
        state = {}

        def unit(p, avals, final, tok=None):
            acc = state.setdefault(p, dict(state.get(0, {})))
            for a in avals:
                u = u_s[a, 0, rs] + u_s[a, 1, rs] if p == 0 else u_s[a, p - 1, rs]
                if tok is not None:
                    u = u + tok
                for i in range(max(a, half * HB), half * HB + HB):
                    t = u * kf_s[i - a, p, rs]
                    acc[i] = t if i not in acc else (acc[i] - t if p == 2 else acc[i] + t)
            if final and p:
                for i, v in acc.items():
                    c_s[i + 1, 2 - p, rs] = v

        subs = UCUT if half else (range(HB),)
        return [functools.partial(unit, p, avals, n == len(subs) - 1)
                for p in range(3) for n, avals in enumerate(subs)]

    def inv_stage(i):
        q = TB // 4
        for g in range(NLB):
            re, im = [], []
            for b in range(4):
                rows = slice(g * TB + b * q, g * TB + (b + 1) * q)
                cr, ci_ = c_s[i + 1, 0, rows], c_s[i + 1, 1, rows]
                pr, pi = c_s[i, 0, rows], c_s[i, 1, rows]
                re.append(cr + pi if b in (0, 3) else cr - pi)
                im.append(ci_ - pr if b in (0, 3) else ci_ + pr)
            pe = jnp.concatenate([re[0] + re[2], re[1] + re[3], im[0] - im[2], im[1] - im[3]], axis=0)
            po = jnp.concatenate([re[0] - re[2], re[1] - re[3], im[0] + im[2], im[1] + im[3]], axis=0)
            for par, pp in enumerate((pe, po)):
                ph, plo = _split(pp)
                y_s[g, pl.ds(i * TB + par, hb, stride=2), :] = jnp.dot(
                    inv_s[par], jnp.concatenate([ph, ph, plo], axis=0).astype(BF16),
                    preferred_element_type=F32)

    def relayout(t):
        w_copies[t].wait()

        def body(i, _):
            for dd in range(32):
                dp = i * 32 + dd
                a = pltpu.bitcast(wraw[t, 2 * dp], U32)
                b = pltpu.bitcast(wraw[t, 2 * dp + 1], U32)
                lo = (a & jnp.uint32(0xFFFF)) | (b << 16)
                hi = (a >> 16) | (b & jnp.uint32(0xFFFF0000))
                wt[pl.ds(t * H * WP + dp, 16, stride=WP), :] = lo
                wt[pl.ds((t * H + 16) * WP + dp, 16, stride=WP), :] = hi
            return 0
        lax.fori_loop(0, D // 64, body, 0)

    def wslab(t, h):
        s0 = (t * H + (h % 2) * 16 + h // 2) * WP
        return pltpu.bitcast(wt[s0:s0 + D // 2, :], BF16)

    def loop(n, fn):
        def body(j, _):
            fn(j)
            return 0
        lax.fori_loop(0, n, body, 0)

    def norm_rows(c):
        r0 = c * TB if isinstance(c, int) else pl.multiple_of(c * TB, TB)
        hl_s[pl.ds(r0, TB), :] = _ln(x_s[pl.ds(r0 + LAG * SEG, TB), :].astype(F32)).astype(BF16)

    def pre_queries(c):
        for sub in range(2):
            r0 = pl.multiple_of((2 * c + sub) * QR, 16)
            hl = hl_s[pl.ds(r0, QR), :]
            for hd in range(NQH):
                qh_s[hd, pl.ds(r0, QR), :] = jnp.dot(
                    hl, wslab(0, hd), preferred_element_type=F32).astype(BF16)

    nch = NA * SEG // TB
    QR = NA * SEG // 8
    with jax.named_scope("conv_a"):
        loop(HB // 2, lambda j: fwd_stage((2 * j, 2 * j + 1), True))
    with jax.named_scope("conv_b"):
        for c in w_copies:
            c.start()
        loop(NPOS // 10, lambda j: [u() for n in range(10) for u in mac_units(pl.multiple_of(80 * j, 16) + 8 * n, 0)])
        loop(HB // 2, lambda j: (inv_stage(2 * j), inv_stage(2 * j + 1)))
    with jax.named_scope("conv_c"):
        for c in late_copies:
            c.wait()
        loop(HB // 2, lambda j: fwd_stage((HB + 2 * j, HB + 2 * j + 1), False))
    with jax.named_scope("norm"):
        xa_copy.wait()
        norm_rows(0)
        loop(nch // 2, lambda c: (norm_rows(2 * c + 1), norm_rows(2 * c + 2)))
    with jax.named_scope("rel0"):
        relayout(0)
    with jax.named_scope("preq"):
        loop(4, pre_queries)
    with jax.named_scope("rel1"):
        relayout(1)
    with jax.named_scope("rel2"):
        relayout(2)

    scale = DH ** -0.5

    def masks(mode, q0=0):
        rows = ROWS if mode == 0 else ROWS - SEG
        qi = lax.broadcasted_iota(jnp.int32, (rows - q0, rows), 0) + q0
        kj = lax.broadcasted_iota(jnp.int32, (rows - q0, rows), 1)

        def layer_of(i):
            xl = (i - 2 * M) // SEG if mode == 0 else mode - 1
            return jnp.where(i < 2 * M, i // M, xl)
        same = layer_of(qi) == layer_of(kj)
        vis = same & ((qi < 2 * M) | (qi >= kj))
        fill = jnp.where(same, -1e9, -jnp.inf).astype(F32)
        return vis, fill

    mem0 = mem0_ref[...].astype(F32)
    hbuf[0:16, :] = jnp.concatenate([mem0, mem0], axis=0).astype(BF16)
    hbuf[16:48, :] = _ln(x_s[0:SEG, :].astype(F32)).astype(BF16)
    obuf[...] = jnp.zeros((2 * SEG, D), F32)
    x2_s[...] = jnp.zeros(x2_s.shape, F32)

    def seg_row(seg):
        if isinstance(seg, int):
            return min(max(seg, 0), NSEG - 1) * SEG
        return pl.multiple_of(jnp.clip(seg, 0, NSEG - 1) * SEG, SEG)

    def gate(xa, r0):
        y = jnp.concatenate([y_s[g, pl.ds(r0, SEG), :] for g in range(NLB)], axis=1)
        return xa + _r(_r(_ln(xa)) * y)

    def attention(h, vis, fill, chained, before_oproj=None, early=None):
        q0 = h.shape[0] - vis.shape[0]
        if early is not None:
            hrest = jnp.concatenate([h[:2 * M], h[2 * M + SEG:]], axis=0)
            qrow = pl.multiple_of(early * SEG, SEG)
            units = [u for n in range(PPS)
                     for u in mac_units(pl.multiple_of(early * (8 * PPS), 8 * PPS) + 8 * n, 1)]

        def proj(g):
            if g == 0 and chained and q0 == 0:
                kc = D - 128
                part = [jnp.dot(h[:, :kc], wslab(0, j)[:kc], preferred_element_type=F32)
                        for j in range(HG)]
                q = [(jnp.dot(h[:, kc:], wslab(0, j)[kc:], preferred_element_type=F32)
                      + part[j]).astype(BF16) for j in range(HG)]
                return [q] + [[jnp.dot(h, wslab(t, j), preferred_element_type=F32).astype(BF16)
                               for j in range(HG)] for t in range(1, 3)]
            res = [[None] * HG for _ in range(3)]
            order = [(t, j) for j in range(HG) for t in range(2)] + [(2, j) for j in range(HG)]
            for n, (t, j) in enumerate(order):
                hd = g * HG + j
                pre = early is not None and t == 0 and hd < NQH
                lhs = hrest if pre else (h if t else h[q0:])
                r = jnp.dot(lhs, wslab(t, hd), preferred_element_type=F32)
                if early is not None and n % TOKP[0] == TOKP[1] and units:
                    units.pop(0)(jnp.minimum(jnp.abs(r[0:8]), 0.0))
                r = r.astype(BF16)
                if pre:
                    r = jnp.concatenate([r[:2 * M], qh_s[hd, pl.ds(qrow, SEG), :], r[2 * M:]], axis=0)
                res[t][j] = r
            return res

        def probs(qkv):
            scs = [lax.dot_general(qkv[0][j], qkv[1][j], (((1,), (1,)), ((), ())),
                                   preferred_element_type=F32) for j in range(HG)]
            ps = []
            for sc in scs:
                sc = jnp.where(vis, sc * scale, fill)
                e = jnp.exp(sc - jnp.max(sc, axis=-1, keepdims=True))
                den = jnp.sum(e, axis=-1, keepdims=True)
                r = pl.reciprocal(den, approx=True)
                r = r * (2.0 - den * r)
                ps.append((e * r).astype(BF16))
            return ps

        def oproj(os_, h0):
            oc = jnp.concatenate(os_, axis=1)
            k0, k1 = h0 * DH, (h0 + len(os_)) * DH
            return [jnp.dot(oc, wo_s[k0:k1, n * 128:(n + 1) * 128], preferred_element_type=F32)
                    for n in range(NLB)]

        heads = []
        qkv = proj(0)
        oa = None
        for g in range(NG):
            ps = probs(qkv)
            vs = qkv[2]
            if g + 1 < NG:
                qkv = proj(g + 1)
            else:
                if before_oproj is not None:
                    before_oproj()
                oa = oproj(heads[:H // 2], 0)
            heads += [jnp.dot(ps[j], vs[j], preferred_element_type=F32).astype(BF16)
                      for j in range(HG)]
        assert early is None or not units
        ob = oproj(heads[H // 2:], H // 2)
        return jnp.concatenate([b + a for a, b in zip(oa, ob)], axis=1)

    def post2(s):
        r3 = seg_row(s - 1 - LAG)
        xo = gate(_r(x2_s[(s + 4 - 1 - LAG) % 4] + obuf[SEG:2 * SEG, :]), r3)
        out_s[pl.ds(r3, SEG), :] = xo.astype(BF16)

    def step(s, mode, vis, fill, chained=False, before_oproj=None, early=None):
        if mode == 0:
            h = hbuf[...]
        elif mode == 1:
            h = hbuf[0:48, :]
        else:
            h = jnp.concatenate([hbuf[0:16, :], hbuf[48:80, :]], axis=0)
        last = isinstance(s, int) and s == NSEG + LAG - 1
        if last:
            post2(s)
            obuf[SEG:2 * SEG, :] = _r(attention(h, vis, fill, chained))
            return
        r1 = seg_row(s - 1)
        xb2 = _r(gate(_r(x_s[pl.ds(r1, SEG), :].astype(F32) + obuf[0:SEG, :]), r1))
        h2n = _ln(xb2).astype(BF16)
        if mode != 1:
            post2(s)
        x2_s[(s + 4 - 1) % 4] = xb2
        if mode != 2:
            h1n = _ln(x_s[pl.ds(seg_row(s + 1), SEG), :].astype(F32)).astype(BF16)

        o = attention(h, vis, fill, chained, before_oproj, early)

        mem2 = mem0 if mode == 1 else o[M:2 * M]
        hbuf[0:16, :] = jnp.concatenate([o[0:M], mem2], axis=0).astype(BF16)
        if mode != 2:
            hbuf[16:48, :] = h1n
        hbuf[48:80, :] = h2n
        if mode == 0:
            obuf[...] = _r(o[2 * M:])
        elif mode == 1:
            obuf[0:SEG, :] = _r(o[2 * M:])
        else:
            obuf[SEG:2 * SEG, :] = _r(o[2 * M:])

    with jax.named_scope("pro"):
        vis, fill = masks(1)
        step(0, 1, vis, fill, False, wo_copy.wait)
        step(1, 1, vis, fill, True)
    xb_copy.wait()
    vis, fill = masks(0)
    with jax.named_scope("main_a"):
        loop(NA, lambda i: step(i + LAG, 0, vis, fill, early=i))
    with jax.named_scope("conv_e"):
        loop(HB // 2, lambda j: (inv_stage(HB + 2 * j), inv_stage(HB + 2 * j + 1)))
    with jax.named_scope("main_b"):
        loop(NSEG - LAG - NA, lambda i: step(i + LAG + NA, 0, vis, fill))
    done = (NSEG - 1 - LAG) * SEG
    out_a = pltpu.make_async_copy(out_s.at[0:done, :], out_hbm.at[0:done, :], sem_x.at[1])
    out_a.start()
    with jax.named_scope("epi"):
        vis, fill = masks(2)
        step(NSEG, 2, vis, fill)
        step(NSEG + 1, 2, *masks(2, 2 * M), True)
    post2(NSEG + LAG)
    out_b = pltpu.make_async_copy(out_s.at[done:S, :], out_hbm.at[done:S, :], sem_x.at[2])
    out_b.start()
    out_a.wait()
    out_b.wait()


@jax.jit
def pallas_interleave_layers__memory_aug_recurrent_mem_tr__ssm_conv_h3__prompt_kernel(
    A_x, A_mem0, A_Wq, A_Wk, A_Wv, A_Wo, A_seg_len,
    B_q, B_k, B_v, B_shift_k, B_ssm_k, B_ssm_D,
):
    del A_seg_len, B_q
    assert A_x.shape == (1, S, D) and A_Wq.shape == (D, H, DH)
    vm = pl.BlockSpec(memory_space=pltpu.VMEM)
    hbm = pl.BlockSpec(memory_space=pl.ANY)
    out = pl.pallas_call(
        _kernel,
        out_shape=jax.ShapeDtypeStruct((S, D), BF16),
        in_specs=[hbm, vm, hbm, hbm, hbm, hbm, hbm, hbm, vm, hbm, vm],
        out_specs=hbm,
        scratch_shapes=[
            pltpu.VMEM((S, D), BF16),
            pltpu.VMEM((S, D), BF16),
            pltpu.VMEM((S, D), BF16),
            pltpu.VMEM((NB, D, TB), BF16),
            pltpu.VMEM((3, D, H, DH), BF16),
            pltpu.VMEM(((3 * H + 1) * WP, 128), U32),
            pltpu.VMEM((H * DH, D), BF16),
            pltpu.VMEM((TB, TB), BF16),
            pltpu.VMEM((2, TB, TB), BF16),
            pltpu.VMEM((2, TB // 2, 3 * TB), BF16),
            pltpu.VMEM((2, NLB, S // 2 + 8, 128), F32),
            pltpu.VMEM((NB, 2, NLB * TB, 128), F32),
            pltpu.VMEM((NB, 3, NLB * TB, 128), F32),
            pltpu.VMEM((NB + 1, 2, NLB * TB, 128), F32),
            pltpu.VMEM((NLB, S + 8, 128), F32),
            pltpu.VMEM((ROWS, D), BF16),
            pltpu.VMEM((2 * SEG, D), F32),
            pltpu.VMEM((4, SEG, D), F32),
            pltpu.VMEM((S, D), BF16),
            pltpu.VMEM((NA * SEG, D), BF16),
            pltpu.VMEM((NQH, NA * SEG, DH), BF16),
            pltpu.SemaphoreType.DMA((3 * (NB // 2) + 1,)),
            pltpu.SemaphoreType.DMA((4,)),
            pltpu.SemaphoreType.DMA((4,)),
        ],
        compiler_params=pltpu.CompilerParams(vmem_limit_bytes=120 * 1024 * 1024),
    )(A_x.reshape(S, D), A_mem0.reshape(M, D), A_Wq, A_Wk, A_Wv,
      A_Wo.reshape(H * DH, D), B_k.reshape(S, D), B_v.reshape(S, D),
      B_shift_k.T, B_ssm_k, B_ssm_D)
    return out.reshape(1, S, D)
```

```python
import functools
import math

import jax
import jax.numpy as jnp
from jax import lax
import jax.experimental.pallas as pl
import jax.experimental.pallas.tpu as pltpu

F32 = jnp.float32
BF16 = jnp.bfloat16
U32 = jnp.uint32

S = 2048
D = 640
H = 32
DH = 128
M = 8
SEG = 32
NSEG = S // SEG
KS = 4
LAG = 2
ROWS = 2 * M + 2 * SEG
HG = 4
NG = H // HG
NLB = D // 128
TB = 128
NB = S // TB
HB = NB // 2
NPOS = NLB * TB // 8
NA = 20
PPS = 4
UCUT = (range(0, 3), range(3, 6), range(6, 9), range(9, 16))
TOKP = (2, 1)
NQH = 26
WP = 324


def _ln(x):
    m = jnp.mean(x, axis=-1, keepdims=True)
    c = x - m
    v = jnp.mean(c * c, axis=-1, keepdims=True)
    return c * lax.rsqrt(v + 1e-5)


def _r(x):
    return x.astype(BF16).astype(F32)


def _split(x):
    hi = pltpu.bitcast(pltpu.bitcast(x, U32) & jnp.uint32(0xFFFF0000), F32)
    return hi, x - hi


def _bf(x):
    return jnp.concatenate([x[:, g:g + 128].astype(BF16)
                            for g in range(0, x.shape[1], 128)], axis=1)


def _basis(r, t):
    b = r & 63
    f = jnp.where(b < 32, 2 * b, 2 * b - 63)
    n = ((2 * f + 1) * t - jnp.where(r >= 64, TB, 0)) & (4 * TB - 1)
    n = jnp.where(n >= 2 * TB, n - 4 * TB, n)
    return jnp.cos(n.astype(F32) * (2.0 * math.pi / (4 * TB)))


def _halves(x):
    w = pltpu.bitcast(x, U32)
    return (pltpu.bitcast(w << 16, F32),
            pltpu.bitcast(w & jnp.uint32(0xFFFF0000), F32))


def _kernel(x_hbm, mem0_ref, wq_hbm, wk_hbm, wv_hbm, wo_hbm,
            k_hbm, v_hbm, shk_ref, ssmk_hbm, ssmd_ref,
            out_hbm,
            x_s, k_s, v_s, ssmk_s, wraw, wt_q, wt_kv, wo_s,
            perm_s, fu_s, inv_s, kpad, u_s, kf_s, c_s, y_s,
            hbuf, obuf, x2_s, out_s, hl_s, qh_s,
            sem_c, sem_w, sem_x):
    XH = (LAG + NA) * SEG

    def conv_copies(j):
        r0 = j * TB if isinstance(j, int) else pl.multiple_of(j * TB, TB)
        return (
            pltpu.make_async_copy(ssmk_hbm.at[:, pl.ds(r0, TB)], ssmk_s.at[j], sem_c.at[j]),
            pltpu.make_async_copy(k_hbm.at[pl.ds(r0, TB), :], k_s.at[pl.ds(r0, TB), :], sem_c.at[HB + j]),
            pltpu.make_async_copy(v_hbm.at[pl.ds(r0, TB), :], v_s.at[pl.ds(r0, TB), :], sem_c.at[NB + j]),
        )
    late_copies = [pltpu.make_async_copy(ssmk_hbm.at[:, pl.ds(j * TB, TB)], ssmk_s.at[j], sem_c.at[3 * HB])
                   for j in range(HB, NB)]
    late_copies += [pltpu.make_async_copy(src.at[S // 2:, :], dst.at[S // 2:, :], sem_c.at[3 * HB])
                    for src, dst in ((k_hbm, k_s), (v_hbm, v_s))]
    w_copies = [pltpu.make_async_copy(w, wraw.at[t], sem_w.at[t])
                for t, w in enumerate((wq_hbm, wk_hbm, wv_hbm))]
    wo_copy = pltpu.make_async_copy(wo_hbm, wo_s, sem_w.at[3])
    xa_copy = pltpu.make_async_copy(x_hbm.at[0:XH, :], x_s.at[0:XH, :], sem_x.at[0])
    xb_copy = pltpu.make_async_copy(x_hbm.at[XH:, :], x_s.at[XH:, :], sem_x.at[3])
    for j in range(HB):
        for c in conv_copies(j):
            c.start()
    for c in late_copies:
        c.start()
    xa_copy.start()
    wo_copy.start(priority=1)
    xb_copy.start(priority=1)

    hb = TB // 2
    ri = lax.broadcasted_iota(jnp.int32, (TB, TB), 0)
    ci = lax.broadcasted_iota(jnp.int32, (TB, TB), 1)
    perm_s[...] = jnp.where(ci == 2 * (ri & 63) + (ri >> 6), 1.0, 0.0).astype(BF16)
    tab = _basis(ri, 2 * (ci & 63) + (ci >> 6))
    hi, lo = _split(tab)
    fu_s[0] = jnp.where(ci < hb, hi, pltpu.roll(lo, hb, 1)).astype(BF16)
    fu_s[1] = jnp.where(ci < hb, pltpu.roll(hi, hb, 1), lo).astype(BF16)
    gh, gl = _split(tab.T * (1.0 / TB))
    ginv = _bf(jnp.concatenate([gh, gl, gh], axis=1))
    inv_s[0] = ginv[:hb]
    inv_s[1] = ginv[hb:]

    shk_t = shk_ref[...].astype(F32)
    taps = [[shk_t[j:j + 1, g * 128:(g + 1) * 128] for g in range(NLB)] for j in range(KS)]
    dvec = ssmd_ref[...].astype(F32).reshape(1, D)
    for g in range(NLB):
        kpad[0, g, 0:8, :] = jnp.zeros((8, 128), F32)
        kpad[1, g, 0:8, :] = jnp.zeros((8, 128), F32)
    c_s[0] = jnp.zeros(c_s.shape[1:], F32)

    def spectrum(e, o):
        fe = jnp.dot(fu_s[0], jnp.concatenate([e, e], axis=0).astype(BF16), preferred_element_type=F32)
        fo = jnp.dot(fu_s[1], jnp.concatenate([o, o], axis=0).astype(BF16), preferred_element_type=F32)
        return ((fe[:hb] + fo[:hb], fe[hb:] + fo[hb:]), (fe[:hb] - fo[:hb], fo[hb:] - fe[hb:]))

    def fwd_stage(js, first):
        if first:
            for j in js:
                for c in conv_copies(j):
                    c.wait()
        kts = [lax.dot_general(perm_s[...], ssmk_s[j], (((1,), (1,)), ((), ())),
                               preferred_element_type=F32) for j in js]
        for j, kt in zip(js, kts):
            r0 = pl.multiple_of(j * TB, TB)
            q0 = pl.multiple_of(j * hb, hb) + 8
            for g in range(NLB):
                lb = slice(g * 128, (g + 1) * 128)
                halves = (slice(g * TB, g * TB + hb), slice(g * TB + hb, (g + 1) * TB))
                for rows, (kr, ki) in zip(halves, spectrum(kt[:hb, lb], kt[hb:, lb])):
                    if first:
                        kr = kr + jnp.where(j == 0, dvec[:, lb], 0.0)
                    kf_s[j, 0, rows] = kr
                    kf_s[j, 1, rows] = ki - kr
                    kf_s[j, 2, rows] = kr + ki
                ke, ko = _halves(k_s[pl.ds(r0, TB), lb])
                ve, vo = _halves(v_s[pl.ds(r0, TB), lb])
                kpad[0, g, pl.ds(q0, hb), :] = ke
                kpad[1, g, pl.ds(q0, hb), :] = ko
                ke1 = kpad[0, g, pl.ds(q0 - 1, hb), :]
                ko1 = kpad[1, g, pl.ds(q0 - 1, hb), :]
                ko2 = kpad[1, g, pl.ds(q0 - 2, hb), :]
                t0, t1, t2, t3 = (taps[t][g] for t in range(KS))
                e = (ke * t0 + ko1 * t1 + ke1 * t2 + ko2 * t3) * ve
                o = (ko * t0 + ke * t1 + ko1 * t2 + ke1 * t3) * vo
                for rows, (ur, ui) in zip(halves, spectrum(e, o)):
                    u_s[j, 0, rows] = ur
                    u_s[j, 1, rows] = ui

    def mac_units(row, half):
        rs = pl.ds(row, 8)
        state = {}

        def unit(p, avals, final, tok=None):
            acc = state.setdefault(p, dict(state.get(0, {})))
            for a in avals:
                u = u_s[a, 0, rs] + u_s[a, 1, rs] if p == 0 else u_s[a, p - 1, rs]
                if tok is not None:
                    u = u + tok
                for i in range(max(a, half * HB), half * HB + HB):
                    t = u * kf_s[i - a, p, rs]
                    acc[i] = t if i not in acc else (acc[i] - t if p == 2 else acc[i] + t)
            if final and p:
                for i, v in acc.items():
                    c_s[i + 1, 2 - p, rs] = v

        subs = UCUT if half else (range(HB),)
        return [functools.partial(unit, p, avals, n == len(subs) - 1)
                for p in range(3) for n, avals in enumerate(subs)]

    def inv_stage(i):
        q = TB // 4
        for g in range(NLB):
            re, im = [], []
            for b in range(4):
                rows = slice(g * TB + b * q, g * TB + (b + 1) * q)
                cr, ci_ = c_s[i + 1, 0, rows], c_s[i + 1, 1, rows]
                pr, pi = c_s[i, 0, rows], c_s[i, 1, rows]
                re.append(cr + pi if b in (0, 3) else cr - pi)
                im.append(ci_ - pr if b in (0, 3) else ci_ + pr)
            pe = jnp.concatenate([re[0] + re[2], re[1] + re[3], im[0] - im[2], im[1] - im[3]], axis=0)
            po = jnp.concatenate([re[0] - re[2], re[1] - re[3], im[0] + im[2], im[1] + im[3]], axis=0)
            for par, pp in enumerate((pe, po)):
                ph, plo = _split(pp)
                y_s[g, pl.ds(i * TB + par, hb, stride=2), :] = jnp.dot(
                    inv_s[par], jnp.concatenate([ph, ph, plo], axis=0).astype(BF16),
                    preferred_element_type=F32)

    def relayout_rows(t, dst, base, dp, tok=None):
        a = pltpu.bitcast(wraw[t, 2 * dp], U32)
        b = pltpu.bitcast(wraw[t, 2 * dp + 1], U32)
        if tok is not None:
            a = a | tok
        dst[pl.ds(base + dp, 16, stride=WP), :] = (a & jnp.uint32(0xFFFF)) | (b << 16)
        dst[pl.ds(base + 16 * WP + dp, 16, stride=WP), :] = (
            (a >> 16) | (b & jnp.uint32(0xFFFF0000)))

    def wslab(t, h):
        s0 = (max(t - 1, 0) * H + (h % 2) * 16 + h // 2) * WP
        return pltpu.bitcast((wt_kv if t else wt_q)[s0:s0 + D // 2, :], BF16)

    def loop(n, fn):
        def body(j, _):
            fn(j)
            return 0
        lax.fori_loop(0, n, body, 0)

    def norm_rows(c):
        r0 = c * TB if isinstance(c, int) else pl.multiple_of(c * TB, TB)
        hl_s[pl.ds(r0, TB), :] = _ln(x_s[pl.ds(r0 + LAG * SEG, TB), :].astype(F32)).astype(BF16)

    def pre_queries(c, t=None):
        if t is not None:
            pltpu.make_async_copy(wk_hbm, wraw.at[t], sem_w.at[t]).wait()
            base = (t - 1) * (H * WP)
        per = -(-(D // 2) // (2 * NQH))
        dp = 0
        for sub in range(2):
            r0 = pl.multiple_of((2 * c + sub) * QR, QR)
            hl = hl_s[pl.ds(r0, QR), :]
            for hd in range(NQH):
                r = jnp.dot(hl, wslab(0, hd), preferred_element_type=F32)
                qh_s[hd, pl.ds(r0, QR), :] = r.astype(BF16)
                if t is not None:
                    tok = pltpu.bitcast(jnp.minimum(jnp.abs(r[0:16]), 0.0), U32)
                    for _ in range(per):
                        if dp < D // 2:
                            relayout_rows(t, wt_kv, base, dp, tok)
                            dp += 1

    nch = NA * SEG // TB
    QR = TB // 2
    with jax.named_scope("conv_a"):
        loop(HB // 2, lambda j: fwd_stage((2 * j, 2 * j + 1), True))
    with jax.named_scope("conv_b"):
        for c in w_copies:
            c.start()
        loop(NPOS // 10, lambda j: [u() for n in range(10) for u in mac_units(pl.multiple_of(80 * j, 16) + 8 * n, 0)])
        loop(HB // 2, lambda j: (inv_stage(2 * j), inv_stage(2 * j + 1)))
    with jax.named_scope("conv_c"):
        for c in late_copies:
            c.wait()
        loop(HB // 2, lambda j: fwd_stage((HB + 2 * j, HB + 2 * j + 1), False))
    with jax.named_scope("norm"):
        xa_copy.wait()
        norm_rows(0)
        loop(nch // 2, lambda c: (norm_rows(2 * c + 1), norm_rows(2 * c + 2)))
    with jax.named_scope("rel0"):
        w_copies[0].wait()
        loop(D // 64, lambda i: [relayout_rows(0, wt_q, 0, i * 32 + dd) for dd in range(32)])
    with jax.named_scope("preq"):
        loop(nch - 2, pre_queries)
    with jax.named_scope("preq_rel"):
        loop(2, lambda i: pre_queries(i + nch - 2, i + 1))

    scale = DH ** -0.5

    def masks(mode, q0=0):
        rows = ROWS if mode == 0 else ROWS - SEG
        qi = lax.broadcasted_iota(jnp.int32, (rows - q0, rows), 0) + q0
        kj = lax.broadcasted_iota(jnp.int32, (rows - q0, rows), 1)

        def layer_of(i):
            xl = (i - 2 * M) // SEG if mode == 0 else mode - 1
            return jnp.where(i < 2 * M, i // M, xl)
        same = layer_of(qi) == layer_of(kj)
        vis = same & ((qi < 2 * M) | (qi >= kj))
        fill = jnp.where(same, -1e9, -jnp.inf).astype(F32)
        return vis, fill

    mem0 = mem0_ref[...].astype(F32)
    hbuf[0:16, :] = jnp.concatenate([mem0, mem0], axis=0).astype(BF16)
    hbuf[16:48, :] = _ln(x_s[0:SEG, :].astype(F32)).astype(BF16)
    obuf[...] = jnp.zeros((2 * SEG, D), F32)
    x2_s[...] = jnp.zeros(x2_s.shape, F32)

    def seg_row(seg):
        if isinstance(seg, int):
            return min(max(seg, 0), NSEG - 1) * SEG
        return pl.multiple_of(jnp.clip(seg, 0, NSEG - 1) * SEG, SEG)

    def gate(xa, r0):
        y = jnp.concatenate([y_s[g, pl.ds(r0, SEG), :] for g in range(NLB)], axis=1)
        return xa + _r(_r(_ln(xa)) * y)

    def attention(h, vis, fill, chained, before_oproj=None, early=None):
        q0 = h.shape[0] - vis.shape[0]
        if early is not None:
            hrest = jnp.concatenate([h[:2 * M], h[2 * M + SEG:]], axis=0)
            qrow = pl.multiple_of(early * SEG, SEG)
            units = [u for n in range(PPS)
                     for u in mac_units(pl.multiple_of(early * (8 * PPS), 8 * PPS) + 8 * n, 1)]

        def proj(g):
            if g == 0 and chained and q0 == 0:
                kc = D - 128
                part = [jnp.dot(h[:, :kc], wslab(0, j)[:kc], preferred_element_type=F32)
                        for j in range(HG)]
                q = [(jnp.dot(h[:, kc:], wslab(0, j)[kc:], preferred_element_type=F32)
                      + part[j]).astype(BF16) for j in range(HG)]
                return [q] + [[jnp.dot(h, wslab(t, j), preferred_element_type=F32).astype(BF16)
                               for j in range(HG)] for t in range(1, 3)]
            res = [[None] * HG for _ in range(3)]
            order = [(t, j) for j in range(HG) for t in range(2)] + [(2, j) for j in range(HG)]
            for n, (t, j) in enumerate(order):
                hd = g * HG + j
                pre = early is not None and t == 0 and hd < NQH
                lhs = hrest if pre else (h if t else h[q0:])
                r = jnp.dot(lhs, wslab(t, hd), preferred_element_type=F32)
                if early is not None and n % TOKP[0] == TOKP[1] and units:
                    units.pop(0)(jnp.minimum(jnp.abs(r[0:8]), 0.0))
                r = r.astype(BF16)
                if pre:
                    r = jnp.concatenate([r[:2 * M], qh_s[hd, pl.ds(qrow, SEG), :], r[2 * M:]], axis=0)
                res[t][j] = r
            return res

        def probs(qkv):
            scs = [lax.dot_general(qkv[0][j], qkv[1][j], (((1,), (1,)), ((), ())),
                                   preferred_element_type=F32) for j in range(HG)]
            ps = []
            for sc in scs:
                sc = jnp.where(vis, sc * scale, fill)
                e = jnp.exp(sc - jnp.max(sc, axis=-1, keepdims=True))
                den = jnp.sum(e, axis=-1, keepdims=True)
                r = pl.reciprocal(den, approx=True)
                r = r * (2.0 - den * r)
                ps.append((e * r).astype(BF16))
            return ps

        def oproj(os_, h0):
            oc = jnp.concatenate(os_, axis=1)
            k0, k1 = h0 * DH, (h0 + len(os_)) * DH
            return [jnp.dot(oc, wo_s[k0:k1, n * 128:(n + 1) * 128], preferred_element_type=F32)
                    for n in range(NLB)]

        heads = []
        qkv = proj(0)
        oa = None
        for g in range(NG):
            ps = probs(qkv)
            vs = qkv[2]
            if g + 1 < NG:
                qkv = proj(g + 1)
            else:
                if before_oproj is not None:
                    before_oproj()
                oa = oproj(heads[:H // 2], 0)
            heads += [jnp.dot(ps[j], vs[j], preferred_element_type=F32).astype(BF16)
                      for j in range(HG)]
        assert early is None or not units
        ob = oproj(heads[H // 2:], H // 2)
        return jnp.concatenate([b + a for a, b in zip(oa, ob)], axis=1)

    def post2(s):
        r3 = seg_row(s - 1 - LAG)
        xo = gate(_r(x2_s[(s + 4 - 1 - LAG) % 4] + obuf[SEG:2 * SEG, :]), r3)
        out_s[pl.ds(r3, SEG), :] = xo.astype(BF16)

    def step(s, mode, vis, fill, chained=False, before_oproj=None, early=None):
        if mode == 0:
            h = hbuf[...]
        elif mode == 1:
            h = hbuf[0:48, :]
        else:
            h = jnp.concatenate([hbuf[0:16, :], hbuf[48:80, :]], axis=0)
        last = isinstance(s, int) and s == NSEG + LAG - 1
        if last:
            post2(s)
            obuf[SEG:2 * SEG, :] = _r(attention(h, vis, fill, chained))
            return
        r1 = seg_row(s - 1)
        xb2 = _r(gate(_r(x_s[pl.ds(r1, SEG), :].astype(F32) + obuf[0:SEG, :]), r1))
        h2n = _ln(xb2).astype(BF16)
        if mode != 1:
            post2(s)
        x2_s[(s + 4 - 1) % 4] = xb2
        if mode != 2:
            h1n = _ln(x_s[pl.ds(seg_row(s + 1), SEG), :].astype(F32)).astype(BF16)

        o = attention(h, vis, fill, chained, before_oproj, early)

        mem2 = mem0 if mode == 1 else o[M:2 * M]
        hbuf[0:16, :] = jnp.concatenate([o[0:M], mem2], axis=0).astype(BF16)
        if mode != 2:
            hbuf[16:48, :] = h1n
        hbuf[48:80, :] = h2n
        if mode == 0:
            obuf[...] = _r(o[2 * M:])
        elif mode == 1:
            obuf[0:SEG, :] = _r(o[2 * M:])
        else:
            obuf[SEG:2 * SEG, :] = _r(o[2 * M:])

    with jax.named_scope("pro"):
        vis, fill = masks(1)
        step(0, 1, vis, fill, False, wo_copy.wait)
        step(1, 1, vis, fill, True)
    xb_copy.wait()
    vis, fill = masks(0)
    with jax.named_scope("main_a"):
        loop(NA, lambda i: step(i + LAG, 0, vis, fill, early=i))
    with jax.named_scope("conv_e"):
        loop(HB // 2, lambda j: (inv_stage(HB + 2 * j), inv_stage(HB + 2 * j + 1)))
    with jax.named_scope("main_b"):
        loop(NSEG - LAG - NA, lambda i: step(i + LAG + NA, 0, vis, fill))
    done = (NSEG - 1 - LAG) * SEG
    out_a = pltpu.make_async_copy(out_s.at[0:done, :], out_hbm.at[0:done, :], sem_x.at[1])
    out_a.start()
    with jax.named_scope("epi"):
        vis, fill = masks(2)
        step(NSEG, 2, vis, fill)
        step(NSEG + 1, 2, *masks(2, 2 * M), True)
    post2(NSEG + LAG)
    out_b = pltpu.make_async_copy(out_s.at[done:S, :], out_hbm.at[done:S, :], sem_x.at[2])
    out_b.start()
    out_a.wait()
    out_b.wait()


@jax.jit
def pallas_interleave_layers__memory_aug_recurrent_mem_tr__ssm_conv_h3__prompt_kernel(
    A_x, A_mem0, A_Wq, A_Wk, A_Wv, A_Wo, A_seg_len,
    B_q, B_k, B_v, B_shift_k, B_ssm_k, B_ssm_D,
):
    del A_seg_len, B_q
    assert A_x.shape == (1, S, D) and A_Wq.shape == (D, H, DH)
    vm = pl.BlockSpec(memory_space=pltpu.VMEM)
    hbm = pl.BlockSpec(memory_space=pl.ANY)
    out = pl.pallas_call(
        _kernel,
        out_shape=jax.ShapeDtypeStruct((S, D), BF16),
        in_specs=[hbm, vm, hbm, hbm, hbm, hbm, hbm, hbm, vm, hbm, vm],
        out_specs=hbm,
        scratch_shapes=[
            pltpu.VMEM((S, D), BF16),
            pltpu.VMEM((S, D), BF16),
            pltpu.VMEM((S, D), BF16),
            pltpu.VMEM((NB, D, TB), BF16),
            pltpu.VMEM((3, D, H, DH), BF16),
            pltpu.VMEM(((H + 1) * WP, 128), U32),
            pltpu.VMEM(((2 * H + 1) * WP, 128), U32),
            pltpu.VMEM((H * DH, D), BF16),
            pltpu.VMEM((TB, TB), BF16),
            pltpu.VMEM((2, TB, TB), BF16),
            pltpu.VMEM((2, TB // 2, 3 * TB), BF16),
            pltpu.VMEM((2, NLB, S // 2 + 8, 128), F32),
            pltpu.VMEM((NB, 2, NLB * TB, 128), F32),
            pltpu.VMEM((NB, 3, NLB * TB, 128), F32),
            pltpu.VMEM((NB + 1, 2, NLB * TB, 128), F32),
            pltpu.VMEM((NLB, S + 8, 128), F32),
            pltpu.VMEM((ROWS, D), BF16),
            pltpu.VMEM((2 * SEG, D), F32),
            pltpu.VMEM((4, SEG, D), F32),
            pltpu.VMEM((S, D), BF16),
            pltpu.VMEM((NA * SEG, D), BF16),
            pltpu.VMEM((NQH, NA * SEG, DH), BF16),
            pltpu.SemaphoreType.DMA((3 * (NB // 2) + 1,)),
            pltpu.SemaphoreType.DMA((4,)),
            pltpu.SemaphoreType.DMA((4,)),
        ],
        compiler_params=pltpu.CompilerParams(vmem_limit_bytes=120 * 1024 * 1024),
    )(A_x.reshape(S, D), A_mem0.reshape(M, D), A_Wq, A_Wk, A_Wv,
      A_Wo.reshape(H * DH, D), B_k.reshape(S, D), B_v.reshape(S, D),
      B_shift_k.T, B_ssm_k, B_ssm_D)
    return out.reshape(1, S, D)
```

```python
import functools
import math

import jax
import jax.numpy as jnp
from jax import lax
import jax.experimental.pallas as pl
import jax.experimental.pallas.tpu as pltpu

F32 = jnp.float32
BF16 = jnp.bfloat16
U32 = jnp.uint32

S = 2048
D = 640
H = 32
DH = 128
M = 8
SEG = 32
NSEG = S // SEG
KS = 4
LAG = 2
ROWS = 2 * M + 2 * SEG
HG = 4
NG = H // HG
NLB = D // 128
TB = 128
NB = S // TB
HB = NB // 2
NPOS = NLB * TB // 8
NA = 20
PPS = 4
UCUT = (range(0, 3), range(3, 6), range(6, 9), range(9, 16))
TOKP = (2, 1)
NQH = 26
WP = 324


def _ln(x):
    m = jnp.mean(x, axis=-1, keepdims=True)
    c = x - m
    v = jnp.mean(c * c, axis=-1, keepdims=True)
    return c * lax.rsqrt(v + 1e-5)


def _r(x):
    return x.astype(BF16).astype(F32)


def _split(x):
    hi = pltpu.bitcast(pltpu.bitcast(x, U32) & jnp.uint32(0xFFFF0000), F32)
    return hi, x - hi


def _bf(x):
    return jnp.concatenate([x[:, g:g + 128].astype(BF16)
                            for g in range(0, x.shape[1], 128)], axis=1)


def _basis(r, t):
    b = r & 63
    f = jnp.where(b < 32, 2 * b, 2 * b - 63)
    n = ((2 * f + 1) * t - jnp.where(r >= 64, TB, 0)) & (4 * TB - 1)
    n = jnp.where(n >= 2 * TB, n - 4 * TB, n)
    return jnp.cos(n.astype(F32) * (2.0 * math.pi / (4 * TB)))


def _halves(x):
    w = pltpu.bitcast(x, U32)
    return (pltpu.bitcast(w << 16, F32),
            pltpu.bitcast(w & jnp.uint32(0xFFFF0000), F32))


def _kernel(x_hbm, mem0_hbm, wq_hbm, wk_hbm, wv_hbm, wo_hbm,
            k_hbm, v_hbm, shk_hbm, ssmk_hbm, ssmd_hbm,
            out_hbm,
            x_s, k_s, v_s, ssmk_s, wraw, wt_q, wt_kv, wo_s,
            perm_s, fu_s, inv_s, kpad, u_s, kf_s, c_s, y_s,
            hbuf, obuf, x2_s, out_s, hl_s, qh_s, mem0_ref, shk_ref, ssmd_ref,
            sem_c, sem_w, sem_x):
    XH = (LAG + NA) * SEG

    def conv_copies(j):
        r0 = j * TB if isinstance(j, int) else pl.multiple_of(j * TB, TB)
        return (
            pltpu.make_async_copy(ssmk_hbm.at[:, pl.ds(r0, TB)], ssmk_s.at[j], sem_c.at[j]),
            pltpu.make_async_copy(k_hbm.at[pl.ds(r0, TB), :], k_s.at[pl.ds(r0, TB), :], sem_c.at[HB + j]),
            pltpu.make_async_copy(v_hbm.at[pl.ds(r0, TB), :], v_s.at[pl.ds(r0, TB), :], sem_c.at[NB + j]),
        )
    late_copies = [pltpu.make_async_copy(ssmk_hbm.at[:, pl.ds(j * TB, TB)], ssmk_s.at[j], sem_c.at[3 * HB])
                   for j in range(HB, NB)]
    late_copies += [pltpu.make_async_copy(src.at[S // 2:, :], dst.at[S // 2:, :], sem_c.at[3 * HB])
                    for src, dst in ((k_hbm, k_s), (v_hbm, v_s))]
    w_copies = [pltpu.make_async_copy(w, wraw.at[t], sem_w.at[t])
                for t, w in enumerate((wq_hbm, wk_hbm, wv_hbm))]
    wo_copy = pltpu.make_async_copy(wo_hbm, wo_s, sem_w.at[3])
    xa_copy = pltpu.make_async_copy(x_hbm.at[0:XH, :], x_s.at[0:XH, :], sem_x.at[0])
    xb_copy = pltpu.make_async_copy(x_hbm.at[XH:, :], x_s.at[XH:, :], sem_x.at[3])
    small_copies = [pltpu.make_async_copy(src, dst, sem_x.at[4])
                    for src, dst in ((shk_hbm, shk_ref), (ssmd_hbm, ssmd_ref), (mem0_hbm, mem0_ref))]
    for c in small_copies:
        c.start()
    for j in range(2):
        for c in conv_copies(j):
            c.start()

    hb = TB // 2
    ri = lax.broadcasted_iota(jnp.int32, (TB, TB), 0)
    ci = lax.broadcasted_iota(jnp.int32, (TB, TB), 1)
    perm_s[...] = jnp.where(ci == 2 * (ri & 63) + (ri >> 6), 1.0, 0.0).astype(BF16)
    tab = _basis(ri, 2 * (ci & 63) + (ci >> 6))
    hi, lo = _split(tab)
    fu_s[0] = jnp.where(ci < hb, hi, pltpu.roll(lo, hb, 1)).astype(BF16)
    fu_s[1] = jnp.where(ci < hb, pltpu.roll(hi, hb, 1), lo).astype(BF16)
    gh, gl = _split(tab.T * (1.0 / TB))
    ginv = _bf(jnp.concatenate([gh, gl, gh], axis=1))
    inv_s[0] = ginv[:hb]
    inv_s[1] = ginv[hb:]

    for c in small_copies:
        c.wait()
    for j in range(2, HB):
        for c in conv_copies(j):
            c.start()
    for c in late_copies:
        c.start()
    xa_copy.start()
    wo_copy.start(priority=1)
    xb_copy.start(priority=1)
    shk_t = shk_ref[...].astype(F32)
    taps = [[shk_t[j:j + 1, g * 128:(g + 1) * 128] for g in range(NLB)] for j in range(KS)]
    dvec = ssmd_ref[...].astype(F32).reshape(1, D)
    for g in range(NLB):
        kpad[0, g, 0:8, :] = jnp.zeros((8, 128), F32)
        kpad[1, g, 0:8, :] = jnp.zeros((8, 128), F32)
    c_s[0] = jnp.zeros(c_s.shape[1:], F32)

    def spectrum(e, o):
        fe = jnp.dot(fu_s[0], jnp.concatenate([e, e], axis=0).astype(BF16), preferred_element_type=F32)
        fo = jnp.dot(fu_s[1], jnp.concatenate([o, o], axis=0).astype(BF16), preferred_element_type=F32)
        return ((fe[:hb] + fo[:hb], fe[hb:] + fo[hb:]), (fe[:hb] - fo[:hb], fo[hb:] - fe[hb:]))

    def fwd_stage(js, first):
        if first:
            for j in js:
                for c in conv_copies(j):
                    c.wait()
        kts = [lax.dot_general(perm_s[...], ssmk_s[j], (((1,), (1,)), ((), ())),
                               preferred_element_type=F32) for j in js]
        for j, kt in zip(js, kts):
            r0 = pl.multiple_of(j * TB, TB)
            q0 = pl.multiple_of(j * hb, hb) + 8
            for g in range(NLB):
                lb = slice(g * 128, (g + 1) * 128)
                halves = (slice(g * TB, g * TB + hb), slice(g * TB + hb, (g + 1) * TB))
                for rows, (kr, ki) in zip(halves, spectrum(kt[:hb, lb], kt[hb:, lb])):
                    if first:
                        kr = kr + jnp.where(j == 0, dvec[:, lb], 0.0)
                    kf_s[j, 0, rows] = kr
                    kf_s[j, 1, rows] = ki - kr
                    kf_s[j, 2, rows] = kr + ki
                ke, ko = _halves(k_s[pl.ds(r0, TB), lb])
                ve, vo = _halves(v_s[pl.ds(r0, TB), lb])
                kpad[0, g, pl.ds(q0, hb), :] = ke
                kpad[1, g, pl.ds(q0, hb), :] = ko
                ke1 = kpad[0, g, pl.ds(q0 - 1, hb), :]
                ko1 = kpad[1, g, pl.ds(q0 - 1, hb), :]
                ko2 = kpad[1, g, pl.ds(q0 - 2, hb), :]
                t0, t1, t2, t3 = (taps[t][g] for t in range(KS))
                e = (ke * t0 + ko1 * t1 + ke1 * t2 + ko2 * t3) * ve
                o = (ko * t0 + ke * t1 + ko1 * t2 + ke1 * t3) * vo
                for rows, (ur, ui) in zip(halves, spectrum(e, o)):
                    u_s[j, 0, rows] = ur
                    u_s[j, 1, rows] = ui

    def mac_units(row, half):
        rs = pl.ds(row, 8)
        state = {}

        def unit(p, avals, final, tok=None):
            acc = state.setdefault(p, dict(state.get(0, {})))
            for a in avals:
                u = u_s[a, 0, rs] + u_s[a, 1, rs] if p == 0 else u_s[a, p - 1, rs]
                if tok is not None:
                    u = u + tok
                for i in range(max(a, half * HB), half * HB + HB):
                    t = u * kf_s[i - a, p, rs]
                    acc[i] = t if i not in acc else (acc[i] - t if p == 2 else acc[i] + t)
            if final and p:
                for i, v in acc.items():
                    c_s[i + 1, 2 - p, rs] = v

        subs = UCUT if half else (range(HB),)
        return [functools.partial(unit, p, avals, n == len(subs) - 1)
                for p in range(3) for n, avals in enumerate(subs)]

    def inv_stage(i):
        q = TB // 4
        for g in range(NLB):
            re, im = [], []
            for b in range(4):
                rows = slice(g * TB + b * q, g * TB + (b + 1) * q)
                cr, ci_ = c_s[i + 1, 0, rows], c_s[i + 1, 1, rows]
                pr, pi = c_s[i, 0, rows], c_s[i, 1, rows]
                re.append(cr + pi if b in (0, 3) else cr - pi)
                im.append(ci_ - pr if b in (0, 3) else ci_ + pr)
            pe = jnp.concatenate([re[0] + re[2], re[1] + re[3], im[0] - im[2], im[1] - im[3]], axis=0)
            po = jnp.concatenate([re[0] - re[2], re[1] - re[3], im[0] + im[2], im[1] + im[3]], axis=0)
            for par, pp in enumerate((pe, po)):
                ph, plo = _split(pp)
                y_s[g, pl.ds(i * TB + par, hb, stride=2), :] = jnp.dot(
                    inv_s[par], jnp.concatenate([ph, ph, plo], axis=0).astype(BF16),
                    preferred_element_type=F32)

    def relayout_rows(t, dst, base, dp, tok=None):
        a = pltpu.bitcast(wraw[t, 2 * dp], U32)
        b = pltpu.bitcast(wraw[t, 2 * dp + 1], U32)
        if tok is not None:
            a = a | tok
        dst[pl.ds(base + dp, 16, stride=WP), :] = (a & jnp.uint32(0xFFFF)) | (b << 16)
        dst[pl.ds(base + 16 * WP + dp, 16, stride=WP), :] = (
            (a >> 16) | (b & jnp.uint32(0xFFFF0000)))

    def wslab(t, h):
        s0 = (max(t - 1, 0) * H + (h % 2) * 16 + h // 2) * WP
        return pltpu.bitcast((wt_kv if t else wt_q)[s0:s0 + D // 2, :], BF16)

    def loop(n, fn):
        def body(j, _):
            fn(j)
            return 0
        lax.fori_loop(0, n, body, 0)

    def norm_rows(c):
        r0 = c * TB if isinstance(c, int) else pl.multiple_of(c * TB, TB)
        hl_s[pl.ds(r0, TB), :] = _ln(x_s[pl.ds(r0 + LAG * SEG, TB), :].astype(F32)).astype(BF16)

    def pre_queries(c, t=None):
        if t is not None:
            pltpu.make_async_copy(wraw.at[t], wraw.at[t], sem_w.at[t]).wait()
            base = (t - 1) * (H * WP)
        per = -(-(D // 2) // (2 * NQH))
        dp = 0
        for sub in range(2):
            r0 = pl.multiple_of((2 * c + sub) * QR, QR)
            hl = hl_s[pl.ds(r0, QR), :]
            for hd in range(NQH):
                r = jnp.dot(hl, wslab(0, hd), preferred_element_type=F32)
                qh_s[hd, pl.ds(r0, QR), :] = r.astype(BF16)
                if t is not None:
                    tok = pltpu.bitcast(jnp.minimum(jnp.abs(r[0:16]), 0.0), U32)
                    for _ in range(per):
                        if dp < D // 2:
                            relayout_rows(t, wt_kv, base, dp, tok)
                            dp += 1

    nch = NA * SEG // TB
    QR = TB // 2
    with jax.named_scope("conv_a"):
        loop(HB // 2, lambda j: fwd_stage((2 * j, 2 * j + 1), True))
    with jax.named_scope("conv_b"):
        for c in w_copies:
            c.start()
        loop(NPOS // 10, lambda j: [u() for n in range(10) for u in mac_units(pl.multiple_of(80 * j, 16) + 8 * n, 0)])
        loop(HB // 2, lambda j: (inv_stage(2 * j), inv_stage(2 * j + 1)))
    with jax.named_scope("conv_c"):
        for c in late_copies:
            c.wait()
        loop(HB // 2, lambda j: fwd_stage((HB + 2 * j, HB + 2 * j + 1), False))
    with jax.named_scope("norm"):
        xa_copy.wait()
        norm_rows(0)
        loop(nch // 2, lambda c: (norm_rows(2 * c + 1), norm_rows(2 * c + 2)))
    with jax.named_scope("rel0"):
        w_copies[0].wait()
        loop(D // 64, lambda i: [relayout_rows(0, wt_q, 0, i * 32 + dd) for dd in range(32)])
    with jax.named_scope("preq"):
        loop(nch - 2, pre_queries)
    with jax.named_scope("preq_rel"):
        loop(2, lambda i: pre_queries(i + nch - 2, i + 1))

    scale = DH ** -0.5

    def masks(mode, q0=0):
        rows = ROWS if mode == 0 else ROWS - SEG
        qi = lax.broadcasted_iota(jnp.int32, (rows - q0, rows), 0) + q0
        kj = lax.broadcasted_iota(jnp.int32, (rows - q0, rows), 1)

        def layer_of(i):
            xl = (i - 2 * M) // SEG if mode == 0 else mode - 1
            return jnp.where(i < 2 * M, i // M, xl)
        same = layer_of(qi) == layer_of(kj)
        vis = same & ((qi < 2 * M) | (qi >= kj))
        fill = jnp.where(same, -1e9, -jnp.inf).astype(F32)
        return vis, fill

    mem0 = mem0_ref[...].astype(F32)
    hbuf[0:16, :] = jnp.concatenate([mem0, mem0], axis=0).astype(BF16)
    hbuf[16:48, :] = _ln(x_s[0:SEG, :].astype(F32)).astype(BF16)
    obuf[...] = jnp.zeros((2 * SEG, D), F32)
    x2_s[...] = jnp.zeros(x2_s.shape, F32)

    def seg_row(seg):
        if isinstance(seg, int):
            return min(max(seg, 0), NSEG - 1) * SEG
        return pl.multiple_of(jnp.clip(seg, 0, NSEG - 1) * SEG, SEG)

    def gate(xa, r0):
        y = jnp.concatenate([y_s[g, pl.ds(r0, SEG), :] for g in range(NLB)], axis=1)
        return xa + _r(_r(_ln(xa)) * y)

    def attention(h, vis, fill, chained, before_oproj=None, early=None):
        q0 = h.shape[0] - vis.shape[0]
        if early is not None:
            hrest = jnp.concatenate([h[:2 * M], h[2 * M + SEG:]], axis=0)
            qrow = pl.multiple_of(early * SEG, SEG)
            units = [u for n in range(PPS)
                     for u in mac_units(pl.multiple_of(early * (8 * PPS), 8 * PPS) + 8 * n, 1)]

        def proj(g):
            if g == 0 and chained and q0 == 0:
                kc = D - 128
                part = [jnp.dot(h[:, :kc], wslab(0, j)[:kc], preferred_element_type=F32)
                        for j in range(HG)]
                q = [(jnp.dot(h[:, kc:], wslab(0, j)[kc:], preferred_element_type=F32)
                      + part[j]).astype(BF16) for j in range(HG)]
                return [q] + [[jnp.dot(h, wslab(t, j), preferred_element_type=F32).astype(BF16)
                               for j in range(HG)] for t in range(1, 3)]
            res = [[None] * HG for _ in range(3)]
            order = [(t, j) for j in range(HG) for t in range(2)] + [(2, j) for j in range(HG)]
            for n, (t, j) in enumerate(order):
                hd = g * HG + j
                pre = early is not None and t == 0 and hd < NQH
                lhs = hrest if pre else (h if t else h[q0:])
                r = jnp.dot(lhs, wslab(t, hd), preferred_element_type=F32)
                if early is not None and n % TOKP[0] == TOKP[1] and units:
                    units.pop(0)(jnp.minimum(jnp.abs(r[0:8]), 0.0))
                r = r.astype(BF16)
                if pre:
                    r = jnp.concatenate([r[:2 * M], qh_s[hd, pl.ds(qrow, SEG), :], r[2 * M:]], axis=0)
                res[t][j] = r
            return res

        def probs(qkv):
            scs = [lax.dot_general(qkv[0][j], qkv[1][j], (((1,), (1,)), ((), ())),
                                   preferred_element_type=F32) for j in range(HG)]
            ps = []
            for sc in scs:
                sc = jnp.where(vis, sc * scale, fill)
                e = jnp.exp(sc - jnp.max(sc, axis=-1, keepdims=True))
                den = jnp.sum(e, axis=-1, keepdims=True)
                r = pl.reciprocal(den, approx=True)
                r = r * (2.0 - den * r)
                ps.append((e * r).astype(BF16))
            return ps

        def oproj(os_, h0):
            oc = jnp.concatenate(os_, axis=1)
            k0, k1 = h0 * DH, (h0 + len(os_)) * DH
            return [jnp.dot(oc, wo_s[k0:k1, n * 128:(n + 1) * 128], preferred_element_type=F32)
                    for n in range(NLB)]

        heads = []
        qkv = proj(0)
        oa = None
        for g in range(NG):
            ps = probs(qkv)
            vs = qkv[2]
            if g + 1 < NG:
                qkv = proj(g + 1)
            else:
                if before_oproj is not None:
                    before_oproj()
                oa = oproj(heads[:H // 2], 0)
            heads += [jnp.dot(ps[j], vs[j], preferred_element_type=F32).astype(BF16)
                      for j in range(HG)]
        assert early is None or not units
        ob = oproj(heads[H // 2:], H // 2)
        return jnp.concatenate([b + a for a, b in zip(oa, ob)], axis=1)

    def post2(s):
        r3 = seg_row(s - 1 - LAG)
        xo = gate(_r(x2_s[(s + 4 - 1 - LAG) % 4] + obuf[SEG:2 * SEG, :]), r3)
        out_s[pl.ds(r3, SEG), :] = xo.astype(BF16)

    def step(s, mode, vis, fill, chained=False, before_oproj=None, early=None):
        if mode == 0:
            h = hbuf[...]
        elif mode == 1:
            h = hbuf[0:48, :]
        else:
            h = jnp.concatenate([hbuf[0:16, :], hbuf[48:80, :]], axis=0)
        last = isinstance(s, int) and s == NSEG + LAG - 1
        if last:
            post2(s)
            obuf[SEG:2 * SEG, :] = _r(attention(h, vis, fill, chained))
            return
        r1 = seg_row(s - 1)
        xb2 = _r(gate(_r(x_s[pl.ds(r1, SEG), :].astype(F32) + obuf[0:SEG, :]), r1))
        h2n = _ln(xb2).astype(BF16)
        if mode != 1:
            post2(s)
        x2_s[(s + 4 - 1) % 4] = xb2
        if mode != 2:
            h1n = _ln(x_s[pl.ds(seg_row(s + 1), SEG), :].astype(F32)).astype(BF16)

        o = attention(h, vis, fill, chained, before_oproj, early)

        mem2 = mem0 if mode == 1 else o[M:2 * M]
        hbuf[0:16, :] = jnp.concatenate([o[0:M], mem2], axis=0).astype(BF16)
        if mode != 2:
            hbuf[16:48, :] = h1n
        hbuf[48:80, :] = h2n
        if mode == 0:
            obuf[...] = _r(o[2 * M:])
        elif mode == 1:
            obuf[0:SEG, :] = _r(o[2 * M:])
        else:
            obuf[SEG:2 * SEG, :] = _r(o[2 * M:])

    with jax.named_scope("pro"):
        vis, fill = masks(1)
        step(0, 1, vis, fill, False, wo_copy.wait)
        step(1, 1, vis, fill, True)
    xb_copy.wait()
    vis, fill = masks(0)
    with jax.named_scope("main_a"):
        loop(NA, lambda i: step(i + LAG, 0, vis, fill, early=i))
    with jax.named_scope("conv_e"):
        loop(HB // 2, lambda j: (inv_stage(HB + 2 * j), inv_stage(HB + 2 * j + 1)))
    with jax.named_scope("main_b"):
        loop(NSEG - LAG - NA, lambda i: step(i + LAG + NA, 0, vis, fill))
    done = (NSEG - 1 - LAG) * SEG
    out_a = pltpu.make_async_copy(out_s.at[0:done, :], out_hbm.at[0:done, :], sem_x.at[1])
    out_a.start()
    with jax.named_scope("epi"):
        vis, fill = masks(2)
        step(NSEG, 2, vis, fill)
        step(NSEG + 1, 2, *masks(2, 2 * M), True)
    post2(NSEG + LAG)
    out_b = pltpu.make_async_copy(out_s.at[done:S, :], out_hbm.at[done:S, :], sem_x.at[2])
    out_b.start()
    out_a.wait()
    out_b.wait()


@jax.jit
def pallas_interleave_layers__memory_aug_recurrent_mem_tr__ssm_conv_h3__prompt_kernel(
    A_x, A_mem0, A_Wq, A_Wk, A_Wv, A_Wo, A_seg_len,
    B_q, B_k, B_v, B_shift_k, B_ssm_k, B_ssm_D,
):
    del A_seg_len, B_q
    assert A_x.shape == (1, S, D) and A_Wq.shape == (D, H, DH)
    hbm = pl.BlockSpec(memory_space=pl.ANY)
    out = pl.pallas_call(
        _kernel,
        out_shape=jax.ShapeDtypeStruct((S, D), BF16),
        in_specs=[hbm] * 11,
        out_specs=hbm,
        scratch_shapes=[
            pltpu.VMEM((S, D), BF16),
            pltpu.VMEM((S, D), BF16),
            pltpu.VMEM((S, D), BF16),
            pltpu.VMEM((NB, D, TB), BF16),
            pltpu.VMEM((3, D, H, DH), BF16),
            pltpu.VMEM(((H + 1) * WP, 128), U32),
            pltpu.VMEM(((2 * H + 1) * WP, 128), U32),
            pltpu.VMEM((H * DH, D), BF16),
            pltpu.VMEM((TB, TB), BF16),
            pltpu.VMEM((2, TB, TB), BF16),
            pltpu.VMEM((2, TB // 2, 3 * TB), BF16),
            pltpu.VMEM((2, NLB, S // 2 + 8, 128), F32),
            pltpu.VMEM((NB, 2, NLB * TB, 128), F32),
            pltpu.VMEM((NB, 3, NLB * TB, 128), F32),
            pltpu.VMEM((NB + 1, 2, NLB * TB, 128), F32),
            pltpu.VMEM((NLB, S + 8, 128), F32),
            pltpu.VMEM((ROWS, D), BF16),
            pltpu.VMEM((2 * SEG, D), F32),
            pltpu.VMEM((4, SEG, D), F32),
            pltpu.VMEM((S, D), BF16),
            pltpu.VMEM((NA * SEG, D), BF16),
            pltpu.VMEM((NQH, NA * SEG, DH), BF16),
            pltpu.VMEM((M, D), BF16),
            pltpu.VMEM((KS, D), BF16),
            pltpu.VMEM((D,), BF16),
            pltpu.SemaphoreType.DMA((3 * (NB // 2) + 1,)),
            pltpu.SemaphoreType.DMA((4,)),
            pltpu.SemaphoreType.DMA((5,)),
        ],
        compiler_params=pltpu.CompilerParams(vmem_limit_bytes=120 * 1024 * 1024),
    )(A_x.reshape(S, D), A_mem0.reshape(M, D), A_Wq, A_Wk, A_Wv,
      A_Wo.reshape(H * DH, D), B_k.reshape(S, D), B_v.reshape(S, D),
      B_shift_k.T, B_ssm_k, B_ssm_D)
    return out.reshape(1, S, D)
```

```python
import functools
import math

import jax
import jax.numpy as jnp
from jax import lax
import jax.experimental.pallas as pl
import jax.experimental.pallas.tpu as pltpu

F32 = jnp.float32
BF16 = jnp.bfloat16
U32 = jnp.uint32

S = 2048
D = 640
H = 32
DH = 128
M = 8
SEG = 32
NSEG = S // SEG
KS = 4
LAG = 2
ROWS = 2 * M + 2 * SEG
HG = 4
NG = H // HG
NLB = D // 128
TB = 128
NB = S // TB
HB = NB // 2
NPOS = NLB * TB // 8
NA = 20
PPS = 4
UCUT = (range(0, 3), range(3, 6), range(6, 9), range(9, 16))
TOKP = (2, 1)
NQH = 26
WP = 324


def _ln(x):
    m = jnp.mean(x, axis=-1, keepdims=True)
    c = x - m
    v = jnp.mean(c * c, axis=-1, keepdims=True)
    return c * lax.rsqrt(v + 1e-5)


def _r(x):
    return x.astype(BF16).astype(F32)


def _split(x):
    hi = pltpu.bitcast(pltpu.bitcast(x, U32) & jnp.uint32(0xFFFF0000), F32)
    return hi, x - hi


def _bf(x):
    return jnp.concatenate([x[:, g:g + 128].astype(BF16)
                            for g in range(0, x.shape[1], 128)], axis=1)


def _basis(r, t):
    b = r & 63
    f = jnp.where(b < 32, 2 * b, 2 * b - 63)
    n = ((2 * f + 1) * t - jnp.where(r >= 64, TB, 0)) & (4 * TB - 1)
    n = jnp.where(n >= 2 * TB, n - 4 * TB, n)
    return jnp.cos(n.astype(F32) * (2.0 * math.pi / (4 * TB)))


def _halves(x):
    w = pltpu.bitcast(x, U32)
    return (pltpu.bitcast(w << 16, F32),
            pltpu.bitcast(w & jnp.uint32(0xFFFF0000), F32))


def _kernel(x_hbm, mem0_hbm, wq_hbm, wk_hbm, wv_hbm, wo_hbm,
            k_hbm, v_hbm, shk_hbm, ssmk_hbm, ssmd_hbm,
            out_hbm,
            x_s, k_s, v_s, ssmk_s, wraw, wt_q, wt_kv, wo_s,
            perm_s, fu_s, inv_s, kpad, u_s, kf_s, c_s, y_s,
            hbuf, obuf, x2_s, out_s, hl_s, qh_s, mem0_ref, shk_ref, ssmd_ref,
            sem):
    XH = (LAG + NA) * SEG
    SW = 3 * HB

    def conv_copies(j):
        r0 = j * TB if isinstance(j, int) else pl.multiple_of(j * TB, TB)
        return (
            pltpu.make_async_copy(ssmk_hbm.at[:, pl.ds(r0, TB)], ssmk_s.at[j], sem.at[j]),
            pltpu.make_async_copy(k_hbm.at[pl.ds(r0, TB), :], k_s.at[pl.ds(r0, TB), :], sem.at[HB + j]),
            pltpu.make_async_copy(v_hbm.at[pl.ds(r0, TB), :], v_s.at[pl.ds(r0, TB), :], sem.at[NB + j]),
        )
    w_copies = [pltpu.make_async_copy(w, wraw.at[t], sem.at[SW + t])
                for t, w in enumerate((wq_hbm, wk_hbm, wv_hbm))]
    wo_copy = pltpu.make_async_copy(wo_hbm, wo_s, sem.at[SW + 3])
    late_copies = [pltpu.make_async_copy(ssmk_hbm.at[:, pl.ds(j * TB, TB)], ssmk_s.at[j], sem.at[SW + 4])
                   for j in range(HB, NB)]
    late_copies += [pltpu.make_async_copy(src.at[S // 2:, :], dst.at[S // 2:, :], sem.at[SW + 4])
                    for src, dst in ((k_hbm, k_s), (v_hbm, v_s))]
    small_copies = [pltpu.make_async_copy(src, dst, sem.at[SW + 5])
                    for src, dst in ((shk_hbm, shk_ref), (ssmd_hbm, ssmd_ref), (mem0_hbm, mem0_ref))]
    xa_copy = pltpu.make_async_copy(x_hbm.at[0:XH, :], x_s.at[0:XH, :], sem.at[SW + 6])
    xb_copy = pltpu.make_async_copy(x_hbm.at[XH:, :], x_s.at[XH:, :], sem.at[SW + 7])
    for c in (small_copies + [c for j in range(HB) for c in conv_copies(j)] + late_copies
              + [xa_copy] + w_copies + [wo_copy, xb_copy]):
        c.start()

    hb = TB // 2
    ri = lax.broadcasted_iota(jnp.int32, (TB, TB), 0)
    ci = lax.broadcasted_iota(jnp.int32, (TB, TB), 1)
    perm_s[...] = jnp.where(ci == 2 * (ri & 63) + (ri >> 6), 1.0, 0.0).astype(BF16)
    tab = _basis(ri, 2 * (ci & 63) + (ci >> 6))
    hi, lo = _split(tab)
    fu_s[0] = jnp.where(ci < hb, hi, pltpu.roll(lo, hb, 1)).astype(BF16)
    fu_s[1] = jnp.where(ci < hb, pltpu.roll(hi, hb, 1), lo).astype(BF16)
    gh, gl = _split(tab.T * (1.0 / TB))
    ginv = _bf(jnp.concatenate([gh, gl, gh], axis=1))
    inv_s[0] = ginv[:hb]
    inv_s[1] = ginv[hb:]

    for c in small_copies:
        c.wait()
    shk_t = shk_ref[...].astype(F32)
    taps = [[shk_t[j:j + 1, g * 128:(g + 1) * 128] for g in range(NLB)] for j in range(KS)]
    dvec = ssmd_ref[...].astype(F32).reshape(1, D)
    for g in range(NLB):
        kpad[0, g, 0:8, :] = jnp.zeros((8, 128), F32)
        kpad[1, g, 0:8, :] = jnp.zeros((8, 128), F32)
    c_s[0] = jnp.zeros(c_s.shape[1:], F32)

    def spectrum(e, o):
        fe = jnp.dot(fu_s[0], jnp.concatenate([e, e], axis=0).astype(BF16), preferred_element_type=F32)
        fo = jnp.dot(fu_s[1], jnp.concatenate([o, o], axis=0).astype(BF16), preferred_element_type=F32)
        return ((fe[:hb] + fo[:hb], fe[hb:] + fo[hb:]), (fe[:hb] - fo[:hb], fo[hb:] - fe[hb:]))

    def fwd_stage(js, first):
        if first:
            for j in js:
                for c in conv_copies(j):
                    c.wait()
        kts = [lax.dot_general(perm_s[...], ssmk_s[j], (((1,), (1,)), ((), ())),
                               preferred_element_type=F32) for j in js]
        for j, kt in zip(js, kts):
            r0 = pl.multiple_of(j * TB, TB)
            q0 = pl.multiple_of(j * hb, hb) + 8
            for g in range(NLB):
                lb = slice(g * 128, (g + 1) * 128)
                halves = (slice(g * TB, g * TB + hb), slice(g * TB + hb, (g + 1) * TB))
                for rows, (kr, ki) in zip(halves, spectrum(kt[:hb, lb], kt[hb:, lb])):
                    if first:
                        kr = kr + jnp.where(j == 0, dvec[:, lb], 0.0)
                    kf_s[j, 0, rows] = kr
                    kf_s[j, 1, rows] = ki - kr
                    kf_s[j, 2, rows] = kr + ki
                ke, ko = _halves(k_s[pl.ds(r0, TB), lb])
                ve, vo = _halves(v_s[pl.ds(r0, TB), lb])
                kpad[0, g, pl.ds(q0, hb), :] = ke
                kpad[1, g, pl.ds(q0, hb), :] = ko
                ke1 = kpad[0, g, pl.ds(q0 - 1, hb), :]
                ko1 = kpad[1, g, pl.ds(q0 - 1, hb), :]
                ko2 = kpad[1, g, pl.ds(q0 - 2, hb), :]
                t0, t1, t2, t3 = (taps[t][g] for t in range(KS))
                e = (ke * t0 + ko1 * t1 + ke1 * t2 + ko2 * t3) * ve
                o = (ko * t0 + ke * t1 + ko1 * t2 + ke1 * t3) * vo
                for rows, (ur, ui) in zip(halves, spectrum(e, o)):
                    u_s[j, 0, rows] = ur
                    u_s[j, 1, rows] = ui

    def mac_units(row, half):
        rs = pl.ds(row, 8)
        state = {}

        def unit(p, avals, final, tok=None):
            acc = state.setdefault(p, dict(state.get(0, {})))
            for a in avals:
                u = u_s[a, 0, rs] + u_s[a, 1, rs] if p == 0 else u_s[a, p - 1, rs]
                if tok is not None:
                    u = u + tok
                for i in range(max(a, half * HB), half * HB + HB):
                    t = u * kf_s[i - a, p, rs]
                    acc[i] = t if i not in acc else (acc[i] - t if p == 2 else acc[i] + t)
            if final and p:
                for i, v in acc.items():
                    c_s[i + 1, 2 - p, rs] = v

        subs = UCUT if half else (range(HB),)
        return [functools.partial(unit, p, avals, n == len(subs) - 1)
                for p in range(3) for n, avals in enumerate(subs)]

    def inv_stage(i):
        q = TB // 4
        for g in range(NLB):
            re, im = [], []
            for b in range(4):
                rows = slice(g * TB + b * q, g * TB + (b + 1) * q)
                cr, ci_ = c_s[i + 1, 0, rows], c_s[i + 1, 1, rows]
                pr, pi = c_s[i, 0, rows], c_s[i, 1, rows]
                re.append(cr + pi if b in (0, 3) else cr - pi)
                im.append(ci_ - pr if b in (0, 3) else ci_ + pr)
            pe = jnp.concatenate([re[0] + re[2], re[1] + re[3], im[0] - im[2], im[1] - im[3]], axis=0)
            po = jnp.concatenate([re[0] - re[2], re[1] - re[3], im[0] + im[2], im[1] + im[3]], axis=0)
            for par, pp in enumerate((pe, po)):
                ph, plo = _split(pp)
                y_s[g, pl.ds(i * TB + par, hb, stride=2), :] = jnp.dot(
                    inv_s[par], jnp.concatenate([ph, ph, plo], axis=0).astype(BF16),
                    preferred_element_type=F32)

    def relayout_rows(t, dst, base, dp, tok=None):
        a = pltpu.bitcast(wraw[t, 2 * dp], U32)
        b = pltpu.bitcast(wraw[t, 2 * dp + 1], U32)
        if tok is not None:
            a = a | tok
        dst[pl.ds(base + dp, 16, stride=WP), :] = (a & jnp.uint32(0xFFFF)) | (b << 16)
        dst[pl.ds(base + 16 * WP + dp, 16, stride=WP), :] = (
            (a >> 16) | (b & jnp.uint32(0xFFFF0000)))

    def wslab(t, h):
        s0 = (max(t - 1, 0) * H + (h % 2) * 16 + h // 2) * WP
        return pltpu.bitcast((wt_kv if t else wt_q)[s0:s0 + D // 2, :], BF16)

    def loop(n, fn):
        def body(j, _):
            fn(j)
            return 0
        lax.fori_loop(0, n, body, 0)

    def norm_rows(c):
        r0 = c * TB if isinstance(c, int) else pl.multiple_of(c * TB, TB)
        hl_s[pl.ds(r0, TB), :] = _ln(x_s[pl.ds(r0 + LAG * SEG, TB), :].astype(F32)).astype(BF16)

    def pre_queries(c, t=None):
        if t is not None:
            pltpu.make_async_copy(wraw.at[t], wraw.at[t], sem.at[SW + t]).wait()
            base = (t - 1) * (H * WP)
        per = -(-(D // 2) // (2 * NQH))
        dp = 0
        for sub in range(2):
            r0 = pl.multiple_of((2 * c + sub) * QR, QR)
            hl = hl_s[pl.ds(r0, QR), :]
            for hd in range(NQH):
                r = jnp.dot(hl, wslab(0, hd), preferred_element_type=F32)
                qh_s[hd, pl.ds(r0, QR), :] = r.astype(BF16)
                if t is not None:
                    tok = pltpu.bitcast(jnp.minimum(jnp.abs(r[0:16]), 0.0), U32)
                    for _ in range(per):
                        if dp < D // 2:
                            relayout_rows(t, wt_kv, base, dp, tok)
                            dp += 1

    nch = NA * SEG // TB
    QR = TB // 2
    with jax.named_scope("conv_a"):
        loop(HB // 2, lambda j: fwd_stage((2 * j, 2 * j + 1), True))
    with jax.named_scope("conv_b"):
        loop(NPOS // 10, lambda j: [u() for n in range(10) for u in mac_units(pl.multiple_of(80 * j, 16) + 8 * n, 0)])
        loop(HB // 2, lambda j: (inv_stage(2 * j), inv_stage(2 * j + 1)))
    with jax.named_scope("conv_c"):
        for c in late_copies:
            c.wait()
        loop(HB // 2, lambda j: fwd_stage((HB + 2 * j, HB + 2 * j + 1), False))
    with jax.named_scope("norm"):
        xa_copy.wait()
        norm_rows(0)
        loop(nch // 2, lambda c: (norm_rows(2 * c + 1), norm_rows(2 * c + 2)))
    with jax.named_scope("rel0"):
        w_copies[0].wait()
        loop(D // 64, lambda i: [relayout_rows(0, wt_q, 0, i * 32 + dd) for dd in range(32)])
    with jax.named_scope("preq"):
        loop(nch - 2, pre_queries)
    with jax.named_scope("preq_rel"):
        loop(2, lambda i: pre_queries(i + nch - 2, i + 1))

    scale = DH ** -0.5

    def masks(mode, q0=0):
        rows = ROWS if mode == 0 else ROWS - SEG
        qi = lax.broadcasted_iota(jnp.int32, (rows - q0, rows), 0) + q0
        kj = lax.broadcasted_iota(jnp.int32, (rows - q0, rows), 1)

        def layer_of(i):
            xl = (i - 2 * M) // SEG if mode == 0 else mode - 1
            return jnp.where(i < 2 * M, i // M, xl)
        same = layer_of(qi) == layer_of(kj)
        vis = same & ((qi < 2 * M) | (qi >= kj))
        fill = jnp.where(same, -1e9, -jnp.inf).astype(F32)
        return vis, fill

    mem0 = mem0_ref[...].astype(F32)
    hbuf[0:16, :] = jnp.concatenate([mem0, mem0], axis=0).astype(BF16)
    hbuf[16:48, :] = _ln(x_s[0:SEG, :].astype(F32)).astype(BF16)
    obuf[...] = jnp.zeros((2 * SEG, D), F32)
    x2_s[...] = jnp.zeros(x2_s.shape, F32)

    def seg_row(seg):
        if isinstance(seg, int):
            return min(max(seg, 0), NSEG - 1) * SEG
        return pl.multiple_of(jnp.clip(seg, 0, NSEG - 1) * SEG, SEG)

    def gate(xa, r0):
        y = jnp.concatenate([y_s[g, pl.ds(r0, SEG), :] for g in range(NLB)], axis=1)
        return xa + _r(_r(_ln(xa)) * y)

    def attention(h, vis, fill, chained, before_oproj=None, early=None):
        q0 = h.shape[0] - vis.shape[0]
        if early is not None:
            hrest = jnp.concatenate([h[:2 * M], h[2 * M + SEG:]], axis=0)
            qrow = pl.multiple_of(early * SEG, SEG)
            units = [u for n in range(PPS)
                     for u in mac_units(pl.multiple_of(early * (8 * PPS), 8 * PPS) + 8 * n, 1)]

        def proj(g):
            if g == 0 and chained and q0 == 0:
                kc = D - 128
                part = [jnp.dot(h[:, :kc], wslab(0, j)[:kc], preferred_element_type=F32)
                        for j in range(HG)]
                q = [(jnp.dot(h[:, kc:], wslab(0, j)[kc:], preferred_element_type=F32)
                      + part[j]).astype(BF16) for j in range(HG)]
                return [q] + [[jnp.dot(h, wslab(t, j), preferred_element_type=F32).astype(BF16)
                               for j in range(HG)] for t in range(1, 3)]
            res = [[None] * HG for _ in range(3)]
            order = [(t, j) for j in range(HG) for t in range(2)] + [(2, j) for j in range(HG)]
            for n, (t, j) in enumerate(order):
                hd = g * HG + j
                pre = early is not None and t == 0 and hd < NQH
                lhs = hrest if pre else (h if t else h[q0:])
                r = jnp.dot(lhs, wslab(t, hd), preferred_element_type=F32)
                if early is not None and n % TOKP[0] == TOKP[1] and units:
                    units.pop(0)(jnp.minimum(jnp.abs(r[0:8]), 0.0))
                r = r.astype(BF16)
                if pre:
                    r = jnp.concatenate([r[:2 * M], qh_s[hd, pl.ds(qrow, SEG), :], r[2 * M:]], axis=0)
                res[t][j] = r
            return res

        def probs(qkv):
            scs = [lax.dot_general(qkv[0][j], qkv[1][j], (((1,), (1,)), ((), ())),
                                   preferred_element_type=F32) for j in range(HG)]
            ps = []
            for sc in scs:
                sc = jnp.where(vis, sc * scale, fill)
                e = jnp.exp(sc - jnp.max(sc, axis=-1, keepdims=True))
                den = jnp.sum(e, axis=-1, keepdims=True)
                r = pl.reciprocal(den, approx=True)
                r = r * (2.0 - den * r)
                ps.append((e * r).astype(BF16))
            return ps

        def oproj(os_, h0):
            oc = jnp.concatenate(os_, axis=1)
            k0, k1 = h0 * DH, (h0 + len(os_)) * DH
            return [jnp.dot(oc, wo_s[k0:k1, n * 128:(n + 1) * 128], preferred_element_type=F32)
                    for n in range(NLB)]

        heads = []
        qkv = proj(0)
        oa = None
        for g in range(NG):
            ps = probs(qkv)
            vs = qkv[2]
            if g + 1 < NG:
                qkv = proj(g + 1)
            else:
                if before_oproj is not None:
                    before_oproj()
                oa = oproj(heads[:H // 2], 0)
            heads += [jnp.dot(ps[j], vs[j], preferred_element_type=F32).astype(BF16)
                      for j in range(HG)]
        assert early is None or not units
        ob = oproj(heads[H // 2:], H // 2)
        return jnp.concatenate([b + a for a, b in zip(oa, ob)], axis=1)

    def post2(s):
        r3 = seg_row(s - 1 - LAG)
        xo = gate(_r(x2_s[(s + 4 - 1 - LAG) % 4] + obuf[SEG:2 * SEG, :]), r3)
        out_s[pl.ds(r3, SEG), :] = xo.astype(BF16)

    def step(s, mode, vis, fill, chained=False, before_oproj=None, early=None):
        if mode == 0:
            h = hbuf[...]
        elif mode == 1:
            h = hbuf[0:48, :]
        else:
            h = jnp.concatenate([hbuf[0:16, :], hbuf[48:80, :]], axis=0)
        last = isinstance(s, int) and s == NSEG + LAG - 1
        if last:
            post2(s)
            obuf[SEG:2 * SEG, :] = _r(attention(h, vis, fill, chained))
            return
        r1 = seg_row(s - 1)
        xb2 = _r(gate(_r(x_s[pl.ds(r1, SEG), :].astype(F32) + obuf[0:SEG, :]), r1))
        h2n = _ln(xb2).astype(BF16)
        if mode != 1:
            post2(s)
        x2_s[(s + 4 - 1) % 4] = xb2
        if mode != 2:
            h1n = _ln(x_s[pl.ds(seg_row(s + 1), SEG), :].astype(F32)).astype(BF16)

        o = attention(h, vis, fill, chained, before_oproj, early)

        mem2 = mem0 if mode == 1 else o[M:2 * M]
        hbuf[0:16, :] = jnp.concatenate([o[0:M], mem2], axis=0).astype(BF16)
        if mode != 2:
            hbuf[16:48, :] = h1n
        hbuf[48:80, :] = h2n
        if mode == 0:
            obuf[...] = _r(o[2 * M:])
        elif mode == 1:
            obuf[0:SEG, :] = _r(o[2 * M:])
        else:
            obuf[SEG:2 * SEG, :] = _r(o[2 * M:])

    with jax.named_scope("pro"):
        vis, fill = masks(1)
        step(0, 1, vis, fill, False, wo_copy.wait)
        step(1, 1, vis, fill, True)
    xb_copy.wait()
    vis, fill = masks(0)
    with jax.named_scope("main_a"):
        loop(NA, lambda i: step(i + LAG, 0, vis, fill, early=i))
    with jax.named_scope("conv_e"):
        loop(HB // 2, lambda j: (inv_stage(HB + 2 * j), inv_stage(HB + 2 * j + 1)))
    with jax.named_scope("main_b"):
        loop(NSEG - LAG - NA, lambda i: step(i + LAG + NA, 0, vis, fill))
    done = (NSEG - 1 - LAG) * SEG
    out_a = pltpu.make_async_copy(out_s.at[0:done, :], out_hbm.at[0:done, :], sem.at[SW + 8])
    out_a.start()
    with jax.named_scope("epi"):
        vis, fill = masks(2)
        step(NSEG, 2, vis, fill)
        step(NSEG + 1, 2, *masks(2, 2 * M), True)
    post2(NSEG + LAG)
    out_b = pltpu.make_async_copy(out_s.at[done:S, :], out_hbm.at[done:S, :], sem.at[SW + 9])
    out_b.start()
    out_a.wait()
    out_b.wait()


@jax.jit
def pallas_interleave_layers__memory_aug_recurrent_mem_tr__ssm_conv_h3__prompt_kernel(
    A_x, A_mem0, A_Wq, A_Wk, A_Wv, A_Wo, A_seg_len,
    B_q, B_k, B_v, B_shift_k, B_ssm_k, B_ssm_D,
):
    del A_seg_len, B_q
    assert A_x.shape == (1, S, D) and A_Wq.shape == (D, H, DH)
    hbm = pl.BlockSpec(memory_space=pl.ANY)
    out = pl.pallas_call(
        _kernel,
        out_shape=jax.ShapeDtypeStruct((S, D), BF16),
        in_specs=[hbm] * 11,
        out_specs=hbm,
        scratch_shapes=[
            pltpu.VMEM((S, D), BF16),
            pltpu.VMEM((S, D), BF16),
            pltpu.VMEM((S, D), BF16),
            pltpu.VMEM((NB, D, TB), BF16),
            pltpu.VMEM((3, D, H, DH), BF16),
            pltpu.VMEM(((H + 1) * WP, 128), U32),
            pltpu.VMEM(((2 * H + 1) * WP, 128), U32),
            pltpu.VMEM((H * DH, D), BF16),
            pltpu.VMEM((TB, TB), BF16),
            pltpu.VMEM((2, TB, TB), BF16),
            pltpu.VMEM((2, TB // 2, 3 * TB), BF16),
            pltpu.VMEM((2, NLB, S // 2 + 8, 128), F32),
            pltpu.VMEM((NB, 2, NLB * TB, 128), F32),
            pltpu.VMEM((NB, 3, NLB * TB, 128), F32),
            pltpu.VMEM((NB + 1, 2, NLB * TB, 128), F32),
            pltpu.VMEM((NLB, S + 8, 128), F32),
            pltpu.VMEM((ROWS, D), BF16),
            pltpu.VMEM((2 * SEG, D), F32),
            pltpu.VMEM((4, SEG, D), F32),
            pltpu.VMEM((S, D), BF16),
            pltpu.VMEM((NA * SEG, D), BF16),
            pltpu.VMEM((NQH, NA * SEG, DH), BF16),
            pltpu.VMEM((M, D), BF16),
            pltpu.VMEM((KS, D), BF16),
            pltpu.VMEM((D,), BF16),
            pltpu.SemaphoreType.DMA((3 * HB + 10,)),
        ],
        compiler_params=pltpu.CompilerParams(vmem_limit_bytes=120 * 1024 * 1024),
    )(A_x.reshape(S, D), A_mem0.reshape(M, D), A_Wq, A_Wk, A_Wv,
      A_Wo.reshape(H * DH, D), B_k.reshape(S, D), B_v.reshape(S, D),
      B_shift_k.T, B_ssm_k, B_ssm_D)
    return out.reshape(1, S, D)
```

```python
import functools
import math

import jax
import jax.numpy as jnp
from jax import lax
import jax.experimental.pallas as pl
import jax.experimental.pallas.tpu as pltpu

F32 = jnp.float32
BF16 = jnp.bfloat16
U32 = jnp.uint32

S = 2048
D = 640
H = 32
DH = 128
M = 8
SEG = 32
NSEG = S // SEG
KS = 4
LAG = 2
ROWS = 2 * M + 2 * SEG
HG = 4
NG = H // HG
NLB = D // 128
TB = 128
NB = S // TB
HB = NB // 2
NPOS = NLB * TB // 8
NA = 20
PPS = 4
UCUT = (range(0, 3), range(3, 6), range(6, 9), range(9, 16))
TOKP = (2, 1)
NQH = 26
WP = 324


def _ln(x):
    m = jnp.mean(x, axis=-1, keepdims=True)
    c = x - m
    v = jnp.mean(c * c, axis=-1, keepdims=True)
    return c * lax.rsqrt(v + 1e-5)


def _r(x):
    return x.astype(BF16).astype(F32)


def _split(x):
    hi = pltpu.bitcast(pltpu.bitcast(x, U32) & jnp.uint32(0xFFFF0000), F32)
    return hi, x - hi


def _bf(x):
    return jnp.concatenate([x[:, g:g + 128].astype(BF16)
                            for g in range(0, x.shape[1], 128)], axis=1)


def _basis(r, t):
    b = r & 63
    f = jnp.where(b < 32, 2 * b, 2 * b - 63)
    n = ((2 * f + 1) * t - jnp.where(r >= 64, TB, 0)) & (4 * TB - 1)
    n = jnp.where(n >= 2 * TB, n - 4 * TB, n)
    return jnp.cos(n.astype(F32) * (2.0 * math.pi / (4 * TB)))


def _halves(x):
    w = pltpu.bitcast(x, U32)
    return (pltpu.bitcast(w << 16, F32),
            pltpu.bitcast(w & jnp.uint32(0xFFFF0000), F32))


def _kernel(x_hbm, mem0_hbm, wq_hbm, wk_hbm, wv_hbm, wo_hbm,
            k_hbm, v_hbm, shk_hbm, ssmk_hbm, ssmd_hbm,
            out_hbm,
            x_s, k_s, v_s, ssmk_s, wraw, wt_q, wt_kv, wo_s,
            perm_s, fu_s, inv_s, kpad, u_s, kf_s, c_s, y_s,
            hbuf, obuf, x2_s, out_s, hl_s, qh_s, mem0_ref, shk_ref, ssmd_ref,
            sem):
    XH = (LAG + NA) * SEG
    SW = HB // 2

    def conv_copies(jp, sm):
        rows = pl.ds(jp * 2 * TB if isinstance(jp, int) else pl.multiple_of(jp * 2 * TB, 2 * TB), 2 * TB)
        return [pltpu.make_async_copy(ssmk_hbm.at[:, rows], ssmk_s.at[jp], sm),
                pltpu.make_async_copy(k_hbm.at[rows, :], k_s.at[rows, :], sm),
                pltpu.make_async_copy(v_hbm.at[rows, :], v_s.at[rows, :], sm)]
    w_copies = [pltpu.make_async_copy(w, wraw.at[t], sem.at[SW + t])
                for t, w in enumerate((wq_hbm, wk_hbm, wv_hbm))]
    wo_copy = pltpu.make_async_copy(wo_hbm, wo_s, sem.at[SW + 3])
    late_copies = [c for jp in range(HB // 2, HB) for c in conv_copies(jp, sem.at[SW + 4])]
    small_copies = [pltpu.make_async_copy(src, dst, sem.at[SW + 5])
                    for src, dst in ((shk_hbm, shk_ref), (ssmd_hbm, ssmd_ref), (mem0_hbm, mem0_ref))]
    xa_copy = pltpu.make_async_copy(x_hbm.at[0:XH, :], x_s.at[0:XH, :], sem.at[SW + 6])
    xb_copy = pltpu.make_async_copy(x_hbm.at[XH:, :], x_s.at[XH:, :], sem.at[SW + 7])
    for c in (small_copies + [c for jp in range(HB // 2) for c in conv_copies(jp, sem.at[jp])] + late_copies
              + [xa_copy] + w_copies + [wo_copy, xb_copy]):
        c.start()

    hb = TB // 2
    ri = lax.broadcasted_iota(jnp.int32, (TB, TB), 0)
    ci = lax.broadcasted_iota(jnp.int32, (TB, TB), 1)
    perm_s[...] = jnp.where(ci == 2 * (ri & 63) + (ri >> 6), 1.0, 0.0).astype(BF16)
    tab = _basis(ri, 2 * (ci & 63) + (ci >> 6))
    hi, lo = _split(tab)
    fu_s[0] = jnp.where(ci < hb, hi, pltpu.roll(lo, hb, 1)).astype(BF16)
    fu_s[1] = jnp.where(ci < hb, pltpu.roll(hi, hb, 1), lo).astype(BF16)
    gh, gl = _split(tab.T * (1.0 / TB))
    ginv = _bf(jnp.concatenate([gh, gl, gh], axis=1))
    inv_s[0] = ginv[:hb]
    inv_s[1] = ginv[hb:]

    for c in small_copies:
        c.wait()
    shk_t = shk_ref[...].astype(F32)
    taps = [[shk_t[j:j + 1, g * 128:(g + 1) * 128] for g in range(NLB)] for j in range(KS)]
    dvec = ssmd_ref[...].astype(F32).reshape(1, D)
    for g in range(NLB):
        kpad[0, g, 0:8, :] = jnp.zeros((8, 128), F32)
        kpad[1, g, 0:8, :] = jnp.zeros((8, 128), F32)
    c_s[0] = jnp.zeros(c_s.shape[1:], F32)

    def spectrum(e, o):
        fe = jnp.dot(fu_s[0], jnp.concatenate([e, e], axis=0).astype(BF16), preferred_element_type=F32)
        fo = jnp.dot(fu_s[1], jnp.concatenate([o, o], axis=0).astype(BF16), preferred_element_type=F32)
        return ((fe[:hb] + fo[:hb], fe[hb:] + fo[hb:]), (fe[:hb] - fo[:hb], fo[hb:] - fe[hb:]))

    def fwd_stage(jp, first):
        if first:
            for c in conv_copies(jp, sem.at[jp]):
                c.wait()
        kts = [lax.dot_general(perm_s[...], ssmk_s[jp, :, n * TB:(n + 1) * TB], (((1,), (1,)), ((), ())),
                               preferred_element_type=F32) for n in range(2)]
        for n, kt in enumerate(kts):
            j = 2 * jp + n
            r0 = pl.multiple_of(j * TB, TB)
            q0 = pl.multiple_of(j * hb, hb) + 8
            for g in range(NLB):
                lb = slice(g * 128, (g + 1) * 128)
                halves = (slice(g * TB, g * TB + hb), slice(g * TB + hb, (g + 1) * TB))
                for rows, (kr, ki) in zip(halves, spectrum(kt[:hb, lb], kt[hb:, lb])):
                    if first and n == 0:
                        kr = kr + jnp.where(j == 0, dvec[:, lb], 0.0)
                    kf_s[j, 0, rows] = kr
                    kf_s[j, 1, rows] = ki - kr
                    kf_s[j, 2, rows] = kr + ki
                ke, ko = _halves(k_s[pl.ds(r0, TB), lb])
                ve, vo = _halves(v_s[pl.ds(r0, TB), lb])
                kpad[0, g, pl.ds(q0, hb), :] = ke
                kpad[1, g, pl.ds(q0, hb), :] = ko
                ke1 = kpad[0, g, pl.ds(q0 - 1, hb), :]
                ko1 = kpad[1, g, pl.ds(q0 - 1, hb), :]
                ko2 = kpad[1, g, pl.ds(q0 - 2, hb), :]
                t0, t1, t2, t3 = (taps[t][g] for t in range(KS))
                e = (ke * t0 + ko1 * t1 + ke1 * t2 + ko2 * t3) * ve
                o = (ko * t0 + ke * t1 + ko1 * t2 + ke1 * t3) * vo
                for rows, (ur, ui) in zip(halves, spectrum(e, o)):
                    u_s[j, 0, rows] = ur
                    u_s[j, 1, rows] = ui

    def mac_units(row, half):
        rs = pl.ds(row, 8)
        state = {}

        def unit(p, avals, final, tok=None):
            acc = state.setdefault(p, dict(state.get(0, {})))
            for a in avals:
                u = u_s[a, 0, rs] + u_s[a, 1, rs] if p == 0 else u_s[a, p - 1, rs]
                if tok is not None:
                    u = u + tok
                for i in range(max(a, half * HB), half * HB + HB):
                    t = u * kf_s[i - a, p, rs]
                    acc[i] = t if i not in acc else (acc[i] - t if p == 2 else acc[i] + t)
            if final and p:
                for i, v in acc.items():
                    c_s[i + 1, 2 - p, rs] = v

        subs = UCUT if half else (range(HB),)
        return [functools.partial(unit, p, avals, n == len(subs) - 1)
                for p in range(3) for n, avals in enumerate(subs)]

    def inv_stage(i):
        q = TB // 4
        for g in range(NLB):
            re, im = [], []
            for b in range(4):
                rows = slice(g * TB + b * q, g * TB + (b + 1) * q)
                cr, ci_ = c_s[i + 1, 0, rows], c_s[i + 1, 1, rows]
                pr, pi = c_s[i, 0, rows], c_s[i, 1, rows]
                re.append(cr + pi if b in (0, 3) else cr - pi)
                im.append(ci_ - pr if b in (0, 3) else ci_ + pr)
            pe = jnp.concatenate([re[0] + re[2], re[1] + re[3], im[0] - im[2], im[1] - im[3]], axis=0)
            po = jnp.concatenate([re[0] - re[2], re[1] - re[3], im[0] + im[2], im[1] + im[3]], axis=0)
            for par, pp in enumerate((pe, po)):
                ph, plo = _split(pp)
                y_s[g, pl.ds(i * TB + par, hb, stride=2), :] = jnp.dot(
                    inv_s[par], jnp.concatenate([ph, ph, plo], axis=0).astype(BF16),
                    preferred_element_type=F32)

    def relayout_rows(t, dst, base, dp, tok=None):
        a = pltpu.bitcast(wraw[t, 2 * dp], U32)
        b = pltpu.bitcast(wraw[t, 2 * dp + 1], U32)
        if tok is not None:
            a = a | tok
        dst[pl.ds(base + dp, 16, stride=WP), :] = (a & jnp.uint32(0xFFFF)) | (b << 16)
        dst[pl.ds(base + 16 * WP + dp, 16, stride=WP), :] = (
            (a >> 16) | (b & jnp.uint32(0xFFFF0000)))

    def wslab(t, h):
        s0 = (max(t - 1, 0) * H + (h % 2) * 16 + h // 2) * WP
        return pltpu.bitcast((wt_kv if t else wt_q)[s0:s0 + D // 2, :], BF16)

    def loop(n, fn):
        def body(j, _):
            fn(j)
            return 0
        lax.fori_loop(0, n, body, 0)

    def norm_rows(c):
        r0 = c * TB if isinstance(c, int) else pl.multiple_of(c * TB, TB)
        hl_s[pl.ds(r0, TB), :] = _ln(x_s[pl.ds(r0 + LAG * SEG, TB), :].astype(F32)).astype(BF16)

    def pre_queries(c, t=None):
        if t is not None:
            pltpu.make_async_copy(wraw.at[t], wraw.at[t], sem.at[SW + t]).wait()
            base = (t - 1) * (H * WP)
        per = -(-(D // 2) // (2 * NQH))
        dp = 0
        for sub in range(2):
            r0 = pl.multiple_of((2 * c + sub) * QR, QR)
            hl = hl_s[pl.ds(r0, QR), :]
            for hd in range(NQH):
                r = jnp.dot(hl, wslab(0, hd), preferred_element_type=F32)
                qh_s[hd, pl.ds(r0, QR), :] = r.astype(BF16)
                if t is not None:
                    tok = pltpu.bitcast(jnp.minimum(jnp.abs(r[0:16]), 0.0), U32)
                    for _ in range(per):
                        if dp < D // 2:
                            relayout_rows(t, wt_kv, base, dp, tok)
                            dp += 1

    nch = NA * SEG // TB
    QR = TB // 2
    with jax.named_scope("conv_a"):
        loop(HB // 2, lambda j: fwd_stage(j, True))
    with jax.named_scope("conv_b"):
        loop(NPOS // 10, lambda j: [u() for n in range(10) for u in mac_units(pl.multiple_of(80 * j, 16) + 8 * n, 0)])
        loop(HB // 2, lambda j: (inv_stage(2 * j), inv_stage(2 * j + 1)))
    with jax.named_scope("conv_c"):
        for c in late_copies:
            c.wait()
        loop(HB // 2, lambda j: fwd_stage(HB // 2 + j, False))
    with jax.named_scope("norm"):
        xa_copy.wait()
        norm_rows(0)
        loop(nch // 2, lambda c: (norm_rows(2 * c + 1), norm_rows(2 * c + 2)))
    with jax.named_scope("rel0"):
        w_copies[0].wait()
        loop(D // 64, lambda i: [relayout_rows(0, wt_q, 0, i * 32 + dd) for dd in range(32)])
    with jax.named_scope("preq"):
        loop(nch - 2, pre_queries)
    with jax.named_scope("preq_rel"):
        loop(2, lambda i: pre_queries(i + nch - 2, i + 1))

    scale = DH ** -0.5

    def masks(mode, q0=0):
        rows = ROWS if mode == 0 else ROWS - SEG
        qi = lax.broadcasted_iota(jnp.int32, (rows - q0, rows), 0) + q0
        kj = lax.broadcasted_iota(jnp.int32, (rows - q0, rows), 1)

        def layer_of(i):
            xl = (i - 2 * M) // SEG if mode == 0 else mode - 1
            return jnp.where(i < 2 * M, i // M, xl)
        same = layer_of(qi) == layer_of(kj)
        vis = same & ((qi < 2 * M) | (qi >= kj))
        fill = jnp.where(same, -1e9, -jnp.inf).astype(F32)
        return vis, fill

    mem0 = mem0_ref[...].astype(F32)
    hbuf[0:16, :] = jnp.concatenate([mem0, mem0], axis=0).astype(BF16)
    hbuf[16:48, :] = _ln(x_s[0:SEG, :].astype(F32)).astype(BF16)
    obuf[...] = jnp.zeros((2 * SEG, D), F32)
    x2_s[...] = jnp.zeros(x2_s.shape, F32)

    def seg_row(seg):
        if isinstance(seg, int):
            return min(max(seg, 0), NSEG - 1) * SEG
        return pl.multiple_of(jnp.clip(seg, 0, NSEG - 1) * SEG, SEG)

    def gate(xa, r0):
        y = jnp.concatenate([y_s[g, pl.ds(r0, SEG), :] for g in range(NLB)], axis=1)
        return xa + _r(_r(_ln(xa)) * y)

    def attention(h, vis, fill, chained, before_oproj=None, early=None):
        q0 = h.shape[0] - vis.shape[0]
        if early is not None:
            hrest = jnp.concatenate([h[:2 * M], h[2 * M + SEG:]], axis=0)
            qrow = pl.multiple_of(early * SEG, SEG)
            units = [u for n in range(PPS)
                     for u in mac_units(pl.multiple_of(early * (8 * PPS), 8 * PPS) + 8 * n, 1)]

        def proj(g):
            if g == 0 and chained and q0 == 0:
                kc = D - 128
                part = [jnp.dot(h[:, :kc], wslab(0, j)[:kc], preferred_element_type=F32)
                        for j in range(HG)]
                q = [(jnp.dot(h[:, kc:], wslab(0, j)[kc:], preferred_element_type=F32)
                      + part[j]).astype(BF16) for j in range(HG)]
                return [q] + [[jnp.dot(h, wslab(t, j), preferred_element_type=F32).astype(BF16)
                               for j in range(HG)] for t in range(1, 3)]
            res = [[None] * HG for _ in range(3)]
            order = [(t, j) for j in range(HG) for t in range(2)] + [(2, j) for j in range(HG)]
            for n, (t, j) in enumerate(order):
                hd = g * HG + j
                pre = early is not None and t == 0 and hd < NQH
                lhs = hrest if pre else (h if t else h[q0:])
                r = jnp.dot(lhs, wslab(t, hd), preferred_element_type=F32)
                if early is not None and n % TOKP[0] == TOKP[1] and units:
                    units.pop(0)(jnp.minimum(jnp.abs(r[0:8]), 0.0))
                r = r.astype(BF16)
                if pre:
                    r = jnp.concatenate([r[:2 * M], qh_s[hd, pl.ds(qrow, SEG), :], r[2 * M:]], axis=0)
                res[t][j] = r
            return res

        def probs(qkv):
            scs = [lax.dot_general(qkv[0][j], qkv[1][j], (((1,), (1,)), ((), ())),
                                   preferred_element_type=F32) for j in range(HG)]
            ps = []
            for sc in scs:
                sc = jnp.where(vis, sc * scale, fill)
                e = jnp.exp(sc - jnp.max(sc, axis=-1, keepdims=True))
                den = jnp.sum(e, axis=-1, keepdims=True)
                r = pl.reciprocal(den, approx=True)
                r = r * (2.0 - den * r)
                ps.append((e * r).astype(BF16))
            return ps

        def oproj(os_, h0):
            oc = jnp.concatenate(os_, axis=1)
            k0, k1 = h0 * DH, (h0 + len(os_)) * DH
            return [jnp.dot(oc, wo_s[k0:k1, n * 128:(n + 1) * 128], preferred_element_type=F32)
                    for n in range(NLB)]

        heads = []
        qkv = proj(0)
        oa = None
        for g in range(NG):
            ps = probs(qkv)
            vs = qkv[2]
            if g + 1 < NG:
                qkv = proj(g + 1)
            else:
                if before_oproj is not None:
                    before_oproj()
                oa = oproj(heads[:H // 2], 0)
            heads += [jnp.dot(ps[j], vs[j], preferred_element_type=F32).astype(BF16)
                      for j in range(HG)]
        assert early is None or not units
        ob = oproj(heads[H // 2:], H // 2)
        return jnp.concatenate([b + a for a, b in zip(oa, ob)], axis=1)

    def post2(s):
        r3 = seg_row(s - 1 - LAG)
        xo = gate(_r(x2_s[(s + 4 - 1 - LAG) % 4] + obuf[SEG:2 * SEG, :]), r3)
        out_s[pl.ds(r3, SEG), :] = xo.astype(BF16)

    def step(s, mode, vis, fill, chained=False, before_oproj=None, early=None):
        if mode == 0:
            h = hbuf[...]
        elif mode == 1:
            h = hbuf[0:48, :]
        else:
            h = jnp.concatenate([hbuf[0:16, :], hbuf[48:80, :]], axis=0)
        last = isinstance(s, int) and s == NSEG + LAG - 1
        if last:
            post2(s)
            obuf[SEG:2 * SEG, :] = _r(attention(h, vis, fill, chained))
            return
        r1 = seg_row(s - 1)
        xb2 = _r(gate(_r(x_s[pl.ds(r1, SEG), :].astype(F32) + obuf[0:SEG, :]), r1))
        h2n = _ln(xb2).astype(BF16)
        if mode != 1:
            post2(s)
        x2_s[(s + 4 - 1) % 4] = xb2
        if mode != 2:
            h1n = _ln(x_s[pl.ds(seg_row(s + 1), SEG), :].astype(F32)).astype(BF16)

        o = attention(h, vis, fill, chained, before_oproj, early)

        mem2 = mem0 if mode == 1 else o[M:2 * M]
        hbuf[0:16, :] = jnp.concatenate([o[0:M], mem2], axis=0).astype(BF16)
        if mode != 2:
            hbuf[16:48, :] = h1n
        hbuf[48:80, :] = h2n
        if mode == 0:
            obuf[...] = _r(o[2 * M:])
        elif mode == 1:
            obuf[0:SEG, :] = _r(o[2 * M:])
        else:
            obuf[SEG:2 * SEG, :] = _r(o[2 * M:])

    with jax.named_scope("pro"):
        vis, fill = masks(1)
        step(0, 1, vis, fill, False, wo_copy.wait)
        step(1, 1, vis, fill, True)
    xb_copy.wait()
    vis, fill = masks(0)
    with jax.named_scope("main_a"):
        loop(NA, lambda i: step(i + LAG, 0, vis, fill, early=i))
    with jax.named_scope("conv_e"):
        loop(HB // 2, lambda j: (inv_stage(HB + 2 * j), inv_stage(HB + 2 * j + 1)))
    with jax.named_scope("main_b"):
        loop(NSEG - LAG - NA, lambda i: step(i + LAG + NA, 0, vis, fill))
    done = (NSEG - 1 - LAG) * SEG
    out_a = pltpu.make_async_copy(out_s.at[0:done, :], out_hbm.at[0:done, :], sem.at[SW + 8])
    out_a.start()
    with jax.named_scope("epi"):
        vis, fill = masks(2)
        step(NSEG, 2, vis, fill)
        step(NSEG + 1, 2, *masks(2, 2 * M), True)
    post2(NSEG + LAG)
    out_b = pltpu.make_async_copy(out_s.at[done:S, :], out_hbm.at[done:S, :], sem.at[SW + 9])
    out_b.start()
    out_a.wait()
    out_b.wait()


@jax.jit
def pallas_interleave_layers__memory_aug_recurrent_mem_tr__ssm_conv_h3__prompt_kernel(
    A_x, A_mem0, A_Wq, A_Wk, A_Wv, A_Wo, A_seg_len,
    B_q, B_k, B_v, B_shift_k, B_ssm_k, B_ssm_D,
):
    del A_seg_len, B_q
    assert A_x.shape == (1, S, D) and A_Wq.shape == (D, H, DH)
    hbm = pl.BlockSpec(memory_space=pl.ANY)
    out = pl.pallas_call(
        _kernel,
        out_shape=jax.ShapeDtypeStruct((S, D), BF16),
        in_specs=[hbm] * 11,
        out_specs=hbm,
        scratch_shapes=[
            pltpu.VMEM((S, D), BF16),
            pltpu.VMEM((S, D), BF16),
            pltpu.VMEM((S, D), BF16),
            pltpu.VMEM((HB, D, 2 * TB), BF16),
            pltpu.VMEM((3, D, H, DH), BF16),
            pltpu.VMEM(((H + 1) * WP, 128), U32),
            pltpu.VMEM(((2 * H + 1) * WP, 128), U32),
            pltpu.VMEM((H * DH, D), BF16),
            pltpu.VMEM((TB, TB), BF16),
            pltpu.VMEM((2, TB, TB), BF16),
            pltpu.VMEM((2, TB // 2, 3 * TB), BF16),
            pltpu.VMEM((2, NLB, S // 2 + 8, 128), F32),
            pltpu.VMEM((NB, 2, NLB * TB, 128), F32),
            pltpu.VMEM((NB, 3, NLB * TB, 128), F32),
            pltpu.VMEM((NB + 1, 2, NLB * TB, 128), F32),
            pltpu.VMEM((NLB, S + 8, 128), F32),
            pltpu.VMEM((ROWS, D), BF16),
            pltpu.VMEM((2 * SEG, D), F32),
            pltpu.VMEM((4, SEG, D), F32),
            pltpu.VMEM((S, D), BF16),
            pltpu.VMEM((NA * SEG, D), BF16),
            pltpu.VMEM((NQH, NA * SEG, DH), BF16),
            pltpu.VMEM((M, D), BF16),
            pltpu.VMEM((KS, D), BF16),
            pltpu.VMEM((D,), BF16),
            pltpu.SemaphoreType.DMA((HB // 2 + 10,)),
        ],
        compiler_params=pltpu.CompilerParams(vmem_limit_bytes=120 * 1024 * 1024),
    )(A_x.reshape(S, D), A_mem0.reshape(M, D), A_Wq, A_Wk, A_Wv,
      A_Wo.reshape(H * DH, D), B_k.reshape(S, D), B_v.reshape(S, D),
      B_shift_k.T, B_ssm_k, B_ssm_D)
    return out.reshape(1, S, D)
```

```python
import functools
import math

import jax
import jax.numpy as jnp
from jax import lax
import jax.experimental.pallas as pl
import jax.experimental.pallas.tpu as pltpu

F32 = jnp.float32
BF16 = jnp.bfloat16
U32 = jnp.uint32

S = 2048
D = 640
H = 32
DH = 128
M = 8
SEG = 32
NSEG = S // SEG
KS = 4
LAG = 2
ROWS = 2 * M + 2 * SEG
HG = 4
NG = H // HG
NLB = D // 128
TB = 128
NB = S // TB
HB = NB // 2
NPOS = NLB * TB // 8
NA = 20
PPS = 4
UCUT = (range(0, 3), range(3, 6), range(6, 9), range(9, 16))
TOKP = (2, 1)
NQH = 26
UB = 2
WP = 324


def _ln(x):
    m = jnp.mean(x, axis=-1, keepdims=True)
    c = x - m
    v = jnp.mean(c * c, axis=-1, keepdims=True)
    return c * lax.rsqrt(v + 1e-5)


def _r(x):
    return x.astype(BF16).astype(F32)


def _split(x):
    hi = pltpu.bitcast(pltpu.bitcast(x, U32) & jnp.uint32(0xFFFF0000), F32)
    return hi, x - hi


def _bf(x):
    return jnp.concatenate([x[:, g:g + 128].astype(BF16)
                            for g in range(0, x.shape[1], 128)], axis=1)


def _basis(r, t):
    b = r & 63
    f = jnp.where(b < 32, 2 * b, 2 * b - 63)
    n = ((2 * f + 1) * t - jnp.where(r >= 64, TB, 0)) & (4 * TB - 1)
    n = jnp.where(n >= 2 * TB, n - 4 * TB, n)
    return jnp.cos(n.astype(F32) * (2.0 * math.pi / (4 * TB)))


def _halves(x):
    w = pltpu.bitcast(x, U32)
    return (pltpu.bitcast(w << 16, F32),
            pltpu.bitcast(w & jnp.uint32(0xFFFF0000), F32))


def _kernel(x_hbm, mem0_hbm, wq_hbm, wk_hbm, wv_hbm, wo_hbm,
            k_hbm, v_hbm, shk_hbm, ssmk_hbm, ssmd_hbm,
            out_hbm,
            x_s, k_s, v_s, ssmk_s, wraw, wt_q, wt_kv, wo_s, wo_t,
            perm_s, fu_s, inv_s, kpad, u_s, kf_s, c_s, y_s,
            hbuf, obuf, x2_s, out_s, hl_s, qh_s, mem0_ref, shk_ref, ssmd_ref,
            sem):
    XH = (LAG + NA) * SEG
    SW = HB // 2

    def conv_copies(jp, sm):
        rows = pl.ds(jp * 2 * TB if isinstance(jp, int) else pl.multiple_of(jp * 2 * TB, 2 * TB), 2 * TB)
        return [pltpu.make_async_copy(ssmk_hbm.at[:, rows], ssmk_s.at[jp], sm),
                pltpu.make_async_copy(k_hbm.at[rows, :], k_s.at[rows, :], sm),
                pltpu.make_async_copy(v_hbm.at[rows, :], v_s.at[rows, :], sm)]
    w_copies = [pltpu.make_async_copy(w, wraw.at[t], sem.at[SW + t])
                for t, w in enumerate((wq_hbm, wk_hbm, wv_hbm))]
    wo_copy = pltpu.make_async_copy(wo_hbm, wo_s, sem.at[SW + 3])
    late_copies = [c for jp in range(HB // 2, HB) for c in conv_copies(jp, sem.at[SW + 4])]
    small_copies = [pltpu.make_async_copy(src, dst, sem.at[SW + 5])
                    for src, dst in ((shk_hbm, shk_ref), (ssmd_hbm, ssmd_ref), (mem0_hbm, mem0_ref))]
    xa_copy = pltpu.make_async_copy(x_hbm.at[0:XH, :], x_s.at[0:XH, :], sem.at[SW + 6])
    xb_copy = pltpu.make_async_copy(x_hbm.at[XH:, :], x_s.at[XH:, :], sem.at[SW + 7])
    for c in (small_copies + [c for jp in range(HB // 2) for c in conv_copies(jp, sem.at[jp])] + late_copies
              + [xa_copy] + w_copies + [wo_copy, xb_copy]):
        c.start()

    hb = TB // 2
    ri = lax.broadcasted_iota(jnp.int32, (TB, TB), 0)
    ci = lax.broadcasted_iota(jnp.int32, (TB, TB), 1)
    perm_s[...] = jnp.where(ci == 2 * (ri & 63) + (ri >> 6), 1.0, 0.0).astype(BF16)
    tab = _basis(ri, 2 * (ci & 63) + (ci >> 6))
    hi, lo = _split(tab)
    fu_s[0] = jnp.where(ci < hb, hi, pltpu.roll(lo, hb, 1)).astype(BF16)
    fu_s[1] = jnp.where(ci < hb, pltpu.roll(hi, hb, 1), lo).astype(BF16)
    gh, gl = _split(tab.T * (1.0 / TB))
    ginv = _bf(jnp.concatenate([gh, gl, gh], axis=1))
    inv_s[0] = ginv[:hb]
    inv_s[1] = ginv[hb:]

    for c in small_copies:
        c.wait()
    shk_t = shk_ref[...].astype(F32)
    taps = [[shk_t[j:j + 1, g * 128:(g + 1) * 128] for g in range(NLB)] for j in range(KS)]
    dvec = ssmd_ref[...].astype(F32).reshape(1, D)
    for g in range(NLB):
        kpad[0, g, 0:8, :] = jnp.zeros((8, 128), F32)
        kpad[1, g, 0:8, :] = jnp.zeros((8, 128), F32)
    c_s[0] = jnp.zeros(c_s.shape[1:], F32)

    def spectrum(e, o):
        fe = jnp.dot(fu_s[0], jnp.concatenate([e, e], axis=0).astype(BF16), preferred_element_type=F32)
        fo = jnp.dot(fu_s[1], jnp.concatenate([o, o], axis=0).astype(BF16), preferred_element_type=F32)
        return ((fe[:hb] + fo[:hb], fe[hb:] + fo[hb:]), (fe[:hb] - fo[:hb], fo[hb:] - fe[hb:]))

    def fwd_stage(jp, first):
        if first:
            for c in conv_copies(jp, sem.at[jp]):
                c.wait()
        kts = [lax.dot_general(perm_s[...], ssmk_s[jp, :, n * TB:(n + 1) * TB], (((1,), (1,)), ((), ())),
                               preferred_element_type=F32) for n in range(2)]
        for n, kt in enumerate(kts):
            j = 2 * jp + n
            r0 = pl.multiple_of(j * TB, TB)
            q0 = pl.multiple_of(j * hb, hb) + 8
            for g in range(NLB):
                lb = slice(g * 128, (g + 1) * 128)
                halves = (slice(g * TB, g * TB + hb), slice(g * TB + hb, (g + 1) * TB))
                for rows, (kr, ki) in zip(halves, spectrum(kt[:hb, lb], kt[hb:, lb])):
                    if first and n == 0:
                        kr = kr + jnp.where(j == 0, dvec[:, lb], 0.0)
                    kf_s[j, 0, rows] = kr
                    kf_s[j, 1, rows] = ki - kr
                    kf_s[j, 2, rows] = kr + ki
                ke, ko = _halves(k_s[pl.ds(r0, TB), lb])
                ve, vo = _halves(v_s[pl.ds(r0, TB), lb])
                kpad[0, g, pl.ds(q0, hb), :] = ke
                kpad[1, g, pl.ds(q0, hb), :] = ko
                ke1 = kpad[0, g, pl.ds(q0 - 1, hb), :]
                ko1 = kpad[1, g, pl.ds(q0 - 1, hb), :]
                ko2 = kpad[1, g, pl.ds(q0 - 2, hb), :]
                t0, t1, t2, t3 = (taps[t][g] for t in range(KS))
                e = (ke * t0 + ko1 * t1 + ke1 * t2 + ko2 * t3) * ve
                o = (ko * t0 + ke * t1 + ko1 * t2 + ke1 * t3) * vo
                for rows, (ur, ui) in zip(halves, spectrum(e, o)):
                    u_s[j, 0, rows] = ur
                    u_s[j, 1, rows] = ui

    def mac_units(row, half):
        rs = pl.ds(row, 8)
        state = {}

        def unit(p, avals, final, tok=None):
            acc = state.setdefault(p, dict(state.get(0, {})))
            for a in avals:
                u = u_s[a, 0, rs] + u_s[a, 1, rs] if p == 0 else u_s[a, p - 1, rs]
                if tok is not None:
                    u = u + tok
                for i in range(max(a, half * HB), half * HB + HB):
                    t = u * kf_s[i - a, p, rs]
                    acc[i] = t if i not in acc else (acc[i] - t if p == 2 else acc[i] + t)
            if final and p:
                for i, v in acc.items():
                    c_s[i + 1, 2 - p, rs] = v

        subs = UCUT if half else (range(HB),)
        return [functools.partial(unit, p, avals, n == len(subs) - 1)
                for p in range(3) for n, avals in enumerate(subs)]

    def inv_stage(i):
        q = TB // 4
        for g in range(NLB):
            re, im = [], []
            for b in range(4):
                rows = slice(g * TB + b * q, g * TB + (b + 1) * q)
                cr, ci_ = c_s[i + 1, 0, rows], c_s[i + 1, 1, rows]
                pr, pi = c_s[i, 0, rows], c_s[i, 1, rows]
                re.append(cr + pi if b in (0, 3) else cr - pi)
                im.append(ci_ - pr if b in (0, 3) else ci_ + pr)
            pe = jnp.concatenate([re[0] + re[2], re[1] + re[3], im[0] - im[2], im[1] - im[3]], axis=0)
            po = jnp.concatenate([re[0] - re[2], re[1] - re[3], im[0] + im[2], im[1] + im[3]], axis=0)
            for par, pp in enumerate((pe, po)):
                ph, plo = _split(pp)
                y_s[g, pl.ds(i * TB + par, hb, stride=2), :] = jnp.dot(
                    inv_s[par], jnp.concatenate([ph, ph, plo], axis=0).astype(BF16),
                    preferred_element_type=F32)

    def relayout_rows(t, dst, base, dp, tok=None):
        a = pltpu.bitcast(wraw[t, 2 * dp], U32)
        b = pltpu.bitcast(wraw[t, 2 * dp + 1], U32)
        if tok is not None:
            a = a | tok
        dst[pl.ds(base + dp, 16, stride=WP), :] = (a & jnp.uint32(0xFFFF)) | (b << 16)
        dst[pl.ds(base + 16 * WP + dp, 16, stride=WP), :] = (
            (a >> 16) | (b & jnp.uint32(0xFFFF0000)))

    def wslab(t, h):
        s0 = (max(t - 1, 0) * H + (h % 2) * 16 + h // 2) * WP
        return pltpu.bitcast((wt_kv if t else wt_q)[s0:s0 + D // 2, :], BF16)

    def loop(n, fn):
        def body(j, _):
            fn(j)
            return 0
        lax.fori_loop(0, n, body, 0)

    def norm_rows(c):
        r0 = c * TB if isinstance(c, int) else pl.multiple_of(c * TB, TB)
        hl_s[pl.ds(r0, TB), :] = _ln(x_s[pl.ds(r0 + LAG * SEG, TB), :].astype(F32)).astype(BF16)

    def pre_queries(c, t=None):
        if t is not None:
            pltpu.make_async_copy(wraw.at[t], wraw.at[t], sem.at[SW + t]).wait()
            base = (t - 1) * (H * WP)
        per = -(-(D // 2) // (2 * NQH))
        dp = 0
        for sub in range(2):
            r0 = pl.multiple_of((2 * c + sub) * QR, QR)
            hl = hl_s[pl.ds(r0, QR), :]
            for hd in range(NQH):
                r = jnp.dot(hl, wslab(0, hd), preferred_element_type=F32)
                qh_s[hd, pl.ds(r0, QR), :] = r.astype(BF16)
                if t is not None:
                    tok = pltpu.bitcast(jnp.minimum(jnp.abs(r[0:16]), 0.0), U32)
                    for _ in range(per):
                        if dp < D // 2:
                            relayout_rows(t, wt_kv, base, dp, tok)
                            dp += 1

    nch = NA * SEG // TB
    QR = TB // 2
    with jax.named_scope("conv_a"):
        loop(HB // 2, lambda j: fwd_stage(j, True))
    with jax.named_scope("conv_b"):
        loop(NPOS // 10, lambda j: [u() for n in range(10) for u in mac_units(pl.multiple_of(80 * j, 16) + 8 * n, 0)])
        loop(HB // 2, lambda j: (inv_stage(2 * j), inv_stage(2 * j + 1)))
    with jax.named_scope("conv_c"):
        for c in late_copies:
            c.wait()
        loop(HB // 2, lambda j: fwd_stage(HB // 2 + j, False))
    with jax.named_scope("norm"):
        xa_copy.wait()
        norm_rows(0)
        loop(nch // 2, lambda c: (norm_rows(2 * c + 1), norm_rows(2 * c + 2)))
    with jax.named_scope("rel0"):
        w_copies[0].wait()
        loop(D // 64, lambda i: [relayout_rows(0, wt_q, 0, i * 32 + dd) for dd in range(32)])
    with jax.named_scope("preq"):
        loop(nch - 2, pre_queries)
    with jax.named_scope("preq_rel"):
        loop(2, lambda i: pre_queries(i + nch - 2, i + 1))

    scale = DH ** -0.5

    def masks(mode, q0=0):
        rows = ROWS if mode == 0 else ROWS - SEG
        qi = lax.broadcasted_iota(jnp.int32, (rows - q0, 128), 0) + q0
        kj = lax.broadcasted_iota(jnp.int32, (rows - q0, 128), 1)

        def layer_of(i):
            xl = (i - 2 * M) // SEG if mode == 0 else mode - 1
            return jnp.where(i < 2 * M, i // M, xl)
        same = (layer_of(qi) == layer_of(kj)) & (kj < rows)
        vis = same & ((qi < 2 * M) | (qi >= kj))
        fill = jnp.where(same, -1e9 / scale, -jnp.inf).astype(F32)
        return vis, fill

    mem0 = mem0_ref[...].astype(F32)
    hbuf[0:16, :] = jnp.concatenate([mem0, mem0], axis=0).astype(BF16)
    hbuf[16:48, :] = _ln(x_s[0:SEG, :].astype(F32)).astype(BF16)
    obuf[...] = jnp.zeros((2 * SEG, D), F32)
    x2_s[...] = jnp.zeros(x2_s.shape, F32)

    def seg_row(seg):
        if isinstance(seg, int):
            return min(max(seg, 0), NSEG - 1) * SEG
        return pl.multiple_of(jnp.clip(seg, 0, NSEG - 1) * SEG, SEG)

    def gate(xa, r0):
        y = jnp.concatenate([y_s[g, pl.ds(r0, SEG), :] for g in range(NLB)], axis=1)
        return xa + _r(_r(_ln(xa)) * y)

    def attention(h, vis, fill, chained, before_oproj=None, early=None):
        q0 = h.shape[0] - vis.shape[0]
        if early is not None:
            hrest = jnp.concatenate([h[:2 * M], h[2 * M + SEG:]], axis=0)
            qrow = pl.multiple_of(early * SEG, SEG)
            units = [u for n in range(PPS)
                     for u in mac_units(pl.multiple_of(early * (8 * PPS), 8 * PPS) + 8 * n, 1)]

        def proj(g):
            if g == 0 and chained and q0 == 0:
                kc = D - 128
                part = [jnp.dot(h[:, :kc], wslab(0, j)[:kc], preferred_element_type=F32)
                        for j in range(HG)]
                q = [(jnp.dot(h[:, kc:], wslab(0, j)[kc:], preferred_element_type=F32)
                      + part[j]).astype(BF16) for j in range(HG)]
                return [q] + [[jnp.dot(h, wslab(t, j), preferred_element_type=F32)
                               for j in range(HG)] for t in range(1, 3)]
            res = [[None] * HG for _ in range(3)]
            order = [(t, j) for j in range(HG) for t in range(2)] + [(2, j) for j in range(HG)]
            for n, (t, j) in enumerate(order):
                hd = g * HG + j
                pre = early is not None and t == 0 and hd < NQH
                lhs = hrest if pre else (h if t else h[q0:])
                r = jnp.dot(lhs, wslab(t, hd), preferred_element_type=F32)
                if early is not None and n % TOKP[0] == TOKP[1] and units:
                    units.pop(0)(jnp.minimum(jnp.abs(r[0:8]), 0.0))
                if t == 0:
                    r = r.astype(BF16)
                if pre:
                    r = jnp.concatenate([r[:2 * M], qh_s[hd, pl.ds(qrow, SEG), :], r[2 * M:]], axis=0)
                res[t][j] = r
            return res

        def pad(kv):
            return jnp.concatenate([kv, jnp.zeros((128 - kv.shape[0], DH), F32)], axis=0).astype(BF16)

        def probs(qkv):
            scs = [lax.dot_general(qkv[0][j], pad(qkv[1][j]), (((1,), (1,)), ((), ())),
                                   preferred_element_type=F32) for j in range(HG)]
            ps = []
            for sc in scs:
                sc = jnp.where(vis, sc, fill)
                e = jnp.exp2((sc - jnp.max(sc, axis=-1, keepdims=True)) * (scale * math.log2(math.e)))
                den = jnp.sum(e, axis=-1, keepdims=True)
                r = pl.reciprocal(den, approx=True)
                r = r * (2.0 - den * r)
                ps.append((e * r).astype(BF16))
            return ps

        def oproj(os_, h0):
            oc = jnp.concatenate(os_, axis=1).astype(BF16)
            k0, k1 = h0 * DH, (h0 + len(os_)) * DH
            res = []
            for n in range(NLB):
                if before_oproj is not None:
                    w = wo_s[k0:k1, n * 128:(n + 1) * 128]
                    wo_t[n, k0 // 2:k1 // 2, :] = pltpu.bitcast(w, U32)
                else:
                    w = pltpu.bitcast(wo_t[n, k0 // 2:k1 // 2, :], BF16)
                res.append(jnp.dot(oc, w, preferred_element_type=F32))
            return res

        heads = []
        qkv = proj(0)
        oa = None
        for g in range(NG):
            ps = probs(qkv)
            vs = qkv[2]
            if g + 1 < NG:
                qkv = proj(g + 1)
            else:
                if before_oproj is not None:
                    before_oproj()
                oa = oproj(heads[:H // 2], 0)
            heads += [jnp.dot(ps[j], pad(vs[j]), preferred_element_type=F32)
                      for j in range(HG)]
        assert early is None or not units
        ob = oproj(heads[H // 2:], H // 2)
        return jnp.concatenate([b + a for a, b in zip(oa, ob)], axis=1)

    def post2(s):
        r3 = seg_row(s - 1 - LAG)
        xo = gate(_r(x2_s[(s + 4 - 1 - LAG) % 4] + obuf[SEG:2 * SEG, :]), r3)
        out_s[pl.ds(r3, SEG), :] = xo.astype(BF16)

    def step(s, mode, vis, fill, chained=False, before_oproj=None, early=None):
        if mode == 0:
            h = hbuf[...]
        elif mode == 1:
            h = hbuf[0:48, :]
        else:
            h = jnp.concatenate([hbuf[0:16, :], hbuf[48:80, :]], axis=0)
        last = isinstance(s, int) and s == NSEG + LAG - 1
        if last:
            post2(s)
            obuf[SEG:2 * SEG, :] = _r(attention(h, vis, fill, chained))
            return
        r1 = seg_row(s - 1)
        xb2 = _r(gate(_r(x_s[pl.ds(r1, SEG), :].astype(F32) + obuf[0:SEG, :]), r1))
        h2n = _ln(xb2).astype(BF16)
        if mode != 1:
            post2(s)
        x2_s[(s + 4 - 1) % 4] = xb2
        if mode != 2:
            h1n = _ln(x_s[pl.ds(seg_row(s + 1), SEG), :].astype(F32)).astype(BF16)

        o = attention(h, vis, fill, chained, before_oproj, early)

        mem2 = mem0 if mode == 1 else o[M:2 * M]
        hbuf[0:16, :] = jnp.concatenate([o[0:M], mem2], axis=0).astype(BF16)
        if mode != 2:
            hbuf[16:48, :] = h1n
        hbuf[48:80, :] = h2n
        if mode == 0:
            obuf[...] = _r(o[2 * M:])
        elif mode == 1:
            obuf[0:SEG, :] = _r(o[2 * M:])
        else:
            obuf[SEG:2 * SEG, :] = _r(o[2 * M:])

    with jax.named_scope("pro"):
        vis, fill = masks(1)
        step(0, 1, vis, fill, False, wo_copy.wait)
        step(1, 1, vis, fill, True)
    xb_copy.wait()
    vis, fill = masks(0)
    with jax.named_scope("main_a"):
        loop(NA, lambda i: step(i + LAG, 0, vis, fill, early=i))
    with jax.named_scope("conv_e"):
        loop(HB // 2, lambda j: (inv_stage(HB + 2 * j), inv_stage(HB + 2 * j + 1)))
    with jax.named_scope("main_b"):
        loop((NSEG - LAG - NA) // UB, lambda i: [step(UB * i + u + LAG + NA, 0, vis, fill, u > 0)
                                                 for u in range(UB)])
    done = (NSEG - 1 - LAG) * SEG
    out_a = pltpu.make_async_copy(out_s.at[0:done, :], out_hbm.at[0:done, :], sem.at[SW + 8])
    out_a.start()
    with jax.named_scope("epi"):
        vis, fill = masks(2)
        step(NSEG, 2, vis, fill)
        step(NSEG + 1, 2, *masks(2, 2 * M), True)
    post2(NSEG + LAG)
    out_b = pltpu.make_async_copy(out_s.at[done:S, :], out_hbm.at[done:S, :], sem.at[SW + 9])
    out_b.start()
    out_a.wait()
    out_b.wait()


@jax.jit
def pallas_interleave_layers__memory_aug_recurrent_mem_tr__ssm_conv_h3__prompt_kernel(
    A_x, A_mem0, A_Wq, A_Wk, A_Wv, A_Wo, A_seg_len,
    B_q, B_k, B_v, B_shift_k, B_ssm_k, B_ssm_D,
):
    del A_seg_len, B_q
    assert A_x.shape == (1, S, D) and A_Wq.shape == (D, H, DH)
    hbm = pl.BlockSpec(memory_space=pl.ANY)
    out = pl.pallas_call(
        _kernel,
        out_shape=jax.ShapeDtypeStruct((S, D), BF16),
        in_specs=[hbm] * 11,
        out_specs=hbm,
        scratch_shapes=[
            pltpu.VMEM((S, D), BF16),
            pltpu.VMEM((S, D), BF16),
            pltpu.VMEM((S, D), BF16),
            pltpu.VMEM((HB, D, 2 * TB), BF16),
            pltpu.VMEM((3, D, H, DH), BF16),
            pltpu.VMEM(((H + 1) * WP, 128), U32),
            pltpu.VMEM(((2 * H + 1) * WP, 128), U32),
            pltpu.VMEM((H * DH, D), BF16),
            pltpu.VMEM((NLB, H * DH // 2, 128), U32),
            pltpu.VMEM((TB, TB), BF16),
            pltpu.VMEM((2, TB, TB), BF16),
            pltpu.VMEM((2, TB // 2, 3 * TB), BF16),
            pltpu.VMEM((2, NLB, S // 2 + 8, 128), F32),
            pltpu.VMEM((NB, 2, NLB * TB, 128), F32),
            pltpu.VMEM((NB, 3, NLB * TB, 128), F32),
            pltpu.VMEM((NB + 1, 2, NLB * TB, 128), F32),
            pltpu.VMEM((NLB, S + 8, 128), F32),
            pltpu.VMEM((ROWS, D), BF16),
            pltpu.VMEM((2 * SEG, D), F32),
            pltpu.VMEM((4, SEG, D), F32),
            pltpu.VMEM((S, D), BF16),
            pltpu.VMEM((NA * SEG, D), BF16),
            pltpu.VMEM((NQH, NA * SEG, DH), BF16),
            pltpu.VMEM((M, D), BF16),
            pltpu.VMEM((KS, D), BF16),
            pltpu.VMEM((D,), BF16),
            pltpu.SemaphoreType.DMA((HB // 2 + 10,)),
        ],
        compiler_params=pltpu.CompilerParams(vmem_limit_bytes=120 * 1024 * 1024),
    )(A_x.reshape(S, D), A_mem0.reshape(M, D), A_Wq, A_Wk, A_Wv,
      A_Wo.reshape(H * DH, D), B_k.reshape(S, D), B_v.reshape(S, D),
      B_shift_k.T, B_ssm_k, B_ssm_D)
    return out.reshape(1, S, D)
```

```python
import functools
import math

import jax
import jax.numpy as jnp
from jax import lax
import jax.experimental.pallas as pl
import jax.experimental.pallas.tpu as pltpu

F32 = jnp.float32
BF16 = jnp.bfloat16
U32 = jnp.uint32

S = 2048
D = 640
H = 32
DH = 128
M = 8
SEG = 32
NSEG = S // SEG
KS = 4
LAG = 2
ROWS = 2 * M + 2 * SEG
HG = 4
NG = H // HG
NLB = D // 128
TB = 128
NB = S // TB
HB = NB // 2
NPOS = NLB * TB // 8
NA = 20
PPS = 4
UCUT = (range(0, 3), range(3, 6), range(6, 9), range(9, 16))
TOKP = (2, 1)
NQH = 26
UA = 2
UB = 3
WP = 324


def _ln(x, toks=None):
    m = jnp.mean(x, axis=-1, keepdims=True)
    c = x - m
    v = jnp.mean(c * c, axis=-1, keepdims=True)
    r = lax.rsqrt(v + 1e-5)
    if toks is not None:
        toks.append(jnp.minimum(r, 0.0))
    return c * r


def _r(x):
    return x.astype(BF16).astype(F32)


def _split(x):
    hi = pltpu.bitcast(pltpu.bitcast(x, U32) & jnp.uint32(0xFFFF0000), F32)
    return hi, x - hi


def _bf(x):
    return jnp.concatenate([x[:, g:g + 128].astype(BF16)
                            for g in range(0, x.shape[1], 128)], axis=1)


def _basis(r, t):
    b = r & 63
    f = jnp.where(b < 32, 2 * b, 2 * b - 63)
    n = ((2 * f + 1) * t - jnp.where(r >= 64, TB, 0)) & (4 * TB - 1)
    n = jnp.where(n >= 2 * TB, n - 4 * TB, n)
    return jnp.cos(n.astype(F32) * (2.0 * math.pi / (4 * TB)))


def _halves(x):
    w = pltpu.bitcast(x, U32)
    return (pltpu.bitcast(w << 16, F32),
            pltpu.bitcast(w & jnp.uint32(0xFFFF0000), F32))


def _kernel(x_hbm, mem0_hbm, wq_hbm, wk_hbm, wv_hbm, wo_hbm,
            k_hbm, v_hbm, shk_hbm, ssmk_hbm, ssmd_hbm,
            out_hbm,
            x_s, k_s, v_s, ssmk_s, wraw, wt_q, wt_kv, wo_s, wo_t,
            perm_s, fu_s, inv_s, kpad, u_s, kf_s, c_s, y_s,
            hbuf, obuf, x2_s, out_s, hl_s, qh_s, mem0_ref, shk_ref, ssmd_ref,
            sem):
    XH = (LAG + NA) * SEG
    SW = HB // 2

    def conv_copies(jp, sm):
        rows = pl.ds(jp * 2 * TB if isinstance(jp, int) else pl.multiple_of(jp * 2 * TB, 2 * TB), 2 * TB)
        return [pltpu.make_async_copy(ssmk_hbm.at[:, rows], ssmk_s.at[jp], sm),
                pltpu.make_async_copy(k_hbm.at[rows, :], k_s.at[rows, :], sm),
                pltpu.make_async_copy(v_hbm.at[rows, :], v_s.at[rows, :], sm)]
    w_copies = [pltpu.make_async_copy(w, wraw.at[t], sem.at[SW + t])
                for t, w in enumerate((wq_hbm, wk_hbm, wv_hbm))]
    wo_copy = pltpu.make_async_copy(wo_hbm, wo_s, sem.at[SW + 3])
    late_copies = [c for jp in range(HB // 2, HB) for c in conv_copies(jp, sem.at[SW + 4])]
    small_copies = [pltpu.make_async_copy(src, dst, sem.at[SW + 5])
                    for src, dst in ((shk_hbm, shk_ref), (ssmd_hbm, ssmd_ref), (mem0_hbm, mem0_ref))]
    xa_copy = pltpu.make_async_copy(x_hbm.at[0:XH, :], x_s.at[0:XH, :], sem.at[SW + 6])
    xb_copy = pltpu.make_async_copy(x_hbm.at[XH:, :], x_s.at[XH:, :], sem.at[SW + 7])
    for c in (small_copies + [c for jp in range(HB // 2) for c in conv_copies(jp, sem.at[jp])] + late_copies
              + [xa_copy] + w_copies + [wo_copy, xb_copy]):
        c.start()

    hb = TB // 2
    ri = lax.broadcasted_iota(jnp.int32, (TB, TB), 0)
    ci = lax.broadcasted_iota(jnp.int32, (TB, TB), 1)
    perm_s[...] = jnp.where(ci == 2 * (ri & 63) + (ri >> 6), 1.0, 0.0).astype(BF16)
    tab = _basis(ri, 2 * (ci & 63) + (ci >> 6))
    hi, lo = _split(tab)
    fu_s[0] = jnp.where(ci < hb, hi, pltpu.roll(lo, hb, 1)).astype(BF16)
    fu_s[1] = jnp.where(ci < hb, pltpu.roll(hi, hb, 1), lo).astype(BF16)
    gh, gl = _split(tab.T * (1.0 / TB))
    ginv = _bf(jnp.concatenate([gh, gl, gh], axis=1))
    inv_s[0] = ginv[:hb]
    inv_s[1] = ginv[hb:]

    for c in small_copies:
        c.wait()
    shk_t = shk_ref[...].astype(F32)
    taps = [[shk_t[j:j + 1, g * 128:(g + 1) * 128] for g in range(NLB)] for j in range(KS)]
    dvec = ssmd_ref[...].astype(F32).reshape(1, D)
    for g in range(NLB):
        kpad[0, g, 0:8, :] = jnp.zeros((8, 128), F32)
        kpad[1, g, 0:8, :] = jnp.zeros((8, 128), F32)
    c_s[0] = jnp.zeros(c_s.shape[1:], F32)

    def spectrum(e, o):
        fe = jnp.dot(fu_s[0], jnp.concatenate([e, e], axis=0).astype(BF16), preferred_element_type=F32)
        fo = jnp.dot(fu_s[1], jnp.concatenate([o, o], axis=0).astype(BF16), preferred_element_type=F32)
        return ((fe[:hb] + fo[:hb], fe[hb:] + fo[hb:]), (fe[:hb] - fo[:hb], fo[hb:] - fe[hb:]))

    def fwd_stage(jp, first):
        if first:
            for c in conv_copies(jp, sem.at[jp]):
                c.wait()
        kts = [lax.dot_general(perm_s[...], ssmk_s[jp, :, n * TB:(n + 1) * TB], (((1,), (1,)), ((), ())),
                               preferred_element_type=F32) for n in range(2)]
        for n, kt in enumerate(kts):
            j = 2 * jp + n
            r0 = pl.multiple_of(j * TB, TB)
            q0 = pl.multiple_of(j * hb, hb) + 8
            for g in range(NLB):
                lb = slice(g * 128, (g + 1) * 128)
                halves = (slice(g * TB, g * TB + hb), slice(g * TB + hb, (g + 1) * TB))
                for rows, (kr, ki) in zip(halves, spectrum(kt[:hb, lb], kt[hb:, lb])):
                    if first and n == 0:
                        kr = kr + jnp.where(j == 0, dvec[:, lb], 0.0)
                    kf_s[j, 0, rows] = kr
                    kf_s[j, 1, rows] = ki - kr
                    kf_s[j, 2, rows] = kr + ki
                ke, ko = _halves(k_s[pl.ds(r0, TB), lb])
                ve, vo = _halves(v_s[pl.ds(r0, TB), lb])
                kpad[0, g, pl.ds(q0, hb), :] = ke
                kpad[1, g, pl.ds(q0, hb), :] = ko
                ke1 = kpad[0, g, pl.ds(q0 - 1, hb), :]
                ko1 = kpad[1, g, pl.ds(q0 - 1, hb), :]
                ko2 = kpad[1, g, pl.ds(q0 - 2, hb), :]
                t0, t1, t2, t3 = (taps[t][g] for t in range(KS))
                e = (ke * t0 + ko1 * t1 + ke1 * t2 + ko2 * t3) * ve
                o = (ko * t0 + ke * t1 + ko1 * t2 + ke1 * t3) * vo
                for rows, (ur, ui) in zip(halves, spectrum(e, o)):
                    u_s[j, 0, rows] = ur
                    u_s[j, 1, rows] = ui

    def mac_units(row, half):
        rs = pl.ds(row, 8)
        state = {}

        def unit(p, avals, final, tok=None):
            acc = state.setdefault(p, dict(state.get(0, {})))
            for a in avals:
                u = u_s[a, 0, rs] + u_s[a, 1, rs] if p == 0 else u_s[a, p - 1, rs]
                if tok is not None:
                    u = u + tok
                for i in range(max(a, half * HB), half * HB + HB):
                    t = u * kf_s[i - a, p, rs]
                    acc[i] = t if i not in acc else (acc[i] - t if p == 2 else acc[i] + t)
            if final and p:
                for i, v in acc.items():
                    c_s[i + 1, 2 - p, rs] = v

        subs = UCUT if half else (range(HB),)
        return [functools.partial(unit, p, avals, n == len(subs) - 1)
                for p in range(3) for n, avals in enumerate(subs)]

    def inv_stage(i):
        q = TB // 4
        for g in range(NLB):
            re, im = [], []
            for b in range(4):
                rows = slice(g * TB + b * q, g * TB + (b + 1) * q)
                cr, ci_ = c_s[i + 1, 0, rows], c_s[i + 1, 1, rows]
                pr, pi = c_s[i, 0, rows], c_s[i, 1, rows]
                re.append(cr + pi if b in (0, 3) else cr - pi)
                im.append(ci_ - pr if b in (0, 3) else ci_ + pr)
            pe = jnp.concatenate([re[0] + re[2], re[1] + re[3], im[0] - im[2], im[1] - im[3]], axis=0)
            po = jnp.concatenate([re[0] - re[2], re[1] - re[3], im[0] + im[2], im[1] + im[3]], axis=0)
            for par, pp in enumerate((pe, po)):
                ph, plo = _split(pp)
                y_s[g, pl.ds(i * TB + par, hb, stride=2), :] = jnp.dot(
                    inv_s[par], jnp.concatenate([ph, ph, plo], axis=0).astype(BF16),
                    preferred_element_type=F32)

    def relayout_rows(t, dst, base, dp, tok=None):
        a = pltpu.bitcast(wraw[t, 2 * dp], U32)
        b = pltpu.bitcast(wraw[t, 2 * dp + 1], U32)
        if tok is not None:
            a = a | tok
        dst[pl.ds(base + dp, 16, stride=WP), :] = (a & jnp.uint32(0xFFFF)) | (b << 16)
        dst[pl.ds(base + 16 * WP + dp, 16, stride=WP), :] = (
            (a >> 16) | (b & jnp.uint32(0xFFFF0000)))

    def wslab(t, h):
        s0 = (max(t - 1, 0) * H + (h % 2) * 16 + h // 2) * WP
        return pltpu.bitcast((wt_kv if t else wt_q)[s0:s0 + D // 2, :], BF16)

    def loop(n, fn):
        def body(j, _):
            fn(j)
            return 0
        lax.fori_loop(0, n, body, 0)

    def norm_rows(c):
        r0 = c * TB if isinstance(c, int) else pl.multiple_of(c * TB, TB)
        hl_s[pl.ds(r0, TB), :] = _ln(x_s[pl.ds(r0 + LAG * SEG, TB), :].astype(F32)).astype(BF16)

    def pre_queries(c, t=None):
        if t is not None:
            pltpu.make_async_copy(wraw.at[t], wraw.at[t], sem.at[SW + t]).wait()
            base = (t - 1) * (H * WP)
        per = -(-(D // 2) // (2 * NQH))
        dp = 0
        for sub in range(2):
            r0 = pl.multiple_of((2 * c + sub) * QR, QR)
            hl = hl_s[pl.ds(r0, QR), :]
            for hd in range(NQH):
                r = jnp.dot(hl, wslab(0, hd), preferred_element_type=F32)
                qh_s[hd, pl.ds(r0, QR), :] = r.astype(BF16)
                if t is not None:
                    tok = pltpu.bitcast(jnp.minimum(jnp.abs(r[0:16]), 0.0), U32)
                    for _ in range(per):
                        if dp < D // 2:
                            relayout_rows(t, wt_kv, base, dp, tok)
                            dp += 1

    nch = NA * SEG // TB
    QR = TB // 2
    with jax.named_scope("conv_a"):
        loop(HB // 2, lambda j: fwd_stage(j, True))
    with jax.named_scope("conv_b"):
        loop(NPOS // 10, lambda j: [u() for n in range(10) for u in mac_units(pl.multiple_of(80 * j, 16) + 8 * n, 0)])
        loop(HB // 2, lambda j: (inv_stage(2 * j), inv_stage(2 * j + 1)))
    with jax.named_scope("conv_c"):
        for c in late_copies:
            c.wait()
        loop(HB // 2, lambda j: fwd_stage(HB // 2 + j, False))
    with jax.named_scope("norm"):
        xa_copy.wait()
        norm_rows(0)
        loop(nch // 2, lambda c: (norm_rows(2 * c + 1), norm_rows(2 * c + 2)))
    with jax.named_scope("rel0"):
        w_copies[0].wait()
        loop(D // 64, lambda i: [relayout_rows(0, wt_q, 0, i * 32 + dd) for dd in range(32)])
    with jax.named_scope("preq"):
        loop(nch - 2, pre_queries)
    with jax.named_scope("preq_rel"):
        loop(2, lambda i: pre_queries(i + nch - 2, i + 1))

    scale = DH ** -0.5

    def masks(mode, q0=0):
        rows = ROWS if mode == 0 else ROWS - SEG
        qi = lax.broadcasted_iota(jnp.int32, (rows - q0, 128), 0) + q0
        kj = lax.broadcasted_iota(jnp.int32, (rows - q0, 128), 1)

        def layer_of(i):
            xl = (i - 2 * M) // SEG if mode == 0 else mode - 1
            return jnp.where(i < 2 * M, i // M, xl)
        same = (layer_of(qi) == layer_of(kj)) & (kj < rows)
        vis = same & ((qi < 2 * M) | (qi >= kj))
        fill = jnp.where(same, -1e9 / scale, -jnp.inf).astype(F32)
        return vis, fill

    mem0 = mem0_ref[...].astype(F32)
    hbuf[0:16, :] = jnp.concatenate([mem0, mem0], axis=0).astype(BF16)
    hbuf[16:48, :] = _ln(x_s[0:SEG, :].astype(F32)).astype(BF16)
    obuf[...] = jnp.zeros((2 * SEG, D), F32)
    x2_s[...] = jnp.zeros(x2_s.shape, F32)

    def seg_row(seg):
        if isinstance(seg, int):
            return min(max(seg, 0), NSEG - 1) * SEG
        return pl.multiple_of(jnp.clip(seg, 0, NSEG - 1) * SEG, SEG)

    def gate(xa, r0, toks=None):
        y = jnp.concatenate([y_s[g, pl.ds(r0, xa.shape[0]), :] for g in range(NLB)], axis=1)
        return xa + _ln(xa, toks) * y

    def attention(h, vis, fill, chained, before_oproj=None, early=None, due=()):
        q0 = h.shape[0] - vis.shape[0]
        if early is not None:
            hrest = jnp.concatenate([h[:2 * M], h[2 * M + SEG:]], axis=0)
            qrow = pl.multiple_of(early * SEG, SEG)
            units = [u for n in range(PPS)
                     for u in mac_units(pl.multiple_of(early * (8 * PPS), 8 * PPS) + 8 * n, 1)]

        def proj(g):
            res = [[None] * HG for _ in range(3)]
            order = [(t, j) for j in range(HG) for t in range(2)] + [(2, j) for j in range(HG)]
            def operand(t, j):
                pre = early is not None and t == 0 and g * HG + j < NQH
                return pre, hrest if pre else (h if t else h[q0:])

            kc = D - 128
            nsplit = 4 if g == 0 and chained else 0
            part = [jnp.dot(operand(t, j)[1][:, :kc], wslab(t, j)[:kc], preferred_element_type=F32)
                    for t, j in order[:nsplit]]
            for n, (t, j) in enumerate(order):
                hd = g * HG + j
                pre, lhs = operand(t, j)
                if n < nsplit:
                    r = jnp.dot(lhs[:, kc:], wslab(t, hd)[kc:], preferred_element_type=F32) + part[n]
                else:
                    r = jnp.dot(lhs, wslab(t, hd), preferred_element_type=F32)
                if early is not None and n % TOKP[0] == TOKP[1] and units:
                    units.pop(0)(jnp.minimum(jnp.abs(r[0:8]), 0.0))
                if t == 0:
                    r = r.astype(BF16)
                if pre:
                    r = jnp.concatenate([r[:2 * M], qh_s[hd, pl.ds(qrow, SEG), :], r[2 * M:]], axis=0)
                res[t][j] = r
            return res

        def pad(kv):
            return jnp.concatenate([kv, jnp.zeros((128 - kv.shape[0], DH), F32)], axis=0).astype(BF16)

        def probs(qkv, g):
            scs = [lax.dot_general(qkv[0][j], pad(qkv[1][j]), (((1,), (1,)), ((), ())),
                                   preferred_element_type=F32) for j in range(HG)]
            ps = []
            for sc in scs:
                sc = jnp.where(vis, sc, fill)
                e = jnp.exp2((sc - jnp.max(sc, axis=-1, keepdims=True)) * (scale * math.log2(math.e)))
                den = jnp.sum(e, axis=-1, keepdims=True)
                if not ps and g >= NG - len(due):
                    e = jnp.concatenate([e[:16] + due[g - NG + len(due)], e[16:]], axis=0)
                r = pl.reciprocal(den, approx=True)
                r = r * (2.0 - den * r)
                ps.append((e * r).astype(BF16))
            return ps

        def oproj(os_, h0):
            oc = jnp.concatenate(os_, axis=1).astype(BF16)
            k0, k1 = h0 * DH, (h0 + len(os_)) * DH
            res = []
            for n in range(NLB):
                if before_oproj is not None:
                    w = wo_s[k0:k1, n * 128:(n + 1) * 128]
                    wo_t[n, k0 // 2:k1 // 2, :] = pltpu.bitcast(w, U32)
                else:
                    w = pltpu.bitcast(wo_t[n, k0 // 2:k1 // 2, :], BF16)
                res.append(jnp.dot(oc, w, preferred_element_type=F32))
            return res

        heads = []
        qkv = proj(0)
        oa = None
        for g in range(NG):
            ps = probs(qkv, g)
            vs = qkv[2]
            if g + 1 < NG:
                qkv = proj(g + 1)
            else:
                if before_oproj is not None:
                    before_oproj()
                oa = oproj(heads[:H // 2], 0)
            heads += [jnp.dot(ps[j], pad(vs[j]), preferred_element_type=F32)
                      for j in range(HG)]
        assert early is None or not units
        ob = oproj(heads[H // 2:], H // 2)
        return jnp.concatenate([b + a for a, b in zip(oa, ob)], axis=1)

    def post2(s, toks=None):
        r3 = seg_row(s - 1 - LAG)
        for r in (0, 16):
            xc = _r(x2_s[(s + 4 - 1 - LAG) % 4, r:r + 16] + obuf[SEG + r:SEG + r + 16, :])
            out_s[pl.ds(r3 + r, 16), :] = gate(xc, r3 + r, toks).astype(BF16)

    def step(s, mode, vis, fill, chained=False, before_oproj=None, early=None):
        if mode == 0:
            h = hbuf[...]
        elif mode == 1:
            h = hbuf[0:48, :]
        else:
            h = jnp.concatenate([hbuf[0:16, :], hbuf[48:80, :]], axis=0)
        toks = []
        if mode != 1:
            post2(s, toks)
        if isinstance(s, int) and s == NSEG + LAG - 1:
            obuf[SEG:2 * SEG, :] = attention(h, vis, fill, chained, due=toks)
            return
        r1 = seg_row(s - 1)
        rn = seg_row(s + 1)
        h1n, h2n = [], []
        for r in (0, 16):
            xa = _r(x_s[pl.ds(r1 + r, 16), :].astype(F32) + obuf[r:r + 16, :])
            xb2 = _r(gate(xa, r1 + r))
            h2n.append(_ln(xb2, toks).astype(BF16))
            x2_s[(s + 4 - 1) % 4, r:r + 16] = xb2
        if mode != 2:
            for r in (0, 16):
                h1n.append(_ln(x_s[pl.ds(rn + r, 16), :].astype(F32), toks).astype(BF16))

        o = attention(h, vis, fill, chained, before_oproj, early, toks)

        mem2 = mem0 if mode == 1 else o[M:2 * M]
        hbuf[0:16, :] = jnp.concatenate([o[0:M], mem2], axis=0).astype(BF16)
        for n, v in enumerate(h1n):
            hbuf[16 + 16 * n:32 + 16 * n, :] = v
        for n, v in enumerate(h2n):
            hbuf[48 + 16 * n:64 + 16 * n, :] = v
        if mode == 0:
            obuf[...] = o[2 * M:]
        elif mode == 1:
            obuf[0:SEG, :] = o[2 * M:]
        else:
            obuf[SEG:2 * SEG, :] = o[2 * M:]

    with jax.named_scope("pro"):
        vis, fill = masks(1)
        step(0, 1, vis, fill, False, wo_copy.wait)
        step(1, 1, vis, fill, True)
    xb_copy.wait()
    vis, fill = masks(0)
    with jax.named_scope("main_a"):
        loop(NA // UA, lambda i: [step(UA * i + u + LAG, 0, vis, fill, u > 0, early=UA * i + u)
                                  for u in range(UA)])
    with jax.named_scope("conv_e"):
        loop(HB // 2, lambda j: (inv_stage(HB + 2 * j), inv_stage(HB + 2 * j + 1)))
    with jax.named_scope("main_b"):
        loop((NSEG - LAG - NA) // UB, lambda i: [step(UB * i + u + LAG + NA, 0, vis, fill, u > 0)
                                                 for u in range(UB)])
    done = (NSEG - 1 - LAG) * SEG
    out_a = pltpu.make_async_copy(out_s.at[0:done, :], out_hbm.at[0:done, :], sem.at[SW + 8])
    out_a.start()
    with jax.named_scope("epi"):
        vis, fill = masks(2)
        step(NSEG, 2, vis, fill)
        step(NSEG + 1, 2, *masks(2, 2 * M), True)
    post2(NSEG + LAG)
    out_b = pltpu.make_async_copy(out_s.at[done:S, :], out_hbm.at[done:S, :], sem.at[SW + 9])
    out_b.start()
    out_a.wait()
    out_b.wait()


@jax.jit
def pallas_interleave_layers__memory_aug_recurrent_mem_tr__ssm_conv_h3__prompt_kernel(
    A_x, A_mem0, A_Wq, A_Wk, A_Wv, A_Wo, A_seg_len,
    B_q, B_k, B_v, B_shift_k, B_ssm_k, B_ssm_D,
):
    del A_seg_len, B_q
    assert A_x.shape == (1, S, D) and A_Wq.shape == (D, H, DH)
    hbm = pl.BlockSpec(memory_space=pl.ANY)
    out = pl.pallas_call(
        _kernel,
        out_shape=jax.ShapeDtypeStruct((S, D), BF16),
        in_specs=[hbm] * 11,
        out_specs=hbm,
        scratch_shapes=[
            pltpu.VMEM((S, D), BF16),
            pltpu.VMEM((S, D), BF16),
            pltpu.VMEM((S, D), BF16),
            pltpu.VMEM((HB, D, 2 * TB), BF16),
            pltpu.VMEM((3, D, H, DH), BF16),
            pltpu.VMEM(((H + 1) * WP, 128), U32),
            pltpu.VMEM(((2 * H + 1) * WP, 128), U32),
            pltpu.VMEM((H * DH, D), BF16),
            pltpu.VMEM((NLB, H * DH // 2, 128), U32),
            pltpu.VMEM((TB, TB), BF16),
            pltpu.VMEM((2, TB, TB), BF16),
            pltpu.VMEM((2, TB // 2, 3 * TB), BF16),
            pltpu.VMEM((2, NLB, S // 2 + 8, 128), F32),
            pltpu.VMEM((NB, 2, NLB * TB, 128), F32),
            pltpu.VMEM((NB, 3, NLB * TB, 128), F32),
            pltpu.VMEM((NB + 1, 2, NLB * TB, 128), F32),
            pltpu.VMEM((NLB, S + 8, 128), F32),
            pltpu.VMEM((ROWS, D), BF16),
            pltpu.VMEM((2 * SEG, D), F32),
            pltpu.VMEM((4, SEG, D), F32),
            pltpu.VMEM((S, D), BF16),
            pltpu.VMEM((NA * SEG, D), BF16),
            pltpu.VMEM((NQH, NA * SEG, DH), BF16),
            pltpu.VMEM((M, D), BF16),
            pltpu.VMEM((KS, D), BF16),
            pltpu.VMEM((D,), BF16),
            pltpu.SemaphoreType.DMA((HB // 2 + 10,)),
        ],
        compiler_params=pltpu.CompilerParams(vmem_limit_bytes=120 * 1024 * 1024),
    )(A_x.reshape(S, D), A_mem0.reshape(M, D), A_Wq, A_Wk, A_Wv,
      A_Wo.reshape(H * DH, D), B_k.reshape(S, D), B_v.reshape(S, D),
      B_shift_k.T, B_ssm_k, B_ssm_D)
    return out.reshape(1, S, D)
```

```python
import functools
import math

import jax
import jax.numpy as jnp
from jax import lax
import jax.experimental.pallas as pl
import jax.experimental.pallas.tpu as pltpu

F32 = jnp.float32
BF16 = jnp.bfloat16
U32 = jnp.uint32

S = 2048
D = 640
H = 32
DH = 128
M = 8
SEG = 32
NSEG = S // SEG
KS = 4
LAG = 2
ROWS = 2 * M + 2 * SEG
HG = 4
NG = H // HG
NLB = D // 128
TB = 128
NB = S // TB
HB = NB // 2
NPOS = NLB * TB // 8
NA = 20
PPS = 4
UCUT = (range(0, 3), range(3, 6), range(6, 9), range(9, 16))
TOKP = (2, 1)
NQH = 28
UA = 2
UB = 3
WP = 324


def _ln(x, toks=None):
    m = jnp.mean(x, axis=-1, keepdims=True)
    c = x - m
    v = jnp.mean(c * c, axis=-1, keepdims=True)
    r = lax.rsqrt(v + 1e-5)
    if toks is not None:
        toks.append(jnp.minimum(r, 0.0))
    return c * r


def _r(x):
    return x.astype(BF16).astype(F32)


def _split(x):
    hi = pltpu.bitcast(pltpu.bitcast(x, U32) & jnp.uint32(0xFFFF0000), F32)
    return hi, x - hi


def _bf(x):
    return jnp.concatenate([x[:, g:g + 128].astype(BF16)
                            for g in range(0, x.shape[1], 128)], axis=1)


def _basis(r, t):
    b = r & 63
    f = jnp.where(b < 32, 2 * b, 2 * b - 63)
    n = ((2 * f + 1) * t - jnp.where(r >= 64, TB, 0)) & (4 * TB - 1)
    n = jnp.where(n >= 2 * TB, n - 4 * TB, n)
    return jnp.cos(n.astype(F32) * (2.0 * math.pi / (4 * TB)))


def _halves(x):
    w = pltpu.bitcast(x, U32)
    return (pltpu.bitcast(w << 16, F32),
            pltpu.bitcast(w & jnp.uint32(0xFFFF0000), F32))


def _kernel(x_hbm, mem0_hbm, wq_hbm, wk_hbm, wv_hbm, wo_hbm,
            k_hbm, v_hbm, shk_hbm, ssmk_hbm, ssmd_hbm,
            out_hbm,
            x_s, k_s, v_s, ssmk_s, wraw, wt_q, wt_kv, wo_s, wo_t,
            perm_s, fu_s, inv_s, kpad, u_s, kf_s, c_s, y_s,
            hbuf, obuf, x2_s, out_s, hl_s, qh_s, mem0_ref, shk_ref, ssmd_ref,
            sem):
    XH = (LAG + NA) * SEG
    SW = HB // 2

    def conv_copies(jp, sm):
        rows = pl.ds(jp * 2 * TB if isinstance(jp, int) else pl.multiple_of(jp * 2 * TB, 2 * TB), 2 * TB)
        return [pltpu.make_async_copy(ssmk_hbm.at[:, rows], ssmk_s.at[jp], sm),
                pltpu.make_async_copy(k_hbm.at[rows, :], k_s.at[rows, :], sm),
                pltpu.make_async_copy(v_hbm.at[rows, :], v_s.at[rows, :], sm)]
    w_copies = [pltpu.make_async_copy(w, wraw.at[t], sem.at[SW + t])
                for t, w in enumerate((wq_hbm, wk_hbm, wv_hbm))]
    wo_copy = pltpu.make_async_copy(wo_hbm, wo_s, sem.at[SW + 3])
    late_copies = [c for jp in range(HB // 2, HB) for c in conv_copies(jp, sem.at[SW + 4])]
    small_copies = [pltpu.make_async_copy(src, dst, sem.at[SW + 5])
                    for src, dst in ((shk_hbm, shk_ref), (ssmd_hbm, ssmd_ref), (mem0_hbm, mem0_ref))]
    xa_copy = pltpu.make_async_copy(x_hbm.at[0:XH, :], x_s.at[0:XH, :], sem.at[SW + 6])
    xb_copy = pltpu.make_async_copy(x_hbm.at[XH:, :], x_s.at[XH:, :], sem.at[SW + 7])
    for c in (small_copies + [c for jp in range(HB // 2) for c in conv_copies(jp, sem.at[jp])] + late_copies
              + [xa_copy] + w_copies + [wo_copy, xb_copy]):
        c.start()

    hb = TB // 2
    ri = lax.broadcasted_iota(jnp.int32, (TB, TB), 0)
    ci = lax.broadcasted_iota(jnp.int32, (TB, TB), 1)
    perm_s[...] = jnp.where(ci == 2 * (ri & 63) + (ri >> 6), 1.0, 0.0).astype(BF16)
    tab = _basis(ri, 2 * (ci & 63) + (ci >> 6))
    hi, lo = _split(tab)
    fu_s[0] = jnp.where(ci < hb, hi, pltpu.roll(lo, hb, 1)).astype(BF16)
    fu_s[1] = jnp.where(ci < hb, pltpu.roll(hi, hb, 1), lo).astype(BF16)
    gh, gl = _split(tab.T * (1.0 / TB))
    ginv = _bf(jnp.concatenate([gh, gl, gh], axis=1))
    inv_s[0] = ginv[:hb]
    inv_s[1] = ginv[hb:]

    for c in small_copies:
        c.wait()
    shk_t = shk_ref[...].astype(F32)
    taps = [[shk_t[j:j + 1, g * 128:(g + 1) * 128] for g in range(NLB)] for j in range(KS)]
    dvec = ssmd_ref[...].astype(F32).reshape(1, D)
    for g in range(NLB):
        kpad[0, g, 0:8, :] = jnp.zeros((8, 128), F32)
        kpad[1, g, 0:8, :] = jnp.zeros((8, 128), F32)
    c_s[0] = jnp.zeros(c_s.shape[1:], F32)

    def spectrum(e, o):
        fe = jnp.dot(fu_s[0], jnp.concatenate([e, e], axis=0).astype(BF16), preferred_element_type=F32)
        fo = jnp.dot(fu_s[1], jnp.concatenate([o, o], axis=0).astype(BF16), preferred_element_type=F32)
        return ((fe[:hb] + fo[:hb], fe[hb:] + fo[hb:]), (fe[:hb] - fo[:hb], fo[hb:] - fe[hb:]))

    def fwd_stage(jp, first):
        if first:
            for c in conv_copies(jp, sem.at[jp]):
                c.wait()
        kts = [lax.dot_general(perm_s[...], ssmk_s[jp, :, n * TB:(n + 1) * TB], (((1,), (1,)), ((), ())),
                               preferred_element_type=F32) for n in range(2)]
        for n, kt in enumerate(kts):
            j = 2 * jp + n
            r0 = pl.multiple_of(j * TB, TB)
            q0 = pl.multiple_of(j * hb, hb) + 8
            for g in range(NLB):
                lb = slice(g * 128, (g + 1) * 128)
                halves = (slice(g * TB, g * TB + hb), slice(g * TB + hb, (g + 1) * TB))
                for rows, (kr, ki) in zip(halves, spectrum(kt[:hb, lb], kt[hb:, lb])):
                    if first and n == 0:
                        kr = kr + jnp.where(j == 0, dvec[:, lb], 0.0)
                    kf_s[j, 0, rows] = kr
                    kf_s[j, 1, rows] = ki - kr
                    kf_s[j, 2, rows] = kr + ki
                ke, ko = _halves(k_s[pl.ds(r0, TB), lb])
                ve, vo = _halves(v_s[pl.ds(r0, TB), lb])
                kpad[0, g, pl.ds(q0, hb), :] = ke
                kpad[1, g, pl.ds(q0, hb), :] = ko
                ke1 = kpad[0, g, pl.ds(q0 - 1, hb), :]
                ko1 = kpad[1, g, pl.ds(q0 - 1, hb), :]
                ko2 = kpad[1, g, pl.ds(q0 - 2, hb), :]
                t0, t1, t2, t3 = (taps[t][g] for t in range(KS))
                e = (ke * t0 + ko1 * t1 + ke1 * t2 + ko2 * t3) * ve
                o = (ko * t0 + ke * t1 + ko1 * t2 + ke1 * t3) * vo
                for rows, (ur, ui) in zip(halves, spectrum(e, o)):
                    u_s[j, 0, rows] = ur
                    u_s[j, 1, rows] = ui

    def mac_units(row, half):
        rs = pl.ds(row, 8)
        state = {}

        def unit(p, avals, final, tok=None):
            acc = state.setdefault(p, dict(state.get(0, {})))
            for a in avals:
                u = u_s[a, 0, rs] + u_s[a, 1, rs] if p == 0 else u_s[a, p - 1, rs]
                if tok is not None:
                    u = u + tok
                for i in range(max(a, half * HB), half * HB + HB):
                    t = u * kf_s[i - a, p, rs]
                    acc[i] = t if i not in acc else (acc[i] - t if p == 2 else acc[i] + t)
            if final and p:
                for i, v in acc.items():
                    c_s[i + 1, 2 - p, rs] = v

        subs = UCUT if half else (range(HB),)
        return [functools.partial(unit, p, avals, n == len(subs) - 1)
                for p in range(3) for n, avals in enumerate(subs)]

    def inv_stage(i):
        q = TB // 4
        for g in range(NLB):
            re, im = [], []
            for b in range(4):
                rows = slice(g * TB + b * q, g * TB + (b + 1) * q)
                cr, ci_ = c_s[i + 1, 0, rows], c_s[i + 1, 1, rows]
                pr, pi = c_s[i, 0, rows], c_s[i, 1, rows]
                re.append(cr + pi if b in (0, 3) else cr - pi)
                im.append(ci_ - pr if b in (0, 3) else ci_ + pr)
            pe = jnp.concatenate([re[0] + re[2], re[1] + re[3], im[0] - im[2], im[1] - im[3]], axis=0)
            po = jnp.concatenate([re[0] - re[2], re[1] - re[3], im[0] + im[2], im[1] + im[3]], axis=0)
            for par, pp in enumerate((pe, po)):
                ph, plo = _split(pp)
                y_s[g, pl.ds(i * TB + par, hb, stride=2), :] = jnp.dot(
                    inv_s[par], jnp.concatenate([ph, ph, plo], axis=0).astype(BF16),
                    preferred_element_type=F32)

    def relayout_rows(t, dst, base, dp, tok=None):
        a = pltpu.bitcast(wraw[t, 2 * dp], U32)
        b = pltpu.bitcast(wraw[t, 2 * dp + 1], U32)
        if tok is not None:
            a = a | tok
        dst[pl.ds(base + dp, 16, stride=WP), :] = (a & jnp.uint32(0xFFFF)) | (b << 16)
        dst[pl.ds(base + 16 * WP + dp, 16, stride=WP), :] = (
            (a >> 16) | (b & jnp.uint32(0xFFFF0000)))

    def wslab(t, h):
        s0 = (max(t - 1, 0) * H + (h % 2) * 16 + h // 2) * WP
        return pltpu.bitcast((wt_kv if t else wt_q)[s0:s0 + D // 2, :], BF16)

    def loop(n, fn):
        def body(j, _):
            fn(j)
            return 0
        lax.fori_loop(0, n, body, 0)

    def norm_rows(c):
        nr = NA * SEG // 4
        r0 = pl.multiple_of(c * nr, 16)
        for r in range(0, nr, 16):
            hl_s[pl.ds(r0 + r, 16), :] = _ln(
                x_s[pl.ds(r0 + r + LAG * SEG, 16), :].astype(F32)).astype(BF16)

    def pre_queries(c, t=None):
        if t is not None:
            pltpu.make_async_copy(wraw.at[t], wraw.at[t], sem.at[SW + t]).wait()
            base = (t - 1) * (H * WP)
        per = -(-(D // 2) // (2 * NQH))
        dp = 0
        for sub in range(2):
            r0 = pl.multiple_of((2 * c + sub) * QR, QR)
            hl = hl_s[pl.ds(r0, QR), :]
            for hd in range(NQH):
                r = jnp.dot(hl, wslab(0, hd), preferred_element_type=F32)
                qh_s[hd, pl.ds(r0, QR), :] = r.astype(BF16)
                if t is not None:
                    tok = pltpu.bitcast(jnp.minimum(jnp.abs(r[0:16]), 0.0), U32)
                    for _ in range(per):
                        if dp < D // 2:
                            relayout_rows(t, wt_kv, base, dp, tok)
                            dp += 1

    nch = NA * SEG // TB
    QR = TB // 2
    with jax.named_scope("conv_a"):
        loop(HB // 2, lambda j: fwd_stage(j, True))
    with jax.named_scope("conv_b"):
        loop(NPOS // 10, lambda j: [u() for n in range(10) for u in mac_units(pl.multiple_of(80 * j, 16) + 8 * n, 0)])
        loop(HB // 2, lambda j: (inv_stage(2 * j), inv_stage(2 * j + 1)))
    with jax.named_scope("conv_c"):
        for c in late_copies:
            c.wait()
        xa_copy.wait()
        loop(HB // 2, lambda j: (fwd_stage(HB // 2 + j, False), norm_rows(j)))
    with jax.named_scope("rel0"):
        w_copies[0].wait()
        loop(D // 64, lambda i: [relayout_rows(0, wt_q, 0, i * 32 + dd) for dd in range(32)])
    with jax.named_scope("preq"):
        loop(nch - 2, pre_queries)
    with jax.named_scope("preq_rel"):
        loop(2, lambda i: pre_queries(i + nch - 2, i + 1))

    scale = DH ** -0.5

    def masks(mode, q0=0):
        rows = ROWS if mode == 0 else ROWS - SEG
        qi = lax.broadcasted_iota(jnp.int32, (rows - q0, 128), 0) + q0
        kj = lax.broadcasted_iota(jnp.int32, (rows - q0, 128), 1)

        def layer_of(i):
            xl = (i - 2 * M) // SEG if mode == 0 else mode - 1
            return jnp.where(i < 2 * M, i // M, xl)
        same = (layer_of(qi) == layer_of(kj)) & (kj < rows)
        vis = same & ((qi < 2 * M) | (qi >= kj))
        fill = jnp.where(same, -1e9 / scale, -jnp.inf).astype(F32)
        return vis, fill

    mem0 = mem0_ref[...].astype(F32)
    hbuf[0:16, :] = jnp.concatenate([mem0, mem0], axis=0).astype(BF16)
    hbuf[16:48, :] = _ln(x_s[0:SEG, :].astype(F32)).astype(BF16)
    obuf[...] = jnp.zeros((2 * SEG, D), F32)
    x2_s[...] = jnp.zeros(x2_s.shape, F32)

    def seg_row(seg):
        if isinstance(seg, int):
            return min(max(seg, 0), NSEG - 1) * SEG
        return pl.multiple_of(jnp.clip(seg, 0, NSEG - 1) * SEG, SEG)

    def gate(xa, r0, toks=None):
        y = jnp.concatenate([y_s[g, pl.ds(r0, xa.shape[0]), :] for g in range(NLB)], axis=1)
        return xa + _ln(xa, toks) * y

    def attention(h, vis, fill, chained, before_oproj=None, early=None, due=()):
        q0 = h.shape[0] - vis.shape[0]
        if early is not None:
            hrest = jnp.concatenate([h[:2 * M], h[2 * M + SEG:]], axis=0)
            qrow = pl.multiple_of(early * SEG, SEG)
            units = [u for n in range(PPS)
                     for u in mac_units(pl.multiple_of(early * (8 * PPS), 8 * PPS) + 8 * n, 1)]

        def proj(g):
            res = [[None] * HG for _ in range(3)]
            order = [(t, j) for j in range(HG) for t in range(2)] + [(2, j) for j in range(HG)]
            def operand(t, j):
                pre = early is not None and t == 0 and g * HG + j < NQH
                return pre, hrest if pre else (h if t else h[q0:])

            kc = D - 128
            nsplit = 4 if g == 0 and chained else 0
            part = [jnp.dot(operand(t, j)[1][:, :kc], wslab(t, j)[:kc], preferred_element_type=F32)
                    for t, j in order[:nsplit]]
            for n, (t, j) in enumerate(order):
                hd = g * HG + j
                pre, lhs = operand(t, j)
                if n < nsplit:
                    r = jnp.dot(lhs[:, kc:], wslab(t, hd)[kc:], preferred_element_type=F32) + part[n]
                else:
                    r = jnp.dot(lhs, wslab(t, hd), preferred_element_type=F32)
                if early is not None and n % TOKP[0] == TOKP[1] and units:
                    units.pop(0)(jnp.minimum(jnp.abs(r[0:8]), 0.0))
                if t == 0:
                    r = r.astype(BF16)
                if pre:
                    r = jnp.concatenate([r[:2 * M], qh_s[hd, pl.ds(qrow, SEG), :], r[2 * M:]], axis=0)
                res[t][j] = r
            return res

        def pad(kv):
            return jnp.concatenate([kv, jnp.zeros((128 - kv.shape[0], DH), F32)], axis=0).astype(BF16)

        def probs(qkv, g):
            scs = [lax.dot_general(qkv[0][j], pad(qkv[1][j]), (((1,), (1,)), ((), ())),
                                   preferred_element_type=F32) for j in range(HG)]
            ps = []
            for sc in scs:
                sc = jnp.where(vis, sc, fill)
                e = jnp.exp2((sc - jnp.max(sc, axis=-1, keepdims=True)) * (scale * math.log2(math.e)))
                den = jnp.sum(e, axis=-1, keepdims=True)
                if not ps and g >= NG - len(due):
                    e = jnp.concatenate([e[:16] + due[g - NG + len(due)], e[16:]], axis=0)
                r = pl.reciprocal(den, approx=True)
                r = r * (2.0 - den * r)
                ps.append((e * r).astype(BF16))
            return ps

        def oproj(os_, h0):
            oc = jnp.concatenate(os_, axis=1).astype(BF16)
            k0, k1 = h0 * DH, (h0 + len(os_)) * DH
            res = []
            for n in range(NLB):
                if before_oproj is not None:
                    w = wo_s[k0:k1, n * 128:(n + 1) * 128]
                    wo_t[n, k0 // 2:k1 // 2, :] = pltpu.bitcast(w, U32)
                else:
                    w = pltpu.bitcast(wo_t[n, k0 // 2:k1 // 2, :], BF16)
                res.append(jnp.dot(oc, w, preferred_element_type=F32))
            return res

        heads = []
        qkv = proj(0)
        oa = None
        for g in range(NG):
            ps = probs(qkv, g)
            vs = qkv[2]
            if g + 1 < NG:
                qkv = proj(g + 1)
            else:
                if before_oproj is not None:
                    before_oproj()
                oa = oproj(heads[:H // 2], 0)
            heads += [jnp.dot(ps[j], pad(vs[j]), preferred_element_type=F32)
                      for j in range(HG)]
        assert early is None or not units
        ob = oproj(heads[H // 2:], H // 2)
        return jnp.concatenate([b + a for a, b in zip(oa, ob)], axis=1)

    def post2(s, toks=None):
        r3 = seg_row(s - 1 - LAG)
        for r in (0, 16):
            xc = _r(x2_s[(s + 4 - 1 - LAG) % 4, r:r + 16] + obuf[SEG + r:SEG + r + 16, :])
            out_s[pl.ds(r3 + r, 16), :] = gate(xc, r3 + r, toks).astype(BF16)

    def step(s, mode, vis, fill, chained=False, before_oproj=None, early=None):
        if mode == 0:
            h = hbuf[...]
        elif mode == 1:
            h = hbuf[0:48, :]
        else:
            h = jnp.concatenate([hbuf[0:16, :], hbuf[48:80, :]], axis=0)
        toks = []
        if mode != 1:
            post2(s, toks)
        if isinstance(s, int) and s == NSEG + LAG - 1:
            obuf[SEG:2 * SEG, :] = attention(h, vis, fill, chained, due=toks)
            return
        r1 = seg_row(s - 1)
        rn = seg_row(s + 1)
        h1n, h2n = [], []
        for r in (0, 16):
            xa = _r(x_s[pl.ds(r1 + r, 16), :].astype(F32) + obuf[r:r + 16, :])
            xb2 = _r(gate(xa, r1 + r))
            h2n.append(_ln(xb2, toks).astype(BF16))
            x2_s[(s + 4 - 1) % 4, r:r + 16] = xb2
        if mode != 2:
            for r in (0, 16):
                h1n.append(_ln(x_s[pl.ds(rn + r, 16), :].astype(F32), toks).astype(BF16))

        o = attention(h, vis, fill, chained, before_oproj, early, toks)

        mem2 = mem0 if mode == 1 else o[M:2 * M]
        hbuf[0:16, :] = jnp.concatenate([o[0:M], mem2], axis=0).astype(BF16)
        for n, v in enumerate(h1n):
            hbuf[16 + 16 * n:32 + 16 * n, :] = v
        for n, v in enumerate(h2n):
            hbuf[48 + 16 * n:64 + 16 * n, :] = v
        if mode == 0:
            obuf[...] = o[2 * M:]
        elif mode == 1:
            obuf[0:SEG, :] = o[2 * M:]
        else:
            obuf[SEG:2 * SEG, :] = o[2 * M:]

    with jax.named_scope("pro"):
        vis, fill = masks(1)
        step(0, 1, vis, fill, False, wo_copy.wait)
        step(1, 1, vis, fill, True)
    xb_copy.wait()
    vis, fill = masks(0)
    with jax.named_scope("main_a"):
        loop(NA // UA, lambda i: [step(UA * i + u + LAG, 0, vis, fill, u > 0, early=UA * i + u)
                                  for u in range(UA)])
    with jax.named_scope("conv_e"):
        loop(HB // 2, lambda j: (inv_stage(HB + 2 * j), inv_stage(HB + 2 * j + 1)))
    with jax.named_scope("main_b"):
        loop((NSEG - LAG - NA) // UB, lambda i: [step(UB * i + u + LAG + NA, 0, vis, fill, u > 0)
                                                 for u in range(UB)])
    done = (NSEG - 1 - LAG) * SEG
    out_a = pltpu.make_async_copy(out_s.at[0:done, :], out_hbm.at[0:done, :], sem.at[SW + 8])
    out_a.start()
    with jax.named_scope("epi"):
        vis, fill = masks(2)
        step(NSEG, 2, vis, fill)
        step(NSEG + 1, 2, *masks(2, 2 * M), True)
    post2(NSEG + LAG)
    out_b = pltpu.make_async_copy(out_s.at[done:S, :], out_hbm.at[done:S, :], sem.at[SW + 9])
    out_b.start()
    out_a.wait()
    out_b.wait()


@jax.jit
def pallas_interleave_layers__memory_aug_recurrent_mem_tr__ssm_conv_h3__prompt_kernel(
    A_x, A_mem0, A_Wq, A_Wk, A_Wv, A_Wo, A_seg_len,
    B_q, B_k, B_v, B_shift_k, B_ssm_k, B_ssm_D,
):
    del A_seg_len, B_q
    assert A_x.shape == (1, S, D) and A_Wq.shape == (D, H, DH)
    hbm = pl.BlockSpec(memory_space=pl.ANY)
    out = pl.pallas_call(
        _kernel,
        out_shape=jax.ShapeDtypeStruct((S, D), BF16),
        in_specs=[hbm] * 11,
        out_specs=hbm,
        scratch_shapes=[
            pltpu.VMEM((S, D), BF16),
            pltpu.VMEM((S, D), BF16),
            pltpu.VMEM((S, D), BF16),
            pltpu.VMEM((HB, D, 2 * TB), BF16),
            pltpu.VMEM((3, D, H, DH), BF16),
            pltpu.VMEM(((H + 1) * WP, 128), U32),
            pltpu.VMEM(((2 * H + 1) * WP, 128), U32),
            pltpu.VMEM((H * DH, D), BF16),
            pltpu.VMEM((NLB, H * DH // 2, 128), U32),
            pltpu.VMEM((TB, TB), BF16),
            pltpu.VMEM((2, TB, TB), BF16),
            pltpu.VMEM((2, TB // 2, 3 * TB), BF16),
            pltpu.VMEM((2, NLB, S // 2 + 8, 128), F32),
            pltpu.VMEM((NB, 2, NLB * TB, 128), F32),
            pltpu.VMEM((NB, 3, NLB * TB, 128), F32),
            pltpu.VMEM((NB + 1, 2, NLB * TB, 128), F32),
            pltpu.VMEM((NLB, S + 8, 128), F32),
            pltpu.VMEM((ROWS, D), BF16),
            pltpu.VMEM((2 * SEG, D), F32),
            pltpu.VMEM((4, SEG, D), F32),
            pltpu.VMEM((S, D), BF16),
            pltpu.VMEM((NA * SEG, D), BF16),
            pltpu.VMEM((NQH, NA * SEG, DH), BF16),
            pltpu.VMEM((M, D), BF16),
            pltpu.VMEM((KS, D), BF16),
            pltpu.VMEM((D,), BF16),
            pltpu.SemaphoreType.DMA((HB // 2 + 10,)),
        ],
        compiler_params=pltpu.CompilerParams(vmem_limit_bytes=120 * 1024 * 1024),
    )(A_x.reshape(S, D), A_mem0.reshape(M, D), A_Wq, A_Wk, A_Wv,
      A_Wo.reshape(H * DH, D), B_k.reshape(S, D), B_v.reshape(S, D),
      B_shift_k.T, B_ssm_k, B_ssm_D)
    return out.reshape(1, S, D)
```

```python
import functools
import math

import jax
import jax.numpy as jnp
from jax import lax
import jax.experimental.pallas as pl
import jax.experimental.pallas.tpu as pltpu

F32 = jnp.float32
BF16 = jnp.bfloat16
U32 = jnp.uint32

S = 2048
D = 640
H = 32
DH = 128
M = 8
SEG = 32
NSEG = S // SEG
KS = 4
LAG = 2
ROWS = 2 * M + 2 * SEG
HG = 4
NG = H // HG
NLB = D // 128
TB = 128
NB = S // TB
HB = NB // 2
NPOS = NLB * TB // 8
NA = 20
PPS = 4
UCUT = tuple(range(a, a + 2) for a in range(0, 12, 2)) + (range(12, 16),)
NQH = 28
UA = 2
UB = 3
UI = 4
WP = 324


def _ln(x, toks=None):
    m = jnp.mean(x, axis=-1, keepdims=True)
    c = x - m
    v = jnp.mean(c * c, axis=-1, keepdims=True)
    r = lax.rsqrt(v + 1e-5)
    if toks is not None:
        toks.append(jnp.minimum(r, 0.0))
    return c * r


def _r(x):
    return x.astype(BF16).astype(F32)


def _split(x):
    hi = pltpu.bitcast(pltpu.bitcast(x, U32) & jnp.uint32(0xFFFF0000), F32)
    return hi, x - hi


def _bf(x):
    return jnp.concatenate([x[:, g:g + 128].astype(BF16)
                            for g in range(0, x.shape[1], 128)], axis=1)


def _basis(r, t):
    b = r & 63
    f = jnp.where(b < 32, 2 * b, 2 * b - 63)
    n = ((2 * f + 1) * t - jnp.where(r >= 64, TB, 0)) & (4 * TB - 1)
    n = jnp.where(n >= 2 * TB, n - 4 * TB, n)
    return jnp.cos(n.astype(F32) * (2.0 * math.pi / (4 * TB)))


def _halves(x):
    w = pltpu.bitcast(x, U32)
    return (pltpu.bitcast(w << 16, F32),
            pltpu.bitcast(w & jnp.uint32(0xFFFF0000), F32))


def _kernel(x_hbm, mem0_hbm, wq_hbm, wk_hbm, wv_hbm, wo_hbm,
            k_hbm, v_hbm, shk_hbm, ssmk_hbm, ssmd_hbm,
            out_hbm,
            x_s, k_s, v_s, ssmk_s, wraw, wt_q, wt_kv, wo_s, wo_t,
            perm_s, fu_s, inv_s, kpad, u_s, kf_s, c_s, y_s,
            hbuf, obuf, x2_s, out_s, hl_s, qh_s, mem0_ref, shk_ref, ssmd_ref,
            sem):
    XH = (LAG + NA) * SEG
    SW = HB // 2

    def conv_copies(jp, sm):
        rows = pl.ds(jp * 2 * TB if isinstance(jp, int) else pl.multiple_of(jp * 2 * TB, 2 * TB), 2 * TB)
        return [pltpu.make_async_copy(ssmk_hbm.at[:, rows], ssmk_s.at[jp], sm),
                pltpu.make_async_copy(k_hbm.at[rows, :], k_s.at[rows, :], sm),
                pltpu.make_async_copy(v_hbm.at[rows, :], v_s.at[rows, :], sm)]
    w_copies = [pltpu.make_async_copy(w, wraw.at[t], sem.at[SW + t])
                for t, w in enumerate((wq_hbm, wk_hbm, wv_hbm))]
    wo_copy = pltpu.make_async_copy(wo_hbm, wo_s, sem.at[SW + 3])
    late_copies = [c for jp in range(HB // 2, HB) for c in conv_copies(jp, sem.at[SW + 4])]
    small_copies = [pltpu.make_async_copy(src, dst, sem.at[SW + 5])
                    for src, dst in ((shk_hbm, shk_ref), (ssmd_hbm, ssmd_ref), (mem0_hbm, mem0_ref))]
    xa_copy = pltpu.make_async_copy(x_hbm.at[0:XH, :], x_s.at[0:XH, :], sem.at[SW + 6])
    xb_copy = pltpu.make_async_copy(x_hbm.at[XH:, :], x_s.at[XH:, :], sem.at[SW + 7])
    for c in (small_copies + [c for jp in range(HB // 2) for c in conv_copies(jp, sem.at[jp])] + late_copies
              + [xa_copy] + w_copies + [wo_copy, xb_copy]):
        c.start()

    hb = TB // 2
    ri = lax.broadcasted_iota(jnp.int32, (TB, TB), 0)
    ci = lax.broadcasted_iota(jnp.int32, (TB, TB), 1)
    perm_s[...] = jnp.where(ci == 2 * (ri & 63) + (ri >> 6), 1.0, 0.0).astype(BF16)
    tab = _basis(ri, 2 * (ci & 63) + (ci >> 6))
    hi, lo = _split(tab)
    fu_s[0] = jnp.where(ci < hb, hi, pltpu.roll(lo, hb, 1)).astype(BF16)
    fu_s[1] = jnp.where(ci < hb, pltpu.roll(hi, hb, 1), lo).astype(BF16)
    gh, gl = _split(tab.T * (1.0 / TB))
    ginv = _bf(jnp.concatenate([gh, gl, gh], axis=1))
    inv_s[0] = ginv[:hb]
    inv_s[1] = ginv[hb:]

    for c in small_copies:
        c.wait()
    shk_t = shk_ref[...].astype(F32)
    taps = [[shk_t[j:j + 1, g * 128:(g + 1) * 128] for g in range(NLB)] for j in range(KS)]
    dvec = ssmd_ref[...].astype(F32).reshape(1, D)
    for g in range(NLB):
        kpad[0, g, 0:8, :] = jnp.zeros((8, 128), F32)
        kpad[1, g, 0:8, :] = jnp.zeros((8, 128), F32)
    c_s[0] = jnp.zeros(c_s.shape[1:], F32)

    def spectrum(e, o):
        fe = jnp.dot(fu_s[0], jnp.concatenate([e, e], axis=0).astype(BF16), preferred_element_type=F32)
        fo = jnp.dot(fu_s[1], jnp.concatenate([o, o], axis=0).astype(BF16), preferred_element_type=F32)
        return ((fe[:hb] + fo[:hb], fe[hb:] + fo[hb:]), (fe[:hb] - fo[:hb], fo[hb:] - fe[hb:]))

    def fwd_stage(jp, first):
        if first:
            for c in conv_copies(jp, sem.at[jp]):
                c.wait()
        kts = [lax.dot_general(perm_s[...], ssmk_s[jp, :, n * TB:(n + 1) * TB], (((1,), (1,)), ((), ())),
                               preferred_element_type=F32) for n in range(2)]
        for n, kt in enumerate(kts):
            j = 2 * jp + n
            r0 = pl.multiple_of(j * TB, TB)
            q0 = pl.multiple_of(j * hb, hb) + 8
            for g in range(NLB):
                lb = slice(g * 128, (g + 1) * 128)
                halves = (slice(g * TB, g * TB + hb), slice(g * TB + hb, (g + 1) * TB))
                for rows, (kr, ki) in zip(halves, spectrum(kt[:hb, lb], kt[hb:, lb])):
                    if first and n == 0:
                        kr = kr + jnp.where(j == 0, dvec[:, lb], 0.0)
                    kf_s[j, 0, rows] = kr
                    kf_s[j, 1, rows] = ki - kr
                    kf_s[j, 2, rows] = kr + ki
                ke, ko = _halves(k_s[pl.ds(r0, TB), lb])
                ve, vo = _halves(v_s[pl.ds(r0, TB), lb])
                kpad[0, g, pl.ds(q0, hb), :] = ke
                kpad[1, g, pl.ds(q0, hb), :] = ko
                ke1 = kpad[0, g, pl.ds(q0 - 1, hb), :]
                ko1 = kpad[1, g, pl.ds(q0 - 1, hb), :]
                ko2 = kpad[1, g, pl.ds(q0 - 2, hb), :]
                t0, t1, t2, t3 = (taps[t][g] for t in range(KS))
                e = (ke * t0 + ko1 * t1 + ke1 * t2 + ko2 * t3) * ve
                o = (ko * t0 + ke * t1 + ko1 * t2 + ke1 * t3) * vo
                for rows, (ur, ui) in zip(halves, spectrum(e, o)):
                    u_s[j, 0, rows] = ur
                    u_s[j, 1, rows] = ui

    def mac_units(row, half):
        rs = pl.ds(row, 8)
        state = {}

        def unit(p, avals, final, tok=None):
            acc = state.setdefault(p, dict(state.get(0, {})))
            for a in avals:
                u = u_s[a, 0, rs] + u_s[a, 1, rs] if p == 0 else u_s[a, p - 1, rs]
                if tok is not None:
                    u = u + tok
                for i in range(max(a, half * HB), half * HB + HB):
                    t = u * kf_s[i - a, p, rs]
                    acc[i] = t if i not in acc else (acc[i] - t if p == 2 else acc[i] + t)
            if final and p:
                for i, v in acc.items():
                    c_s[i + 1, 2 - p, rs] = v

        subs = UCUT if half else (range(HB),)
        return [functools.partial(unit, p, avals, n == len(subs) - 1)
                for p in range(3) for n, avals in enumerate(subs)]

    def inv_stage(i):
        q = TB // 4
        for g in range(NLB):
            re, im = [], []
            for b in range(4):
                rows = slice(g * TB + b * q, g * TB + (b + 1) * q)
                cr, ci_ = c_s[i + 1, 0, rows], c_s[i + 1, 1, rows]
                pr, pi = c_s[i, 0, rows], c_s[i, 1, rows]
                re.append(cr + pi if b in (0, 3) else cr - pi)
                im.append(ci_ - pr if b in (0, 3) else ci_ + pr)
            pe = jnp.concatenate([re[0] + re[2], re[1] + re[3], im[0] - im[2], im[1] - im[3]], axis=0)
            po = jnp.concatenate([re[0] - re[2], re[1] - re[3], im[0] + im[2], im[1] + im[3]], axis=0)
            for par, pp in enumerate((pe, po)):
                ph, plo = _split(pp)
                y_s[g, pl.ds(i * TB + par, hb, stride=2), :] = jnp.dot(
                    inv_s[par], jnp.concatenate([ph, ph, plo], axis=0).astype(BF16),
                    preferred_element_type=F32)

    def relayout_rows(t, dst, base, dp, tok=None):
        a = pltpu.bitcast(wraw[t, 2 * dp], U32)
        b = pltpu.bitcast(wraw[t, 2 * dp + 1], U32)
        if tok is not None:
            a = a | tok
        dst[pl.ds(base + dp, 16, stride=WP), :] = (a & jnp.uint32(0xFFFF)) | (b << 16)
        dst[pl.ds(base + 16 * WP + dp, 16, stride=WP), :] = (
            (a >> 16) | (b & jnp.uint32(0xFFFF0000)))

    def wslab(t, h):
        s0 = (max(t - 1, 0) * H + (h % 2) * 16 + h // 2) * WP
        return pltpu.bitcast((wt_kv if t else wt_q)[s0:s0 + D // 2, :], BF16)

    def loop(n, fn):
        def body(j, _):
            fn(j)
            return 0
        lax.fori_loop(0, n, body, 0)

    def norm_rows(c):
        nr = NA * SEG // 4
        r0 = pl.multiple_of(c * nr, 16)
        for r in range(0, nr, 16):
            hl_s[pl.ds(r0 + r, 16), :] = _ln(
                x_s[pl.ds(r0 + r + LAG * SEG, 16), :].astype(F32)).astype(BF16)

    def pre_queries(c, t=None):
        if t is not None:
            pltpu.make_async_copy(wraw.at[t], wraw.at[t], sem.at[SW + t]).wait()
            base = (t - 1) * (H * WP)
        per = -(-(D // 2) // (2 * NQH))
        dp = 0
        for sub in range(2):
            r0 = pl.multiple_of((2 * c + sub) * QR, QR)
            hl = hl_s[pl.ds(r0, QR), :]
            for hd in range(NQH):
                r = jnp.dot(hl, wslab(0, hd), preferred_element_type=F32)
                qh_s[hd, pl.ds(r0, QR), :] = r.astype(BF16)
                if t is not None:
                    tok = pltpu.bitcast(jnp.minimum(jnp.abs(r[0:16]), 0.0), U32)
                    for _ in range(per):
                        if dp < D // 2:
                            relayout_rows(t, wt_kv, base, dp, tok)
                            dp += 1

    nch = NA * SEG // TB
    QR = TB // 2
    with jax.named_scope("conv_a"):
        loop(HB // 2, lambda j: fwd_stage(j, True))
    with jax.named_scope("conv_b"):
        loop(NPOS // 10, lambda j: [u() for n in range(10) for u in mac_units(pl.multiple_of(80 * j, 16) + 8 * n, 0)])
        loop(HB // UI, lambda j: [inv_stage(UI * j + u) for u in range(UI)])
    with jax.named_scope("conv_c"):
        for c in late_copies:
            c.wait()
        xa_copy.wait()
        loop(HB // 2, lambda j: (fwd_stage(HB // 2 + j, False), norm_rows(j)))
    with jax.named_scope("rel0"):
        w_copies[0].wait()
        loop(D // 64, lambda i: [relayout_rows(0, wt_q, 0, i * 32 + dd) for dd in range(32)])
    with jax.named_scope("preq"):
        loop(nch - 2, pre_queries)
    with jax.named_scope("preq_rel"):
        loop(2, lambda i: pre_queries(i + nch - 2, i + 1))

    scale = DH ** -0.5

    def masks(mode, q0=0):
        rows = ROWS if mode == 0 else ROWS - SEG
        qi = lax.broadcasted_iota(jnp.int32, (rows - q0, 128), 0) + q0
        kj = lax.broadcasted_iota(jnp.int32, (rows - q0, 128), 1)

        def layer_of(i):
            xl = (i - 2 * M) // SEG if mode == 0 else mode - 1
            return jnp.where(i < 2 * M, i // M, xl)
        same = (layer_of(qi) == layer_of(kj)) & (kj < rows)
        vis = same & ((qi < 2 * M) | (qi >= kj))
        fill = jnp.where(same, -1e9 / scale, -jnp.inf).astype(F32)
        return vis, fill

    mem0 = mem0_ref[...].astype(F32)
    hbuf[0:16, :] = jnp.concatenate([mem0, mem0], axis=0).astype(BF16)
    hbuf[16:48, :] = _ln(x_s[0:SEG, :].astype(F32)).astype(BF16)
    obuf[...] = jnp.zeros((2 * SEG, D), F32)
    x2_s[...] = jnp.zeros(x2_s.shape, F32)

    def seg_row(seg):
        if isinstance(seg, int):
            return min(max(seg, 0), NSEG - 1) * SEG
        return pl.multiple_of(jnp.clip(seg, 0, NSEG - 1) * SEG, SEG)

    def gate(xa, r0, toks=None):
        y = jnp.concatenate([y_s[g, pl.ds(r0, xa.shape[0]), :] for g in range(NLB)], axis=1)
        return xa + _ln(xa, toks) * y

    def attention(h, vis, fill, chained, before_oproj=None, early=None, due=()):
        q0 = h.shape[0] - vis.shape[0]
        if early is not None:
            hrest = jnp.concatenate([h[:2 * M], h[2 * M + SEG:]], axis=0)
            qrow = pl.multiple_of(early * SEG, SEG)
            units = [u for n in range(PPS)
                     for u in mac_units(pl.multiple_of(early * (8 * PPS), 8 * PPS) + 8 * n, 1)]

        def proj(g):
            res = [[None] * HG for _ in range(3)]
            order = [(t, j) for j in range(HG) for t in range(2)] + [(2, j) for j in range(HG)]
            def operand(t, j):
                pre = early is not None and t == 0 and g * HG + j < NQH
                return pre, hrest if pre else (h if t else h[q0:])

            kc = D - 128
            nsplit = 4 if g == 0 and chained else 0
            part = [jnp.dot(operand(t, j)[1][:, :kc], wslab(t, j)[:kc], preferred_element_type=F32)
                    for t, j in order[:nsplit]]
            for n, (t, j) in enumerate(order):
                hd = g * HG + j
                pre, lhs = operand(t, j)
                if n < nsplit:
                    r = jnp.dot(lhs[:, kc:], wslab(t, hd)[kc:], preferred_element_type=F32) + part[n]
                else:
                    r = jnp.dot(lhs, wslab(t, hd), preferred_element_type=F32)
                if early is not None and units:
                    units.pop(0)(jnp.minimum(jnp.abs(r[0:8]), 0.0))
                if t == 0:
                    r = r.astype(BF16)
                if pre:
                    r = jnp.concatenate([r[:2 * M], qh_s[hd, pl.ds(qrow, SEG), :], r[2 * M:]], axis=0)
                res[t][j] = r
            return res

        def pad(kv):
            return jnp.concatenate([kv, jnp.zeros((128 - kv.shape[0], DH), F32)], axis=0).astype(BF16)

        def probs(qkv, g):
            scs = [lax.dot_general(qkv[0][j], pad(qkv[1][j]), (((1,), (1,)), ((), ())),
                                   preferred_element_type=F32) for j in range(HG)]
            ps = []
            for sc in scs:
                sc = jnp.where(vis, sc, fill)
                e = jnp.exp2((sc - jnp.max(sc, axis=-1, keepdims=True)) * (scale * math.log2(math.e)))
                den = jnp.sum(e, axis=-1, keepdims=True)
                if not ps and g >= NG - len(due):
                    e = jnp.concatenate([e[:16] + due[g - NG + len(due)], e[16:]], axis=0)
                r = pl.reciprocal(den, approx=True)
                r = r * (2.0 - den * r)
                ps.append((e * r).astype(BF16))
            return ps

        def oproj(os_, h0):
            oc = jnp.concatenate(os_, axis=1).astype(BF16)
            k0, k1 = h0 * DH, (h0 + len(os_)) * DH
            res = []
            for n in range(NLB):
                if before_oproj is not None:
                    w = wo_s[k0:k1, n * 128:(n + 1) * 128]
                    wo_t[n, k0 // 2:k1 // 2, :] = pltpu.bitcast(w, U32)
                else:
                    w = pltpu.bitcast(wo_t[n, k0 // 2:k1 // 2, :], BF16)
                res.append(jnp.dot(oc, w, preferred_element_type=F32))
            return res

        heads = []
        qkv = proj(0)
        oa = None
        for g in range(NG):
            ps = probs(qkv, g)
            vs = qkv[2]
            if g + 1 < NG:
                qkv = proj(g + 1)
            else:
                if before_oproj is not None:
                    before_oproj()
                oa = oproj(heads[:H // 2], 0)
            heads += [jnp.dot(ps[j], pad(vs[j]), preferred_element_type=F32)
                      for j in range(HG)]
        assert early is None or not units
        ob = oproj(heads[H // 2:], H // 2)
        return jnp.concatenate([b + a for a, b in zip(oa, ob)], axis=1)

    def post2(s, toks=None):
        r3 = seg_row(s - 1 - LAG)
        for r in (0, 16):
            xc = _r(x2_s[(s + 4 - 1 - LAG) % 4, r:r + 16] + obuf[SEG + r:SEG + r + 16, :])
            out_s[pl.ds(r3 + r, 16), :] = gate(xc, r3 + r, toks).astype(BF16)

    def step(s, mode, vis, fill, chained=False, before_oproj=None, early=None):
        if mode == 0:
            h = hbuf[...]
        elif mode == 1:
            h = hbuf[0:48, :]
        else:
            h = jnp.concatenate([hbuf[0:16, :], hbuf[48:80, :]], axis=0)
        toks = []
        if mode != 1:
            post2(s, toks)
        if isinstance(s, int) and s == NSEG + LAG - 1:
            obuf[SEG:2 * SEG, :] = attention(h, vis, fill, chained, due=toks)
            return
        r1 = seg_row(s - 1)
        rn = seg_row(s + 1)
        h1n, h2n = [], []
        for r in (0, 16):
            xa = _r(x_s[pl.ds(r1 + r, 16), :].astype(F32) + obuf[r:r + 16, :])
            xb2 = _r(gate(xa, r1 + r))
            h2n.append(_ln(xb2, toks).astype(BF16))
            x2_s[(s + 4 - 1) % 4, r:r + 16] = xb2
        if mode != 2:
            for r in (0, 16):
                h1n.append(_ln(x_s[pl.ds(rn + r, 16), :].astype(F32), toks).astype(BF16))

        o = attention(h, vis, fill, chained, before_oproj, early, toks)

        mem2 = mem0 if mode == 1 else o[M:2 * M]
        hbuf[0:16, :] = jnp.concatenate([o[0:M], mem2], axis=0).astype(BF16)
        for n, v in enumerate(h1n):
            hbuf[16 + 16 * n:32 + 16 * n, :] = v
        for n, v in enumerate(h2n):
            hbuf[48 + 16 * n:64 + 16 * n, :] = v
        if mode == 0:
            obuf[...] = o[2 * M:]
        elif mode == 1:
            obuf[0:SEG, :] = o[2 * M:]
        else:
            obuf[SEG:2 * SEG, :] = o[2 * M:]

    with jax.named_scope("pro"):
        vis, fill = masks(1)
        step(0, 1, vis, fill, False, wo_copy.wait)
        step(1, 1, vis, fill, True)
    xb_copy.wait()
    vis, fill = masks(0)
    with jax.named_scope("main_a"):
        loop(NA // UA, lambda i: [step(UA * i + u + LAG, 0, vis, fill, u > 0, early=UA * i + u)
                                  for u in range(UA)])
    with jax.named_scope("conv_e"):
        loop(HB // UI, lambda j: [inv_stage(HB + UI * j + u) for u in range(UI)])
    with jax.named_scope("main_b"):
        loop((NSEG - LAG - NA) // UB, lambda i: [step(UB * i + u + LAG + NA, 0, vis, fill, u > 0)
                                                 for u in range(UB)])
    done = (NSEG - 1 - LAG) * SEG
    out_a = pltpu.make_async_copy(out_s.at[0:done, :], out_hbm.at[0:done, :], sem.at[SW + 8])
    out_a.start()
    with jax.named_scope("epi"):
        vis, fill = masks(2)
        step(NSEG, 2, vis, fill)
        step(NSEG + 1, 2, *masks(2, 2 * M), True)
    post2(NSEG + LAG)
    out_b = pltpu.make_async_copy(out_s.at[done:S, :], out_hbm.at[done:S, :], sem.at[SW + 9])
    out_b.start()
    out_a.wait()
    out_b.wait()


@jax.jit
def pallas_interleave_layers__memory_aug_recurrent_mem_tr__ssm_conv_h3__prompt_kernel(
    A_x, A_mem0, A_Wq, A_Wk, A_Wv, A_Wo, A_seg_len,
    B_q, B_k, B_v, B_shift_k, B_ssm_k, B_ssm_D,
):
    del A_seg_len, B_q
    assert A_x.shape == (1, S, D) and A_Wq.shape == (D, H, DH)
    hbm = pl.BlockSpec(memory_space=pl.ANY)
    out = pl.pallas_call(
        _kernel,
        out_shape=jax.ShapeDtypeStruct((S, D), BF16),
        in_specs=[hbm] * 11,
        out_specs=hbm,
        scratch_shapes=[
            pltpu.VMEM((S, D), BF16),
            pltpu.VMEM((S, D), BF16),
            pltpu.VMEM((S, D), BF16),
            pltpu.VMEM((HB, D, 2 * TB), BF16),
            pltpu.VMEM((3, D, H, DH), BF16),
            pltpu.VMEM(((H + 1) * WP, 128), U32),
            pltpu.VMEM(((2 * H + 1) * WP, 128), U32),
            pltpu.VMEM((H * DH, D), BF16),
            pltpu.VMEM((NLB, H * DH // 2, 128), U32),
            pltpu.VMEM((TB, TB), BF16),
            pltpu.VMEM((2, TB, TB), BF16),
            pltpu.VMEM((2, TB // 2, 3 * TB), BF16),
            pltpu.VMEM((2, NLB, S // 2 + 8, 128), F32),
            pltpu.VMEM((NB, 2, NLB * TB, 128), F32),
            pltpu.VMEM((NB, 3, NLB * TB, 128), F32),
            pltpu.VMEM((NB + 1, 2, NLB * TB, 128), F32),
            pltpu.VMEM((NLB, S + 8, 128), F32),
            pltpu.VMEM((ROWS, D), BF16),
            pltpu.VMEM((2 * SEG, D), F32),
            pltpu.VMEM((4, SEG, D), F32),
            pltpu.VMEM((S, D), BF16),
            pltpu.VMEM((NA * SEG, D), BF16),
            pltpu.VMEM((NQH, NA * SEG, DH), BF16),
            pltpu.VMEM((M, D), BF16),
            pltpu.VMEM((KS, D), BF16),
            pltpu.VMEM((D,), BF16),
            pltpu.SemaphoreType.DMA((HB // 2 + 10,)),
        ],
        compiler_params=pltpu.CompilerParams(vmem_limit_bytes=120 * 1024 * 1024),
    )(A_x.reshape(S, D), A_mem0.reshape(M, D), A_Wq, A_Wk, A_Wv,
      A_Wo.reshape(H * DH, D), B_k.reshape(S, D), B_v.reshape(S, D),
      B_shift_k.T, B_ssm_k, B_ssm_D)
    return out.reshape(1, S, D)
```

```python
import functools
import math

import jax
import jax.numpy as jnp
from jax import lax
import jax.experimental.pallas as pl
import jax.experimental.pallas.tpu as pltpu

F32 = jnp.float32
BF16 = jnp.bfloat16
U32 = jnp.uint32

S = 2048
D = 640
H = 32
DH = 128
M = 8
SEG = 32
NSEG = S // SEG
KS = 4
LAG = 2
ROWS = 2 * M + 2 * SEG
HG = 4
NG = H // HG
NLB = D // 128
TB = 128
NB = S // TB
HB = NB // 2
NPOS = NLB * TB // 8
NA = 20
PPS = 4
UCUT = tuple(range(a, a + 2) for a in range(0, 12, 2)) + (range(12, 16),)
NQH = 30
UA = 2
UB = 3
UI = 4
WP = 324


def _ln(x, toks=None):
    m = jnp.mean(x, axis=-1, keepdims=True)
    c = x - m
    v = jnp.mean(c * c, axis=-1, keepdims=True)
    r = lax.rsqrt(v + 1e-5)
    if toks is not None:
        toks.append(jnp.minimum(r, 0.0))
    return c * r


def _r(x):
    return x.astype(BF16).astype(F32)


def _split(x):
    hi = pltpu.bitcast(pltpu.bitcast(x, U32) & jnp.uint32(0xFFFF0000), F32)
    return hi, x - hi


def _bf(x):
    return jnp.concatenate([x[:, g:g + 128].astype(BF16)
                            for g in range(0, x.shape[1], 128)], axis=1)


def _basis(r, t):
    b = r & 63
    f = jnp.where(b < 32, 2 * b, 2 * b - 63)
    n = ((2 * f + 1) * t - jnp.where(r >= 64, TB, 0)) & (4 * TB - 1)
    n = jnp.where(n >= 2 * TB, n - 4 * TB, n)
    return jnp.cos(n.astype(F32) * (2.0 * math.pi / (4 * TB)))


def _halves(x):
    w = pltpu.bitcast(x, U32)
    return (pltpu.bitcast(w << 16, F32),
            pltpu.bitcast(w & jnp.uint32(0xFFFF0000), F32))


def _kernel(x_hbm, mem0_hbm, wq_hbm, wk_hbm, wv_hbm, wo_hbm,
            k_hbm, v_hbm, shk_hbm, ssmk_hbm, ssmd_hbm,
            out_hbm,
            x_s, k_s, v_s, ssmk_s, wraw, wt_q, wt_kv, wo_s, wo_t,
            perm_s, fu_s, inv_s, kpad, u_s, kf_s, c_s, y_s,
            hbuf, obuf, x2_s, out_s, hl_s, qh_s, mem0_ref, shk_ref, ssmd_ref,
            sem):
    XH = (LAG + NA) * SEG
    SW = HB + HB // 2

    def pair_rows(jp):
        r0 = jp * 2 * TB
        return pl.ds(r0 if isinstance(jp, int) else pl.multiple_of(r0, 2 * TB), 2 * TB)

    def ssmk_copy(jp):
        return pltpu.make_async_copy(ssmk_hbm.at[:, pair_rows(jp)], ssmk_s.at[jp], sem.at[jp])

    def kv_copies(rows, sm):
        return [pltpu.make_async_copy(k_hbm.at[rows, :], k_s.at[rows, :], sm),
                pltpu.make_async_copy(v_hbm.at[rows, :], v_s.at[rows, :], sm)]
    w_copies = [pltpu.make_async_copy(w, wraw.at[t], sem.at[SW + t])
                for t, w in enumerate((wq_hbm, wk_hbm, wv_hbm))]
    wo_copy = pltpu.make_async_copy(wo_hbm, wo_s, sem.at[SW + 3])
    late_copies = kv_copies(pl.ds(S // 2, S // 2), sem.at[SW + 4])
    small_copies = [pltpu.make_async_copy(src, dst, sem.at[SW + 5])
                    for src, dst in ((shk_hbm, shk_ref), (ssmd_hbm, ssmd_ref), (mem0_hbm, mem0_ref))]
    xa_copy = pltpu.make_async_copy(x_hbm.at[0:XH, :], x_s.at[0:XH, :], sem.at[SW + 6])
    xb_copy = pltpu.make_async_copy(x_hbm.at[XH:, :], x_s.at[XH:, :], sem.at[SW + 7])
    for c in (small_copies + [ssmk_copy(jp) for jp in range(HB)]
              + [c for jp in range(HB // 2) for c in kv_copies(pair_rows(jp), sem.at[HB + jp])]
              + [xa_copy, w_copies[0]] + late_copies + w_copies[1:] + [wo_copy, xb_copy]):
        c.start()

    hb = TB // 2
    ri = lax.broadcasted_iota(jnp.int32, (TB, TB), 0)
    ci = lax.broadcasted_iota(jnp.int32, (TB, TB), 1)
    perm_s[...] = jnp.where(ci == 2 * (ri & 63) + (ri >> 6), 1.0, 0.0).astype(BF16)
    tab = _basis(ri, 2 * (ci & 63) + (ci >> 6))
    hi, lo = _split(tab)
    fu_s[0] = jnp.where(ci < hb, hi, pltpu.roll(lo, hb, 1)).astype(BF16)
    fu_s[1] = jnp.where(ci < hb, pltpu.roll(hi, hb, 1), lo).astype(BF16)
    gh, gl = _split(tab.T * (1.0 / TB))
    ginv = _bf(jnp.concatenate([gh, gl, gh], axis=1))
    inv_s[0] = ginv[:hb]
    inv_s[1] = ginv[hb:]

    for c in small_copies:
        c.wait()
    shk_t = shk_ref[...].astype(F32)
    taps = [[shk_t[j:j + 1, g * 128:(g + 1) * 128] for g in range(NLB)] for j in range(KS)]
    dvec = ssmd_ref[...].astype(F32).reshape(1, D)
    for g in range(NLB):
        kpad[0, g, 0:8, :] = jnp.zeros((8, 128), F32)
        kpad[1, g, 0:8, :] = jnp.zeros((8, 128), F32)
    c_s[0] = jnp.zeros(c_s.shape[1:], F32)

    def spectrum(e, o):
        fe = jnp.dot(fu_s[0], jnp.concatenate([e, e], axis=0).astype(BF16), preferred_element_type=F32)
        fo = jnp.dot(fu_s[1], jnp.concatenate([o, o], axis=0).astype(BF16), preferred_element_type=F32)
        return ((fe[:hb] + fo[:hb], fe[hb:] + fo[hb:]), (fe[:hb] - fo[:hb], fo[hb:] - fe[hb:]))

    def freq_rows(g):
        return slice(g * TB, g * TB + hb), slice(g * TB + hb, (g + 1) * TB)

    def fwd_k(jq):
        for jp in (2 * jq, 2 * jq + 1):
            ssmk_copy(jp).wait()

        def transposed(n):
            blk = ssmk_s[2 * jq + n // 2, :, (n % 2) * TB:(n % 2 + 1) * TB]
            return lax.dot_general(perm_s[...], blk, (((1,), (1,)), ((), ())),
                                   preferred_element_type=F32)
        nxt = transposed(0)
        for n in range(4):
            kt = nxt
            if n < 3:
                nxt = transposed(n + 1)
            j = 4 * jq + n
            for g in range(NLB):
                lb = slice(g * 128, (g + 1) * 128)
                for rows, (kr, ki) in zip(freq_rows(g), spectrum(kt[:hb, lb], kt[hb:, lb])):
                    if n == 0:
                        kr = kr + jnp.where(j == 0, dvec[:, lb], 0.0)
                    kf_s[j, 0, rows] = kr
                    kf_s[j, 1, rows] = ki - kr
                    kf_s[j, 2, rows] = kr + ki

    def fwd_u(jq, first):
        if first:
            for jp in (2 * jq, 2 * jq + 1):
                for c in kv_copies(pair_rows(jp), sem.at[HB + jp]):
                    c.wait()
        for j in [4 * jq + n for n in range(4)]:
            r0 = pl.multiple_of(j * TB, TB)
            q0 = pl.multiple_of(j * hb, hb) + 8
            for g in range(NLB):
                lb = slice(g * 128, (g + 1) * 128)
                ke, ko = _halves(k_s[pl.ds(r0, TB), lb])
                ve, vo = _halves(v_s[pl.ds(r0, TB), lb])
                kpad[0, g, pl.ds(q0, hb), :] = ke
                kpad[1, g, pl.ds(q0, hb), :] = ko
                ke1 = kpad[0, g, pl.ds(q0 - 1, hb), :]
                ko1 = kpad[1, g, pl.ds(q0 - 1, hb), :]
                ko2 = kpad[1, g, pl.ds(q0 - 2, hb), :]
                t0, t1, t2, t3 = (taps[t][g] for t in range(KS))
                e = (ke * t0 + ko1 * t1 + ke1 * t2 + ko2 * t3) * ve
                o = (ko * t0 + ke * t1 + ko1 * t2 + ke1 * t3) * vo
                for rows, (ur, ui) in zip(freq_rows(g), spectrum(e, o)):
                    u_s[j, 0, rows] = ur
                    u_s[j, 1, rows] = ui

    def mac_units(row, half):
        rs = pl.ds(row, 8)
        state = {}

        def unit(p, avals, final, tok=None):
            acc = state.setdefault(p, dict(state.get(0, {})))
            for a in avals:
                u = u_s[a, 0, rs] + u_s[a, 1, rs] if p == 0 else u_s[a, p - 1, rs]
                if tok is not None:
                    u = u + tok
                for i in range(max(a, half * HB), half * HB + HB):
                    t = u * kf_s[i - a, p, rs]
                    acc[i] = t if i not in acc else (acc[i] - t if p == 2 else acc[i] + t)
            if final and p:
                for i, v in acc.items():
                    c_s[i + 1, 2 - p, rs] = v

        subs = UCUT if half else (range(HB),)
        return [functools.partial(unit, p, avals, n == len(subs) - 1)
                for p in range(3) for n, avals in enumerate(subs)]

    def inv_stage(i):
        q = TB // 4
        for g in range(NLB):
            re, im = [], []
            for b in range(4):
                rows = slice(g * TB + b * q, g * TB + (b + 1) * q)
                cr, ci_ = c_s[i + 1, 0, rows], c_s[i + 1, 1, rows]
                pr, pi = c_s[i, 0, rows], c_s[i, 1, rows]
                re.append(cr + pi if b in (0, 3) else cr - pi)
                im.append(ci_ - pr if b in (0, 3) else ci_ + pr)
            pe = jnp.concatenate([re[0] + re[2], re[1] + re[3], im[0] - im[2], im[1] - im[3]], axis=0)
            po = jnp.concatenate([re[0] - re[2], re[1] - re[3], im[0] + im[2], im[1] + im[3]], axis=0)
            for par, pp in enumerate((pe, po)):
                ph, plo = _split(pp)
                y_s[g, pl.ds(i * TB + par, hb, stride=2), :] = jnp.dot(
                    inv_s[par], jnp.concatenate([ph, ph, plo], axis=0).astype(BF16),
                    preferred_element_type=F32)

    def relayout_rows(t, dst, base, dp, tok=None):
        a = pltpu.bitcast(wraw[t, 2 * dp], U32)
        b = pltpu.bitcast(wraw[t, 2 * dp + 1], U32)
        if tok is not None:
            a = a | tok
        dst[pl.ds(base + dp, 16, stride=WP), :] = (a & jnp.uint32(0xFFFF)) | (b << 16)
        dst[pl.ds(base + 16 * WP + dp, 16, stride=WP), :] = (
            (a >> 16) | (b & jnp.uint32(0xFFFF0000)))

    def wslab(t, h):
        s0 = (max(t - 1, 0) * H + (h % 2) * 16 + h // 2) * WP
        return pltpu.bitcast((wt_kv if t else wt_q)[s0:s0 + D // 2, :], BF16)

    def loop(n, fn):
        def body(j, _):
            fn(j)
            return 0
        lax.fori_loop(0, n, body, 0)

    def norm_rows(c):
        nr = NA * SEG // (HB // UI)
        r0 = pl.multiple_of(c * nr, 16)
        for r in range(0, nr, 16):
            hl_s[pl.ds(r0 + r, 16), :] = _ln(
                x_s[pl.ds(r0 + r + LAG * SEG, 16), :].astype(F32)).astype(BF16)

    def pre_queries(c, t=None):
        if t is not None:
            pltpu.make_async_copy(wraw.at[t], wraw.at[t], sem.at[SW + t]).wait()
            base = (t - 1) * (H * WP)
        per = -(-(D // 2) // (2 * NQH))
        dp = 0
        for sub in range(2):
            r0 = pl.multiple_of((2 * c + sub) * QR, QR)
            hl = hl_s[pl.ds(r0, QR), :]
            for hd in range(NQH):
                r = jnp.dot(hl, wslab(0, hd), preferred_element_type=F32)
                qh_s[hd, pl.ds(r0, QR), :] = r.astype(BF16)
                if t is not None:
                    tok = pltpu.bitcast(jnp.minimum(jnp.abs(r[0:16]), 0.0), U32)
                    for _ in range(per):
                        if dp < D // 2:
                            relayout_rows(t, wt_kv, base, dp, tok)
                            dp += 1

    nch = NA * SEG // TB
    QR = TB // 2
    with jax.named_scope("conv_k"):
        loop(HB // 2, fwd_k)
    with jax.named_scope("conv_u"):
        loop(HB // 4, lambda j: fwd_u(j, True))
    with jax.named_scope("conv_b"):
        loop(NPOS // 10, lambda j: [u() for n in range(10)
                                    for u in mac_units(pl.multiple_of(80 * j, 16) + 8 * n, 0)])
        xa_copy.wait()
        loop(HB // UI, lambda j: ([inv_stage(UI * j + u) for u in range(UI)], norm_rows(j)))
    with jax.named_scope("rel0"):
        w_copies[0].wait()
        loop(D // 64, lambda i: [relayout_rows(0, wt_q, 0, i * 32 + dd) for dd in range(32)])
    with jax.named_scope("preq"):
        loop(nch - 2, pre_queries)
    with jax.named_scope("conv_c"):
        for c in late_copies:
            c.wait()
        loop(HB // 4, lambda j: fwd_u(HB // 4 + j, False))
    with jax.named_scope("preq_rel"):
        loop(2, lambda i: pre_queries(i + nch - 2, i + 1))

    scale = DH ** -0.5

    def masks(mode, q0=0):
        rows = ROWS if mode == 0 else ROWS - SEG
        qi = lax.broadcasted_iota(jnp.int32, (rows - q0, 128), 0) + q0
        kj = lax.broadcasted_iota(jnp.int32, (rows - q0, 128), 1)

        def layer_of(i):
            xl = (i - 2 * M) // SEG if mode == 0 else mode - 1
            return jnp.where(i < 2 * M, i // M, xl)
        same = (layer_of(qi) == layer_of(kj)) & (kj < rows)
        vis = same & ((qi < 2 * M) | (qi >= kj))
        fill = jnp.where(same, -1e9 / scale, -jnp.inf).astype(F32)
        return vis, fill

    mem0 = mem0_ref[...].astype(F32)
    hbuf[0:16, :] = jnp.concatenate([mem0, mem0], axis=0).astype(BF16)
    hbuf[16:48, :] = _ln(x_s[0:SEG, :].astype(F32)).astype(BF16)
    obuf[...] = jnp.zeros((2 * SEG, D), F32)
    x2_s[...] = jnp.zeros(x2_s.shape, F32)

    def seg_row(seg):
        if isinstance(seg, int):
            return min(max(seg, 0), NSEG - 1) * SEG
        return pl.multiple_of(jnp.clip(seg, 0, NSEG - 1) * SEG, SEG)

    def gate(xa, r0, toks=None):
        y = jnp.concatenate([y_s[g, pl.ds(r0, xa.shape[0]), :] for g in range(NLB)], axis=1)
        return xa + _ln(xa, toks) * y

    def attention(h, vis, fill, chained, before_oproj=None, early=None, due=()):
        q0 = h.shape[0] - vis.shape[0]
        if early is not None:
            hrest = jnp.concatenate([h[:2 * M], h[2 * M + SEG:]], axis=0)
            qrow = pl.multiple_of(early * SEG, SEG)
            units = [u for n in range(PPS)
                     for u in mac_units(pl.multiple_of(early * (8 * PPS), 8 * PPS) + 8 * n, 1)]

        def proj(g):
            res = [[None] * HG for _ in range(3)]
            order = [(t, j) for j in range(HG) for t in range(2)] + [(2, j) for j in range(HG)]
            def operand(t, j):
                pre = early is not None and t == 0 and g * HG + j < NQH
                return pre, hrest if pre else (h if t else h[q0:])

            kc = D - 128
            nsplit = 4 if g == 0 and chained else 0
            part = [jnp.dot(operand(t, j)[1][:, :kc], wslab(t, j)[:kc], preferred_element_type=F32)
                    for t, j in order[:nsplit]]
            for n, (t, j) in enumerate(order):
                hd = g * HG + j
                pre, lhs = operand(t, j)
                if n < nsplit:
                    r = jnp.dot(lhs[:, kc:], wslab(t, hd)[kc:], preferred_element_type=F32) + part[n]
                else:
                    r = jnp.dot(lhs, wslab(t, hd), preferred_element_type=F32)
                if early is not None and units:
                    units.pop(0)(jnp.minimum(jnp.abs(r[0:8]), 0.0))
                if t == 0:
                    r = r.astype(BF16)
                if pre:
                    r = jnp.concatenate([r[:2 * M], qh_s[hd, pl.ds(qrow, SEG), :], r[2 * M:]], axis=0)
                res[t][j] = r
            return res

        def pad(kv):
            return jnp.concatenate([kv, jnp.zeros((128 - kv.shape[0], DH), F32)], axis=0).astype(BF16)

        def probs(qkv, g):
            scs = [lax.dot_general(qkv[0][j], pad(qkv[1][j]), (((1,), (1,)), ((), ())),
                                   preferred_element_type=F32) for j in range(HG)]
            ps = []
            for sc in scs:
                sc = jnp.where(vis, sc, fill)
                e = jnp.exp2((sc - jnp.max(sc, axis=-1, keepdims=True)) * (scale * math.log2(math.e)))
                den = jnp.sum(e, axis=-1, keepdims=True)
                if not ps and g >= NG - len(due):
                    e = jnp.concatenate([e[:16] + due[g - NG + len(due)], e[16:]], axis=0)
                r = pl.reciprocal(den, approx=True)
                r = r * (2.0 - den * r)
                ps.append((e * r).astype(BF16))
            return ps

        def oproj(os_, h0):
            oc = jnp.concatenate(os_, axis=1).astype(BF16)
            k0, k1 = h0 * DH, (h0 + len(os_)) * DH
            res = []
            for n in range(NLB):
                if before_oproj is not None:
                    w = wo_s[k0:k1, n * 128:(n + 1) * 128]
                    wo_t[n, k0 // 2:k1 // 2, :] = pltpu.bitcast(w, U32)
                else:
                    w = pltpu.bitcast(wo_t[n, k0 // 2:k1 // 2, :], BF16)
                res.append(jnp.dot(oc, w, preferred_element_type=F32))
            return res

        heads = []
        qkv = proj(0)
        oa = None
        for g in range(NG):
            ps = probs(qkv, g)
            vs = qkv[2]
            if g + 1 < NG:
                qkv = proj(g + 1)
            else:
                if before_oproj is not None:
                    before_oproj()
                oa = oproj(heads[:H // 2], 0)
            heads += [jnp.dot(ps[j], pad(vs[j]), preferred_element_type=F32)
                      for j in range(HG)]
        assert early is None or not units
        ob = oproj(heads[H // 2:], H // 2)
        return jnp.concatenate([b + a for a, b in zip(oa, ob)], axis=1)

    def post2(s, toks=None):
        r3 = seg_row(s - 1 - LAG)
        for r in (0, 16):
            xc = _r(x2_s[(s + 4 - 1 - LAG) % 4, r:r + 16] + obuf[SEG + r:SEG + r + 16, :])
            out_s[pl.ds(r3 + r, 16), :] = gate(xc, r3 + r, toks).astype(BF16)

    def step(s, mode, vis, fill, chained=False, before_oproj=None, early=None):
        if mode == 0:
            h = hbuf[...]
        elif mode == 1:
            h = hbuf[0:48, :]
        else:
            h = jnp.concatenate([hbuf[0:16, :], hbuf[48:80, :]], axis=0)
        toks = []
        if mode != 1:
            post2(s, toks)
        if isinstance(s, int) and s == NSEG + LAG - 1:
            obuf[SEG:2 * SEG, :] = attention(h, vis, fill, chained, due=toks)
            return
        r1 = seg_row(s - 1)
        rn = seg_row(s + 1)
        h1n, h2n = [], []
        for r in (0, 16):
            xa = _r(x_s[pl.ds(r1 + r, 16), :].astype(F32) + obuf[r:r + 16, :])
            xb2 = _r(gate(xa, r1 + r))
            h2n.append(_ln(xb2, toks).astype(BF16))
            x2_s[(s + 4 - 1) % 4, r:r + 16] = xb2
        if mode != 2:
            for r in (0, 16):
                h1n.append(_ln(x_s[pl.ds(rn + r, 16), :].astype(F32), toks).astype(BF16))

        o = attention(h, vis, fill, chained, before_oproj, early, toks)

        mem2 = mem0 if mode == 1 else o[M:2 * M]
        hbuf[0:16, :] = jnp.concatenate([o[0:M], mem2], axis=0).astype(BF16)
        for n, v in enumerate(h1n):
            hbuf[16 + 16 * n:32 + 16 * n, :] = v
        for n, v in enumerate(h2n):
            hbuf[48 + 16 * n:64 + 16 * n, :] = v
        if mode == 0:
            obuf[...] = o[2 * M:]
        elif mode == 1:
            obuf[0:SEG, :] = o[2 * M:]
        else:
            obuf[SEG:2 * SEG, :] = o[2 * M:]

    with jax.named_scope("pro"):
        vis, fill = masks(1)
        step(0, 1, vis, fill, False, wo_copy.wait)
        step(1, 1, vis, fill, True)
    xb_copy.wait()
    vis, fill = masks(0)
    with jax.named_scope("main_a"):
        loop(NA // UA, lambda i: [step(UA * i + u + LAG, 0, vis, fill, u > 0, early=UA * i + u)
                                  for u in range(UA)])
    with jax.named_scope("conv_e"):
        loop(HB // UI, lambda j: [inv_stage(HB + UI * j + u) for u in range(UI)])
    with jax.named_scope("main_b"):
        loop((NSEG - LAG - NA) // UB, lambda i: [step(UB * i + u + LAG + NA, 0, vis, fill, u > 0)
                                                 for u in range(UB)])
    done = (NSEG - 1 - LAG) * SEG
    out_a = pltpu.make_async_copy(out_s.at[0:done, :], out_hbm.at[0:done, :], sem.at[SW + 8])
    out_a.start()
    with jax.named_scope("epi"):
        vis, fill = masks(2)
        step(NSEG, 2, vis, fill)
        step(NSEG + 1, 2, *masks(2, 2 * M), True)
    post2(NSEG + LAG)
    out_b = pltpu.make_async_copy(out_s.at[done:S, :], out_hbm.at[done:S, :], sem.at[SW + 9])
    out_b.start()
    out_a.wait()
    out_b.wait()


@jax.jit
def pallas_interleave_layers__memory_aug_recurrent_mem_tr__ssm_conv_h3__prompt_kernel(
    A_x, A_mem0, A_Wq, A_Wk, A_Wv, A_Wo, A_seg_len,
    B_q, B_k, B_v, B_shift_k, B_ssm_k, B_ssm_D,
):
    del A_seg_len, B_q
    assert A_x.shape == (1, S, D) and A_Wq.shape == (D, H, DH)
    hbm = pl.BlockSpec(memory_space=pl.ANY)
    out = pl.pallas_call(
        _kernel,
        out_shape=jax.ShapeDtypeStruct((S, D), BF16),
        in_specs=[hbm] * 11,
        out_specs=hbm,
        scratch_shapes=[
            pltpu.VMEM((S, D), BF16),
            pltpu.VMEM((S, D), BF16),
            pltpu.VMEM((S, D), BF16),
            pltpu.VMEM((HB, D, 2 * TB), BF16),
            pltpu.VMEM((3, D, H, DH), BF16),
            pltpu.VMEM(((H + 1) * WP, 128), U32),
            pltpu.VMEM(((2 * H + 1) * WP, 128), U32),
            pltpu.VMEM((H * DH, D), BF16),
            pltpu.VMEM((NLB, H * DH // 2, 128), U32),
            pltpu.VMEM((TB, TB), BF16),
            pltpu.VMEM((2, TB, TB), BF16),
            pltpu.VMEM((2, TB // 2, 3 * TB), BF16),
            pltpu.VMEM((2, NLB, S // 2 + 8, 128), F32),
            pltpu.VMEM((NB, 2, NLB * TB, 128), F32),
            pltpu.VMEM((NB, 3, NLB * TB, 128), F32),
            pltpu.VMEM((NB + 1, 2, NLB * TB, 128), F32),
            pltpu.VMEM((NLB, S + 8, 128), F32),
            pltpu.VMEM((ROWS, D), BF16),
            pltpu.VMEM((2 * SEG, D), F32),
            pltpu.VMEM((4, SEG, D), F32),
            pltpu.VMEM((S, D), BF16),
            pltpu.VMEM((NA * SEG, D), BF16),
            pltpu.VMEM((NQH, NA * SEG, DH), BF16),
            pltpu.VMEM((M, D), BF16),
            pltpu.VMEM((KS, D), BF16),
            pltpu.VMEM((D,), BF16),
            pltpu.SemaphoreType.DMA((HB + HB // 2 + 10,)),
        ],
        compiler_params=pltpu.CompilerParams(vmem_limit_bytes=120 * 1024 * 1024),
    )(A_x.reshape(S, D), A_mem0.reshape(M, D), A_Wq, A_Wk, A_Wv,
      A_Wo.reshape(H * DH, D), B_k.reshape(S, D), B_v.reshape(S, D),
      B_shift_k.T, B_ssm_k, B_ssm_D)
    return out.reshape(1, S, D)
```

```python
import functools
import math

import jax
import jax.numpy as jnp
from jax import lax
import jax.experimental.pallas as pl
import jax.experimental.pallas.tpu as pltpu

F32 = jnp.float32
BF16 = jnp.bfloat16
U32 = jnp.uint32

S = 2048
D = 640
H = 32
DH = 128
M = 8
SEG = 32
NSEG = S // SEG
KS = 4
LAG = 2
ROWS = 2 * M + 2 * SEG
HG = 4
NG = H // HG
NLB = D // 128
TB = 128
NB = S // TB
HB = NB // 2
NPOS = NLB * TB // 8
NA = 20
PPS = 4
UCUT = tuple(range(a, a + 2) for a in range(0, 12, 2)) + (range(12, 16),)
NQH = 31
UA = 2
UB = 3
UI = 4
WP = 324


def _ln(x, toks=None):
    m = jnp.mean(x, axis=-1, keepdims=True)
    c = x - m
    v = jnp.mean(c * c, axis=-1, keepdims=True)
    r = lax.rsqrt(v + 1e-5)
    if toks is not None:
        toks.append(jnp.minimum(r, 0.0))
    return c * r


def _r(x):
    return x.astype(BF16).astype(F32)


def _split(x):
    hi = pltpu.bitcast(pltpu.bitcast(x, U32) & jnp.uint32(0xFFFF0000), F32)
    return hi, x - hi


def _pk(x):
    return pltpu.bitcast(x.astype(BF16), U32)


def _upk(w):
    return pltpu.bitcast(w, BF16)


def _basis(r, t):
    b = r & 63
    f = jnp.where(b < 32, 2 * b, 2 * b - 63)
    n = ((2 * f + 1) * t - jnp.where(r >= 64, TB, 0)) & (4 * TB - 1)
    n = jnp.where(n >= 2 * TB, n - 4 * TB, n)
    return jnp.cos(n.astype(F32) * (2.0 * math.pi / (4 * TB)))


def _halves(x):
    w = pltpu.bitcast(x, U32)
    return (pltpu.bitcast(w << 16, F32),
            pltpu.bitcast(w & jnp.uint32(0xFFFF0000), F32))


def _kernel(x_hbm, mem0_hbm, wq_hbm, wk_hbm, wv_hbm, wo_hbm,
            k_hbm, v_hbm, shk_hbm, ssmk_hbm, ssmd_hbm,
            out_hbm,
            x_s, k_s, v_s, ssmk_s, wraw, wt_q, wt_kv, wo_s, wo_t,
            perm_s, fu_s, inv_s, kpad, u_s, kf_s, c_s, y_s,
            hbuf, obuf, x2_s, out_s, hl_s, qh_s, mem0_ref, shk_ref, ssmd_ref,
            sem):
    XH = (LAG + NA) * SEG
    SW = HB + HB // 2

    def pair_rows(jp):
        r0 = jp * 2 * TB
        return pl.ds(r0 if isinstance(jp, int) else pl.multiple_of(r0, 2 * TB), 2 * TB)

    def ssmk_copy(jp):
        return pltpu.make_async_copy(ssmk_hbm.at[:, pair_rows(jp)], ssmk_s.at[jp], sem.at[jp])

    def kv_copies(rows, sm):
        return [pltpu.make_async_copy(k_hbm.at[rows, :], k_s.at[rows, :], sm),
                pltpu.make_async_copy(v_hbm.at[rows, :], v_s.at[rows, :], sm)]
    w_copies = [pltpu.make_async_copy(w, wraw.at[t], sem.at[SW + t])
                for t, w in enumerate((wq_hbm, wk_hbm, wv_hbm))]
    wo_copy = pltpu.make_async_copy(wo_hbm, wo_s, sem.at[SW + 3])
    late_copies = kv_copies(pl.ds(S // 2, S // 2), sem.at[SW + 4])
    small_copies = [pltpu.make_async_copy(src, dst, sem.at[SW + 5])
                    for src, dst in ((shk_hbm, shk_ref), (ssmd_hbm, ssmd_ref), (mem0_hbm, mem0_ref))]
    xa_copy = pltpu.make_async_copy(x_hbm.at[0:XH, :], x_s.at[0:XH, :], sem.at[SW + 6])
    xb_copy = pltpu.make_async_copy(x_hbm.at[XH:, :], x_s.at[XH:, :], sem.at[SW + 7])
    for c in (small_copies + [ssmk_copy(jp) for jp in range(HB)]
              + [c for jp in range(HB // 2) for c in kv_copies(pair_rows(jp), sem.at[HB + jp])]
              + [xa_copy, w_copies[0]] + late_copies + w_copies[1:] + [wo_copy, xb_copy]):
        c.start()

    hb = TB // 2
    ri = lax.broadcasted_iota(jnp.int32, (TB, TB), 0)
    ci = lax.broadcasted_iota(jnp.int32, (TB, TB), 1)
    perm_s[...] = _pk(jnp.where(ci == 2 * (ri & 63) + (ri >> 6), 1.0, 0.0))
    tab = _basis(ri, 2 * (ci & 63) + (ci >> 6))
    hi, lo = _split(tab)
    fu_s[0] = _pk(jnp.where(ci < hb, hi, pltpu.roll(lo, hb, 1)))
    fu_s[1] = _pk(jnp.where(ci < hb, pltpu.roll(hi, hb, 1), lo))
    gh, gl = _split(tab.T * (1.0 / TB))
    inv_s[0] = _pk(gh)
    inv_s[1] = _pk(gl)

    for c in small_copies:
        c.wait()
    shk_t = shk_ref[...].astype(F32)
    taps = [[shk_t[j:j + 1, g * 128:(g + 1) * 128] for g in range(NLB)] for j in range(KS)]
    dvec = ssmd_ref[...].astype(F32).reshape(1, D)
    for g in range(NLB):
        kpad[0, g, 0:8, :] = jnp.zeros((8, 128), F32)
        kpad[1, g, 0:8, :] = jnp.zeros((8, 128), F32)
    c_s[0] = jnp.zeros(c_s.shape[1:], F32)

    def spectrum(e, o):
        fe = jnp.dot(_upk(fu_s[0]), jnp.concatenate([e, e], axis=0).astype(BF16), preferred_element_type=F32)
        fo = jnp.dot(_upk(fu_s[1]), jnp.concatenate([o, o], axis=0).astype(BF16), preferred_element_type=F32)
        return ((fe[:hb] + fo[:hb], fe[hb:] + fo[hb:]), (fe[:hb] - fo[:hb], fo[hb:] - fe[hb:]))

    def freq_rows(g):
        return slice(g * TB, g * TB + hb), slice(g * TB + hb, (g + 1) * TB)

    def fwd_k(jq):
        for jp in (2 * jq, 2 * jq + 1):
            ssmk_copy(jp).wait()

        def transposed(n):
            blk = ssmk_s[2 * jq + n // 2, :, (n % 2) * TB:(n % 2 + 1) * TB]
            return lax.dot_general(_upk(perm_s[...]), blk, (((1,), (1,)), ((), ())),
                                   preferred_element_type=F32)
        nxt = transposed(0)
        for n in range(4):
            kt = nxt
            if n < 3:
                nxt = transposed(n + 1)
            j = 4 * jq + n
            for g in range(NLB):
                lb = slice(g * 128, (g + 1) * 128)
                for rows, (kr, ki) in zip(freq_rows(g), spectrum(kt[:hb, lb], kt[hb:, lb])):
                    if n == 0:
                        kr = kr + jnp.where(j == 0, dvec[:, lb], 0.0)
                    kf_s[j, 0, rows] = kr
                    kf_s[j, 1, rows] = ki - kr
                    kf_s[j, 2, rows] = kr + ki

    def fwd_u(jq, first):
        if first:
            for jp in (2 * jq, 2 * jq + 1):
                for c in kv_copies(pair_rows(jp), sem.at[HB + jp]):
                    c.wait()
        for j in [4 * jq + n for n in range(4)]:
            r0 = pl.multiple_of(j * TB, TB)
            q0 = pl.multiple_of(j * hb, hb) + 8
            for g in range(NLB):
                lb = slice(g * 128, (g + 1) * 128)
                ke, ko = _halves(k_s[pl.ds(r0, TB), lb])
                ve, vo = _halves(v_s[pl.ds(r0, TB), lb])
                kpad[0, g, pl.ds(q0, hb), :] = ke
                kpad[1, g, pl.ds(q0, hb), :] = ko
                ke1 = kpad[0, g, pl.ds(q0 - 1, hb), :]
                ko1 = kpad[1, g, pl.ds(q0 - 1, hb), :]
                ko2 = kpad[1, g, pl.ds(q0 - 2, hb), :]
                t0, t1, t2, t3 = (taps[t][g] for t in range(KS))
                e = (ke * t0 + ko1 * t1 + ke1 * t2 + ko2 * t3) * ve
                o = (ko * t0 + ke * t1 + ko1 * t2 + ke1 * t3) * vo
                for rows, (ur, ui) in zip(freq_rows(g), spectrum(e, o)):
                    u_s[j, 0, rows] = ur
                    u_s[j, 1, rows] = ui

    def mac_units(row, half):
        rs = pl.ds(row, 8)
        state = {}

        def unit(p, avals, final, tok=None):
            acc = state.setdefault(p, dict(state.get(0, {})))
            for a in avals:
                u = u_s[a, 0, rs] + u_s[a, 1, rs] if p == 0 else u_s[a, p - 1, rs]
                if tok is not None:
                    u = u + tok
                for i in range(max(a, half * HB), half * HB + HB):
                    t = u * kf_s[i - a, p, rs]
                    acc[i] = t if i not in acc else (acc[i] - t if p == 2 else acc[i] + t)
            if final and p:
                for i, v in acc.items():
                    c_s[i + 1, 2 - p, rs] = v

        subs = UCUT if half else (range(HB),)
        return [functools.partial(unit, p, avals, n == len(subs) - 1)
                for p in range(3) for n, avals in enumerate(subs)]

    def inv_stage(i):
        q = TB // 4
        for g in range(NLB):
            re, im = [], []
            for b in range(4):
                rows = slice(g * TB + b * q, g * TB + (b + 1) * q)
                cr, ci_ = c_s[i + 1, 0, rows], c_s[i + 1, 1, rows]
                pr, pi = c_s[i, 0, rows], c_s[i, 1, rows]
                re.append(cr + pi if b in (0, 3) else cr - pi)
                im.append(ci_ - pr if b in (0, 3) else ci_ + pr)
            pe = jnp.concatenate([re[0] + re[2], re[1] + re[3], im[0] - im[2], im[1] - im[3]], axis=0)
            po = jnp.concatenate([re[0] - re[2], re[1] - re[3], im[0] + im[2], im[1] + im[3]], axis=0)
            for par, pp in enumerate((pe, po)):
                ph, plo = _split(pp)
                gh_, gl_ = (inv_s[n, par * q:(par + 1) * q] for n in range(2))
                y_s[g, pl.ds(i * TB + par, hb, stride=2), :] = jnp.dot(
                    _upk(jnp.concatenate([gh_, gl_, gh_], axis=1)),
                    jnp.concatenate([ph, ph, plo], axis=0).astype(BF16),
                    preferred_element_type=F32)

    def relayout_rows(t, dst, base, dp, tok=None):
        a = pltpu.bitcast(wraw[t, 2 * dp], U32)
        b = pltpu.bitcast(wraw[t, 2 * dp + 1], U32)
        if tok is not None:
            a = a | tok
        dst[pl.ds(base + dp, 16, stride=WP), :] = (a & jnp.uint32(0xFFFF)) | (b << 16)
        dst[pl.ds(base + 16 * WP + dp, 16, stride=WP), :] = (
            (a >> 16) | (b & jnp.uint32(0xFFFF0000)))

    def wslab(t, h):
        s0 = (max(t - 1, 0) * H + (h % 2) * 16 + h // 2) * WP
        return pltpu.bitcast((wt_kv if t else wt_q)[s0:s0 + D // 2, :], BF16)

    def loop(n, fn):
        def body(j, _):
            fn(j)
            return 0
        lax.fori_loop(0, n, body, 0)

    def norm_rows(c):
        nr = NA * SEG // (HB // UI)
        r0 = pl.multiple_of(c * nr, 16)
        for r in range(0, nr, 16):
            hl_s[pl.ds(r0 + r, 16), :] = _ln(
                x_s[pl.ds(r0 + r + LAG * SEG, 16), :].astype(F32)).astype(BF16)

    def pre_queries(c, t=None):
        if t is not None:
            pltpu.make_async_copy(wraw.at[t], wraw.at[t], sem.at[SW + t]).wait()
            base = (t - 1) * (H * WP)
        per = -(-(D // 2) // (2 * NQH))
        dp = 0
        for sub in range(2):
            r0 = pl.multiple_of((2 * c + sub) * QR, QR)
            hl = hl_s[pl.ds(r0, QR), :]
            for hd in range(NQH):
                r = jnp.dot(hl, wslab(0, hd), preferred_element_type=F32)
                qh_s[hd, pl.ds(r0, QR), :] = r.astype(BF16)
                if t is not None:
                    tok = pltpu.bitcast(jnp.minimum(jnp.abs(r[0:16]), 0.0), U32)
                    for _ in range(per):
                        if dp < D // 2:
                            relayout_rows(t, wt_kv, base, dp, tok)
                            dp += 1

    nch = NA * SEG // TB
    QR = TB // 2
    with jax.named_scope("conv_k"):
        loop(HB // 2, fwd_k)
    with jax.named_scope("conv_u"):
        loop(HB // 4, lambda j: fwd_u(j, True))
    with jax.named_scope("conv_b"):
        loop(NPOS // 10, lambda j: [u() for n in range(10)
                                    for u in mac_units(pl.multiple_of(80 * j, 16) + 8 * n, 0)])
        xa_copy.wait()
        loop(HB // UI, lambda j: ([inv_stage(UI * j + u) for u in range(UI)], norm_rows(j)))
    with jax.named_scope("rel0"):
        w_copies[0].wait()
        loop(D // 64, lambda i: [relayout_rows(0, wt_q, 0, i * 32 + dd) for dd in range(32)])
    with jax.named_scope("preq"):
        loop(nch - 2, pre_queries)
    with jax.named_scope("conv_c"):
        for c in late_copies:
            c.wait()
        loop(HB // 4, lambda j: fwd_u(HB // 4 + j, False))
    with jax.named_scope("preq_rel"):
        loop(2, lambda i: pre_queries(i + nch - 2, i + 1))

    scale = DH ** -0.5

    def masks(mode, q0=0):
        rows = ROWS if mode == 0 else ROWS - SEG
        qi = lax.broadcasted_iota(jnp.int32, (rows - q0, 128), 0) + q0
        kj = lax.broadcasted_iota(jnp.int32, (rows - q0, 128), 1)

        def layer_of(i):
            xl = (i - 2 * M) // SEG if mode == 0 else mode - 1
            return jnp.where(i < 2 * M, i // M, xl)
        same = (layer_of(qi) == layer_of(kj)) & (kj < rows)
        vis = same & ((qi < 2 * M) | (qi >= kj))
        fill = jnp.where(same, -1e9 / scale, -jnp.inf).astype(F32)
        return vis, fill

    mem0 = mem0_ref[...].astype(F32)
    hbuf[0:16, :] = jnp.concatenate([mem0, mem0], axis=0).astype(BF16)
    hbuf[16:48, :] = _ln(x_s[0:SEG, :].astype(F32)).astype(BF16)
    obuf[...] = jnp.zeros((2 * SEG, D), F32)
    x2_s[...] = jnp.zeros(x2_s.shape, F32)

    def seg_row(seg):
        if isinstance(seg, int):
            return min(max(seg, 0), NSEG - 1) * SEG
        return pl.multiple_of(jnp.clip(seg, 0, NSEG - 1) * SEG, SEG)

    def gate(xa, r0, toks=None):
        y = jnp.concatenate([y_s[g, pl.ds(r0, xa.shape[0]), :] for g in range(NLB)], axis=1)
        return xa + _ln(xa, toks) * y

    def attention(h, vis, fill, chained, before_oproj=None, early=None, due=()):
        q0 = h.shape[0] - vis.shape[0]
        if early is not None:
            hrest = jnp.concatenate([h[:2 * M], h[2 * M + SEG:]], axis=0)
            qrow = pl.multiple_of(early * SEG, SEG)
            units = [u for n in range(PPS)
                     for u in mac_units(pl.multiple_of(early * (8 * PPS), 8 * PPS) + 8 * n, 1)]

        def proj(g):
            res = [[None] * HG for _ in range(3)]
            order = [(t, j) for j in range(HG) for t in range(2)] + [(2, j) for j in range(HG)]
            def operand(t, j):
                pre = early is not None and t == 0 and g * HG + j < NQH
                return pre, hrest if pre else (h if t else h[q0:])

            kc = D - 128
            nsplit = 4 if g == 0 and chained else 0
            part = [jnp.dot(operand(t, j)[1][:, :kc], wslab(t, j)[:kc], preferred_element_type=F32)
                    for t, j in order[:nsplit]]
            for n, (t, j) in enumerate(order):
                hd = g * HG + j
                pre, lhs = operand(t, j)
                if n < nsplit:
                    r = jnp.dot(lhs[:, kc:], wslab(t, hd)[kc:], preferred_element_type=F32) + part[n]
                else:
                    r = jnp.dot(lhs, wslab(t, hd), preferred_element_type=F32)
                if early is not None and units:
                    units.pop(0)(jnp.minimum(jnp.abs(r[0:8]), 0.0))
                if t == 0:
                    r = r.astype(BF16)
                if pre:
                    r = jnp.concatenate([r[:2 * M], qh_s[hd, pl.ds(qrow, SEG), :], r[2 * M:]], axis=0)
                res[t][j] = r
            return res

        def pad(kv):
            return jnp.concatenate([kv, jnp.zeros((128 - kv.shape[0], DH), F32)], axis=0).astype(BF16)

        def probs(qkv, g):
            scs = [lax.dot_general(qkv[0][j], pad(qkv[1][j]), (((1,), (1,)), ((), ())),
                                   preferred_element_type=F32) for j in range(HG)]
            ps = []
            for sc in scs:
                sc = jnp.where(vis, sc, fill)
                e = jnp.exp2((sc - jnp.max(sc, axis=-1, keepdims=True)) * (scale * math.log2(math.e)))
                den = jnp.sum(e, axis=-1, keepdims=True)
                if not ps and g >= NG - len(due):
                    e = jnp.concatenate([e[:16] + due[g - NG + len(due)], e[16:]], axis=0)
                r = pl.reciprocal(den, approx=True)
                r = r * (2.0 - den * r)
                ps.append((e * r).astype(BF16))
            return ps

        def oproj(os_, h0):
            oc = jnp.concatenate(os_, axis=1).astype(BF16)
            k0, k1 = h0 * DH, (h0 + len(os_)) * DH
            res = []
            for n in range(NLB):
                if before_oproj is not None:
                    w = wo_s[k0:k1, n * 128:(n + 1) * 128]
                    wo_t[n, k0 // 2:k1 // 2, :] = pltpu.bitcast(w, U32)
                else:
                    w = pltpu.bitcast(wo_t[n, k0 // 2:k1 // 2, :], BF16)
                res.append(jnp.dot(oc, w, preferred_element_type=F32))
            return res

        heads = []
        qkv = proj(0)
        oa = None
        for g in range(NG):
            ps = probs(qkv, g)
            vs = qkv[2]
            if g + 1 < NG:
                qkv = proj(g + 1)
            else:
                if before_oproj is not None:
                    before_oproj()
                oa = oproj(heads[:H // 2], 0)
            heads += [jnp.dot(ps[j], pad(vs[j]), preferred_element_type=F32)
                      for j in range(HG)]
        assert early is None or not units
        ob = oproj(heads[H // 2:], H // 2)
        return jnp.concatenate([b + a for a, b in zip(oa, ob)], axis=1)

    def post2(s, toks=None):
        r3 = seg_row(s - 1 - LAG)
        for r in (0, 16):
            xc = _r(x2_s[(s + 4 - 1 - LAG) % 4, r:r + 16] + obuf[SEG + r:SEG + r + 16, :])
            out_s[pl.ds(r3 + r, 16), :] = gate(xc, r3 + r, toks).astype(BF16)

    def step(s, mode, vis, fill, chained=False, before_oproj=None, early=None):
        if mode == 0:
            h = hbuf[...]
        elif mode == 1:
            h = hbuf[0:48, :]
        else:
            h = jnp.concatenate([hbuf[0:16, :], hbuf[48:80, :]], axis=0)
        toks = []
        if mode != 1:
            post2(s, toks)
        if isinstance(s, int) and s == NSEG + LAG - 1:
            obuf[SEG:2 * SEG, :] = attention(h, vis, fill, chained, due=toks)
            return
        r1 = seg_row(s - 1)
        rn = seg_row(s + 1)
        h1n, h2n = [], []
        for r in (0, 16):
            xa = _r(x_s[pl.ds(r1 + r, 16), :].astype(F32) + obuf[r:r + 16, :])
            xb2 = _r(gate(xa, r1 + r))
            h2n.append(_ln(xb2, toks).astype(BF16))
            x2_s[(s + 4 - 1) % 4, r:r + 16] = xb2
        if mode != 2:
            for r in (0, 16):
                h1n.append(_ln(x_s[pl.ds(rn + r, 16), :].astype(F32), toks).astype(BF16))

        o = attention(h, vis, fill, chained, before_oproj, early, toks)

        mem2 = mem0 if mode == 1 else o[M:2 * M]
        hbuf[0:16, :] = jnp.concatenate([o[0:M], mem2], axis=0).astype(BF16)
        for n, v in enumerate(h1n):
            hbuf[16 + 16 * n:32 + 16 * n, :] = v
        for n, v in enumerate(h2n):
            hbuf[48 + 16 * n:64 + 16 * n, :] = v
        if mode == 0:
            obuf[...] = o[2 * M:]
        elif mode == 1:
            obuf[0:SEG, :] = o[2 * M:]
        else:
            obuf[SEG:2 * SEG, :] = o[2 * M:]

    with jax.named_scope("pro"):
        vis, fill = masks(1)
        step(0, 1, vis, fill, False, wo_copy.wait)
        step(1, 1, vis, fill, True)
    xb_copy.wait()
    vis, fill = masks(0)
    with jax.named_scope("main_a"):
        loop(NA // UA, lambda i: [step(UA * i + u + LAG, 0, vis, fill, u > 0, early=UA * i + u)
                                  for u in range(UA)])
    with jax.named_scope("conv_e"):
        loop(HB // UI, lambda j: [inv_stage(HB + UI * j + u) for u in range(UI)])
    with jax.named_scope("main_b"):
        loop((NSEG - LAG - NA) // UB, lambda i: [step(UB * i + u + LAG + NA, 0, vis, fill, u > 0)
                                                 for u in range(UB)])
    done = (NSEG - 1 - LAG) * SEG
    out_a = pltpu.make_async_copy(out_s.at[0:done, :], out_hbm.at[0:done, :], sem.at[SW + 8])
    out_a.start()
    with jax.named_scope("epi"):
        vis, fill = masks(2)
        step(NSEG, 2, vis, fill)
        step(NSEG + 1, 2, *masks(2, 2 * M), True)
    post2(NSEG + LAG)
    out_b = pltpu.make_async_copy(out_s.at[done:S, :], out_hbm.at[done:S, :], sem.at[SW + 9])
    out_b.start()
    out_a.wait()
    out_b.wait()


@jax.jit
def pallas_interleave_layers__memory_aug_recurrent_mem_tr__ssm_conv_h3__prompt_kernel(
    A_x, A_mem0, A_Wq, A_Wk, A_Wv, A_Wo, A_seg_len,
    B_q, B_k, B_v, B_shift_k, B_ssm_k, B_ssm_D,
):
    del A_seg_len, B_q
    assert A_x.shape == (1, S, D) and A_Wq.shape == (D, H, DH)
    hbm = pl.BlockSpec(memory_space=pl.ANY)
    out = pl.pallas_call(
        _kernel,
        out_shape=jax.ShapeDtypeStruct((S, D), BF16),
        in_specs=[hbm] * 11,
        out_specs=hbm,
        scratch_shapes=[
            pltpu.VMEM((S, D), BF16),
            pltpu.VMEM((S, D), BF16),
            pltpu.VMEM((S, D), BF16),
            pltpu.VMEM((HB, D, 2 * TB), BF16),
            pltpu.VMEM((3, D, H, DH), BF16),
            pltpu.VMEM(((H + 1) * WP, 128), U32),
            pltpu.VMEM(((2 * H + 1) * WP, 128), U32),
            pltpu.VMEM((H * DH, D), BF16),
            pltpu.VMEM((NLB, H * DH // 2, 128), U32),
            pltpu.VMEM((TB // 2, TB), U32),
            pltpu.VMEM((2, TB // 2, TB), U32),
            pltpu.VMEM((2, TB // 2, TB), U32),
            pltpu.VMEM((2, NLB, S // 2 + 8, 128), F32),
            pltpu.VMEM((NB, 2, NLB * TB, 128), F32),
            pltpu.VMEM((NB, 3, NLB * TB, 128), F32),
            pltpu.VMEM((NB + 1, 2, NLB * TB, 128), F32),
            pltpu.VMEM((NLB, S + 8, 128), F32),
            pltpu.VMEM((ROWS, D), BF16),
            pltpu.VMEM((2 * SEG, D), F32),
            pltpu.VMEM((4, SEG, D), F32),
            pltpu.VMEM((S, D), BF16),
            pltpu.VMEM((NA * SEG, D), BF16),
            pltpu.VMEM((NQH, NA * SEG, DH), BF16),
            pltpu.VMEM((M, D), BF16),
            pltpu.VMEM((KS, D), BF16),
            pltpu.VMEM((D,), BF16),
            pltpu.SemaphoreType.DMA((HB + HB // 2 + 10,)),
        ],
        compiler_params=pltpu.CompilerParams(vmem_limit_bytes=120 * 1024 * 1024),
    )(A_x.reshape(S, D), A_mem0.reshape(M, D), A_Wq, A_Wk, A_Wv,
      A_Wo.reshape(H * DH, D), B_k.reshape(S, D), B_v.reshape(S, D),
      B_shift_k.T, B_ssm_k, B_ssm_D)
    return out.reshape(1, S, D)
```

```python
import functools
import math

import jax
import jax.numpy as jnp
from jax import lax
import jax.experimental.pallas as pl
import jax.experimental.pallas.tpu as pltpu

F32 = jnp.float32
BF16 = jnp.bfloat16
U32 = jnp.uint32

S = 2048
D = 640
H = 32
DH = 128
M = 8
SEG = 32
NSEG = S // SEG
KS = 4
LAG = 2
ROWS = 2 * M + 2 * SEG
HG = 4
NG = H // HG
NLB = D // 128
TB = 128
NB = S // TB
HB = NB // 2
NPOS = NLB * TB // 8
NA = 20
PPS = 4
UCUT = tuple(range(a, a + 2) for a in range(0, 12, 2)) + (range(12, 16),)
NQH = 31
UA = 2
UB = 3
UI = 4
WP = 324


def _ln(x, toks=None):
    m = jnp.mean(x, axis=-1, keepdims=True)
    c = x - m
    v = jnp.mean(c * c, axis=-1, keepdims=True)
    r = lax.rsqrt(v + 1e-5)
    if toks is not None:
        toks.append(jnp.minimum(r, 0.0))
    return c * r


def _r(x):
    return x.astype(BF16).astype(F32)


def _split(x):
    hi = pltpu.bitcast(pltpu.bitcast(x, U32) & jnp.uint32(0xFFFF0000), F32)
    return hi, x - hi


def _pk(x):
    return pltpu.bitcast(x.astype(BF16), U32)


def _upk(w):
    return pltpu.bitcast(w, BF16)


def _basis(r, t):
    b = r & 63
    f = jnp.where(b < 32, 2 * b, 2 * b - 63)
    n = ((2 * f + 1) * t - jnp.where(r >= 64, TB, 0)) & (4 * TB - 1)
    n = jnp.where(n >= 2 * TB, n - 4 * TB, n)
    return jnp.cos(n.astype(F32) * (2.0 * math.pi / (4 * TB)))


def _halves(x):
    w = pltpu.bitcast(x, U32)
    return (pltpu.bitcast(w << 16, F32),
            pltpu.bitcast(w & jnp.uint32(0xFFFF0000), F32))


def _kernel(x_hbm, mem0_hbm, wq_hbm, wk_hbm, wv_hbm, wo_hbm,
            k_hbm, v_hbm, shk_hbm, ssmk_hbm, ssmd_hbm,
            out_hbm,
            x_s, k_s, v_s, ssmk_s, wraw, wt_q, wt_kv, wo_s, wo_t,
            perm_s, fu_s, inv_s, kpad, u_s, kf_s, c_s, y_s,
            hbuf, obuf, x2_s, out_s, hl_s, qh_s, mem0_ref, shk_ref, ssmd_ref,
            sem):
    X0, XH = LAG * SEG, (LAG + NA) * SEG
    SW = HB + HB // 2

    def pair_rows(jp):
        r0 = jp * 2 * TB
        return pl.ds(r0 if isinstance(jp, int) else pl.multiple_of(r0, 2 * TB), 2 * TB)

    def ssmk_copy(jp):
        return pltpu.make_async_copy(ssmk_hbm.at[:, pair_rows(jp)], ssmk_s.at[jp], sem.at[jp])

    def kv_copies(rows, sm):
        return [pltpu.make_async_copy(k_hbm.at[rows, :], k_s.at[rows, :], sm),
                pltpu.make_async_copy(v_hbm.at[rows, :], v_s.at[rows, :], sm)]
    w_copies = [pltpu.make_async_copy(w, wraw.at[t], sem.at[SW + t])
                for t, w in enumerate((wq_hbm, wk_hbm, wv_hbm))]
    wo_copy = pltpu.make_async_copy(wo_hbm, wo_s, sem.at[SW + 3])
    late_copies = kv_copies(pl.ds(S // 2, S // 2), sem.at[SW + 4])
    small_copies = [pltpu.make_async_copy(src, dst, sem.at[SW + 5])
                    for src, dst in ((shk_hbm, shk_ref), (ssmd_hbm, ssmd_ref), (mem0_hbm, mem0_ref))]
    xa_copy = pltpu.make_async_copy(x_hbm.at[X0:XH, :], x_s.at[X0:XH, :], sem.at[SW + 6])
    late_copies += [pltpu.make_async_copy(x_hbm.at[a:b, :], x_s.at[a:b, :], sem.at[SW + 4])
                    for a, b in ((0, X0), (XH, XH + SEG))]
    xb_copy = pltpu.make_async_copy(x_hbm.at[XH + SEG:, :], x_s.at[XH + SEG:, :], sem.at[SW + 7])
    for c in (small_copies + [ssmk_copy(jp) for jp in range(HB)]
              + [c for jp in range(HB // 2) for c in kv_copies(pair_rows(jp), sem.at[HB + jp])]
              + [xa_copy, w_copies[0]] + late_copies + w_copies[1:] + [wo_copy]):
        c.start()

    hb = TB // 2
    ri = lax.broadcasted_iota(jnp.int32, (TB, TB), 0)
    ci = lax.broadcasted_iota(jnp.int32, (TB, TB), 1)
    perm_s[...] = _pk(jnp.where(ci == 2 * (ri & 63) + (ri >> 6), 1.0, 0.0))
    tab = _basis(ri, 2 * (ci & 63) + (ci >> 6))
    hi, lo = _split(tab)
    fu_s[0] = _pk(jnp.where(ci < hb, hi, pltpu.roll(lo, hb, 1)))
    fu_s[1] = _pk(jnp.where(ci < hb, pltpu.roll(hi, hb, 1), lo))
    gh, gl = _split(tab.T * (1.0 / TB))
    inv_s[0] = _pk(gh)
    inv_s[1] = _pk(gl)

    for c in small_copies:
        c.wait()
    shk_t = shk_ref[...].astype(F32)
    taps = [[shk_t[j:j + 1, g * 128:(g + 1) * 128] for g in range(NLB)] for j in range(KS)]
    dvec = ssmd_ref[...].astype(F32).reshape(1, D)
    for g in range(NLB):
        kpad[0, g, 0:8, :] = jnp.zeros((8, 128), F32)
        kpad[1, g, 0:8, :] = jnp.zeros((8, 128), F32)
    c_s[0] = jnp.zeros(c_s.shape[1:], F32)

    def spectrum(e, o):
        fe = jnp.dot(_upk(fu_s[0]), jnp.concatenate([e, e], axis=0).astype(BF16), preferred_element_type=F32)
        fo = jnp.dot(_upk(fu_s[1]), jnp.concatenate([o, o], axis=0).astype(BF16), preferred_element_type=F32)
        return ((fe[:hb] + fo[:hb], fe[hb:] + fo[hb:]), (fe[:hb] - fo[:hb], fo[hb:] - fe[hb:]))

    def freq_rows(g):
        return slice(g * TB, g * TB + hb), slice(g * TB + hb, (g + 1) * TB)

    def fwd_k(jq):
        for jp in (2 * jq, 2 * jq + 1):
            ssmk_copy(jp).wait()

        def transposed(n):
            blk = ssmk_s[2 * jq + n // 2, :, (n % 2) * TB:(n % 2 + 1) * TB]
            return lax.dot_general(_upk(perm_s[...]), blk, (((1,), (1,)), ((), ())),
                                   preferred_element_type=F32)
        nxt = transposed(0)
        for n in range(4):
            kt = nxt
            if n < 3:
                nxt = transposed(n + 1)
            j = 4 * jq + n
            for g in range(NLB):
                lb = slice(g * 128, (g + 1) * 128)
                for rows, (kr, ki) in zip(freq_rows(g), spectrum(kt[:hb, lb], kt[hb:, lb])):
                    if n == 0:
                        kr = kr + jnp.where(j == 0, dvec[:, lb], 0.0)
                    kf_s[j, 0, rows] = kr
                    kf_s[j, 1, rows] = ki - kr
                    kf_s[j, 2, rows] = kr + ki

    def fwd_u(jq, first):
        if first:
            for jp in (2 * jq, 2 * jq + 1):
                for c in kv_copies(pair_rows(jp), sem.at[HB + jp]):
                    c.wait()
        for j in [4 * jq + n for n in range(4)]:
            r0 = pl.multiple_of(j * TB, TB)
            q0 = pl.multiple_of(j * hb, hb) + 8
            for g in range(NLB):
                lb = slice(g * 128, (g + 1) * 128)
                ke, ko = _halves(k_s[pl.ds(r0, TB), lb])
                ve, vo = _halves(v_s[pl.ds(r0, TB), lb])
                kpad[0, g, pl.ds(q0, hb), :] = ke
                kpad[1, g, pl.ds(q0, hb), :] = ko
                ke1 = kpad[0, g, pl.ds(q0 - 1, hb), :]
                ko1 = kpad[1, g, pl.ds(q0 - 1, hb), :]
                ko2 = kpad[1, g, pl.ds(q0 - 2, hb), :]
                t0, t1, t2, t3 = (taps[t][g] for t in range(KS))
                e = (ke * t0 + ko1 * t1 + ke1 * t2 + ko2 * t3) * ve
                o = (ko * t0 + ke * t1 + ko1 * t2 + ke1 * t3) * vo
                for rows, (ur, ui) in zip(freq_rows(g), spectrum(e, o)):
                    u_s[j, 0, rows] = ur
                    u_s[j, 1, rows] = ui

    def mac_units(row, half):
        rs = pl.ds(row, 8)
        state = {}

        def unit(p, avals, final, tok=None):
            acc = state.setdefault(p, dict(state.get(0, {})))
            for a in avals:
                u = u_s[a, 0, rs] + u_s[a, 1, rs] if p == 0 else u_s[a, p - 1, rs]
                if tok is not None:
                    u = u + tok
                for i in range(max(a, half * HB), half * HB + HB):
                    t = u * kf_s[i - a, p, rs]
                    acc[i] = t if i not in acc else (acc[i] - t if p == 2 else acc[i] + t)
            if final and p:
                for i, v in acc.items():
                    c_s[i + 1, 2 - p, rs] = v

        subs = UCUT if half else (range(HB),)
        return [functools.partial(unit, p, avals, n == len(subs) - 1)
                for p in range(3) for n, avals in enumerate(subs)]

    def inv_stage(i):
        q = TB // 4
        for g in range(NLB):
            re, im = [], []
            for b in range(4):
                rows = slice(g * TB + b * q, g * TB + (b + 1) * q)
                cr, ci_ = c_s[i + 1, 0, rows], c_s[i + 1, 1, rows]
                pr, pi = c_s[i, 0, rows], c_s[i, 1, rows]
                re.append(cr + pi if b in (0, 3) else cr - pi)
                im.append(ci_ - pr if b in (0, 3) else ci_ + pr)
            pe = jnp.concatenate([re[0] + re[2], re[1] + re[3], im[0] - im[2], im[1] - im[3]], axis=0)
            po = jnp.concatenate([re[0] - re[2], re[1] - re[3], im[0] + im[2], im[1] + im[3]], axis=0)
            for par, pp in enumerate((pe, po)):
                ph, plo = _split(pp)
                gh_, gl_ = (inv_s[n, par * q:(par + 1) * q] for n in range(2))
                y_s[g, pl.ds(i * TB + par, hb, stride=2), :] = jnp.dot(
                    _upk(jnp.concatenate([gh_, gl_, gh_], axis=1)),
                    jnp.concatenate([ph, ph, plo], axis=0).astype(BF16),
                    preferred_element_type=F32)

    def relayout_rows(t, dst, base, dp, tok=None):
        a = pltpu.bitcast(wraw[t, 2 * dp], U32)
        b = pltpu.bitcast(wraw[t, 2 * dp + 1], U32)
        if tok is not None:
            a = a | tok
        dst[pl.ds(base + dp, 16, stride=WP), :] = (a & jnp.uint32(0xFFFF)) | (b << 16)
        dst[pl.ds(base + 16 * WP + dp, 16, stride=WP), :] = (
            (a >> 16) | (b & jnp.uint32(0xFFFF0000)))

    def wslab(t, h):
        s0 = (max(t - 1, 0) * H + (h % 2) * 16 + h // 2) * WP
        return pltpu.bitcast((wt_kv if t else wt_q)[s0:s0 + D // 2, :], BF16)

    def loop(n, fn):
        def body(j, _):
            fn(j)
            return 0
        lax.fori_loop(0, n, body, 0)

    def norm_rows(c):
        nr = NA * SEG // (HB // UI)
        r0 = pl.multiple_of(c * nr, 16)
        for r in range(0, nr, 16):
            hl_s[pl.ds(r0 + r, 16), :] = _ln(
                x_s[pl.ds(r0 + r + LAG * SEG, 16), :].astype(F32)).astype(BF16)

    def pre_queries(c, t=None):
        if t is not None:
            pltpu.make_async_copy(wraw.at[t], wraw.at[t], sem.at[SW + t]).wait()
            base = (t - 1) * (H * WP)
        per = -(-(D // 2) // (2 * NQH))
        dp = 0
        for sub in range(2):
            r0 = pl.multiple_of((2 * c + sub) * QR, QR)
            hl = hl_s[pl.ds(r0, QR), :]
            for hd in range(NQH):
                r = jnp.dot(hl, wslab(0, hd), preferred_element_type=F32)
                qh_s[hd, pl.ds(r0, QR), :] = r.astype(BF16)
                if t is not None:
                    tok = pltpu.bitcast(jnp.minimum(jnp.abs(r[0:16]), 0.0), U32)
                    for _ in range(per):
                        if dp < D // 2:
                            relayout_rows(t, wt_kv, base, dp, tok)
                            dp += 1

    nch = NA * SEG // TB
    QR = TB // 2
    with jax.named_scope("conv_k"):
        loop(HB // 2, fwd_k)
    with jax.named_scope("conv_u"):
        loop(HB // 4, lambda j: fwd_u(j, True))
    with jax.named_scope("conv_b"):
        loop(NPOS // 10, lambda j: [u() for n in range(10)
                                    for u in mac_units(pl.multiple_of(80 * j, 16) + 8 * n, 0)])
        xa_copy.wait()
        loop(HB // UI, lambda j: ([inv_stage(UI * j + u) for u in range(UI)], norm_rows(j)))
    with jax.named_scope("rel0"):
        w_copies[0].wait()
        loop(D // 64, lambda i: [relayout_rows(0, wt_q, 0, i * 32 + dd) for dd in range(32)])
    with jax.named_scope("preq"):
        loop(nch - 2, pre_queries)
    with jax.named_scope("conv_c"):
        for c in late_copies:
            c.wait()
        loop(HB // 4, lambda j: fwd_u(HB // 4 + j, False))
    with jax.named_scope("preq_rel"):
        loop(2, lambda i: pre_queries(i + nch - 2, i + 1))

    scale = DH ** -0.5

    def masks(mode, q0=0):
        rows = ROWS if mode == 0 else ROWS - SEG
        qi = lax.broadcasted_iota(jnp.int32, (rows - q0, 128), 0) + q0
        kj = lax.broadcasted_iota(jnp.int32, (rows - q0, 128), 1)

        def layer_of(i):
            xl = (i - 2 * M) // SEG if mode == 0 else mode - 1
            return jnp.where(i < 2 * M, i // M, xl)
        same = (layer_of(qi) == layer_of(kj)) & (kj < rows)
        vis = same & ((qi < 2 * M) | (qi >= kj))
        fill = jnp.where(same, -1e9 / scale, -jnp.inf).astype(F32)
        return vis, fill

    mem0 = mem0_ref[...].astype(F32)
    hbuf[0:16, :] = jnp.concatenate([mem0, mem0], axis=0).astype(BF16)
    hbuf[16:48, :] = _ln(x_s[0:SEG, :].astype(F32)).astype(BF16)
    obuf[...] = jnp.zeros((2 * SEG, D), F32)
    x2_s[...] = jnp.zeros(x2_s.shape, F32)

    def seg_row(seg):
        if isinstance(seg, int):
            return min(max(seg, 0), NSEG - 1) * SEG
        return pl.multiple_of(jnp.clip(seg, 0, NSEG - 1) * SEG, SEG)

    def gate(xa, r0, toks=None):
        y = jnp.concatenate([y_s[g, pl.ds(r0, xa.shape[0]), :] for g in range(NLB)], axis=1)
        return xa + _ln(xa, toks) * y

    def attention(h, vis, fill, chained, before_oproj=None, early=None, due=()):
        q0 = h.shape[0] - vis.shape[0]
        if early is not None:
            hrest = jnp.concatenate([h[:2 * M], h[2 * M + SEG:]], axis=0)
            qrow = pl.multiple_of(early * SEG, SEG)
            units = [u for n in range(PPS)
                     for u in mac_units(pl.multiple_of(early * (8 * PPS), 8 * PPS) + 8 * n, 1)]

        def proj(g):
            res = [[None] * HG for _ in range(3)]
            order = [(t, j) for j in range(HG) for t in range(2)] + [(2, j) for j in range(HG)]
            def operand(t, j):
                pre = early is not None and t == 0 and g * HG + j < NQH
                return pre, hrest if pre else (h if t else h[q0:])

            kc = D - 128
            nsplit = 4 if g == 0 and chained else 0
            part = [jnp.dot(operand(t, j)[1][:, :kc], wslab(t, j)[:kc], preferred_element_type=F32)
                    for t, j in order[:nsplit]]
            for n, (t, j) in enumerate(order):
                hd = g * HG + j
                pre, lhs = operand(t, j)
                if n < nsplit:
                    r = jnp.dot(lhs[:, kc:], wslab(t, hd)[kc:], preferred_element_type=F32) + part[n]
                else:
                    r = jnp.dot(lhs, wslab(t, hd), preferred_element_type=F32)
                if early is not None and units:
                    units.pop(0)(jnp.minimum(jnp.abs(r[0:8]), 0.0))
                if t == 0:
                    r = r.astype(BF16)
                if pre:
                    r = jnp.concatenate([r[:2 * M], qh_s[hd, pl.ds(qrow, SEG), :], r[2 * M:]], axis=0)
                res[t][j] = r
            return res

        def pad(kv):
            return jnp.concatenate([kv, jnp.zeros((128 - kv.shape[0], DH), F32)], axis=0).astype(BF16)

        def probs(qkv, g):
            scs = [lax.dot_general(qkv[0][j], pad(qkv[1][j]), (((1,), (1,)), ((), ())),
                                   preferred_element_type=F32) for j in range(HG)]
            ps = []
            for sc in scs:
                sc = jnp.where(vis, sc, fill)
                e = jnp.exp2((sc - jnp.max(sc, axis=-1, keepdims=True)) * (scale * math.log2(math.e)))
                den = jnp.sum(e, axis=-1, keepdims=True)
                if not ps and g >= NG - len(due):
                    e = jnp.concatenate([e[:16] + due[g - NG + len(due)], e[16:]], axis=0)
                r = pl.reciprocal(den, approx=True)
                r = r * (2.0 - den * r)
                ps.append((e * r).astype(BF16))
            return ps

        def oproj(os_, h0):
            oc = jnp.concatenate(os_, axis=1).astype(BF16)
            k0, k1 = h0 * DH, (h0 + len(os_)) * DH
            res = []
            for n in range(NLB):
                if before_oproj is not None:
                    w = wo_s[k0:k1, n * 128:(n + 1) * 128]
                    wo_t[n, k0 // 2:k1 // 2, :] = pltpu.bitcast(w, U32)
                else:
                    w = pltpu.bitcast(wo_t[n, k0 // 2:k1 // 2, :], BF16)
                res.append(jnp.dot(oc, w, preferred_element_type=F32))
            return res

        heads = []
        qkv = proj(0)
        oa = None
        for g in range(NG):
            ps = probs(qkv, g)
            vs = qkv[2]
            if g + 1 < NG:
                qkv = proj(g + 1)
            else:
                if before_oproj is not None:
                    before_oproj()
                oa = oproj(heads[:H // 2], 0)
            heads += [jnp.dot(ps[j], pad(vs[j]), preferred_element_type=F32)
                      for j in range(HG)]
        assert early is None or not units
        ob = oproj(heads[H // 2:], H // 2)
        return jnp.concatenate([b + a for a, b in zip(oa, ob)], axis=1)

    def post2(s, toks=None):
        r3 = seg_row(s - 1 - LAG)
        for r in (0, 16):
            xc = _r(x2_s[(s + 4 - 1 - LAG) % 4, r:r + 16] + obuf[SEG + r:SEG + r + 16, :])
            out_s[pl.ds(r3 + r, 16), :] = gate(xc, r3 + r, toks).astype(BF16)

    def step(s, mode, vis, fill, chained=False, before_oproj=None, early=None):
        if mode == 0:
            h = hbuf[...]
        elif mode == 1:
            h = hbuf[0:48, :]
        else:
            h = jnp.concatenate([hbuf[0:16, :], hbuf[48:80, :]], axis=0)
        toks = []
        if mode != 1:
            post2(s, toks)
        if isinstance(s, int) and s == NSEG + LAG - 1:
            obuf[SEG:2 * SEG, :] = attention(h, vis, fill, chained, due=toks)
            return
        r1 = seg_row(s - 1)
        rn = seg_row(s + 1)
        h1n, h2n = [], []
        for r in (0, 16):
            xa = _r(x_s[pl.ds(r1 + r, 16), :].astype(F32) + obuf[r:r + 16, :])
            xb2 = _r(gate(xa, r1 + r))
            h2n.append(_ln(xb2, toks).astype(BF16))
            x2_s[(s + 4 - 1) % 4, r:r + 16] = xb2
        if mode != 2:
            for r in (0, 16):
                h1n.append(_ln(x_s[pl.ds(rn + r, 16), :].astype(F32), toks).astype(BF16))

        o = attention(h, vis, fill, chained, before_oproj, early, toks)

        mem2 = mem0 if mode == 1 else o[M:2 * M]
        hbuf[0:16, :] = jnp.concatenate([o[0:M], mem2], axis=0).astype(BF16)
        for n, v in enumerate(h1n):
            hbuf[16 + 16 * n:32 + 16 * n, :] = v
        for n, v in enumerate(h2n):
            hbuf[48 + 16 * n:64 + 16 * n, :] = v
        if mode == 0:
            obuf[...] = o[2 * M:]
        elif mode == 1:
            obuf[0:SEG, :] = o[2 * M:]
        else:
            obuf[SEG:2 * SEG, :] = o[2 * M:]

    with jax.named_scope("pro"):
        vis, fill = masks(1)
        step(0, 1, vis, fill, False, wo_copy.wait)
        step(1, 1, vis, fill, True)
    xb_copy.start()
    vis, fill = masks(0)
    with jax.named_scope("main_a"):
        loop(NA // UA, lambda i: [step(UA * i + u + LAG, 0, vis, fill, u > 0, early=UA * i + u)
                                  for u in range(UA)])
    xb_copy.wait()
    with jax.named_scope("conv_e"):
        loop(HB // UI, lambda j: [inv_stage(HB + UI * j + u) for u in range(UI)])
    with jax.named_scope("main_b"):
        loop((NSEG - LAG - NA) // UB, lambda i: [step(UB * i + u + LAG + NA, 0, vis, fill, u > 0)
                                                 for u in range(UB)])
    done = (NSEG - 1 - LAG) * SEG
    out_a = pltpu.make_async_copy(out_s.at[0:done, :], out_hbm.at[0:done, :], sem.at[SW + 8])
    out_a.start()
    with jax.named_scope("epi"):
        vis, fill = masks(2)
        step(NSEG, 2, vis, fill)
        step(NSEG + 1, 2, *masks(2, 2 * M), True)
    post2(NSEG + LAG)
    out_b = pltpu.make_async_copy(out_s.at[done:S, :], out_hbm.at[done:S, :], sem.at[SW + 9])
    out_b.start()
    out_a.wait()
    out_b.wait()


@jax.jit
def pallas_interleave_layers__memory_aug_recurrent_mem_tr__ssm_conv_h3__prompt_kernel(
    A_x, A_mem0, A_Wq, A_Wk, A_Wv, A_Wo, A_seg_len,
    B_q, B_k, B_v, B_shift_k, B_ssm_k, B_ssm_D,
):
    del A_seg_len, B_q
    assert A_x.shape == (1, S, D) and A_Wq.shape == (D, H, DH)
    hbm = pl.BlockSpec(memory_space=pl.ANY)
    out = pl.pallas_call(
        _kernel,
        out_shape=jax.ShapeDtypeStruct((S, D), BF16),
        in_specs=[hbm] * 11,
        out_specs=hbm,
        scratch_shapes=[
            pltpu.VMEM((S, D), BF16),
            pltpu.VMEM((S, D), BF16),
            pltpu.VMEM((S, D), BF16),
            pltpu.VMEM((HB, D, 2 * TB), BF16),
            pltpu.VMEM((3, D, H, DH), BF16),
            pltpu.VMEM(((H + 1) * WP, 128), U32),
            pltpu.VMEM(((2 * H + 1) * WP, 128), U32),
            pltpu.VMEM((H * DH, D), BF16),
            pltpu.VMEM((NLB, H * DH // 2, 128), U32),
            pltpu.VMEM((TB // 2, TB), U32),
            pltpu.VMEM((2, TB // 2, TB), U32),
            pltpu.VMEM((2, TB // 2, TB), U32),
            pltpu.VMEM((2, NLB, S // 2 + 8, 128), F32),
            pltpu.VMEM((NB, 2, NLB * TB, 128), F32),
            pltpu.VMEM((NB, 3, NLB * TB, 128), F32),
            pltpu.VMEM((NB + 1, 2, NLB * TB, 128), F32),
            pltpu.VMEM((NLB, S + 8, 128), F32),
            pltpu.VMEM((ROWS, D), BF16),
            pltpu.VMEM((2 * SEG, D), F32),
            pltpu.VMEM((4, SEG, D), F32),
            pltpu.VMEM((S, D), BF16),
            pltpu.VMEM((NA * SEG, D), BF16),
            pltpu.VMEM((NQH, NA * SEG, DH), BF16),
            pltpu.VMEM((M, D), BF16),
            pltpu.VMEM((KS, D), BF16),
            pltpu.VMEM((D,), BF16),
            pltpu.SemaphoreType.DMA((HB + HB // 2 + 10,)),
        ],
        compiler_params=pltpu.CompilerParams(vmem_limit_bytes=120 * 1024 * 1024),
    )(A_x.reshape(S, D), A_mem0.reshape(M, D), A_Wq, A_Wk, A_Wv,
      A_Wo.reshape(H * DH, D), B_k.reshape(S, D), B_v.reshape(S, D),
      B_shift_k.T, B_ssm_k, B_ssm_D)
    return out.reshape(1, S, D)
```

```python
import contextlib
import functools
import math

import jax
import jax.numpy as jnp
from jax import lax
import jax.experimental.pallas as pl
import jax.experimental.pallas.tpu as pltpu

F32 = jnp.float32
BF16 = jnp.bfloat16
U32 = jnp.uint32

S = 2048
D = 640
H = 32
DH = 128
M = 8
SEG = 32
NSEG = S // SEG
KS = 4
LAG = 2
ROWS = 2 * M + 2 * SEG
HG = 4
NG = H // HG
NLB = D // 128
TB = 128
NB = S // TB
HB = NB // 2
NPOS = NLB * TB // 8
NA = 20
PPS = 4
UCUT = tuple(range(a, a + 2) for a in range(0, 12, 2)) + (range(12, 16),)
NQH = 31
UA = 2
UB = 3
UI = 4
WP = 324


PROFILE = False


def _scope(name):
    return jax.named_scope(name) if PROFILE else contextlib.nullcontext()


def _ln(x, toks=None):
    m = jnp.mean(x, axis=-1, keepdims=True)
    c = x - m
    v = jnp.mean(c * c, axis=-1, keepdims=True)
    r = lax.rsqrt(v + 1e-5)
    if toks is not None:
        toks.append(jnp.minimum(r, 0.0))
    return c * r


def _r(x):
    return x.astype(BF16).astype(F32)


def _split(x):
    hi = pltpu.bitcast(pltpu.bitcast(x, U32) & jnp.uint32(0xFFFF0000), F32)
    return hi, x - hi


def _pk(x):
    return pltpu.bitcast(x.astype(BF16), U32)


def _upk(w):
    return pltpu.bitcast(w, BF16)


def _basis(r, t):
    b = r & 63
    f = jnp.where(b < 32, 2 * b, 2 * b - 63)
    n = ((2 * f + 1) * t - jnp.where(r >= 64, TB, 0)) & (4 * TB - 1)
    n = jnp.where(n >= 2 * TB, n - 4 * TB, n)
    return jnp.cos(n.astype(F32) * (2.0 * math.pi / (4 * TB)))


def _halves(x):
    w = pltpu.bitcast(x, U32)
    return (pltpu.bitcast(w << 16, F32),
            pltpu.bitcast(w & jnp.uint32(0xFFFF0000), F32))


def _kernel(x_hbm, mem0_hbm, wq_hbm, wk_hbm, wv_hbm, wo_hbm,
            k_hbm, v_hbm, shk_hbm, ssmk_hbm, ssmd_hbm,
            out_hbm,
            x_s, k_s, v_s, ssmk_s, wraw, wt_q, wt_kv, wo_s, wo_t,
            perm_s, fu_s, inv_s, kpad, u_s, kf_s, c_s, y_s,
            hbuf, obuf, x2_s, out_s, hl_s, qh_s, mem0_ref, shk_ref, ssmd_ref,
            sem):
    X0, XH = LAG * SEG, (LAG + NA) * SEG
    SW = HB + HB // 2

    def pair_rows(jp):
        r0 = jp * 2 * TB
        return pl.ds(r0 if isinstance(jp, int) else pl.multiple_of(r0, 2 * TB), 2 * TB)

    def ssmk_copy(jp):
        return pltpu.make_async_copy(ssmk_hbm.at[:, pair_rows(jp)], ssmk_s.at[jp], sem.at[jp])

    def kv_copies(rows, sm):
        return [pltpu.make_async_copy(k_hbm.at[rows, :], k_s.at[rows, :], sm),
                pltpu.make_async_copy(v_hbm.at[rows, :], v_s.at[rows, :], sm)]
    w_copies = [pltpu.make_async_copy(w, wraw.at[t], sem.at[SW + t])
                for t, w in enumerate((wq_hbm, wk_hbm, wv_hbm))]
    wo_copy = pltpu.make_async_copy(wo_hbm, wo_s, sem.at[SW + 3])
    late_copies = kv_copies(pl.ds(S // 2, S // 2), sem.at[SW + 4])
    small_copies = [pltpu.make_async_copy(src, dst, sem.at[SW + 5])
                    for src, dst in ((shk_hbm, shk_ref), (ssmd_hbm, ssmd_ref), (mem0_hbm, mem0_ref))]
    xa_copy = pltpu.make_async_copy(x_hbm.at[X0:XH, :], x_s.at[X0:XH, :], sem.at[SW + 6])
    late_copies += [pltpu.make_async_copy(x_hbm.at[a:b, :], x_s.at[a:b, :], sem.at[SW + 4])
                    for a, b in ((0, X0), (XH, XH + SEG))]
    xb_copy = pltpu.make_async_copy(x_hbm.at[XH + SEG:, :], x_s.at[XH + SEG:, :], sem.at[SW + 7])
    for c in (small_copies + [ssmk_copy(jp) for jp in range(HB)]
              + [c for jp in range(HB // 2) for c in kv_copies(pair_rows(jp), sem.at[HB + jp])]
              + [xa_copy, w_copies[0]] + late_copies + w_copies[1:] + [wo_copy]):
        c.start()

    hb = TB // 2
    ri = lax.broadcasted_iota(jnp.int32, (TB, TB), 0)
    ci = lax.broadcasted_iota(jnp.int32, (TB, TB), 1)
    perm_s[...] = _pk(jnp.where(ci == 2 * (ri & 63) + (ri >> 6), 1.0, 0.0))
    tab = _basis(ri, 2 * (ci & 63) + (ci >> 6))
    hi, lo = _split(tab)
    fu_s[0] = _pk(jnp.where(ci < hb, hi, pltpu.roll(lo, hb, 1)))
    fu_s[1] = _pk(jnp.where(ci < hb, pltpu.roll(hi, hb, 1), lo))
    gh, gl = _split(tab.T * (1.0 / TB))
    inv_s[0] = _pk(gh)
    inv_s[1] = _pk(gl)

    for c in small_copies:
        c.wait()
    shk_t = shk_ref[...].astype(F32)
    taps = [[shk_t[j:j + 1, g * 128:(g + 1) * 128] for g in range(NLB)] for j in range(KS)]
    dvec = ssmd_ref[...].astype(F32).reshape(1, D)
    for g in range(NLB):
        kpad[0, g, 0:8, :] = jnp.zeros((8, 128), F32)
        kpad[1, g, 0:8, :] = jnp.zeros((8, 128), F32)
    c_s[0] = jnp.zeros(c_s.shape[1:], F32)

    def spectrum(e, o):
        fe = jnp.dot(_upk(fu_s[0]), jnp.concatenate([e, e], axis=0).astype(BF16), preferred_element_type=F32)
        fo = jnp.dot(_upk(fu_s[1]), jnp.concatenate([o, o], axis=0).astype(BF16), preferred_element_type=F32)
        return ((fe[:hb] + fo[:hb], fe[hb:] + fo[hb:]), (fe[:hb] - fo[:hb], fo[hb:] - fe[hb:]))

    def freq_rows(g):
        return slice(g * TB, g * TB + hb), slice(g * TB + hb, (g + 1) * TB)

    def fwd_k(jq):
        for jp in (2 * jq, 2 * jq + 1):
            ssmk_copy(jp).wait()

        def transposed(n):
            blk = ssmk_s[2 * jq + n // 2, :, (n % 2) * TB:(n % 2 + 1) * TB]
            return lax.dot_general(_upk(perm_s[...]), blk, (((1,), (1,)), ((), ())),
                                   preferred_element_type=F32)
        nxt = transposed(0)
        for n in range(4):
            kt = nxt
            if n < 3:
                nxt = transposed(n + 1)
            j = 4 * jq + n
            for g in range(NLB):
                lb = slice(g * 128, (g + 1) * 128)
                for rows, (kr, ki) in zip(freq_rows(g), spectrum(kt[:hb, lb], kt[hb:, lb])):
                    if n == 0:
                        kr = kr + jnp.where(j == 0, dvec[:, lb], 0.0)
                    kf_s[j, 0, rows] = kr
                    kf_s[j, 1, rows] = ki - kr
                    kf_s[j, 2, rows] = kr + ki

    def fwd_u(jq, first):
        if first:
            for jp in (2 * jq, 2 * jq + 1):
                for c in kv_copies(pair_rows(jp), sem.at[HB + jp]):
                    c.wait()
        for j in [4 * jq + n for n in range(4)]:
            r0 = pl.multiple_of(j * TB, TB)
            q0 = pl.multiple_of(j * hb, hb) + 8
            for g in range(NLB):
                lb = slice(g * 128, (g + 1) * 128)
                ke, ko = _halves(k_s[pl.ds(r0, TB), lb])
                ve, vo = _halves(v_s[pl.ds(r0, TB), lb])
                kpad[0, g, pl.ds(q0, hb), :] = ke
                kpad[1, g, pl.ds(q0, hb), :] = ko
                ke1 = kpad[0, g, pl.ds(q0 - 1, hb), :]
                ko1 = kpad[1, g, pl.ds(q0 - 1, hb), :]
                ko2 = kpad[1, g, pl.ds(q0 - 2, hb), :]
                t0, t1, t2, t3 = (taps[t][g] for t in range(KS))
                e = (ke * t0 + ko1 * t1 + ke1 * t2 + ko2 * t3) * ve
                o = (ko * t0 + ke * t1 + ko1 * t2 + ke1 * t3) * vo
                for rows, (ur, ui) in zip(freq_rows(g), spectrum(e, o)):
                    u_s[j, 0, rows] = ur
                    u_s[j, 1, rows] = ui

    def mac_units(row, half):
        rs = pl.ds(row, 8)
        state = {}

        def unit(p, avals, final, tok=None):
            acc = state.setdefault(p, dict(state.get(0, {})))
            for a in avals:
                u = u_s[a, 0, rs] + u_s[a, 1, rs] if p == 0 else u_s[a, p - 1, rs]
                if tok is not None:
                    u = u + tok
                for i in range(max(a, half * HB), half * HB + HB):
                    t = u * kf_s[i - a, p, rs]
                    acc[i] = t if i not in acc else (acc[i] - t if p == 2 else acc[i] + t)
            if final and p:
                for i, v in acc.items():
                    c_s[i + 1, 2 - p, rs] = v

        subs = UCUT if half else (range(HB),)
        return [functools.partial(unit, p, avals, n == len(subs) - 1)
                for p in range(3) for n, avals in enumerate(subs)]

    def inv_stage(i):
        q = TB // 4
        for g in range(NLB):
            re, im = [], []
            for b in range(4):
                rows = slice(g * TB + b * q, g * TB + (b + 1) * q)
                cr, ci_ = c_s[i + 1, 0, rows], c_s[i + 1, 1, rows]
                pr, pi = c_s[i, 0, rows], c_s[i, 1, rows]
                re.append(cr + pi if b in (0, 3) else cr - pi)
                im.append(ci_ - pr if b in (0, 3) else ci_ + pr)
            pe = jnp.concatenate([re[0] + re[2], re[1] + re[3], im[0] - im[2], im[1] - im[3]], axis=0)
            po = jnp.concatenate([re[0] - re[2], re[1] - re[3], im[0] + im[2], im[1] + im[3]], axis=0)
            for par, pp in enumerate((pe, po)):
                ph, plo = _split(pp)
                gh_, gl_ = (inv_s[n, par * q:(par + 1) * q] for n in range(2))
                y_s[g, pl.ds(i * TB + par, hb, stride=2), :] = jnp.dot(
                    _upk(jnp.concatenate([gh_, gl_, gh_], axis=1)),
                    jnp.concatenate([ph, ph, plo], axis=0).astype(BF16),
                    preferred_element_type=F32)

    def relayout_rows(t, dst, base, dp, tok=None):
        a = pltpu.bitcast(wraw[t, 2 * dp], U32)
        b = pltpu.bitcast(wraw[t, 2 * dp + 1], U32)
        if tok is not None:
            a = a | tok
        dst[pl.ds(base + dp, 16, stride=WP), :] = (a & jnp.uint32(0xFFFF)) | (b << 16)
        dst[pl.ds(base + 16 * WP + dp, 16, stride=WP), :] = (
            (a >> 16) | (b & jnp.uint32(0xFFFF0000)))

    def wslab(t, h):
        s0 = (max(t - 1, 0) * H + (h % 2) * 16 + h // 2) * WP
        return pltpu.bitcast((wt_kv if t else wt_q)[s0:s0 + D // 2, :], BF16)

    def loop(n, fn):
        def body(j, _):
            fn(j)
            return 0
        lax.fori_loop(0, n, body, 0)

    def norm_rows(c):
        nr = NA * SEG // (HB // UI)
        r0 = pl.multiple_of(c * nr, 16)
        for r in range(0, nr, 16):
            hl_s[pl.ds(r0 + r, 16), :] = _ln(
                x_s[pl.ds(r0 + r + LAG * SEG, 16), :].astype(F32)).astype(BF16)

    def pre_queries(c, t=None):
        if t is not None:
            pltpu.make_async_copy(wraw.at[t], wraw.at[t], sem.at[SW + t]).wait()
            base = (t - 1) * (H * WP)
        per = -(-(D // 2) // (2 * NQH))
        dp = 0
        for sub in range(2):
            r0 = pl.multiple_of((2 * c + sub) * QR, QR)
            hl = hl_s[pl.ds(r0, QR), :]
            for hd in range(NQH):
                r = jnp.dot(hl, wslab(0, hd), preferred_element_type=F32)
                qh_s[hd, pl.ds(r0, QR), :] = r.astype(BF16)
                if t is not None:
                    tok = pltpu.bitcast(jnp.minimum(jnp.abs(r[0:16]), 0.0), U32)
                    for _ in range(per):
                        if dp < D // 2:
                            relayout_rows(t, wt_kv, base, dp, tok)
                            dp += 1

    nch = NA * SEG // TB
    QR = TB // 2
    with _scope("conv_k"):
        loop(HB // 2, fwd_k)
    with _scope("conv_u"):
        loop(HB // 4, lambda j: fwd_u(j, True))
    with _scope("conv_b"):
        loop(NPOS // 10, lambda j: [u() for n in range(10)
                                    for u in mac_units(pl.multiple_of(80 * j, 16) + 8 * n, 0)])
        xa_copy.wait()
        loop(HB // UI, lambda j: ([inv_stage(UI * j + u) for u in range(UI)], norm_rows(j)))
    with _scope("rel0"):
        w_copies[0].wait()
        loop(D // 64, lambda i: [relayout_rows(0, wt_q, 0, i * 32 + dd) for dd in range(32)])
    with _scope("preq"):
        loop(nch - 2, pre_queries)
    with _scope("conv_c"):
        for c in late_copies:
            c.wait()
        loop(HB // 4, lambda j: fwd_u(HB // 4 + j, False))
    with _scope("preq_rel"):
        loop(2, lambda i: pre_queries(i + nch - 2, i + 1))

    scale = DH ** -0.5

    def masks(mode, q0=0):
        rows = ROWS if mode == 0 else ROWS - SEG
        qi = lax.broadcasted_iota(jnp.int32, (rows - q0, 128), 0) + q0
        kj = lax.broadcasted_iota(jnp.int32, (rows - q0, 128), 1)

        def layer_of(i):
            xl = (i - 2 * M) // SEG if mode == 0 else mode - 1
            return jnp.where(i < 2 * M, i // M, xl)
        same = (layer_of(qi) == layer_of(kj)) & (kj < rows)
        vis = same & ((qi < 2 * M) | (qi >= kj))
        fill = jnp.where(same, -1e9 / scale, -jnp.inf).astype(F32)
        return vis, fill

    mem0 = mem0_ref[...].astype(F32)
    hbuf[0:16, :] = jnp.concatenate([mem0, mem0], axis=0).astype(BF16)
    hbuf[16:48, :] = _ln(x_s[0:SEG, :].astype(F32)).astype(BF16)
    obuf[...] = jnp.zeros((2 * SEG, D), F32)
    x2_s[...] = jnp.zeros(x2_s.shape, F32)

    def seg_row(seg):
        if isinstance(seg, int):
            return min(max(seg, 0), NSEG - 1) * SEG
        return pl.multiple_of(jnp.clip(seg, 0, NSEG - 1) * SEG, SEG)

    def gate(xa, r0, toks=None):
        y = jnp.concatenate([y_s[g, pl.ds(r0, xa.shape[0]), :] for g in range(NLB)], axis=1)
        return xa + _ln(xa, toks) * y

    def attention(h, vis, fill, chained, before_oproj=None, early=None, due=()):
        q0 = h.shape[0] - vis.shape[0]
        if early is not None:
            hrest = jnp.concatenate([h[:2 * M], h[2 * M + SEG:]], axis=0)
            qrow = pl.multiple_of(early * SEG, SEG)
            units = [u for n in range(PPS)
                     for u in mac_units(pl.multiple_of(early * (8 * PPS), 8 * PPS) + 8 * n, 1)]

        def proj(g):
            res = [[None] * HG for _ in range(3)]
            order = [(t, j) for j in range(HG) for t in range(2)] + [(2, j) for j in range(HG)]

            def operand(t, j):
                pre = early is not None and t == 0 and g * HG + j < NQH
                return pre, hrest if pre else (h if t else h[q0:])

            kc = D - 128
            nsplit = 4 if g == 0 and chained else 0
            part = [jnp.dot(operand(t, j)[1][:, :kc], wslab(t, j)[:kc], preferred_element_type=F32)
                    for t, j in order[:nsplit]]
            for n, (t, j) in enumerate(order):
                hd = g * HG + j
                pre, lhs = operand(t, j)
                if n < nsplit:
                    r = jnp.dot(lhs[:, kc:], wslab(t, hd)[kc:], preferred_element_type=F32) + part[n]
                else:
                    r = jnp.dot(lhs, wslab(t, hd), preferred_element_type=F32)
                if early is not None and units:
                    units.pop(0)(jnp.minimum(jnp.abs(r[0:8]), 0.0))
                if t == 0:
                    r = r.astype(BF16)
                if pre:
                    r = jnp.concatenate([r[:2 * M], qh_s[hd, pl.ds(qrow, SEG), :], r[2 * M:]], axis=0)
                res[t][j] = r
            return res

        def pad(kv):
            return jnp.concatenate([kv, jnp.zeros((128 - kv.shape[0], DH), F32)], axis=0).astype(BF16)

        def probs(qkv, g):
            scs = [lax.dot_general(qkv[0][j], pad(qkv[1][j]), (((1,), (1,)), ((), ())),
                                   preferred_element_type=F32) for j in range(HG)]
            ps = []
            for sc in scs:
                sc = jnp.where(vis, sc, fill)
                e = jnp.exp2((sc - jnp.max(sc, axis=-1, keepdims=True)) * (scale * math.log2(math.e)))
                den = jnp.sum(e, axis=-1, keepdims=True)
                if not ps and g >= NG - len(due):
                    e = jnp.concatenate([e[:16] + due[g - NG + len(due)], e[16:]], axis=0)
                r = pl.reciprocal(den, approx=True)
                r = r * (2.0 - den * r)
                ps.append((e * r).astype(BF16))
            return ps

        def oproj(os_, h0):
            oc = jnp.concatenate(os_, axis=1).astype(BF16)
            k0, k1 = h0 * DH, (h0 + len(os_)) * DH
            res = []
            for n in range(NLB):
                if before_oproj is not None:
                    w = wo_s[k0:k1, n * 128:(n + 1) * 128]
                    wo_t[n, k0 // 2:k1 // 2, :] = pltpu.bitcast(w, U32)
                else:
                    w = pltpu.bitcast(wo_t[n, k0 // 2:k1 // 2, :], BF16)
                res.append(jnp.dot(oc, w, preferred_element_type=F32))
            return res

        heads = []
        qkv = proj(0)
        oa = None
        for g in range(NG):
            ps = probs(qkv, g)
            vs = qkv[2]
            if g + 1 < NG:
                qkv = proj(g + 1)
            else:
                if before_oproj is not None:
                    before_oproj()
                oa = oproj(heads[:H // 2], 0)
            heads += [jnp.dot(ps[j], pad(vs[j]), preferred_element_type=F32)
                      for j in range(HG)]
        assert early is None or not units
        ob = oproj(heads[H // 2:], H // 2)
        return jnp.concatenate([b + a for a, b in zip(oa, ob)], axis=1)

    def post2(s, toks=None):
        r3 = seg_row(s - 1 - LAG)
        for r in (0, 16):
            xc = _r(x2_s[(s + 4 - 1 - LAG) % 4, r:r + 16] + obuf[SEG + r:SEG + r + 16, :])
            out_s[pl.ds(r3 + r, 16), :] = gate(xc, r3 + r, toks).astype(BF16)

    def step(s, mode, vis, fill, chained=False, before_oproj=None, early=None):
        if mode == 0:
            h = hbuf[...]
        elif mode == 1:
            h = hbuf[0:48, :]
        else:
            live = lax.broadcasted_iota(jnp.int32, (2 * M, D), 0) >= M
            mem = jnp.where(live, hbuf[0:16, :].astype(F32), 0.0).astype(BF16)
            h = jnp.concatenate([mem, hbuf[48:80, :]], axis=0)
        toks = []
        if mode != 1:
            post2(s, toks)
        if isinstance(s, int) and s == NSEG + LAG - 1:
            obuf[SEG:2 * SEG, :] = attention(h, vis, fill, chained, due=toks)
            return
        r1 = seg_row(s - 1)
        rn = seg_row(s + 1)
        h1n, h2n = [], []
        for r in (0, 16):
            xa = _r(x_s[pl.ds(r1 + r, 16), :].astype(F32) + obuf[r:r + 16, :])
            xb2 = _r(gate(xa, r1 + r))
            h2n.append(_ln(xb2, toks).astype(BF16))
            x2_s[(s + 4 - 1) % 4, r:r + 16] = xb2
        if mode != 2:
            for r in (0, 16):
                h1n.append(_ln(x_s[pl.ds(rn + r, 16), :].astype(F32), toks).astype(BF16))

        o = attention(h, vis, fill, chained, before_oproj, early, toks)

        mem2 = mem0 if mode == 1 else o[M:2 * M]
        hbuf[0:16, :] = jnp.concatenate([o[0:M], mem2], axis=0).astype(BF16)
        for n, v in enumerate(h1n):
            hbuf[16 + 16 * n:32 + 16 * n, :] = v
        for n, v in enumerate(h2n):
            hbuf[48 + 16 * n:64 + 16 * n, :] = v
        if mode == 0:
            obuf[...] = o[2 * M:]
        elif mode == 1:
            obuf[0:SEG, :] = o[2 * M:]
        else:
            obuf[SEG:2 * SEG, :] = o[2 * M:]

    with _scope("pro"):
        vis, fill = masks(1)
        step(0, 1, vis, fill, False, wo_copy.wait)
        step(1, 1, vis, fill, True)
    xb_copy.start()
    vis, fill = masks(0)
    with _scope("main_a"):
        loop(NA // UA, lambda i: [step(UA * i + u + LAG, 0, vis, fill, u > 0, early=UA * i + u)
                                  for u in range(UA)])
    xb_copy.wait()
    with _scope("conv_e"):
        loop(HB // UI, lambda j: [inv_stage(HB + UI * j + u) for u in range(UI)])
    with _scope("main_b"):
        loop((NSEG - LAG - NA) // UB, lambda i: [step(UB * i + u + LAG + NA, 0, vis, fill, u > 0)
                                                 for u in range(UB)])
    done = (NSEG - 1 - LAG) * SEG
    out_a = pltpu.make_async_copy(out_s.at[0:done, :], out_hbm.at[0:done, :], sem.at[SW + 8])
    out_a.start()
    with _scope("epi"):
        vis, fill = masks(2)
        step(NSEG, 2, vis, fill)
        step(NSEG + 1, 2, *masks(2, 2 * M), True)
    post2(NSEG + LAG)
    out_b = pltpu.make_async_copy(out_s.at[done:S, :], out_hbm.at[done:S, :], sem.at[SW + 9])
    out_b.start()
    out_a.wait()
    out_b.wait()


@jax.jit
def pallas_interleave_layers__memory_aug_recurrent_mem_tr__ssm_conv_h3__prompt_kernel(
    A_x, A_mem0, A_Wq, A_Wk, A_Wv, A_Wo, A_seg_len,
    B_q, B_k, B_v, B_shift_k, B_ssm_k, B_ssm_D,
):
    del A_seg_len, B_q
    assert A_x.shape == (1, S, D) and A_Wq.shape == (D, H, DH)
    hbm = pl.BlockSpec(memory_space=pl.ANY)
    out = pl.pallas_call(
        _kernel,
        out_shape=jax.ShapeDtypeStruct((S, D), BF16),
        in_specs=[hbm] * 11,
        out_specs=hbm,
        scratch_shapes=[
            pltpu.VMEM((S, D), BF16),
            pltpu.VMEM((S, D), BF16),
            pltpu.VMEM((S, D), BF16),
            pltpu.VMEM((HB, D, 2 * TB), BF16),
            pltpu.VMEM((3, D, H, DH), BF16),
            pltpu.VMEM(((H + 1) * WP, 128), U32),
            pltpu.VMEM(((2 * H + 1) * WP, 128), U32),
            pltpu.VMEM((H * DH, D), BF16),
            pltpu.VMEM((NLB, H * DH // 2, 128), U32),
            pltpu.VMEM((TB // 2, TB), U32),
            pltpu.VMEM((2, TB // 2, TB), U32),
            pltpu.VMEM((2, TB // 2, TB), U32),
            pltpu.VMEM((2, NLB, S // 2 + 8, 128), F32),
            pltpu.VMEM((NB, 2, NLB * TB, 128), F32),
            pltpu.VMEM((NB, 3, NLB * TB, 128), F32),
            pltpu.VMEM((NB + 1, 2, NLB * TB, 128), F32),
            pltpu.VMEM((NLB, S + 8, 128), F32),
            pltpu.VMEM((ROWS, D), BF16),
            pltpu.VMEM((2 * SEG, D), F32),
            pltpu.VMEM((4, SEG, D), F32),
            pltpu.VMEM((S, D), BF16),
            pltpu.VMEM((NA * SEG, D), BF16),
            pltpu.VMEM((NQH, NA * SEG, DH), BF16),
            pltpu.VMEM((M, D), BF16),
            pltpu.VMEM((KS, D), BF16),
            pltpu.VMEM((D,), BF16),
            pltpu.SemaphoreType.DMA((HB + HB // 2 + 10,)),
        ],
        compiler_params=pltpu.CompilerParams(vmem_limit_bytes=120 * 1024 * 1024),
    )(A_x.reshape(S, D), A_mem0.reshape(M, D), A_Wq, A_Wk, A_Wv,
      A_Wo.reshape(H * DH, D), B_k.reshape(S, D), B_v.reshape(S, D),
      B_shift_k.T, B_ssm_k, B_ssm_D)
    return out.reshape(1, S, D)
```

```python
import contextlib
import functools
import math

import jax
import jax.numpy as jnp
from jax import lax
import jax.experimental.pallas as pl
import jax.experimental.pallas.tpu as pltpu

F32 = jnp.float32
BF16 = jnp.bfloat16
U32 = jnp.uint32

S = 2048
D = 640
H = 32
DH = 128
M = 8
SEG = 32
NSEG = S // SEG
KS = 4
LAG = 2
ROWS = 2 * M + 2 * SEG
HG = 4
NG = H // HG
NLB = D // 128
TB = 128
NB = S // TB
HB = NB // 2
NPOS = NLB * TB // 8
NA = 20
PPS = 4
UCUT = tuple(range(a, a + 2) for a in range(0, 12, 2)) + (range(12, 16),)
NQH = 32
UA = 2
UB = 3
UI = 4
WP = 324


PROFILE = False


def _scope(name):
    return jax.named_scope(name) if PROFILE else contextlib.nullcontext()


def _ln(x, toks=None):
    m = jnp.mean(x, axis=-1, keepdims=True)
    c = x - m
    v = jnp.mean(c * c, axis=-1, keepdims=True)
    r = lax.rsqrt(v + 1e-5)
    if toks is not None:
        toks.append(jnp.minimum(r, 0.0))
    return c * r


def _r(x):
    return x.astype(BF16).astype(F32)


def _split(x):
    hi = pltpu.bitcast(pltpu.bitcast(x, U32) & jnp.uint32(0xFFFF0000), F32)
    return hi, x - hi


def _pk(x):
    return pltpu.bitcast(x.astype(BF16), U32)


def _upk(w):
    return pltpu.bitcast(w, BF16)


def _basis(r, t):
    b = r & 63
    f = jnp.where(b < 32, 2 * b, 2 * b - 63)
    n = ((2 * f + 1) * t - jnp.where(r >= 64, TB, 0)) & (4 * TB - 1)
    n = jnp.where(n >= 2 * TB, n - 4 * TB, n)
    return jnp.cos(n.astype(F32) * (2.0 * math.pi / (4 * TB)))


def _halves(x):
    w = pltpu.bitcast(x, U32)
    return (pltpu.bitcast(w << 16, F32),
            pltpu.bitcast(w & jnp.uint32(0xFFFF0000), F32))


def _kernel(x_hbm, mem0_hbm, wq_hbm, wk_hbm, wv_hbm, wo_hbm,
            k_hbm, v_hbm, shk_hbm, ssmk_hbm, ssmd_hbm,
            out_hbm,
            x_s, k_s, v_s, ssmk_s, wraw, wt_q, wt_kv, wo_s, wo_t,
            perm_s, fu_s, inv_s, kpad, u_s, kf_s, c_s, y_s,
            hbuf, obuf, x2_s, out_s, hl_s, qh_s, mem0_ref, shk_ref, ssmd_ref,
            sem):
    X0, XH = LAG * SEG, (LAG + NA) * SEG
    SW = HB + HB // 2

    def pair_rows(jp):
        r0 = jp * 2 * TB
        return pl.ds(r0 if isinstance(jp, int) else pl.multiple_of(r0, 2 * TB), 2 * TB)

    def ssmk_copy(jp):
        return pltpu.make_async_copy(ssmk_hbm.at[:, pair_rows(jp)], ssmk_s.at[jp], sem.at[jp])

    def kv_copies(rows, sm):
        return [pltpu.make_async_copy(k_hbm.at[rows, :], k_s.at[rows, :], sm),
                pltpu.make_async_copy(v_hbm.at[rows, :], v_s.at[rows, :], sm)]
    DQ = 192
    wq_early = [pltpu.make_async_copy(wq_hbm.at[n * DQ:(n + 1) * DQ], wraw.at[0, n * DQ:(n + 1) * DQ],
                                      sem.at[SW + 10 + n]) for n in range(2)]
    w_copies = [pltpu.make_async_copy(wq_hbm.at[2 * DQ:], wraw.at[0, 2 * DQ:], sem.at[SW])]
    w_copies += [pltpu.make_async_copy(w, wraw.at[t], sem.at[SW + t])
                 for t, w in ((1, wk_hbm), (2, wv_hbm))]
    wo_copy = pltpu.make_async_copy(wo_hbm, wo_s, sem.at[SW + 3])
    late_copies = kv_copies(pl.ds(S // 2, S // 2), sem.at[SW + 4])
    small_copies = [pltpu.make_async_copy(src, dst, sem.at[SW + 5])
                    for src, dst in ((shk_hbm, shk_ref), (ssmd_hbm, ssmd_ref), (mem0_hbm, mem0_ref))]
    xa_copy = pltpu.make_async_copy(x_hbm.at[X0:XH, :], x_s.at[X0:XH, :], sem.at[SW + 6])
    late_copies += [pltpu.make_async_copy(x_hbm.at[a:b, :], x_s.at[a:b, :], sem.at[SW + 4])
                    for a, b in ((0, X0), (XH, XH + SEG))]
    xb_copy = pltpu.make_async_copy(x_hbm.at[XH + SEG:, :], x_s.at[XH + SEG:, :], sem.at[SW + 7])
    for c in (small_copies + [ssmk_copy(jp) for jp in range(HB)]
              + [c for jp in range(HB // 2) for c in kv_copies(pair_rows(jp), sem.at[HB + jp])]
              + [xa_copy] + wq_early + [w_copies[0]] + late_copies + w_copies[1:] + [wo_copy]):
        c.start()

    hb = TB // 2
    ri = lax.broadcasted_iota(jnp.int32, (TB, TB), 0)
    ci = lax.broadcasted_iota(jnp.int32, (TB, TB), 1)
    perm_s[...] = _pk(jnp.where(ci == 2 * (ri & 63) + (ri >> 6), 1.0, 0.0))
    tab = _basis(ri, 2 * (ci & 63) + (ci >> 6))
    hi, lo = _split(tab)
    fu_s[0] = _pk(jnp.where(ci < hb, hi, pltpu.roll(lo, hb, 1)))
    fu_s[1] = _pk(jnp.where(ci < hb, pltpu.roll(hi, hb, 1), lo))
    gh, gl = _split(tab.T * (1.0 / TB))
    inv_s[0] = _pk(gh)
    inv_s[1] = _pk(gl)

    for c in small_copies:
        c.wait()
    shk_t = shk_ref[...].astype(F32)
    taps = [[shk_t[j:j + 1, g * 128:(g + 1) * 128] for g in range(NLB)] for j in range(KS)]
    dvec = ssmd_ref[...].astype(F32).reshape(1, D)
    for g in range(NLB):
        kpad[0, g, 0:8, :] = jnp.zeros((8, 128), F32)
        kpad[1, g, 0:8, :] = jnp.zeros((8, 128), F32)
    c_s[0] = jnp.zeros(c_s.shape[1:], F32)

    def spectrum(e, o):
        fe = jnp.dot(_upk(fu_s[0]), jnp.concatenate([e, e], axis=0).astype(BF16), preferred_element_type=F32)
        fo = jnp.dot(_upk(fu_s[1]), jnp.concatenate([o, o], axis=0).astype(BF16), preferred_element_type=F32)
        return ((fe[:hb] + fo[:hb], fe[hb:] + fo[hb:]), (fe[:hb] - fo[:hb], fo[hb:] - fe[hb:]))

    def freq_rows(g):
        return slice(g * TB, g * TB + hb), slice(g * TB + hb, (g + 1) * TB)

    def fwd_k(jq):
        for jp in (2 * jq, 2 * jq + 1):
            ssmk_copy(jp).wait()

        def transposed(n):
            blk = ssmk_s[2 * jq + n // 2, :, (n % 2) * TB:(n % 2 + 1) * TB]
            return lax.dot_general(_upk(perm_s[...]), blk, (((1,), (1,)), ((), ())),
                                   preferred_element_type=F32)
        nxt = transposed(0)
        for n in range(4):
            kt = nxt
            if n < 3:
                nxt = transposed(n + 1)
            j = 4 * jq + n
            for g in range(NLB):
                lb = slice(g * 128, (g + 1) * 128)
                for rows, (kr, ki) in zip(freq_rows(g), spectrum(kt[:hb, lb], kt[hb:, lb])):
                    if n == 0:
                        kr = kr + jnp.where(j == 0, dvec[:, lb], 0.0)
                    kf_s[j, 0, rows] = kr
                    kf_s[j, 1, rows] = ki - kr
                    kf_s[j, 2, rows] = kr + ki

    def fwd_u(jq, first):
        if first:
            for jp in (2 * jq, 2 * jq + 1):
                for c in kv_copies(pair_rows(jp), sem.at[HB + jp]):
                    c.wait()
        for j in [4 * jq + n for n in range(4)]:
            r0 = pl.multiple_of(j * TB, TB)
            q0 = pl.multiple_of(j * hb, hb) + 8
            for g in range(NLB):
                lb = slice(g * 128, (g + 1) * 128)
                ke, ko = _halves(k_s[pl.ds(r0, TB), lb])
                ve, vo = _halves(v_s[pl.ds(r0, TB), lb])
                kpad[0, g, pl.ds(q0, hb), :] = ke
                kpad[1, g, pl.ds(q0, hb), :] = ko
                ke1 = kpad[0, g, pl.ds(q0 - 1, hb), :]
                ko1 = kpad[1, g, pl.ds(q0 - 1, hb), :]
                ko2 = kpad[1, g, pl.ds(q0 - 2, hb), :]
                t0, t1, t2, t3 = (taps[t][g] for t in range(KS))
                e = (ke * t0 + ko1 * t1 + ke1 * t2 + ko2 * t3) * ve
                o = (ko * t0 + ke * t1 + ko1 * t2 + ke1 * t3) * vo
                for rows, (ur, ui) in zip(freq_rows(g), spectrum(e, o)):
                    u_s[j, 0, rows] = ur
                    u_s[j, 1, rows] = ui

    def mac_units(row, half):
        rs = pl.ds(row, 8)
        state = {}

        def unit(p, avals, final, tok=None):
            acc = state.setdefault(p, dict(state.get(0, {})))
            for a in avals:
                u = u_s[a, 0, rs] + u_s[a, 1, rs] if p == 0 else u_s[a, p - 1, rs]
                if tok is not None:
                    u = u + tok
                for i in range(max(a, half * HB), half * HB + HB):
                    t = u * kf_s[i - a, p, rs]
                    acc[i] = t if i not in acc else (acc[i] - t if p == 2 else acc[i] + t)
            if final and p:
                for i, v in acc.items():
                    c_s[i + 1, 2 - p, rs] = v

        subs = UCUT if half else (range(HB),)
        return [functools.partial(unit, p, avals, n == len(subs) - 1)
                for p in range(3) for n, avals in enumerate(subs)]

    def inv_stage(i, units=None):
        q = TB // 4
        for g in range(NLB):
            re, im = [], []
            for b in range(4):
                rows = slice(g * TB + b * q, g * TB + (b + 1) * q)
                cr, ci_ = c_s[i + 1, 0, rows], c_s[i + 1, 1, rows]
                pr, pi = c_s[i, 0, rows], c_s[i, 1, rows]
                re.append(cr + pi if b in (0, 3) else cr - pi)
                im.append(ci_ - pr if b in (0, 3) else ci_ + pr)
            pe = jnp.concatenate([re[0] + re[2], re[1] + re[3], im[0] - im[2], im[1] - im[3]], axis=0)
            po = jnp.concatenate([re[0] - re[2], re[1] - re[3], im[0] + im[2], im[1] + im[3]], axis=0)
            for par, pp in enumerate((pe, po)):
                ph, plo = _split(pp)
                gh_, gl_ = (inv_s[n, par * q:(par + 1) * q] for n in range(2))
                y = jnp.dot(_upk(jnp.concatenate([gh_, gl_, gh_], axis=1)),
                            jnp.concatenate([ph, ph, plo], axis=0).astype(BF16),
                            preferred_element_type=F32)
                y_s[g, pl.ds(i * TB + par, hb, stride=2), :] = y
                if units:
                    tok = pltpu.bitcast(jnp.minimum(jnp.abs(y[0:16]), 0.0), U32)
                    for _ in range(3):
                        if units:
                            units.pop(0)(tok)

    def relayout_rows(t, dst, base, dp, tok=None):
        a = pltpu.bitcast(wraw[t, 2 * dp], U32)
        b = pltpu.bitcast(wraw[t, 2 * dp + 1], U32)
        if tok is not None:
            a = a | tok
        dst[pl.ds(base + dp, 16, stride=WP), :] = (a & jnp.uint32(0xFFFF)) | (b << 16)
        dst[pl.ds(base + 16 * WP + dp, 16, stride=WP), :] = (
            (a >> 16) | (b & jnp.uint32(0xFFFF0000)))

    def wslab(t, h):
        s0 = (max(t - 1, 0) * H + (h % 2) * 16 + h // 2) * WP
        return pltpu.bitcast((wt_kv if t else wt_q)[s0:s0 + D // 2, :], BF16)

    def loop(n, fn):
        def body(j, _):
            fn(j)
            return 0
        lax.fori_loop(0, n, body, 0)

    def norm_rows(c):
        nr = NA * SEG // (HB // UI)
        r0 = pl.multiple_of(c * nr, 16)
        for r in range(0, nr, 16):
            hl_s[pl.ds(r0 + r, 16), :] = _ln(
                x_s[pl.ds(r0 + r + LAG * SEG, 16), :].astype(F32)).astype(BF16)

    def pre_queries(c, t=None):
        if t is not None:
            pltpu.make_async_copy(wraw.at[t], wraw.at[t], sem.at[SW + t]).wait()
            base = (t - 1) * (H * WP)
        per = -(-(D // 2) // (2 * NQH))
        dp = 0
        for sub in range(2):
            r0 = pl.multiple_of((2 * c + sub) * QR, QR)
            hl = hl_s[pl.ds(r0, QR), :]
            for hd in range(NQH):
                r = jnp.dot(hl, wslab(0, hd), preferred_element_type=F32)
                qh_s[hd, pl.ds(r0, QR), :] = r.astype(BF16)
                if t is not None:
                    tok = pltpu.bitcast(jnp.minimum(jnp.abs(r[0:16]), 0.0), U32)
                    for _ in range(per):
                        if dp < D // 2:
                            relayout_rows(t, wt_kv, base, dp, tok)
                            dp += 1

    nch = NA * SEG // TB
    QR = TB // 2
    with _scope("conv_k"):
        loop(HB // 2, fwd_k)
    with _scope("conv_u"):
        loop(HB // 4, lambda j: fwd_u(j, True))
    with _scope("conv_b"):
        loop(NPOS // 10, lambda j: [u() for n in range(10)
                                    for u in mac_units(pl.multiple_of(80 * j, 16) + 8 * n, 0)])
        xa_copy.wait()

        def inv_first(j):
            pltpu.make_async_copy(wraw.at[0, 0:DQ], wraw.at[0, 0:DQ], sem.at[SW + 10 + j]).wait()
            units = [functools.partial(relayout_rows, 0, wt_q, 0, j * (DQ // 2) + dd)
                     for dd in range(DQ // 2)]
            for u in range(UI):
                inv_stage(UI * j + u, units)
            assert not units
            norm_rows(j)
        loop(HB // UI, inv_first)
    with _scope("rel0"):
        w_copies[0].wait()
        loop((D - 2 * DQ) // 64,
             lambda i: [relayout_rows(0, wt_q, 0, DQ + i * 32 + dd) for dd in range(32)])
    with _scope("preq"):
        loop(nch - 2, pre_queries)
    with _scope("conv_c"):
        for c in late_copies:
            c.wait()
        loop(HB // 4, lambda j: fwd_u(HB // 4 + j, False))
    with _scope("preq_rel"):
        loop(2, lambda i: pre_queries(i + nch - 2, i + 1))

    scale = DH ** -0.5

    def masks(mode, q0=0):
        rows = ROWS if mode == 0 else ROWS - SEG
        qi = lax.broadcasted_iota(jnp.int32, (rows - q0, 128), 0) + q0
        kj = lax.broadcasted_iota(jnp.int32, (rows - q0, 128), 1)

        def layer_of(i):
            xl = (i - 2 * M) // SEG if mode == 0 else mode - 1
            return jnp.where(i < 2 * M, i // M, xl)
        same = (layer_of(qi) == layer_of(kj)) & (kj < rows)
        vis = same & ((qi < 2 * M) | (qi >= kj))
        fill = jnp.where(same, -1e9 / scale, -jnp.inf).astype(F32)
        return vis, fill

    mem0 = mem0_ref[...].astype(F32)
    hbuf[0:16, :] = jnp.concatenate([mem0, mem0], axis=0).astype(BF16)
    hbuf[16:48, :] = _ln(x_s[0:SEG, :].astype(F32)).astype(BF16)
    obuf[...] = jnp.zeros((2 * SEG, D), F32)
    x2_s[...] = jnp.zeros(x2_s.shape, F32)

    def seg_row(seg):
        if isinstance(seg, int):
            return min(max(seg, 0), NSEG - 1) * SEG
        return pl.multiple_of(jnp.clip(seg, 0, NSEG - 1) * SEG, SEG)

    def gate(xa, r0, toks=None):
        y = jnp.concatenate([y_s[g, pl.ds(r0, xa.shape[0]), :] for g in range(NLB)], axis=1)
        return xa + _ln(xa, toks) * y

    def attention(h, vis, fill, chained, before_oproj=None, early=None, due=()):
        q0 = h.shape[0] - vis.shape[0]
        if early is not None:
            hrest = jnp.concatenate([h[:2 * M], h[2 * M + SEG:]], axis=0)
            qrow = pl.multiple_of(early * SEG, SEG)
            units = [u for n in range(PPS)
                     for u in mac_units(pl.multiple_of(early * (8 * PPS), 8 * PPS) + 8 * n, 1)]

        def proj(g):
            res = [[None] * HG for _ in range(3)]
            order = [(t, j) for j in range(HG) for t in range(2)] + [(2, j) for j in range(HG)]

            def operand(t, j):
                pre = early is not None and t == 0 and g * HG + j < NQH
                return pre, hrest if pre else (h if t else h[q0:])

            kc = D - 128
            nsplit = 4 if g == 0 and chained else 0
            part = [jnp.dot(operand(t, j)[1][:, :kc], wslab(t, j)[:kc], preferred_element_type=F32)
                    for t, j in order[:nsplit]]
            for n, (t, j) in enumerate(order):
                hd = g * HG + j
                pre, lhs = operand(t, j)
                if n < nsplit:
                    r = jnp.dot(lhs[:, kc:], wslab(t, hd)[kc:], preferred_element_type=F32) + part[n]
                else:
                    r = jnp.dot(lhs, wslab(t, hd), preferred_element_type=F32)
                if early is not None and units:
                    units.pop(0)(jnp.minimum(jnp.abs(r[0:8]), 0.0))
                if t == 0:
                    r = r.astype(BF16)
                if pre:
                    r = jnp.concatenate([r[:2 * M], qh_s[hd, pl.ds(qrow, SEG), :], r[2 * M:]], axis=0)
                res[t][j] = r
            return res

        def pad(kv):
            return jnp.concatenate([kv, jnp.zeros((128 - kv.shape[0], DH), F32)], axis=0).astype(BF16)

        def probs(qkv, g):
            scs = [lax.dot_general(qkv[0][j], pad(qkv[1][j]), (((1,), (1,)), ((), ())),
                                   preferred_element_type=F32) for j in range(HG)]
            ps = []
            for sc in scs:
                sc = jnp.where(vis, sc, fill)
                e = jnp.exp2((sc - jnp.max(sc, axis=-1, keepdims=True)) * (scale * math.log2(math.e)))
                den = jnp.sum(e, axis=-1, keepdims=True)
                if not ps and g >= NG - len(due):
                    e = jnp.concatenate([e[:16] + due[g - NG + len(due)], e[16:]], axis=0)
                r = pl.reciprocal(den, approx=True)
                r = r * (2.0 - den * r)
                ps.append((e * r).astype(BF16))
            return ps

        def oproj(os_, h0):
            oc = jnp.concatenate(os_, axis=1).astype(BF16)
            k0, k1 = h0 * DH, (h0 + len(os_)) * DH
            res = []
            for n in range(NLB):
                if before_oproj is not None:
                    w = wo_s[k0:k1, n * 128:(n + 1) * 128]
                    wo_t[n, k0 // 2:k1 // 2, :] = pltpu.bitcast(w, U32)
                else:
                    w = pltpu.bitcast(wo_t[n, k0 // 2:k1 // 2, :], BF16)
                res.append(jnp.dot(oc, w, preferred_element_type=F32))
            return res

        heads = []
        qkv = proj(0)
        oa = None
        for g in range(NG):
            ps = probs(qkv, g)
            vs = qkv[2]
            if g + 1 < NG:
                qkv = proj(g + 1)
            else:
                if before_oproj is not None:
                    before_oproj()
                oa = oproj(heads[:H // 2], 0)
            heads += [jnp.dot(ps[j], pad(vs[j]), preferred_element_type=F32)
                      for j in range(HG)]
        assert early is None or not units
        ob = oproj(heads[H // 2:], H // 2)
        return jnp.concatenate([b + a for a, b in zip(oa, ob)], axis=1)

    def post2(s, toks=None):
        r3 = seg_row(s - 1 - LAG)
        for r in (0, 16):
            xc = _r(x2_s[(s + 4 - 1 - LAG) % 4, r:r + 16] + obuf[SEG + r:SEG + r + 16, :])
            out_s[pl.ds(r3 + r, 16), :] = gate(xc, r3 + r, toks).astype(BF16)

    def step(s, mode, vis, fill, chained=False, before_oproj=None, early=None):
        if mode == 0:
            h = hbuf[...]
        elif mode == 1:
            h = hbuf[0:48, :]
        else:
            live = lax.broadcasted_iota(jnp.int32, (2 * M, D), 0) >= M
            mem = jnp.where(live, hbuf[0:16, :].astype(F32), 0.0).astype(BF16)
            h = jnp.concatenate([mem, hbuf[48:80, :]], axis=0)
        toks = []
        if mode != 1:
            post2(s, toks)
        if isinstance(s, int) and s == NSEG + LAG - 1:
            obuf[SEG:2 * SEG, :] = attention(h, vis, fill, chained, due=toks)
            return
        r1 = seg_row(s - 1)
        rn = seg_row(s + 1)
        h1n, h2n = [], []
        for r in (0, 16):
            xa = _r(x_s[pl.ds(r1 + r, 16), :].astype(F32) + obuf[r:r + 16, :])
            xb2 = _r(gate(xa, r1 + r))
            h2n.append(_ln(xb2, toks).astype(BF16))
            x2_s[(s + 4 - 1) % 4, r:r + 16] = xb2
        if mode != 2:
            for r in (0, 16):
                h1n.append(_ln(x_s[pl.ds(rn + r, 16), :].astype(F32), toks).astype(BF16))

        o = attention(h, vis, fill, chained, before_oproj, early, toks)

        mem2 = mem0 if mode == 1 else o[M:2 * M]
        hbuf[0:16, :] = jnp.concatenate([o[0:M], mem2], axis=0).astype(BF16)
        for n, v in enumerate(h1n):
            hbuf[16 + 16 * n:32 + 16 * n, :] = v
        for n, v in enumerate(h2n):
            hbuf[48 + 16 * n:64 + 16 * n, :] = v
        if mode == 0:
            obuf[...] = o[2 * M:]
        elif mode == 1:
            obuf[0:SEG, :] = o[2 * M:]
        else:
            obuf[SEG:2 * SEG, :] = o[2 * M:]

    with _scope("pro"):
        vis, fill = masks(1)
        step(0, 1, vis, fill, False, wo_copy.wait)
        step(1, 1, vis, fill, True)
    xb_copy.start()
    vis, fill = masks(0)
    with _scope("main_a"):
        loop(NA // UA, lambda i: [step(UA * i + u + LAG, 0, vis, fill, u > 0, early=UA * i + u)
                                  for u in range(UA)])
    xb_copy.wait()
    with _scope("conv_e"):
        loop(HB // UI, lambda j: [inv_stage(HB + UI * j + u) for u in range(UI)])
    with _scope("main_b"):
        loop((NSEG - LAG - NA) // UB, lambda i: [step(UB * i + u + LAG + NA, 0, vis, fill, u > 0)
                                                 for u in range(UB)])
    done = (NSEG - 1 - LAG) * SEG
    out_a = pltpu.make_async_copy(out_s.at[0:done, :], out_hbm.at[0:done, :], sem.at[SW + 8])
    out_a.start()
    with _scope("epi"):
        vis, fill = masks(2)
        step(NSEG, 2, vis, fill)
        step(NSEG + 1, 2, *masks(2, 2 * M), True)
    post2(NSEG + LAG)
    out_b = pltpu.make_async_copy(out_s.at[done:S, :], out_hbm.at[done:S, :], sem.at[SW + 9])
    out_b.start()
    out_a.wait()
    out_b.wait()


@jax.jit
def pallas_interleave_layers__memory_aug_recurrent_mem_tr__ssm_conv_h3__prompt_kernel(
    A_x, A_mem0, A_Wq, A_Wk, A_Wv, A_Wo, A_seg_len,
    B_q, B_k, B_v, B_shift_k, B_ssm_k, B_ssm_D,
):
    del A_seg_len, B_q
    assert A_x.shape == (1, S, D) and A_Wq.shape == (D, H, DH)
    hbm = pl.BlockSpec(memory_space=pl.ANY)
    out = pl.pallas_call(
        _kernel,
        out_shape=jax.ShapeDtypeStruct((S, D), BF16),
        in_specs=[hbm] * 11,
        out_specs=hbm,
        scratch_shapes=[
            pltpu.VMEM((S, D), BF16),
            pltpu.VMEM((S, D), BF16),
            pltpu.VMEM((S, D), BF16),
            pltpu.VMEM((HB, D, 2 * TB), BF16),
            pltpu.VMEM((3, D, H, DH), BF16),
            pltpu.VMEM(((H + 1) * WP, 128), U32),
            pltpu.VMEM(((2 * H + 1) * WP, 128), U32),
            pltpu.VMEM((H * DH, D), BF16),
            pltpu.VMEM((NLB, H * DH // 2, 128), U32),
            pltpu.VMEM((TB // 2, TB), U32),
            pltpu.VMEM((2, TB // 2, TB), U32),
            pltpu.VMEM((2, TB // 2, TB), U32),
            pltpu.VMEM((2, NLB, S // 2 + 8, 128), F32),
            pltpu.VMEM((NB, 2, NLB * TB, 128), F32),
            pltpu.VMEM((NB, 3, NLB * TB, 128), F32),
            pltpu.VMEM((NB + 1, 2, NLB * TB, 128), F32),
            pltpu.VMEM((NLB, S + 8, 128), F32),
            pltpu.VMEM((ROWS, D), BF16),
            pltpu.VMEM((2 * SEG, D), F32),
            pltpu.VMEM((4, SEG, D), F32),
            pltpu.VMEM((S, D), BF16),
            pltpu.VMEM((NA * SEG, D), BF16),
            pltpu.VMEM((NQH, NA * SEG, DH), BF16),
            pltpu.VMEM((M, D), BF16),
            pltpu.VMEM((KS, D), BF16),
            pltpu.VMEM((D,), BF16),
            pltpu.SemaphoreType.DMA((HB + HB // 2 + 12,)),
        ],
        compiler_params=pltpu.CompilerParams(vmem_limit_bytes=120 * 1024 * 1024),
    )(A_x.reshape(S, D), A_mem0.reshape(M, D), A_Wq, A_Wk, A_Wv,
      A_Wo.reshape(H * DH, D), B_k.reshape(S, D), B_v.reshape(S, D),
      B_shift_k.T, B_ssm_k, B_ssm_D)
    return out.reshape(1, S, D)
```

```python
import contextlib
import functools
import math

import jax
import jax.numpy as jnp
from jax import lax
import jax.experimental.pallas as pl
import jax.experimental.pallas.tpu as pltpu

F32 = jnp.float32
BF16 = jnp.bfloat16
U32 = jnp.uint32

S = 2048
D = 640
H = 32
DH = 128
M = 8
SEG = 32
NSEG = S // SEG
KS = 4
LAG = 2
ROWS = 2 * M + 2 * SEG
HG = 4
NG = H // HG
NLB = D // 128
TB = 128
NB = S // TB
HB = NB // 2
NPOS = NLB * TB // 8
NA = 20
PPS = 4
UCUT = tuple(range(a, a + 2) for a in range(0, 12, 2)) + (range(12, 16),)
NQH = 32
UA = 2
UB = 3
UI = 4
WP = 324


PROFILE = False


def _scope(name):
    return jax.named_scope(name) if PROFILE else contextlib.nullcontext()


def _ln(x, toks=None):
    m = jnp.mean(x, axis=-1, keepdims=True)
    c = x - m
    v = jnp.mean(c * c, axis=-1, keepdims=True)
    r = lax.rsqrt(v + 1e-5)
    if toks is not None:
        toks.append(jnp.minimum(r, 0.0))
    return c * r


def _r(x):
    return x.astype(BF16).astype(F32)


def _split(x):
    hi = pltpu.bitcast(pltpu.bitcast(x, U32) & jnp.uint32(0xFFFF0000), F32)
    return hi, x - hi


def _pk(x):
    return pltpu.bitcast(x.astype(BF16), U32)


def _upk(w):
    return pltpu.bitcast(w, BF16)


def _basis(r, t):
    b = r & 63
    f = jnp.where(b < 32, 2 * b, 2 * b - 63)
    n = ((2 * f + 1) * t - jnp.where(r >= 64, TB, 0)) & (4 * TB - 1)
    n = jnp.where(n >= 2 * TB, n - 4 * TB, n)
    return jnp.cos(n.astype(F32) * (2.0 * math.pi / (4 * TB)))


def _halves(x):
    w = pltpu.bitcast(x, U32)
    return (pltpu.bitcast(w << 16, F32),
            pltpu.bitcast(w & jnp.uint32(0xFFFF0000), F32))


def _kernel(x_hbm, mem0_hbm, wq_hbm, wk_hbm, wv_hbm, wo_hbm,
            k_hbm, v_hbm, shk_hbm, ssmk_hbm, ssmd_hbm,
            out_hbm,
            x_s, k_s, v_s, ssmk_s, wraw, wt_q, wt_kv, wo_s, wo_t,
            perm_s, fu_s, inv_s, kpad, u_s, kf_s, c_s, y_s,
            hbuf, obuf, x2_s, out_s, hl_s, qh_s, mem0_ref, shk_ref, ssmd_ref,
            sem):
    X0, XH = LAG * SEG, (LAG + NA) * SEG
    SW = HB + HB // 2

    def pair_rows(jp):
        r0 = jp * 2 * TB
        return pl.ds(r0 if isinstance(jp, int) else pl.multiple_of(r0, 2 * TB), 2 * TB)

    def ssmk_copy(jp):
        return pltpu.make_async_copy(ssmk_hbm.at[:, pair_rows(jp)], ssmk_s.at[jp], sem.at[jp])

    def kv_copies(rows, sm):
        return [pltpu.make_async_copy(k_hbm.at[rows, :], k_s.at[rows, :], sm),
                pltpu.make_async_copy(v_hbm.at[rows, :], v_s.at[rows, :], sm)]
    DQ = 192
    wq_early = [pltpu.make_async_copy(wq_hbm.at[n * DQ:(n + 1) * DQ], wraw.at[0, n * DQ:(n + 1) * DQ],
                                      sem.at[SW + 10 + n]) for n in range(2)]
    w_copies = [pltpu.make_async_copy(wq_hbm.at[2 * DQ:], wraw.at[0, 2 * DQ:], sem.at[SW])]
    w_copies += [pltpu.make_async_copy(w.at[n * (D // 2):(n + 1) * (D // 2)],
                                       wraw.at[t, n * (D // 2):(n + 1) * (D // 2)],
                                       sem.at[SW + 11 * n + t])
                 for t, w in ((1, wk_hbm), (2, wv_hbm)) for n in range(2)]
    wo_copy = pltpu.make_async_copy(wo_hbm, wo_s, sem.at[SW + 3])
    late_copies = kv_copies(pl.ds(S // 2, S // 2), sem.at[SW + 4])
    small_copies = [pltpu.make_async_copy(src, dst, sem.at[SW + 5])
                    for src, dst in ((shk_hbm, shk_ref), (ssmd_hbm, ssmd_ref), (mem0_hbm, mem0_ref))]
    xa_copy = pltpu.make_async_copy(x_hbm.at[X0:XH, :], x_s.at[X0:XH, :], sem.at[SW + 6])
    late_copies += [pltpu.make_async_copy(x_hbm.at[a:b, :], x_s.at[a:b, :], sem.at[SW + 4])
                    for a, b in ((0, X0), (XH, XH + SEG))]
    xb_copy = pltpu.make_async_copy(x_hbm.at[XH + SEG:, :], x_s.at[XH + SEG:, :], sem.at[SW + 7])
    for c in (small_copies + [ssmk_copy(jp) for jp in range(HB)]
              + [c for jp in range(HB // 2) for c in kv_copies(pair_rows(jp), sem.at[HB + jp])]
              + [xa_copy] + wq_early + [w_copies[0]] + late_copies + w_copies[1:] + [wo_copy]):
        c.start()

    hb = TB // 2
    ri = lax.broadcasted_iota(jnp.int32, (TB, TB), 0)
    ci = lax.broadcasted_iota(jnp.int32, (TB, TB), 1)
    perm_s[...] = _pk(jnp.where(ci == 2 * (ri & 63) + (ri >> 6), 1.0, 0.0))
    tab = _basis(ri, 2 * (ci & 63) + (ci >> 6))
    hi, lo = _split(tab)
    fu_s[0] = _pk(jnp.where(ci < hb, hi, pltpu.roll(lo, hb, 1)))
    fu_s[1] = _pk(jnp.where(ci < hb, pltpu.roll(hi, hb, 1), lo))
    gh, gl = _split(tab.T * (1.0 / TB))
    inv_s[0] = _pk(gh)
    inv_s[1] = _pk(gl)

    for c in small_copies:
        c.wait()
    shk_t = shk_ref[...].astype(F32)
    taps = [[shk_t[j:j + 1, g * 128:(g + 1) * 128] for g in range(NLB)] for j in range(KS)]
    dvec = ssmd_ref[...].astype(F32).reshape(1, D)
    for g in range(NLB):
        kpad[0, g, 0:8, :] = jnp.zeros((8, 128), F32)
        kpad[1, g, 0:8, :] = jnp.zeros((8, 128), F32)
    c_s[0] = jnp.zeros(c_s.shape[1:], F32)

    def spectrum(e, o):
        fe = jnp.dot(_upk(fu_s[0]), jnp.concatenate([e, e], axis=0).astype(BF16), preferred_element_type=F32)
        fo = jnp.dot(_upk(fu_s[1]), jnp.concatenate([o, o], axis=0).astype(BF16), preferred_element_type=F32)
        return ((fe[:hb] + fo[:hb], fe[hb:] + fo[hb:]), (fe[:hb] - fo[:hb], fo[hb:] - fe[hb:]))

    def freq_rows(g):
        return slice(g * TB, g * TB + hb), slice(g * TB + hb, (g + 1) * TB)

    def fwd_k(jq):
        for jp in (2 * jq, 2 * jq + 1):
            ssmk_copy(jp).wait()

        def transposed(n):
            blk = ssmk_s[2 * jq + n // 2, :, (n % 2) * TB:(n % 2 + 1) * TB]
            return lax.dot_general(_upk(perm_s[...]), blk, (((1,), (1,)), ((), ())),
                                   preferred_element_type=F32)
        nxt = transposed(0)
        for n in range(4):
            kt = nxt
            if n < 3:
                nxt = transposed(n + 1)
            j = 4 * jq + n
            for g in range(NLB):
                lb = slice(g * 128, (g + 1) * 128)
                for rows, (kr, ki) in zip(freq_rows(g), spectrum(kt[:hb, lb], kt[hb:, lb])):
                    if n == 0:
                        kr = kr + jnp.where(j == 0, dvec[:, lb], 0.0)
                    kf_s[j, 0, rows] = kr
                    kf_s[j, 1, rows] = ki - kr
                    kf_s[j, 2, rows] = kr + ki

    def fwd_u(jq, first):
        if first:
            for jp in (2 * jq, 2 * jq + 1):
                for c in kv_copies(pair_rows(jp), sem.at[HB + jp]):
                    c.wait()
        for j in [4 * jq + n for n in range(4)]:
            r0 = pl.multiple_of(j * TB, TB)
            q0 = pl.multiple_of(j * hb, hb) + 8
            for g in range(NLB):
                lb = slice(g * 128, (g + 1) * 128)
                ke, ko = _halves(k_s[pl.ds(r0, TB), lb])
                ve, vo = _halves(v_s[pl.ds(r0, TB), lb])
                kpad[0, g, pl.ds(q0, hb), :] = ke
                kpad[1, g, pl.ds(q0, hb), :] = ko
                ke1 = kpad[0, g, pl.ds(q0 - 1, hb), :]
                ko1 = kpad[1, g, pl.ds(q0 - 1, hb), :]
                ko2 = kpad[1, g, pl.ds(q0 - 2, hb), :]
                t0, t1, t2, t3 = (taps[t][g] for t in range(KS))
                e = (ke * t0 + ko1 * t1 + ke1 * t2 + ko2 * t3) * ve
                o = (ko * t0 + ke * t1 + ko1 * t2 + ke1 * t3) * vo
                for rows, (ur, ui) in zip(freq_rows(g), spectrum(e, o)):
                    u_s[j, 0, rows] = ur
                    u_s[j, 1, rows] = ui

    def mac_units(row, half):
        rs = pl.ds(row, 8)
        state = {}

        def unit(p, avals, final, tok=None):
            acc = state.setdefault(p, dict(state.get(0, {})))
            for a in avals:
                u = u_s[a, 0, rs] + u_s[a, 1, rs] if p == 0 else u_s[a, p - 1, rs]
                if tok is not None:
                    u = u + tok
                for i in range(max(a, half * HB), half * HB + HB):
                    t = u * kf_s[i - a, p, rs]
                    acc[i] = t if i not in acc else (acc[i] - t if p == 2 else acc[i] + t)
            if final and p:
                for i, v in acc.items():
                    c_s[i + 1, 2 - p, rs] = v

        subs = UCUT if half else (range(HB),)
        return [functools.partial(unit, p, avals, n == len(subs) - 1)
                for p in range(3) for n, avals in enumerate(subs)]

    def inv_stage(i, units=None):
        q = TB // 4
        for g in range(NLB):
            re, im = [], []
            for b in range(4):
                rows = slice(g * TB + b * q, g * TB + (b + 1) * q)
                cr, ci_ = c_s[i + 1, 0, rows], c_s[i + 1, 1, rows]
                pr, pi = c_s[i, 0, rows], c_s[i, 1, rows]
                re.append(cr + pi if b in (0, 3) else cr - pi)
                im.append(ci_ - pr if b in (0, 3) else ci_ + pr)
            pe = jnp.concatenate([re[0] + re[2], re[1] + re[3], im[0] - im[2], im[1] - im[3]], axis=0)
            po = jnp.concatenate([re[0] - re[2], re[1] - re[3], im[0] + im[2], im[1] + im[3]], axis=0)
            for par, pp in enumerate((pe, po)):
                ph, plo = _split(pp)
                gh_, gl_ = (inv_s[n, par * q:(par + 1) * q] for n in range(2))
                y = jnp.dot(_upk(jnp.concatenate([gh_, gl_, gh_], axis=1)),
                            jnp.concatenate([ph, ph, plo], axis=0).astype(BF16),
                            preferred_element_type=F32)
                y_s[g, pl.ds(i * TB + par, hb, stride=2), :] = y
                if units:
                    tok = pltpu.bitcast(jnp.minimum(jnp.abs(y[0:16]), 0.0), U32)
                    for _ in range(3):
                        if units:
                            units.pop(0)(tok)

    def relayout_rows(t, dst, base, dp, tok=None):
        a = pltpu.bitcast(wraw[t, 2 * dp], U32)
        b = pltpu.bitcast(wraw[t, 2 * dp + 1], U32)
        if tok is not None:
            a = a | tok
        dst[pl.ds(base + dp, 16, stride=WP), :] = (a & jnp.uint32(0xFFFF)) | (b << 16)
        dst[pl.ds(base + 16 * WP + dp, 16, stride=WP), :] = (
            (a >> 16) | (b & jnp.uint32(0xFFFF0000)))

    def wslab(t, h):
        s0 = (max(t - 1, 0) * H + (h % 2) * 16 + h // 2) * WP
        return pltpu.bitcast((wt_kv if t else wt_q)[s0:s0 + D // 2, :], BF16)

    def loop(n, fn):
        def body(j, _):
            fn(j)
            return 0
        lax.fori_loop(0, n, body, 0)

    def norm_rows(c):
        nr = NA * SEG // (HB // UI)
        r0 = pl.multiple_of(c * nr, 16)
        for r in range(0, nr, 16):
            hl_s[pl.ds(r0 + r, 16), :] = _ln(
                x_s[pl.ds(r0 + r + LAG * SEG, 16), :].astype(F32)).astype(BF16)

    def pre_queries(c, t=None):
        per = -(-(D // 4) // NQH)
        for sub in range(2):
            if t is not None:
                half = wraw.at[t, sub * (D // 2):(sub + 1) * (D // 2)]
                pltpu.make_async_copy(half, half, sem.at[SW + 11 * sub + t]).wait()
                base = (t - 1) * (H * WP)
                dp = sub * (D // 4)
            r0 = pl.multiple_of((2 * c + sub) * QR, QR)
            hl = hl_s[pl.ds(r0, QR), :]
            for hd in range(NQH):
                r = jnp.dot(hl, wslab(0, hd), preferred_element_type=F32)
                qh_s[hd, pl.ds(r0, QR), :] = r.astype(BF16)
                if t is not None:
                    tok = pltpu.bitcast(jnp.minimum(jnp.abs(r[0:16]), 0.0), U32)
                    for _ in range(per):
                        if dp < (sub + 1) * (D // 4):
                            relayout_rows(t, wt_kv, base, dp, tok)
                            dp += 1

    nch = NA * SEG // TB
    QR = TB // 2
    with _scope("conv_k"):
        loop(HB // 2, fwd_k)
    with _scope("conv_u"):
        loop(HB // 4, lambda j: fwd_u(j, True))
    with _scope("conv_b"):
        loop(NPOS // 10, lambda j: [u() for n in range(10)
                                    for u in mac_units(pl.multiple_of(80 * j, 16) + 8 * n, 0)])
        xa_copy.wait()

        def inv_first(j):
            part = wraw.at[0, pl.ds(j * DQ, DQ)]
            pltpu.make_async_copy(part, part, sem.at[SW + 10 + j]).wait()
            units = [functools.partial(relayout_rows, 0, wt_q, 0, j * (DQ // 2) + dd)
                     for dd in range(DQ // 2)]
            for u in range(UI):
                inv_stage(UI * j + u, units)
            assert not units
            norm_rows(j)
        loop(HB // UI, inv_first)
    with _scope("rel0"):
        w_copies[0].wait()
        loop((D - 2 * DQ) // 64,
             lambda i: [relayout_rows(0, wt_q, 0, DQ + i * 32 + dd) for dd in range(32)])
    with _scope("preq"):
        loop(nch - 2, pre_queries)
    with _scope("conv_c"):
        for c in late_copies:
            c.wait()
        loop(HB // 4, lambda j: fwd_u(HB // 4 + j, False))
    with _scope("preq_rel"):
        loop(2, lambda i: pre_queries(i + nch - 2, i + 1))

    scale = DH ** -0.5

    def masks(mode, q0=0):
        rows = ROWS if mode == 0 else ROWS - SEG
        qi = lax.broadcasted_iota(jnp.int32, (rows - q0, 128), 0) + q0
        kj = lax.broadcasted_iota(jnp.int32, (rows - q0, 128), 1)

        def layer_of(i):
            xl = (i - 2 * M) // SEG if mode == 0 else mode - 1
            return jnp.where(i < 2 * M, i // M, xl)
        same = (layer_of(qi) == layer_of(kj)) & (kj < rows)
        vis = same & ((qi < 2 * M) | (qi >= kj))
        fill = jnp.where(same, -1e9 / scale, -jnp.inf).astype(F32)
        return vis, fill

    mem0 = mem0_ref[...].astype(F32)
    hbuf[0:16, :] = jnp.concatenate([mem0, mem0], axis=0).astype(BF16)
    hbuf[16:48, :] = _ln(x_s[0:SEG, :].astype(F32)).astype(BF16)
    obuf[...] = jnp.zeros((2 * SEG, D), F32)
    x2_s[...] = jnp.zeros(x2_s.shape, F32)

    def seg_row(seg):
        if isinstance(seg, int):
            return min(max(seg, 0), NSEG - 1) * SEG
        return pl.multiple_of(jnp.clip(seg, 0, NSEG - 1) * SEG, SEG)

    def gate(xa, r0, toks=None):
        y = jnp.concatenate([y_s[g, pl.ds(r0, xa.shape[0]), :] for g in range(NLB)], axis=1)
        return xa + _ln(xa, toks) * y

    def attention(h, vis, fill, chained, before_oproj=None, early=None, due=()):
        q0 = h.shape[0] - vis.shape[0]
        if early is not None:
            hrest = jnp.concatenate([h[:2 * M], h[2 * M + SEG:]], axis=0)
            qrow = pl.multiple_of(early * SEG, SEG)
            units = [u for n in range(PPS)
                     for u in mac_units(pl.multiple_of(early * (8 * PPS), 8 * PPS) + 8 * n, 1)]

        def proj(g):
            res = [[None] * HG for _ in range(3)]
            order = [(t, j) for j in range(HG) for t in range(2)] + [(2, j) for j in range(HG)]

            def operand(t, j):
                pre = early is not None and t == 0 and g * HG + j < NQH
                return pre, hrest if pre else (h if t else h[q0:])

            kc = D - 128
            nsplit = 4 if g == 0 and chained else 0
            part = [jnp.dot(operand(t, j)[1][:, :kc], wslab(t, j)[:kc], preferred_element_type=F32)
                    for t, j in order[:nsplit]]
            for n, (t, j) in enumerate(order):
                hd = g * HG + j
                pre, lhs = operand(t, j)
                if n < nsplit:
                    r = jnp.dot(lhs[:, kc:], wslab(t, hd)[kc:], preferred_element_type=F32) + part[n]
                else:
                    r = jnp.dot(lhs, wslab(t, hd), preferred_element_type=F32)
                if early is not None and units:
                    units.pop(0)(jnp.minimum(jnp.abs(r[0:8]), 0.0))
                if t == 0:
                    r = r.astype(BF16)
                if pre:
                    r = jnp.concatenate([r[:2 * M], qh_s[hd, pl.ds(qrow, SEG), :], r[2 * M:]], axis=0)
                res[t][j] = r
            return res

        def pad(kv):
            return jnp.concatenate([kv, jnp.zeros((128 - kv.shape[0], DH), F32)], axis=0).astype(BF16)

        def probs(qkv, g):
            scs = [lax.dot_general(qkv[0][j], pad(qkv[1][j]), (((1,), (1,)), ((), ())),
                                   preferred_element_type=F32) for j in range(HG)]
            ps = []
            for sc in scs:
                sc = jnp.where(vis, sc, fill)
                e = jnp.exp2((sc - jnp.max(sc, axis=-1, keepdims=True)) * (scale * math.log2(math.e)))
                den = jnp.sum(e, axis=-1, keepdims=True)
                if not ps and g >= NG - len(due):
                    e = jnp.concatenate([e[:16] + due[g - NG + len(due)], e[16:]], axis=0)
                r = pl.reciprocal(den, approx=True)
                r = r * (2.0 - den * r)
                ps.append((e * r).astype(BF16))
            return ps

        def oproj(os_, h0):
            oc = jnp.concatenate(os_, axis=1).astype(BF16)
            k0, k1 = h0 * DH, (h0 + len(os_)) * DH
            res = []
            for n in range(NLB):
                if before_oproj is not None:
                    w = wo_s[k0:k1, n * 128:(n + 1) * 128]
                    wo_t[n, k0 // 2:k1 // 2, :] = pltpu.bitcast(w, U32)
                else:
                    w = pltpu.bitcast(wo_t[n, k0 // 2:k1 // 2, :], BF16)
                res.append(jnp.dot(oc, w, preferred_element_type=F32))
            return res

        heads = []
        qkv = proj(0)
        oa = None
        for g in range(NG):
            ps = probs(qkv, g)
            vs = qkv[2]
            if g + 1 < NG:
                qkv = proj(g + 1)
            else:
                if before_oproj is not None:
                    before_oproj()
                oa = oproj(heads[:H // 2], 0)
            heads += [jnp.dot(ps[j], pad(vs[j]), preferred_element_type=F32)
                      for j in range(HG)]
        assert early is None or not units
        ob = oproj(heads[H // 2:], H // 2)
        return jnp.concatenate([b + a for a, b in zip(oa, ob)], axis=1)

    def post2(s, toks=None):
        r3 = seg_row(s - 1 - LAG)
        for r in (0, 16):
            xc = _r(x2_s[(s + 4 - 1 - LAG) % 4, r:r + 16] + obuf[SEG + r:SEG + r + 16, :])
            out_s[pl.ds(r3 + r, 16), :] = gate(xc, r3 + r, toks).astype(BF16)

    def step(s, mode, vis, fill, chained=False, before_oproj=None, early=None):
        if mode == 0:
            h = hbuf[...]
        elif mode == 1:
            h = hbuf[0:48, :]
        else:
            live = lax.broadcasted_iota(jnp.int32, (2 * M, D), 0) >= M
            mem = jnp.where(live, hbuf[0:16, :].astype(F32), 0.0).astype(BF16)
            h = jnp.concatenate([mem, hbuf[48:80, :]], axis=0)
        toks = []
        if mode != 1:
            post2(s, toks)
        if isinstance(s, int) and s == NSEG + LAG - 1:
            obuf[SEG:2 * SEG, :] = attention(h, vis, fill, chained, due=toks)
            return
        r1 = seg_row(s - 1)
        rn = seg_row(s + 1)
        h1n, h2n = [], []
        for r in (0, 16):
            xa = _r(x_s[pl.ds(r1 + r, 16), :].astype(F32) + obuf[r:r + 16, :])
            xb2 = _r(gate(xa, r1 + r))
            h2n.append(_ln(xb2, toks).astype(BF16))
            x2_s[(s + 4 - 1) % 4, r:r + 16] = xb2
        if mode != 2:
            for r in (0, 16):
                h1n.append(_ln(x_s[pl.ds(rn + r, 16), :].astype(F32), toks).astype(BF16))

        o = attention(h, vis, fill, chained, before_oproj, early, toks)

        mem2 = mem0 if mode == 1 else o[M:2 * M]
        hbuf[0:16, :] = jnp.concatenate([o[0:M], mem2], axis=0).astype(BF16)
        for n, v in enumerate(h1n):
            hbuf[16 + 16 * n:32 + 16 * n, :] = v
        for n, v in enumerate(h2n):
            hbuf[48 + 16 * n:64 + 16 * n, :] = v
        if mode == 0:
            obuf[...] = o[2 * M:]
        elif mode == 1:
            obuf[0:SEG, :] = o[2 * M:]
        else:
            obuf[SEG:2 * SEG, :] = o[2 * M:]

    with _scope("pro"):
        vis, fill = masks(1)
        step(0, 1, vis, fill, False, wo_copy.wait)
        step(1, 1, vis, fill, True)
    xb_copy.start()
    vis, fill = masks(0)
    with _scope("main_a"):
        loop(NA // UA, lambda i: [step(UA * i + u + LAG, 0, vis, fill, u > 0, early=UA * i + u)
                                  for u in range(UA)])
    xb_copy.wait()
    with _scope("conv_e"):
        loop(HB // UI, lambda j: [inv_stage(HB + UI * j + u) for u in range(UI)])
    with _scope("main_b"):
        loop((NSEG - LAG - NA) // UB, lambda i: [step(UB * i + u + LAG + NA, 0, vis, fill, u > 0)
                                                 for u in range(UB)])
    done = (NSEG - 1 - LAG) * SEG
    out_a = pltpu.make_async_copy(out_s.at[0:done, :], out_hbm.at[0:done, :], sem.at[SW + 8])
    out_a.start()
    with _scope("epi"):
        vis, fill = masks(2)
        step(NSEG, 2, vis, fill)
        step(NSEG + 1, 2, *masks(2, 2 * M), True)
    post2(NSEG + LAG)
    out_b = pltpu.make_async_copy(out_s.at[done:S, :], out_hbm.at[done:S, :], sem.at[SW + 9])
    out_b.start()
    out_a.wait()
    out_b.wait()


@jax.jit
def pallas_interleave_layers__memory_aug_recurrent_mem_tr__ssm_conv_h3__prompt_kernel(
    A_x, A_mem0, A_Wq, A_Wk, A_Wv, A_Wo, A_seg_len,
    B_q, B_k, B_v, B_shift_k, B_ssm_k, B_ssm_D,
):
    del A_seg_len, B_q
    assert A_x.shape == (1, S, D) and A_Wq.shape == (D, H, DH)
    hbm = pl.BlockSpec(memory_space=pl.ANY)
    out = pl.pallas_call(
        _kernel,
        out_shape=jax.ShapeDtypeStruct((S, D), BF16),
        in_specs=[hbm] * 11,
        out_specs=hbm,
        scratch_shapes=[
            pltpu.VMEM((S, D), BF16),
            pltpu.VMEM((S, D), BF16),
            pltpu.VMEM((S, D), BF16),
            pltpu.VMEM((HB, D, 2 * TB), BF16),
            pltpu.VMEM((3, D, H, DH), BF16),
            pltpu.VMEM(((H + 1) * WP, 128), U32),
            pltpu.VMEM(((2 * H + 1) * WP, 128), U32),
            pltpu.VMEM((H * DH, D), BF16),
            pltpu.VMEM((NLB, H * DH // 2, 128), U32),
            pltpu.VMEM((TB // 2, TB), U32),
            pltpu.VMEM((2, TB // 2, TB), U32),
            pltpu.VMEM((2, TB // 2, TB), U32),
            pltpu.VMEM((2, NLB, S // 2 + 8, 128), F32),
            pltpu.VMEM((NB, 2, NLB * TB, 128), F32),
            pltpu.VMEM((NB, 3, NLB * TB, 128), F32),
            pltpu.VMEM((NB + 1, 2, NLB * TB, 128), F32),
            pltpu.VMEM((NLB, S + 8, 128), F32),
            pltpu.VMEM((ROWS, D), BF16),
            pltpu.VMEM((2 * SEG, D), F32),
            pltpu.VMEM((4, SEG, D), F32),
            pltpu.VMEM((S, D), BF16),
            pltpu.VMEM((NA * SEG, D), BF16),
            pltpu.VMEM((NQH, NA * SEG, DH), BF16),
            pltpu.VMEM((M, D), BF16),
            pltpu.VMEM((KS, D), BF16),
            pltpu.VMEM((D,), BF16),
            pltpu.SemaphoreType.DMA((HB + HB // 2 + 14,)),
        ],
        compiler_params=pltpu.CompilerParams(vmem_limit_bytes=120 * 1024 * 1024),
    )(A_x.reshape(S, D), A_mem0.reshape(M, D), A_Wq, A_Wk, A_Wv,
      A_Wo.reshape(H * DH, D), B_k.reshape(S, D), B_v.reshape(S, D),
      B_shift_k.T, B_ssm_k, B_ssm_D)
    return out.reshape(1, S, D)
```

```python
import contextlib
import functools
import math

import jax
import jax.numpy as jnp
from jax import lax
import jax.experimental.pallas as pl
import jax.experimental.pallas.tpu as pltpu

F32 = jnp.float32
BF16 = jnp.bfloat16
U32 = jnp.uint32

S = 2048
D = 640
H = 32
DH = 128
M = 8
SEG = 32
NSEG = S // SEG
KS = 4
LAG = 2
ROWS = 2 * M + 2 * SEG
HG = 4
NG = H // HG
NLB = D // 128
TB = 128
NB = S // TB
HB = NB // 2
NPOS = NLB * TB // 8
NA = 20
PPS = 4
UCUT = tuple(range(a, a + 2) for a in range(0, 12, 2)) + (range(12, 16),)
NQH = 32
UA = 2
UB = 3
UI = 4
WP = 324


PROFILE = False


def _scope(name):
    return jax.named_scope(name) if PROFILE else contextlib.nullcontext()


def _ln(x, toks=None):
    m = jnp.mean(x, axis=-1, keepdims=True)
    c = x - m
    v = jnp.mean(c * c, axis=-1, keepdims=True)
    r = lax.rsqrt(v + 1e-5)
    if toks is not None:
        toks.append(jnp.minimum(r, 0.0))
    return c * r


def _r(x):
    return x.astype(BF16).astype(F32)


def _split(x):
    hi = pltpu.bitcast(pltpu.bitcast(x, U32) & jnp.uint32(0xFFFF0000), F32)
    return hi, x - hi


def _pk(x):
    return pltpu.bitcast(x.astype(BF16), U32)


def _upk(w):
    return pltpu.bitcast(w, BF16)


def _basis(r, t):
    b = r & 63
    f = jnp.where(b < 32, 2 * b, 2 * b - 63)
    n = ((2 * f + 1) * t - jnp.where(r >= 64, TB, 0)) & (4 * TB - 1)
    n = jnp.where(n >= 2 * TB, n - 4 * TB, n)
    return jnp.cos(n.astype(F32) * (2.0 * math.pi / (4 * TB)))


def _halves(x):
    w = pltpu.bitcast(x, U32)
    return (pltpu.bitcast(w << 16, F32),
            pltpu.bitcast(w & jnp.uint32(0xFFFF0000), F32))


def _kernel(x_hbm, mem0_hbm, wq_hbm, wk_hbm, wv_hbm, wo_hbm,
            k_hbm, v_hbm, shk_hbm, ssmk_hbm, ssmd_hbm,
            out_hbm,
            x_s, k_s, v_s, ssmk_s, wraw, wt_q, wt_kv, wo_s, wo_t,
            perm_s, fu_s, inv_s, kpad, u_s, kf_s, c_s, y_s,
            hbuf, obuf, x2_s, out_s, hl_s, qh_s, mem0_ref, shk_ref, ssmd_ref,
            sem):
    X0, XH = LAG * SEG, (LAG + NA) * SEG
    SW = HB + HB // 2

    def pair_rows(jp):
        r0 = jp * 2 * TB
        return pl.ds(r0 if isinstance(jp, int) else pl.multiple_of(r0, 2 * TB), 2 * TB)

    def ssmk_copy(jp):
        return pltpu.make_async_copy(ssmk_hbm.at[:, pair_rows(jp)], ssmk_s.at[jp], sem.at[jp])

    def kv_copies(rows, sm):
        return [pltpu.make_async_copy(k_hbm.at[rows, :], k_s.at[rows, :], sm),
                pltpu.make_async_copy(v_hbm.at[rows, :], v_s.at[rows, :], sm)]
    DQ = 192
    wq_early = [pltpu.make_async_copy(wq_hbm.at[n * DQ:(n + 1) * DQ], wraw.at[0, n * DQ:(n + 1) * DQ],
                                      sem.at[SW + 10 + n]) for n in range(2)]
    w_copies = [pltpu.make_async_copy(wq_hbm.at[2 * DQ:], wraw.at[0, 2 * DQ:], sem.at[SW])]
    w_copies += [pltpu.make_async_copy(w.at[n * (D // 2):(n + 1) * (D // 2)],
                                       wraw.at[t, n * (D // 2):(n + 1) * (D // 2)],
                                       sem.at[SW + 11 * n + t])
                 for t, w in ((1, wk_hbm), (2, wv_hbm)) for n in range(2)]
    wo_copy = pltpu.make_async_copy(wo_hbm, wo_s, sem.at[SW + 3])
    late_copies = kv_copies(pl.ds(S // 2, S // 2), sem.at[SW + 4])
    small_copies = [pltpu.make_async_copy(src, dst, sem.at[SW + 5])
                    for src, dst in ((shk_hbm, shk_ref), (ssmd_hbm, ssmd_ref), (mem0_hbm, mem0_ref))]
    xa_copy = pltpu.make_async_copy(x_hbm.at[X0:XH, :], x_s.at[X0:XH, :], sem.at[SW + 6])
    late_copies += [pltpu.make_async_copy(x_hbm.at[a:b, :], x_s.at[a:b, :], sem.at[SW + 4])
                    for a, b in ((0, X0), (XH, XH + SEG))]
    xb_copy = pltpu.make_async_copy(x_hbm.at[XH + SEG:, :], x_s.at[XH + SEG:, :], sem.at[SW + 7])
    for c in (small_copies + [ssmk_copy(jp) for jp in range(HB)]
              + [c for jp in range(HB // 2) for c in kv_copies(pair_rows(jp), sem.at[HB + jp])]
              + [xa_copy] + wq_early + [w_copies[0]] + late_copies + w_copies[1:] + [wo_copy]):
        c.start()

    hb = TB // 2
    ri = lax.broadcasted_iota(jnp.int32, (TB, TB), 0)
    ci = lax.broadcasted_iota(jnp.int32, (TB, TB), 1)
    perm_s[...] = _pk(jnp.where(ci == 2 * (ri & 63) + (ri >> 6), 1.0, 0.0))
    tab = _basis(ri, 2 * (ci & 63) + (ci >> 6))
    hi, lo = _split(tab)
    fu_s[0] = _pk(jnp.where(ci < hb, hi, pltpu.roll(lo, hb, 1)))
    fu_s[1] = _pk(jnp.where(ci < hb, pltpu.roll(hi, hb, 1), lo))
    gh, gl = _split(tab.T * (1.0 / TB))
    inv_s[0] = _pk(gh)
    inv_s[1] = _pk(gl)

    for c in small_copies:
        c.wait()
    shk_t = shk_ref[...].astype(F32)
    taps = [[shk_t[j:j + 1, g * 128:(g + 1) * 128] for g in range(NLB)] for j in range(KS)]
    dvec = ssmd_ref[...].astype(F32).reshape(1, D)
    for g in range(NLB):
        kpad[0, g, 0:8, :] = jnp.zeros((8, 128), F32)
        kpad[1, g, 0:8, :] = jnp.zeros((8, 128), F32)
    c_s[0] = jnp.zeros(c_s.shape[1:], F32)
    hbuf[0:16, :] = jnp.concatenate([mem0_ref[...].astype(F32)] * 2, axis=0).astype(BF16)
    obuf[...] = jnp.zeros((2 * SEG, D), F32)
    x2_s[...] = jnp.zeros(x2_s.shape, F32)

    def spectrum(e, o):
        fe = jnp.dot(_upk(fu_s[0]), jnp.concatenate([e, e], axis=0).astype(BF16), preferred_element_type=F32)
        fo = jnp.dot(_upk(fu_s[1]), jnp.concatenate([o, o], axis=0).astype(BF16), preferred_element_type=F32)
        return ((fe[:hb] + fo[:hb], fe[hb:] + fo[hb:]), (fe[:hb] - fo[:hb], fo[hb:] - fe[hb:]))

    def freq_rows(g):
        return slice(g * TB, g * TB + hb), slice(g * TB + hb, (g + 1) * TB)

    def fwd_k(jq):
        for jp in (2 * jq, 2 * jq + 1):
            ssmk_copy(jp).wait()

        def transposed(n):
            blk = ssmk_s[2 * jq + n // 2, :, (n % 2) * TB:(n % 2 + 1) * TB]
            return lax.dot_general(_upk(perm_s[...]), blk, (((1,), (1,)), ((), ())),
                                   preferred_element_type=F32)
        nxt = transposed(0)
        for n in range(4):
            kt = nxt
            if n < 3:
                nxt = transposed(n + 1)
            j = 4 * jq + n
            for g in range(NLB):
                lb = slice(g * 128, (g + 1) * 128)
                for rows, (kr, ki) in zip(freq_rows(g), spectrum(kt[:hb, lb], kt[hb:, lb])):
                    if n == 0:
                        kr = kr + jnp.where(j == 0, dvec[:, lb], 0.0)
                    kf_s[j, 0, rows] = kr
                    kf_s[j, 1, rows] = ki - kr
                    kf_s[j, 2, rows] = kr + ki

    def fwd_u(jq, first):
        if first:
            for jp in (2 * jq, 2 * jq + 1):
                for c in kv_copies(pair_rows(jp), sem.at[HB + jp]):
                    c.wait()
        for j in [4 * jq + n for n in range(4)]:
            r0 = pl.multiple_of(j * TB, TB)
            q0 = pl.multiple_of(j * hb, hb) + 8
            for g in range(NLB):
                lb = slice(g * 128, (g + 1) * 128)
                ke, ko = _halves(k_s[pl.ds(r0, TB), lb])
                ve, vo = _halves(v_s[pl.ds(r0, TB), lb])
                kpad[0, g, pl.ds(q0, hb), :] = ke
                kpad[1, g, pl.ds(q0, hb), :] = ko
                ke1 = kpad[0, g, pl.ds(q0 - 1, hb), :]
                ko1 = kpad[1, g, pl.ds(q0 - 1, hb), :]
                ko2 = kpad[1, g, pl.ds(q0 - 2, hb), :]
                t0, t1, t2, t3 = (taps[t][g] for t in range(KS))
                e = (ke * t0 + ko1 * t1 + ke1 * t2 + ko2 * t3) * ve
                o = (ko * t0 + ke * t1 + ko1 * t2 + ke1 * t3) * vo
                for rows, (ur, ui) in zip(freq_rows(g), spectrum(e, o)):
                    u_s[j, 0, rows] = ur
                    u_s[j, 1, rows] = ui

    def mac_units(row, half):
        rs = pl.ds(row, 8)
        state = {}

        def unit(p, avals, final, tok=None):
            acc = state.setdefault(p, dict(state.get(0, {})))
            for a in avals:
                u = u_s[a, 0, rs] + u_s[a, 1, rs] if p == 0 else u_s[a, p - 1, rs]
                if tok is not None:
                    u = u + tok
                for i in range(max(a, half * HB), half * HB + HB):
                    t = u * kf_s[i - a, p, rs]
                    acc[i] = t if i not in acc else (acc[i] - t if p == 2 else acc[i] + t)
            if final and p:
                for i, v in acc.items():
                    c_s[i + 1, 2 - p, rs] = v

        subs = UCUT if half else (range(HB),)
        return [functools.partial(unit, p, avals, n == len(subs) - 1)
                for p in range(3) for n, avals in enumerate(subs)]

    def inv_stage(i, units=None):
        q = TB // 4
        for g in range(NLB):
            re, im = [], []
            for b in range(4):
                rows = slice(g * TB + b * q, g * TB + (b + 1) * q)
                cr, ci_ = c_s[i + 1, 0, rows], c_s[i + 1, 1, rows]
                pr, pi = c_s[i, 0, rows], c_s[i, 1, rows]
                re.append(cr + pi if b in (0, 3) else cr - pi)
                im.append(ci_ - pr if b in (0, 3) else ci_ + pr)
            pe = jnp.concatenate([re[0] + re[2], re[1] + re[3], im[0] - im[2], im[1] - im[3]], axis=0)
            po = jnp.concatenate([re[0] - re[2], re[1] - re[3], im[0] + im[2], im[1] + im[3]], axis=0)
            for par, pp in enumerate((pe, po)):
                ph, plo = _split(pp)
                gh_, gl_ = (inv_s[n, par * q:(par + 1) * q] for n in range(2))
                y = jnp.dot(_upk(jnp.concatenate([gh_, gl_, gh_], axis=1)),
                            jnp.concatenate([ph, ph, plo], axis=0).astype(BF16),
                            preferred_element_type=F32)
                y_s[g, pl.ds(i * TB + par, hb, stride=2), :] = y
                if units:
                    tok = pltpu.bitcast(jnp.minimum(jnp.abs(y[0:16]), 0.0), U32)
                    for _ in range(3):
                        if units:
                            units.pop(0)(tok)

    def relayout_rows(t, dst, base, dp, tok=None):
        a = pltpu.bitcast(wraw[t, 2 * dp], U32)
        b = pltpu.bitcast(wraw[t, 2 * dp + 1], U32)
        if tok is not None:
            a = a | tok
        dst[pl.ds(base + dp, 16, stride=WP), :] = (a & jnp.uint32(0xFFFF)) | (b << 16)
        dst[pl.ds(base + 16 * WP + dp, 16, stride=WP), :] = (
            (a >> 16) | (b & jnp.uint32(0xFFFF0000)))

    def wslab(t, h):
        s0 = (max(t - 1, 0) * H + (h % 2) * 16 + h // 2) * WP
        return pltpu.bitcast((wt_kv if t else wt_q)[s0:s0 + D // 2, :], BF16)

    def loop(n, fn):
        def body(j, _):
            fn(j)
            return 0
        lax.fori_loop(0, n, body, 0)

    def norm_rows(c):
        nr = NA * SEG // (HB // UI)
        r0 = pl.multiple_of(c * nr, 16)
        for r in range(0, nr, 16):
            hl_s[pl.ds(r0 + r, 16), :] = _ln(
                x_s[pl.ds(r0 + r + LAG * SEG, 16), :].astype(F32)).astype(BF16)

    def pre_queries(c, t=None):
        per = -(-(D // 4) // NQH)
        for sub in range(2):
            if t is not None:
                half = wraw.at[t, sub * (D // 2):(sub + 1) * (D // 2)]
                pltpu.make_async_copy(half, half, sem.at[SW + 11 * sub + t]).wait()
                base = (t - 1) * (H * WP)
                dp = sub * (D // 4)
            r0 = pl.multiple_of((2 * c + sub) * QR, QR)
            hl = hl_s[pl.ds(r0, QR), :]
            for hd in range(NQH):
                r = jnp.dot(hl, wslab(0, hd), preferred_element_type=F32)
                qh_s[hd, pl.ds(r0, QR), :] = r.astype(BF16)
                if t is not None:
                    tok = pltpu.bitcast(jnp.minimum(jnp.abs(r[0:16]), 0.0), U32)
                    for _ in range(per):
                        if dp < (sub + 1) * (D // 4):
                            relayout_rows(t, wt_kv, base, dp, tok)
                            dp += 1

    nch = NA * SEG // TB
    QR = TB // 2
    with _scope("conv_k"):
        loop(HB // 2, fwd_k)
    with _scope("conv_u"):
        loop(HB // 4, lambda j: fwd_u(j, True))
    with _scope("conv_b"):
        loop(NPOS // 10, lambda j: [u() for n in range(10)
                                    for u in mac_units(pl.multiple_of(80 * j, 16) + 8 * n, 0)])
        xa_copy.wait()

        def inv_first(j):
            part = wraw.at[0, pl.ds(j * DQ, DQ)]
            pltpu.make_async_copy(part, part, sem.at[SW + 10 + j]).wait()
            units = [functools.partial(relayout_rows, 0, wt_q, 0, j * (DQ // 2) + dd)
                     for dd in range(DQ // 2)]
            for u in range(UI):
                inv_stage(UI * j + u, units)
            assert not units
            norm_rows(j)
        loop(HB // UI, inv_first)
    with _scope("rel0"):
        w_copies[0].wait()
        loop((D - 2 * DQ) // 64,
             lambda i: [relayout_rows(0, wt_q, 0, DQ + i * 32 + dd) for dd in range(32)])
    with _scope("preq"):
        loop(nch - 2, pre_queries)
    with _scope("conv_c"):
        for c in late_copies:
            c.wait()

        def fwd_u_late(j):
            r0 = pl.multiple_of(j * 16, 16)
            hbuf[pl.ds(16 + r0, 16), :] = _ln(x_s[pl.ds(r0, 16), :].astype(F32)).astype(BF16)
            fwd_u(HB // 4 + j, False)
        loop(HB // 4, fwd_u_late)
    with _scope("preq_rel"):
        loop(2, lambda i: pre_queries(i + nch - 2, i + 1))

    scale = DH ** -0.5

    def masks(mode, q0=0):
        rows = ROWS if mode == 0 else ROWS - SEG
        qi = lax.broadcasted_iota(jnp.int32, (rows - q0, 128), 0) + q0
        kj = lax.broadcasted_iota(jnp.int32, (rows - q0, 128), 1)

        def layer_of(i):
            xl = (i - 2 * M) // SEG if mode == 0 else mode - 1
            return jnp.where(i < 2 * M, i // M, xl)
        same = (layer_of(qi) == layer_of(kj)) & (kj < rows)
        vis = same & ((qi < 2 * M) | (qi >= kj))
        fill = jnp.where(same, -1e9 / scale, -jnp.inf).astype(F32)
        return vis, fill

    mem0 = mem0_ref[...].astype(F32)

    def seg_row(seg):
        if isinstance(seg, int):
            return min(max(seg, 0), NSEG - 1) * SEG
        return pl.multiple_of(jnp.clip(seg, 0, NSEG - 1) * SEG, SEG)

    def gate(xa, r0, toks=None):
        y = jnp.concatenate([y_s[g, pl.ds(r0, xa.shape[0]), :] for g in range(NLB)], axis=1)
        return xa + _ln(xa, toks) * y

    def attention(h, vis, fill, chained, before_oproj=None, early=None, due=()):
        q0 = h.shape[0] - vis.shape[0]
        if early is not None:
            hrest = jnp.concatenate([h[:2 * M], h[2 * M + SEG:]], axis=0)
            qrow = pl.multiple_of(early * SEG, SEG)
            units = [u for n in range(PPS)
                     for u in mac_units(pl.multiple_of(early * (8 * PPS), 8 * PPS) + 8 * n, 1)]

        def proj(g):
            res = [[None] * HG for _ in range(3)]
            order = [(t, j) for j in range(HG) for t in range(2)] + [(2, j) for j in range(HG)]

            def operand(t, j):
                pre = early is not None and t == 0 and g * HG + j < NQH
                return pre, hrest if pre else (h if t else h[q0:])

            kc = D - 128
            nsplit = 4 if g == 0 and chained else 0
            part = [jnp.dot(operand(t, j)[1][:, :kc], wslab(t, j)[:kc], preferred_element_type=F32)
                    for t, j in order[:nsplit]]
            for n, (t, j) in enumerate(order):
                hd = g * HG + j
                pre, lhs = operand(t, j)
                if n < nsplit:
                    r = jnp.dot(lhs[:, kc:], wslab(t, hd)[kc:], preferred_element_type=F32) + part[n]
                else:
                    r = jnp.dot(lhs, wslab(t, hd), preferred_element_type=F32)
                if early is not None and units:
                    units.pop(0)(jnp.minimum(jnp.abs(r[0:8]), 0.0))
                if t == 0:
                    r = r.astype(BF16)
                if pre:
                    r = jnp.concatenate([r[:2 * M], qh_s[hd, pl.ds(qrow, SEG), :], r[2 * M:]], axis=0)
                res[t][j] = r
            return res

        def pad(kv):
            return jnp.concatenate([kv, jnp.zeros((128 - kv.shape[0], DH), F32)], axis=0).astype(BF16)

        def probs(qkv, g):
            scs = [lax.dot_general(qkv[0][j], pad(qkv[1][j]), (((1,), (1,)), ((), ())),
                                   preferred_element_type=F32) for j in range(HG)]
            ps = []
            for sc in scs:
                sc = jnp.where(vis, sc, fill)
                e = jnp.exp2((sc - jnp.max(sc, axis=-1, keepdims=True)) * (scale * math.log2(math.e)))
                den = jnp.sum(e, axis=-1, keepdims=True)
                if not ps and g >= NG - len(due):
                    e = jnp.concatenate([e[:16] + due[g - NG + len(due)], e[16:]], axis=0)
                r = pl.reciprocal(den, approx=True)
                r = r * (2.0 - den * r)
                ps.append((e * r).astype(BF16))
            return ps

        def oproj(os_, h0):
            oc = jnp.concatenate(os_, axis=1).astype(BF16)
            k0, k1 = h0 * DH, (h0 + len(os_)) * DH
            res = []
            for n in range(NLB):
                if before_oproj is not None:
                    w = wo_s[k0:k1, n * 128:(n + 1) * 128]
                    wo_t[n, k0 // 2:k1 // 2, :] = pltpu.bitcast(w, U32)
                else:
                    w = pltpu.bitcast(wo_t[n, k0 // 2:k1 // 2, :], BF16)
                res.append(jnp.dot(oc, w, preferred_element_type=F32))
            return res

        heads = []
        qkv = proj(0)
        oa = None
        for g in range(NG):
            ps = probs(qkv, g)
            vs = qkv[2]
            if g + 1 < NG:
                qkv = proj(g + 1)
            else:
                if before_oproj is not None:
                    before_oproj()
                oa = oproj(heads[:H // 2], 0)
            heads += [jnp.dot(ps[j], pad(vs[j]), preferred_element_type=F32)
                      for j in range(HG)]
        assert early is None or not units
        ob = oproj(heads[H // 2:], H // 2)
        return jnp.concatenate([b + a for a, b in zip(oa, ob)], axis=1)

    def post2(s, toks=None):
        r3 = seg_row(s - 1 - LAG)
        for r in (0, 16):
            xc = _r(x2_s[(s + 4 - 1 - LAG) % 4, r:r + 16] + obuf[SEG + r:SEG + r + 16, :])
            out_s[pl.ds(r3 + r, 16), :] = gate(xc, r3 + r, toks).astype(BF16)

    def step(s, mode, vis, fill, chained=False, before_oproj=None, early=None):
        if mode == 0:
            h = hbuf[...]
        elif mode == 1:
            h = hbuf[0:48, :]
        else:
            live = lax.broadcasted_iota(jnp.int32, (2 * M, D), 0) >= M
            mem = jnp.where(live, hbuf[0:16, :].astype(F32), 0.0).astype(BF16)
            h = jnp.concatenate([mem, hbuf[48:80, :]], axis=0)
        toks = []
        if mode != 1:
            post2(s, toks)
        if isinstance(s, int) and s == NSEG + LAG - 1:
            obuf[SEG:2 * SEG, :] = attention(h, vis, fill, chained, due=toks)
            return
        r1 = seg_row(s - 1)
        rn = seg_row(s + 1)
        h1n, h2n = [], []
        for r in (0, 16):
            xa = _r(x_s[pl.ds(r1 + r, 16), :].astype(F32) + obuf[r:r + 16, :])
            xb2 = _r(gate(xa, r1 + r))
            h2n.append(_ln(xb2, toks).astype(BF16))
            x2_s[(s + 4 - 1) % 4, r:r + 16] = xb2
        if mode != 2:
            for r in (0, 16):
                h1n.append(_ln(x_s[pl.ds(rn + r, 16), :].astype(F32), toks).astype(BF16))

        o = attention(h, vis, fill, chained, before_oproj, early, toks)

        mem2 = mem0 if mode == 1 else o[M:2 * M]
        hbuf[0:16, :] = jnp.concatenate([o[0:M], mem2], axis=0).astype(BF16)
        for n, v in enumerate(h1n):
            hbuf[16 + 16 * n:32 + 16 * n, :] = v
        for n, v in enumerate(h2n):
            hbuf[48 + 16 * n:64 + 16 * n, :] = v
        if mode == 0:
            obuf[...] = o[2 * M:]
        elif mode == 1:
            obuf[0:SEG, :] = o[2 * M:]
        else:
            obuf[SEG:2 * SEG, :] = o[2 * M:]

    with _scope("pro"):
        vis, fill = masks(1)
        step(0, 1, vis, fill, False, wo_copy.wait)
        step(1, 1, vis, fill, True)
    xb_copy.start()
    vis, fill = masks(0)
    with _scope("main_a"):
        loop(NA // UA, lambda i: [step(UA * i + u + LAG, 0, vis, fill, u > 0, early=UA * i + u)
                                  for u in range(UA)])
    xb_copy.wait()
    with _scope("conv_e"):
        loop(HB // UI, lambda j: [inv_stage(HB + UI * j + u) for u in range(UI)])
    with _scope("main_b"):
        loop((NSEG - LAG - NA) // UB, lambda i: [step(UB * i + u + LAG + NA, 0, vis, fill, u > 0)
                                                 for u in range(UB)])
    done = (NSEG - 1 - LAG) * SEG
    out_a = pltpu.make_async_copy(out_s.at[0:done, :], out_hbm.at[0:done, :], sem.at[SW + 8])
    out_a.start()
    with _scope("epi"):
        vis, fill = masks(2)
        step(NSEG, 2, vis, fill)
        step(NSEG + 1, 2, *masks(2, 2 * M), True)
    post2(NSEG + LAG)
    out_b = pltpu.make_async_copy(out_s.at[done:S, :], out_hbm.at[done:S, :], sem.at[SW + 9])
    out_b.start()
    out_a.wait()
    out_b.wait()


@jax.jit
def pallas_interleave_layers__memory_aug_recurrent_mem_tr__ssm_conv_h3__prompt_kernel(
    A_x, A_mem0, A_Wq, A_Wk, A_Wv, A_Wo, A_seg_len,
    B_q, B_k, B_v, B_shift_k, B_ssm_k, B_ssm_D,
):
    del A_seg_len, B_q
    assert A_x.shape == (1, S, D) and A_Wq.shape == (D, H, DH)
    hbm = pl.BlockSpec(memory_space=pl.ANY)
    out = pl.pallas_call(
        _kernel,
        out_shape=jax.ShapeDtypeStruct((S, D), BF16),
        in_specs=[hbm] * 11,
        out_specs=hbm,
        scratch_shapes=[
            pltpu.VMEM((S, D), BF16),
            pltpu.VMEM((S, D), BF16),
            pltpu.VMEM((S, D), BF16),
            pltpu.VMEM((HB, D, 2 * TB), BF16),
            pltpu.VMEM((3, D, H, DH), BF16),
            pltpu.VMEM(((H + 1) * WP, 128), U32),
            pltpu.VMEM(((2 * H + 1) * WP, 128), U32),
            pltpu.VMEM((H * DH, D), BF16),
            pltpu.VMEM((NLB, H * DH // 2, 128), U32),
            pltpu.VMEM((TB // 2, TB), U32),
            pltpu.VMEM((2, TB // 2, TB), U32),
            pltpu.VMEM((2, TB // 2, TB), U32),
            pltpu.VMEM((2, NLB, S // 2 + 8, 128), F32),
            pltpu.VMEM((NB, 2, NLB * TB, 128), F32),
            pltpu.VMEM((NB, 3, NLB * TB, 128), F32),
            pltpu.VMEM((NB + 1, 2, NLB * TB, 128), F32),
            pltpu.VMEM((NLB, S + 8, 128), F32),
            pltpu.VMEM((ROWS, D), BF16),
            pltpu.VMEM((2 * SEG, D), F32),
            pltpu.VMEM((4, SEG, D), F32),
            pltpu.VMEM((S, D), BF16),
            pltpu.VMEM((NA * SEG, D), BF16),
            pltpu.VMEM((NQH, NA * SEG, DH), BF16),
            pltpu.VMEM((M, D), BF16),
            pltpu.VMEM((KS, D), BF16),
            pltpu.VMEM((D,), BF16),
            pltpu.SemaphoreType.DMA((HB + HB // 2 + 14,)),
        ],
        compiler_params=pltpu.CompilerParams(vmem_limit_bytes=120 * 1024 * 1024),
    )(A_x.reshape(S, D), A_mem0.reshape(M, D), A_Wq, A_Wk, A_Wv,
      A_Wo.reshape(H * DH, D), B_k.reshape(S, D), B_v.reshape(S, D),
      B_shift_k.T, B_ssm_k, B_ssm_D)
    return out.reshape(1, S, D)
```

```python
import contextlib
import functools
import math

import jax
import jax.numpy as jnp
from jax import lax
import jax.experimental.pallas as pl
import jax.experimental.pallas.tpu as pltpu

F32 = jnp.float32
BF16 = jnp.bfloat16
U32 = jnp.uint32

S = 2048
D = 640
H = 32
DH = 128
M = 8
SEG = 32
NSEG = S // SEG
KS = 4
LAG = 2
ROWS = 2 * M + 2 * SEG
HG = 4
NG = H // HG
NLB = D // 128
TB = 128
NB = S // TB
HB = NB // 2
NPOS = NLB * TB // 8
NA = 20
PPS = 4
UCUT = tuple(range(a, a + 2) for a in range(0, 12, 2)) + (range(12, 16),)
NQH = 32
UA = 2
UB = 3
UI = 4
WP = 324


PROFILE = False


def _scope(name):
    return jax.named_scope(name) if PROFILE else contextlib.nullcontext()


def _ln(x, toks=None):
    m = jnp.mean(x, axis=-1, keepdims=True)
    c = x - m
    v = jnp.mean(c * c, axis=-1, keepdims=True)
    r = lax.rsqrt(v + 1e-5)
    if toks is not None:
        toks.append(jnp.minimum(r, 0.0))
    return c * r


def _r(x):
    return x.astype(BF16).astype(F32)


def _split(x):
    hi = pltpu.bitcast(pltpu.bitcast(x, U32) & jnp.uint32(0xFFFF0000), F32)
    return hi, x - hi


def _pk(x):
    return pltpu.bitcast(x.astype(BF16), U32)


def _upk(w):
    return pltpu.bitcast(w, BF16)


def _basis(r, t):
    b = r & 63
    f = jnp.where(b < 32, 2 * b, 2 * b - 63)
    n = ((2 * f + 1) * t - jnp.where(r >= 64, TB, 0)) & (4 * TB - 1)
    n = jnp.where(n >= 2 * TB, n - 4 * TB, n)
    return jnp.cos(n.astype(F32) * (2.0 * math.pi / (4 * TB)))


def _halves(x):
    w = pltpu.bitcast(x, U32)
    return (pltpu.bitcast(w << 16, F32),
            pltpu.bitcast(w & jnp.uint32(0xFFFF0000), F32))


def _kernel(x_hbm, mem0_hbm, wq_hbm, wk_hbm, wv_hbm, wo_hbm,
            k_hbm, v_hbm, shk_hbm, ssmk_hbm, ssmd_hbm,
            out_hbm,
            x_s, k_s, v_s, ssmk_s, wraw, wt_q, wt_kv, wo_s, wo_t,
            perm_s, fu_s, inv_s, kpad, u_s, kf_s, c_s, y_s,
            hbuf, obuf, x2_s, out_s, hl_s, qh_s, mem0_ref, shk_ref, ssmd_ref,
            sem):
    X0, XH = LAG * SEG, (LAG + NA) * SEG
    SW = HB + HB // 2

    def pair_rows(jp):
        r0 = jp * 2 * TB
        return pl.ds(r0 if isinstance(jp, int) else pl.multiple_of(r0, 2 * TB), 2 * TB)

    def ssmk_copy(jp):
        return pltpu.make_async_copy(ssmk_hbm.at[:, pair_rows(jp)], ssmk_s.at[jp], sem.at[jp])

    def kv_copies(rows, sm):
        return [pltpu.make_async_copy(k_hbm.at[rows, :], k_s.at[rows, :], sm),
                pltpu.make_async_copy(v_hbm.at[rows, :], v_s.at[rows, :], sm)]
    DQ = 192
    wq_early = [pltpu.make_async_copy(wq_hbm.at[n * DQ:(n + 1) * DQ], wraw.at[0, n * DQ:(n + 1) * DQ],
                                      sem.at[SW + 10 + n]) for n in range(2)]
    w_copies = [pltpu.make_async_copy(wq_hbm.at[2 * DQ:], wraw.at[0, 2 * DQ:], sem.at[SW])]
    w_copies += [pltpu.make_async_copy(w.at[n * (D // 2):(n + 1) * (D // 2)],
                                       wraw.at[t, n * (D // 2):(n + 1) * (D // 2)],
                                       sem.at[SW + 11 * n + t])
                 for t, w in ((1, wk_hbm), (2, wv_hbm)) for n in range(2)]
    wo_copy = pltpu.make_async_copy(wo_hbm, wo_s, sem.at[SW + 3])
    late_copies = kv_copies(pl.ds(S // 2, S // 2), sem.at[SW + 4])
    small_copies = [pltpu.make_async_copy(src, dst, sem.at[SW + 5])
                    for src, dst in ((shk_hbm, shk_ref), (ssmd_hbm, ssmd_ref), (mem0_hbm, mem0_ref))]
    XM = XH - 2 * TB
    xa_copy = pltpu.make_async_copy(x_hbm.at[X0:XM, :], x_s.at[X0:XM, :], sem.at[SW + 6])
    late_copies += [pltpu.make_async_copy(x_hbm.at[a:b, :], x_s.at[a:b, :], sem.at[SW + 4])
                    for a, b in ((0, X0), (XM, XH + SEG))]
    xb_copy = pltpu.make_async_copy(x_hbm.at[XH + SEG:, :], x_s.at[XH + SEG:, :], sem.at[SW + 7])
    for c in (small_copies + [ssmk_copy(jp) for jp in range(HB)]
              + [c for jp in range(HB // 2) for c in kv_copies(pair_rows(jp), sem.at[HB + jp])]
              + [xa_copy] + wq_early + [w_copies[0]] + late_copies + w_copies[1:] + [wo_copy]):
        c.start()

    hb = TB // 2
    ri = lax.broadcasted_iota(jnp.int32, (TB, TB), 0)
    ci = lax.broadcasted_iota(jnp.int32, (TB, TB), 1)
    perm_s[...] = _pk(jnp.where(ci == 2 * (ri & 63) + (ri >> 6), 1.0, 0.0))
    tab = _basis(ri, 2 * (ci & 63) + (ci >> 6))
    hi, lo = _split(tab)
    fu_s[0] = _pk(jnp.where(ci < hb, hi, pltpu.roll(lo, hb, 1)))
    fu_s[1] = _pk(jnp.where(ci < hb, pltpu.roll(hi, hb, 1), lo))
    gh, gl = _split(tab.T * (1.0 / TB))
    inv_s[0] = _pk(gh)
    inv_s[1] = _pk(gl)

    for c in small_copies:
        c.wait()
    shk_t = shk_ref[...].astype(F32)
    taps = [[shk_t[j:j + 1, g * 128:(g + 1) * 128] for g in range(NLB)] for j in range(KS)]
    dvec = ssmd_ref[...].astype(F32).reshape(1, D)
    for g in range(NLB):
        kpad[0, g, 0:8, :] = jnp.zeros((8, 128), F32)
        kpad[1, g, 0:8, :] = jnp.zeros((8, 128), F32)
    c_s[0] = jnp.zeros(c_s.shape[1:], F32)
    hbuf[0:16, :] = jnp.concatenate([mem0_ref[...].astype(F32)] * 2, axis=0).astype(BF16)
    obuf[...] = jnp.zeros((2 * SEG, D), F32)
    x2_s[...] = jnp.zeros(x2_s.shape, F32)

    def spectrum(e, o):
        fe = jnp.dot(_upk(fu_s[0]), jnp.concatenate([e, e], axis=0).astype(BF16), preferred_element_type=F32)
        fo = jnp.dot(_upk(fu_s[1]), jnp.concatenate([o, o], axis=0).astype(BF16), preferred_element_type=F32)
        return ((fe[:hb] + fo[:hb], fe[hb:] + fo[hb:]), (fe[:hb] - fo[:hb], fo[hb:] - fe[hb:]))

    def freq_rows(g):
        return slice(g * TB, g * TB + hb), slice(g * TB + hb, (g + 1) * TB)

    def fwd_k(jq):
        def transposed(n):
            if n % 2 == 0:
                ssmk_copy(2 * jq + n // 2).wait()
            blk = ssmk_s[2 * jq + n // 2, :, (n % 2) * TB:(n % 2 + 1) * TB]
            return lax.dot_general(_upk(perm_s[...]), blk, (((1,), (1,)), ((), ())),
                                   preferred_element_type=F32)
        nxt = transposed(0)
        for n in range(4):
            kt = nxt
            if n < 3:
                nxt = transposed(n + 1)
            j = 4 * jq + n
            for g in range(NLB):
                lb = slice(g * 128, (g + 1) * 128)
                for rows, (kr, ki) in zip(freq_rows(g), spectrum(kt[:hb, lb], kt[hb:, lb])):
                    if n == 0:
                        kr = kr + jnp.where(j == 0, dvec[:, lb], 0.0)
                    kf_s[j, 0, rows] = kr
                    kf_s[j, 1, rows] = ki - kr
                    kf_s[j, 2, rows] = kr + ki

    def fwd_u(jq, first):
        if first:
            for jp in (2 * jq, 2 * jq + 1):
                for c in kv_copies(pair_rows(jp), sem.at[HB + jp]):
                    c.wait()
        for j in [4 * jq + n for n in range(4)]:
            r0 = pl.multiple_of(j * TB, TB)
            q0 = pl.multiple_of(j * hb, hb) + 8
            for g in range(NLB):
                lb = slice(g * 128, (g + 1) * 128)
                ke, ko = _halves(k_s[pl.ds(r0, TB), lb])
                ve, vo = _halves(v_s[pl.ds(r0, TB), lb])
                kpad[0, g, pl.ds(q0, hb), :] = ke
                kpad[1, g, pl.ds(q0, hb), :] = ko
                ke1 = kpad[0, g, pl.ds(q0 - 1, hb), :]
                ko1 = kpad[1, g, pl.ds(q0 - 1, hb), :]
                ko2 = kpad[1, g, pl.ds(q0 - 2, hb), :]
                t0, t1, t2, t3 = (taps[t][g] for t in range(KS))
                e = (ke * t0 + ko1 * t1 + ke1 * t2 + ko2 * t3) * ve
                o = (ko * t0 + ke * t1 + ko1 * t2 + ke1 * t3) * vo
                for rows, (ur, ui) in zip(freq_rows(g), spectrum(e, o)):
                    u_s[j, 0, rows] = ur
                    u_s[j, 1, rows] = ui

    def mac_units(row, half):
        rs = pl.ds(row, 8)
        state = {}

        def unit(p, avals, final, tok=None):
            acc = state.setdefault(p, dict(state.get(0, {})))
            for a in avals:
                u = u_s[a, 0, rs] + u_s[a, 1, rs] if p == 0 else u_s[a, p - 1, rs]
                if tok is not None:
                    u = u + tok
                for i in range(max(a, half * HB), half * HB + HB):
                    t = u * kf_s[i - a, p, rs]
                    acc[i] = t if i not in acc else (acc[i] - t if p == 2 else acc[i] + t)
            if final and p:
                for i, v in acc.items():
                    c_s[i + 1, 2 - p, rs] = v

        subs = UCUT if half else (range(HB),)
        return [functools.partial(unit, p, avals, n == len(subs) - 1)
                for p in range(3) for n, avals in enumerate(subs)]

    def inv_stage(i, units=None):
        q = TB // 4
        for g in range(NLB):
            re, im = [], []
            for b in range(4):
                rows = slice(g * TB + b * q, g * TB + (b + 1) * q)
                cr, ci_ = c_s[i + 1, 0, rows], c_s[i + 1, 1, rows]
                pr, pi = c_s[i, 0, rows], c_s[i, 1, rows]
                re.append(cr + pi if b in (0, 3) else cr - pi)
                im.append(ci_ - pr if b in (0, 3) else ci_ + pr)
            pe = jnp.concatenate([re[0] + re[2], re[1] + re[3], im[0] - im[2], im[1] - im[3]], axis=0)
            po = jnp.concatenate([re[0] - re[2], re[1] - re[3], im[0] + im[2], im[1] + im[3]], axis=0)
            for par, pp in enumerate((pe, po)):
                ph, plo = _split(pp)
                gh_, gl_ = (inv_s[n, par * q:(par + 1) * q] for n in range(2))
                y = jnp.dot(_upk(jnp.concatenate([gh_, gl_, gh_], axis=1)),
                            jnp.concatenate([ph, ph, plo], axis=0).astype(BF16),
                            preferred_element_type=F32)
                y_s[g, pl.ds(i * TB + par, hb, stride=2), :] = y
                if units:
                    tok = pltpu.bitcast(jnp.minimum(jnp.abs(y[0:16]), 0.0), U32)
                    for _ in range(3):
                        if units:
                            units.pop(0)(tok)

    def relayout_rows(t, dst, base, dp, tok=None):
        a = pltpu.bitcast(wraw[t, 2 * dp], U32)
        b = pltpu.bitcast(wraw[t, 2 * dp + 1], U32)
        if tok is not None:
            a = a | tok
        dst[pl.ds(base + dp, 16, stride=WP), :] = (a & jnp.uint32(0xFFFF)) | (b << 16)
        dst[pl.ds(base + 16 * WP + dp, 16, stride=WP), :] = (
            (a >> 16) | (b & jnp.uint32(0xFFFF0000)))

    def wslab(t, h):
        s0 = (max(t - 1, 0) * H + (h % 2) * 16 + h // 2) * WP
        return pltpu.bitcast((wt_kv if t else wt_q)[s0:s0 + D // 2, :], BF16)

    def loop(n, fn):
        def body(j, _):
            fn(j)
            return 0
        lax.fori_loop(0, n, body, 0)

    def norm_rows(r0, nr):
        r0 = pl.multiple_of(r0, 16)
        for r in range(0, nr, 16):
            hl_s[pl.ds(r0 + r, 16), :] = _ln(
                x_s[pl.ds(r0 + r + LAG * SEG, 16), :].astype(F32)).astype(BF16)

    def pre_queries(c, t=None):
        per = -(-(D // 4) // NQH)
        for sub in range(2):
            if t is not None:
                half = wraw.at[t, sub * (D // 2):(sub + 1) * (D // 2)]
                pltpu.make_async_copy(half, half, sem.at[SW + 11 * sub + t]).wait()
                base = (t - 1) * (H * WP)
                dp = sub * (D // 4)
            r0 = pl.multiple_of((2 * c + sub) * QR, QR)
            hl = hl_s[pl.ds(r0, QR), :]
            for hd in range(NQH):
                r = jnp.dot(hl, wslab(0, hd), preferred_element_type=F32)
                qh_s[hd, pl.ds(r0, QR), :] = r.astype(BF16)
                if t is not None:
                    tok = pltpu.bitcast(jnp.minimum(jnp.abs(r[0:16]), 0.0), U32)
                    for _ in range(per):
                        if dp < (sub + 1) * (D // 4):
                            relayout_rows(t, wt_kv, base, dp, tok)
                            dp += 1

    nch = NA * SEG // TB
    QR = TB // 2
    with _scope("conv_k"):
        loop(HB // 2, fwd_k)
    with _scope("conv_u"):
        loop(HB // 4, lambda j: fwd_u(j, True))
    with _scope("conv_b"):
        loop(NPOS // 10, lambda j: [u() for n in range(10)
                                    for u in mac_units(pl.multiple_of(80 * j, 16) + 8 * n, 0)])
        xa_copy.wait()

        def inv_first(j):
            part = wraw.at[0, pl.ds(j * DQ, DQ)]
            pltpu.make_async_copy(part, part, sem.at[SW + 10 + j]).wait()
            units = [functools.partial(relayout_rows, 0, wt_q, 0, j * (DQ // 2) + dd)
                     for dd in range(DQ // 2)]
            for u in range(UI):
                inv_stage(UI * j + u, units)
            assert not units
            norm_rows(j * ((XM - X0) // 2), (XM - X0) // 2)
        loop(HB // UI, inv_first)
    with _scope("rel0"):
        w_copies[0].wait()
        loop((D - 2 * DQ) // 64,
             lambda i: [relayout_rows(0, wt_q, 0, DQ + i * 32 + dd) for dd in range(32)])
    with _scope("preq"):
        loop(nch - 2, pre_queries)
    with _scope("conv_c"):
        for c in late_copies:
            c.wait()

        def fwd_u_late(j):
            r0 = pl.multiple_of(j * 16, 16)
            hbuf[pl.ds(16 + r0, 16), :] = _ln(x_s[pl.ds(r0, 16), :].astype(F32)).astype(BF16)
            norm_rows(XM - X0 + j * TB, TB)
            fwd_u(HB // 4 + j, False)
        loop(HB // 4, fwd_u_late)
    with _scope("preq_rel"):
        loop(2, lambda i: pre_queries(i + nch - 2, i + 1))

    scale = DH ** -0.5

    def masks(mode, q0=0):
        rows = ROWS if mode == 0 else ROWS - SEG
        qi = lax.broadcasted_iota(jnp.int32, (rows - q0, 128), 0) + q0
        kj = lax.broadcasted_iota(jnp.int32, (rows - q0, 128), 1)

        def layer_of(i):
            xl = (i - 2 * M) // SEG if mode == 0 else mode - 1
            return jnp.where(i < 2 * M, i // M, xl)
        same = (layer_of(qi) == layer_of(kj)) & (kj < rows)
        vis = same & ((qi < 2 * M) | (qi >= kj))
        fill = jnp.where(same, -1e9 / scale, -jnp.inf).astype(F32)
        return vis, fill

    mem0 = mem0_ref[...].astype(F32)

    def seg_row(seg):
        if isinstance(seg, int):
            return min(max(seg, 0), NSEG - 1) * SEG
        return pl.multiple_of(jnp.clip(seg, 0, NSEG - 1) * SEG, SEG)

    def gate(xa, r0, toks=None):
        y = jnp.concatenate([y_s[g, pl.ds(r0, xa.shape[0]), :] for g in range(NLB)], axis=1)
        return xa + _ln(xa, toks) * y

    def attention(h, vis, fill, chained, before_oproj=None, early=None, due=()):
        q0 = h.shape[0] - vis.shape[0]
        if early is not None:
            hrest = jnp.concatenate([h[:2 * M], h[2 * M + SEG:]], axis=0)
            qrow = pl.multiple_of(early * SEG, SEG)
            units = [u for n in range(PPS)
                     for u in mac_units(pl.multiple_of(early * (8 * PPS), 8 * PPS) + 8 * n, 1)]

        def proj(g):
            res = [[None] * HG for _ in range(3)]
            order = [(t, j) for j in range(HG) for t in range(2)] + [(2, j) for j in range(HG)]

            def operand(t, j):
                pre = early is not None and t == 0 and g * HG + j < NQH
                return pre, hrest if pre else (h if t else h[q0:])

            kc = D - 128
            nsplit = 4 if g == 0 and chained else 0
            part = [jnp.dot(operand(t, j)[1][:, :kc], wslab(t, j)[:kc], preferred_element_type=F32)
                    for t, j in order[:nsplit]]
            for n, (t, j) in enumerate(order):
                hd = g * HG + j
                pre, lhs = operand(t, j)
                if n < nsplit:
                    r = jnp.dot(lhs[:, kc:], wslab(t, hd)[kc:], preferred_element_type=F32) + part[n]
                else:
                    r = jnp.dot(lhs, wslab(t, hd), preferred_element_type=F32)
                if early is not None and units:
                    units.pop(0)(jnp.minimum(jnp.abs(r[0:8]), 0.0))
                if t == 0:
                    r = r.astype(BF16)
                if pre:
                    r = jnp.concatenate([r[:2 * M], qh_s[hd, pl.ds(qrow, SEG), :], r[2 * M:]], axis=0)
                res[t][j] = r
            return res

        def pad(kv):
            return jnp.concatenate([kv, jnp.zeros((128 - kv.shape[0], DH), F32)], axis=0).astype(BF16)

        def probs(qkv, g):
            scs = [lax.dot_general(qkv[0][j], pad(qkv[1][j]), (((1,), (1,)), ((), ())),
                                   preferred_element_type=F32) for j in range(HG)]
            ps = []
            for sc in scs:
                sc = jnp.where(vis, sc, fill)
                e = jnp.exp2((sc - jnp.max(sc, axis=-1, keepdims=True)) * (scale * math.log2(math.e)))
                den = jnp.sum(e, axis=-1, keepdims=True)
                if not ps and g >= NG - len(due):
                    e = jnp.concatenate([e[:16] + due[g - NG + len(due)], e[16:]], axis=0)
                r = pl.reciprocal(den, approx=True)
                r = r * (2.0 - den * r)
                ps.append((e * r).astype(BF16))
            return ps

        def oproj(os_, h0):
            oc = jnp.concatenate(os_, axis=1).astype(BF16)
            k0, k1 = h0 * DH, (h0 + len(os_)) * DH
            res = []
            for n in range(NLB):
                if before_oproj is not None:
                    w = wo_s[k0:k1, n * 128:(n + 1) * 128]
                    wo_t[n, k0 // 2:k1 // 2, :] = pltpu.bitcast(w, U32)
                else:
                    w = pltpu.bitcast(wo_t[n, k0 // 2:k1 // 2, :], BF16)
                res.append(jnp.dot(oc, w, preferred_element_type=F32))
            return res

        heads = []
        qkv = proj(0)
        oa = None
        for g in range(NG):
            ps = probs(qkv, g)
            vs = qkv[2]
            if g + 1 < NG:
                qkv = proj(g + 1)
            else:
                if before_oproj is not None:
                    before_oproj()
                oa = oproj(heads[:H // 2], 0)
            heads += [jnp.dot(ps[j], pad(vs[j]), preferred_element_type=F32)
                      for j in range(HG)]
        assert early is None or not units
        ob = oproj(heads[H // 2:], H // 2)
        return jnp.concatenate([b + a for a, b in zip(oa, ob)], axis=1)

    def post2(s, toks=None):
        r3 = seg_row(s - 1 - LAG)
        for r in (0, 16):
            xc = _r(x2_s[(s + 4 - 1 - LAG) % 4, r:r + 16] + obuf[SEG + r:SEG + r + 16, :])
            out_s[pl.ds(r3 + r, 16), :] = gate(xc, r3 + r, toks).astype(BF16)

    def step(s, mode, vis, fill, chained=False, before_oproj=None, early=None):
        if mode == 0:
            h = hbuf[...]
        elif mode == 1:
            h = hbuf[0:48, :]
        else:
            live = lax.broadcasted_iota(jnp.int32, (2 * M, D), 0) >= M
            mem = jnp.where(live, hbuf[0:16, :].astype(F32), 0.0).astype(BF16)
            h = jnp.concatenate([mem, hbuf[48:80, :]], axis=0)
        toks = []
        if mode != 1:
            post2(s, toks)
        if isinstance(s, int) and s == NSEG + LAG - 1:
            obuf[SEG:2 * SEG, :] = attention(h, vis, fill, chained, due=toks)
            return
        r1 = seg_row(s - 1)
        rn = seg_row(s + 1)
        h1n, h2n = [], []
        for r in (0, 16):
            xa = _r(x_s[pl.ds(r1 + r, 16), :].astype(F32) + obuf[r:r + 16, :])
            xb2 = _r(gate(xa, r1 + r))
            h2n.append(_ln(xb2, toks).astype(BF16))
            x2_s[(s + 4 - 1) % 4, r:r + 16] = xb2
        if mode != 2:
            for r in (0, 16):
                h1n.append(_ln(x_s[pl.ds(rn + r, 16), :].astype(F32), toks).astype(BF16))

        o = attention(h, vis, fill, chained, before_oproj, early, toks)

        mem2 = mem0 if mode == 1 else o[M:2 * M]
        hbuf[0:16, :] = jnp.concatenate([o[0:M], mem2], axis=0).astype(BF16)
        for n, v in enumerate(h1n):
            hbuf[16 + 16 * n:32 + 16 * n, :] = v
        for n, v in enumerate(h2n):
            hbuf[48 + 16 * n:64 + 16 * n, :] = v
        if mode == 0:
            obuf[...] = o[2 * M:]
        elif mode == 1:
            obuf[0:SEG, :] = o[2 * M:]
        else:
            obuf[SEG:2 * SEG, :] = o[2 * M:]

    with _scope("pro"):
        vis, fill = masks(1)
        step(0, 1, vis, fill, False, wo_copy.wait)
        step(1, 1, vis, fill, True)
    xb_copy.start()
    vis, fill = masks(0)
    with _scope("main_a"):
        loop(NA // UA, lambda i: [step(UA * i + u + LAG, 0, vis, fill, u > 0, early=UA * i + u)
                                  for u in range(UA)])
    xb_copy.wait()
    with _scope("conv_e"):
        loop(HB // UI, lambda j: [inv_stage(HB + UI * j + u) for u in range(UI)])
    with _scope("main_b"):
        loop((NSEG - LAG - NA) // UB, lambda i: [step(UB * i + u + LAG + NA, 0, vis, fill, u > 0)
                                                 for u in range(UB)])
    done = (NSEG - 1 - LAG) * SEG
    out_a = pltpu.make_async_copy(out_s.at[0:done, :], out_hbm.at[0:done, :], sem.at[SW + 8])
    out_a.start()
    with _scope("epi"):
        vis, fill = masks(2)
        step(NSEG, 2, vis, fill)
        step(NSEG + 1, 2, *masks(2, 2 * M), True)
    post2(NSEG + LAG)
    out_b = pltpu.make_async_copy(out_s.at[done:S, :], out_hbm.at[done:S, :], sem.at[SW + 9])
    out_b.start()
    out_a.wait()
    out_b.wait()


@jax.jit
def pallas_interleave_layers__memory_aug_recurrent_mem_tr__ssm_conv_h3__prompt_kernel(
    A_x, A_mem0, A_Wq, A_Wk, A_Wv, A_Wo, A_seg_len,
    B_q, B_k, B_v, B_shift_k, B_ssm_k, B_ssm_D,
):
    del A_seg_len, B_q
    assert A_x.shape == (1, S, D) and A_Wq.shape == (D, H, DH)
    hbm = pl.BlockSpec(memory_space=pl.ANY)
    out = pl.pallas_call(
        _kernel,
        out_shape=jax.ShapeDtypeStruct((S, D), BF16),
        in_specs=[hbm] * 11,
        out_specs=hbm,
        scratch_shapes=[
            pltpu.VMEM((S, D), BF16),
            pltpu.VMEM((S, D), BF16),
            pltpu.VMEM((S, D), BF16),
            pltpu.VMEM((HB, D, 2 * TB), BF16),
            pltpu.VMEM((3, D, H, DH), BF16),
            pltpu.VMEM(((H + 1) * WP, 128), U32),
            pltpu.VMEM(((2 * H + 1) * WP, 128), U32),
            pltpu.VMEM((H * DH, D), BF16),
            pltpu.VMEM((NLB, H * DH // 2, 128), U32),
            pltpu.VMEM((TB // 2, TB), U32),
            pltpu.VMEM((2, TB // 2, TB), U32),
            pltpu.VMEM((2, TB // 2, TB), U32),
            pltpu.VMEM((2, NLB, S // 2 + 8, 128), F32),
            pltpu.VMEM((NB, 2, NLB * TB, 128), F32),
            pltpu.VMEM((NB, 3, NLB * TB, 128), F32),
            pltpu.VMEM((NB + 1, 2, NLB * TB, 128), F32),
            pltpu.VMEM((NLB, S + 8, 128), F32),
            pltpu.VMEM((ROWS, D), BF16),
            pltpu.VMEM((2 * SEG, D), F32),
            pltpu.VMEM((4, SEG, D), F32),
            pltpu.VMEM((S, D), BF16),
            pltpu.VMEM((NA * SEG, D), BF16),
            pltpu.VMEM((NQH, NA * SEG, DH), BF16),
            pltpu.VMEM((M, D), BF16),
            pltpu.VMEM((KS, D), BF16),
            pltpu.VMEM((D,), BF16),
            pltpu.SemaphoreType.DMA((HB + HB // 2 + 14,)),
        ],
        compiler_params=pltpu.CompilerParams(vmem_limit_bytes=120 * 1024 * 1024),
    )(A_x.reshape(S, D), A_mem0.reshape(M, D), A_Wq, A_Wk, A_Wv,
      A_Wo.reshape(H * DH, D), B_k.reshape(S, D), B_v.reshape(S, D),
      B_shift_k.T, B_ssm_k, B_ssm_D)
    return out.reshape(1, S, D)
```

```python
import contextlib
import functools
import math

import jax
import jax.numpy as jnp
from jax import lax
import jax.experimental.pallas as pl
import jax.experimental.pallas.tpu as pltpu

F32 = jnp.float32
BF16 = jnp.bfloat16
U32 = jnp.uint32

S = 2048
D = 640
H = 32
DH = 128
M = 8
SEG = 32
NSEG = S // SEG
KS = 4
LAG = 2
ROWS = 2 * M + 2 * SEG
HG = 4
NG = H // HG
NLB = D // 128
TB = 128
NB = S // TB
HB = NB // 2
NPOS = NLB * TB // 8
NA = 20
PPS = 4
UCUT = tuple(range(a, a + 2) for a in range(0, 12, 2)) + (range(12, 16),)
NQH = 32
UA = 2
UB = 3
UI = 4
WP = 324


PROFILE = False


def _scope(name):
    return jax.named_scope(name) if PROFILE else contextlib.nullcontext()


def _ln(x, toks=None):
    m = jnp.mean(x, axis=-1, keepdims=True)
    c = x - m
    v = jnp.mean(c * c, axis=-1, keepdims=True)
    r = lax.rsqrt(v + 1e-5)
    if toks is not None:
        toks.append(jnp.minimum(r, 0.0))
    return c * r


def _r(x):
    return x.astype(BF16).astype(F32)


def _split(x):
    hi = pltpu.bitcast(pltpu.bitcast(x, U32) & jnp.uint32(0xFFFF0000), F32)
    return hi, x - hi


def _pk(x):
    return pltpu.bitcast(x.astype(BF16), U32)


def _upk(w):
    return pltpu.bitcast(w, BF16)


def _basis(r, t):
    b = r & 63
    f = jnp.where(b < 32, 2 * b, 2 * b - 63)
    n = ((2 * f + 1) * t - jnp.where(r >= 64, TB, 0)) & (4 * TB - 1)
    n = jnp.where(n >= 2 * TB, n - 4 * TB, n)
    return jnp.cos(n.astype(F32) * (2.0 * math.pi / (4 * TB)))


def _halves(x):
    w = pltpu.bitcast(x, U32)
    return (pltpu.bitcast(w << 16, F32),
            pltpu.bitcast(w & jnp.uint32(0xFFFF0000), F32))


def _kernel(x_hbm, mem0_hbm, wq_hbm, wk_hbm, wv_hbm, wo_hbm,
            k_hbm, v_hbm, shk_hbm, ssmk_hbm, ssmd_hbm,
            out_hbm,
            x_s, wt_q, wt_kv, wo_s, wo_t,
            perm_s, fu_s, inv_s, u_s, kf_s, c_s, y_s,
            hbuf, sbuf, obuf, x2_s, out_s, qh_s, mem0_ref, shk_ref, ssmd_ref,
            sem):
    X0, XH = LAG * SEG, (LAG + NA) * SEG
    SW = HB + HB // 2
    hb = TB // 2
    wo_copy = pltpu.make_async_copy(wo_hbm, wo_s, sem.at[SW + 3])
    xb_copy = pltpu.make_async_copy(x_hbm.at[XH + SEG:, :], x_s.at[XH + SEG:, :], sem.at[SW + 7])

    def mac_units(row, half):
        rs = pl.ds(row, 8)
        state = {}

        def unit(p, avals, final, tok=None):
            acc = state.setdefault(p, dict(state.get(0, {})))
            for a in avals:
                u = u_s[a, 0, rs] + u_s[a, 1, rs] if p == 0 else u_s[a, p - 1, rs]
                if tok is not None:
                    u = u + tok
                for i in range(max(a, half * HB), half * HB + HB):
                    t = u * kf_s[i - a, p, rs]
                    acc[i] = t if i not in acc else (acc[i] - t if p == 2 else acc[i] + t)
            if final and p:
                for i, v in acc.items():
                    c_s[i + 1, 2 - p, rs] = v

        subs = UCUT if half else (range(HB),)
        return [functools.partial(unit, p, avals, n == len(subs) - 1)
                for p in range(3) for n, avals in enumerate(subs)]

    def inv_stage(i, units=None):
        q = TB // 4
        for g in range(NLB):
            re, im = [], []
            for b in range(4):
                rows = slice(g * TB + b * q, g * TB + (b + 1) * q)
                cr, ci_ = c_s[i + 1, 0, rows], c_s[i + 1, 1, rows]
                pr, pi = c_s[i, 0, rows], c_s[i, 1, rows]
                re.append(cr + pi if b in (0, 3) else cr - pi)
                im.append(ci_ - pr if b in (0, 3) else ci_ + pr)
            pe = jnp.concatenate([re[0] + re[2], re[1] + re[3], im[0] - im[2], im[1] - im[3]], axis=0)
            po = jnp.concatenate([re[0] - re[2], re[1] - re[3], im[0] + im[2], im[1] + im[3]], axis=0)
            for par, pp in enumerate((pe, po)):
                ph, plo = _split(pp)
                gh_, gl_ = (inv_s[n, par * q:(par + 1) * q] for n in range(2))
                y = jnp.dot(_upk(jnp.concatenate([gh_, gl_, gh_], axis=1)),
                            jnp.concatenate([ph, ph, plo], axis=0).astype(BF16),
                            preferred_element_type=F32)
                y_s[g, pl.ds(i * TB + par, hb, stride=2), :] = y
                if units:
                    tok = pltpu.bitcast(jnp.minimum(jnp.abs(y[0:16]), 0.0), U32)
                    for _ in range(3):
                        if units:
                            units.pop(0)(tok)

    def wslab(t, h):
        s0 = (max(t - 1, 0) * H + (h % 2) * 16 + h // 2) * WP
        return pltpu.bitcast((wt_kv if t else wt_q)[s0:s0 + D // 2, :], BF16)

    def loop(n, fn):
        def body(j, _):
            fn(j)
            return 0
        lax.fori_loop(0, n, body, 0)

    def phase0(k_s, v_s, ssmk_s, wraw, kpad, hl_s):

        def pair_rows(jp):
            r0 = jp * 2 * TB
            return pl.ds(r0 if isinstance(jp, int) else pl.multiple_of(r0, 2 * TB), 2 * TB)

        def ssmk_copy(jp):
            return pltpu.make_async_copy(ssmk_hbm.at[:, pair_rows(jp)], ssmk_s.at[jp], sem.at[jp])

        def kv_copies(rows, sm):
            return [pltpu.make_async_copy(k_hbm.at[rows, :], k_s.at[rows, :], sm),
                    pltpu.make_async_copy(v_hbm.at[rows, :], v_s.at[rows, :], sm)]
        DQ = 192
        wq_early = [pltpu.make_async_copy(wq_hbm.at[n * DQ:(n + 1) * DQ], wraw.at[0, n * DQ:(n + 1) * DQ],
                                          sem.at[SW + 10 + n]) for n in range(2)]
        w_copies = [pltpu.make_async_copy(wq_hbm.at[2 * DQ:], wraw.at[0, 2 * DQ:], sem.at[SW])]
        w_copies += [pltpu.make_async_copy(w.at[n * (D // 2):(n + 1) * (D // 2)],
                                           wraw.at[t, n * (D // 2):(n + 1) * (D // 2)],
                                           sem.at[SW + 11 * n + t])
                     for t, w in ((1, wk_hbm), (2, wv_hbm)) for n in range(2)]
        late_copies = kv_copies(pl.ds(S // 2, S // 2), sem.at[SW + 4])
        small_copies = [pltpu.make_async_copy(src, dst, sem.at[SW + 5])
                        for src, dst in ((shk_hbm, shk_ref), (ssmd_hbm, ssmd_ref), (mem0_hbm, mem0_ref))]
        XM = XH - 2 * TB
        xa_copy = pltpu.make_async_copy(x_hbm.at[X0:XM, :], x_s.at[X0:XM, :], sem.at[SW + 6])
        late_copies += [pltpu.make_async_copy(x_hbm.at[a:b, :], x_s.at[a:b, :], sem.at[SW + 4])
                        for a, b in ((0, X0), (XM, XH + SEG))]
        for c in (small_copies + [ssmk_copy(jp) for jp in range(HB)]
                  + [c for jp in range(HB // 2) for c in kv_copies(pair_rows(jp), sem.at[HB + jp])]
                  + [xa_copy] + wq_early + [w_copies[0]] + late_copies + w_copies[1:] + [wo_copy]):
            c.start()

        ri = lax.broadcasted_iota(jnp.int32, (TB, TB), 0)
        ci = lax.broadcasted_iota(jnp.int32, (TB, TB), 1)
        perm_s[...] = _pk(jnp.where(ci == 2 * (ri & 63) + (ri >> 6), 1.0, 0.0))
        tab = _basis(ri, 2 * (ci & 63) + (ci >> 6))
        hi, lo = _split(tab)
        fu_s[0] = _pk(jnp.where(ci < hb, hi, pltpu.roll(lo, hb, 1)))
        fu_s[1] = _pk(jnp.where(ci < hb, pltpu.roll(hi, hb, 1), lo))
        gh, gl = _split(tab.T * (1.0 / TB))
        inv_s[0] = _pk(gh)
        inv_s[1] = _pk(gl)

        for c in small_copies:
            c.wait()
        shk_t = shk_ref[...].astype(F32)
        taps = [[shk_t[j:j + 1, g * 128:(g + 1) * 128] for g in range(NLB)] for j in range(KS)]
        dvec = ssmd_ref[...].astype(F32).reshape(1, D)
        for g in range(NLB):
            kpad[0, g, 0:8, :] = jnp.zeros((8, 128), F32)
            kpad[1, g, 0:8, :] = jnp.zeros((8, 128), F32)
        c_s[0] = jnp.zeros(c_s.shape[1:], F32)
        hbuf[0:16, :] = jnp.concatenate([mem0_ref[...].astype(F32)] * 2, axis=0).astype(BF16)
        obuf[...] = jnp.zeros((2 * SEG, D), F32)
        x2_s[...] = jnp.zeros(x2_s.shape, F32)

        def spectrum(e, o):
            fe = jnp.dot(_upk(fu_s[0]), jnp.concatenate([e, e], axis=0).astype(BF16), preferred_element_type=F32)
            fo = jnp.dot(_upk(fu_s[1]), jnp.concatenate([o, o], axis=0).astype(BF16), preferred_element_type=F32)
            return ((fe[:hb] + fo[:hb], fe[hb:] + fo[hb:]), (fe[:hb] - fo[:hb], fo[hb:] - fe[hb:]))

        def freq_rows(g):
            return slice(g * TB, g * TB + hb), slice(g * TB + hb, (g + 1) * TB)

        def fwd_k(jq):
            def transposed(n):
                if n % 2 == 0:
                    ssmk_copy(2 * jq + n // 2).wait()
                blk = ssmk_s[2 * jq + n // 2, :, (n % 2) * TB:(n % 2 + 1) * TB]
                return lax.dot_general(_upk(perm_s[...]), blk, (((1,), (1,)), ((), ())),
                                       preferred_element_type=F32)
            nxt = transposed(0)
            for n in range(4):
                kt = nxt
                if n < 3:
                    nxt = transposed(n + 1)
                j = 4 * jq + n
                for g in range(NLB):
                    lb = slice(g * 128, (g + 1) * 128)
                    for rows, (kr, ki) in zip(freq_rows(g), spectrum(kt[:hb, lb], kt[hb:, lb])):
                        if n == 0:
                            kr = kr + jnp.where(j == 0, dvec[:, lb], 0.0)
                        kf_s[j, 0, rows] = kr
                        kf_s[j, 1, rows] = ki - kr
                        kf_s[j, 2, rows] = kr + ki

        def fwd_u(jq, first):
            if first:
                for jp in (2 * jq, 2 * jq + 1):
                    for c in kv_copies(pair_rows(jp), sem.at[HB + jp]):
                        c.wait()
            for j in [4 * jq + n for n in range(4)]:
                r0 = pl.multiple_of(j * TB, TB)
                q0 = pl.multiple_of(j * hb, hb) + 8
                for g in range(NLB):
                    lb = slice(g * 128, (g + 1) * 128)
                    ke, ko = _halves(k_s[pl.ds(r0, TB), lb])
                    ve, vo = _halves(v_s[pl.ds(r0, TB), lb])
                    kpad[0, g, pl.ds(q0, hb), :] = ke
                    kpad[1, g, pl.ds(q0, hb), :] = ko
                    ke1 = kpad[0, g, pl.ds(q0 - 1, hb), :]
                    ko1 = kpad[1, g, pl.ds(q0 - 1, hb), :]
                    ko2 = kpad[1, g, pl.ds(q0 - 2, hb), :]
                    t0, t1, t2, t3 = (taps[t][g] for t in range(KS))
                    e = (ke * t0 + ko1 * t1 + ke1 * t2 + ko2 * t3) * ve
                    o = (ko * t0 + ke * t1 + ko1 * t2 + ke1 * t3) * vo
                    for rows, (ur, ui) in zip(freq_rows(g), spectrum(e, o)):
                        u_s[j, 0, rows] = ur
                        u_s[j, 1, rows] = ui

        def relayout_rows(t, dst, base, dp, tok=None):
            a = pltpu.bitcast(wraw[t, 2 * dp], U32)
            b = pltpu.bitcast(wraw[t, 2 * dp + 1], U32)
            if tok is not None:
                a = a | tok
            dst[pl.ds(base + dp, 16, stride=WP), :] = (a & jnp.uint32(0xFFFF)) | (b << 16)
            dst[pl.ds(base + 16 * WP + dp, 16, stride=WP), :] = (
                (a >> 16) | (b & jnp.uint32(0xFFFF0000)))

        def norm_rows(r0, nr):
            r0 = pl.multiple_of(r0, 16)
            for r in range(0, nr, 16):
                hl_s[pl.ds(r0 + r, 16), :] = _ln(
                    x_s[pl.ds(r0 + r + LAG * SEG, 16), :].astype(F32)).astype(BF16)

        def pre_queries(c, t=None):
            per = -(-(D // 4) // NQH)
            for sub in range(2):
                if t is not None:
                    half = wraw.at[t, sub * (D // 2):(sub + 1) * (D // 2)]
                    pltpu.make_async_copy(half, half, sem.at[SW + 11 * sub + t]).wait()
                    base = (t - 1) * (H * WP)
                    dp = sub * (D // 4)
                r0 = pl.multiple_of((2 * c + sub) * QR, QR)
                hl = hl_s[pl.ds(r0, QR), :]
                for hd in range(NQH):
                    r = jnp.dot(hl, wslab(0, hd), preferred_element_type=F32)
                    qh_s[hd, pl.ds(r0, QR), :] = r.astype(BF16)
                    if t is not None:
                        tok = pltpu.bitcast(jnp.minimum(jnp.abs(r[0:16]), 0.0), U32)
                        for _ in range(per):
                            if dp < (sub + 1) * (D // 4):
                                relayout_rows(t, wt_kv, base, dp, tok)
                                dp += 1

        nch = NA * SEG // TB
        QR = TB // 2
        with _scope("conv_k"):
            loop(HB // 2, fwd_k)
        with _scope("conv_u"):
            loop(HB // 4, lambda j: fwd_u(j, True))
        with _scope("conv_b"):
            loop(NPOS // 10, lambda j: [u() for n in range(10)
                                        for u in mac_units(pl.multiple_of(80 * j, 16) + 8 * n, 0)])
            xa_copy.wait()

            def inv_first(j):
                part = wraw.at[0, pl.ds(j * DQ, DQ)]
                pltpu.make_async_copy(part, part, sem.at[SW + 10 + j]).wait()
                units = [functools.partial(relayout_rows, 0, wt_q, 0, j * (DQ // 2) + dd)
                         for dd in range(DQ // 2)]
                for u in range(UI):
                    inv_stage(UI * j + u, units)
                assert not units
                norm_rows(j * ((XM - X0) // 2), (XM - X0) // 2)
            loop(HB // UI, inv_first)
        with _scope("rel0"):
            w_copies[0].wait()
            loop((D - 2 * DQ) // 64,
                 lambda i: [relayout_rows(0, wt_q, 0, DQ + i * 32 + dd) for dd in range(32)])
        with _scope("preq"):
            loop(nch - 2, pre_queries)
        with _scope("conv_c"):
            for c in late_copies:
                c.wait()

            def fwd_u_late(j):
                r0 = pl.multiple_of(j * 16, 16)
                hbuf[pl.ds(16 + r0, 16), :] = _ln(x_s[pl.ds(r0, 16), :].astype(F32)).astype(BF16)
                norm_rows(XM - X0 + j * TB, TB)
                fwd_u(HB // 4 + j, False)
            loop(HB // 4, fwd_u_late)
        with _scope("preq_rel"):
            loop(2, lambda i: pre_queries(i + nch - 2, i + 1))

    pl.run_scoped(
        phase0,
        pltpu.VMEM((S, D), BF16),
        pltpu.VMEM((S, D), BF16),
        pltpu.VMEM((HB, D, 2 * TB), BF16),
        pltpu.VMEM((3, D, H, DH), BF16),
        pltpu.VMEM((2, NLB, S // 2 + 8, 128), F32),
        pltpu.VMEM((NA * SEG, D), BF16),
    )

    def phase1(cq, ckv, co):
        scale = DH ** -0.5

        def masks(mode, q0=0):
            rows = ROWS if mode == 0 else ROWS - SEG
            qi = lax.broadcasted_iota(jnp.int32, (rows - q0, 128), 0) + q0
            kj = lax.broadcasted_iota(jnp.int32, (rows - q0, 128), 1)

            def layer_of(i):
                xl = (i - 2 * M) // SEG if mode == 0 else mode - 1
                return jnp.where(i < 2 * M, i // M, xl)
            same = (layer_of(qi) == layer_of(kj)) & (kj < rows)
            vis = same & ((qi < 2 * M) | (qi >= kj))
            fill = jnp.where(same, -1e9 / scale, -jnp.inf).astype(F32)
            return vis, fill

        mem0 = mem0_ref[...].astype(F32)

        def seg_row(seg):
            if isinstance(seg, int):
                return min(max(seg, 0), NSEG - 1) * SEG
            return pl.multiple_of(jnp.clip(seg, 0, NSEG - 1) * SEG, SEG)

        def gate(xa, r0, toks=None):
            y = jnp.concatenate([y_s[g, pl.ds(r0, xa.shape[0]), :] for g in range(NLB)], axis=1)
            return xa + _ln(xa, toks) * y

        KH = 256

        def mm(a, b):
            return jnp.dot(a, b, preferred_element_type=F32)

        def row_sums(x1, x2, m_a, m_b):
            (a11, a12), (a21, a22) = x1, x2
            ms = m_a + m_b
            cat = lambda u, v: jnp.concatenate([u, v], axis=0)
            return [a11 + a22, cat(ms, a21 + a22), cat(m_a, a11), cat(m_b, a22),
                    cat(ms, a11 + a12), a21 - a11, a12 - a22]

        def combine(m):
            m1, m2, m3, m4, m5, m16, m17 = m
            m24, m35 = m2 + m4, m3 + m5
            r = 2 * M
            return (jnp.concatenate([m24[:r], m17 + m4[r:] - m5[r:], m24[r:]], axis=0),
                    jnp.concatenate([m35[:r], m35[r:], m16 - m2[r:] + m3[r:]], axis=0))

        def sums_of(b11, b12, b21, b22):
            b11, b12, b21, b22 = (_upk(b).astype(F32) for b in (b11, b12, b21, b22))
            return [_pk(v) for v in (b11 + b22, b12 - b22, b21 - b11, b11 + b12, b21 + b22)]

        def slab_rows(t, h):
            return (wt_kv if t else wt_q), (max(t - 1, 0) * H + (h % 2) * 16 + h // 2) * WP

        def qkv_sum_unit(t, pr, r0, nr, tok=None):
            src, s1 = slab_rows(t, 0)
            s1 = s1 + pr * WP
            s2 = s1 + 16 * WP
            b11 = src[pl.ds(s1 + r0, nr), :]
            if tok is not None:
                b11 = b11 | pltpu.bitcast(tok, U32)
            sm = sums_of(b11, src[pl.ds(s2 + r0, nr), :],
                         src[pl.ds(s1 + 128 + r0, nr), :], src[pl.ds(s2 + 128 + r0, nr), :])
            dst, d0 = (ckv if t else cq), (max(t - 1, 0) * 16 + pr) * 640
            for n, v in enumerate(sm):
                dst[pl.ds(d0 + n * 128 + r0, nr), :] = v

        def o_sum_unit(np_, i, r0, nr, tok=None):
            ka = ((i // 2) * 4 + i % 2) * 64 + r0
            b11 = wo_t[2 * np_, pl.ds(ka, nr), :]
            if tok is not None:
                b11 = b11 | pltpu.bitcast(tok, U32)
            sm = sums_of(b11, wo_t[2 * np_ + 1, pl.ds(ka, nr), :],
                         wo_t[2 * np_, pl.ds(ka + 128, nr), :], wo_t[2 * np_ + 1, pl.ds(ka + 128, nr), :])
            for n, v in enumerate(sm):
                co[pl.ds((np_ * 5 + n) * 1024 + i * 64 + r0, nr), :] = v

        def attention(h, vis, fill, chained, before_oproj=None, early=None, due=(), fast=False,
                      units=()):
            q0 = h.shape[0] - vis.shape[0]
            units = list(units)
            per = -(-len(units) // 96)
            r = 2 * M
            if early is not None:
                hrest = jnp.concatenate([h[:r], h[r + SEG:]], axis=0)
                qrow = pl.multiple_of(early * SEG, SEG)
            if fast:
                sb = sbuf[...]
                ms = sb[5 * SEG:]
                cat = lambda u, v: jnp.concatenate([u, v], axis=0)
                lhs = [sb[0:SEG], cat(ms, sb[SEG:2 * SEG]), h[:r + SEG, :KH],
                       cat(h[:r, KH:2 * KH], h[r + SEG:, KH:2 * KH]), cat(ms, sb[2 * SEG:3 * SEG]),
                       sb[3 * SEG:4 * SEG], sb[4 * SEG:5 * SEG]]

            def feed(x):
                if units:
                    tok = jnp.minimum(jnp.abs(x[0:16]), 0.0)
                    for u in units[:per]:
                        u(tok)
                    del units[:per]

            def proj(g):
                res = [[None] * HG for _ in range(3)]
                plain, pairs = [], []
                for t, j in [(t, j) for j in range(HG) for t in range(2)] + [(2, j) for j in range(HG)]:
                    pre = early is not None and t == 0 and g * HG + j < NQH
                    if pre or not fast:
                        plain.append((t, j, pre))
                    elif j % 2 == 0:
                        pairs.append((t, j))

                def csum(t, j, n):
                    d0 = (max(t - 1, 0) * 16 + (g * HG + j) // 2) * 640 + n * 128
                    return _upk((ckv if t else cq)[d0:d0 + 128, :])

                def free_part(t, j):
                    m1 = mm(lhs[0], csum(t, j, 0))
                    return m1, mm(lhs[5], csum(t, j, 3)) + m1, mm(lhs[6], csum(t, j, 4)) + m1

                def do_pair(t, j, fp):
                    w1, w2 = wslab(t, g * HG + j), wslab(t, g * HG + j + 1)
                    m1, m16, m17 = fp
                    feed(m16)
                    m = [m1, mm(lhs[1], w1[:KH]), mm(lhs[2], csum(t, j, 1)), mm(lhs[3], csum(t, j, 2)),
                         mm(lhs[4], w2[KH:2 * KH]), m16, m17]
                    feed(m[4])
                    for n, (c, w) in enumerate(zip(combine(m), (w1, w2))):
                        c = mm(h[:, 2 * KH:], w[2 * KH:]) + c
                        res[t][j + n] = c.astype(BF16) if t == 0 else c

                def do_plain(t, j, pre, part=None):
                    hd = g * HG + j
                    x = hrest if pre else (h if t else h[q0:])
                    if part is None:
                        y = mm(x, wslab(t, hd))
                    else:
                        y = mm(x[:, 2 * KH:], wslab(t, hd)[2 * KH:]) + part
                    feed(y)
                    if t == 0:
                        y = y.astype(BF16)
                    if pre:
                        y = jnp.concatenate([y[:r], qh_s[hd, pl.ds(qrow, SEG), :], y[r:]], axis=0)
                    res[t][j] = y

                first = g == 0 and chained
                fps = [free_part(t, j) for t, j in pairs] if first else None
                nsplit = 4 if first and not fast else 0
                parts = [mm((h if t else h[q0:])[:, :2 * KH], wslab(t, j)[:2 * KH])
                         for t, j, _ in plain[:nsplit]]
                jobs = sorted([(t, j, None) for t, j in pairs] + plain,
                              key=lambda x: (x[0] == 2, x[1], x[0]))
                np_ = 0
                for t, j, pre in jobs:
                    if pre is None:
                        do_pair(t, j, fps[pairs.index((t, j))] if first else free_part(t, j))
                    else:
                        do_plain(t, j, pre, parts[np_] if np_ < nsplit else None)
                        np_ += 1
                return res

            def pad(kv):
                return jnp.concatenate([kv, jnp.zeros((128 - kv.shape[0], DH), F32)],
                                       axis=0).astype(BF16)

            def probs(qkv, g):
                scs = [lax.dot_general(qkv[0][j], pad(qkv[1][j]), (((1,), (1,)), ((), ())),
                                       preferred_element_type=F32) for j in range(HG)]
                ps = []
                for sc in scs:
                    sc = jnp.where(vis, sc, fill)
                    e = jnp.exp2((sc - jnp.max(sc, axis=-1, keepdims=True))
                                 * (scale * math.log2(math.e)))
                    den = jnp.sum(e, axis=-1, keepdims=True)
                    if not ps and g >= NG - len(due):
                        e = jnp.concatenate([e[:16] + due[g - NG + len(due)], e[16:]], axis=0)
                    rc = pl.reciprocal(den, approx=True)
                    rc = rc * (2.0 - den * rc)
                    ps.append((e * rc).astype(BF16))
                return ps

            def oproj(os_, h0, acc):
                ext = lambda n, y: y if acc is None else y + acc[n]
                oc = jnp.concatenate(os_, axis=1).astype(BF16)
                k0, k1 = h0 * DH, (h0 + len(os_)) * DH
                res = []
                if fast:
                    ia = [n for n in range(len(os_)) if n % 4 < 2]
                    oa_, ob_ = (jnp.concatenate([os_[n + d] for n in ia], axis=1) for d in (0, 2))
                    ls = [v.astype(BF16) for v in row_sums(
                        (oa_[r:r + SEG], ob_[r:r + SEG]), (oa_[r + SEG:], ob_[r + SEG:]),
                        oa_[:r], ob_[:r])]
                    for np_ in range(2):
                        def cs(n):
                            d0 = (np_ * 5 + n) * 1024 + h0 * 32
                            return _upk(co[d0:d0 + len(os_) * 32, :])

                        def pw(n, d):
                            return _upk(jnp.concatenate(
                                [wo_t[n, (h0 + i + d) * 64:(h0 + i + d + 1) * 64, :] for i in ia], axis=0))
                        ws = [cs(0), pw(2 * np_, 0), cs(1), cs(2), pw(2 * np_ + 1, 2), cs(3), cs(4)]
                        for n in range(7):
                            res.append(ext(len(res), mm(ls[n], ws[n])))
                    res.append(ext(len(res), mm(oc, _upk(wo_t[NLB - 1, k0 // 2:k1 // 2, :]))))
                    return res
                for n in range(NLB):
                    if before_oproj is not None:
                        w = wo_s[k0:k1, n * 128:(n + 1) * 128]
                        wo_t[n, k0 // 2:k1 // 2, :] = pltpu.bitcast(w, U32)
                    else:
                        w = _upk(wo_t[n, k0 // 2:k1 // 2, :])
                    res.append(ext(n, mm(oc, w)))
                return res

            heads = []
            qkv = proj(0)
            oa = None
            for g in range(NG):
                ps = probs(qkv, g)
                vs = qkv[2]
                if g + 1 < NG:
                    qkv = proj(g + 1)
                else:
                    if before_oproj is not None:
                        before_oproj()
                    oa = oproj(heads[:H // 2], 0, None)
                heads += [mm(ps[j], pad(vs[j])) for j in range(HG)]
            assert not units
            o = oproj(heads[H // 2:], H // 2, oa)
            if fast:
                cols = []
                for np_ in range(2):
                    m = o[7 * np_:7 * np_ + 7]
                    cols += combine(m[:5] + [m[5] + m[0], m[6] + m[0]])
                o = cols + [o[14]]
            return jnp.concatenate(o, axis=1)

        def post2(s, toks=None):
            r3 = seg_row(s - 1 - LAG)
            for r in (0, 16):
                xc = _r(x2_s[(s + 4 - 1 - LAG) % 4, r:r + 16] + obuf[SEG + r:SEG + r + 16, :])
                out_s[pl.ds(r3 + r, 16), :] = gate(xc, r3 + r, toks).astype(BF16)

        def step(s, mode, vis, fill, chained=False, before_oproj=None, early=None, units=()):
            if mode == 0:
                h = hbuf[...]
            elif mode == 1:
                h = hbuf[0:48, :]
            else:
                live = lax.broadcasted_iota(jnp.int32, (2 * M, D), 0) >= M
                mem = jnp.where(live, hbuf[0:16, :].astype(F32), 0.0).astype(BF16)
                h = jnp.concatenate([mem, hbuf[48:80, :]], axis=0)
            toks = []
            if mode != 1:
                post2(s, toks)
            if isinstance(s, int) and s == NSEG + LAG - 1:
                obuf[SEG:2 * SEG, :] = attention(h, vis, fill, chained, due=toks)
                return
            r1 = seg_row(s - 1)
            rn = seg_row(s + 1)
            h1n, h2n = [], []
            for r in (0, 16):
                xa = _r(x_s[pl.ds(r1 + r, 16), :].astype(F32) + obuf[r:r + 16, :])
                xb2 = _r(gate(xa, r1 + r))
                h2n.append(_ln(xb2, toks))
                x2_s[(s + 4 - 1) % 4, r:r + 16] = xb2
            if mode != 2:
                for r in (0, 16):
                    h1n.append(_ln(x_s[pl.ds(rn + r, 16), :].astype(F32), toks))

            if early is not None:
                mrow = pl.multiple_of(early * (8 * PPS), 8 * PPS)
                units = [functools.partial(lambda u, tok: u(tok[0:8]), u)
                         for n in range(PPS) for u in mac_units(mrow + 8 * n, 1)]
                units += [functools.partial(qkv_sum_unit, 0, jnp.minimum(early, 15), r0, 16)
                          for r0 in range(0, 128, 16)]

            o = attention(h, vis, fill, chained, before_oproj, early, toks, mode == 0, units)

            mem2 = mem0 if mode == 1 else o[M:2 * M]
            mem = jnp.concatenate([o[0:M], mem2], axis=0)
            hbuf[0:16, :] = mem.astype(BF16)
            for n, v in enumerate(h1n):
                hbuf[16 + 16 * n:32 + 16 * n, :] = v.astype(BF16)
            for n, v in enumerate(h2n):
                hbuf[48 + 16 * n:64 + 16 * n, :] = v.astype(BF16)
            if mode != 2:
                sbuf[5 * SEG:, :] = (mem[:, :KH] + mem[:, KH:2 * KH]).astype(BF16)
                for n, (x1, x2) in enumerate(zip(h1n, h2n)):
                    a11, a12, a21, a22 = x1[:, :KH], x1[:, KH:2 * KH], x2[:, :KH], x2[:, KH:2 * KH]
                    for i, v in enumerate((a11 + a22, a21 + a22, a11 + a12, a21 - a11, a12 - a22)):
                        sbuf[i * SEG + 16 * n:i * SEG + 16 * n + 16, :] = v.astype(BF16)
            if mode == 0:
                obuf[...] = o[2 * M:]
            elif mode == 1:
                obuf[0:SEG, :] = o[2 * M:]
            else:
                obuf[SEG:2 * SEG, :] = o[2 * M:]

        with _scope("pro"):
            vis, fill = masks(1)
            kv_units = [functools.partial(qkv_sum_unit, t, pr, r0, 16)
                        for t in (1, 2) for pr in range(16) for r0 in range(0, 128, 16)]
            o_units = [functools.partial(o_sum_unit, np_, i, r0, 16)
                       for np_ in range(2) for i in range(16) for r0 in range(0, 64, 16)]
            step(0, 1, vis, fill, False, wo_copy.wait, units=kv_units[:192])
            step(1, 1, vis, fill, True, units=kv_units[192:] + o_units)
        xb_copy.start()
        vis, fill = masks(0)
        with _scope("main_a"):
            loop(NA // UA, lambda i: [step(UA * i + u + LAG, 0, vis, fill, u > 0, early=UA * i + u)
                                      for u in range(UA)])
        xb_copy.wait()
        with _scope("conv_e"):
            loop(HB // UI, lambda j: [inv_stage(HB + UI * j + u) for u in range(UI)])
        with _scope("main_b"):
            loop((NSEG - LAG - NA) // UB, lambda i: [step(UB * i + u + LAG + NA, 0, vis, fill, u > 0)
                                                     for u in range(UB)])
        done = (NSEG - 1 - LAG) * SEG
        out_a = pltpu.make_async_copy(out_s.at[0:done, :], out_hbm.at[0:done, :], sem.at[SW + 8])
        out_a.start()
        with _scope("epi"):
            vis, fill = masks(2)
            step(NSEG, 2, vis, fill)
            step(NSEG + 1, 2, *masks(2, 2 * M), True)
        post2(NSEG + LAG)
        out_b = pltpu.make_async_copy(out_s.at[done:S, :], out_hbm.at[done:S, :], sem.at[SW + 9])
        out_b.start()
        out_a.wait()
        out_b.wait()

    pl.run_scoped(
        phase1,
        pltpu.VMEM((H // 2 * 5 * 128, 128), U32),
        pltpu.VMEM((H * 5 * 128, 128), U32),
        pltpu.VMEM((2 * 5 * (H * DH // 4), 128), U32),
    )


@jax.jit
def pallas_interleave_layers__memory_aug_recurrent_mem_tr__ssm_conv_h3__prompt_kernel(
    A_x, A_mem0, A_Wq, A_Wk, A_Wv, A_Wo, A_seg_len,
    B_q, B_k, B_v, B_shift_k, B_ssm_k, B_ssm_D,
):
    del A_seg_len, B_q
    assert A_x.shape == (1, S, D) and A_Wq.shape == (D, H, DH)
    hbm = pl.BlockSpec(memory_space=pl.ANY)
    out = pl.pallas_call(
        _kernel,
        out_shape=jax.ShapeDtypeStruct((S, D), BF16),
        in_specs=[hbm] * 11,
        out_specs=hbm,
        scratch_shapes=[
            pltpu.VMEM((S, D), BF16),
            pltpu.VMEM(((H + 1) * WP, 128), U32),
            pltpu.VMEM(((2 * H + 1) * WP, 128), U32),
            pltpu.VMEM((H * DH, D), BF16),
            pltpu.VMEM((NLB, H * DH // 2, 128), U32),
            pltpu.VMEM((TB // 2, TB), U32),
            pltpu.VMEM((2, TB // 2, TB), U32),
            pltpu.VMEM((2, TB // 2, TB), U32),
            pltpu.VMEM((NB, 2, NLB * TB, 128), F32),
            pltpu.VMEM((NB, 3, NLB * TB, 128), F32),
            pltpu.VMEM((NB + 1, 2, NLB * TB, 128), F32),
            pltpu.VMEM((NLB, S + 8, 128), F32),
            pltpu.VMEM((ROWS, D), BF16),
            pltpu.VMEM((5 * SEG + 2 * M, 256), BF16),
            pltpu.VMEM((2 * SEG, D), F32),
            pltpu.VMEM((4, SEG, D), F32),
            pltpu.VMEM((S, D), BF16),
            pltpu.VMEM((NQH, NA * SEG, DH), BF16),
            pltpu.VMEM((M, D), BF16),
            pltpu.VMEM((KS, D), BF16),
            pltpu.VMEM((D,), BF16),
            pltpu.SemaphoreType.DMA((HB + HB // 2 + 14,)),
        ],
        compiler_params=pltpu.CompilerParams(vmem_limit_bytes=120 * 1024 * 1024),
    )(A_x.reshape(S, D), A_mem0.reshape(M, D), A_Wq, A_Wk, A_Wv,
      A_Wo.reshape(H * DH, D), B_k.reshape(S, D), B_v.reshape(S, D),
      B_shift_k.T, B_ssm_k, B_ssm_D)
    return out.reshape(1, S, D)
```

```python
import contextlib
import functools
import math

import jax
import jax.numpy as jnp
from jax import lax
import jax.experimental.pallas as pl
import jax.experimental.pallas.tpu as pltpu

F32 = jnp.float32
BF16 = jnp.bfloat16
U32 = jnp.uint32

S = 2048
D = 640
H = 32
DH = 128
M = 8
SEG = 32
NSEG = S // SEG
KS = 4
LAG = 2
ROWS = 2 * M + 2 * SEG
HG = 4
NG = H // HG
NLB = D // 128
TB = 128
NB = S // TB
HB = NB // 2
NPOS = NLB * TB // 8
NA = 20
PPS = 4
UCUT = tuple(range(a, a + 2) for a in range(0, 12, 2)) + (range(12, 16),)
NQH = 32
UA = 2
UB = 3
UI = 4
WP = 324


PROFILE = False


def _scope(name):
    return jax.named_scope(name) if PROFILE else contextlib.nullcontext()


def _ln(x, toks=None):
    m = jnp.mean(x, axis=-1, keepdims=True)
    c = x - m
    v = jnp.mean(c * c, axis=-1, keepdims=True)
    r = lax.rsqrt(v + 1e-5)
    if toks is not None:
        toks.append(jnp.minimum(r, 0.0))
    return c * r


def _r(x):
    return x.astype(BF16).astype(F32)


def _split(x):
    hi = pltpu.bitcast(pltpu.bitcast(x, U32) & jnp.uint32(0xFFFF0000), F32)
    return hi, x - hi


def _pk(x):
    return pltpu.bitcast(x.astype(BF16), U32)


def _upk(w):
    return pltpu.bitcast(w, BF16)


def _basis(r, t):
    b = r & 63
    f = jnp.where(b < 32, 2 * b, 2 * b - 63)
    n = ((2 * f + 1) * t - jnp.where(r >= 64, TB, 0)) & (4 * TB - 1)
    n = jnp.where(n >= 2 * TB, n - 4 * TB, n)
    return jnp.cos(n.astype(F32) * (2.0 * math.pi / (4 * TB)))


def _halves(x):
    w = pltpu.bitcast(x, U32)
    return (pltpu.bitcast(w << 16, F32),
            pltpu.bitcast(w & jnp.uint32(0xFFFF0000), F32))


def _kernel(x_hbm, mem0_hbm, wq_hbm, wk_hbm, wv_hbm, wo_hbm,
            k_hbm, v_hbm, shk_hbm, ssmk_hbm, ssmd_hbm,
            out_hbm,
            x_s, wt_q, wt_kv, wo_s, wo_t,
            perm_s, fu_s, inv_s, u_s, kf_s, c_s, y_s,
            obuf, x2_s, out_s, qh_s, hbuf, sbuf, mem0_ref, shk_ref, ssmd_ref,
            sem):
    X0, XH = LAG * SEG, (LAG + NA) * SEG
    SW = HB + HB // 2
    hb = TB // 2
    wo_copy = pltpu.make_async_copy(wo_hbm, wo_s, sem.at[SW + 3])
    xb_copy = pltpu.make_async_copy(x_hbm.at[XH + SEG:, :], x_s.at[XH + SEG:, :], sem.at[SW + 7])

    def mac_units(row, half):
        rs = pl.ds(row, 8)
        state = {}

        def unit(p, avals, final, tok=None):
            acc = state.setdefault(p, dict(state.get(0, {})))
            for a in avals:
                u = u_s[a, 0, rs] + u_s[a, 1, rs] if p == 0 else u_s[a, p - 1, rs]
                if tok is not None:
                    u = u + tok
                for i in range(max(a, half * HB), half * HB + HB):
                    t = u * kf_s[i - a, p, rs]
                    acc[i] = t if i not in acc else (acc[i] - t if p == 2 else acc[i] + t)
            if final and p:
                for i, v in acc.items():
                    c_s[i + 1, 2 - p, rs] = v

        subs = UCUT if half else (range(HB),)
        return [functools.partial(unit, p, avals, n == len(subs) - 1)
                for p in range(3) for n, avals in enumerate(subs)]

    def inv_stage(i, units=None):
        q = TB // 4
        for g in range(NLB):
            re, im = [], []
            for b in range(4):
                rows = slice(g * TB + b * q, g * TB + (b + 1) * q)
                cr, ci_ = c_s[i + 1, 0, rows], c_s[i + 1, 1, rows]
                pr, pi = c_s[i, 0, rows], c_s[i, 1, rows]
                re.append(cr + pi if b in (0, 3) else cr - pi)
                im.append(ci_ - pr if b in (0, 3) else ci_ + pr)
            pe = jnp.concatenate([re[0] + re[2], re[1] + re[3], im[0] - im[2], im[1] - im[3]], axis=0)
            po = jnp.concatenate([re[0] - re[2], re[1] - re[3], im[0] + im[2], im[1] + im[3]], axis=0)
            for par, pp in enumerate((pe, po)):
                ph, plo = _split(pp)
                gh_, gl_ = (inv_s[n, par * q:(par + 1) * q] for n in range(2))
                y = jnp.dot(_upk(jnp.concatenate([gh_, gl_, gh_], axis=1)),
                            jnp.concatenate([ph, ph, plo], axis=0).astype(BF16),
                            preferred_element_type=F32)
                y_s[g, pl.ds(i * TB + par, hb, stride=2), :] = y
                if units:
                    tok = pltpu.bitcast(jnp.minimum(jnp.abs(y[0:16]), 0.0), U32)
                    for _ in range(3):
                        if units:
                            units.pop(0)(tok)

    def wslab(t, h):
        s0 = (max(t - 1, 0) * H + (h % 2) * 16 + h // 2) * WP
        return pltpu.bitcast((wt_kv if t else wt_q)[s0:s0 + D // 2, :], BF16)

    def loop(n, fn):
        def body(j, _):
            fn(j)
            return 0
        lax.fori_loop(0, n, body, 0)

    def phase0(k_s, v_s, ssmk_s, wraw, kpad, hl_s):

        def pair_rows(jp):
            r0 = jp * 2 * TB
            return pl.ds(r0 if isinstance(jp, int) else pl.multiple_of(r0, 2 * TB), 2 * TB)

        def ssmk_copy(jp):
            return pltpu.make_async_copy(ssmk_hbm.at[:, pair_rows(jp)], ssmk_s.at[jp], sem.at[jp])

        def kv_copies(rows, sm):
            return [pltpu.make_async_copy(k_hbm.at[rows, :], k_s.at[rows, :], sm),
                    pltpu.make_async_copy(v_hbm.at[rows, :], v_s.at[rows, :], sm)]
        DQ = 192
        wq_early = [pltpu.make_async_copy(wq_hbm.at[n * DQ:(n + 1) * DQ], wraw.at[0, n * DQ:(n + 1) * DQ],
                                          sem.at[SW + 10 + n]) for n in range(2)]
        w_copies = [pltpu.make_async_copy(wq_hbm.at[2 * DQ:], wraw.at[0, 2 * DQ:], sem.at[SW])]
        w_copies += [pltpu.make_async_copy(w.at[n * (D // 2):(n + 1) * (D // 2)],
                                           wraw.at[t, n * (D // 2):(n + 1) * (D // 2)],
                                           sem.at[SW + 11 * n + t])
                     for t, w in ((1, wk_hbm), (2, wv_hbm)) for n in range(2)]
        late_copies = kv_copies(pl.ds(S // 2, S // 2), sem.at[SW + 4])
        small_copies = [pltpu.make_async_copy(src, dst, sem.at[SW + 5])
                        for src, dst in ((shk_hbm, shk_ref), (ssmd_hbm, ssmd_ref), (mem0_hbm, mem0_ref))]
        XM = XH - 2 * TB
        xa_copy = pltpu.make_async_copy(x_hbm.at[X0:XM, :], x_s.at[X0:XM, :], sem.at[SW + 6])
        late_copies += [pltpu.make_async_copy(x_hbm.at[a:b, :], x_s.at[a:b, :], sem.at[SW + 4])
                        for a, b in ((0, X0), (XM, XH + SEG))]
        for c in (small_copies + [ssmk_copy(jp) for jp in range(HB)]
                  + [c for jp in range(HB // 2) for c in kv_copies(pair_rows(jp), sem.at[HB + jp])]
                  + [xa_copy] + wq_early + [w_copies[0]] + late_copies + w_copies[1:] + [wo_copy]):
            c.start()

        ri = lax.broadcasted_iota(jnp.int32, (TB, TB), 0)
        ci = lax.broadcasted_iota(jnp.int32, (TB, TB), 1)
        perm_s[...] = _pk(jnp.where(ci == 2 * (ri & 63) + (ri >> 6), 1.0, 0.0))
        tab = _basis(ri, 2 * (ci & 63) + (ci >> 6))
        hi, lo = _split(tab)
        fu_s[0] = _pk(jnp.where(ci < hb, hi, pltpu.roll(lo, hb, 1)))
        fu_s[1] = _pk(jnp.where(ci < hb, pltpu.roll(hi, hb, 1), lo))
        gh, gl = _split(tab.T * (1.0 / TB))
        inv_s[0] = _pk(gh)
        inv_s[1] = _pk(gl)

        for c in small_copies:
            c.wait()
        shk_t = shk_ref[...].astype(F32)
        taps = [[shk_t[j:j + 1, g * 128:(g + 1) * 128] for g in range(NLB)] for j in range(KS)]
        dvec = ssmd_ref[...].astype(F32).reshape(1, D)
        for g in range(NLB):
            kpad[0, g, 0:8, :] = jnp.zeros((8, 128), F32)
            kpad[1, g, 0:8, :] = jnp.zeros((8, 128), F32)
        c_s[0] = jnp.zeros(c_s.shape[1:], F32)
        hbuf[0:16, :] = jnp.concatenate([mem0_ref[...].astype(F32)] * 2, axis=0).astype(BF16)
        obuf[...] = jnp.zeros((2 * SEG, D), F32)
        x2_s[...] = jnp.zeros(x2_s.shape, F32)

        def spectrum(e, o):
            fe = jnp.dot(_upk(fu_s[0]), jnp.concatenate([e, e], axis=0).astype(BF16), preferred_element_type=F32)
            fo = jnp.dot(_upk(fu_s[1]), jnp.concatenate([o, o], axis=0).astype(BF16), preferred_element_type=F32)
            return ((fe[:hb] + fo[:hb], fe[hb:] + fo[hb:]), (fe[:hb] - fo[:hb], fo[hb:] - fe[hb:]))

        def freq_rows(g):
            return slice(g * TB, g * TB + hb), slice(g * TB + hb, (g + 1) * TB)

        def fwd_k(jq):
            def transposed(n):
                if n % 2 == 0:
                    ssmk_copy(2 * jq + n // 2).wait()
                blk = ssmk_s[2 * jq + n // 2, :, (n % 2) * TB:(n % 2 + 1) * TB]
                return lax.dot_general(_upk(perm_s[...]), blk, (((1,), (1,)), ((), ())),
                                       preferred_element_type=F32)
            nxt = transposed(0)
            for n in range(4):
                kt = nxt
                if n < 3:
                    nxt = transposed(n + 1)
                j = 4 * jq + n
                for g in range(NLB):
                    lb = slice(g * 128, (g + 1) * 128)
                    for rows, (kr, ki) in zip(freq_rows(g), spectrum(kt[:hb, lb], kt[hb:, lb])):
                        if n == 0:
                            kr = kr + jnp.where(j == 0, dvec[:, lb], 0.0)
                        kf_s[j, 0, rows] = kr
                        kf_s[j, 1, rows] = ki - kr
                        kf_s[j, 2, rows] = kr + ki

        def fwd_u(jq, first):
            if first:
                for jp in (2 * jq, 2 * jq + 1):
                    for c in kv_copies(pair_rows(jp), sem.at[HB + jp]):
                        c.wait()
            for j in [4 * jq + n for n in range(4)]:
                r0 = pl.multiple_of(j * TB, TB)
                q0 = pl.multiple_of(j * hb, hb) + 8
                for g in range(NLB):
                    lb = slice(g * 128, (g + 1) * 128)
                    ke, ko = _halves(k_s[pl.ds(r0, TB), lb])
                    ve, vo = _halves(v_s[pl.ds(r0, TB), lb])
                    kpad[0, g, pl.ds(q0, hb), :] = ke
                    kpad[1, g, pl.ds(q0, hb), :] = ko
                    ke1 = kpad[0, g, pl.ds(q0 - 1, hb), :]
                    ko1 = kpad[1, g, pl.ds(q0 - 1, hb), :]
                    ko2 = kpad[1, g, pl.ds(q0 - 2, hb), :]
                    t0, t1, t2, t3 = (taps[t][g] for t in range(KS))
                    e = (ke * t0 + ko1 * t1 + ke1 * t2 + ko2 * t3) * ve
                    o = (ko * t0 + ke * t1 + ko1 * t2 + ke1 * t3) * vo
                    for rows, (ur, ui) in zip(freq_rows(g), spectrum(e, o)):
                        u_s[j, 0, rows] = ur
                        u_s[j, 1, rows] = ui

        def relayout_rows(t, dst, base, dp, tok=None):
            a = pltpu.bitcast(wraw[t, 2 * dp], U32)
            b = pltpu.bitcast(wraw[t, 2 * dp + 1], U32)
            if tok is not None:
                a = a | tok
            dst[pl.ds(base + dp, 16, stride=WP), :] = (a & jnp.uint32(0xFFFF)) | (b << 16)
            dst[pl.ds(base + 16 * WP + dp, 16, stride=WP), :] = (
                (a >> 16) | (b & jnp.uint32(0xFFFF0000)))

        def norm_rows(r0, nr):
            r0 = pl.multiple_of(r0, 16)
            for r in range(0, nr, 16):
                hl_s[pl.ds(r0 + r, 16), :] = _ln(
                    x_s[pl.ds(r0 + r + LAG * SEG, 16), :].astype(F32)).astype(BF16)

        def pre_queries(c, t=None):
            per = -(-(D // 4) // NQH)
            for sub in range(2):
                if t is not None:
                    half = wraw.at[t, sub * (D // 2):(sub + 1) * (D // 2)]
                    pltpu.make_async_copy(half, half, sem.at[SW + 11 * sub + t]).wait()
                    base = (t - 1) * (H * WP)
                    dp = sub * (D // 4)
                r0 = pl.multiple_of((2 * c + sub) * QR, QR)
                hl = hl_s[pl.ds(r0, QR), :]
                for hd in range(NQH):
                    r = jnp.dot(hl, wslab(0, hd), preferred_element_type=F32)
                    qh_s[hd, pl.ds(r0, QR), :] = r.astype(BF16)
                    if t is not None:
                        tok = pltpu.bitcast(jnp.minimum(jnp.abs(r[0:16]), 0.0), U32)
                        for _ in range(per):
                            if dp < (sub + 1) * (D // 4):
                                relayout_rows(t, wt_kv, base, dp, tok)
                                dp += 1

        nch = NA * SEG // TB
        QR = TB // 2
        with _scope("conv_k"):
            loop(HB // 2, fwd_k)
        with _scope("conv_u"):
            loop(HB // 4, lambda j: fwd_u(j, True))
        with _scope("conv_b"):
            loop(NPOS // 10, lambda j: [u() for n in range(10)
                                        for u in mac_units(pl.multiple_of(80 * j, 16) + 8 * n, 0)])
            xa_copy.wait()

            def inv_first(j):
                part = wraw.at[0, pl.ds(j * DQ, DQ)]
                pltpu.make_async_copy(part, part, sem.at[SW + 10 + j]).wait()
                units = [functools.partial(relayout_rows, 0, wt_q, 0, j * (DQ // 2) + dd)
                         for dd in range(DQ // 2)]
                for u in range(UI):
                    inv_stage(UI * j + u, units)
                assert not units
                norm_rows(j * ((XM - X0) // 2), (XM - X0) // 2)
            loop(HB // UI, inv_first)
        with _scope("rel0"):
            w_copies[0].wait()
            loop((D - 2 * DQ) // 64,
                 lambda i: [relayout_rows(0, wt_q, 0, DQ + i * 32 + dd) for dd in range(32)])
        with _scope("preq"):
            loop(nch - 2, pre_queries)
        with _scope("conv_c"):
            for c in late_copies:
                c.wait()

            def fwd_u_late(j):
                r0 = pl.multiple_of(j * 16, 16)
                hbuf[pl.ds(16 + r0, 16), :] = _ln(x_s[pl.ds(r0, 16), :].astype(F32)).astype(BF16)
                norm_rows(XM - X0 + j * TB, TB)
                fwd_u(HB // 4 + j, False)
            loop(HB // 4, fwd_u_late)
        with _scope("preq_rel"):
            loop(2, lambda i: pre_queries(i + nch - 2, i + 1))

    pl.run_scoped(
        phase0,
        pltpu.VMEM((S, D), BF16),
        pltpu.VMEM((S, D), BF16),
        pltpu.VMEM((HB, D, 2 * TB), BF16),
        pltpu.VMEM((3, D, H, DH), BF16),
        pltpu.VMEM((2, NLB, S // 2 + 32, 128), F32),
        pltpu.VMEM((NA * SEG, D), BF16),
    )

    def phase1(cq, ckv, co):
        scale = DH ** -0.5

        def masks(mode, q0=0):
            rows = ROWS if mode == 0 else ROWS - SEG
            qi = lax.broadcasted_iota(jnp.int32, (rows - q0, 128), 0) + q0
            kj = lax.broadcasted_iota(jnp.int32, (rows - q0, 128), 1)

            def layer_of(i):
                xl = (i - 2 * M) // SEG if mode == 0 else mode - 1
                return jnp.where(i < 2 * M, i // M, xl)
            same = (layer_of(qi) == layer_of(kj)) & (kj < rows)
            vis = same & ((qi < 2 * M) | (qi >= kj))
            fill = jnp.where(same, -1e9 / scale, -jnp.inf).astype(F32)
            return vis, fill

        mem0 = mem0_ref[...].astype(F32)

        def seg_row(seg):
            if isinstance(seg, int):
                return min(max(seg, 0), NSEG - 1) * SEG
            return pl.multiple_of(jnp.clip(seg, 0, NSEG - 1) * SEG, SEG)

        def gate(xa, r0, toks=None):
            y = jnp.concatenate([y_s[g, pl.ds(r0, xa.shape[0]), :] for g in range(NLB)], axis=1)
            return xa + _ln(xa, toks) * y

        KH = 256

        def mm(a, b):
            return jnp.dot(a, b, preferred_element_type=F32)

        def row_sums(x1, x2, m_a, m_b):
            (a11, a12), (a21, a22) = x1, x2
            ms = m_a + m_b
            cat = lambda u, v: jnp.concatenate([u, v], axis=0)
            return [a11 + a22, cat(ms, a21 + a22), cat(m_a, a11), cat(m_b, a22),
                    cat(ms, a11 + a12), a21 - a11, a12 - a22]

        def combine(m):
            m1, m2, m3, m4, m5, m16, m17 = m
            m24, m35 = m2 + m4, m3 + m5
            r = 2 * M
            return (jnp.concatenate([m24[:r], m17 + m4[r:] - m5[r:], m24[r:]], axis=0),
                    jnp.concatenate([m35[:r], m35[r:], m16 - m2[r:] + m3[r:]], axis=0))

        def sums_of(b11, b12, b21, b22):
            b11, b12, b21, b22 = (_upk(b).astype(F32) for b in (b11, b12, b21, b22))
            return [_pk(v) for v in (b11 + b22, b12 - b22, b21 - b11, b11 + b12, b21 + b22)]

        def slab_rows(t, h):
            return (wt_kv if t else wt_q), (max(t - 1, 0) * H + (h % 2) * 16 + h // 2) * WP

        def qkv_sum_unit(t, pr, r0, nr, tok=None):
            src, s1 = slab_rows(t, 0)
            s1 = s1 + pr * WP
            s2 = s1 + 16 * WP
            b11 = src[pl.ds(s1 + r0, nr), :]
            if tok is not None:
                b11 = b11 | pltpu.bitcast(tok, U32)
            sm = sums_of(b11, src[pl.ds(s2 + r0, nr), :],
                         src[pl.ds(s1 + 128 + r0, nr), :], src[pl.ds(s2 + 128 + r0, nr), :])
            dst, d0 = (ckv if t else cq), (max(t - 1, 0) * 16 + pr) * 640
            for n, v in enumerate(sm):
                dst[pl.ds(d0 + n * 128 + r0, nr), :] = v

        def o_sum_unit(np_, i, r0, nr, tok=None):
            ka = ((i // 2) * 4 + i % 2) * 64 + r0
            b11 = wo_t[2 * np_, pl.ds(ka, nr), :]
            if tok is not None:
                b11 = b11 | pltpu.bitcast(tok, U32)
            sm = sums_of(b11, wo_t[2 * np_ + 1, pl.ds(ka, nr), :],
                         wo_t[2 * np_, pl.ds(ka + 128, nr), :], wo_t[2 * np_ + 1, pl.ds(ka + 128, nr), :])
            for n, v in enumerate(sm):
                co[pl.ds((np_ * 5 + n) * 1024 + i * 64 + r0, nr), :] = v

        def attention(h, vis, fill, chained, before_oproj=None, early=None, due=(), fast=False,
                      units=()):
            q0 = h.shape[0] - vis.shape[0]
            units = list(units)
            per = -(-len(units) // 96)
            r = 2 * M
            if early is not None:
                hrest = jnp.concatenate([h[:r], h[r + SEG:]], axis=0)
                qrow = pl.multiple_of(early * SEG, SEG)
            if fast:
                sb = sbuf[...]
                ms = sb[5 * SEG:]
                cat = lambda u, v: jnp.concatenate([u, v], axis=0)
                lhs = [sb[0:SEG], cat(ms, sb[SEG:2 * SEG]), h[:r + SEG, :KH],
                       cat(h[:r, KH:2 * KH], h[r + SEG:, KH:2 * KH]), cat(ms, sb[2 * SEG:3 * SEG]),
                       sb[3 * SEG:4 * SEG], sb[4 * SEG:5 * SEG]]

            def feed(x):
                if units:
                    tok = jnp.minimum(jnp.abs(x[0:16]), 0.0)
                    for u in units[:per]:
                        u(tok)
                    del units[:per]

            def proj(g):
                res = [[None] * HG for _ in range(3)]
                plain, pairs = [], []
                for t, j in [(t, j) for j in range(HG) for t in range(2)] + [(2, j) for j in range(HG)]:
                    pre = early is not None and t == 0 and g * HG + j < NQH
                    if pre or not fast:
                        plain.append((t, j, pre))
                    elif j % 2 == 0:
                        pairs.append((t, j))

                def csum(t, j, n):
                    d0 = (max(t - 1, 0) * 16 + (g * HG + j) // 2) * 640 + n * 128
                    return _upk((ckv if t else cq)[d0:d0 + 128, :])

                def free_part(t, j):
                    m1 = mm(lhs[0], csum(t, j, 0))
                    return m1, mm(lhs[5], csum(t, j, 3)) + m1, mm(lhs[6], csum(t, j, 4)) + m1

                def do_pair(t, j, fp):
                    w1, w2 = wslab(t, g * HG + j), wslab(t, g * HG + j + 1)
                    m1, m16, m17 = fp
                    feed(m16)
                    m = [m1, mm(lhs[1], w1[:KH]), mm(lhs[2], csum(t, j, 1)), mm(lhs[3], csum(t, j, 2)),
                         mm(lhs[4], w2[KH:2 * KH]), m16, m17]
                    feed(m[4])
                    for n, (c, w) in enumerate(zip(combine(m), (w1, w2))):
                        c = mm(h[:, 2 * KH:], w[2 * KH:]) + c
                        res[t][j + n] = c.astype(BF16) if t == 0 else c

                def do_plain(t, j, pre, part=None):
                    hd = g * HG + j
                    x = hrest if pre else (h if t else h[q0:])
                    if part is None:
                        y = mm(x, wslab(t, hd))
                    else:
                        y = mm(x[:, 2 * KH:], wslab(t, hd)[2 * KH:]) + part
                    feed(y)
                    if t == 0:
                        y = y.astype(BF16)
                    if pre:
                        y = jnp.concatenate([y[:r], qh_s[hd, pl.ds(qrow, SEG), :], y[r:]], axis=0)
                    res[t][j] = y

                first = g == 0 and chained
                fps = [free_part(t, j) for t, j in pairs] if first else None
                nsplit = 4 if first and not fast else 0
                parts = [mm((h if t else h[q0:])[:, :2 * KH], wslab(t, j)[:2 * KH])
                         for t, j, _ in plain[:nsplit]]
                jobs = sorted([(t, j, None) for t, j in pairs] + plain,
                              key=lambda x: (x[0] == 2, x[1], x[0]))
                np_ = 0
                for t, j, pre in jobs:
                    if pre is None:
                        do_pair(t, j, fps[pairs.index((t, j))] if first else free_part(t, j))
                    else:
                        do_plain(t, j, pre, parts[np_] if np_ < nsplit else None)
                        np_ += 1
                return res

            def pad(kv):
                return jnp.concatenate([kv, jnp.zeros((128 - kv.shape[0], DH), F32)],
                                       axis=0).astype(BF16)

            def probs(qkv, g):
                scs = [lax.dot_general(qkv[0][j], pad(qkv[1][j]), (((1,), (1,)), ((), ())),
                                       preferred_element_type=F32) for j in range(HG)]
                ps = []
                for sc in scs:
                    sc = jnp.where(vis, sc, fill)
                    e = jnp.exp2((sc - jnp.max(sc, axis=-1, keepdims=True))
                                 * (scale * math.log2(math.e)))
                    den = jnp.sum(e, axis=-1, keepdims=True)
                    if not ps and g >= NG - len(due):
                        e = jnp.concatenate([e[:16] + due[g - NG + len(due)], e[16:]], axis=0)
                    rc = pl.reciprocal(den, approx=True)
                    rc = rc * (2.0 - den * rc)
                    ps.append((e * rc).astype(BF16))
                return ps

            def oproj(os_, h0, acc, mid=None):
                ext = lambda n, y: y if acc is None else y + acc[n]
                oc = jnp.concatenate(os_, axis=1).astype(BF16)
                k0, k1 = h0 * DH, (h0 + len(os_)) * DH
                res = []
                if fast:
                    ia = [n for n in range(len(os_)) if n % 4 < 2]
                    oa_, ob_ = (jnp.concatenate([os_[n + d] for n in ia], axis=1) for d in (0, 2))
                    ls = [v.astype(BF16) for v in row_sums(
                        (oa_[r:r + SEG], ob_[r:r + SEG]), (oa_[r + SEG:], ob_[r + SEG:]),
                        oa_[:r], ob_[:r])]
                    for np_ in range(2):
                        def cs(n):
                            d0 = (np_ * 5 + n) * 1024 + h0 * 32
                            return _upk(co[d0:d0 + len(os_) * 32, :])

                        def pw(n, d):
                            return _upk(jnp.concatenate(
                                [wo_t[n, (h0 + i + d) * 64:(h0 + i + d + 1) * 64, :] for i in ia], axis=0))
                        ws = [cs(0), pw(2 * np_, 0), cs(1), cs(2), pw(2 * np_ + 1, 2), cs(3), cs(4)]
                        for n in range(7):
                            if mid is not None and len(res) == 9:
                                mid()
                            res.append(ext(len(res), mm(ls[n], ws[n])))
                    res.append(ext(len(res), mm(oc, _upk(wo_t[NLB - 1, k0 // 2:k1 // 2, :]))))
                    return res
                for n in range(NLB):
                    if before_oproj is not None:
                        w = wo_s[k0:k1, n * 128:(n + 1) * 128]
                        wo_t[n, k0 // 2:k1 // 2, :] = pltpu.bitcast(w, U32)
                    else:
                        w = _upk(wo_t[n, k0 // 2:k1 // 2, :])
                    res.append(ext(n, mm(oc, w)))
                if mid is not None:
                    mid()
                return res

            heads = []
            qkv = proj(0)
            oa = None
            for g in range(NG):
                ps = probs(qkv, g)
                vs = qkv[2]

                def weigh():
                    heads.extend(mm(ps[j], pad(vs[j])) for j in range(HG))
                if g + 1 < NG:
                    qkv = proj(g + 1)
                    weigh()
                else:
                    if before_oproj is not None:
                        before_oproj()
                    oa = oproj(heads[:H // 2], 0, None, weigh)
            assert not units
            o = oproj(heads[H // 2:], H // 2, oa)
            if fast:
                cols = []
                for np_ in range(2):
                    m = o[7 * np_:7 * np_ + 7]
                    cols += combine(m[:5] + [m[5] + m[0], m[6] + m[0]])
                o = cols + [o[14]]
            return jnp.concatenate(o, axis=1)

        def post2(s, toks=None):
            r3 = seg_row(s - 1 - LAG)
            for r in (0, 16):
                xc = _r(x2_s[(s + 4 - 1 - LAG) % 4, r:r + 16] + obuf[SEG + r:SEG + r + 16, :])
                out_s[pl.ds(r3 + r, 16), :] = gate(xc, r3 + r, toks).astype(BF16)

        def step(s, mode, vis, fill, chained=False, before_oproj=None, early=None, units=()):
            if mode == 0:
                h = hbuf[...]
            elif mode == 1:
                h = hbuf[0:48, :]
            else:
                live = lax.broadcasted_iota(jnp.int32, (2 * M, D), 0) >= M
                mem = jnp.where(live, hbuf[0:16, :].astype(F32), 0.0).astype(BF16)
                h = jnp.concatenate([mem, hbuf[48:80, :]], axis=0)
            toks = []
            if mode != 1:
                post2(s, toks)
            if isinstance(s, int) and s == NSEG + LAG - 1:
                obuf[SEG:2 * SEG, :] = attention(h, vis, fill, chained, due=toks)
                return
            r1 = seg_row(s - 1)
            rn = seg_row(s + 1)
            h1n, h2n = [], []
            for r in (0, 16):
                xa = _r(x_s[pl.ds(r1 + r, 16), :].astype(F32) + obuf[r:r + 16, :])
                xb2 = _r(gate(xa, r1 + r))
                h2n.append(_ln(xb2, toks))
                x2_s[(s + 4 - 1) % 4, r:r + 16] = xb2
            if mode != 2:
                for r in (0, 16):
                    h1n.append(_ln(x_s[pl.ds(rn + r, 16), :].astype(F32), toks))

            if early is not None:
                mrow = pl.multiple_of(early * (8 * PPS), 8 * PPS)
                units = [functools.partial(lambda u, tok: u(tok[0:8]), u)
                         for n in range(PPS) for u in mac_units(mrow + 8 * n, 1)]
                units += [functools.partial(qkv_sum_unit, 0, jnp.minimum(early, 15), r0, 16)
                          for r0 in range(0, 128, 16)]

            o = attention(h, vis, fill, chained, before_oproj, early, toks, mode == 0, units)

            mem2 = mem0 if mode == 1 else o[M:2 * M]
            mem = jnp.concatenate([o[0:M], mem2], axis=0)
            hbuf[0:16, :] = mem.astype(BF16)
            for n, v in enumerate(h1n):
                hbuf[16 + 16 * n:32 + 16 * n, :] = v.astype(BF16)
            for n, v in enumerate(h2n):
                hbuf[48 + 16 * n:64 + 16 * n, :] = v.astype(BF16)
            if mode != 2:
                sbuf[5 * SEG:, :] = (mem[:, :KH] + mem[:, KH:2 * KH]).astype(BF16)
                for n, (x1, x2) in enumerate(zip(h1n, h2n)):
                    a11, a12, a21, a22 = x1[:, :KH], x1[:, KH:2 * KH], x2[:, :KH], x2[:, KH:2 * KH]
                    for i, v in enumerate((a11 + a22, a21 + a22, a11 + a12, a21 - a11, a12 - a22)):
                        sbuf[i * SEG + 16 * n:i * SEG + 16 * n + 16, :] = v.astype(BF16)
            if mode == 0:
                obuf[...] = o[2 * M:]
            elif mode == 1:
                obuf[0:SEG, :] = o[2 * M:]
            else:
                obuf[SEG:2 * SEG, :] = o[2 * M:]

        with _scope("pro"):
            vis, fill = masks(1)
            kv_units = [functools.partial(qkv_sum_unit, t, pr, r0, 16)
                        for t in (1, 2) for pr in range(16) for r0 in range(0, 128, 16)]
            o_units = [functools.partial(o_sum_unit, np_, i, r0, 16)
                       for np_ in range(2) for i in range(16) for r0 in range(0, 64, 16)]
            step(0, 1, vis, fill, False, wo_copy.wait, units=kv_units[:192])
            step(1, 1, vis, fill, True, units=kv_units[192:] + o_units)
        xb_copy.start()
        vis, fill = masks(0)
        with _scope("main_a"):
            loop(NA // UA, lambda i: [step(UA * i + u + LAG, 0, vis, fill, u > 0, early=UA * i + u)
                                      for u in range(UA)])
        xb_copy.wait()
        with _scope("conv_e"):
            loop(HB // UI, lambda j: [inv_stage(HB + UI * j + u) for u in range(UI)])
        with _scope("main_b"):
            loop((NSEG - LAG - NA) // UB, lambda i: [step(UB * i + u + LAG + NA, 0, vis, fill, u > 0)
                                                     for u in range(UB)])
        done = (NSEG - 1 - LAG) * SEG
        out_a = pltpu.make_async_copy(out_s.at[0:done, :], out_hbm.at[0:done, :], sem.at[SW + 8])
        out_a.start()
        with _scope("epi"):
            vis, fill = masks(2)
            step(NSEG, 2, vis, fill)
            step(NSEG + 1, 2, *masks(2, 2 * M), True)
        post2(NSEG + LAG)
        out_b = pltpu.make_async_copy(out_s.at[done:S, :], out_hbm.at[done:S, :], sem.at[SW + 9])
        out_b.start()
        out_a.wait()
        out_b.wait()

    pl.run_scoped(
        phase1,
        pltpu.VMEM((H // 2 * 5 * 128, 128), U32),
        pltpu.VMEM((H * 5 * 128, 128), U32),
        pltpu.VMEM((2 * 5 * (H * DH // 4), 128), U32),
    )


@jax.jit
def pallas_interleave_layers__memory_aug_recurrent_mem_tr__ssm_conv_h3__prompt_kernel(
    A_x, A_mem0, A_Wq, A_Wk, A_Wv, A_Wo, A_seg_len,
    B_q, B_k, B_v, B_shift_k, B_ssm_k, B_ssm_D,
):
    del A_seg_len, B_q
    assert A_x.shape == (1, S, D) and A_Wq.shape == (D, H, DH)
    hbm = pl.BlockSpec(memory_space=pl.ANY)
    out = pl.pallas_call(
        _kernel,
        out_shape=jax.ShapeDtypeStruct((S, D), BF16),
        in_specs=[hbm] * 11,
        out_specs=hbm,
        scratch_shapes=[
            pltpu.VMEM((S, D), BF16),
            pltpu.VMEM((H * WP + 352, 128), U32),
            pltpu.VMEM((2 * H * WP + 352, 128), U32),
            pltpu.VMEM((H * DH, D), BF16),
            pltpu.VMEM((NLB, H * DH // 2, 128), U32),
            pltpu.VMEM((TB // 2, TB), U32),
            pltpu.VMEM((2, TB // 2, TB), U32),
            pltpu.VMEM((2, TB // 2, TB), U32),
            pltpu.VMEM((NB, 2, NLB * TB, 128), F32),
            pltpu.VMEM((NB, 3, NLB * TB, 128), F32),
            pltpu.VMEM((NB + 1, 2, NLB * TB, 128), F32),
            pltpu.VMEM((NLB, S + 32, 128), F32),
            pltpu.VMEM((2 * SEG, D), F32),
            pltpu.VMEM((4, SEG, D), F32),
            pltpu.VMEM((S, D), BF16),
            pltpu.VMEM((NQH, NA * SEG, DH), BF16),
            pltpu.VMEM((ROWS, D), BF16),
            pltpu.VMEM((5 * SEG + 2 * M, 256), BF16),
            pltpu.VMEM((M, D), BF16),
            pltpu.VMEM((KS, D), BF16),
            pltpu.VMEM((D,), BF16),
            pltpu.SemaphoreType.DMA((HB + HB // 2 + 14,)),
        ],
        compiler_params=pltpu.CompilerParams(vmem_limit_bytes=120 * 1024 * 1024),
    )(A_x.reshape(S, D), A_mem0.reshape(M, D), A_Wq, A_Wk, A_Wv,
      A_Wo.reshape(H * DH, D), B_k.reshape(S, D), B_v.reshape(S, D),
      B_shift_k.T, B_ssm_k, B_ssm_D)
    return out.reshape(1, S, D)
```

```python
import contextlib
import functools
import math

import jax
import jax.numpy as jnp
from jax import lax
import jax.experimental.pallas as pl
import jax.experimental.pallas.tpu as pltpu

F32 = jnp.float32
BF16 = jnp.bfloat16
U32 = jnp.uint32

S = 2048
D = 640
H = 32
DH = 128
M = 8
SEG = 32
NSEG = S // SEG
KS = 4
LAG = 2
ROWS = 2 * M + 2 * SEG
HG = 4
NG = H // HG
NLB = D // 128
TB = 128
NB = S // TB
HB = NB // 2
NPOS = NLB * TB // 8
NA = 20
PPS = 4
UCUT = tuple(range(a, a + 2) for a in range(0, 12, 2)) + (range(12, 16),)
NQH = 32
UA = 2
UB = 3
UI = 4
WP = 324


PROFILE = False


def _scope(name):
    return jax.named_scope(name) if PROFILE else contextlib.nullcontext()


def _ln(x, toks=None):
    m = jnp.mean(x, axis=-1, keepdims=True)
    c = x - m
    v = jnp.mean(c * c, axis=-1, keepdims=True)
    r = lax.rsqrt(v + 1e-5)
    if toks is not None:
        toks.append(jnp.minimum(r, 0.0))
    return c * r


def _r(x):
    return x.astype(BF16).astype(F32)


def _split(x):
    hi = pltpu.bitcast(pltpu.bitcast(x, U32) & jnp.uint32(0xFFFF0000), F32)
    return hi, x - hi


def _pk(x):
    return pltpu.bitcast(x.astype(BF16), U32)


def _upk(w):
    return pltpu.bitcast(w, BF16)


def _basis(r, t):
    b = r & 63
    f = jnp.where(b < 32, 2 * b, 2 * b - 63)
    n = ((2 * f + 1) * t - jnp.where(r >= 64, TB, 0)) & (4 * TB - 1)
    n = jnp.where(n >= 2 * TB, n - 4 * TB, n)
    return jnp.cos(n.astype(F32) * (2.0 * math.pi / (4 * TB)))


def _halves(x):
    w = pltpu.bitcast(x, U32)
    return (pltpu.bitcast(w << 16, F32),
            pltpu.bitcast(w & jnp.uint32(0xFFFF0000), F32))


def _kernel(x_hbm, mem0_hbm, wq_hbm, wk_hbm, wv_hbm, wo_hbm,
            k_hbm, v_hbm, shk_hbm, ssmk_hbm, ssmd_hbm,
            out_hbm,
            x_s, wt_q, wt_kv, wo_s, wo_t,
            perm_s, fu_s, inv_s, u_s, kf_s, c_s, y_s,
            obuf, x2_s, out_s, qh_s, hbuf, sbuf, mem0_ref,
            sem):
    X0, XH = LAG * SEG, (LAG + NA) * SEG
    SW = HB + HB // 2
    hb = TB // 2
    wo_copy = pltpu.make_async_copy(wo_hbm, wo_s, sem.at[SW + 3])
    xb_copy = pltpu.make_async_copy(x_hbm.at[XH + SEG:, :], x_s.at[XH + SEG:, :], sem.at[SW + 7])

    def mac_units(row, half):
        rs = pl.ds(row, 8)
        state = {}

        def unit(p, avals, final, tok=None):
            acc = state.setdefault(p, dict(state.get(0, {})))
            for a in avals:
                u = u_s[a, 0, rs] + u_s[a, 1, rs] if p == 0 else u_s[a, p - 1, rs]
                if tok is not None:
                    u = u + tok
                for i in range(max(a, half * HB), half * HB + HB):
                    t = u * kf_s[i - a, p, rs]
                    acc[i] = t if i not in acc else (acc[i] - t if p == 2 else acc[i] + t)
            if final and p:
                for i, v in acc.items():
                    c_s[i + 1, 2 - p, rs] = v

        subs = UCUT if half else (range(HB),)
        return [functools.partial(unit, p, avals, n == len(subs) - 1)
                for p in range(3) for n, avals in enumerate(subs)]

    def inv_stage(i, units=None):
        q = TB // 4
        for g in range(NLB):
            re, im = [], []
            for b in range(4):
                rows = slice(g * TB + b * q, g * TB + (b + 1) * q)
                cr, ci_ = c_s[i + 1, 0, rows], c_s[i + 1, 1, rows]
                pr, pi = c_s[i, 0, rows], c_s[i, 1, rows]
                re.append(cr + pi if b in (0, 3) else cr - pi)
                im.append(ci_ - pr if b in (0, 3) else ci_ + pr)
            pe = jnp.concatenate([re[0] + re[2], re[1] + re[3], im[0] - im[2], im[1] - im[3]], axis=0)
            po = jnp.concatenate([re[0] - re[2], re[1] - re[3], im[0] + im[2], im[1] + im[3]], axis=0)
            for par, pp in enumerate((pe, po)):
                ph, plo = _split(pp)
                gh_, gl_ = (inv_s[n, par * q:(par + 1) * q] for n in range(2))
                y = jnp.dot(_upk(jnp.concatenate([gh_, gl_, gh_], axis=1)),
                            jnp.concatenate([ph, ph, plo], axis=0).astype(BF16),
                            preferred_element_type=F32)
                y_s[g, pl.ds(i * TB + par, hb, stride=2), :] = y
                if units:
                    tok = pltpu.bitcast(jnp.minimum(jnp.abs(y[0:16]), 0.0), U32)
                    for _ in range(3):
                        if units:
                            units.pop(0)(tok)

    def wslab(t, h):
        s0 = (max(t - 1, 0) * H + (h % 2) * 16 + h // 2) * WP
        return pltpu.bitcast((wt_kv if t else wt_q)[s0:s0 + D // 2, :], BF16)

    def loop(n, fn):
        def body(j, _):
            fn(j)
            return 0
        lax.fori_loop(0, n, body, 0)

    def phase0(k_s, v_s, ssmk_s, wraw, kpad, hl_s, shk_ref, ssmd_ref):

        def pair_rows(jp):
            r0 = jp * 2 * TB
            return pl.ds(r0 if isinstance(jp, int) else pl.multiple_of(r0, 2 * TB), 2 * TB)

        def ssmk_copy(jp):
            return pltpu.make_async_copy(ssmk_hbm.at[:, pair_rows(jp)], ssmk_s.at[jp], sem.at[jp])

        def kv_copies(rows, sm):
            return [pltpu.make_async_copy(k_hbm.at[rows, :], k_s.at[rows, :], sm),
                    pltpu.make_async_copy(v_hbm.at[rows, :], v_s.at[rows, :], sm)]
        DQ = 192
        wq_early = [pltpu.make_async_copy(wq_hbm.at[n * DQ:(n + 1) * DQ], wraw.at[0, n * DQ:(n + 1) * DQ],
                                          sem.at[SW + 10 + n]) for n in range(2)]
        w_copies = [pltpu.make_async_copy(wq_hbm.at[2 * DQ:], wraw.at[0, 2 * DQ:], sem.at[SW])]
        w_copies += [pltpu.make_async_copy(w.at[n * (D // 2):(n + 1) * (D // 2)],
                                           wraw.at[t, n * (D // 2):(n + 1) * (D // 2)],
                                           sem.at[SW + 11 * n + t])
                     for t, w in ((1, wk_hbm), (2, wv_hbm)) for n in range(2)]
        late_copies = kv_copies(pl.ds(S // 2, S // 2), sem.at[SW + 4])
        small_copies = [pltpu.make_async_copy(src, dst, sem.at[SW + 5])
                        for src, dst in ((shk_hbm, shk_ref), (ssmd_hbm, ssmd_ref), (mem0_hbm, mem0_ref.at[0:M]))]
        XM = XH - 2 * TB
        xa_copy = pltpu.make_async_copy(x_hbm.at[X0:XM, :], x_s.at[X0:XM, :], sem.at[SW + 6])
        late_copies += [pltpu.make_async_copy(x_hbm.at[a:b, :], x_s.at[a:b, :], sem.at[SW + 4])
                        for a, b in ((0, X0), (XM, XH + SEG))]
        for c in (small_copies + [ssmk_copy(jp) for jp in range(HB)]
                  + [c for jp in range(HB // 2) for c in kv_copies(pair_rows(jp), sem.at[HB + jp])]
                  + [xa_copy] + wq_early + [w_copies[0]] + late_copies + w_copies[1:] + [wo_copy]):
            c.start()

        ri = lax.broadcasted_iota(jnp.int32, (TB, TB), 0)
        ci = lax.broadcasted_iota(jnp.int32, (TB, TB), 1)
        perm_s[...] = _pk(jnp.where(ci == 2 * (ri & 63) + (ri >> 6), 1.0, 0.0))
        tab = _basis(ri, 2 * (ci & 63) + (ci >> 6))
        hi, lo = _split(tab)
        fu_s[0] = _pk(jnp.where(ci < hb, hi, pltpu.roll(lo, hb, 1)))
        fu_s[1] = _pk(jnp.where(ci < hb, pltpu.roll(hi, hb, 1), lo))
        gh, gl = _split(tab.T * (1.0 / TB))
        inv_s[0] = _pk(gh)
        inv_s[1] = _pk(gl)

        for c in small_copies:
            c.wait()
        shk_t = shk_ref[...].astype(F32)
        taps = [[shk_t[j:j + 1, g * 128:(g + 1) * 128] for g in range(NLB)] for j in range(KS)]
        dvec = ssmd_ref[...].astype(F32).reshape(1, D)
        for g in range(NLB):
            kpad[0, g, 0:8, :] = jnp.zeros((8, 128), F32)
            kpad[1, g, 0:8, :] = jnp.zeros((8, 128), F32)
        c_s[0] = jnp.zeros(c_s.shape[1:], F32)
        hbuf[0:16, :] = jnp.concatenate([mem0_ref[0:M, :].astype(F32)] * 2, axis=0).astype(BF16)
        obuf[...] = jnp.zeros((2 * SEG, D), F32)
        x2_s[...] = jnp.zeros(x2_s.shape, F32)

        def spectrum(e, o):
            fe = jnp.dot(_upk(fu_s[0]), jnp.concatenate([e, e], axis=0).astype(BF16), preferred_element_type=F32)
            fo = jnp.dot(_upk(fu_s[1]), jnp.concatenate([o, o], axis=0).astype(BF16), preferred_element_type=F32)
            return ((fe[:hb] + fo[:hb], fe[hb:] + fo[hb:]), (fe[:hb] - fo[:hb], fo[hb:] - fe[hb:]))

        def freq_rows(g):
            return slice(g * TB, g * TB + hb), slice(g * TB + hb, (g + 1) * TB)

        def fwd_k(jq):
            def transposed(n):
                if n % 2 == 0:
                    ssmk_copy(2 * jq + n // 2).wait()
                blk = ssmk_s[2 * jq + n // 2, :, (n % 2) * TB:(n % 2 + 1) * TB]
                return lax.dot_general(_upk(perm_s[...]), blk, (((1,), (1,)), ((), ())),
                                       preferred_element_type=F32)
            nxt = transposed(0)
            for n in range(4):
                kt = nxt
                if n < 3:
                    nxt = transposed(n + 1)
                j = 4 * jq + n
                for g in range(NLB):
                    lb = slice(g * 128, (g + 1) * 128)
                    for rows, (kr, ki) in zip(freq_rows(g), spectrum(kt[:hb, lb], kt[hb:, lb])):
                        if n == 0:
                            kr = kr + jnp.where(j == 0, dvec[:, lb], 0.0)
                        kf_s[j, 0, rows] = kr
                        kf_s[j, 1, rows] = ki - kr
                        kf_s[j, 2, rows] = kr + ki

        def fwd_u(jq, first):
            if first:
                for jp in (2 * jq, 2 * jq + 1):
                    for c in kv_copies(pair_rows(jp), sem.at[HB + jp]):
                        c.wait()
            for j in [4 * jq + n for n in range(4)]:
                r0 = pl.multiple_of(j * TB, TB)
                q0 = pl.multiple_of(j * hb, hb) + 8
                for g in range(NLB):
                    lb = slice(g * 128, (g + 1) * 128)
                    ke, ko = _halves(k_s[pl.ds(r0, TB), lb])
                    ve, vo = _halves(v_s[pl.ds(r0, TB), lb])
                    kpad[0, g, pl.ds(q0, hb), :] = ke
                    kpad[1, g, pl.ds(q0, hb), :] = ko
                    ke1 = kpad[0, g, pl.ds(q0 - 1, hb), :]
                    ko1 = kpad[1, g, pl.ds(q0 - 1, hb), :]
                    ko2 = kpad[1, g, pl.ds(q0 - 2, hb), :]
                    t0, t1, t2, t3 = (taps[t][g] for t in range(KS))
                    e = (ke * t0 + ko1 * t1 + ke1 * t2 + ko2 * t3) * ve
                    o = (ko * t0 + ke * t1 + ko1 * t2 + ke1 * t3) * vo
                    for rows, (ur, ui) in zip(freq_rows(g), spectrum(e, o)):
                        u_s[j, 0, rows] = ur
                        u_s[j, 1, rows] = ui

        def relayout_rows(t, dst, base, dp, tok=None):
            a = pltpu.bitcast(wraw[t, 2 * dp], U32)
            b = pltpu.bitcast(wraw[t, 2 * dp + 1], U32)
            if tok is not None:
                a = a | tok
            dst[pl.ds(base + dp, 16, stride=WP), :] = (a & jnp.uint32(0xFFFF)) | (b << 16)
            dst[pl.ds(base + 16 * WP + dp, 16, stride=WP), :] = (
                (a >> 16) | (b & jnp.uint32(0xFFFF0000)))

        def norm_rows(r0, nr):
            r0 = pl.multiple_of(r0, 16)
            for r in range(0, nr, 16):
                hl_s[pl.ds(r0 + r, 16), :] = _ln(
                    x_s[pl.ds(r0 + r + LAG * SEG, 16), :].astype(F32)).astype(BF16)

        def pre_queries(c, t=None):
            per = -(-(D // 4) // NQH)
            for sub in range(2):
                if t is not None:
                    half = wraw.at[t, sub * (D // 2):(sub + 1) * (D // 2)]
                    pltpu.make_async_copy(half, half, sem.at[SW + 11 * sub + t]).wait()
                    base = (t - 1) * (H * WP)
                    dp = sub * (D // 4)
                r0 = pl.multiple_of((2 * c + sub) * QR, QR)
                hl = hl_s[pl.ds(r0, QR), :]
                for hd in range(NQH):
                    r = jnp.dot(hl, wslab(0, hd), preferred_element_type=F32)
                    qh_s[hd, pl.ds(r0, QR), :] = r.astype(BF16)
                    if t is not None:
                        tok = pltpu.bitcast(jnp.minimum(jnp.abs(r[0:16]), 0.0), U32)
                        for _ in range(per):
                            if dp < (sub + 1) * (D // 4):
                                relayout_rows(t, wt_kv, base, dp, tok)
                                dp += 1

        nch = NA * SEG // TB
        QR = TB // 2
        with _scope("conv_k"):
            loop(HB // 2, fwd_k)
        with _scope("conv_u"):
            loop(HB // 4, lambda j: fwd_u(j, True))
        with _scope("conv_b"):
            loop(NPOS // 10, lambda j: [u() for n in range(10)
                                        for u in mac_units(pl.multiple_of(80 * j, 16) + 8 * n, 0)])
            xa_copy.wait()

            def inv_first(j):
                part = wraw.at[0, pl.ds(j * DQ, DQ)]
                pltpu.make_async_copy(part, part, sem.at[SW + 10 + j]).wait()
                units = [functools.partial(relayout_rows, 0, wt_q, 0, j * (DQ // 2) + dd)
                         for dd in range(DQ // 2)]
                for u in range(UI):
                    inv_stage(UI * j + u, units)
                assert not units
                norm_rows(j * ((XM - X0) // 2), (XM - X0) // 2)
            loop(HB // UI, inv_first)
        with _scope("rel0"):
            w_copies[0].wait()
            loop((D - 2 * DQ) // 64,
                 lambda i: [relayout_rows(0, wt_q, 0, DQ + i * 32 + dd) for dd in range(32)])
        with _scope("preq"):
            loop(nch - 2, pre_queries)
        with _scope("conv_c"):
            for c in late_copies:
                c.wait()

            def fwd_u_late(j):
                r0 = pl.multiple_of(j * 16, 16)
                hbuf[pl.ds(16 + r0, 16), :] = _ln(x_s[pl.ds(r0, 16), :].astype(F32)).astype(BF16)
                norm_rows(XM - X0 + j * TB, TB)
                fwd_u(HB // 4 + j, False)
            loop(HB // 4, fwd_u_late)
        with _scope("preq_rel"):
            loop(2, lambda i: pre_queries(i + nch - 2, i + 1))

    pl.run_scoped(
        phase0,
        pltpu.VMEM((S, D), BF16),
        pltpu.VMEM((S, D), BF16),
        pltpu.VMEM((HB, D, 2 * TB), BF16),
        pltpu.VMEM((3, D, H, DH), BF16),
        pltpu.VMEM((2, NLB, S // 2 + 32, 128), F32),
        pltpu.VMEM((NA * SEG, D), BF16),
        pltpu.VMEM((KS, D), BF16),
        pltpu.VMEM((D,), BF16),
    )

    def phase1(cq, ckv, co):
        scale = DH ** -0.5

        def masks(mode, q0=0):
            rows = ROWS if mode == 0 else ROWS - SEG
            qi = lax.broadcasted_iota(jnp.int32, (rows - q0, 128), 0) + q0
            kj = lax.broadcasted_iota(jnp.int32, (rows - q0, 128), 1)

            def layer_of(i):
                xl = (i - 2 * M) // SEG if mode == 0 else mode - 1
                return jnp.where(i < 2 * M, i // M, xl)
            same = (layer_of(qi) == layer_of(kj)) & (kj < rows)
            vis = same & ((qi < 2 * M) | (qi >= kj))
            fill = jnp.where(same, -1e9 / scale, -jnp.inf).astype(F32)
            return vis, fill

        mem0 = mem0_ref[0:M, :].astype(F32)

        def seg_row(seg):
            if isinstance(seg, int):
                return min(max(seg, 0), NSEG - 1) * SEG
            return pl.multiple_of(jnp.clip(seg, 0, NSEG - 1) * SEG, SEG)

        def gate(xa, r0, toks=None):
            y = jnp.concatenate([y_s[g, pl.ds(r0, xa.shape[0]), :] for g in range(NLB)], axis=1)
            return xa + _ln(xa, toks) * y

        KH = 256

        def mm(a, b):
            return jnp.dot(a, b, preferred_element_type=F32)

        def row_sums(x1, x2, m_a, m_b):
            (a11, a12), (a21, a22) = x1, x2
            ms = m_a + m_b
            cat = lambda u, v: jnp.concatenate([u, v], axis=0)
            return [a11 + a22, cat(ms, a21 + a22), cat(m_a, a11), cat(m_b, a22),
                    cat(ms, a11 + a12), a21 - a11, a12 - a22]

        def combine(m):
            m1, m2, m3, m4, m5, m16, m17 = m
            m24, m35 = m2 + m4, m3 + m5
            r = 2 * M
            return (jnp.concatenate([m24[:r], m17 + m4[r:] - m5[r:], m24[r:]], axis=0),
                    jnp.concatenate([m35[:r], m35[r:], m16 - m2[r:] + m3[r:]], axis=0))

        def sums_of(b11, b12, b21, b22):
            b11, b12, b21, b22 = (_upk(b).astype(F32) for b in (b11, b12, b21, b22))
            return [_pk(v) for v in (b11 + b22, b12 - b22, b21 - b11, b11 + b12, b21 + b22)]

        def slab_rows(t, h):
            return (wt_kv if t else wt_q), (max(t - 1, 0) * H + (h % 2) * 16 + h // 2) * WP

        def qkv_sum_unit(t, pr, r0, nr, tok=None):
            src, s1 = slab_rows(t, 0)
            s1 = s1 + pr * WP
            s2 = s1 + 16 * WP
            b11 = src[pl.ds(s1 + r0, nr), :]
            if tok is not None:
                b11 = b11 | pltpu.bitcast(tok, U32)
            sm = sums_of(b11, src[pl.ds(s2 + r0, nr), :],
                         src[pl.ds(s1 + 128 + r0, nr), :], src[pl.ds(s2 + 128 + r0, nr), :])
            dst, d0 = (ckv if t else cq), (max(t - 1, 0) * 16 + pr) * 640
            for n, v in enumerate(sm):
                dst[pl.ds(d0 + n * 128 + r0, nr), :] = v

        def o_sum_unit(np_, i, r0, nr, tok=None):
            ka = ((i // 2) * 4 + i % 2) * 64 + r0
            b11 = wo_t[2 * np_, pl.ds(ka, nr), :]
            if tok is not None:
                b11 = b11 | pltpu.bitcast(tok, U32)
            sm = sums_of(b11, wo_t[2 * np_ + 1, pl.ds(ka, nr), :],
                         wo_t[2 * np_, pl.ds(ka + 128, nr), :], wo_t[2 * np_ + 1, pl.ds(ka + 128, nr), :])
            for n, v in enumerate(sm):
                co[pl.ds((np_ * 5 + n) * 1024 + i * 64 + r0, nr), :] = v

        def attention(h, vis, fill, chained, before_oproj=None, early=None, due=(), fast=False,
                      units=()):
            q0 = h.shape[0] - vis.shape[0]
            units = list(units)
            per = -(-len(units) // 96)
            r = 2 * M
            if early is not None:
                hrest = jnp.concatenate([h[:r], h[r + SEG:]], axis=0)
                qrow = pl.multiple_of(early * SEG, SEG)
            if fast:
                sb = sbuf[0:5 * SEG + r, :]
                ms = sb[5 * SEG:]
                cat = lambda u, v: jnp.concatenate([u, v], axis=0)
                lhs = [sb[0:SEG], cat(ms, sb[SEG:2 * SEG]), h[:r + SEG, :KH],
                       cat(h[:r, KH:2 * KH], h[r + SEG:, KH:2 * KH]), cat(ms, sb[2 * SEG:3 * SEG]),
                       sb[3 * SEG:4 * SEG], sb[4 * SEG:5 * SEG]]

            def feed(x):
                if units:
                    tok = jnp.minimum(jnp.abs(x[0:16]), 0.0)
                    for u in units[:per]:
                        u(tok)
                    del units[:per]

            def proj(g):
                res = [[None] * HG for _ in range(3)]
                plain, pairs = [], []
                for t, j in [(t, j) for j in range(HG) for t in range(2)] + [(2, j) for j in range(HG)]:
                    pre = early is not None and t == 0 and g * HG + j < NQH
                    if pre or not fast:
                        plain.append((t, j, pre))
                    elif j % 2 == 0:
                        pairs.append((t, j))

                def csum(t, j, n):
                    d0 = (max(t - 1, 0) * 16 + (g * HG + j) // 2) * 640 + n * 128
                    return _upk((ckv if t else cq)[d0:d0 + 128, :])

                def free_part(t, j):
                    m1 = mm(lhs[0], csum(t, j, 0))
                    return m1, mm(lhs[5], csum(t, j, 3)) + m1, mm(lhs[6], csum(t, j, 4)) + m1

                def do_pair(t, j, fp):
                    w1, w2 = wslab(t, g * HG + j), wslab(t, g * HG + j + 1)
                    m1, m16, m17 = fp
                    feed(m16)
                    m = [m1, mm(lhs[1], w1[:KH]), mm(lhs[2], csum(t, j, 1)), mm(lhs[3], csum(t, j, 2)),
                         mm(lhs[4], w2[KH:2 * KH]), m16, m17]
                    feed(m[4])
                    for n, (c, w) in enumerate(zip(combine(m), (w1, w2))):
                        c = mm(h[:, 2 * KH:], w[2 * KH:]) + c
                        res[t][j + n] = c.astype(BF16) if t == 0 else c

                def do_plain(t, j, pre, part=None):
                    hd = g * HG + j
                    x = hrest if pre else (h if t else h[q0:])
                    if part is None:
                        y = mm(x, wslab(t, hd))
                    else:
                        y = mm(x[:, 2 * KH:], wslab(t, hd)[2 * KH:]) + part
                    feed(y)
                    if t == 0:
                        y = y.astype(BF16)
                    if pre:
                        y = jnp.concatenate([y[:r], qh_s[hd, pl.ds(qrow, SEG), :], y[r:]], axis=0)
                    res[t][j] = y

                first = g == 0 and chained
                fps = [free_part(t, j) for t, j in pairs] if first else None
                nsplit = 4 if first and not fast else 0
                parts = [mm((h if t else h[q0:])[:, :2 * KH], wslab(t, j)[:2 * KH])
                         for t, j, _ in plain[:nsplit]]
                jobs = sorted([(t, j, None) for t, j in pairs] + plain,
                              key=lambda x: (x[0] == 2, x[1], x[0]))
                np_ = 0
                for t, j, pre in jobs:
                    if pre is None:
                        do_pair(t, j, fps[pairs.index((t, j))] if first else free_part(t, j))
                    else:
                        do_plain(t, j, pre, parts[np_] if np_ < nsplit else None)
                        np_ += 1
                return res

            def pad(kv):
                return jnp.concatenate([kv, jnp.zeros((128 - kv.shape[0], DH), F32)],
                                       axis=0).astype(BF16)

            def probs(qkv, g):
                scs = [lax.dot_general(qkv[0][j], pad(qkv[1][j]), (((1,), (1,)), ((), ())),
                                       preferred_element_type=F32) for j in range(HG)]
                ps = []
                for sc in scs:
                    sc = jnp.where(vis, sc, fill)
                    e = jnp.exp2((sc - jnp.max(sc, axis=-1, keepdims=True))
                                 * (scale * math.log2(math.e)))
                    den = jnp.sum(e, axis=-1, keepdims=True)
                    if not ps and g >= NG - len(due):
                        e = jnp.concatenate([e[:16] + due[g - NG + len(due)], e[16:]], axis=0)
                    rc = pl.reciprocal(den, approx=True)
                    rc = rc * (2.0 - den * rc)
                    ps.append((e * rc).astype(BF16))
                return ps

            def oproj(os_, h0, acc, mid=None):
                ext = lambda n, y: y if acc is None else y + acc[n]
                oc = jnp.concatenate(os_, axis=1).astype(BF16)
                k0, k1 = h0 * DH, (h0 + len(os_)) * DH
                res = []
                if fast:
                    ia = [n for n in range(len(os_)) if n % 4 < 2]
                    oa_, ob_ = (jnp.concatenate([os_[n + d] for n in ia], axis=1) for d in (0, 2))
                    ls = [v.astype(BF16) for v in row_sums(
                        (oa_[r:r + SEG], ob_[r:r + SEG]), (oa_[r + SEG:], ob_[r + SEG:]),
                        oa_[:r], ob_[:r])]
                    for np_ in range(2):
                        def cs(n):
                            d0 = (np_ * 5 + n) * 1024 + h0 * 32
                            return _upk(co[d0:d0 + len(os_) * 32, :])

                        def pw(n, d):
                            return _upk(jnp.concatenate(
                                [wo_t[n, (h0 + i + d) * 64:(h0 + i + d + 1) * 64, :] for i in ia], axis=0))
                        ws = [cs(0), pw(2 * np_, 0), cs(1), cs(2), pw(2 * np_ + 1, 2), cs(3), cs(4)]
                        for n in range(7):
                            if mid is not None and len(res) == 9:
                                mid()
                            res.append(ext(len(res), mm(ls[n], ws[n])))
                    res.append(ext(len(res), mm(oc, _upk(wo_t[NLB - 1, k0 // 2:k1 // 2, :]))))
                    return res
                for n in range(NLB):
                    if before_oproj is not None:
                        w = wo_s[k0:k1, n * 128:(n + 1) * 128]
                        wo_t[n, k0 // 2:k1 // 2, :] = pltpu.bitcast(w, U32)
                    else:
                        w = _upk(wo_t[n, k0 // 2:k1 // 2, :])
                    res.append(ext(n, mm(oc, w)))
                if mid is not None:
                    mid()
                return res

            heads = []
            qkv = proj(0)
            oa = None
            for g in range(NG):
                ps = probs(qkv, g)
                vs = qkv[2]

                def weigh():
                    heads.extend(mm(ps[j], pad(vs[j])) for j in range(HG))
                if g + 1 < NG:
                    qkv = proj(g + 1)
                    weigh()
                else:
                    if before_oproj is not None:
                        before_oproj()
                    oa = oproj(heads[:H // 2], 0, None, weigh)
            assert not units
            o = oproj(heads[H // 2:], H // 2, oa)
            if fast:
                cols = []
                for np_ in range(2):
                    m = o[7 * np_:7 * np_ + 7]
                    cols += combine(m[:5] + [m[5] + m[0], m[6] + m[0]])
                o = cols + [o[14]]
            return jnp.concatenate(o, axis=1)

        def post2(s, toks=None):
            r3 = seg_row(s - 1 - LAG)
            for r in (0, 16):
                xc = _r(x2_s[(s + 4 - 1 - LAG) % 4, r:r + 16] + obuf[SEG + r:SEG + r + 16, :])
                out_s[pl.ds(r3 + r, 16), :] = gate(xc, r3 + r, toks).astype(BF16)

        def step(s, mode, vis, fill, chained=False, before_oproj=None, early=None, units=()):
            if mode == 0:
                h = hbuf[0:ROWS, :]
            elif mode == 1:
                h = hbuf[0:48, :]
            else:
                live = lax.broadcasted_iota(jnp.int32, (2 * M, D), 0) >= M
                mem = jnp.where(live, hbuf[0:16, :].astype(F32), 0.0).astype(BF16)
                h = jnp.concatenate([mem, hbuf[48:80, :]], axis=0)
            toks = []
            if mode != 1:
                post2(s, toks)
            if isinstance(s, int) and s == NSEG + LAG - 1:
                obuf[SEG:2 * SEG, :] = attention(h, vis, fill, chained, due=toks)
                return
            r1 = seg_row(s - 1)
            rn = seg_row(s + 1)
            h1n, h2n = [], []
            for r in (0, 16):
                xa = _r(x_s[pl.ds(r1 + r, 16), :].astype(F32) + obuf[r:r + 16, :])
                xb2 = _r(gate(xa, r1 + r))
                h2n.append(_ln(xb2, toks))
                x2_s[(s + 4 - 1) % 4, r:r + 16] = xb2
            if mode != 2:
                for r in (0, 16):
                    h1n.append(_ln(x_s[pl.ds(rn + r, 16), :].astype(F32), toks))

            if early is not None:
                mrow = pl.multiple_of(early * (8 * PPS), 8 * PPS)
                units = [functools.partial(lambda u, tok: u(tok[0:8]), u)
                         for n in range(PPS) for u in mac_units(mrow + 8 * n, 1)]
                units += [functools.partial(qkv_sum_unit, 0, jnp.minimum(early, 15), r0, 16)
                          for r0 in range(0, 128, 16)]

            o = attention(h, vis, fill, chained, before_oproj, early, toks, mode == 0, units)

            mem2 = mem0 if mode == 1 else o[M:2 * M]
            mem = jnp.concatenate([o[0:M], mem2], axis=0)
            hbuf[0:16, :] = mem.astype(BF16)
            for n, v in enumerate(h1n):
                hbuf[16 + 16 * n:32 + 16 * n, :] = v.astype(BF16)
            for n, v in enumerate(h2n):
                hbuf[48 + 16 * n:64 + 16 * n, :] = v.astype(BF16)
            if mode != 2:
                sbuf[5 * SEG:5 * SEG + 2 * M, :] = (mem[:, :KH] + mem[:, KH:2 * KH]).astype(BF16)
                for n, (x1, x2) in enumerate(zip(h1n, h2n)):
                    a11, a12, a21, a22 = x1[:, :KH], x1[:, KH:2 * KH], x2[:, :KH], x2[:, KH:2 * KH]
                    for i, v in enumerate((a11 + a22, a21 + a22, a11 + a12, a21 - a11, a12 - a22)):
                        sbuf[i * SEG + 16 * n:i * SEG + 16 * n + 16, :] = v.astype(BF16)
            if mode == 0:
                obuf[...] = o[2 * M:]
            elif mode == 1:
                obuf[0:SEG, :] = o[2 * M:]
            else:
                obuf[SEG:2 * SEG, :] = o[2 * M:]

        with _scope("pro"):
            vis, fill = masks(1)
            kv_units = [functools.partial(qkv_sum_unit, t, pr, r0, 16)
                        for t in (1, 2) for pr in range(16) for r0 in range(0, 128, 16)]
            o_units = [functools.partial(o_sum_unit, np_, i, r0, 16)
                       for np_ in range(2) for i in range(16) for r0 in range(0, 64, 16)]
            step(0, 1, vis, fill, False, wo_copy.wait, units=kv_units[:192])
            step(1, 1, vis, fill, True, units=kv_units[192:] + o_units)
        xb_copy.start()
        vis, fill = masks(0)
        with _scope("main_a"):
            loop(NA // UA, lambda i: [step(UA * i + u + LAG, 0, vis, fill, u > 0, early=UA * i + u)
                                      for u in range(UA)])
        xb_copy.wait()
        with _scope("conv_e"):
            loop(HB // UI, lambda j: [inv_stage(HB + UI * j + u) for u in range(UI)])
        with _scope("main_b"):
            loop((NSEG - LAG - NA) // UB, lambda i: [step(UB * i + u + LAG + NA, 0, vis, fill, u > 0)
                                                     for u in range(UB)])
        done = (NSEG - 1 - LAG) * SEG
        out_a = pltpu.make_async_copy(out_s.at[0:done, :], out_hbm.at[0:done, :], sem.at[SW + 8])
        out_a.start()
        with _scope("epi"):
            vis, fill = masks(2)
            step(NSEG, 2, vis, fill)
            step(NSEG + 1, 2, *masks(2, 2 * M), True)
        post2(NSEG + LAG)
        out_b = pltpu.make_async_copy(out_s.at[done:S, :], out_hbm.at[done:S, :], sem.at[SW + 9])
        out_b.start()
        out_a.wait()
        out_b.wait()

    pl.run_scoped(
        phase1,
        pltpu.VMEM((H // 2 * 5 * 128, 128), U32),
        pltpu.VMEM((H * 5 * 128, 128), U32),
        pltpu.VMEM((2 * 5 * (H * DH // 4), 128), U32),
    )


@jax.jit
def pallas_interleave_layers__memory_aug_recurrent_mem_tr__ssm_conv_h3__prompt_kernel(
    A_x, A_mem0, A_Wq, A_Wk, A_Wv, A_Wo, A_seg_len,
    B_q, B_k, B_v, B_shift_k, B_ssm_k, B_ssm_D,
):
    del A_seg_len, B_q
    assert A_x.shape == (1, S, D) and A_Wq.shape == (D, H, DH)
    hbm = pl.BlockSpec(memory_space=pl.ANY)
    out = pl.pallas_call(
        _kernel,
        out_shape=jax.ShapeDtypeStruct((S, D), BF16),
        in_specs=[hbm] * 11,
        out_specs=hbm,
        scratch_shapes=[
            pltpu.VMEM((S, D), BF16),
            pltpu.VMEM((H * WP + 352, 128), U32),
            pltpu.VMEM((2 * H * WP + 352, 128), U32),
            pltpu.VMEM((H * DH, D), BF16),
            pltpu.VMEM((NLB, H * DH // 2, 128), U32),
            pltpu.VMEM((TB // 2, TB), U32),
            pltpu.VMEM((2, TB // 2, TB), U32),
            pltpu.VMEM((2, TB // 2, TB), U32),
            pltpu.VMEM((NB, 2, NLB * TB, 128), F32),
            pltpu.VMEM((NB, 3, NLB * TB, 128), F32),
            pltpu.VMEM((NB + 1, 2, NLB * TB, 128), F32),
            pltpu.VMEM((NLB, S + 32, 128), F32),
            pltpu.VMEM((2 * SEG, D), F32),
            pltpu.VMEM((4, SEG, D), F32),
            pltpu.VMEM((S, D), BF16),
            pltpu.VMEM((NQH, NA * SEG, DH), BF16),
            pltpu.VMEM((128, D), BF16),
            pltpu.VMEM((6 * SEG, 256), BF16),
            pltpu.VMEM((64, D), BF16),
            pltpu.SemaphoreType.DMA((HB + HB // 2 + 14,)),
        ],
        compiler_params=pltpu.CompilerParams(vmem_limit_bytes=120 * 1024 * 1024),
    )(A_x.reshape(S, D), A_mem0.reshape(M, D), A_Wq, A_Wk, A_Wv,
      A_Wo.reshape(H * DH, D), B_k.reshape(S, D), B_v.reshape(S, D),
      B_shift_k.T, B_ssm_k, B_ssm_D)
    return out.reshape(1, S, D)
```

```python
import contextlib
import functools
import math

import jax
import jax.numpy as jnp
from jax import lax
import jax.experimental.pallas as pl
import jax.experimental.pallas.tpu as pltpu

F32 = jnp.float32
BF16 = jnp.bfloat16
U32 = jnp.uint32

S = 2048
D = 640
H = 32
DH = 128
M = 8
SEG = 32
NSEG = S // SEG
KS = 4
LAG = 2
ROWS = 2 * M + 2 * SEG
NLB = D // 128
TB = 128
NB = S // TB
HB = NB // 2
NPOS = NLB * TB // 8
NA = 20
PPS = 4
UCUT = tuple(range(a, a + 2) for a in range(0, 12, 2)) + (range(12, 16),)
NQH = 32
UA = 2
UB = 3
UI = 4
WP = 324


STRASSEN = (
    (((1, 0), (0, 1)), ((1, 0), (0, 1)), ((1, 0), (0, 1)), None),
    (((-1, 0), (1, 0)), ((1, 1), (0, 0)), ((0, 0), (0, 1)), None),
    (((0, 1), (0, -1)), ((0, 0), (1, 1)), ((1, 0), (0, 0)), None),
    (((0, 0), (1, 1)), ((1, 0), (0, 0)), ((0, 0), (1, -1)), ((1, 1), (1, 0))),
    (((1, 0), (0, 0)), ((0, 1), (0, -1)), ((0, 1), (0, 1)), ((1, 0), (0, 1))),
    (((0, 0), (0, 1)), ((-1, 0), (1, 0)), ((1, 0), (1, 0)), ((0, 1), (1, 0))),
    (((1, 1), (0, 0)), ((0, 0), (0, 1)), ((-1, 1), (0, 0)), ((1, 1), (0, 1))),
)
HOPKERR = (
    (((1, 0, 0), (0, 0, 0)), ((1, 0, 1), (-1, 0, 0), (0, 0, 0)), ((1, 0, 0), (1, 0, 0)), None),
    (((1, 1, 0), (0, 0, 0)), ((0, 0, 0), (1, 0, 0), (0, 0, 0)), ((1, -1, 0), (0, 0, 0)), None),
    (((-1, 0, 0), (1, 0, 1)), ((0, 0, 1), (0, 0, 0), (1, 0, 0)), ((1, 0, -1), (1, 0, 0)), None),
    (((0, 1, 0), (0, -1, 0)), ((0, 0, 0), (1, 1, 0), (0, -1, 0)), ((0, 1, 0), (0, 0, 0)), None),
    (((0, 1, 1), (0, -1, 0)), ((0, 0, 0), (0, 0, 1), (0, 1, 0)), ((0, 1, 0), (0, 1, -1)), None),
    (((0, 0, 1), (0, 0, 0)), ((0, 0, 0), (0, 0, -1), (1, 0, 1)), ((0, 0, 1), (0, 0, 0)), None),
    (((-1, 0, 0), (1, 0, 0)), ((1, 1, 0), (0, 0, 0), (-1, 0, 0)), ((0, 0, 0), (1, 0, 0)),
     ((1, 0, 0), (1, 0, 0))),
    (((1, 0, 0), (0, 1, 0)), ((0, 1, 0), (1, 0, 0), (0, 0, 0)), ((0, 1, 0), (1, 0, 0)),
     ((0, 1, 0), (1, 0, 0))),
    (((0, 0, 0), (1, 1, 0)), ((0, 1, 0), (0, 0, 0), (0, 0, 0)), ((0, 0, 0), (-1, 1, 0)),
     ((1, 1, 0), (-1, 1, 0))),
    (((0, 0, 0), (1, 0, 1)), ((0, 0, 1), (0, 0, 0), (0, 0, 0)), ((-1, 0, 1), (-1, 0, 1)),
     ((1, 0, 1), (0, 0, 1))),
    (((-1, 0, -1), (1, 0, 1)), ((0, 0, 0), (0, 0, 0), (1, 0, 0)), ((-1, 0, 1), (0, 0, 0)),
     ((1, 0, 1), (1, 0, 0))),
    (((0, 0, 0), (0, 1, 0)), ((0, -1, 0), (0, 1, 1), (0, 0, 0)), ((0, 1, 0), (0, 1, 0)),
     ((0, 1, 0), (0, 1, 0))),
    (((0, 1, 1), (0, 0, 0)), ((0, 0, 0), (0, 0, 1), (0, 0, 0)), ((0, -1, 1), (0, -1, 1)),
     ((0, 1, 0), (0, -1, 1))),
    (((0, -1, -1), (0, 1, 1)), ((0, 0, 0), (0, 0, 0), (0, 1, 0)), ((0, 0, 0), (0, 1, -1)),
     ((0, 0, 1), (0, 1, -1))),
    (((0, 0, 0), (0, 0, 1)), ((0, 0, -1), (0, 0, 0), (0, 1, 1)), ((0, 0, 0), (0, 0, 1)),
     ((0, 0, 1), (0, 0, 1))),
)
BLOCKS = ([(HOPKERR, (0, 1, 2), (3 * i, 3 * i + 1, 3 * i + 2)) for i in range(10)]
          + [(STRASSEN, (3, 4), (2 * i, 2 * i + 1)) for i in range(16)]
          + [(STRASSEN, (0, 1), (30, 31))])
GROUPS = [tuple(range(a, b)) for a, b in ((0, 6), (6, 12), (12, 18), (18, 24), (24, 32))]
NSUM = 10 * 9 + 17 * 5


def _nz(mat):
    return tuple((i, j, c) for i, row in enumerate(mat) for j, c in enumerate(row) if c)


def _summed(alg):
    return [p for p, e in enumerate(alg) if len(_nz(e[1])) > 1]


def _slot(b, p):
    sm = _summed(BLOCKS[b][0])
    if p not in sm:
        return None
    return (9 * b if b < 10 else 90 + 5 * (b - 10)) + sm.index(p)


def _lin(terms):
    terms = sorted(terms, key=lambda t: -t[0])
    acc = terms[0][1]
    for c, v in terms[1:]:
        acc = acc + v if c > 0 else acc - v
    return acc


class _Acc:
    def __init__(self):
        self.d = {}

    def add(self, key, c, v):
        if key not in self.d:
            self.d[key] = (c, v)
            return
        c0, v0 = self.d[key]
        self.d[key] = (c0, v0 + v) if c == c0 else (1, _lin([(c0, v0), (c, v)]))

    def route(self, e, ns, y):
        r = 0 if e[3] is None else 2 * M
        for row, n, c in _nz(e[2]):
            self.add((row + 1, ns[n]), c, y[r:])
        if r:
            for n, c in enumerate(e[3][1]):
                if c:
                    self.add((0, ns[n]), c, y[:r])

    def rows(self, n):
        assert all(self.d[(i, n)][0] == 1 for i in range(3))
        return jnp.concatenate([self.d[(i, n)][1] for i in range(3)], axis=0)


def _row_sigs():
    xs, ms = [], []
    for alg, dts, _ in BLOCKS:
        for e in alg:
            x = tuple((r, dts[k], c) for r, k, c in _nz(e[0]))
            if len(x) > 1 and x not in xs:
                xs.append(x)
            if e[3] is not None:
                m = tuple((dts[k], c) for k, c in enumerate(e[3][0]) if c)
                if len(m) > 1 and m not in ms:
                    ms.append(m)
    return xs, ms


XSIG, MSIG = _row_sigs()
PROFILE = False


def _scope(name):
    return jax.named_scope(name) if PROFILE else contextlib.nullcontext()


def _ln(x, toks=None):
    m = jnp.mean(x, axis=-1, keepdims=True)
    c = x - m
    v = jnp.mean(c * c, axis=-1, keepdims=True)
    r = lax.rsqrt(v + 1e-5)
    if toks is not None:
        toks.append(jnp.minimum(r, 0.0))
    return c * r


def _r(x):
    return x.astype(BF16).astype(F32)


def _split(x):
    hi = pltpu.bitcast(pltpu.bitcast(x, U32) & jnp.uint32(0xFFFF0000), F32)
    return hi, x - hi


def _pk(x):
    return pltpu.bitcast(x.astype(BF16), U32)


def _upk(w):
    return pltpu.bitcast(w, BF16)


def _basis(r, t):
    b = r & 63
    f = jnp.where(b < 32, 2 * b, 2 * b - 63)
    n = ((2 * f + 1) * t - jnp.where(r >= 64, TB, 0)) & (4 * TB - 1)
    n = jnp.where(n >= 2 * TB, n - 4 * TB, n)
    return jnp.cos(n.astype(F32) * (2.0 * math.pi / (4 * TB)))


def _halves(x):
    w = pltpu.bitcast(x, U32)
    return (pltpu.bitcast(w << 16, F32),
            pltpu.bitcast(w & jnp.uint32(0xFFFF0000), F32))


def _kernel(x_hbm, mem0_hbm, wq_hbm, wk_hbm, wv_hbm, wo_hbm,
            k_hbm, v_hbm, shk_hbm, ssmk_hbm, ssmd_hbm,
            out_hbm,
            x_s, wt_q, wt_kv, wo_s, wo_t,
            perm_s, fu_s, inv_s, u_s, kf_s, c_s, y_s,
            obuf, x2_s, out_s, qh_s, hbuf, sbuf, mem0_ref,
            sem):
    X0, XH = LAG * SEG, (LAG + NA) * SEG
    SW = HB + HB // 2
    hb = TB // 2
    wo_copy = pltpu.make_async_copy(wo_hbm, wo_s, sem.at[SW + 3])
    xb_copy = pltpu.make_async_copy(x_hbm.at[XH + SEG:, :], x_s.at[XH + SEG:, :], sem.at[SW + 7])

    def mac_units(row, half):
        rs = pl.ds(row, 8)
        state = {}

        def unit(p, avals, final, tok=None):
            acc = state.setdefault(p, dict(state.get(0, {})))
            for a in avals:
                u = u_s[a, 0, rs] + u_s[a, 1, rs] if p == 0 else u_s[a, p - 1, rs]
                if tok is not None:
                    u = u + tok
                for i in range(max(a, half * HB), half * HB + HB):
                    t = u * kf_s[i - a, p, rs]
                    acc[i] = t if i not in acc else (acc[i] - t if p == 2 else acc[i] + t)
            if final and p:
                for i, v in acc.items():
                    c_s[i + 1, 2 - p, rs] = v

        subs = UCUT if half else (range(HB),)
        return [functools.partial(unit, p, avals, n == len(subs) - 1)
                for p in range(3) for n, avals in enumerate(subs)]

    def inv_stage(i, units=None):
        q = TB // 4
        for g in range(NLB):
            re, im = [], []
            for b in range(4):
                rows = slice(g * TB + b * q, g * TB + (b + 1) * q)
                cr, ci_ = c_s[i + 1, 0, rows], c_s[i + 1, 1, rows]
                pr, pi = c_s[i, 0, rows], c_s[i, 1, rows]
                re.append(cr + pi if b in (0, 3) else cr - pi)
                im.append(ci_ - pr if b in (0, 3) else ci_ + pr)
            pe = jnp.concatenate([re[0] + re[2], re[1] + re[3], im[0] - im[2], im[1] - im[3]], axis=0)
            po = jnp.concatenate([re[0] - re[2], re[1] - re[3], im[0] + im[2], im[1] + im[3]], axis=0)
            for par, pp in enumerate((pe, po)):
                ph, plo = _split(pp)
                gh_, gl_ = (inv_s[n, par * q:(par + 1) * q] for n in range(2))
                y = jnp.dot(_upk(jnp.concatenate([gh_, gl_, gh_], axis=1)),
                            jnp.concatenate([ph, ph, plo], axis=0).astype(BF16),
                            preferred_element_type=F32)
                y_s[g, pl.ds(i * TB + par, hb, stride=2), :] = y
                if units:
                    tok = pltpu.bitcast(jnp.minimum(jnp.abs(y[0:16]), 0.0), U32)
                    for _ in range(3):
                        if units:
                            units.pop(0)(tok)

    def wslab(t, h):
        s0 = (max(t - 1, 0) * H + (h % 2) * 16 + h // 2) * WP
        return pltpu.bitcast((wt_kv if t else wt_q)[s0:s0 + D // 2, :], BF16)

    def loop(n, fn):
        def body(j, _):
            fn(j)
            return 0
        lax.fori_loop(0, n, body, 0)

    def phase0(k_s, v_s, ssmk_s, wraw, kpad, hl_s, shk_ref, ssmd_ref):

        def pair_rows(jp):
            r0 = jp * 2 * TB
            return pl.ds(r0 if isinstance(jp, int) else pl.multiple_of(r0, 2 * TB), 2 * TB)

        def ssmk_copy(jp):
            return pltpu.make_async_copy(ssmk_hbm.at[:, pair_rows(jp)], ssmk_s.at[jp], sem.at[jp])

        def kv_copies(rows, sm):
            return [pltpu.make_async_copy(k_hbm.at[rows, :], k_s.at[rows, :], sm),
                    pltpu.make_async_copy(v_hbm.at[rows, :], v_s.at[rows, :], sm)]
        DQ = 192
        wq_early = [pltpu.make_async_copy(wq_hbm.at[n * DQ:(n + 1) * DQ], wraw.at[0, n * DQ:(n + 1) * DQ],
                                          sem.at[SW + 10 + n]) for n in range(2)]
        w_copies = [pltpu.make_async_copy(wq_hbm.at[2 * DQ:], wraw.at[0, 2 * DQ:], sem.at[SW])]
        w_copies += [pltpu.make_async_copy(w.at[n * (D // 2):(n + 1) * (D // 2)],
                                           wraw.at[t, n * (D // 2):(n + 1) * (D // 2)],
                                           sem.at[SW + 11 * n + t])
                     for t, w in ((1, wk_hbm), (2, wv_hbm)) for n in range(2)]
        late_copies = kv_copies(pl.ds(S // 2, S // 2), sem.at[SW + 4])
        small_copies = [pltpu.make_async_copy(src, dst, sem.at[SW + 5])
                        for src, dst in ((shk_hbm, shk_ref), (ssmd_hbm, ssmd_ref), (mem0_hbm, mem0_ref.at[0:M]))]
        XM = XH - 2 * TB
        xa_copy = pltpu.make_async_copy(x_hbm.at[X0:XM, :], x_s.at[X0:XM, :], sem.at[SW + 6])
        late_copies += [pltpu.make_async_copy(x_hbm.at[a:b, :], x_s.at[a:b, :], sem.at[SW + 4])
                        for a, b in ((0, X0), (XM, XH + SEG))]
        for c in (small_copies + [ssmk_copy(jp) for jp in range(HB)]
                  + [c for jp in range(HB // 2) for c in kv_copies(pair_rows(jp), sem.at[HB + jp])]
                  + [xa_copy] + wq_early + [w_copies[0]] + late_copies + w_copies[1:] + [wo_copy]):
            c.start()

        ri = lax.broadcasted_iota(jnp.int32, (TB, TB), 0)
        ci = lax.broadcasted_iota(jnp.int32, (TB, TB), 1)
        perm_s[...] = _pk(jnp.where(ci == 2 * (ri & 63) + (ri >> 6), 1.0, 0.0))
        tab = _basis(ri, 2 * (ci & 63) + (ci >> 6))
        hi, lo = _split(tab)
        fu_s[0] = _pk(jnp.where(ci < hb, hi, pltpu.roll(lo, hb, 1)))
        fu_s[1] = _pk(jnp.where(ci < hb, pltpu.roll(hi, hb, 1), lo))
        gh, gl = _split(tab.T * (1.0 / TB))
        inv_s[0] = _pk(gh)
        inv_s[1] = _pk(gl)

        for c in small_copies:
            c.wait()
        shk_t = shk_ref[...].astype(F32)
        taps = [[shk_t[j:j + 1, g * 128:(g + 1) * 128] for g in range(NLB)] for j in range(KS)]
        dvec = ssmd_ref[...].astype(F32).reshape(1, D)
        for g in range(NLB):
            kpad[0, g, 0:8, :] = jnp.zeros((8, 128), F32)
            kpad[1, g, 0:8, :] = jnp.zeros((8, 128), F32)
        c_s[0] = jnp.zeros(c_s.shape[1:], F32)
        hbuf[0:16, :] = jnp.concatenate([mem0_ref[0:M, :].astype(F32)] * 2, axis=0).astype(BF16)
        obuf[...] = jnp.zeros((2 * SEG, D), F32)
        x2_s[...] = jnp.zeros(x2_s.shape, F32)

        def spectrum(e, o):
            fe = jnp.dot(_upk(fu_s[0]), jnp.concatenate([e, e], axis=0).astype(BF16), preferred_element_type=F32)
            fo = jnp.dot(_upk(fu_s[1]), jnp.concatenate([o, o], axis=0).astype(BF16), preferred_element_type=F32)
            return ((fe[:hb] + fo[:hb], fe[hb:] + fo[hb:]), (fe[:hb] - fo[:hb], fo[hb:] - fe[hb:]))

        def freq_rows(g):
            return slice(g * TB, g * TB + hb), slice(g * TB + hb, (g + 1) * TB)

        def fwd_k(jq):
            def transposed(n):
                if n % 2 == 0:
                    ssmk_copy(2 * jq + n // 2).wait()
                blk = ssmk_s[2 * jq + n // 2, :, (n % 2) * TB:(n % 2 + 1) * TB]
                return lax.dot_general(_upk(perm_s[...]), blk, (((1,), (1,)), ((), ())),
                                       preferred_element_type=F32)
            nxt = transposed(0)
            for n in range(4):
                kt = nxt
                if n < 3:
                    nxt = transposed(n + 1)
                j = 4 * jq + n
                for g in range(NLB):
                    lb = slice(g * 128, (g + 1) * 128)
                    for rows, (kr, ki) in zip(freq_rows(g), spectrum(kt[:hb, lb], kt[hb:, lb])):
                        if n == 0:
                            kr = kr + jnp.where(j == 0, dvec[:, lb], 0.0)
                        kf_s[j, 0, rows] = kr
                        kf_s[j, 1, rows] = ki - kr
                        kf_s[j, 2, rows] = kr + ki

        def fwd_u(jq, first):
            if first:
                for jp in (2 * jq, 2 * jq + 1):
                    for c in kv_copies(pair_rows(jp), sem.at[HB + jp]):
                        c.wait()
            for j in [4 * jq + n for n in range(4)]:
                r0 = pl.multiple_of(j * TB, TB)
                q0 = pl.multiple_of(j * hb, hb) + 8
                for g in range(NLB):
                    lb = slice(g * 128, (g + 1) * 128)
                    ke, ko = _halves(k_s[pl.ds(r0, TB), lb])
                    ve, vo = _halves(v_s[pl.ds(r0, TB), lb])
                    kpad[0, g, pl.ds(q0, hb), :] = ke
                    kpad[1, g, pl.ds(q0, hb), :] = ko
                    ke1 = kpad[0, g, pl.ds(q0 - 1, hb), :]
                    ko1 = kpad[1, g, pl.ds(q0 - 1, hb), :]
                    ko2 = kpad[1, g, pl.ds(q0 - 2, hb), :]
                    t0, t1, t2, t3 = (taps[t][g] for t in range(KS))
                    e = (ke * t0 + ko1 * t1 + ke1 * t2 + ko2 * t3) * ve
                    o = (ko * t0 + ke * t1 + ko1 * t2 + ke1 * t3) * vo
                    for rows, (ur, ui) in zip(freq_rows(g), spectrum(e, o)):
                        u_s[j, 0, rows] = ur
                        u_s[j, 1, rows] = ui

        def relayout_rows(t, dst, base, dp, tok=None):
            a = pltpu.bitcast(wraw[t, 2 * dp], U32)
            b = pltpu.bitcast(wraw[t, 2 * dp + 1], U32)
            if tok is not None:
                a = a | tok
            dst[pl.ds(base + dp, 16, stride=WP), :] = (a & jnp.uint32(0xFFFF)) | (b << 16)
            dst[pl.ds(base + 16 * WP + dp, 16, stride=WP), :] = (
                (a >> 16) | (b & jnp.uint32(0xFFFF0000)))

        def norm_rows(r0, nr):
            r0 = pl.multiple_of(r0, 16)
            for r in range(0, nr, 16):
                hl_s[pl.ds(r0 + r, 16), :] = _ln(
                    x_s[pl.ds(r0 + r + LAG * SEG, 16), :].astype(F32)).astype(BF16)

        def pre_queries(c, t=None):
            per = -(-(D // 4) // NQH)
            for sub in range(2):
                if t is not None:
                    half = wraw.at[t, sub * (D // 2):(sub + 1) * (D // 2)]
                    pltpu.make_async_copy(half, half, sem.at[SW + 11 * sub + t]).wait()
                    base = (t - 1) * (H * WP)
                    dp = sub * (D // 4)
                r0 = pl.multiple_of((2 * c + sub) * QR, QR)
                hl = hl_s[pl.ds(r0, QR), :]
                for hd in range(NQH):
                    r = jnp.dot(hl, wslab(0, hd), preferred_element_type=F32)
                    qh_s[hd, pl.ds(r0, QR), :] = r.astype(BF16)
                    if t is not None:
                        tok = pltpu.bitcast(jnp.minimum(jnp.abs(r[0:16]), 0.0), U32)
                        for _ in range(per):
                            if dp < (sub + 1) * (D // 4):
                                relayout_rows(t, wt_kv, base, dp, tok)
                                dp += 1

        nch = NA * SEG // TB
        QR = TB // 2
        with _scope("conv_k"):
            loop(HB // 2, fwd_k)
        with _scope("conv_u"):
            loop(HB // 4, lambda j: fwd_u(j, True))
        with _scope("conv_b"):
            loop(NPOS // 10, lambda j: [u() for n in range(10)
                                        for u in mac_units(pl.multiple_of(80 * j, 16) + 8 * n, 0)])
            xa_copy.wait()

            def inv_first(j):
                part = wraw.at[0, pl.ds(j * DQ, DQ)]
                pltpu.make_async_copy(part, part, sem.at[SW + 10 + j]).wait()
                units = [functools.partial(relayout_rows, 0, wt_q, 0, j * (DQ // 2) + dd)
                         for dd in range(DQ // 2)]
                for u in range(UI):
                    inv_stage(UI * j + u, units)
                assert not units
                norm_rows(j * ((XM - X0) // 2), (XM - X0) // 2)
            loop(HB // UI, inv_first)
        with _scope("rel0"):
            w_copies[0].wait()
            loop((D - 2 * DQ) // 64,
                 lambda i: [relayout_rows(0, wt_q, 0, DQ + i * 32 + dd) for dd in range(32)])
        with _scope("preq"):
            loop(nch - 2, pre_queries)
        with _scope("conv_c"):
            for c in late_copies:
                c.wait()

            def fwd_u_late(j):
                r0 = pl.multiple_of(j * 16, 16)
                hbuf[pl.ds(16 + r0, 16), :] = _ln(x_s[pl.ds(r0, 16), :].astype(F32)).astype(BF16)
                norm_rows(XM - X0 + j * TB, TB)
                fwd_u(HB // 4 + j, False)
            loop(HB // 4, fwd_u_late)
        with _scope("preq_rel"):
            loop(2, lambda i: pre_queries(i + nch - 2, i + 1))

    pl.run_scoped(
        phase0,
        pltpu.VMEM((S, D), BF16),
        pltpu.VMEM((S, D), BF16),
        pltpu.VMEM((HB, D, 2 * TB), BF16),
        pltpu.VMEM((3, D, H, DH), BF16),
        pltpu.VMEM((2, NLB, S // 2 + 32, 128), F32),
        pltpu.VMEM((NA * SEG, D), BF16),
        pltpu.VMEM((KS, D), BF16),
        pltpu.VMEM((D,), BF16),
    )

    def phase1(cq, ckv, co):
        scale = DH ** -0.5

        def masks(mode, q0=0):
            rows = ROWS if mode == 0 else ROWS - SEG
            qi = lax.broadcasted_iota(jnp.int32, (rows - q0, 128), 0) + q0
            kj = lax.broadcasted_iota(jnp.int32, (rows - q0, 128), 1)

            def layer_of(i):
                xl = (i - 2 * M) // SEG if mode == 0 else mode - 1
                return jnp.where(i < 2 * M, i // M, xl)
            same = (layer_of(qi) == layer_of(kj)) & (kj < rows)
            vis = same & ((qi < 2 * M) | (qi >= kj))
            fill = jnp.where(same, -1e9 / scale, -jnp.inf).astype(F32)
            return vis, fill

        mem0 = mem0_ref[0:M, :].astype(F32)

        def seg_row(seg):
            if isinstance(seg, int):
                return min(max(seg, 0), NSEG - 1) * SEG
            return pl.multiple_of(jnp.clip(seg, 0, NSEG - 1) * SEG, SEG)

        def gate(xa, r0, toks=None):
            y = jnp.concatenate([y_s[g, pl.ds(r0, xa.shape[0]), :] for g in range(NLB)], axis=1)
            return xa + _ln(xa, toks) * y

        def mm(a, b):
            return jnp.dot(a, b, preferred_element_type=F32)

        def cat(vs, axis=0):
            return vs[0] if len(vs) == 1 else jnp.concatenate(vs, axis=axis)

        def plain_tile(t, dt, hd, r0=0, nr=64):
            if t == 3:
                return wo_t[dt, pl.ds(hd * 64 + r0, nr), :]
            s0 = (max(t - 1, 0) * H + (hd % 2) * 16 + hd // 2) * WP
            return (wt_kv if t else wt_q)[pl.ds(s0 + dt * 64 + r0, nr), :]

        def sum_ref(t):
            return (cq, ckv, ckv, co)[t], (NSUM * 64 if t == 2 else 0)

        def wtile(t, b, p):
            alg, dts, hds = BLOCKS[b]
            if _slot(b, p) is None:
                (k, n, _), = _nz(alg[p][1])
                return plain_tile(t, dts[n], hds[k]) if t == 3 else plain_tile(t, dts[k], hds[n])
            ref, r0 = sum_ref(t)
            r0 += _slot(b, p) * 64
            return ref[r0:r0 + 64, :]

        def sum_unit(t, alg, dts, hds, slot0, r0, tok):
            src = {}
            for k in range(len(dts)):
                for n in range(len(dts)):
                    w = (plain_tile(t, dts[n], hds[k], r0, 8) if t == 3
                         else plain_tile(t, dts[k], hds[n], r0, 8))
                    if k != n:
                        w = w | pltpu.bitcast(tok[0:8], U32)
                    src[k, n] = _upk(w).astype(F32)
            ref, base = sum_ref(t)
            for i, p in enumerate(_summed(alg)):
                ref[pl.ds(base + (slot0 + i) * 64 + r0, 8), :] = _pk(
                    _lin([(c, src[k, n]) for k, n, c in _nz(alg[p][1])]))

        def sum_units(t):
            return [functools.partial(sum_unit, t, *BLOCKS[b], _slot(b, _summed(BLOCKS[b][0])[0]), r0)
                    for b in range(len(BLOCKS)) for r0 in range(0, 64, 8)]

        def attention(h, vis, fill, chained, before_oproj=None, early=None, due=(), fast=False,
                      units=()):
            q0 = h.shape[0] - vis.shape[0]
            r = 2 * M
            units, due = list(units), list(due)
            nprod = sum(len(b[0]) for b in BLOCKS) + 2
            ncall = 3 * H if not fast else (3 * nprod if early is None else 2 * nprod + 5 * H)
            nunit, state = len(units), [0]
            if early is not None:
                hrest = jnp.concatenate([h[:r], h[r + SEG:]], axis=0)
                qrow = pl.multiple_of(early * SEG, SEG)
            if fast:
                sb = sbuf[0:16 * len(XSIG) + 8 * len(MSIG), :]

            def feed(x, weight=1):
                state[0] += weight
                n = -(-nunit * state[0] // ncall) - (nunit - len(units))
                if n > 0:
                    tok = jnp.minimum(jnp.abs(x[0:16]), 0.0)
                    for u in units[:n]:
                        u(tok)
                    del units[:n]

            def left(e, dts):
                x = tuple((row, dts[k], c) for row, k, c in _nz(e[0]))
                if len(x) > 1:
                    parts = [_upk(sb[16 * XSIG.index(x):16 * XSIG.index(x) + 16])]
                else:
                    row, dt, _ = x[0]
                    parts = [h[r + row * SEG:r + (row + 1) * SEG, dt * 128:(dt + 1) * 128]]
                if e[3] is not None:
                    m = tuple((dts[k], c) for k, c in enumerate(e[3][0]) if c)
                    if len(m) > 1:
                        m0 = 16 * len(XSIG) + 8 * MSIG.index(m)
                        parts.insert(0, _upk(sb[m0:m0 + 8]))
                    else:
                        parts.insert(0, h[:r, m[0][0] * 128:(m[0][0] + 1) * 128])
                return cat(parts)

            def proj(g):
                hds = GROUPS[g]
                res = [{} for _ in range(3)]
                first = g == 0 and chained
                kc = D - 128

                def plain(t, hd, part=None):
                    pre = early is not None and t == 0
                    x = hrest if pre else (h if t else h[q0:])
                    if part is None:
                        y = mm(x, wslab(t, hd))
                    else:
                        y = mm(x[:, kc:], wslab(t, hd)[kc:]) + part
                    feed(y, 5 if fast else 1)
                    if t == 0:
                        y = y.astype(BF16)
                    if pre:
                        y = jnp.concatenate([y[:r], qh_s[hd, pl.ds(qrow, SEG), :], y[r:]], axis=0)
                    res[t][hd] = y

                if not fast:
                    order = [(t, hd) for hd in hds for t in range(2)] + [(2, hd) for hd in hds]
                    parts = [mm((h if t else h[q0:])[:, :kc], wslab(t, hd)[:kc])
                             for t, hd in order[:4 if first else 0]]
                    for n, (t, hd) in enumerate(order):
                        plain(t, hd, parts[n] if n < len(parts) else None)
                    return res

                blocks = sorted((b for b in range(len(BLOCKS)) if BLOCKS[b][2][0] in hds),
                                key=lambda b: (max(BLOCKS[b][2]) - 2 * (b < 10), b))
                accs = [_Acc() for _ in range(3)]
                ts = [t for t in range(3) if t or early is None]

                def run(t, b, sel):
                    alg, dts, bh = BLOCKS[b]
                    for p, e in enumerate(alg):
                        if sel(e):
                            y = mm(left(e, dts), _upk(wtile(t, b, p)))
                            feed(y)
                            accs[t].route(e, bh, y)

                lead = [(t, b) for t in ts[:2] for b in blocks] if first else []
                for t, b in lead:
                    run(t, b, lambda e: e[3] is None)
                todo = list(hds) if early is not None else []
                for t in ts:
                    for b in blocks:
                        run(t, b, (lambda e: e[3] is not None) if (t, b) in lead else (lambda e: True))
                        for _ in range(2):
                            if todo and t == 1:
                                plain(0, todo.pop(0))
                    for hd in hds:
                        y = accs[t].rows(hd)
                        if hd >= 30:
                            y = mm(h[:, 256:384], _upk(plain_tile(t, 2, hd))) + y
                            feed(y)
                        res[t][hd] = y.astype(BF16) if t == 0 else y
                assert not todo
                return res

            def pad(kv):
                return jnp.concatenate([kv, jnp.zeros((128 - kv.shape[0], DH), F32)],
                                       axis=0).astype(BF16)

            def probs(qkv, g):
                scs = [lax.dot_general(qkv[0][hd], pad(qkv[1][hd]), (((1,), (1,)), ((), ())),
                                       preferred_element_type=F32) for hd in GROUPS[g]]
                ps = []
                for n, sc in enumerate(scs):
                    sc = jnp.where(vis, sc, fill)
                    e = jnp.exp2((sc - jnp.max(sc, axis=-1, keepdims=True))
                                 * (scale * math.log2(math.e)))
                    den = jnp.sum(e, axis=-1, keepdims=True)
                    if due and g >= 1 and n in ((0, 5) if g > 2 else (0,)):
                        e = jnp.concatenate([e[:16] + due.pop(0), e[16:]], axis=0)
                    rc = pl.reciprocal(den, approx=True)
                    rc = rc * (2.0 - den * rc)
                    ps.append((e * rc).astype(BF16))
                return ps

            def oproj(h0, h1, acc, mid=None):
                def put(key, y):
                    acc[key] = y + acc[key] if key in acc else y

                if not fast:
                    oc = jnp.concatenate(heads[h0:h1], axis=1).astype(BF16)
                    for n in range(NLB):
                        if before_oproj is not None:
                            w = wo_s[h0 * DH:h1 * DH, n * 128:(n + 1) * 128]
                            wo_t[n, h0 * 64:h1 * 64, :] = pltpu.bitcast(w, U32)
                        else:
                            w = _upk(wo_t[n, h0 * 64:h1 * 64, :])
                        put(n, mm(oc, w))
                        if mid is not None and n == NLB - 2:
                            mid()
                    return
                for dts in ((0, 1, 2), (3, 4), (0, 1)):
                    bs = [b for b in range(len(BLOCKS))
                          if BLOCKS[b][1] == dts and h0 <= BLOCKS[b][2][0] < h1]
                    if mid is not None and dts == (3, 4):
                        mid()
                    for p, e in enumerate(BLOCKS[bs[0]][0]) if bs else ():
                        ls = []
                        for b in bs:
                            o = [heads[hd] for hd in BLOCKS[b][2]]
                            parts = [_lin([(c, o[k][r + row * SEG:r + (row + 1) * SEG])
                                           for row, k, c in _nz(e[0])])]
                            if e[3] is not None:
                                parts.insert(0, _lin([(c, o[k][:r])
                                                      for k, c in enumerate(e[3][0]) if c]))
                            ls.append(cat(parts))
                        put((dts, p), mm(cat(ls, 1).astype(BF16),
                                         _upk(cat([wtile(3, b, p) for b in bs]))))
                if h1 == H:
                    put(2, mm(jnp.concatenate(heads[30:], axis=1).astype(BF16),
                              _upk(wo_t[2, 30 * 64:, :])))

            heads, acc = [], {}
            qkv = proj(0)
            for g in range(len(GROUPS)):
                ps = probs(qkv, g)
                vs = [qkv[2][hd] for hd in GROUPS[g]]

                def weigh():
                    heads.extend(mm(p_, pad(v_)) for p_, v_ in zip(ps, vs))
                if g + 1 < len(GROUPS):
                    qkv = proj(g + 1)
                    weigh()
                else:
                    if before_oproj is not None:
                        before_oproj()
                    oproj(0, 18, acc, weigh)
            assert not units and not due
            oproj(18, H, acc)
            if not fast:
                return jnp.concatenate([acc[n] for n in range(NLB)], axis=1)
            out = _Acc()
            for key, y in acc.items():
                if key != 2:
                    out.route((HOPKERR if len(key[0]) == 3 else STRASSEN)[key[1]], key[0], y)
            return jnp.concatenate([out.rows(n) + acc[2] if n == 2 else out.rows(n)
                                    for n in range(NLB)], axis=1)

        def post2(s, toks=None):
            r3 = seg_row(s - 1 - LAG)
            for r in (0, 16):
                xc = _r(x2_s[(s + 4 - 1 - LAG) % 4, r:r + 16] + obuf[SEG + r:SEG + r + 16, :])
                out_s[pl.ds(r3 + r, 16), :] = gate(xc, r3 + r, toks).astype(BF16)

        def step(s, mode, vis, fill, chained=False, before_oproj=None, early=None, units=()):
            if mode == 0:
                h = hbuf[0:ROWS, :]
            elif mode == 1:
                h = hbuf[0:48, :]
            else:
                live = lax.broadcasted_iota(jnp.int32, (2 * M, D), 0) >= M
                mem = jnp.where(live, hbuf[0:16, :].astype(F32), 0.0).astype(BF16)
                h = jnp.concatenate([mem, hbuf[48:80, :]], axis=0)
            toks = []
            if mode != 1:
                post2(s, toks)
            if isinstance(s, int) and s == NSEG + LAG - 1:
                obuf[SEG:2 * SEG, :] = attention(h, vis, fill, chained, due=toks)
                return
            r1 = seg_row(s - 1)
            rn = seg_row(s + 1)
            h1n, h2n = [], []
            for r in (0, 16):
                xa = _r(x_s[pl.ds(r1 + r, 16), :].astype(F32) + obuf[r:r + 16, :])
                xb2 = _r(gate(xa, r1 + r))
                h2n.append(_ln(xb2, toks))
                x2_s[(s + 4 - 1) % 4, r:r + 16] = xb2
            if mode != 2:
                for r in (0, 16):
                    h1n.append(_ln(x_s[pl.ds(rn + r, 16), :].astype(F32), toks))

            if early is not None:
                mrow = pl.multiple_of(early * (8 * PPS), 8 * PPS)
                units = [functools.partial(lambda u, tok: u(tok[0:8]), u)
                         for n in range(PPS) for u in mac_units(mrow + 8 * n, 1)]
                tb = early // 2
                units += [functools.partial(sum_unit, 0, HOPKERR, (0, 1, 2),
                                            (3 * tb, 3 * tb + 1, 3 * tb + 2), 9 * tb,
                                            (early % 2) * 32 + r0) for r0 in range(0, 32, 8)]
                pb = jnp.minimum(early, 16)
                k0, h0 = jnp.where(pb < 16, 3, 0), 2 * jnp.minimum(pb, 15)
                units += [functools.partial(sum_unit, 0, STRASSEN, (k0, k0 + 1), (h0, h0 + 1),
                                            90 + 5 * pb, r0) for r0 in range(0, 64, 8)]

            o = attention(h, vis, fill, chained, before_oproj, early, toks, mode == 0, units)

            mem2 = mem0 if mode == 1 else o[M:2 * M]
            mem = jnp.concatenate([o[0:M], mem2], axis=0)
            hbuf[0:16, :] = mem.astype(BF16)
            for n, v in enumerate(h1n):
                hbuf[16 + 16 * n:32 + 16 * n, :] = v.astype(BF16)
            for n, v in enumerate(h2n):
                hbuf[48 + 16 * n:64 + 16 * n, :] = v.astype(BF16)
            if mode != 2:
                tile = lambda v, dt: v[:, dt * 128:(dt + 1) * 128]
                for i, sig in enumerate(MSIG):
                    m0 = 16 * len(XSIG) + 8 * i
                    sbuf[m0:m0 + 8, :] = _pk(_lin([(c, tile(mem, dt)) for dt, c in sig]))
                for n, xy in enumerate(zip(h1n, h2n)):
                    for i, sig in enumerate(XSIG):
                        sbuf[16 * i + 8 * n:16 * i + 8 * n + 8, :] = _pk(
                            _lin([(c, tile(xy[row], dt)) for row, dt, c in sig]))
            if mode == 0:
                obuf[...] = o[2 * M:]
            elif mode == 1:
                obuf[0:SEG, :] = o[2 * M:]
            else:
                obuf[SEG:2 * SEG, :] = o[2 * M:]

        with _scope("pro"):
            vis, fill = masks(1)
            kv_units = sum_units(1) + sum_units(2)
            cut = len(kv_units) * 3 // 4
            step(0, 1, vis, fill, False, wo_copy.wait, units=kv_units[:cut])
            step(1, 1, vis, fill, True, units=kv_units[cut:] + sum_units(3))
        xb_copy.start()
        vis, fill = masks(0)
        with _scope("main_a"):
            loop(NA // UA, lambda i: [step(UA * i + u + LAG, 0, vis, fill, u > 0, early=UA * i + u)
                                      for u in range(UA)])
        xb_copy.wait()
        with _scope("conv_e"):
            loop(HB // UI, lambda j: [inv_stage(HB + UI * j + u) for u in range(UI)])
        with _scope("main_b"):
            loop((NSEG - LAG - NA) // UB, lambda i: [step(UB * i + u + LAG + NA, 0, vis, fill, u > 0)
                                                     for u in range(UB)])
        done = (NSEG - 1 - LAG) * SEG
        out_a = pltpu.make_async_copy(out_s.at[0:done, :], out_hbm.at[0:done, :], sem.at[SW + 8])
        out_a.start()
        with _scope("epi"):
            vis, fill = masks(2)
            step(NSEG, 2, vis, fill)
            step(NSEG + 1, 2, *masks(2, 2 * M), True)
        post2(NSEG + LAG)
        out_b = pltpu.make_async_copy(out_s.at[done:S, :], out_hbm.at[done:S, :], sem.at[SW + 9])
        out_b.start()
        out_a.wait()
        out_b.wait()

    pl.run_scoped(
        phase1,
        pltpu.VMEM((NSUM * 64, 128), U32),
        pltpu.VMEM((2 * NSUM * 64, 128), U32),
        pltpu.VMEM((NSUM * 64, 128), U32),
    )


@jax.jit
def pallas_interleave_layers__memory_aug_recurrent_mem_tr__ssm_conv_h3__prompt_kernel(
    A_x, A_mem0, A_Wq, A_Wk, A_Wv, A_Wo, A_seg_len,
    B_q, B_k, B_v, B_shift_k, B_ssm_k, B_ssm_D,
):
    del A_seg_len, B_q
    assert A_x.shape == (1, S, D) and A_Wq.shape == (D, H, DH)
    hbm = pl.BlockSpec(memory_space=pl.ANY)
    out = pl.pallas_call(
        _kernel,
        out_shape=jax.ShapeDtypeStruct((S, D), BF16),
        in_specs=[hbm] * 11,
        out_specs=hbm,
        scratch_shapes=[
            pltpu.VMEM((S, D), BF16),
            pltpu.VMEM((H * WP + 352, 128), U32),
            pltpu.VMEM((2 * H * WP + 352, 128), U32),
            pltpu.VMEM((H * DH, D), BF16),
            pltpu.VMEM((NLB, H * DH // 2, 128), U32),
            pltpu.VMEM((TB // 2, TB), U32),
            pltpu.VMEM((2, TB // 2, TB), U32),
            pltpu.VMEM((2, TB // 2, TB), U32),
            pltpu.VMEM((NB, 2, NLB * TB, 128), F32),
            pltpu.VMEM((NB, 3, NLB * TB, 128), F32),
            pltpu.VMEM((NB + 1, 2, NLB * TB, 128), F32),
            pltpu.VMEM((NLB, S + 32, 128), F32),
            pltpu.VMEM((2 * SEG, D), F32),
            pltpu.VMEM((4, SEG, D), F32),
            pltpu.VMEM((S, D), BF16),
            pltpu.VMEM((NQH, NA * SEG, DH), BF16),
            pltpu.VMEM((128, D), BF16),
            pltpu.VMEM((320, 128), U32),
            pltpu.VMEM((64, D), BF16),
            pltpu.SemaphoreType.DMA((HB + HB // 2 + 14,)),
        ],
        compiler_params=pltpu.CompilerParams(vmem_limit_bytes=120 * 1024 * 1024),
    )(A_x.reshape(S, D), A_mem0.reshape(M, D), A_Wq, A_Wk, A_Wv,
      A_Wo.reshape(H * DH, D), B_k.reshape(S, D), B_v.reshape(S, D),
      B_shift_k.T, B_ssm_k, B_ssm_D)
    return out.reshape(1, S, D)
```

```python
import contextlib
import functools
import math

import jax
import jax.numpy as jnp
from jax import lax
import jax.experimental.pallas as pl
import jax.experimental.pallas.tpu as pltpu

F32 = jnp.float32
BF16 = jnp.bfloat16
U32 = jnp.uint32

S = 2048
D = 640
H = 32
DH = 128
M = 8
SEG = 32
NSEG = S // SEG
KS = 4
LAG = 2
ROWS = 2 * M + 2 * SEG
NLB = D // 128
TB = 128
NB = S // TB
HB = NB // 2
NPOS = NLB * TB // 8
NA = 20
PPS = 4
UCUT = tuple(range(a, a + 2) for a in range(0, 12, 2)) + (range(12, 16),)
NQH = 32
UA = 2
UB = 3
UI = 4
WP = 324


STRASSEN = (
    (((1, 0), (0, 1)), ((1, 0), (0, 1)), ((1, 0), (0, 1)), None),
    (((-1, 0), (1, 0)), ((1, 1), (0, 0)), ((0, 0), (0, 1)), None),
    (((0, 1), (0, -1)), ((0, 0), (1, 1)), ((1, 0), (0, 0)), None),
    (((0, 0), (1, 1)), ((1, 0), (0, 0)), ((0, 0), (1, -1)), ((1, 1), (1, 0))),
    (((1, 0), (0, 0)), ((0, 1), (0, -1)), ((0, 1), (0, 1)), ((1, 0), (0, 1))),
    (((0, 0), (0, 1)), ((-1, 0), (1, 0)), ((1, 0), (1, 0)), ((0, 1), (1, 0))),
    (((1, 1), (0, 0)), ((0, 0), (0, 1)), ((-1, 1), (0, 0)), ((1, 1), (0, 1))),
)
HOPKERR = (
    (((1, 0, 0), (0, 0, 0)), ((1, 0, 1), (-1, 0, 0), (0, 0, 0)), ((1, 0, 0), (1, 0, 0)), None),
    (((1, 1, 0), (0, 0, 0)), ((0, 0, 0), (1, 0, 0), (0, 0, 0)), ((1, -1, 0), (0, 0, 0)), None),
    (((-1, 0, 0), (1, 0, 1)), ((0, 0, 1), (0, 0, 0), (1, 0, 0)), ((1, 0, -1), (1, 0, 0)), None),
    (((0, 1, 0), (0, -1, 0)), ((0, 0, 0), (1, 1, 0), (0, -1, 0)), ((0, 1, 0), (0, 0, 0)), None),
    (((0, 1, 1), (0, -1, 0)), ((0, 0, 0), (0, 0, 1), (0, 1, 0)), ((0, 1, 0), (0, 1, -1)), None),
    (((0, 0, 1), (0, 0, 0)), ((0, 0, 0), (0, 0, -1), (1, 0, 1)), ((0, 0, 1), (0, 0, 0)), None),
    (((-1, 0, 0), (1, 0, 0)), ((1, 1, 0), (0, 0, 0), (-1, 0, 0)), ((0, 0, 0), (1, 0, 0)),
     ((1, 0, 0), (1, 0, 0))),
    (((1, 0, 0), (0, 1, 0)), ((0, 1, 0), (1, 0, 0), (0, 0, 0)), ((0, 1, 0), (1, 0, 0)),
     ((0, 1, 0), (1, 0, 0))),
    (((0, 0, 0), (1, 1, 0)), ((0, 1, 0), (0, 0, 0), (0, 0, 0)), ((0, 0, 0), (-1, 1, 0)),
     ((1, 1, 0), (-1, 1, 0))),
    (((0, 0, 0), (1, 0, 1)), ((0, 0, 1), (0, 0, 0), (0, 0, 0)), ((-1, 0, 1), (-1, 0, 1)),
     ((1, 0, 1), (0, 0, 1))),
    (((-1, 0, -1), (1, 0, 1)), ((0, 0, 0), (0, 0, 0), (1, 0, 0)), ((-1, 0, 1), (0, 0, 0)),
     ((1, 0, 1), (1, 0, 0))),
    (((0, 0, 0), (0, 1, 0)), ((0, -1, 0), (0, 1, 1), (0, 0, 0)), ((0, 1, 0), (0, 1, 0)),
     ((0, 1, 0), (0, 1, 0))),
    (((0, 1, 1), (0, 0, 0)), ((0, 0, 0), (0, 0, 1), (0, 0, 0)), ((0, -1, 1), (0, -1, 1)),
     ((0, 1, 0), (0, -1, 1))),
    (((0, -1, -1), (0, 1, 1)), ((0, 0, 0), (0, 0, 0), (0, 1, 0)), ((0, 0, 0), (0, 1, -1)),
     ((0, 0, 1), (0, 1, -1))),
    (((0, 0, 0), (0, 0, 1)), ((0, 0, -1), (0, 0, 0), (0, 1, 1)), ((0, 0, 0), (0, 0, 1)),
     ((0, 0, 1), (0, 0, 1))),
)
BLOCKS = ([(HOPKERR, (0, 1, 2), (3 * i, 3 * i + 1, 3 * i + 2)) for i in range(10)]
          + [(STRASSEN, (3, 4), (2 * i, 2 * i + 1)) for i in range(16)]
          + [(STRASSEN, (0, 1), (30, 31))])
GROUPS = [tuple(range(a, b)) for a, b in ((0, 6), (6, 12), (12, 18), (18, 24), (24, 32))]
NSUM = 10 * 9 + 17 * 5


def _nz(mat):
    return tuple((i, j, c) for i, row in enumerate(mat) for j, c in enumerate(row) if c)


def _summed(alg):
    return [p for p, e in enumerate(alg) if len(_nz(e[1])) > 1]


def _slot(b, p):
    sm = _summed(BLOCKS[b][0])
    if p not in sm:
        return None
    return (9 * b if b < 10 else 90 + 5 * (b - 10)) + sm.index(p)


def _lin(terms):
    terms = sorted(terms, key=lambda t: -t[0])
    acc = terms[0][1]
    for c, v in terms[1:]:
        acc = acc + v if c > 0 else acc - v
    return acc


class _Acc:
    def __init__(self):
        self.d = {}

    def add(self, key, c, v):
        if key not in self.d:
            self.d[key] = (c, v)
            return
        c0, v0 = self.d[key]
        self.d[key] = (c0, v0 + v) if c == c0 else (1, _lin([(c0, v0), (c, v)]))

    def route(self, e, ns, y):
        r = 0 if e[3] is None else 2 * M
        for row, n, c in _nz(e[2]):
            self.add((row + 1, ns[n]), c, y[r:])
        if r:
            for n, c in enumerate(e[3][1]):
                if c:
                    self.add((0, ns[n]), c, y[:r])

    def rows(self, n):
        assert all(self.d[(i, n)][0] == 1 for i in range(3))
        return jnp.concatenate([self.d[(i, n)][1] for i in range(3)], axis=0)


def _row_sigs():
    xs, ms = [], []
    for alg, dts, _ in BLOCKS:
        for e in alg:
            x = tuple((r, dts[k], c) for r, k, c in _nz(e[0]))
            if len(x) > 1 and x not in xs:
                xs.append(x)
            if e[3] is not None:
                m = tuple((dts[k], c) for k, c in enumerate(e[3][0]) if c)
                if len(m) > 1 and m not in ms:
                    ms.append(m)
    return xs, ms


XSIG, MSIG = _row_sigs()
PROFILE = False


def _scope(name):
    return jax.named_scope(name) if PROFILE else contextlib.nullcontext()


def _ln(x, toks=None):
    m = jnp.mean(x, axis=-1, keepdims=True)
    c = x - m
    v = jnp.mean(c * c, axis=-1, keepdims=True)
    r = lax.rsqrt(v + 1e-5)
    if toks is not None:
        toks.append(jnp.minimum(r, 0.0))
    return c * r


def _r(x):
    return x.astype(BF16).astype(F32)


def _split(x):
    hi = pltpu.bitcast(pltpu.bitcast(x, U32) & jnp.uint32(0xFFFF0000), F32)
    return hi, x - hi


def _pk(x):
    return pltpu.bitcast(x.astype(BF16), U32)


def _upk(w):
    return pltpu.bitcast(w, BF16)


def _basis(r, t):
    b = r & 63
    f = jnp.where(b < 32, 2 * b, 2 * b - 63)
    n = ((2 * f + 1) * t - jnp.where(r >= 64, TB, 0)) & (4 * TB - 1)
    n = jnp.where(n >= 2 * TB, n - 4 * TB, n)
    return jnp.cos(n.astype(F32) * (2.0 * math.pi / (4 * TB)))


def _halves(x):
    w = pltpu.bitcast(x, U32)
    return (pltpu.bitcast(w << 16, F32),
            pltpu.bitcast(w & jnp.uint32(0xFFFF0000), F32))


def _kernel(x_hbm, mem0_hbm, wq_hbm, wk_hbm, wv_hbm, wo_hbm,
            k_hbm, v_hbm, shk_hbm, ssmk_hbm, ssmd_hbm,
            out_hbm,
            x_s, wt_q, wt_kv, wo_s, wo_t,
            perm_s, fu_s, inv_s, u_s, kf_s, c_s, y_s,
            obuf, x2_s, out_s, qh_s, hbuf, sbuf, mem0_ref,
            sem):
    X0, XH = LAG * SEG, (LAG + NA) * SEG
    SW = HB + HB // 2
    hb = TB // 2
    wo_copy = pltpu.make_async_copy(wo_hbm, wo_s, sem.at[SW + 3])
    xb_copy = pltpu.make_async_copy(x_hbm.at[XH + SEG:, :], x_s.at[XH + SEG:, :], sem.at[SW + 7])

    def mac_units(row, half):
        rs = pl.ds(row, 8)
        state = {}

        def unit(p, avals, final, tok=None):
            acc = state.setdefault(p, dict(state.get(0, {})))
            for a in avals:
                u = u_s[a, 0, rs] + u_s[a, 1, rs] if p == 0 else u_s[a, p - 1, rs]
                if tok is not None:
                    u = u + tok
                for i in range(max(a, half * HB), half * HB + HB):
                    t = u * kf_s[i - a, p, rs]
                    acc[i] = t if i not in acc else (acc[i] - t if p == 2 else acc[i] + t)
            if final and p:
                for i, v in acc.items():
                    c_s[i + 1, 2 - p, rs] = v

        subs = UCUT if half else (range(HB),)
        return [functools.partial(unit, p, avals, n == len(subs) - 1)
                for p in range(3) for n, avals in enumerate(subs)]

    def inv_stage(i, units=None):
        q = TB // 4
        for g in range(NLB):
            re, im = [], []
            for b in range(4):
                rows = slice(g * TB + b * q, g * TB + (b + 1) * q)
                cr, ci_ = c_s[i + 1, 0, rows], c_s[i + 1, 1, rows]
                pr, pi = c_s[i, 0, rows], c_s[i, 1, rows]
                re.append(cr + pi if b in (0, 3) else cr - pi)
                im.append(ci_ - pr if b in (0, 3) else ci_ + pr)
            pe = jnp.concatenate([re[0] + re[2], re[1] + re[3], im[0] - im[2], im[1] - im[3]], axis=0)
            po = jnp.concatenate([re[0] - re[2], re[1] - re[3], im[0] + im[2], im[1] + im[3]], axis=0)
            for par, pp in enumerate((pe, po)):
                ph, plo = _split(pp)
                gh_, gl_ = (inv_s[n, par * q:(par + 1) * q] for n in range(2))
                y = jnp.dot(_upk(jnp.concatenate([gh_, gl_, gh_], axis=1)),
                            jnp.concatenate([ph, ph, plo], axis=0).astype(BF16),
                            preferred_element_type=F32)
                y_s[g, pl.ds(i * TB + par, hb, stride=2), :] = y
                if units:
                    tok = pltpu.bitcast(jnp.minimum(jnp.abs(y[0:16]), 0.0), U32)
                    for _ in range(3):
                        if units:
                            units.pop(0)(tok)

    def wslab(t, h):
        s0 = (max(t - 1, 0) * H + (h % 2) * 16 + h // 2) * WP
        return pltpu.bitcast((wt_kv if t else wt_q)[s0:s0 + D // 2, :], BF16)

    def loop(n, fn):
        def body(j, _):
            fn(j)
            return 0
        lax.fori_loop(0, n, body, 0)

    def phase0(k_s, v_s, ssmk_s, wraw, kpad, hl_s, shk_ref, ssmd_ref):

        def pair_rows(jp):
            r0 = jp * 2 * TB
            return pl.ds(r0 if isinstance(jp, int) else pl.multiple_of(r0, 2 * TB), 2 * TB)

        def ssmk_copy(jp):
            return pltpu.make_async_copy(ssmk_hbm.at[:, pair_rows(jp)], ssmk_s.at[jp], sem.at[jp])

        def kv_copies(rows, sm):
            return [pltpu.make_async_copy(k_hbm.at[rows, :], k_s.at[rows, :], sm),
                    pltpu.make_async_copy(v_hbm.at[rows, :], v_s.at[rows, :], sm)]
        DQ = 192
        wq_early = [pltpu.make_async_copy(wq_hbm.at[n * DQ:(n + 1) * DQ], wraw.at[0, n * DQ:(n + 1) * DQ],
                                          sem.at[SW + 10 + n]) for n in range(2)]
        w_copies = [pltpu.make_async_copy(wq_hbm.at[2 * DQ:], wraw.at[0, 2 * DQ:], sem.at[SW])]
        w_copies += [pltpu.make_async_copy(w.at[n * (D // 2):(n + 1) * (D // 2)],
                                           wraw.at[t, n * (D // 2):(n + 1) * (D // 2)],
                                           sem.at[SW + 11 * n + t])
                     for t, w in ((1, wk_hbm), (2, wv_hbm)) for n in range(2)]
        late_copies = kv_copies(pl.ds(S // 2, S // 2), sem.at[SW + 4])
        small_copies = [pltpu.make_async_copy(src, dst, sem.at[SW + 5])
                        for src, dst in ((shk_hbm, shk_ref), (ssmd_hbm, ssmd_ref), (mem0_hbm, mem0_ref.at[0:M]))]
        XM = XH - 2 * TB
        xa_copy = pltpu.make_async_copy(x_hbm.at[X0:XM, :], x_s.at[X0:XM, :], sem.at[SW + 6])
        late_copies += [pltpu.make_async_copy(x_hbm.at[a:b, :], x_s.at[a:b, :], sem.at[SW + 4])
                        for a, b in ((0, X0), (XM, XH + SEG))]
        for c in (small_copies + [ssmk_copy(jp) for jp in range(HB)]
                  + [c for jp in range(HB // 2) for c in kv_copies(pair_rows(jp), sem.at[HB + jp])]
                  + [xa_copy] + wq_early + [w_copies[0]] + late_copies + w_copies[1:] + [wo_copy]):
            c.start()

        ri = lax.broadcasted_iota(jnp.int32, (TB, TB), 0)
        ci = lax.broadcasted_iota(jnp.int32, (TB, TB), 1)
        perm_s[...] = _pk(jnp.where(ci == 2 * (ri & 63) + (ri >> 6), 1.0, 0.0))
        tab = _basis(ri, 2 * (ci & 63) + (ci >> 6))
        hi, lo = _split(tab)
        fu_s[0] = _pk(jnp.where(ci < hb, hi, pltpu.roll(lo, hb, 1)))
        fu_s[1] = _pk(jnp.where(ci < hb, pltpu.roll(hi, hb, 1), lo))
        gh, gl = _split(tab.T * (1.0 / TB))
        inv_s[0] = _pk(gh)
        inv_s[1] = _pk(gl)

        for c in small_copies:
            c.wait()
        shk_t = shk_ref[...].astype(F32)
        taps = [[shk_t[j:j + 1, g * 128:(g + 1) * 128] for g in range(NLB)] for j in range(KS)]
        dvec = ssmd_ref[...].astype(F32).reshape(1, D)
        for g in range(NLB):
            kpad[0, g, 0:8, :] = jnp.zeros((8, 128), F32)
            kpad[1, g, 0:8, :] = jnp.zeros((8, 128), F32)
        c_s[0] = jnp.zeros(c_s.shape[1:], F32)
        hbuf[0:16, :] = jnp.concatenate([mem0_ref[0:M, :].astype(F32)] * 2, axis=0).astype(BF16)
        obuf[...] = jnp.zeros((2 * SEG, D), F32)
        x2_s[...] = jnp.zeros(x2_s.shape, F32)

        def spectrum(e, o):
            fe = jnp.dot(_upk(fu_s[0]), jnp.concatenate([e, e], axis=0).astype(BF16), preferred_element_type=F32)
            fo = jnp.dot(_upk(fu_s[1]), jnp.concatenate([o, o], axis=0).astype(BF16), preferred_element_type=F32)
            return ((fe[:hb] + fo[:hb], fe[hb:] + fo[hb:]), (fe[:hb] - fo[:hb], fo[hb:] - fe[hb:]))

        def freq_rows(g):
            return slice(g * TB, g * TB + hb), slice(g * TB + hb, (g + 1) * TB)

        def fwd_k(jq):
            def transposed(n):
                if n % 2 == 0:
                    ssmk_copy(2 * jq + n // 2).wait()
                blk = ssmk_s[2 * jq + n // 2, :, (n % 2) * TB:(n % 2 + 1) * TB]
                return lax.dot_general(_upk(perm_s[...]), blk, (((1,), (1,)), ((), ())),
                                       preferred_element_type=F32)
            nxt = transposed(0)
            for n in range(4):
                kt = nxt
                if n < 3:
                    nxt = transposed(n + 1)
                j = 4 * jq + n
                for g in range(NLB):
                    lb = slice(g * 128, (g + 1) * 128)
                    for rows, (kr, ki) in zip(freq_rows(g), spectrum(kt[:hb, lb], kt[hb:, lb])):
                        if n == 0:
                            kr = kr + jnp.where(j == 0, dvec[:, lb], 0.0)
                        kf_s[j, 0, rows] = kr
                        kf_s[j, 1, rows] = ki - kr
                        kf_s[j, 2, rows] = kr + ki

        def fwd_u(jq, first):
            if first:
                for jp in (2 * jq, 2 * jq + 1):
                    for c in kv_copies(pair_rows(jp), sem.at[HB + jp]):
                        c.wait()
            for j in [4 * jq + n for n in range(4)]:
                r0 = pl.multiple_of(j * TB, TB)
                q0 = pl.multiple_of(j * hb, hb) + 8
                for g in range(NLB):
                    lb = slice(g * 128, (g + 1) * 128)
                    ke, ko = _halves(k_s[pl.ds(r0, TB), lb])
                    ve, vo = _halves(v_s[pl.ds(r0, TB), lb])
                    kpad[0, g, pl.ds(q0, hb), :] = ke
                    kpad[1, g, pl.ds(q0, hb), :] = ko
                    ke1 = kpad[0, g, pl.ds(q0 - 1, hb), :]
                    ko1 = kpad[1, g, pl.ds(q0 - 1, hb), :]
                    ko2 = kpad[1, g, pl.ds(q0 - 2, hb), :]
                    t0, t1, t2, t3 = (taps[t][g] for t in range(KS))
                    e = (ke * t0 + ko1 * t1 + ke1 * t2 + ko2 * t3) * ve
                    o = (ko * t0 + ke * t1 + ko1 * t2 + ke1 * t3) * vo
                    for rows, (ur, ui) in zip(freq_rows(g), spectrum(e, o)):
                        u_s[j, 0, rows] = ur
                        u_s[j, 1, rows] = ui

        def relayout_rows(t, dst, base, dp, tok=None):
            a = pltpu.bitcast(wraw[t, 2 * dp], U32)
            b = pltpu.bitcast(wraw[t, 2 * dp + 1], U32)
            if tok is not None:
                a = a | tok
            dst[pl.ds(base + dp, 16, stride=WP), :] = (a & jnp.uint32(0xFFFF)) | (b << 16)
            dst[pl.ds(base + 16 * WP + dp, 16, stride=WP), :] = (
                (a >> 16) | (b & jnp.uint32(0xFFFF0000)))

        def norm_rows(r0, nr):
            r0 = pl.multiple_of(r0, 16)
            for r in range(0, nr, 16):
                hl_s[pl.ds(r0 + r, 16), :] = _ln(
                    x_s[pl.ds(r0 + r + LAG * SEG, 16), :].astype(F32)).astype(BF16)

        def pre_queries(c, t=None):
            per = -(-(D // 4) // NQH)
            for sub in range(2):
                if t is not None:
                    half = wraw.at[t, sub * (D // 2):(sub + 1) * (D // 2)]
                    pltpu.make_async_copy(half, half, sem.at[SW + 11 * sub + t]).wait()
                    base = (t - 1) * (H * WP)
                    dp = sub * (D // 4)
                r0 = pl.multiple_of((2 * c + sub) * QR, QR)
                hl = hl_s[pl.ds(r0, QR), :]
                for hd in range(NQH):
                    r = jnp.dot(hl, wslab(0, hd), preferred_element_type=F32)
                    qh_s[hd, pl.ds(r0, QR), :] = r.astype(BF16)
                    if t is not None:
                        tok = pltpu.bitcast(jnp.minimum(jnp.abs(r[0:16]), 0.0), U32)
                        for _ in range(per):
                            if dp < (sub + 1) * (D // 4):
                                relayout_rows(t, wt_kv, base, dp, tok)
                                dp += 1

        nch = NA * SEG // TB
        QR = TB // 2
        with _scope("conv_k"):
            loop(HB // 2, fwd_k)
        with _scope("conv_u"):
            loop(HB // 4, lambda j: fwd_u(j, True))
        with _scope("conv_b"):
            loop(NPOS // 10, lambda j: [u() for n in range(10)
                                        for u in mac_units(pl.multiple_of(80 * j, 16) + 8 * n, 0)])
            xa_copy.wait()

            def inv_first(j):
                part = wraw.at[0, pl.ds(j * DQ, DQ)]
                pltpu.make_async_copy(part, part, sem.at[SW + 10 + j]).wait()
                units = [functools.partial(relayout_rows, 0, wt_q, 0, j * (DQ // 2) + dd)
                         for dd in range(DQ // 2)]
                for u in range(UI):
                    inv_stage(UI * j + u, units)
                assert not units
                norm_rows(j * ((XM - X0) // 2), (XM - X0) // 2)
            loop(HB // UI, inv_first)
        with _scope("rel0"):
            w_copies[0].wait()
            loop((D - 2 * DQ) // 64,
                 lambda i: [relayout_rows(0, wt_q, 0, DQ + i * 32 + dd) for dd in range(32)])
        with _scope("preq"):
            loop(nch - 2, pre_queries)
        with _scope("conv_c"):
            for c in late_copies:
                c.wait()

            def fwd_u_late(j):
                r0 = pl.multiple_of(j * 16, 16)
                hbuf[pl.ds(16 + r0, 16), :] = _ln(x_s[pl.ds(r0, 16), :].astype(F32)).astype(BF16)
                norm_rows(XM - X0 + j * TB, TB)
                fwd_u(HB // 4 + j, False)
            loop(HB // 4, fwd_u_late)
        with _scope("preq_rel"):
            loop(2, lambda i: pre_queries(i + nch - 2, i + 1))

    pl.run_scoped(
        phase0,
        pltpu.VMEM((S, D), BF16),
        pltpu.VMEM((S, D), BF16),
        pltpu.VMEM((HB, D, 2 * TB), BF16),
        pltpu.VMEM((3, D, H, DH), BF16),
        pltpu.VMEM((2, NLB, S // 2 + 32, 128), F32),
        pltpu.VMEM((NA * SEG, D), BF16),
        pltpu.VMEM((KS, D), BF16),
        pltpu.VMEM((D,), BF16),
    )

    def phase1(cq, ckv, co):
        scale = DH ** -0.5

        def masks(mode, q0=0):
            rows = ROWS if mode == 0 else ROWS - SEG
            qi = lax.broadcasted_iota(jnp.int32, (rows - q0, 128), 0) + q0
            kj = lax.broadcasted_iota(jnp.int32, (rows - q0, 128), 1)

            def layer_of(i):
                xl = (i - 2 * M) // SEG if mode == 0 else mode - 1
                return jnp.where(i < 2 * M, i // M, xl)
            same = (layer_of(qi) == layer_of(kj)) & (kj < rows)
            vis = same & ((qi < 2 * M) | (qi >= kj))
            fill = jnp.where(same, -1e9 / scale, -jnp.inf).astype(F32)
            return vis, fill

        mem0 = mem0_ref[0:M, :].astype(F32)

        def seg_row(seg):
            if isinstance(seg, int):
                return min(max(seg, 0), NSEG - 1) * SEG
            return pl.multiple_of(jnp.clip(seg, 0, NSEG - 1) * SEG, SEG)

        def gate(xa, r0, toks=None):
            y = jnp.concatenate([y_s[g, pl.ds(r0, xa.shape[0]), :] for g in range(NLB)], axis=1)
            return xa + _ln(xa, toks) * y

        def mm(a, b):
            return jnp.dot(a, b, preferred_element_type=F32)

        def cat(vs, axis=0):
            return vs[0] if len(vs) == 1 else jnp.concatenate(vs, axis=axis)

        def plain_tile(t, dt, hd, r0=0, nr=64):
            if t == 3:
                return wo_t[dt, pl.ds(hd * 64 + r0, nr), :]
            s0 = (max(t - 1, 0) * H + (hd % 2) * 16 + hd // 2) * WP
            return (wt_kv if t else wt_q)[pl.ds(s0 + dt * 64 + r0, nr), :]

        def sum_ref(t):
            return (cq, ckv, ckv, co)[t], (NSUM * 64 if t == 2 else 0)

        def wtile(t, b, p):
            alg, dts, hds = BLOCKS[b]
            if _slot(b, p) is None:
                (k, n, _), = _nz(alg[p][1])
                return plain_tile(t, dts[n], hds[k]) if t == 3 else plain_tile(t, dts[k], hds[n])
            ref, r0 = sum_ref(t)
            r0 += _slot(b, p) * 64
            return ref[r0:r0 + 64, :]

        def sum_unit(t, alg, dts, hds, slot0, r0, tok):
            src = {}
            for k in range(len(dts)):
                for n in range(len(dts)):
                    w = (plain_tile(t, dts[n], hds[k], r0, 8) if t == 3
                         else plain_tile(t, dts[k], hds[n], r0, 8))
                    if (n - k) % len(dts) == len(dts) - 2:
                        w = w | pltpu.bitcast(tok[0:8], U32)
                    src[k, n] = _upk(w).astype(F32)
            ref, base = sum_ref(t)
            sums = _pk(jnp.concatenate([_lin([(c, src[k, n]) for k, n, c in _nz(alg[p][1])])
                                        for p in _summed(alg)], axis=1))
            for i in range(len(_summed(alg))):
                ref[pl.ds(base + (slot0 + i) * 64 + r0, 8), :] = sums[:, i * 128:(i + 1) * 128]

        def sum_units(t):
            return [functools.partial(sum_unit, t, *BLOCKS[b], _slot(b, _summed(BLOCKS[b][0])[0]), r0)
                    for b in range(len(BLOCKS)) for r0 in range(0, 64, 8)]

        def attention(h, vis, fill, chained, before_oproj=None, early=None, due=(), fast=False,
                      units=()):
            q0 = h.shape[0] - vis.shape[0]
            r = 2 * M
            units, due = list(units), list(due)
            nprod = sum(len(b[0]) for b in BLOCKS) + 2
            ncall = 4 * H - 6 if not fast else (3 * nprod if early is None else 2 * nprod + 5 * H)
            nunit, state = len(units), [0]
            if early is not None:
                hrest = jnp.concatenate([h[:r], h[r + SEG:]], axis=0)
                qrow = pl.multiple_of(early * SEG, SEG)
            if fast:
                sb = sbuf[0:16 * len(XSIG) + 8 * len(MSIG), :]

            def feed(x, weight=1):
                state[0] += weight
                n = -(-nunit * state[0] // ncall) - (nunit - len(units))
                if n > 0:
                    tok = jnp.minimum(jnp.abs(x[0:16]), 0.0)
                    for u in units[:n]:
                        u(tok)
                    del units[:n]

            def left(e, dts):
                x = tuple((row, dts[k], c) for row, k, c in _nz(e[0]))
                if len(x) > 1:
                    parts = [_upk(sb[16 * XSIG.index(x):16 * XSIG.index(x) + 16])]
                else:
                    row, dt, _ = x[0]
                    parts = [h[r + row * SEG:r + (row + 1) * SEG, dt * 128:(dt + 1) * 128]]
                if e[3] is not None:
                    m = tuple((dts[k], c) for k, c in enumerate(e[3][0]) if c)
                    if len(m) > 1:
                        m0 = 16 * len(XSIG) + 8 * MSIG.index(m)
                        parts.insert(0, _upk(sb[m0:m0 + 8]))
                    else:
                        parts.insert(0, h[:r, m[0][0] * 128:(m[0][0] + 1) * 128])
                return cat(parts)

            def proj(g):
                hds = GROUPS[g]
                res = [{} for _ in range(3)]
                first = g == 0 and chained
                kc = D - 128

                def plain(t, hd, part=None):
                    pre = early is not None and t == 0
                    x = hrest if pre else (h if t else h[q0:])
                    if part is None:
                        y = mm(x, wslab(t, hd))
                    else:
                        y = mm(x[:, kc:], wslab(t, hd)[kc:]) + part
                    feed(y, 5 if fast else 1)
                    if t == 0:
                        y = y.astype(BF16)
                    if pre:
                        y = jnp.concatenate([y[:r], qh_s[hd, pl.ds(qrow, SEG), :], y[r:]], axis=0)
                    res[t][hd] = y

                if not fast:
                    order = [(t, hd) for hd in hds for t in range(2)] + [(2, hd) for hd in hds]
                    parts = [mm((h if t else h[q0:])[:, :kc], wslab(t, hd)[:kc])
                             for t, hd in order[:4 if first else 0]]
                    for n, (t, hd) in enumerate(order):
                        plain(t, hd, parts[n] if n < len(parts) else None)
                    return res

                blocks = sorted((b for b in range(len(BLOCKS)) if BLOCKS[b][2][0] in hds),
                                key=lambda b: (max(BLOCKS[b][2]) - 2 * (b < 10), b))
                accs = [_Acc() for _ in range(3)]
                ts = [t for t in range(3) if t or early is None]

                def run(t, b, sel):
                    alg, dts, bh = BLOCKS[b]
                    for p, e in enumerate(alg):
                        if sel(e):
                            y = mm(left(e, dts), _upk(wtile(t, b, p)))
                            feed(y)
                            accs[t].route(e, bh, y)

                lead = [(t, b) for t in ts[:2] for b in blocks] if first else []
                for t, b in lead:
                    run(t, b, lambda e: e[3] is None)
                todo = list(hds) if early is not None else []
                for t in ts:
                    for b in blocks:
                        run(t, b, (lambda e: e[3] is not None) if (t, b) in lead else (lambda e: True))
                        for _ in range(2):
                            if todo and t == 1:
                                plain(0, todo.pop(0))
                    for hd in hds:
                        y = accs[t].rows(hd)
                        if hd >= 30:
                            y = mm(h[:, 256:384], _upk(plain_tile(t, 2, hd))) + y
                            feed(y)
                        res[t][hd] = y.astype(BF16) if t == 0 else y
                assert not todo
                return res

            def pad(kv):
                return jnp.concatenate([kv, jnp.zeros((128 - kv.shape[0], DH), F32)],
                                       axis=0).astype(BF16)

            def probs(qkv, g):
                scs = [lax.dot_general(qkv[0][hd], pad(qkv[1][hd]), (((1,), (1,)), ((), ())),
                                       preferred_element_type=F32) for hd in GROUPS[g]]
                ps = []
                for n, sc in enumerate(scs):
                    sc = jnp.where(vis, sc, fill)
                    e = jnp.exp2((sc - jnp.max(sc, axis=-1, keepdims=True))
                                 * (scale * math.log2(math.e)))
                    den = jnp.sum(e, axis=-1, keepdims=True)
                    if due and g >= 1 and n in ((0, 5) if g > 2 else (0,)):
                        e = jnp.concatenate([e[:16] + due.pop(0), e[16:]], axis=0)
                    rc = pl.reciprocal(den, approx=True)
                    rc = rc * (2.0 - den * rc)
                    ps.append((e * rc).astype(BF16))
                return ps

            def oproj(h0, h1, acc, mid=None):
                def put(key, y):
                    acc[key] = y + acc[key] if key in acc else y

                if not fast:
                    cuts = list(range(h0, h1, 5)) + [h1] if units else [h0, h1]
                    for n in range(NLB):
                        for a, b in zip(cuts, cuts[1:]):
                            if before_oproj is not None:
                                w = wo_s[a * DH:b * DH, n * 128:(n + 1) * 128]
                                wo_t[n, a * 64:b * 64, :] = pltpu.bitcast(w, U32)
                            else:
                                w = _upk(wo_t[n, a * 64:b * 64, :])
                            put(n, mm(jnp.concatenate(heads[a:b], axis=1).astype(BF16), w))
                            feed(acc[n])
                        if mid is not None and n == NLB - 2:
                            mid()
                    return
                for dts in ((0, 1, 2), (3, 4), (0, 1)):
                    bs = [b for b in range(len(BLOCKS))
                          if BLOCKS[b][1] == dts and h0 <= BLOCKS[b][2][0] < h1]
                    if mid is not None and dts == (3, 4):
                        mid()
                    for p, e in enumerate(BLOCKS[bs[0]][0]) if bs else ():
                        ls = []
                        for b in bs:
                            o = [heads[hd] for hd in BLOCKS[b][2]]
                            parts = [_lin([(c, o[k][r + row * SEG:r + (row + 1) * SEG])
                                           for row, k, c in _nz(e[0])])]
                            if e[3] is not None:
                                parts.insert(0, _lin([(c, o[k][:r])
                                                      for k, c in enumerate(e[3][0]) if c]))
                            ls.append(cat(parts))
                        put((dts, p), mm(cat(ls, 1).astype(BF16),
                                         _upk(cat([wtile(3, b, p) for b in bs]))))
                if h1 == H:
                    put(2, mm(jnp.concatenate(heads[30:], axis=1).astype(BF16),
                              _upk(wo_t[2, 30 * 64:, :])))

            heads, acc = [], {}
            qkv = proj(0)
            for g in range(len(GROUPS)):
                ps = probs(qkv, g)
                vs = [qkv[2][hd] for hd in GROUPS[g]]

                def weigh():
                    heads.extend(mm(p_, pad(v_)) for p_, v_ in zip(ps, vs))
                if g + 1 < len(GROUPS):
                    qkv = proj(g + 1)
                    weigh()
                else:
                    if before_oproj is not None:
                        before_oproj()
                    oproj(0, 18, acc, weigh)
            oproj(18, H, acc)
            assert not units and not due
            if not fast:
                return jnp.concatenate([acc[n] for n in range(NLB)], axis=1)
            out = _Acc()
            for key, y in acc.items():
                if key != 2:
                    out.route((HOPKERR if len(key[0]) == 3 else STRASSEN)[key[1]], key[0], y)
            return jnp.concatenate([out.rows(n) + acc[2] if n == 2 else out.rows(n)
                                    for n in range(NLB)], axis=1)

        def post2(s, toks=None):
            r3 = seg_row(s - 1 - LAG)
            for r in (0, 16):
                xc = _r(x2_s[(s + 4 - 1 - LAG) % 4, r:r + 16] + obuf[SEG + r:SEG + r + 16, :])
                out_s[pl.ds(r3 + r, 16), :] = gate(xc, r3 + r, toks).astype(BF16)

        def step(s, mode, vis, fill, chained=False, before_oproj=None, early=None, units=()):
            if mode == 0:
                h = hbuf[0:ROWS, :]
            elif mode == 1:
                h = hbuf[0:48, :]
            else:
                live = lax.broadcasted_iota(jnp.int32, (2 * M, D), 0) >= M
                mem = jnp.where(live, hbuf[0:16, :].astype(F32), 0.0).astype(BF16)
                h = jnp.concatenate([mem, hbuf[48:80, :]], axis=0)
            toks = []
            if mode != 1:
                post2(s, toks)
            if isinstance(s, int) and s == NSEG + LAG - 1:
                obuf[SEG:2 * SEG, :] = attention(h, vis, fill, chained, due=toks)
                return
            r1 = seg_row(s - 1)
            rn = seg_row(s + 1)
            h1n, h2n = [], []
            for r in (0, 16):
                xa = _r(x_s[pl.ds(r1 + r, 16), :].astype(F32) + obuf[r:r + 16, :])
                xb2 = _r(gate(xa, r1 + r))
                h2n.append(_ln(xb2, toks))
                x2_s[(s + 4 - 1) % 4, r:r + 16] = xb2
            if mode != 2:
                for r in (0, 16):
                    h1n.append(_ln(x_s[pl.ds(rn + r, 16), :].astype(F32), toks))

            if early is not None:
                mrow = pl.multiple_of(early * (8 * PPS), 8 * PPS)
                units = [functools.partial(lambda u, tok: u(tok[0:8]), u)
                         for n in range(PPS) for u in mac_units(mrow + 8 * n, 1)]
                tb = early // 2
                units += [functools.partial(sum_unit, 0, HOPKERR, (0, 1, 2),
                                            (3 * tb, 3 * tb + 1, 3 * tb + 2), 9 * tb,
                                            (early % 2) * 32 + r0) for r0 in range(0, 32, 8)]
                pb = jnp.minimum(early, 16)
                k0, h0 = jnp.where(pb < 16, 3, 0), 2 * jnp.minimum(pb, 15)
                units += [functools.partial(sum_unit, 0, STRASSEN, (k0, k0 + 1), (h0, h0 + 1),
                                            90 + 5 * pb, r0) for r0 in range(0, 64, 8)]

            o = attention(h, vis, fill, chained, before_oproj, early, toks, mode == 0, units)

            mem2 = mem0 if mode == 1 else o[M:2 * M]
            mem = jnp.concatenate([o[0:M], mem2], axis=0)
            hbuf[0:16, :] = mem.astype(BF16)
            for n, v in enumerate(h1n):
                hbuf[16 + 16 * n:32 + 16 * n, :] = v.astype(BF16)
            for n, v in enumerate(h2n):
                hbuf[48 + 16 * n:64 + 16 * n, :] = v.astype(BF16)
            if mode != 2:
                tile = lambda v, dt: v[:, dt * 128:(dt + 1) * 128]
                for i, sig in enumerate(MSIG):
                    m0 = 16 * len(XSIG) + 8 * i
                    sbuf[m0:m0 + 8, :] = _pk(_lin([(c, tile(mem, dt)) for dt, c in sig]))
                for n, xy in enumerate(zip(h1n, h2n)):
                    for i, sig in enumerate(XSIG):
                        sbuf[16 * i + 8 * n:16 * i + 8 * n + 8, :] = _pk(
                            _lin([(c, tile(xy[row], dt)) for row, dt, c in sig]))
            if mode == 0:
                obuf[...] = o[2 * M:]
            elif mode == 1:
                obuf[0:SEG, :] = o[2 * M:]
            else:
                obuf[SEG:2 * SEG, :] = o[2 * M:]

        with _scope("pro"):
            vis, fill = masks(1)
            kv_units = sum_units(1) + sum_units(2)
            cut = len(kv_units) * 3 // 4
            step(0, 1, vis, fill, False, wo_copy.wait, units=kv_units[:cut])
            step(1, 1, vis, fill, True, units=kv_units[cut:] + sum_units(3))
        xb_copy.start()
        vis, fill = masks(0)
        with _scope("main_a"):
            loop(NA // UA, lambda i: [step(UA * i + u + LAG, 0, vis, fill, u > 0, early=UA * i + u)
                                      for u in range(UA)])
        xb_copy.wait()
        with _scope("conv_e"):
            loop(HB // UI, lambda j: [inv_stage(HB + UI * j + u) for u in range(UI)])
        with _scope("main_b"):
            loop((NSEG - LAG - NA) // UB, lambda i: [step(UB * i + u + LAG + NA, 0, vis, fill, u > 0)
                                                     for u in range(UB)])
        done = (NSEG - 1 - LAG) * SEG
        out_a = pltpu.make_async_copy(out_s.at[0:done, :], out_hbm.at[0:done, :], sem.at[SW + 8])
        out_a.start()
        with _scope("epi"):
            vis, fill = masks(2)
            step(NSEG, 2, vis, fill)
            step(NSEG + 1, 2, *masks(2, 2 * M), True)
        post2(NSEG + LAG)
        out_b = pltpu.make_async_copy(out_s.at[done:S, :], out_hbm.at[done:S, :], sem.at[SW + 9])
        out_b.start()
        out_a.wait()
        out_b.wait()

    pl.run_scoped(
        phase1,
        pltpu.VMEM((NSUM * 64, 128), U32),
        pltpu.VMEM((2 * NSUM * 64, 128), U32),
        pltpu.VMEM((NSUM * 64, 128), U32),
    )


@jax.jit
def pallas_interleave_layers__memory_aug_recurrent_mem_tr__ssm_conv_h3__prompt_kernel(
    A_x, A_mem0, A_Wq, A_Wk, A_Wv, A_Wo, A_seg_len,
    B_q, B_k, B_v, B_shift_k, B_ssm_k, B_ssm_D,
):
    del A_seg_len, B_q
    assert A_x.shape == (1, S, D) and A_Wq.shape == (D, H, DH)
    hbm = pl.BlockSpec(memory_space=pl.ANY)
    out = pl.pallas_call(
        _kernel,
        out_shape=jax.ShapeDtypeStruct((S, D), BF16),
        in_specs=[hbm] * 11,
        out_specs=hbm,
        scratch_shapes=[
            pltpu.VMEM((S, D), BF16),
            pltpu.VMEM((H * WP + 352, 128), U32),
            pltpu.VMEM((2 * H * WP + 352, 128), U32),
            pltpu.VMEM((H * DH, D), BF16),
            pltpu.VMEM((NLB, H * DH // 2, 128), U32),
            pltpu.VMEM((TB // 2, TB), U32),
            pltpu.VMEM((2, TB // 2, TB), U32),
            pltpu.VMEM((2, TB // 2, TB), U32),
            pltpu.VMEM((NB, 2, NLB * TB, 128), F32),
            pltpu.VMEM((NB, 3, NLB * TB, 128), F32),
            pltpu.VMEM((NB + 1, 2, NLB * TB, 128), F32),
            pltpu.VMEM((NLB, S + 32, 128), F32),
            pltpu.VMEM((2 * SEG, D), F32),
            pltpu.VMEM((4, SEG, D), F32),
            pltpu.VMEM((S, D), BF16),
            pltpu.VMEM((NQH, NA * SEG, DH), BF16),
            pltpu.VMEM((128, D), BF16),
            pltpu.VMEM((320, 128), U32),
            pltpu.VMEM((64, D), BF16),
            pltpu.SemaphoreType.DMA((HB + HB // 2 + 14,)),
        ],
        compiler_params=pltpu.CompilerParams(vmem_limit_bytes=120 * 1024 * 1024),
    )(A_x.reshape(S, D), A_mem0.reshape(M, D), A_Wq, A_Wk, A_Wv,
      A_Wo.reshape(H * DH, D), B_k.reshape(S, D), B_v.reshape(S, D),
      B_shift_k.T, B_ssm_k, B_ssm_D)
    return out.reshape(1, S, D)
```

```python
import contextlib
import functools
import math

import jax
import jax.numpy as jnp
from jax import lax
import jax.experimental.pallas as pl
import jax.experimental.pallas.tpu as pltpu

F32 = jnp.float32
BF16 = jnp.bfloat16
U32 = jnp.uint32

S = 2048
D = 640
H = 32
DH = 128
M = 8
SEG = 32
NSEG = S // SEG
KS = 4
LAG = 2
ROWS = 2 * M + 2 * SEG
NLB = D // 128
TB = 128
NB = S // TB
HB = NB // 2
NPOS = NLB * TB // 8
NA = 20
PPS = 4
UCUT = tuple(range(a, a + 2) for a in range(0, 12, 2)) + (range(12, 16),)
NQH = 32
UA = 2
UB = 3
UI = 4
WP = 324


STRASSEN = (
    (((1, 0), (0, 1)), ((1, 0), (0, 1)), ((1, 0), (0, 1)), None),
    (((-1, 0), (1, 0)), ((1, 1), (0, 0)), ((0, 0), (0, 1)), None),
    (((0, 1), (0, -1)), ((0, 0), (1, 1)), ((1, 0), (0, 0)), None),
    (((0, 0), (1, 1)), ((1, 0), (0, 0)), ((0, 0), (1, -1)), ((1, 1), (1, 0))),
    (((1, 0), (0, 0)), ((0, 1), (0, -1)), ((0, 1), (0, 1)), ((1, 0), (0, 1))),
    (((0, 0), (0, 1)), ((-1, 0), (1, 0)), ((1, 0), (1, 0)), ((0, 1), (1, 0))),
    (((1, 1), (0, 0)), ((0, 0), (0, 1)), ((-1, 1), (0, 0)), ((1, 1), (0, 1))),
)
HOPKERR = (
    (((1, 0, 0), (0, 0, 0)), ((1, 0, 1), (-1, 0, 0), (0, 0, 0)), ((1, 0, 0), (1, 0, 0)), None),
    (((1, 1, 0), (0, 0, 0)), ((0, 0, 0), (1, 0, 0), (0, 0, 0)), ((1, -1, 0), (0, 0, 0)), None),
    (((-1, 0, 0), (1, 0, 1)), ((0, 0, 1), (0, 0, 0), (1, 0, 0)), ((1, 0, -1), (1, 0, 0)), None),
    (((0, 1, 0), (0, -1, 0)), ((0, 0, 0), (1, 1, 0), (0, -1, 0)), ((0, 1, 0), (0, 0, 0)), None),
    (((0, 1, 1), (0, -1, 0)), ((0, 0, 0), (0, 0, 1), (0, 1, 0)), ((0, 1, 0), (0, 1, -1)), None),
    (((0, 0, 1), (0, 0, 0)), ((0, 0, 0), (0, 0, -1), (1, 0, 1)), ((0, 0, 1), (0, 0, 0)), None),
    (((-1, 0, 0), (1, 0, 0)), ((1, 1, 0), (0, 0, 0), (-1, 0, 0)), ((0, 0, 0), (1, 0, 0)),
     ((1, 0, 0), (1, 0, 0))),
    (((1, 0, 0), (0, 1, 0)), ((0, 1, 0), (1, 0, 0), (0, 0, 0)), ((0, 1, 0), (1, 0, 0)),
     ((0, 1, 0), (1, 0, 0))),
    (((0, 0, 0), (1, 1, 0)), ((0, 1, 0), (0, 0, 0), (0, 0, 0)), ((0, 0, 0), (-1, 1, 0)),
     ((1, 1, 0), (-1, 1, 0))),
    (((0, 0, 0), (1, 0, 1)), ((0, 0, 1), (0, 0, 0), (0, 0, 0)), ((-1, 0, 1), (-1, 0, 1)),
     ((1, 0, 1), (0, 0, 1))),
    (((-1, 0, -1), (1, 0, 1)), ((0, 0, 0), (0, 0, 0), (1, 0, 0)), ((-1, 0, 1), (0, 0, 0)),
     ((1, 0, 1), (1, 0, 0))),
    (((0, 0, 0), (0, 1, 0)), ((0, -1, 0), (0, 1, 1), (0, 0, 0)), ((0, 1, 0), (0, 1, 0)),
     ((0, 1, 0), (0, 1, 0))),
    (((0, 1, 1), (0, 0, 0)), ((0, 0, 0), (0, 0, 1), (0, 0, 0)), ((0, -1, 1), (0, -1, 1)),
     ((0, 1, 0), (0, -1, 1))),
    (((0, -1, -1), (0, 1, 1)), ((0, 0, 0), (0, 0, 0), (0, 1, 0)), ((0, 0, 0), (0, 1, -1)),
     ((0, 0, 1), (0, 1, -1))),
    (((0, 0, 0), (0, 0, 1)), ((0, 0, -1), (0, 0, 0), (0, 1, 1)), ((0, 0, 0), (0, 0, 1)),
     ((0, 0, 1), (0, 0, 1))),
)
BLOCKS = ([(HOPKERR, (0, 1, 2), (3 * i, 3 * i + 1, 3 * i + 2)) for i in range(10)]
          + [(STRASSEN, (3, 4), (2 * i, 2 * i + 1)) for i in range(16)]
          + [(STRASSEN, (0, 1), (30, 31))])
GROUPS = [tuple(range(a, b)) for a, b in ((0, 6), (6, 12), (12, 18), (18, 24), (24, 32))]
NSUM = 10 * 9 + 17 * 5


def _nz(mat):
    return tuple((i, j, c) for i, row in enumerate(mat) for j, c in enumerate(row) if c)


def _summed(alg):
    return [p for p, e in enumerate(alg) if len(_nz(e[1])) > 1]


def _slot(b, p):
    sm = _summed(BLOCKS[b][0])
    if p not in sm:
        return None
    return (9 * b if b < 10 else 90 + 5 * (b - 10)) + sm.index(p)


def _lin(terms):
    terms = sorted(terms, key=lambda t: -t[0])
    acc = terms[0][1]
    for c, v in terms[1:]:
        acc = acc + v if c > 0 else acc - v
    return acc


class _Acc:
    def __init__(self):
        self.d = {}

    def add(self, key, c, v):
        if key not in self.d:
            self.d[key] = (c, v)
            return
        c0, v0 = self.d[key]
        self.d[key] = (c0, v0 + v) if c == c0 else (1, _lin([(c0, v0), (c, v)]))

    def route(self, e, ns, y):
        r = 0 if e[3] is None else 2 * M
        for row, n, c in _nz(e[2]):
            self.add((row + 1, ns[n]), c, y[r:])
        if r:
            for n, c in enumerate(e[3][1]):
                if c:
                    self.add((0, ns[n]), c, y[:r])

    def rows(self, n):
        assert all(self.d[(i, n)][0] == 1 for i in range(3))
        return jnp.concatenate([self.d[(i, n)][1] for i in range(3)], axis=0)


def _row_sigs():
    xs, ms = [], []
    for alg, dts, _ in BLOCKS:
        for e in alg:
            x = tuple((r, dts[k], c) for r, k, c in _nz(e[0]))
            if len(x) > 1 and x not in xs:
                xs.append(x)
            if e[3] is not None:
                m = tuple((dts[k], c) for k, c in enumerate(e[3][0]) if c)
                if len(m) > 1 and m not in ms:
                    ms.append(m)
    return xs, ms


XSIG, MSIG = _row_sigs()
PROFILE = False


def _scope(name):
    return jax.named_scope(name) if PROFILE else contextlib.nullcontext()


def _ln(x, toks=None):
    m = jnp.mean(x, axis=-1, keepdims=True)
    c = x - m
    v = jnp.mean(c * c, axis=-1, keepdims=True)
    r = lax.rsqrt(v + 1e-5)
    if toks is not None:
        toks.append(jnp.minimum(r, 0.0))
    return c * r


def _r(x):
    return x.astype(BF16).astype(F32)


def _split(x):
    hi = pltpu.bitcast(pltpu.bitcast(x, U32) & jnp.uint32(0xFFFF0000), F32)
    return hi, x - hi


def _pk(x):
    return pltpu.bitcast(x.astype(BF16), U32)


def _upk(w):
    return pltpu.bitcast(w, BF16)


def _basis(r, t):
    b = r & 63
    f = jnp.where(b < 32, 2 * b, 2 * b - 63)
    n = ((2 * f + 1) * t - jnp.where(r >= 64, TB, 0)) & (4 * TB - 1)
    n = jnp.where(n >= 2 * TB, n - 4 * TB, n)
    return jnp.cos(n.astype(F32) * (2.0 * math.pi / (4 * TB)))


def _halves(x):
    w = pltpu.bitcast(x, U32)
    return (pltpu.bitcast(w << 16, F32),
            pltpu.bitcast(w & jnp.uint32(0xFFFF0000), F32))


def _kernel(x_hbm, mem0_hbm, wq_hbm, wk_hbm, wv_hbm, wo_hbm,
            k_hbm, v_hbm, shk_hbm, ssmk_hbm, ssmd_hbm,
            out_hbm,
            x_s, wt_q, wt_kv, wo_s, wo_t,
            perm_s, fu_s, inv_s, u_s, kf_s, c_s, y_s,
            obuf, x2_s, out_s, qh_s, hbuf, sbuf, mem0_ref,
            sem):
    X0, XH = LAG * SEG, (LAG + NA) * SEG
    SW = HB + HB // 2
    hb = TB // 2
    wo_copy = pltpu.make_async_copy(wo_hbm, wo_s, sem.at[SW + 3])
    xb_copy = pltpu.make_async_copy(x_hbm.at[XH + SEG:, :], x_s.at[XH + SEG:, :], sem.at[SW + 7])

    def mac_units(row, half):
        rs = pl.ds(row, 8)
        state = {}

        def unit(p, avals, final, tok=None):
            acc = state.setdefault(p, dict(state.get(0, {})))
            for a in avals:
                u = u_s[a, 0, rs] + u_s[a, 1, rs] if p == 0 else u_s[a, p - 1, rs]
                if tok is not None:
                    u = u + tok
                for i in range(max(a, half * HB), half * HB + HB):
                    t = u * kf_s[i - a, p, rs]
                    acc[i] = t if i not in acc else (acc[i] - t if p == 2 else acc[i] + t)
            if final and p:
                for i, v in acc.items():
                    c_s[i + 1, 2 - p, rs] = v

        subs = UCUT if half else (range(HB),)
        return [functools.partial(unit, p, avals, n == len(subs) - 1)
                for p in range(3) for n, avals in enumerate(subs)]

    def inv_stage(i, units=None):
        q = TB // 4
        for g in range(NLB):
            re, im = [], []
            for b in range(4):
                rows = slice(g * TB + b * q, g * TB + (b + 1) * q)
                cr, ci_ = c_s[i + 1, 0, rows], c_s[i + 1, 1, rows]
                pr, pi = c_s[i, 0, rows], c_s[i, 1, rows]
                re.append(cr + pi if b in (0, 3) else cr - pi)
                im.append(ci_ - pr if b in (0, 3) else ci_ + pr)
            pe = jnp.concatenate([re[0] + re[2], re[1] + re[3], im[0] - im[2], im[1] - im[3]], axis=0)
            po = jnp.concatenate([re[0] - re[2], re[1] - re[3], im[0] + im[2], im[1] + im[3]], axis=0)
            for par, pp in enumerate((pe, po)):
                ph, plo = _split(pp)
                gh_, gl_ = (inv_s[n, par * q:(par + 1) * q] for n in range(2))
                y = jnp.dot(_upk(jnp.concatenate([gh_, gl_, gh_], axis=1)),
                            jnp.concatenate([ph, ph, plo], axis=0).astype(BF16),
                            preferred_element_type=F32)
                y_s[g, pl.ds(i * TB + par, hb, stride=2), :] = y
                if units:
                    tok = pltpu.bitcast(jnp.minimum(jnp.abs(y[0:16]), 0.0), U32)
                    for _ in range(3):
                        if units:
                            units.pop(0)(tok)

    def wslab(t, h):
        s0 = (max(t - 1, 0) * H + (h % 2) * 16 + h // 2) * WP
        return pltpu.bitcast((wt_kv if t else wt_q)[s0:s0 + D // 2, :], BF16)

    def loop(n, fn):
        def body(j, _):
            fn(j)
            return 0
        lax.fori_loop(0, n, body, 0)

    def phase0(k_s, v_s, ssmk_s, wraw, kpad, hl_s, shk_ref, ssmd_ref):

        def pair_rows(jp):
            r0 = jp * 2 * TB
            return pl.ds(r0 if isinstance(jp, int) else pl.multiple_of(r0, 2 * TB), 2 * TB)

        def ssmk_copy(jp):
            return pltpu.make_async_copy(ssmk_hbm.at[:, pair_rows(jp)], ssmk_s.at[jp], sem.at[jp])

        def kv_copies(rows, sm):
            return [pltpu.make_async_copy(k_hbm.at[rows, :], k_s.at[rows, :], sm),
                    pltpu.make_async_copy(v_hbm.at[rows, :], v_s.at[rows, :], sm)]
        DQ = 192
        wq_early = [pltpu.make_async_copy(wq_hbm.at[n * DQ:(n + 1) * DQ], wraw.at[0, n * DQ:(n + 1) * DQ],
                                          sem.at[SW + 10 + n]) for n in range(2)]
        w_copies = [pltpu.make_async_copy(wq_hbm.at[2 * DQ:], wraw.at[0, 2 * DQ:], sem.at[SW])]
        w_copies += [pltpu.make_async_copy(w.at[n * (D // 2):(n + 1) * (D // 2)],
                                           wraw.at[t, n * (D // 2):(n + 1) * (D // 2)],
                                           sem.at[SW + 11 * n + t])
                     for t, w in ((1, wk_hbm), (2, wv_hbm)) for n in range(2)]
        late_copies = kv_copies(pl.ds(S // 2, S // 2), sem.at[SW + 4])
        small_copies = [pltpu.make_async_copy(src, dst, sem.at[SW + 5])
                        for src, dst in ((shk_hbm, shk_ref), (ssmd_hbm, ssmd_ref), (mem0_hbm, mem0_ref.at[0:M]))]
        XM = XH - 2 * TB
        xa_copy = pltpu.make_async_copy(x_hbm.at[X0:XM, :], x_s.at[X0:XM, :], sem.at[SW + 6])
        late_copies += [pltpu.make_async_copy(x_hbm.at[a:b, :], x_s.at[a:b, :], sem.at[SW + 4])
                        for a, b in ((0, X0), (XM, XH + SEG))]
        for c in (small_copies + [ssmk_copy(jp) for jp in range(HB)]
                  + [c for jp in range(HB // 2) for c in kv_copies(pair_rows(jp), sem.at[HB + jp])]
                  + [xa_copy] + wq_early + [w_copies[0]] + late_copies + w_copies[1:] + [wo_copy]):
            c.start()

        ri = lax.broadcasted_iota(jnp.int32, (TB, TB), 0)
        ci = lax.broadcasted_iota(jnp.int32, (TB, TB), 1)
        perm_s[...] = _pk(jnp.where(ci == 2 * (ri & 63) + (ri >> 6), 1.0, 0.0))
        tab = _basis(ri, 2 * (ci & 63) + (ci >> 6))
        hi, lo = _split(tab)
        fu_s[0] = _pk(jnp.where(ci < hb, hi, pltpu.roll(lo, hb, 1)))
        fu_s[1] = _pk(jnp.where(ci < hb, pltpu.roll(hi, hb, 1), lo))
        gh, gl = _split(tab.T * (1.0 / TB))
        inv_s[0] = _pk(gh)
        inv_s[1] = _pk(gl)

        for c in small_copies:
            c.wait()
        shk_t = shk_ref[...].astype(F32)
        taps = [[shk_t[j:j + 1, g * 128:(g + 1) * 128] for g in range(NLB)] for j in range(KS)]
        dvec = ssmd_ref[...].astype(F32).reshape(1, D)
        for g in range(NLB):
            kpad[0, g, 0:8, :] = jnp.zeros((8, 128), F32)
            kpad[1, g, 0:8, :] = jnp.zeros((8, 128), F32)
        c_s[0] = jnp.zeros(c_s.shape[1:], F32)
        hbuf[0:16, :] = jnp.concatenate([mem0_ref[0:M, :].astype(F32)] * 2, axis=0).astype(BF16)
        obuf[...] = jnp.zeros((2 * SEG, D), F32)
        x2_s[...] = jnp.zeros(x2_s.shape, F32)

        def spectrum(e, o):
            fe = jnp.dot(_upk(fu_s[0]), jnp.concatenate([e, e], axis=0).astype(BF16), preferred_element_type=F32)
            fo = jnp.dot(_upk(fu_s[1]), jnp.concatenate([o, o], axis=0).astype(BF16), preferred_element_type=F32)
            return ((fe[:hb] + fo[:hb], fe[hb:] + fo[hb:]), (fe[:hb] - fo[:hb], fo[hb:] - fe[hb:]))

        def freq_rows(g):
            return slice(g * TB, g * TB + hb), slice(g * TB + hb, (g + 1) * TB)

        def fwd_k(jq):
            def transposed(n):
                if n % 2 == 0:
                    ssmk_copy(2 * jq + n // 2).wait()
                blk = ssmk_s[2 * jq + n // 2, :, (n % 2) * TB:(n % 2 + 1) * TB]
                return lax.dot_general(_upk(perm_s[...]), blk, (((1,), (1,)), ((), ())),
                                       preferred_element_type=F32)
            nxt = transposed(0)
            for n in range(4):
                kt = nxt
                if n < 3:
                    nxt = transposed(n + 1)
                j = 4 * jq + n
                for g in range(NLB):
                    lb = slice(g * 128, (g + 1) * 128)
                    for rows, (kr, ki) in zip(freq_rows(g), spectrum(kt[:hb, lb], kt[hb:, lb])):
                        if n == 0:
                            kr = kr + jnp.where(j == 0, dvec[:, lb], 0.0)
                        kf_s[j, 0, rows] = kr
                        kf_s[j, 1, rows] = ki - kr
                        kf_s[j, 2, rows] = kr + ki

        def fwd_u(jq, first):
            if first:
                for jp in (2 * jq, 2 * jq + 1):
                    for c in kv_copies(pair_rows(jp), sem.at[HB + jp]):
                        c.wait()
            for j in [4 * jq + n for n in range(4)]:
                r0 = pl.multiple_of(j * TB, TB)
                q0 = pl.multiple_of(j * hb, hb) + 8
                for g in range(NLB):
                    lb = slice(g * 128, (g + 1) * 128)
                    ke, ko = _halves(k_s[pl.ds(r0, TB), lb])
                    ve, vo = _halves(v_s[pl.ds(r0, TB), lb])
                    kpad[0, g, pl.ds(q0, hb), :] = ke
                    kpad[1, g, pl.ds(q0, hb), :] = ko
                    ke1 = kpad[0, g, pl.ds(q0 - 1, hb), :]
                    ko1 = kpad[1, g, pl.ds(q0 - 1, hb), :]
                    ko2 = kpad[1, g, pl.ds(q0 - 2, hb), :]
                    t0, t1, t2, t3 = (taps[t][g] for t in range(KS))
                    e = (ke * t0 + ko1 * t1 + ke1 * t2 + ko2 * t3) * ve
                    o = (ko * t0 + ke * t1 + ko1 * t2 + ke1 * t3) * vo
                    for rows, (ur, ui) in zip(freq_rows(g), spectrum(e, o)):
                        u_s[j, 0, rows] = ur
                        u_s[j, 1, rows] = ui

        def relayout_rows(t, dst, base, dp, tok=None):
            a = pltpu.bitcast(wraw[t, 2 * dp], U32)
            b = pltpu.bitcast(wraw[t, 2 * dp + 1], U32)
            if tok is not None:
                a = a | tok
            dst[pl.ds(base + dp, 16, stride=WP), :] = (a & jnp.uint32(0xFFFF)) | (b << 16)
            dst[pl.ds(base + 16 * WP + dp, 16, stride=WP), :] = (
                (a >> 16) | (b & jnp.uint32(0xFFFF0000)))

        def norm_rows(r0, nr):
            r0 = pl.multiple_of(r0, 16)
            for r in range(0, nr, 16):
                hl_s[pl.ds(r0 + r, 16), :] = _ln(
                    x_s[pl.ds(r0 + r + LAG * SEG, 16), :].astype(F32)).astype(BF16)

        def pre_queries(c, t=None):
            per = -(-(D // 4) // NQH)
            for sub in range(2):
                if t is not None:
                    half = wraw.at[t, sub * (D // 2):(sub + 1) * (D // 2)]
                    pltpu.make_async_copy(half, half, sem.at[SW + 11 * sub + t]).wait()
                    base = (t - 1) * (H * WP)
                    dp = sub * (D // 4)
                r0 = pl.multiple_of((2 * c + sub) * QR, QR)
                hl = hl_s[pl.ds(r0, QR), :]
                for hd in range(NQH):
                    r = jnp.dot(hl, wslab(0, hd), preferred_element_type=F32)
                    qh_s[hd, pl.ds(r0, QR), :] = r.astype(BF16)
                    if t is not None:
                        tok = pltpu.bitcast(jnp.minimum(jnp.abs(r[0:16]), 0.0), U32)
                        for _ in range(per):
                            if dp < (sub + 1) * (D // 4):
                                relayout_rows(t, wt_kv, base, dp, tok)
                                dp += 1

        nch = NA * SEG // TB
        QR = TB // 2
        with _scope("conv_k"):
            loop(HB // 2, fwd_k)
        with _scope("conv_u"):
            loop(HB // 4, lambda j: fwd_u(j, True))
        with _scope("conv_b"):
            loop(NPOS // 10, lambda j: [u() for n in range(10)
                                        for u in mac_units(pl.multiple_of(80 * j, 16) + 8 * n, 0)])
            xa_copy.wait()

            def inv_first(j):
                part = wraw.at[0, pl.ds(j * DQ, DQ)]
                pltpu.make_async_copy(part, part, sem.at[SW + 10 + j]).wait()
                units = [functools.partial(relayout_rows, 0, wt_q, 0, j * (DQ // 2) + dd)
                         for dd in range(DQ // 2)]
                for u in range(UI):
                    inv_stage(UI * j + u, units)
                assert not units
                norm_rows(j * ((XM - X0) // 2), (XM - X0) // 2)
            loop(HB // UI, inv_first)
        with _scope("rel0"):
            w_copies[0].wait()
            loop((D - 2 * DQ) // 64,
                 lambda i: [relayout_rows(0, wt_q, 0, DQ + i * 32 + dd) for dd in range(32)])
        with _scope("preq"):
            loop(nch - 2, pre_queries)
        with _scope("conv_c"):
            for c in late_copies:
                c.wait()

            def fwd_u_late(j):
                r0 = pl.multiple_of(j * 16, 16)
                hbuf[pl.ds(16 + r0, 16), :] = _ln(x_s[pl.ds(r0, 16), :].astype(F32)).astype(BF16)
                norm_rows(XM - X0 + j * TB, TB)
                fwd_u(HB // 4 + j, False)
            loop(HB // 4, fwd_u_late)
        with _scope("preq_rel"):
            loop(2, lambda i: pre_queries(i + nch - 2, i + 1))

    pl.run_scoped(
        phase0,
        pltpu.VMEM((S, D), BF16),
        pltpu.VMEM((S, D), BF16),
        pltpu.VMEM((HB, D, 2 * TB), BF16),
        pltpu.VMEM((3, D, H, DH), BF16),
        pltpu.VMEM((2, NLB, S // 2 + 32, 128), F32),
        pltpu.VMEM((NA * SEG, D), BF16),
        pltpu.VMEM((KS, D), BF16),
        pltpu.VMEM((D,), BF16),
    )

    def phase1(cq, ckv, co):
        scale = DH ** -0.5

        def masks(mode, q0=0):
            rows = ROWS if mode == 0 else ROWS - SEG
            qi = lax.broadcasted_iota(jnp.int32, (rows - q0, 128), 0) + q0
            kj = lax.broadcasted_iota(jnp.int32, (rows - q0, 128), 1)

            def layer_of(i):
                xl = (i - 2 * M) // SEG if mode == 0 else mode - 1
                return jnp.where(i < 2 * M, i // M, xl)
            same = (layer_of(qi) == layer_of(kj)) & (kj < rows)
            vis = same & ((qi < 2 * M) | (qi >= kj))
            fill = jnp.where(same, -1e9 / scale, -jnp.inf).astype(F32)
            return vis, fill

        mem0 = mem0_ref[0:M, :].astype(F32)

        def seg_row(seg):
            if isinstance(seg, int):
                return min(max(seg, 0), NSEG - 1) * SEG
            return pl.multiple_of(jnp.clip(seg, 0, NSEG - 1) * SEG, SEG)

        def gate(xa, r0, toks=None):
            y = jnp.concatenate([y_s[g, pl.ds(r0, xa.shape[0]), :] for g in range(NLB)], axis=1)
            return xa + _ln(xa, toks) * y

        def mm(a, b):
            return jnp.dot(a, b, preferred_element_type=F32)

        def cat(vs, axis=0):
            return vs[0] if len(vs) == 1 else jnp.concatenate(vs, axis=axis)

        def plain_tile(t, dt, hd, r0=0, nr=64):
            if t == 3:
                return wo_t[dt, pl.ds(hd * 64 + r0, nr), :]
            s0 = (max(t - 1, 0) * H + (hd % 2) * 16 + hd // 2) * WP
            return (wt_kv if t else wt_q)[pl.ds(s0 + dt * 64 + r0, nr), :]

        def sum_ref(t):
            return (cq, ckv, ckv, co)[t], (NSUM * 64 if t == 2 else 0)

        def wtile(t, b, p):
            alg, dts, hds = BLOCKS[b]
            if _slot(b, p) is None:
                (k, n, _), = _nz(alg[p][1])
                return plain_tile(t, dts[n], hds[k]) if t == 3 else plain_tile(t, dts[k], hds[n])
            ref, r0 = sum_ref(t)
            r0 += _slot(b, p) * 64
            return ref[r0:r0 + 64, :]

        def sum_unit(t, alg, dts, hds, slot0, r0, tok):
            src = {}
            for k in range(len(dts)):
                for n in range(len(dts)):
                    w = (plain_tile(t, dts[n], hds[k], r0, 8) if t == 3
                         else plain_tile(t, dts[k], hds[n], r0, 8))
                    if (n - k) % len(dts) == len(dts) - 2:
                        w = w | pltpu.bitcast(tok[0:8], U32)
                    src[k, n] = _upk(w).astype(F32)
            ref, base = sum_ref(t)
            sums = _pk(jnp.concatenate([_lin([(c, src[k, n]) for k, n, c in _nz(alg[p][1])])
                                        for p in _summed(alg)], axis=1))
            for i in range(len(_summed(alg))):
                ref[pl.ds(base + (slot0 + i) * 64 + r0, 8), :] = sums[:, i * 128:(i + 1) * 128]

        def sum_units(t):
            jobs = [(b, r0) for b in range(len(BLOCKS)) for r0 in range(0, 64, 8)]
            jobs.sort(key=lambda j: (j[0] * 64 + j[1]) / 640 if j[0] < 10
                      else ((j[0] - 10) * 64 + j[1]) / (17 * 64))
            return [functools.partial(sum_unit, t, *BLOCKS[b], _slot(b, _summed(BLOCKS[b][0])[0]), r0)
                    for b, r0 in jobs]

        def attention(h, vis, fill, chained, before_oproj=None, early=None, due=(), fast=False,
                      units=()):
            q0 = h.shape[0] - vis.shape[0]
            r = 2 * M
            units, due = list(units), list(due)
            nprod = sum(len(b[0]) for b in BLOCKS) + 2
            ncall = (3 * H if before_oproj else 4 * H - 4) if not fast else (3 * nprod if early is None else 2 * nprod + 5 * H)
            nunit, state = len(units), [0]
            if early is not None:
                hrest = jnp.concatenate([h[:r], h[r + SEG:]], axis=0)
                qrow = pl.multiple_of(early * SEG, SEG)
            if fast:
                sb = sbuf[0:16 * len(XSIG) + 8 * len(MSIG), :]

            def feed(x, weight=1):
                state[0] += weight
                n = -(-nunit * state[0] // ncall) - (nunit - len(units))
                if n > 0:
                    tok = jnp.minimum(jnp.abs(x[0:16]), 0.0)
                    for u in units[:n]:
                        u(tok)
                    del units[:n]

            def left(e, dts):
                x = tuple((row, dts[k], c) for row, k, c in _nz(e[0]))
                if len(x) > 1:
                    parts = [_upk(sb[16 * XSIG.index(x):16 * XSIG.index(x) + 16])]
                else:
                    row, dt, _ = x[0]
                    parts = [h[r + row * SEG:r + (row + 1) * SEG, dt * 128:(dt + 1) * 128]]
                if e[3] is not None:
                    m = tuple((dts[k], c) for k, c in enumerate(e[3][0]) if c)
                    if len(m) > 1:
                        m0 = 16 * len(XSIG) + 8 * MSIG.index(m)
                        parts.insert(0, _upk(sb[m0:m0 + 8]))
                    else:
                        parts.insert(0, h[:r, m[0][0] * 128:(m[0][0] + 1) * 128])
                return cat(parts)

            def proj(g):
                hds = GROUPS[g]
                res = [{} for _ in range(3)]
                first = g == 0 and chained
                kc = D - 128

                def plain(t, hd, part=None):
                    pre = early is not None and t == 0
                    x = hrest if pre else (h if t else h[q0:])
                    if part is None:
                        y = mm(x, wslab(t, hd))
                    else:
                        y = mm(x[:, kc:], wslab(t, hd)[kc:]) + part
                    feed(y, 5 if fast else 1)
                    if t == 0:
                        y = y.astype(BF16)
                    if pre:
                        y = jnp.concatenate([y[:r], qh_s[hd, pl.ds(qrow, SEG), :], y[r:]], axis=0)
                    res[t][hd] = y

                if not fast:
                    order = [(t, hd) for hd in hds for t in range(2)] + [(2, hd) for hd in hds]
                    parts = [mm((h if t else h[q0:])[:, :kc], wslab(t, hd)[:kc])
                             for t, hd in order[:4 if first else 0]]
                    for n, (t, hd) in enumerate(order):
                        plain(t, hd, parts[n] if n < len(parts) else None)
                    return res

                blocks = sorted((b for b in range(len(BLOCKS)) if BLOCKS[b][2][0] in hds),
                                key=lambda b: (max(BLOCKS[b][2]) - 2 * (b < 10), b))
                accs = [_Acc() for _ in range(3)]
                ts = [t for t in range(3) if t or early is None]

                def run(t, b, sel):
                    alg, dts, bh = BLOCKS[b]
                    for p, e in enumerate(alg):
                        if sel(e):
                            y = mm(left(e, dts), _upk(wtile(t, b, p)))
                            feed(y)
                            accs[t].route(e, bh, y)

                lead = [(t, b) for t in ts[:2] for b in blocks] if first else []
                for t, b in lead:
                    run(t, b, lambda e: e[3] is None)
                todo = list(hds) if early is not None else []
                for t in ts:
                    for b in blocks:
                        run(t, b, (lambda e: e[3] is not None) if (t, b) in lead else (lambda e: True))
                        for _ in range(2):
                            if todo and t == 1:
                                plain(0, todo.pop(0))
                    for hd in hds:
                        y = accs[t].rows(hd)
                        if hd >= 30:
                            y = mm(h[:, 256:384], _upk(plain_tile(t, 2, hd))) + y
                            feed(y)
                        res[t][hd] = y.astype(BF16) if t == 0 else y
                assert not todo
                return res

            def pad(kv):
                return jnp.concatenate([kv, jnp.zeros((128 - kv.shape[0], DH), F32)],
                                       axis=0).astype(BF16)

            def probs(qkv, g):
                scs = [lax.dot_general(qkv[0][hd], pad(qkv[1][hd]), (((1,), (1,)), ((), ())),
                                       preferred_element_type=F32) for hd in GROUPS[g]]
                ps = []
                for n, sc in enumerate(scs):
                    sc = jnp.where(vis, sc, fill)
                    e = jnp.exp2((sc - jnp.max(sc, axis=-1, keepdims=True))
                                 * (scale * math.log2(math.e)))
                    den = jnp.sum(e, axis=-1, keepdims=True)
                    if due and g >= 1 and n in ((0, 5) if g > 2 else (0,)):
                        e = jnp.concatenate([e[:16] + due.pop(0), e[16:]], axis=0)
                    rc = pl.reciprocal(den, approx=True)
                    rc = rc * (2.0 - den * rc)
                    ps.append((e * rc).astype(BF16))
                return ps

            def oproj(h0, h1, acc, mid=None):
                def put(key, y):
                    acc[key] = y + acc[key] if key in acc else y

                if not fast:
                    cuts = list(range(h0, h1, 5)) + [h1] if units else [h0, h1]
                    for n in range(NLB):
                        for a, b in zip(cuts, cuts[1:]):
                            if before_oproj is not None:
                                w = wo_s[a * DH:b * DH, n * 128:(n + 1) * 128]
                                wo_t[n, a * 64:b * 64, :] = pltpu.bitcast(w, U32)
                            else:
                                w = _upk(wo_t[n, a * 64:b * 64, :])
                            put(n, mm(jnp.concatenate(heads[a:b], axis=1).astype(BF16), w))
                            feed(acc[n])
                        if mid is not None and n == NLB - 2:
                            mid()
                    return
                for dts in ((0, 1, 2), (3, 4), (0, 1)):
                    bs = [b for b in range(len(BLOCKS))
                          if BLOCKS[b][1] == dts and h0 <= BLOCKS[b][2][0] < h1]
                    if mid is not None and dts == (3, 4):
                        mid()
                    for p, e in enumerate(BLOCKS[bs[0]][0]) if bs else ():
                        ls = []
                        for b in bs:
                            o = [heads[hd] for hd in BLOCKS[b][2]]
                            parts = [_lin([(c, o[k][r + row * SEG:r + (row + 1) * SEG])
                                           for row, k, c in _nz(e[0])])]
                            if e[3] is not None:
                                parts.insert(0, _lin([(c, o[k][:r])
                                                      for k, c in enumerate(e[3][0]) if c]))
                            ls.append(cat(parts))
                        put((dts, p), mm(cat(ls, 1).astype(BF16),
                                         _upk(cat([wtile(3, b, p) for b in bs]))))
                if h1 == H:
                    put(2, mm(jnp.concatenate(heads[30:], axis=1).astype(BF16),
                              _upk(wo_t[2, 30 * 64:, :])))

            heads, acc = [], {}
            qkv = proj(0)
            for g in range(len(GROUPS)):
                ps = probs(qkv, g)
                vs = [qkv[2][hd] for hd in GROUPS[g]]

                def weigh():
                    heads.extend(mm(p_, pad(v_)) for p_, v_ in zip(ps, vs))
                if g + 1 < len(GROUPS):
                    qkv = proj(g + 1)
                    weigh()
                else:
                    if before_oproj is not None:
                        before_oproj()
                    oproj(0, 18, acc, weigh)
            oproj(18, H, acc)
            assert not units and not due
            if not fast:
                return jnp.concatenate([acc[n] for n in range(NLB)], axis=1)
            out = _Acc()
            for key, y in acc.items():
                if key != 2:
                    out.route((HOPKERR if len(key[0]) == 3 else STRASSEN)[key[1]], key[0], y)
            return jnp.concatenate([out.rows(n) + acc[2] if n == 2 else out.rows(n)
                                    for n in range(NLB)], axis=1)

        def post2(s, toks=None):
            r3 = seg_row(s - 1 - LAG)
            for r in (0, 16):
                xc = _r(x2_s[(s + 4 - 1 - LAG) % 4, r:r + 16] + obuf[SEG + r:SEG + r + 16, :])
                out_s[pl.ds(r3 + r, 16), :] = gate(xc, r3 + r, toks).astype(BF16)

        def step(s, mode, vis, fill, chained=False, before_oproj=None, early=None, units=()):
            if mode == 0:
                h = hbuf[0:ROWS, :]
            elif mode == 1:
                h = hbuf[0:48, :]
            else:
                live = lax.broadcasted_iota(jnp.int32, (2 * M, D), 0) >= M
                mem = jnp.where(live, hbuf[0:16, :].astype(F32), 0.0).astype(BF16)
                h = jnp.concatenate([mem, hbuf[48:80, :]], axis=0)
            toks = []
            if mode != 1:
                post2(s, toks)
            if isinstance(s, int) and s == NSEG + LAG - 1:
                obuf[SEG:2 * SEG, :] = attention(h, vis, fill, chained, due=toks)
                return
            r1 = seg_row(s - 1)
            rn = seg_row(s + 1)
            h1n, h2n = [], []
            for r in (0, 16):
                xa = _r(x_s[pl.ds(r1 + r, 16), :].astype(F32) + obuf[r:r + 16, :])
                xb2 = _r(gate(xa, r1 + r))
                h2n.append(_ln(xb2, toks))
                x2_s[(s + 4 - 1) % 4, r:r + 16] = xb2
            if mode != 2:
                for r in (0, 16):
                    h1n.append(_ln(x_s[pl.ds(rn + r, 16), :].astype(F32), toks))

            if early is not None:
                mrow = pl.multiple_of(early * (8 * PPS), 8 * PPS)
                units = [functools.partial(lambda u, tok: u(tok[0:8]), u)
                         for n in range(PPS) for u in mac_units(mrow + 8 * n, 1)]
                tb = early // 2
                units += [functools.partial(sum_unit, 0, HOPKERR, (0, 1, 2),
                                            (3 * tb, 3 * tb + 1, 3 * tb + 2), 9 * tb,
                                            (early % 2) * 32 + r0) for r0 in range(0, 32, 8)]
                pb = jnp.minimum(early, 16)
                k0, h0 = jnp.where(pb < 16, 3, 0), 2 * jnp.minimum(pb, 15)
                units += [functools.partial(sum_unit, 0, STRASSEN, (k0, k0 + 1), (h0, h0 + 1),
                                            90 + 5 * pb, r0) for r0 in range(0, 64, 8)]

            o = attention(h, vis, fill, chained, before_oproj, early, toks, mode == 0, units)

            mem2 = mem0 if mode == 1 else o[M:2 * M]
            mem = jnp.concatenate([o[0:M], mem2], axis=0)
            hbuf[0:16, :] = mem.astype(BF16)
            for n, v in enumerate(h1n):
                hbuf[16 + 16 * n:32 + 16 * n, :] = v.astype(BF16)
            for n, v in enumerate(h2n):
                hbuf[48 + 16 * n:64 + 16 * n, :] = v.astype(BF16)
            if mode != 2:
                tile = lambda v, dt: v[:, dt * 128:(dt + 1) * 128]
                for i, sig in enumerate(MSIG):
                    m0 = 16 * len(XSIG) + 8 * i
                    sbuf[m0:m0 + 8, :] = _pk(_lin([(c, tile(mem, dt)) for dt, c in sig]))
                for n, xy in enumerate(zip(h1n, h2n)):
                    for i, sig in enumerate(XSIG):
                        sbuf[16 * i + 8 * n:16 * i + 8 * n + 8, :] = _pk(
                            _lin([(c, tile(xy[row], dt)) for row, dt, c in sig]))
            if mode == 0:
                obuf[...] = o[2 * M:]
            elif mode == 1:
                obuf[0:SEG, :] = o[2 * M:]
            else:
                obuf[SEG:2 * SEG, :] = o[2 * M:]

        with _scope("pro"):
            vis, fill = masks(1)
            kv_units = sum_units(1) + sum_units(2)
            cut = len(kv_units) * 2 // 3
            step(0, 1, vis, fill, False, wo_copy.wait, units=kv_units[:cut])
            step(1, 1, vis, fill, True, units=kv_units[cut:] + sum_units(3))
        xb_copy.start()
        vis, fill = masks(0)
        with _scope("main_a"):
            loop(NA // UA, lambda i: [step(UA * i + u + LAG, 0, vis, fill, u > 0, early=UA * i + u)
                                      for u in range(UA)])
        xb_copy.wait()
        with _scope("conv_e"):
            loop(HB // UI, lambda j: [inv_stage(HB + UI * j + u) for u in range(UI)])
        with _scope("main_b"):
            loop((NSEG - LAG - NA) // UB, lambda i: [step(UB * i + u + LAG + NA, 0, vis, fill, u > 0)
                                                     for u in range(UB)])
        done = (NSEG - 1 - LAG) * SEG
        out_a = pltpu.make_async_copy(out_s.at[0:done, :], out_hbm.at[0:done, :], sem.at[SW + 8])
        out_a.start()
        with _scope("epi"):
            vis, fill = masks(2)
            step(NSEG, 2, vis, fill)
            step(NSEG + 1, 2, *masks(2, 2 * M), True)
        post2(NSEG + LAG)
        out_b = pltpu.make_async_copy(out_s.at[done:S, :], out_hbm.at[done:S, :], sem.at[SW + 9])
        out_b.start()
        out_a.wait()
        out_b.wait()

    pl.run_scoped(
        phase1,
        pltpu.VMEM((NSUM * 64, 128), U32),
        pltpu.VMEM((2 * NSUM * 64, 128), U32),
        pltpu.VMEM((NSUM * 64, 128), U32),
    )


@jax.jit
def pallas_interleave_layers__memory_aug_recurrent_mem_tr__ssm_conv_h3__prompt_kernel(
    A_x, A_mem0, A_Wq, A_Wk, A_Wv, A_Wo, A_seg_len,
    B_q, B_k, B_v, B_shift_k, B_ssm_k, B_ssm_D,
):
    del A_seg_len, B_q
    assert A_x.shape == (1, S, D) and A_Wq.shape == (D, H, DH)
    hbm = pl.BlockSpec(memory_space=pl.ANY)
    out = pl.pallas_call(
        _kernel,
        out_shape=jax.ShapeDtypeStruct((S, D), BF16),
        in_specs=[hbm] * 11,
        out_specs=hbm,
        scratch_shapes=[
            pltpu.VMEM((S, D), BF16),
            pltpu.VMEM((H * WP + 352, 128), U32),
            pltpu.VMEM((2 * H * WP + 352, 128), U32),
            pltpu.VMEM((H * DH, D), BF16),
            pltpu.VMEM((NLB, H * DH // 2, 128), U32),
            pltpu.VMEM((TB // 2, TB), U32),
            pltpu.VMEM((2, TB // 2, TB), U32),
            pltpu.VMEM((2, TB // 2, TB), U32),
            pltpu.VMEM((NB, 2, NLB * TB, 128), F32),
            pltpu.VMEM((NB, 3, NLB * TB, 128), F32),
            pltpu.VMEM((NB + 1, 2, NLB * TB, 128), F32),
            pltpu.VMEM((NLB, S + 32, 128), F32),
            pltpu.VMEM((2 * SEG, D), F32),
            pltpu.VMEM((4, SEG, D), F32),
            pltpu.VMEM((S, D), BF16),
            pltpu.VMEM((NQH, NA * SEG, DH), BF16),
            pltpu.VMEM((128, D), BF16),
            pltpu.VMEM((320, 128), U32),
            pltpu.VMEM((64, D), BF16),
            pltpu.SemaphoreType.DMA((HB + HB // 2 + 14,)),
        ],
        compiler_params=pltpu.CompilerParams(vmem_limit_bytes=120 * 1024 * 1024),
    )(A_x.reshape(S, D), A_mem0.reshape(M, D), A_Wq, A_Wk, A_Wv,
      A_Wo.reshape(H * DH, D), B_k.reshape(S, D), B_v.reshape(S, D),
      B_shift_k.T, B_ssm_k, B_ssm_D)
    return out.reshape(1, S, D)
```

```python
import contextlib
import functools
import math

import jax
import jax.numpy as jnp
from jax import lax
import jax.experimental.pallas as pl
import jax.experimental.pallas.tpu as pltpu

F32 = jnp.float32
BF16 = jnp.bfloat16
U32 = jnp.uint32

S = 2048
D = 640
H = 32
DH = 128
M = 8
SEG = 32
NSEG = S // SEG
KS = 4
LAG = 2
ROWS = 2 * M + 2 * SEG
NLB = D // 128
TB = 128
NB = S // TB
HB = NB // 2
NPOS = NLB * TB // 8
NA = 20
PPS = 4
UCUT = tuple(range(a, a + 2) for a in range(0, 12, 2)) + (range(12, 16),)
NQH = 32
UA = 2
UB = 3
UI = 4
WP = 324


STRASSEN = (
    (((1, 0), (0, 1)), ((1, 0), (0, 1)), ((1, 0), (0, 1)), None),
    (((-1, 0), (1, 0)), ((1, 1), (0, 0)), ((0, 0), (0, 1)), None),
    (((0, 1), (0, -1)), ((0, 0), (1, 1)), ((1, 0), (0, 0)), None),
    (((0, 0), (1, 1)), ((1, 0), (0, 0)), ((0, 0), (1, -1)), ((1, 1), (1, 0))),
    (((1, 0), (0, 0)), ((0, 1), (0, -1)), ((0, 1), (0, 1)), ((1, 0), (0, 1))),
    (((0, 0), (0, 1)), ((-1, 0), (1, 0)), ((1, 0), (1, 0)), ((0, 1), (1, 0))),
    (((1, 1), (0, 0)), ((0, 0), (0, 1)), ((-1, 1), (0, 0)), ((1, 1), (0, 1))),
)
HOPKERR = (
    (((1, 0, 0), (0, 0, 0)), ((1, 0, 1), (-1, 0, 0), (0, 0, 0)), ((1, 0, 0), (1, 0, 0)), None),
    (((1, 1, 0), (0, 0, 0)), ((0, 0, 0), (1, 0, 0), (0, 0, 0)), ((1, -1, 0), (0, 0, 0)), None),
    (((-1, 0, 0), (1, 0, 1)), ((0, 0, 1), (0, 0, 0), (1, 0, 0)), ((1, 0, -1), (1, 0, 0)), None),
    (((0, 1, 0), (0, -1, 0)), ((0, 0, 0), (1, 1, 0), (0, -1, 0)), ((0, 1, 0), (0, 0, 0)), None),
    (((0, 1, 1), (0, -1, 0)), ((0, 0, 0), (0, 0, 1), (0, 1, 0)), ((0, 1, 0), (0, 1, -1)), None),
    (((0, 0, 1), (0, 0, 0)), ((0, 0, 0), (0, 0, -1), (1, 0, 1)), ((0, 0, 1), (0, 0, 0)), None),
    (((-1, 0, 0), (1, 0, 0)), ((1, 1, 0), (0, 0, 0), (-1, 0, 0)), ((0, 0, 0), (1, 0, 0)),
     ((1, 0, 0), (1, 0, 0))),
    (((1, 0, 0), (0, 1, 0)), ((0, 1, 0), (1, 0, 0), (0, 0, 0)), ((0, 1, 0), (1, 0, 0)),
     ((0, 1, 0), (1, 0, 0))),
    (((0, 0, 0), (1, 1, 0)), ((0, 1, 0), (0, 0, 0), (0, 0, 0)), ((0, 0, 0), (-1, 1, 0)),
     ((1, 1, 0), (-1, 1, 0))),
    (((0, 0, 0), (1, 0, 1)), ((0, 0, 1), (0, 0, 0), (0, 0, 0)), ((-1, 0, 1), (-1, 0, 1)),
     ((1, 0, 1), (0, 0, 1))),
    (((-1, 0, -1), (1, 0, 1)), ((0, 0, 0), (0, 0, 0), (1, 0, 0)), ((-1, 0, 1), (0, 0, 0)),
     ((1, 0, 1), (1, 0, 0))),
    (((0, 0, 0), (0, 1, 0)), ((0, -1, 0), (0, 1, 1), (0, 0, 0)), ((0, 1, 0), (0, 1, 0)),
     ((0, 1, 0), (0, 1, 0))),
    (((0, 1, 1), (0, 0, 0)), ((0, 0, 0), (0, 0, 1), (0, 0, 0)), ((0, -1, 1), (0, -1, 1)),
     ((0, 1, 0), (0, -1, 1))),
    (((0, -1, -1), (0, 1, 1)), ((0, 0, 0), (0, 0, 0), (0, 1, 0)), ((0, 0, 0), (0, 1, -1)),
     ((0, 0, 1), (0, 1, -1))),
    (((0, 0, 0), (0, 0, 1)), ((0, 0, -1), (0, 0, 0), (0, 1, 1)), ((0, 0, 0), (0, 0, 1)),
     ((0, 0, 1), (0, 0, 1))),
)
BLOCKS = ([(HOPKERR, (0, 1, 2), (3 * i, 3 * i + 1, 3 * i + 2)) for i in range(10)]
          + [(STRASSEN, (3, 4), (2 * i, 2 * i + 1)) for i in range(16)]
          + [(STRASSEN, (0, 1), (30, 31))])
GROUPS = [tuple(range(a, b)) for a, b in ((0, 6), (6, 12), (12, 18), (18, 24), (24, 32))]
NSUM = 10 * 9 + 17 * 5


def _nz(mat):
    return tuple((i, j, c) for i, row in enumerate(mat) for j, c in enumerate(row) if c)


def _summed(alg):
    return [p for p, e in enumerate(alg) if len(_nz(e[1])) > 1]


def _slot(b, p):
    sm = _summed(BLOCKS[b][0])
    if p not in sm:
        return None
    return (9 * b if b < 10 else 90 + 5 * (b - 10)) + sm.index(p)


def _lin(terms):
    terms = sorted(terms, key=lambda t: -t[0])
    acc = terms[0][1]
    for c, v in terms[1:]:
        acc = acc + v if c > 0 else acc - v
    return acc


class _Acc:
    def __init__(self):
        self.d = {}

    def add(self, key, c, v):
        if key not in self.d:
            self.d[key] = (c, v)
            return
        c0, v0 = self.d[key]
        self.d[key] = (c0, v0 + v) if c == c0 else (1, _lin([(c0, v0), (c, v)]))

    def route(self, e, ns, y):
        r = 0 if e[3] is None else 2 * M
        for row, n, c in _nz(e[2]):
            self.add((row + 1, ns[n]), c, y[r:])
        if r:
            for n, c in enumerate(e[3][1]):
                if c:
                    self.add((0, ns[n]), c, y[:r])

    def rows(self, n):
        assert all(self.d[(i, n)][0] == 1 for i in range(3))
        return jnp.concatenate([self.d[(i, n)][1] for i in range(3)], axis=0)


def _row_sigs():
    xs, ms = [], []
    for alg, dts, _ in BLOCKS:
        for e in alg:
            x = tuple((r, dts[k], c) for r, k, c in _nz(e[0]))
            if len(x) > 1 and x not in xs:
                xs.append(x)
            if e[3] is not None:
                m = tuple((dts[k], c) for k, c in enumerate(e[3][0]) if c)
                if len(m) > 1 and m not in ms:
                    ms.append(m)
    return xs, ms


XSIG, MSIG = _row_sigs()
PROFILE = False


def _scope(name):
    return jax.named_scope(name) if PROFILE else contextlib.nullcontext()


def _ln(x, toks=None):
    m = jnp.mean(x, axis=-1, keepdims=True)
    c = x - m
    v = jnp.mean(c * c, axis=-1, keepdims=True)
    r = lax.rsqrt(v + 1e-5)
    if toks is not None:
        toks.append(jnp.minimum(r, 0.0))
    return c * r


def _r(x):
    return x.astype(BF16).astype(F32)


def _split(x):
    hi = pltpu.bitcast(pltpu.bitcast(x, U32) & jnp.uint32(0xFFFF0000), F32)
    return hi, x - hi


def _pk(x):
    return pltpu.bitcast(x.astype(BF16), U32)


def _upk(w):
    return pltpu.bitcast(w, BF16)


def _basis(r, t):
    b = r & 63
    f = jnp.where(b < 32, 2 * b, 2 * b - 63)
    n = ((2 * f + 1) * t - jnp.where(r >= 64, TB, 0)) & (4 * TB - 1)
    n = jnp.where(n >= 2 * TB, n - 4 * TB, n)
    return jnp.cos(n.astype(F32) * (2.0 * math.pi / (4 * TB)))


def _halves(x):
    w = pltpu.bitcast(x, U32)
    return (pltpu.bitcast(w << 16, F32),
            pltpu.bitcast(w & jnp.uint32(0xFFFF0000), F32))


def _kernel(x_hbm, mem0_hbm, wq_hbm, wk_hbm, wv_hbm, wo_hbm,
            k_hbm, v_hbm, shk_hbm, ssmk_hbm, ssmd_hbm,
            out_hbm,
            x_s, wt_q, wt_kv, wo_s, wo_t,
            perm_s, fu_s, inv_s, u_s, kf_s, c_s, y_s,
            obuf, x2_s, out_s, qh_s, hbuf, sbuf, mem0_ref,
            sem):
    X0, XH = LAG * SEG, (LAG + NA) * SEG
    SW = HB + HB // 2
    hb = TB // 2
    wo_copy = pltpu.make_async_copy(wo_hbm, wo_s, sem.at[SW + 3])
    xb_copy = pltpu.make_async_copy(x_hbm.at[XH + SEG:, :], x_s.at[XH + SEG:, :], sem.at[SW + 7])

    def mac_units(row, half):
        rs = pl.ds(row, 8)
        state = {}

        def unit(p, avals, final, tok=None):
            acc = state.setdefault(p, dict(state.get(0, {})))
            for a in avals:
                u = u_s[a, 0, rs] + u_s[a, 1, rs] if p == 0 else u_s[a, p - 1, rs]
                if tok is not None:
                    u = u + tok
                for i in range(max(a, half * HB), half * HB + HB):
                    t = u * kf_s[i - a, p, rs]
                    acc[i] = t if i not in acc else (acc[i] - t if p == 2 else acc[i] + t)
            if final and p:
                for i, v in acc.items():
                    c_s[i + 1, 2 - p, rs] = v

        subs = UCUT if half else (range(HB),)
        return [functools.partial(unit, p, avals, n == len(subs) - 1)
                for p in range(3) for n, avals in enumerate(subs)]

    def inv_stage(i, units=None):
        q = TB // 4
        for g in range(NLB):
            re, im = [], []
            for b in range(4):
                rows = slice(g * TB + b * q, g * TB + (b + 1) * q)
                cr, ci_ = c_s[i + 1, 0, rows], c_s[i + 1, 1, rows]
                pr, pi = c_s[i, 0, rows], c_s[i, 1, rows]
                re.append(cr + pi if b in (0, 3) else cr - pi)
                im.append(ci_ - pr if b in (0, 3) else ci_ + pr)
            pe = jnp.concatenate([re[0] + re[2], re[1] + re[3], im[0] - im[2], im[1] - im[3]], axis=0)
            po = jnp.concatenate([re[0] - re[2], re[1] - re[3], im[0] + im[2], im[1] + im[3]], axis=0)
            for par, pp in enumerate((pe, po)):
                ph, plo = _split(pp)
                gh_, gl_ = (inv_s[n, par * q:(par + 1) * q] for n in range(2))
                y = jnp.dot(_upk(jnp.concatenate([gh_, gl_, gh_], axis=1)),
                            jnp.concatenate([ph, ph, plo], axis=0).astype(BF16),
                            preferred_element_type=F32)
                y_s[g, pl.ds(i * TB + par, hb, stride=2), :] = y
                if units:
                    tok = pltpu.bitcast(jnp.minimum(jnp.abs(y[0:16]), 0.0), U32)
                    for _ in range(3):
                        if units:
                            units.pop(0)(tok)

    def wslab(t, h):
        s0 = (max(t - 1, 0) * H + (h % 2) * 16 + h // 2) * WP
        return pltpu.bitcast((wt_kv if t else wt_q)[s0:s0 + D // 2, :], BF16)

    def loop(n, fn):
        def body(j, _):
            fn(j)
            return 0
        lax.fori_loop(0, n, body, 0)

    def phase0(k_s, v_s, ssmk_s, wraw, kpad, hl_s, shk_ref, ssmd_ref):

        def pair_rows(jp):
            r0 = jp * 2 * TB
            return pl.ds(r0 if isinstance(jp, int) else pl.multiple_of(r0, 2 * TB), 2 * TB)

        def ssmk_copy(jp):
            return pltpu.make_async_copy(ssmk_hbm.at[:, pair_rows(jp)], ssmk_s.at[jp], sem.at[jp])

        def kv_copies(rows, sm):
            return [pltpu.make_async_copy(k_hbm.at[rows, :], k_s.at[rows, :], sm),
                    pltpu.make_async_copy(v_hbm.at[rows, :], v_s.at[rows, :], sm)]
        DQ = 192
        wq_early = [pltpu.make_async_copy(wq_hbm.at[n * DQ:(n + 1) * DQ], wraw.at[0, n * DQ:(n + 1) * DQ],
                                          sem.at[SW + 10 + n]) for n in range(2)]
        w_copies = [pltpu.make_async_copy(wq_hbm.at[2 * DQ:], wraw.at[0, 2 * DQ:], sem.at[SW])]
        w_copies += [pltpu.make_async_copy(w.at[n * (D // 2):(n + 1) * (D // 2)],
                                           wraw.at[t, n * (D // 2):(n + 1) * (D // 2)],
                                           sem.at[SW + 11 * n + t])
                     for t, w in ((1, wk_hbm), (2, wv_hbm)) for n in range(2)]
        late_copies = kv_copies(pl.ds(S // 2, S // 2), sem.at[SW + 4])
        small_copies = [pltpu.make_async_copy(src, dst, sem.at[SW + 5])
                        for src, dst in ((shk_hbm, shk_ref), (ssmd_hbm, ssmd_ref), (mem0_hbm, mem0_ref.at[0:M]))]
        XM = XH - 2 * TB
        xa_copy = pltpu.make_async_copy(x_hbm.at[X0:XM, :], x_s.at[X0:XM, :], sem.at[SW + 6])
        late_copies += [pltpu.make_async_copy(x_hbm.at[a:b, :], x_s.at[a:b, :], sem.at[SW + 4])
                        for a, b in ((0, X0), (XM, XH + SEG))]
        for c in (small_copies + [ssmk_copy(jp) for jp in range(HB)]
                  + [c for jp in range(HB // 2) for c in kv_copies(pair_rows(jp), sem.at[HB + jp])]
                  + [xa_copy] + wq_early + [w_copies[0]] + late_copies + w_copies[1:] + [wo_copy]):
            c.start()

        ri = lax.broadcasted_iota(jnp.int32, (TB, TB), 0)
        ci = lax.broadcasted_iota(jnp.int32, (TB, TB), 1)
        perm_s[...] = _pk(jnp.where(ci == 2 * (ri & 63) + (ri >> 6), 1.0, 0.0))
        tab = _basis(ri, 2 * (ci & 63) + (ci >> 6))
        hi, lo = _split(tab)
        fu_s[0] = _pk(jnp.where(ci < hb, hi, pltpu.roll(lo, hb, 1)))
        fu_s[1] = _pk(jnp.where(ci < hb, pltpu.roll(hi, hb, 1), lo))
        gh, gl = _split(tab.T * (1.0 / TB))
        inv_s[0] = _pk(gh)
        inv_s[1] = _pk(gl)

        for c in small_copies:
            c.wait()
        shk_t = shk_ref[...].astype(F32)
        taps = [[shk_t[j:j + 1, g * 128:(g + 1) * 128] for g in range(NLB)] for j in range(KS)]
        dvec = ssmd_ref[...].astype(F32).reshape(1, D)
        for g in range(NLB):
            kpad[0, g, 0:8, :] = jnp.zeros((8, 128), F32)
            kpad[1, g, 0:8, :] = jnp.zeros((8, 128), F32)
        c_s[0] = jnp.zeros(c_s.shape[1:], F32)
        hbuf[0:16, :] = jnp.concatenate([mem0_ref[0:M, :].astype(F32)] * 2, axis=0).astype(BF16)
        obuf[...] = jnp.zeros((2 * SEG, D), F32)
        x2_s[...] = jnp.zeros(x2_s.shape, F32)

        def spectrum(e, o):
            fe = jnp.dot(_upk(fu_s[0]), jnp.concatenate([e, e], axis=0).astype(BF16), preferred_element_type=F32)
            fo = jnp.dot(_upk(fu_s[1]), jnp.concatenate([o, o], axis=0).astype(BF16), preferred_element_type=F32)
            return ((fe[:hb] + fo[:hb], fe[hb:] + fo[hb:]), (fe[:hb] - fo[:hb], fo[hb:] - fe[hb:]))

        def freq_rows(g):
            return slice(g * TB, g * TB + hb), slice(g * TB + hb, (g + 1) * TB)

        def fwd_k(jq):
            def transposed(n):
                if n % 2 == 0:
                    ssmk_copy(2 * jq + n // 2).wait()
                blk = ssmk_s[2 * jq + n // 2, :, (n % 2) * TB:(n % 2 + 1) * TB]
                return lax.dot_general(_upk(perm_s[...]), blk, (((1,), (1,)), ((), ())),
                                       preferred_element_type=F32)
            nxt = transposed(0)
            for n in range(4):
                kt = nxt
                if n < 3:
                    nxt = transposed(n + 1)
                j = 4 * jq + n
                for g in range(NLB):
                    lb = slice(g * 128, (g + 1) * 128)
                    for rows, (kr, ki) in zip(freq_rows(g), spectrum(kt[:hb, lb], kt[hb:, lb])):
                        if n == 0:
                            kr = kr + jnp.where(j == 0, dvec[:, lb], 0.0)
                        kf_s[j, 0, rows] = kr
                        kf_s[j, 1, rows] = ki - kr
                        kf_s[j, 2, rows] = kr + ki

        def fwd_u(jq, first):
            if first:
                for jp in (2 * jq, 2 * jq + 1):
                    for c in kv_copies(pair_rows(jp), sem.at[HB + jp]):
                        c.wait()
            for j in [4 * jq + n for n in range(4)]:
                r0 = pl.multiple_of(j * TB, TB)
                q0 = pl.multiple_of(j * hb, hb) + 8
                for g in range(NLB):
                    lb = slice(g * 128, (g + 1) * 128)
                    ke, ko = _halves(k_s[pl.ds(r0, TB), lb])
                    ve, vo = _halves(v_s[pl.ds(r0, TB), lb])
                    kpad[0, g, pl.ds(q0, hb), :] = ke
                    kpad[1, g, pl.ds(q0, hb), :] = ko
                    ke1 = kpad[0, g, pl.ds(q0 - 1, hb), :]
                    ko1 = kpad[1, g, pl.ds(q0 - 1, hb), :]
                    ko2 = kpad[1, g, pl.ds(q0 - 2, hb), :]
                    t0, t1, t2, t3 = (taps[t][g] for t in range(KS))
                    e = (ke * t0 + ko1 * t1 + ke1 * t2 + ko2 * t3) * ve
                    o = (ko * t0 + ke * t1 + ko1 * t2 + ke1 * t3) * vo
                    for rows, (ur, ui) in zip(freq_rows(g), spectrum(e, o)):
                        u_s[j, 0, rows] = ur
                        u_s[j, 1, rows] = ui

        def relayout_rows(t, dst, base, dp, tok=None):
            a = pltpu.bitcast(wraw[t, 2 * dp], U32)
            b = pltpu.bitcast(wraw[t, 2 * dp + 1], U32)
            if tok is not None:
                a = a | tok
            dst[pl.ds(base + dp, 16, stride=WP), :] = (a & jnp.uint32(0xFFFF)) | (b << 16)
            dst[pl.ds(base + 16 * WP + dp, 16, stride=WP), :] = (
                (a >> 16) | (b & jnp.uint32(0xFFFF0000)))

        def norm_rows(r0, nr):
            r0 = pl.multiple_of(r0, 16)
            for r in range(0, nr, 16):
                hl_s[pl.ds(r0 + r, 16), :] = _ln(
                    x_s[pl.ds(r0 + r + LAG * SEG, 16), :].astype(F32)).astype(BF16)

        def pre_queries(c, t=None):
            per = -(-(D // 4) // NQH)
            for sub in range(2):
                if t is not None:
                    half = wraw.at[t, sub * (D // 2):(sub + 1) * (D // 2)]
                    pltpu.make_async_copy(half, half, sem.at[SW + 11 * sub + t]).wait()
                    base = (t - 1) * (H * WP)
                    dp = sub * (D // 4)
                r0 = pl.multiple_of((2 * c + sub) * QR, QR)
                hl = hl_s[pl.ds(r0, QR), :]
                for hd in range(NQH):
                    r = jnp.dot(hl, wslab(0, hd), preferred_element_type=F32)
                    qh_s[hd, pl.ds(r0, QR), :] = r.astype(BF16)
                    if t is not None:
                        tok = pltpu.bitcast(jnp.minimum(jnp.abs(r[0:16]), 0.0), U32)
                        for _ in range(per):
                            if dp < (sub + 1) * (D // 4):
                                relayout_rows(t, wt_kv, base, dp, tok)
                                dp += 1

        nch = NA * SEG // TB
        QR = TB // 2
        with _scope("conv_k"):
            loop(HB // 2, fwd_k)
        with _scope("conv_u"):
            loop(HB // 4, lambda j: fwd_u(j, True))
        with _scope("conv_b"):
            loop(NPOS // 10, lambda j: [u() for n in range(10)
                                        for u in mac_units(pl.multiple_of(80 * j, 16) + 8 * n, 0)])
            xa_copy.wait()

            def inv_first(j):
                part = wraw.at[0, pl.ds(j * DQ, DQ)]
                pltpu.make_async_copy(part, part, sem.at[SW + 10 + j]).wait()
                units = [functools.partial(relayout_rows, 0, wt_q, 0, j * (DQ // 2) + dd)
                         for dd in range(DQ // 2)]
                for u in range(UI):
                    inv_stage(UI * j + u, units)
                assert not units
                norm_rows(j * ((XM - X0) // 2), (XM - X0) // 2)
            loop(HB // UI, inv_first)
        with _scope("rel0"):
            w_copies[0].wait()
            loop((D - 2 * DQ) // 64,
                 lambda i: [relayout_rows(0, wt_q, 0, DQ + i * 32 + dd) for dd in range(32)])
        with _scope("preq"):
            loop(nch - 2, pre_queries)
        with _scope("conv_c"):
            for c in late_copies:
                c.wait()

            def fwd_u_late(j):
                r0 = pl.multiple_of(j * 16, 16)
                hbuf[pl.ds(16 + r0, 16), :] = _ln(x_s[pl.ds(r0, 16), :].astype(F32)).astype(BF16)
                norm_rows(XM - X0 + j * TB, TB)
                fwd_u(HB // 4 + j, False)
            loop(HB // 4, fwd_u_late)
        with _scope("preq_rel"):
            loop(2, lambda i: pre_queries(i + nch - 2, i + 1))

    pl.run_scoped(
        phase0,
        pltpu.VMEM((S, D), BF16),
        pltpu.VMEM((S, D), BF16),
        pltpu.VMEM((HB, D, 2 * TB), BF16),
        pltpu.VMEM((3, D, H, DH), BF16),
        pltpu.VMEM((2, NLB, S // 2 + 32, 128), F32),
        pltpu.VMEM((NA * SEG, D), BF16),
        pltpu.VMEM((KS, D), BF16),
        pltpu.VMEM((D,), BF16),
    )

    def phase1(cq, ckv, co):
        scale = DH ** -0.5

        def masks(mode, q0=0):
            rows = ROWS if mode == 0 else ROWS - SEG
            qi = lax.broadcasted_iota(jnp.int32, (rows - q0, 128), 0) + q0
            kj = lax.broadcasted_iota(jnp.int32, (rows - q0, 128), 1)

            def layer_of(i):
                xl = (i - 2 * M) // SEG if mode == 0 else mode - 1
                return jnp.where(i < 2 * M, i // M, xl)
            same = (layer_of(qi) == layer_of(kj)) & (kj < rows)
            vis = same & ((qi < 2 * M) | (qi >= kj))
            fill = jnp.where(same, -1e9 / scale, -jnp.inf).astype(F32)
            return vis, fill

        mem0 = mem0_ref[0:M, :].astype(F32)

        def seg_row(seg):
            if isinstance(seg, int):
                return min(max(seg, 0), NSEG - 1) * SEG
            return pl.multiple_of(jnp.clip(seg, 0, NSEG - 1) * SEG, SEG)

        def gate(xa, r0, toks=None):
            y = jnp.concatenate([y_s[g, pl.ds(r0, xa.shape[0]), :] for g in range(NLB)], axis=1)
            return xa + _ln(xa, toks) * y

        def mm(a, b):
            return jnp.dot(a, b, preferred_element_type=F32)

        def cat(vs, axis=0):
            return vs[0] if len(vs) == 1 else jnp.concatenate(vs, axis=axis)

        def plain_tile(t, dt, hd, r0=0, nr=64):
            if t == 3:
                return wo_t[dt, pl.ds(hd * 64 + r0, nr), :]
            s0 = (max(t - 1, 0) * H + (hd % 2) * 16 + hd // 2) * WP
            return (wt_kv if t else wt_q)[pl.ds(s0 + dt * 64 + r0, nr), :]

        def sum_ref(t):
            return (cq, ckv, ckv, co)[t], (NSUM * 64 if t == 2 else 0)

        def wtile(t, b, p):
            alg, dts, hds = BLOCKS[b]
            if _slot(b, p) is None:
                (k, n, _), = _nz(alg[p][1])
                return plain_tile(t, dts[n], hds[k]) if t == 3 else plain_tile(t, dts[k], hds[n])
            ref, r0 = sum_ref(t)
            r0 += _slot(b, p) * 64
            return ref[r0:r0 + 64, :]

        def sum_unit(t, alg, dts, hds, slot0, r0, tok):
            src = {}
            for k in range(len(dts)):
                for n in range(len(dts)):
                    w = (plain_tile(t, dts[n], hds[k], r0, 8) if t == 3
                         else plain_tile(t, dts[k], hds[n], r0, 8))
                    if (n - k) % len(dts) == len(dts) - 2:
                        w = w | pltpu.bitcast(tok[0:8], U32)
                    src[k, n] = _upk(w).astype(F32)
            ref, base = sum_ref(t)
            sums = _pk(jnp.concatenate([_lin([(c, src[k, n]) for k, n, c in _nz(alg[p][1])])
                                        for p in _summed(alg)], axis=1))
            for i in range(len(_summed(alg))):
                ref[pl.ds(base + (slot0 + i) * 64 + r0, 8), :] = sums[:, i * 128:(i + 1) * 128]

        def sum_units(t):
            jobs = [(b, r0) for b in range(len(BLOCKS)) for r0 in range(0, 64, 8)]
            jobs.sort(key=lambda j: (j[0] * 64 + j[1]) / 640 if j[0] < 10
                      else ((j[0] - 10) * 64 + j[1]) / (17 * 64))
            return [functools.partial(sum_unit, t, *BLOCKS[b], _slot(b, _summed(BLOCKS[b][0])[0]), r0)
                    for b, r0 in jobs]

        def attention(h, vis, fill, chained, before_oproj=None, early=None, due=(), fast=False,
                      units=()):
            q0 = h.shape[0] - vis.shape[0]
            r = 2 * M
            units, due = list(units), list(due)
            nprod = sum(len(b[0]) for b in BLOCKS) + 2
            ncall = (3 * H if before_oproj else 4 * H - 4) if not fast else (3 * nprod if early is None else 2 * nprod + 5 * H)
            nunit, state = len(units), [0]
            if early is not None:
                hrest = jnp.concatenate([h[:r], h[r + SEG:]], axis=0)
                qrow = pl.multiple_of(early * SEG, SEG)
            if fast:
                sb = sbuf[0:16 * len(XSIG) + 8 * len(MSIG), :]

            def feed(x, weight=1):
                state[0] += weight
                n = -(-nunit * state[0] // ncall) - (nunit - len(units))
                if n > 0:
                    tok = jnp.minimum(jnp.abs(x[0:16]), 0.0)
                    for u in units[:n]:
                        u(tok)
                    del units[:n]

            def left(e, dts):
                x = tuple((row, dts[k], c) for row, k, c in _nz(e[0]))
                if len(x) > 1:
                    parts = [_upk(sb[16 * XSIG.index(x):16 * XSIG.index(x) + 16])]
                else:
                    row, dt, _ = x[0]
                    parts = [h[r + row * SEG:r + (row + 1) * SEG, dt * 128:(dt + 1) * 128]]
                if e[3] is not None:
                    m = tuple((dts[k], c) for k, c in enumerate(e[3][0]) if c)
                    if len(m) > 1:
                        m0 = 16 * len(XSIG) + 8 * MSIG.index(m)
                        parts.insert(0, _upk(sb[m0:m0 + 8]))
                    else:
                        parts.insert(0, h[:r, m[0][0] * 128:(m[0][0] + 1) * 128])
                return cat(parts)

            def proj(g, hooks=()):
                hds = GROUPS[g]
                hooks = list(hooks)

                def tick(done, total):
                    if hooks and done * 3 >= total * (3 - len(hooks)):
                        hooks.pop(0)()
                res = [{} for _ in range(3)]
                first = g == 0 and chained
                kc = D - 128

                def plain(t, hd, part=None):
                    pre = early is not None and t == 0
                    x = hrest if pre else (h if t else h[q0:])
                    if part is None:
                        y = mm(x, wslab(t, hd))
                    else:
                        y = mm(x[:, kc:], wslab(t, hd)[kc:]) + part
                    feed(y, 5 if fast else 1)
                    if t == 0:
                        y = y.astype(BF16)
                    if pre:
                        y = jnp.concatenate([y[:r], qh_s[hd, pl.ds(qrow, SEG), :], y[r:]], axis=0)
                    res[t][hd] = y

                if not fast:
                    order = [(t, hd) for hd in hds for t in range(2)] + [(2, hd) for hd in hds]
                    parts = [mm((h if t else h[q0:])[:, :kc], wslab(t, hd)[:kc])
                             for t, hd in order[:4 if first else 0]]
                    for n, (t, hd) in enumerate(order):
                        tick(n, len(order))
                        plain(t, hd, parts[n] if n < len(parts) else None)
                    return res

                blocks = sorted((b for b in range(len(BLOCKS)) if BLOCKS[b][2][0] in hds),
                                key=lambda b: (max(BLOCKS[b][2]) - 2 * (b < 10), b))
                accs = [_Acc() for _ in range(3)]
                ts = [t for t in range(3) if t or early is None]

                def run(t, b, sel):
                    alg, dts, bh = BLOCKS[b]
                    for p, e in enumerate(alg):
                        if sel(e):
                            y = mm(left(e, dts), _upk(wtile(t, b, p)))
                            feed(y)
                            accs[t].route(e, bh, y)

                lead = [(t, b) for t in ts[:2] for b in blocks] if first else []
                for t, b in lead:
                    run(t, b, lambda e: e[3] is None)
                todo = list(hds) if early is not None else []
                start = state[0]
                total = ncall * len(hds) // H
                for t in ts:
                    for b in blocks:
                        tick(state[0] - start, total)
                        run(t, b, (lambda e: e[3] is not None) if (t, b) in lead else (lambda e: True))
                        for _ in range(2):
                            if todo and t == 1:
                                plain(0, todo.pop(0))
                    for hd in hds:
                        y = accs[t].rows(hd)
                        if hd >= 30:
                            y = mm(h[:, 256:384], _upk(plain_tile(t, 2, hd))) + y
                            feed(y)
                        res[t][hd] = y.astype(BF16) if t == 0 else y
                assert not todo and not hooks
                return res

            def pad(kv):
                return jnp.concatenate([kv, jnp.zeros((128 - kv.shape[0], DH), F32)],
                                       axis=0).astype(BF16)

            def probs(qkv, hds):
                scs = [lax.dot_general(qkv[0][hd], pad(qkv[1][hd]), (((1,), (1,)), ((), ())),
                                       preferred_element_type=F32) for hd in hds]
                ps = []
                for n, sc in enumerate(scs):
                    sc = jnp.where(vis, sc, fill)
                    e = jnp.exp2((sc - jnp.max(sc, axis=-1, keepdims=True))
                                 * (scale * math.log2(math.e)))
                    den = jnp.sum(e, axis=-1, keepdims=True)
                    if due and n == 0 and hds[0] >= 6:
                        e = jnp.concatenate([e[:16] + due.pop(0), e[16:]], axis=0)
                    rc = pl.reciprocal(den, approx=True)
                    rc = rc * (2.0 - den * rc)
                    ps.append((e * rc).astype(BF16))
                return ps

            def oproj(h0, h1, acc, mid=()):
                mid = list(mid)

                def put(key, y):
                    acc[key] = y + acc[key] if key in acc else y

                if not fast:
                    cuts = list(range(h0, h1, 5)) + [h1] if units else [h0, h1]
                    for n in range(NLB):
                        for a, b in zip(cuts, cuts[1:]):
                            if before_oproj is not None:
                                w = wo_s[a * DH:b * DH, n * 128:(n + 1) * 128]
                                wo_t[n, a * 64:b * 64, :] = pltpu.bitcast(w, U32)
                            else:
                                w = _upk(wo_t[n, a * 64:b * 64, :])
                            put(n, mm(jnp.concatenate(heads[a:b], axis=1).astype(BF16), w))
                            feed(acc[n])
                        if mid and n in (0, 2, 3):
                            mid.pop(0)()
                    return
                for dts in ((0, 1, 2), (3, 4), (0, 1)):
                    bs = [b for b in range(len(BLOCKS))
                          if BLOCKS[b][1] == dts and h0 <= BLOCKS[b][2][0] < h1]
                    for p, e in enumerate(BLOCKS[bs[0]][0]) if bs else ():
                        if mid and (len(dts), p) in ((3, 4), (3, 12), (2, 3)):
                            mid.pop(0)()
                        ls = []
                        for b in bs:
                            o = [heads[hd] for hd in BLOCKS[b][2]]
                            parts = [_lin([(c, o[k][r + row * SEG:r + (row + 1) * SEG])
                                           for row, k, c in _nz(e[0])])]
                            if e[3] is not None:
                                parts.insert(0, _lin([(c, o[k][:r])
                                                      for k, c in enumerate(e[3][0]) if c]))
                            ls.append(cat(parts))
                        put((dts, p), mm(cat(ls, 1).astype(BF16),
                                         _upk(cat([wtile(3, b, p) for b in bs]))))
                if h1 == H:
                    put(2, mm(jnp.concatenate(heads[30:], axis=1).astype(BF16),
                              _upk(wo_t[2, 30 * 64:, :])))

            heads, acc = [], {}
            qkv = proj(0)
            for g, hds in enumerate(GROUPS):
                ha, hb_ = hds[:len(hds) // 2], hds[len(hds) // 2:]
                cur, ps = qkv, probs(qkv, ha)

                def weigh(sub):
                    heads.extend(mm(ps[hd - hds[0]], pad(cur[2][hd])) for hd in sub)
                hooks = [lambda: ps.extend(probs(cur, hb_)), lambda: weigh(ha)]
                if g + 1 < len(GROUPS):
                    qkv = proj(g + 1, hooks)
                    weigh(hb_)
                else:
                    if before_oproj is not None:
                        before_oproj()
                    oproj(0, 18, acc, hooks + [lambda: weigh(hb_)])
            oproj(18, H, acc)
            assert not units and not due
            if not fast:
                return jnp.concatenate([acc[n] for n in range(NLB)], axis=1)
            out = _Acc()
            for key, y in acc.items():
                if key != 2:
                    out.route((HOPKERR if len(key[0]) == 3 else STRASSEN)[key[1]], key[0], y)
            return jnp.concatenate([out.rows(n) + acc[2] if n == 2 else out.rows(n)
                                    for n in range(NLB)], axis=1)

        def post2(s, toks=None):
            r3 = seg_row(s - 1 - LAG)
            for r in (0, 16):
                xc = _r(x2_s[(s + 4 - 1 - LAG) % 4, r:r + 16] + obuf[SEG + r:SEG + r + 16, :])
                out_s[pl.ds(r3 + r, 16), :] = gate(xc, r3 + r, toks).astype(BF16)

        def step(s, mode, vis, fill, chained=False, before_oproj=None, early=None, units=()):
            if mode == 0:
                h = hbuf[0:ROWS, :]
            elif mode == 1:
                h = hbuf[0:48, :]
            else:
                live = lax.broadcasted_iota(jnp.int32, (2 * M, D), 0) >= M
                mem = jnp.where(live, hbuf[0:16, :].astype(F32), 0.0).astype(BF16)
                h = jnp.concatenate([mem, hbuf[48:80, :]], axis=0)
            toks = []
            if mode != 1:
                post2(s, toks)
            if isinstance(s, int) and s == NSEG + LAG - 1:
                obuf[SEG:2 * SEG, :] = attention(h, vis, fill, chained, due=toks)
                return
            r1 = seg_row(s - 1)
            rn = seg_row(s + 1)
            h1n, h2n = [], []
            for r in (0, 16):
                xa = _r(x_s[pl.ds(r1 + r, 16), :].astype(F32) + obuf[r:r + 16, :])
                xb2 = _r(gate(xa, r1 + r))
                h2n.append(_ln(xb2, toks))
                x2_s[(s + 4 - 1) % 4, r:r + 16] = xb2
            if mode != 2:
                for r in (0, 16):
                    h1n.append(_ln(x_s[pl.ds(rn + r, 16), :].astype(F32), toks))

            if early is not None:
                mrow = pl.multiple_of(early * (8 * PPS), 8 * PPS)
                units = [functools.partial(lambda u, tok: u(tok[0:8]), u)
                         for n in range(PPS) for u in mac_units(mrow + 8 * n, 1)]
                tb = early // 2
                units += [functools.partial(sum_unit, 0, HOPKERR, (0, 1, 2),
                                            (3 * tb, 3 * tb + 1, 3 * tb + 2), 9 * tb,
                                            (early % 2) * 32 + r0) for r0 in range(0, 32, 8)]
                pb = jnp.minimum(early, 16)
                k0, h0 = jnp.where(pb < 16, 3, 0), 2 * jnp.minimum(pb, 15)
                units += [functools.partial(sum_unit, 0, STRASSEN, (k0, k0 + 1), (h0, h0 + 1),
                                            90 + 5 * pb, r0) for r0 in range(0, 64, 8)]

            o = attention(h, vis, fill, chained, before_oproj, early, toks, mode == 0, units)

            mem2 = mem0 if mode == 1 else o[M:2 * M]
            mem = jnp.concatenate([o[0:M], mem2], axis=0)
            hbuf[0:16, :] = mem.astype(BF16)
            for n, v in enumerate(h1n):
                hbuf[16 + 16 * n:32 + 16 * n, :] = v.astype(BF16)
            for n, v in enumerate(h2n):
                hbuf[48 + 16 * n:64 + 16 * n, :] = v.astype(BF16)
            if mode != 2:
                tile = lambda v, dt: v[:, dt * 128:(dt + 1) * 128]
                for i, sig in enumerate(MSIG):
                    m0 = 16 * len(XSIG) + 8 * i
                    sbuf[m0:m0 + 8, :] = _pk(_lin([(c, tile(mem, dt)) for dt, c in sig]))
                for n, xy in enumerate(zip(h1n, h2n)):
                    for i, sig in enumerate(XSIG):
                        sbuf[16 * i + 8 * n:16 * i + 8 * n + 8, :] = _pk(
                            _lin([(c, tile(xy[row], dt)) for row, dt, c in sig]))
            if mode == 0:
                obuf[...] = o[2 * M:]
            elif mode == 1:
                obuf[0:SEG, :] = o[2 * M:]
            else:
                obuf[SEG:2 * SEG, :] = o[2 * M:]

        with _scope("pro"):
            vis, fill = masks(1)
            kv_units = sum_units(1) + sum_units(2)
            cut = len(kv_units) * 2 // 3
            step(0, 1, vis, fill, False, wo_copy.wait, units=kv_units[:cut])
            step(1, 1, vis, fill, True, units=kv_units[cut:] + sum_units(3))
        xb_copy.start()
        vis, fill = masks(0)
        with _scope("main_a"):
            loop(NA // UA, lambda i: [step(UA * i + u + LAG, 0, vis, fill, u > 0, early=UA * i + u)
                                      for u in range(UA)])
        xb_copy.wait()
        with _scope("conv_e"):
            loop(HB // UI, lambda j: [inv_stage(HB + UI * j + u) for u in range(UI)])
        with _scope("main_b"):
            loop((NSEG - LAG - NA) // UB, lambda i: [step(UB * i + u + LAG + NA, 0, vis, fill, u > 0)
                                                     for u in range(UB)])
        done = (NSEG - 1 - LAG) * SEG
        out_a = pltpu.make_async_copy(out_s.at[0:done, :], out_hbm.at[0:done, :], sem.at[SW + 8])
        out_a.start()
        with _scope("epi"):
            vis, fill = masks(2)
            step(NSEG, 2, vis, fill)
            step(NSEG + 1, 2, *masks(2, 2 * M), True)
        post2(NSEG + LAG)
        out_b = pltpu.make_async_copy(out_s.at[done:S, :], out_hbm.at[done:S, :], sem.at[SW + 9])
        out_b.start()
        out_a.wait()
        out_b.wait()

    pl.run_scoped(
        phase1,
        pltpu.VMEM((NSUM * 64, 128), U32),
        pltpu.VMEM((2 * NSUM * 64, 128), U32),
        pltpu.VMEM((NSUM * 64, 128), U32),
    )


@jax.jit
def pallas_interleave_layers__memory_aug_recurrent_mem_tr__ssm_conv_h3__prompt_kernel(
    A_x, A_mem0, A_Wq, A_Wk, A_Wv, A_Wo, A_seg_len,
    B_q, B_k, B_v, B_shift_k, B_ssm_k, B_ssm_D,
):
    del A_seg_len, B_q
    assert A_x.shape == (1, S, D) and A_Wq.shape == (D, H, DH)
    hbm = pl.BlockSpec(memory_space=pl.ANY)
    out = pl.pallas_call(
        _kernel,
        out_shape=jax.ShapeDtypeStruct((S, D), BF16),
        in_specs=[hbm] * 11,
        out_specs=hbm,
        scratch_shapes=[
            pltpu.VMEM((S, D), BF16),
            pltpu.VMEM((H * WP + 352, 128), U32),
            pltpu.VMEM((2 * H * WP + 352, 128), U32),
            pltpu.VMEM((H * DH, D), BF16),
            pltpu.VMEM((NLB, H * DH // 2, 128), U32),
            pltpu.VMEM((TB // 2, TB), U32),
            pltpu.VMEM((2, TB // 2, TB), U32),
            pltpu.VMEM((2, TB // 2, TB), U32),
            pltpu.VMEM((NB, 2, NLB * TB, 128), F32),
            pltpu.VMEM((NB, 3, NLB * TB, 128), F32),
            pltpu.VMEM((NB + 1, 2, NLB * TB, 128), F32),
            pltpu.VMEM((NLB, S + 32, 128), F32),
            pltpu.VMEM((2 * SEG, D), F32),
            pltpu.VMEM((4, SEG, D), F32),
            pltpu.VMEM((S, D), BF16),
            pltpu.VMEM((NQH, NA * SEG, DH), BF16),
            pltpu.VMEM((128, D), BF16),
            pltpu.VMEM((320, 128), U32),
            pltpu.VMEM((64, D), BF16),
            pltpu.SemaphoreType.DMA((HB + HB // 2 + 14,)),
        ],
        compiler_params=pltpu.CompilerParams(vmem_limit_bytes=120 * 1024 * 1024),
    )(A_x.reshape(S, D), A_mem0.reshape(M, D), A_Wq, A_Wk, A_Wv,
      A_Wo.reshape(H * DH, D), B_k.reshape(S, D), B_v.reshape(S, D),
      B_shift_k.T, B_ssm_k, B_ssm_D)
    return out.reshape(1, S, D)
```

```python
import contextlib
import functools
import math

import jax
import jax.numpy as jnp
from jax import lax
import jax.experimental.pallas as pl
import jax.experimental.pallas.tpu as pltpu

F32 = jnp.float32
BF16 = jnp.bfloat16
U32 = jnp.uint32

S = 2048
D = 640
H = 32
DH = 128
M = 8
SEG = 32
NSEG = S // SEG
KS = 4
LAG = 2
ROWS = 2 * M + 2 * SEG
NLB = D // 128
TB = 128
NB = S // TB
HB = NB // 2
NPOS = NLB * TB // 8
NA = 20
PPS = 4
UCUT = tuple(range(a, a + 2) for a in range(0, 12, 2)) + (range(12, 16),)
NQH = 32
UA = 2
UB = 3
UI = 4
WP = 324


STRASSEN = (
    (((1, 0), (0, 1)), ((1, 0), (0, 1)), ((1, 0), (0, 1)), None),
    (((-1, 0), (1, 0)), ((1, 1), (0, 0)), ((0, 0), (0, 1)), None),
    (((0, 1), (0, -1)), ((0, 0), (1, 1)), ((1, 0), (0, 0)), None),
    (((0, 0), (1, 1)), ((1, 0), (0, 0)), ((0, 0), (1, -1)), ((1, 1), (1, 0))),
    (((1, 0), (0, 0)), ((0, 1), (0, -1)), ((0, 1), (0, 1)), ((1, 0), (0, 1))),
    (((0, 0), (0, 1)), ((-1, 0), (1, 0)), ((1, 0), (1, 0)), ((0, 1), (1, 0))),
    (((1, 1), (0, 0)), ((0, 0), (0, 1)), ((-1, 1), (0, 0)), ((1, 1), (0, 1))),
)
HOPKERR = (
    (((1, 0, 0), (0, 0, 0)), ((1, 0, 1), (-1, 0, 0), (0, 0, 0)), ((1, 0, 0), (1, 0, 0)), None),
    (((1, 1, 0), (0, 0, 0)), ((0, 0, 0), (1, 0, 0), (0, 0, 0)), ((1, -1, 0), (0, 0, 0)), None),
    (((-1, 0, 0), (1, 0, 1)), ((0, 0, 1), (0, 0, 0), (1, 0, 0)), ((1, 0, -1), (1, 0, 0)), None),
    (((0, 1, 0), (0, -1, 0)), ((0, 0, 0), (1, 1, 0), (0, -1, 0)), ((0, 1, 0), (0, 0, 0)), None),
    (((0, 1, 1), (0, -1, 0)), ((0, 0, 0), (0, 0, 1), (0, 1, 0)), ((0, 1, 0), (0, 1, -1)), None),
    (((0, 0, 1), (0, 0, 0)), ((0, 0, 0), (0, 0, -1), (1, 0, 1)), ((0, 0, 1), (0, 0, 0)), None),
    (((-1, 0, 0), (1, 0, 0)), ((1, 1, 0), (0, 0, 0), (-1, 0, 0)), ((0, 0, 0), (1, 0, 0)),
     ((1, 0, 0), (1, 0, 0))),
    (((1, 0, 0), (0, 1, 0)), ((0, 1, 0), (1, 0, 0), (0, 0, 0)), ((0, 1, 0), (1, 0, 0)),
     ((0, 1, 0), (1, 0, 0))),
    (((0, 0, 0), (1, 1, 0)), ((0, 1, 0), (0, 0, 0), (0, 0, 0)), ((0, 0, 0), (-1, 1, 0)),
     ((1, 1, 0), (-1, 1, 0))),
    (((0, 0, 0), (1, 0, 1)), ((0, 0, 1), (0, 0, 0), (0, 0, 0)), ((-1, 0, 1), (-1, 0, 1)),
     ((1, 0, 1), (0, 0, 1))),
    (((-1, 0, -1), (1, 0, 1)), ((0, 0, 0), (0, 0, 0), (1, 0, 0)), ((-1, 0, 1), (0, 0, 0)),
     ((1, 0, 1), (1, 0, 0))),
    (((0, 0, 0), (0, 1, 0)), ((0, -1, 0), (0, 1, 1), (0, 0, 0)), ((0, 1, 0), (0, 1, 0)),
     ((0, 1, 0), (0, 1, 0))),
    (((0, 1, 1), (0, 0, 0)), ((0, 0, 0), (0, 0, 1), (0, 0, 0)), ((0, -1, 1), (0, -1, 1)),
     ((0, 1, 0), (0, -1, 1))),
    (((0, -1, -1), (0, 1, 1)), ((0, 0, 0), (0, 0, 0), (0, 1, 0)), ((0, 0, 0), (0, 1, -1)),
     ((0, 0, 1), (0, 1, -1))),
    (((0, 0, 0), (0, 0, 1)), ((0, 0, -1), (0, 0, 0), (0, 1, 1)), ((0, 0, 0), (0, 0, 1)),
     ((0, 0, 1), (0, 0, 1))),
)
BLOCKS = ([(HOPKERR, (0, 1, 2), (3 * i, 3 * i + 1, 3 * i + 2)) for i in range(10)]
          + [(STRASSEN, (3, 4), (2 * i, 2 * i + 1)) for i in range(16)]
          + [(STRASSEN, (0, 1), (30, 31))])
GROUPS = [tuple(range(a, b)) for a, b in ((0, 6), (6, 12), (12, 18), (18, 24), (24, 32))]
NSUM = 10 * 9 + 17 * 5


def _nz(mat):
    return tuple((i, j, c) for i, row in enumerate(mat) for j, c in enumerate(row) if c)


def _summed(alg):
    return [p for p, e in enumerate(alg) if len(_nz(e[1])) > 1]


def _slot(b, p):
    sm = _summed(BLOCKS[b][0])
    if p not in sm:
        return None
    return (9 * b if b < 10 else 90 + 5 * (b - 10)) + sm.index(p)


def _lin(terms):
    terms = sorted(terms, key=lambda t: -t[0])
    acc = terms[0][1]
    for c, v in terms[1:]:
        acc = acc + v if c > 0 else acc - v
    return acc


class _Acc:
    def __init__(self):
        self.d = {}

    def add(self, key, c, v):
        if key not in self.d:
            self.d[key] = (c, v)
            return
        c0, v0 = self.d[key]
        self.d[key] = (c0, v0 + v) if c == c0 else (1, _lin([(c0, v0), (c, v)]))

    def route(self, e, ns, y):
        r = 0 if e[3] is None else 2 * M
        for row, n, c in _nz(e[2]):
            self.add((row + 1, ns[n]), c, y[r:])
        if r:
            for n, c in enumerate(e[3][1]):
                if c:
                    self.add((0, ns[n]), c, y[:r])

    def rows(self, n):
        assert all(self.d[(i, n)][0] == 1 for i in range(3))
        return jnp.concatenate([self.d[(i, n)][1] for i in range(3)], axis=0)


def _row_sigs():
    xs, ms = [], []
    for alg, dts, _ in BLOCKS:
        for e in alg:
            x = tuple((r, dts[k], c) for r, k, c in _nz(e[0]))
            if len(x) > 1 and x not in xs:
                xs.append(x)
            if e[3] is not None:
                m = tuple((dts[k], c) for k, c in enumerate(e[3][0]) if c)
                if len(m) > 1 and m not in ms:
                    ms.append(m)
    return xs, ms


XSIG, MSIG = _row_sigs()
OEXT = 240
PROFILE = False


def _scope(name):
    return jax.named_scope(name) if PROFILE else contextlib.nullcontext()


def _ln(x, toks=None):
    m = jnp.mean(x, axis=-1, keepdims=True)
    c = x - m
    v = jnp.mean(c * c, axis=-1, keepdims=True)
    r = lax.rsqrt(v + 1e-5)
    if toks is not None:
        toks.append(jnp.minimum(r, 0.0))
    return c * r


def _r(x):
    return x.astype(BF16).astype(F32)


def _split(x):
    hi = pltpu.bitcast(pltpu.bitcast(x, U32) & jnp.uint32(0xFFFF0000), F32)
    return hi, x - hi


def _pk(x):
    return pltpu.bitcast(x.astype(BF16), U32)


def _upk(w):
    return pltpu.bitcast(w, BF16)


def _basis(r, t):
    b = r & 63
    f = jnp.where(b < 32, 2 * b, 2 * b - 63)
    n = ((2 * f + 1) * t - jnp.where(r >= 64, TB, 0)) & (4 * TB - 1)
    n = jnp.where(n >= 2 * TB, n - 4 * TB, n)
    return jnp.cos(n.astype(F32) * (2.0 * math.pi / (4 * TB)))


def _halves(x):
    w = pltpu.bitcast(x, U32)
    return (pltpu.bitcast(w << 16, F32),
            pltpu.bitcast(w & jnp.uint32(0xFFFF0000), F32))


def _kernel(x_hbm, mem0_hbm, wq_hbm, wk_hbm, wv_hbm, wo_hbm,
            k_hbm, v_hbm, shk_hbm, ssmk_hbm, ssmd_hbm,
            out_hbm,
            x_s, wt_q, wt_kv, wo_s, wo_t,
            perm_s, fu_s, inv_s, u_s, kf_s, c_s, y_s,
            obuf, x2_s, out_s, qh_s, hbuf, sbuf, mem0_ref,
            sem):
    X0, XH = LAG * SEG, (LAG + NA) * SEG
    SW = HB + HB // 2
    hb = TB // 2
    wo_copy = pltpu.make_async_copy(wo_hbm, wo_s, sem.at[SW + 3])
    xb_copy = pltpu.make_async_copy(x_hbm.at[XH + SEG:, :], x_s.at[XH + SEG:, :], sem.at[SW + 7])

    def mac_units(row, half):
        rs = pl.ds(row, 8)
        state = {}

        def unit(p, avals, final, tok=None):
            acc = state.setdefault(p, dict(state.get(0, {})))
            for a in avals:
                u = u_s[a, 0, rs] + u_s[a, 1, rs] if p == 0 else u_s[a, p - 1, rs]
                if tok is not None:
                    u = u + tok
                for i in range(max(a, half * HB), half * HB + HB):
                    t = u * kf_s[i - a, p, rs]
                    acc[i] = t if i not in acc else (acc[i] - t if p == 2 else acc[i] + t)
            if final and p:
                for i, v in acc.items():
                    c_s[i + 1, 2 - p, rs] = v

        subs = UCUT if half else (range(HB),)
        return [functools.partial(unit, p, avals, n == len(subs) - 1)
                for p in range(3) for n, avals in enumerate(subs)]

    def inv_stage(i, units=None):
        q = TB // 4
        for g in range(NLB):
            re, im = [], []
            for b in range(4):
                rows = slice(g * TB + b * q, g * TB + (b + 1) * q)
                cr, ci_ = c_s[i + 1, 0, rows], c_s[i + 1, 1, rows]
                pr, pi = c_s[i, 0, rows], c_s[i, 1, rows]
                re.append(cr + pi if b in (0, 3) else cr - pi)
                im.append(ci_ - pr if b in (0, 3) else ci_ + pr)
            pe = jnp.concatenate([re[0] + re[2], re[1] + re[3], im[0] - im[2], im[1] - im[3]], axis=0)
            po = jnp.concatenate([re[0] - re[2], re[1] - re[3], im[0] + im[2], im[1] + im[3]], axis=0)
            for par, pp in enumerate((pe, po)):
                ph, plo = _split(pp)
                gh_, gl_ = (inv_s[n, par * q:(par + 1) * q] for n in range(2))
                y = jnp.dot(_upk(jnp.concatenate([gh_, gl_, gh_], axis=1)),
                            jnp.concatenate([ph, ph, plo], axis=0).astype(BF16),
                            preferred_element_type=F32)
                y_s[g, pl.ds(i * TB + par, hb, stride=2), :] = y
                if units:
                    tok = pltpu.bitcast(jnp.minimum(jnp.abs(y[0:16]), 0.0), U32)
                    for _ in range(3):
                        if units:
                            units.pop(0)(tok)

    def wslab(t, h):
        s0 = (max(t - 1, 0) * H + (h % 2) * 16 + h // 2) * WP
        return pltpu.bitcast((wt_kv if t else wt_q)[s0:s0 + D // 2, :], BF16)

    def loop(n, fn):
        def body(j, _):
            fn(j)
            return 0
        lax.fori_loop(0, n, body, 0)

    def phase0(k_s, v_s, ssmk_s, wraw, kpad, hl_s, shk_ref, ssmd_ref):

        def pair_rows(jp):
            r0 = jp * 2 * TB
            return pl.ds(r0 if isinstance(jp, int) else pl.multiple_of(r0, 2 * TB), 2 * TB)

        def ssmk_copy(jp):
            return pltpu.make_async_copy(ssmk_hbm.at[:, pair_rows(jp)], ssmk_s.at[jp], sem.at[jp])

        def kv_copies(rows, sm):
            return [pltpu.make_async_copy(k_hbm.at[rows, :], k_s.at[rows, :], sm),
                    pltpu.make_async_copy(v_hbm.at[rows, :], v_s.at[rows, :], sm)]
        DQ = 192
        wq_early = [pltpu.make_async_copy(wq_hbm.at[n * DQ:(n + 1) * DQ], wraw.at[0, n * DQ:(n + 1) * DQ],
                                          sem.at[SW + 10 + n]) for n in range(2)]
        w_copies = [pltpu.make_async_copy(wq_hbm.at[2 * DQ:], wraw.at[0, 2 * DQ:], sem.at[SW])]
        w_copies += [pltpu.make_async_copy(w.at[n * (D // 2):(n + 1) * (D // 2)],
                                           wraw.at[t, n * (D // 2):(n + 1) * (D // 2)],
                                           sem.at[SW + 11 * n + t])
                     for t, w in ((1, wk_hbm), (2, wv_hbm)) for n in range(2)]
        late_copies = kv_copies(pl.ds(S // 2, S // 2), sem.at[SW + 4])
        small_copies = [pltpu.make_async_copy(src, dst, sem.at[SW + 5])
                        for src, dst in ((shk_hbm, shk_ref), (ssmd_hbm, ssmd_ref), (mem0_hbm, mem0_ref.at[0:M]))]
        XM = XH - 2 * TB
        xa_copy = pltpu.make_async_copy(x_hbm.at[X0:XM, :], x_s.at[X0:XM, :], sem.at[SW + 6])
        late_copies += [pltpu.make_async_copy(x_hbm.at[a:b, :], x_s.at[a:b, :], sem.at[SW + 4])
                        for a, b in ((0, X0), (XM, XH + SEG))]
        for c in (small_copies + [ssmk_copy(jp) for jp in range(HB)]
                  + [c for jp in range(HB // 2) for c in kv_copies(pair_rows(jp), sem.at[HB + jp])]
                  + [xa_copy] + wq_early + [w_copies[0]] + late_copies + w_copies[1:] + [wo_copy]):
            c.start()

        ri = lax.broadcasted_iota(jnp.int32, (TB, TB), 0)
        ci = lax.broadcasted_iota(jnp.int32, (TB, TB), 1)
        perm_s[...] = _pk(jnp.where(ci == 2 * (ri & 63) + (ri >> 6), 1.0, 0.0))
        tab = _basis(ri, 2 * (ci & 63) + (ci >> 6))
        hi, lo = _split(tab)
        fu_s[0] = _pk(jnp.where(ci < hb, hi, pltpu.roll(lo, hb, 1)))
        fu_s[1] = _pk(jnp.where(ci < hb, pltpu.roll(hi, hb, 1), lo))
        gh, gl = _split(tab.T * (1.0 / TB))
        inv_s[0] = _pk(gh)
        inv_s[1] = _pk(gl)

        for c in small_copies:
            c.wait()
        shk_t = shk_ref[...].astype(F32)
        taps = [[shk_t[j:j + 1, g * 128:(g + 1) * 128] for g in range(NLB)] for j in range(KS)]
        dvec = ssmd_ref[...].astype(F32).reshape(1, D)
        for g in range(NLB):
            kpad[0, g, 0:8, :] = jnp.zeros((8, 128), F32)
            kpad[1, g, 0:8, :] = jnp.zeros((8, 128), F32)
        c_s[0] = jnp.zeros(c_s.shape[1:], F32)
        hbuf[0:16, :] = jnp.concatenate([mem0_ref[0:M, :].astype(F32)] * 2, axis=0).astype(BF16)
        obuf[...] = jnp.zeros((2 * SEG, D), F32)
        x2_s[...] = jnp.zeros(x2_s.shape, F32)

        def spectrum(e, o):
            fe = jnp.dot(_upk(fu_s[0]), jnp.concatenate([e, e], axis=0).astype(BF16), preferred_element_type=F32)
            fo = jnp.dot(_upk(fu_s[1]), jnp.concatenate([o, o], axis=0).astype(BF16), preferred_element_type=F32)
            return ((fe[:hb] + fo[:hb], fe[hb:] + fo[hb:]), (fe[:hb] - fo[:hb], fo[hb:] - fe[hb:]))

        def freq_rows(g):
            return slice(g * TB, g * TB + hb), slice(g * TB + hb, (g + 1) * TB)

        def fwd_k(jq):
            def transposed(n):
                if n % 2 == 0:
                    ssmk_copy(2 * jq + n // 2).wait()
                blk = ssmk_s[2 * jq + n // 2, :, (n % 2) * TB:(n % 2 + 1) * TB]
                return lax.dot_general(_upk(perm_s[...]), blk, (((1,), (1,)), ((), ())),
                                       preferred_element_type=F32)
            nxt = transposed(0)
            for n in range(4):
                kt = nxt
                if n < 3:
                    nxt = transposed(n + 1)
                j = 4 * jq + n
                for g in range(NLB):
                    lb = slice(g * 128, (g + 1) * 128)
                    for rows, (kr, ki) in zip(freq_rows(g), spectrum(kt[:hb, lb], kt[hb:, lb])):
                        if n == 0:
                            kr = kr + jnp.where(j == 0, dvec[:, lb], 0.0)
                        kf_s[j, 0, rows] = kr
                        kf_s[j, 1, rows] = ki - kr
                        kf_s[j, 2, rows] = kr + ki

        def fwd_u(jq, first):
            if first:
                for jp in (2 * jq, 2 * jq + 1):
                    for c in kv_copies(pair_rows(jp), sem.at[HB + jp]):
                        c.wait()
            for j in [4 * jq + n for n in range(4)]:
                r0 = pl.multiple_of(j * TB, TB)
                q0 = pl.multiple_of(j * hb, hb) + 8
                for g in range(NLB):
                    lb = slice(g * 128, (g + 1) * 128)
                    ke, ko = _halves(k_s[pl.ds(r0, TB), lb])
                    ve, vo = _halves(v_s[pl.ds(r0, TB), lb])
                    kpad[0, g, pl.ds(q0, hb), :] = ke
                    kpad[1, g, pl.ds(q0, hb), :] = ko
                    ke1 = kpad[0, g, pl.ds(q0 - 1, hb), :]
                    ko1 = kpad[1, g, pl.ds(q0 - 1, hb), :]
                    ko2 = kpad[1, g, pl.ds(q0 - 2, hb), :]
                    t0, t1, t2, t3 = (taps[t][g] for t in range(KS))
                    e = (ke * t0 + ko1 * t1 + ke1 * t2 + ko2 * t3) * ve
                    o = (ko * t0 + ke * t1 + ko1 * t2 + ke1 * t3) * vo
                    for rows, (ur, ui) in zip(freq_rows(g), spectrum(e, o)):
                        u_s[j, 0, rows] = ur
                        u_s[j, 1, rows] = ui

        def relayout_rows(t, dst, base, dp, tok=None):
            a = pltpu.bitcast(wraw[t, 2 * dp], U32)
            b = pltpu.bitcast(wraw[t, 2 * dp + 1], U32)
            if tok is not None:
                a = a | tok
            dst[pl.ds(base + dp, 16, stride=WP), :] = (a & jnp.uint32(0xFFFF)) | (b << 16)
            dst[pl.ds(base + 16 * WP + dp, 16, stride=WP), :] = (
                (a >> 16) | (b & jnp.uint32(0xFFFF0000)))

        def norm_rows(r0, nr):
            r0 = pl.multiple_of(r0, 16)
            for r in range(0, nr, 16):
                hl_s[pl.ds(r0 + r, 16), :] = _ln(
                    x_s[pl.ds(r0 + r + LAG * SEG, 16), :].astype(F32)).astype(BF16)

        def pre_queries(c, t=None):
            per = -(-(D // 4) // NQH)
            for sub in range(2):
                if t is not None:
                    half = wraw.at[t, sub * (D // 2):(sub + 1) * (D // 2)]
                    pltpu.make_async_copy(half, half, sem.at[SW + 11 * sub + t]).wait()
                    base = (t - 1) * (H * WP)
                    dp = sub * (D // 4)
                r0 = pl.multiple_of((2 * c + sub) * QR, QR)
                hl = hl_s[pl.ds(r0, QR), :]
                for hd in range(NQH):
                    r = jnp.dot(hl, wslab(0, hd), preferred_element_type=F32)
                    qh_s[hd, pl.ds(r0, QR), :] = r.astype(BF16)
                    if t is not None:
                        tok = pltpu.bitcast(jnp.minimum(jnp.abs(r[0:16]), 0.0), U32)
                        for _ in range(per):
                            if dp < (sub + 1) * (D // 4):
                                relayout_rows(t, wt_kv, base, dp, tok)
                                dp += 1

        nch = NA * SEG // TB
        QR = TB // 2
        with _scope("conv_k"):
            loop(HB // 2, fwd_k)
        with _scope("conv_u"):
            loop(HB // 4, lambda j: fwd_u(j, True))
        with _scope("conv_b"):
            loop(NPOS // 10, lambda j: [u() for n in range(10)
                                        for u in mac_units(pl.multiple_of(80 * j, 16) + 8 * n, 0)])
            xa_copy.wait()

            def inv_first(j):
                part = wraw.at[0, pl.ds(j * DQ, DQ)]
                pltpu.make_async_copy(part, part, sem.at[SW + 10 + j]).wait()
                units = [functools.partial(relayout_rows, 0, wt_q, 0, j * (DQ // 2) + dd)
                         for dd in range(DQ // 2)]
                for u in range(UI):
                    inv_stage(UI * j + u, units)
                assert not units
                norm_rows(j * ((XM - X0) // 2), (XM - X0) // 2)
            loop(HB // UI, inv_first)
        with _scope("rel0"):
            w_copies[0].wait()
            loop((D - 2 * DQ) // 64,
                 lambda i: [relayout_rows(0, wt_q, 0, DQ + i * 32 + dd) for dd in range(32)])
        with _scope("preq"):
            loop(nch - 2, pre_queries)
        with _scope("conv_c"):
            for c in late_copies:
                c.wait()

            def fwd_u_late(j):
                r0 = pl.multiple_of(j * 16, 16)
                hbuf[pl.ds(16 + r0, 16), :] = _ln(x_s[pl.ds(r0, 16), :].astype(F32)).astype(BF16)
                norm_rows(XM - X0 + j * TB, TB)
                fwd_u(HB // 4 + j, False)
            loop(HB // 4, fwd_u_late)
        with _scope("preq_rel"):
            loop(2, lambda i: pre_queries(i + nch - 2, i + 1))

    pl.run_scoped(
        phase0,
        pltpu.VMEM((S, D), BF16),
        pltpu.VMEM((S, D), BF16),
        pltpu.VMEM((HB, D, 2 * TB), BF16),
        pltpu.VMEM((3, D, H, DH), BF16),
        pltpu.VMEM((2, NLB, S // 2 + 32, 128), F32),
        pltpu.VMEM((NA * SEG, D), BF16),
        pltpu.VMEM((KS, D), BF16),
        pltpu.VMEM((D,), BF16),
    )

    def phase1(cq, ckv, co):
        scale = DH ** -0.5

        def masks(mode, q0=0):
            rows = ROWS if mode == 0 else ROWS - SEG
            qi = lax.broadcasted_iota(jnp.int32, (rows - q0, 128), 0) + q0
            kj = lax.broadcasted_iota(jnp.int32, (rows - q0, 128), 1)

            def layer_of(i):
                xl = (i - 2 * M) // SEG if mode == 0 else mode - 1
                return jnp.where(i < 2 * M, i // M, xl)
            same = (layer_of(qi) == layer_of(kj)) & (kj < rows)
            vis = same & ((qi < 2 * M) | (qi >= kj))
            fill = jnp.where(same, -1e9 / scale, -jnp.inf).astype(F32)
            return vis, fill

        mem0 = mem0_ref[0:M, :].astype(F32)

        def seg_row(seg):
            if isinstance(seg, int):
                return min(max(seg, 0), NSEG - 1) * SEG
            return pl.multiple_of(jnp.clip(seg, 0, NSEG - 1) * SEG, SEG)

        def gate(xa, r0, toks=None):
            y = jnp.concatenate([y_s[g, pl.ds(r0, xa.shape[0]), :] for g in range(NLB)], axis=1)
            return xa + _ln(xa, toks) * y

        def mm(a, b):
            return jnp.dot(a, b, preferred_element_type=F32)

        def cat(vs, axis=0):
            return vs[0] if len(vs) == 1 else jnp.concatenate(vs, axis=axis)

        def plain_tile(t, dt, hd, r0=0, nr=64):
            if t == 3:
                return wo_t[dt, pl.ds(hd * 64 + r0, nr), :]
            s0 = (max(t - 1, 0) * H + (hd % 2) * 16 + hd // 2) * WP
            return (wt_kv if t else wt_q)[pl.ds(s0 + dt * 64 + r0, nr), :]

        def sum_ref(t):
            return (cq, ckv, ckv, co)[t], (NSUM * 64 if t == 2 else 0)

        def wtile(t, b, p):
            alg, dts, hds = BLOCKS[b]
            if _slot(b, p) is None:
                (k, n, _), = _nz(alg[p][1])
                return plain_tile(t, dts[n], hds[k]) if t == 3 else plain_tile(t, dts[k], hds[n])
            ref, r0 = sum_ref(t)
            r0 += _slot(b, p) * 64
            return ref[r0:r0 + 64, :]

        def sum_unit(t, alg, dts, hds, slot0, r0, tok):
            src = {}
            for k in range(len(dts)):
                for n in range(len(dts)):
                    w = (plain_tile(t, dts[n], hds[k], r0, 8) if t == 3
                         else plain_tile(t, dts[k], hds[n], r0, 8))
                    if (n - k) % len(dts) == len(dts) - 2:
                        w = w | pltpu.bitcast(tok[0:8], U32)
                    src[k, n] = _upk(w).astype(F32)
            ref, base = sum_ref(t)
            sums = _pk(jnp.concatenate([_lin([(c, src[k, n]) for k, n, c in _nz(alg[p][1])])
                                        for p in _summed(alg)], axis=1))
            for i in range(len(_summed(alg))):
                ref[pl.ds(base + (slot0 + i) * 64 + r0, 8), :] = sums[:, i * 128:(i + 1) * 128]

        def sum_units(t):
            jobs = [(b, r0) for b in range(len(BLOCKS)) for r0 in range(0, 64, 8)]
            jobs.sort(key=lambda j: (j[0] * 64 + j[1]) / 640 if j[0] < 10
                      else ((j[0] - 10) * 64 + j[1]) / (17 * 64))
            return [functools.partial(sum_unit, t, *BLOCKS[b], _slot(b, _summed(BLOCKS[b][0])[0]), r0)
                    for b, r0 in jobs]

        def attention(h, vis, fill, chained, before_oproj=None, early=None, due=(), fast=False,
                      units=()):
            q0 = h.shape[0] - vis.shape[0]
            r = 2 * M
            units, due = list(units), list(due)
            nprod = sum(len(b[0]) for b in BLOCKS) + 2
            ncall = (3 * H if before_oproj else 4 * H - 4) if not fast else (3 * nprod if early is None else 2 * nprod + 5 * H)
            nunit, state = len(units), [0]
            if early is not None:
                hrest = jnp.concatenate([h[:r], h[r + SEG:]], axis=0)
                qrow = pl.multiple_of(early * SEG, SEG)
            if fast:
                sb = sbuf[0:16 * len(XSIG) + 8 * len(MSIG), :]

            def feed(x, weight=1):
                state[0] += weight
                n = -(-nunit * state[0] // (ncall + OEXT * fast)) - (nunit - len(units))
                if n > 0:
                    tok = jnp.minimum(jnp.abs(x[0:16]), 0.0)
                    for u in units[:n]:
                        u(tok)
                    del units[:n]

            def left(e, dts):
                x = tuple((row, dts[k], c) for row, k, c in _nz(e[0]))
                if len(x) > 1:
                    parts = [_upk(sb[16 * XSIG.index(x):16 * XSIG.index(x) + 16])]
                else:
                    row, dt, _ = x[0]
                    parts = [h[r + row * SEG:r + (row + 1) * SEG, dt * 128:(dt + 1) * 128]]
                if e[3] is not None:
                    m = tuple((dts[k], c) for k, c in enumerate(e[3][0]) if c)
                    if len(m) > 1:
                        m0 = 16 * len(XSIG) + 8 * MSIG.index(m)
                        parts.insert(0, _upk(sb[m0:m0 + 8]))
                    else:
                        parts.insert(0, h[:r, m[0][0] * 128:(m[0][0] + 1) * 128])
                return cat(parts)

            def proj(g, hooks=()):
                hds = GROUPS[g]
                hooks = list(hooks)

                def tick(done, total):
                    if hooks and done * 3 >= total * (3 - len(hooks)):
                        hooks.pop(0)()
                res = [{} for _ in range(3)]
                first = g == 0 and chained
                kc = D - 128

                def plain(t, hd, part=None):
                    pre = early is not None and t == 0
                    x = hrest if pre else (h if t else h[q0:])
                    if part is None:
                        y = mm(x, wslab(t, hd))
                    else:
                        y = mm(x[:, kc:], wslab(t, hd)[kc:]) + part
                    feed(y, 5 if fast else 1)
                    if t == 0:
                        y = y.astype(BF16)
                    if pre:
                        y = jnp.concatenate([y[:r], qh_s[hd, pl.ds(qrow, SEG), :], y[r:]], axis=0)
                    res[t][hd] = y

                if not fast:
                    order = [(t, hd) for hd in hds for t in range(2)] + [(2, hd) for hd in hds]
                    parts = [mm((h if t else h[q0:])[:, :kc], wslab(t, hd)[:kc])
                             for t, hd in order[:4 if first else 0]]
                    for n, (t, hd) in enumerate(order):
                        tick(n, len(order))
                        plain(t, hd, parts[n] if n < len(parts) else None)
                    return res

                blocks = sorted((b for b in range(len(BLOCKS)) if BLOCKS[b][2][0] in hds),
                                key=lambda b: (min(BLOCKS[b][2]) + 2.5 * (b < 10), b))
                accs = [_Acc() for _ in range(3)]
                ts = [t for t in range(3) if t or early is None]

                def run(t, b, sel):
                    alg, dts, bh = BLOCKS[b]
                    for p, e in enumerate(alg):
                        if sel(e):
                            y = mm(left(e, dts), _upk(wtile(t, b, p)))
                            feed(y)
                            accs[t].route(e, bh, y)

                lead = [(t, b) for t in ts[:2] for b in blocks] if first else []
                for t, b in lead:
                    run(t, b, lambda e: e[3] is None)
                todo = list(hds) if early is not None else []
                start = state[0]
                total = ncall * len(hds) // H
                for t in ts:
                    for b in blocks:
                        tick(state[0] - start, total)
                        run(t, b, (lambda e: e[3] is not None) if (t, b) in lead else (lambda e: True))
                        for _ in range(2):
                            if todo and t == 1:
                                plain(0, todo.pop(0))
                    for hd in hds:
                        y = accs[t].rows(hd)
                        if hd >= 30:
                            y = mm(h[:, 256:384], _upk(plain_tile(t, 2, hd))) + y
                            feed(y)
                        res[t][hd] = y.astype(BF16) if t == 0 else y
                assert not todo and not hooks
                return res

            def pad(kv):
                return jnp.concatenate([kv, jnp.zeros((128 - kv.shape[0], DH), F32)],
                                       axis=0).astype(BF16)

            def probs(qkv, hds):
                scs = [lax.dot_general(qkv[0][hd], pad(qkv[1][hd]), (((1,), (1,)), ((), ())),
                                       preferred_element_type=F32) for hd in hds]
                ps = []
                for n, sc in enumerate(scs):
                    sc = jnp.where(vis, sc, fill)
                    e = jnp.exp2((sc - jnp.max(sc, axis=-1, keepdims=True))
                                 * (scale * math.log2(math.e)))
                    den = jnp.sum(e, axis=-1, keepdims=True)
                    if due and n == 0 and hds[0] >= 6:
                        e = jnp.concatenate([e[:16] + due.pop(0), e[16:]], axis=0)
                    rc = pl.reciprocal(den, approx=True)
                    rc = rc * (2.0 - den * rc)
                    ps.append((e * rc).astype(BF16))
                return ps

            def oproj(h0, h1, acc, mid=()):
                mid = list(mid)

                def put(key, y):
                    acc[key] = y + acc[key] if key in acc else y

                if not fast:
                    cuts = list(range(h0, h1, 5)) + [h1] if units else [h0, h1]
                    for n in range(NLB):
                        for a, b in zip(cuts, cuts[1:]):
                            if before_oproj is not None:
                                w = wo_s[a * DH:b * DH, n * 128:(n + 1) * 128]
                                wo_t[n, a * 64:b * 64, :] = pltpu.bitcast(w, U32)
                            else:
                                w = _upk(wo_t[n, a * 64:b * 64, :])
                            put(n, mm(jnp.concatenate(heads[a:b], axis=1).astype(BF16), w))
                            feed(acc[n])
                        if mid and n in (0, 2, 3):
                            mid.pop(0)()
                    return
                for dts in ((0, 1, 2), (3, 4), (0, 1)):
                    bs = [b for b in range(len(BLOCKS))
                          if BLOCKS[b][1] == dts and h0 <= BLOCKS[b][2][0] < h1]
                    for p, e in enumerate(BLOCKS[bs[0]][0]) if bs else ():
                        if mid and (len(dts), p) in ((3, 4), (3, 12), (2, 3)):
                            mid.pop(0)()
                        ls = []
                        for b in bs:
                            o = [heads[hd] for hd in BLOCKS[b][2]]
                            parts = [_lin([(c, o[k][r + row * SEG:r + (row + 1) * SEG])
                                           for row, k, c in _nz(e[0])])]
                            if e[3] is not None:
                                parts.insert(0, _lin([(c, o[k][:r])
                                                      for k, c in enumerate(e[3][0]) if c]))
                            ls.append(cat(parts))
                        put((dts, p), mm(cat(ls, 1).astype(BF16),
                                         _upk(cat([wtile(3, b, p) for b in bs]))))
                        feed(acc[dts, p], len(bs))
                if h1 == H:
                    put(2, mm(jnp.concatenate(heads[30:], axis=1).astype(BF16),
                              _upk(wo_t[2, 30 * 64:, :])))

            heads, acc = [], {}
            qkv = proj(0)
            for g, hds in enumerate(GROUPS):
                ha, hb_ = hds[:len(hds) // 2], hds[len(hds) // 2:]
                cur, ps = qkv, probs(qkv, ha)

                def weigh(sub):
                    heads.extend(mm(ps[hd - hds[0]], pad(cur[2][hd])) for hd in sub)
                hooks = [lambda: ps.extend(probs(cur, hb_)), lambda: weigh(ha)]
                if g + 1 < len(GROUPS):
                    qkv = proj(g + 1, hooks)
                    weigh(hb_)
                else:
                    if before_oproj is not None:
                        before_oproj()
                    oproj(0, 18, acc, hooks + [lambda: weigh(hb_)])
            oproj(18, H, acc)
            assert not units and not due
            if not fast:
                return jnp.concatenate([acc[n] for n in range(NLB)], axis=1)
            out = _Acc()
            for key, y in acc.items():
                if key != 2:
                    out.route((HOPKERR if len(key[0]) == 3 else STRASSEN)[key[1]], key[0], y)
            return jnp.concatenate([out.rows(n) + acc[2] if n == 2 else out.rows(n)
                                    for n in range(NLB)], axis=1)

        def post2(s, toks=None):
            r3 = seg_row(s - 1 - LAG)
            for r in (0, 16):
                xc = _r(x2_s[(s + 4 - 1 - LAG) % 4, r:r + 16] + obuf[SEG + r:SEG + r + 16, :])
                out_s[pl.ds(r3 + r, 16), :] = gate(xc, r3 + r, toks).astype(BF16)

        def step(s, mode, vis, fill, chained=False, before_oproj=None, early=None, units=()):
            if mode == 0:
                h = hbuf[0:ROWS, :]
            elif mode == 1:
                h = hbuf[0:48, :]
            else:
                live = lax.broadcasted_iota(jnp.int32, (2 * M, D), 0) >= M
                mem = jnp.where(live, hbuf[0:16, :].astype(F32), 0.0).astype(BF16)
                h = jnp.concatenate([mem, hbuf[48:80, :]], axis=0)
            toks = []
            if mode != 1:
                post2(s, toks)
            if isinstance(s, int) and s == NSEG + LAG - 1:
                obuf[SEG:2 * SEG, :] = attention(h, vis, fill, chained, due=toks)
                return
            r1 = seg_row(s - 1)
            rn = seg_row(s + 1)
            h1n, h2n = [], []
            for r in (0, 16):
                xa = _r(x_s[pl.ds(r1 + r, 16), :].astype(F32) + obuf[r:r + 16, :])
                xb2 = _r(gate(xa, r1 + r))
                h2n.append(_ln(xb2, toks))
                x2_s[(s + 4 - 1) % 4, r:r + 16] = xb2
            if mode != 2:
                for r in (0, 16):
                    h1n.append(_ln(x_s[pl.ds(rn + r, 16), :].astype(F32), toks))

            if early is not None:
                mrow = pl.multiple_of(early * (8 * PPS), 8 * PPS)
                units = [functools.partial(lambda u, tok: u(tok[0:8]), u)
                         for n in range(PPS) for u in mac_units(mrow + 8 * n, 1)]
                tb = early // 2
                units += [functools.partial(sum_unit, 0, HOPKERR, (0, 1, 2),
                                            (3 * tb, 3 * tb + 1, 3 * tb + 2), 9 * tb,
                                            (early % 2) * 32 + r0) for r0 in range(0, 32, 8)]
                pb = jnp.minimum(early, 16)
                k0, h0 = jnp.where(pb < 16, 3, 0), 2 * jnp.minimum(pb, 15)
                units += [functools.partial(sum_unit, 0, STRASSEN, (k0, k0 + 1), (h0, h0 + 1),
                                            90 + 5 * pb, r0) for r0 in range(0, 64, 8)]

            o = attention(h, vis, fill, chained, before_oproj, early, toks, mode == 0, units)

            mem2 = mem0 if mode == 1 else o[M:2 * M]
            mem = jnp.concatenate([o[0:M], mem2], axis=0)
            hbuf[0:16, :] = mem.astype(BF16)
            for n, v in enumerate(h1n):
                hbuf[16 + 16 * n:32 + 16 * n, :] = v.astype(BF16)
            for n, v in enumerate(h2n):
                hbuf[48 + 16 * n:64 + 16 * n, :] = v.astype(BF16)
            if mode != 2:
                tile = lambda v, dt: v[:, dt * 128:(dt + 1) * 128]
                for i, sig in enumerate(MSIG):
                    m0 = 16 * len(XSIG) + 8 * i
                    sbuf[m0:m0 + 8, :] = _pk(_lin([(c, tile(mem, dt)) for dt, c in sig]))
                for n, xy in enumerate(zip(h1n, h2n)):
                    for i, sig in enumerate(XSIG):
                        sbuf[16 * i + 8 * n:16 * i + 8 * n + 8, :] = _pk(
                            _lin([(c, tile(xy[row], dt)) for row, dt, c in sig]))
            if mode == 0:
                obuf[...] = o[2 * M:]
            elif mode == 1:
                obuf[0:SEG, :] = o[2 * M:]
            else:
                obuf[SEG:2 * SEG, :] = o[2 * M:]

        with _scope("pro"):
            vis, fill = masks(1)
            kv_units = sum_units(1) + sum_units(2)
            cut = len(kv_units) * 2 // 3
            step(0, 1, vis, fill, False, wo_copy.wait, units=kv_units[:cut])
            step(1, 1, vis, fill, True, units=kv_units[cut:] + sum_units(3))
        xb_copy.start()
        vis, fill = masks(0)
        with _scope("main_a"):
            loop(NA // UA, lambda i: [step(UA * i + u + LAG, 0, vis, fill, u > 0, early=UA * i + u)
                                      for u in range(UA)])
        xb_copy.wait()
        with _scope("conv_e"):
            loop(HB // UI, lambda j: [inv_stage(HB + UI * j + u) for u in range(UI)])
        with _scope("main_b"):
            loop((NSEG - LAG - NA) // UB, lambda i: [step(UB * i + u + LAG + NA, 0, vis, fill, u > 0)
                                                     for u in range(UB)])
        done = (NSEG - 1 - LAG) * SEG
        out_a = pltpu.make_async_copy(out_s.at[0:done, :], out_hbm.at[0:done, :], sem.at[SW + 8])
        out_a.start()
        with _scope("epi"):
            vis, fill = masks(2)
            step(NSEG, 2, vis, fill)
            step(NSEG + 1, 2, *masks(2, 2 * M), True)
        post2(NSEG + LAG)
        out_b = pltpu.make_async_copy(out_s.at[done:S, :], out_hbm.at[done:S, :], sem.at[SW + 9])
        out_b.start()
        out_a.wait()
        out_b.wait()

    pl.run_scoped(
        phase1,
        pltpu.VMEM((NSUM * 64, 128), U32),
        pltpu.VMEM((2 * NSUM * 64, 128), U32),
        pltpu.VMEM((NSUM * 64, 128), U32),
    )


@jax.jit
def pallas_interleave_layers__memory_aug_recurrent_mem_tr__ssm_conv_h3__prompt_kernel(
    A_x, A_mem0, A_Wq, A_Wk, A_Wv, A_Wo, A_seg_len,
    B_q, B_k, B_v, B_shift_k, B_ssm_k, B_ssm_D,
):
    del A_seg_len, B_q
    assert A_x.shape == (1, S, D) and A_Wq.shape == (D, H, DH)
    hbm = pl.BlockSpec(memory_space=pl.ANY)
    out = pl.pallas_call(
        _kernel,
        out_shape=jax.ShapeDtypeStruct((S, D), BF16),
        in_specs=[hbm] * 11,
        out_specs=hbm,
        scratch_shapes=[
            pltpu.VMEM((S, D), BF16),
            pltpu.VMEM((H * WP + 352, 128), U32),
            pltpu.VMEM((2 * H * WP + 352, 128), U32),
            pltpu.VMEM((H * DH, D), BF16),
            pltpu.VMEM((NLB, H * DH // 2, 128), U32),
            pltpu.VMEM((TB // 2, TB), U32),
            pltpu.VMEM((2, TB // 2, TB), U32),
            pltpu.VMEM((2, TB // 2, TB), U32),
            pltpu.VMEM((NB, 2, NLB * TB, 128), F32),
            pltpu.VMEM((NB, 3, NLB * TB, 128), F32),
            pltpu.VMEM((NB + 1, 2, NLB * TB, 128), F32),
            pltpu.VMEM((NLB, S + 32, 128), F32),
            pltpu.VMEM((2 * SEG, D), F32),
            pltpu.VMEM((4, SEG, D), F32),
            pltpu.VMEM((S, D), BF16),
            pltpu.VMEM((NQH, NA * SEG, DH), BF16),
            pltpu.VMEM((128, D), BF16),
            pltpu.VMEM((320, 128), U32),
            pltpu.VMEM((64, D), BF16),
            pltpu.SemaphoreType.DMA((HB + HB // 2 + 14,)),
        ],
        compiler_params=pltpu.CompilerParams(vmem_limit_bytes=120 * 1024 * 1024),
    )(A_x.reshape(S, D), A_mem0.reshape(M, D), A_Wq, A_Wk, A_Wv,
      A_Wo.reshape(H * DH, D), B_k.reshape(S, D), B_v.reshape(S, D),
      B_shift_k.T, B_ssm_k, B_ssm_D)
    return out.reshape(1, S, D)
```

```python
import contextlib
import functools
import math

import jax
import jax.numpy as jnp
from jax import lax
import jax.experimental.pallas as pl
import jax.experimental.pallas.tpu as pltpu

F32 = jnp.float32
BF16 = jnp.bfloat16
U32 = jnp.uint32

S = 2048
D = 640
H = 32
DH = 128
M = 8
SEG = 32
NSEG = S // SEG
KS = 4
LAG = 2
ROWS = 2 * M + 2 * SEG
NLB = D // 128
TB = 128
NB = S // TB
HB = NB // 2
NPOS = NLB * TB // 8
NA = 20
PPS = 4
UCUT = tuple(range(a, a + 2) for a in range(0, 12, 2)) + (range(12, 16),)
NQH = 32
UA = 2
UB = 3
UI = 4
WP = 324


STRASSEN = (
    (((1, 0), (0, 1)), ((1, 0), (0, 1)), ((1, 0), (0, 1)), None),
    (((-1, 0), (1, 0)), ((1, 1), (0, 0)), ((0, 0), (0, 1)), None),
    (((0, 1), (0, -1)), ((0, 0), (1, 1)), ((1, 0), (0, 0)), None),
    (((0, 0), (1, 1)), ((1, 0), (0, 0)), ((0, 0), (1, -1)), ((1, 1), (1, 0))),
    (((1, 0), (0, 0)), ((0, 1), (0, -1)), ((0, 1), (0, 1)), ((1, 0), (0, 1))),
    (((0, 0), (0, 1)), ((-1, 0), (1, 0)), ((1, 0), (1, 0)), ((0, 1), (1, 0))),
    (((1, 1), (0, 0)), ((0, 0), (0, 1)), ((-1, 1), (0, 0)), ((1, 1), (0, 1))),
)
HOPKERR = (
    (((1, 0, 0), (0, 0, 0)), ((1, 0, 1), (-1, 0, 0), (0, 0, 0)), ((1, 0, 0), (1, 0, 0)), None),
    (((1, 1, 0), (0, 0, 0)), ((0, 0, 0), (1, 0, 0), (0, 0, 0)), ((1, -1, 0), (0, 0, 0)), None),
    (((-1, 0, 0), (1, 0, 1)), ((0, 0, 1), (0, 0, 0), (1, 0, 0)), ((1, 0, -1), (1, 0, 0)), None),
    (((0, 1, 0), (0, -1, 0)), ((0, 0, 0), (1, 1, 0), (0, -1, 0)), ((0, 1, 0), (0, 0, 0)), None),
    (((0, 1, 1), (0, -1, 0)), ((0, 0, 0), (0, 0, 1), (0, 1, 0)), ((0, 1, 0), (0, 1, -1)), None),
    (((0, 0, 1), (0, 0, 0)), ((0, 0, 0), (0, 0, -1), (1, 0, 1)), ((0, 0, 1), (0, 0, 0)), None),
    (((-1, 0, 0), (1, 0, 0)), ((1, 1, 0), (0, 0, 0), (-1, 0, 0)), ((0, 0, 0), (1, 0, 0)),
     ((1, 0, 0), (1, 0, 0))),
    (((1, 0, 0), (0, 1, 0)), ((0, 1, 0), (1, 0, 0), (0, 0, 0)), ((0, 1, 0), (1, 0, 0)),
     ((0, 1, 0), (1, 0, 0))),
    (((0, 0, 0), (1, 1, 0)), ((0, 1, 0), (0, 0, 0), (0, 0, 0)), ((0, 0, 0), (-1, 1, 0)),
     ((1, 1, 0), (-1, 1, 0))),
    (((0, 0, 0), (1, 0, 1)), ((0, 0, 1), (0, 0, 0), (0, 0, 0)), ((-1, 0, 1), (-1, 0, 1)),
     ((1, 0, 1), (0, 0, 1))),
    (((-1, 0, -1), (1, 0, 1)), ((0, 0, 0), (0, 0, 0), (1, 0, 0)), ((-1, 0, 1), (0, 0, 0)),
     ((1, 0, 1), (1, 0, 0))),
    (((0, 0, 0), (0, 1, 0)), ((0, -1, 0), (0, 1, 1), (0, 0, 0)), ((0, 1, 0), (0, 1, 0)),
     ((0, 1, 0), (0, 1, 0))),
    (((0, 1, 1), (0, 0, 0)), ((0, 0, 0), (0, 0, 1), (0, 0, 0)), ((0, -1, 1), (0, -1, 1)),
     ((0, 1, 0), (0, -1, 1))),
    (((0, -1, -1), (0, 1, 1)), ((0, 0, 0), (0, 0, 0), (0, 1, 0)), ((0, 0, 0), (0, 1, -1)),
     ((0, 0, 1), (0, 1, -1))),
    (((0, 0, 0), (0, 0, 1)), ((0, 0, -1), (0, 0, 0), (0, 1, 1)), ((0, 0, 0), (0, 0, 1)),
     ((0, 0, 1), (0, 0, 1))),
)
BLOCKS = ([(HOPKERR, (0, 1, 2), (3 * i, 3 * i + 1, 3 * i + 2)) for i in range(10)]
          + [(STRASSEN, (3, 4), (2 * i, 2 * i + 1)) for i in range(16)]
          + [(STRASSEN, (0, 1), (30, 31))])
GROUPS = [tuple(range(a, b)) for a, b in ((0, 6), (6, 12), (12, 18), (18, 24), (24, 32))]
NSUM = 10 * 9 + 17 * 5


def _nz(mat):
    return tuple((i, j, c) for i, row in enumerate(mat) for j, c in enumerate(row) if c)


def _summed(alg):
    return [p for p, e in enumerate(alg) if len(_nz(e[1])) > 1]


def _slot(b, p):
    sm = _summed(BLOCKS[b][0])
    if p not in sm:
        return None
    return (9 * b if b < 10 else 90 + 5 * (b - 10)) + sm.index(p)


def _lin(terms):
    terms = sorted(terms, key=lambda t: -t[0])
    acc = terms[0][1]
    for c, v in terms[1:]:
        acc = acc + v if c > 0 else acc - v
    return acc


class _Acc:
    def __init__(self):
        self.d = {}

    def add(self, key, c, v):
        if key not in self.d:
            self.d[key] = (c, v)
            return
        c0, v0 = self.d[key]
        self.d[key] = (c0, v0 + v) if c == c0 else (1, _lin([(c0, v0), (c, v)]))

    def route(self, e, ns, y):
        if e[3] is not None:
            ym, y = y[:2 * M], y[2 * M:]
            for n, c in enumerate(e[3][1]):
                if c:
                    self.add((0, ns[n]), c, ym)
        for row, n, c in _nz(e[2]):
            self.add((row + 1, ns[n]), c, y)

    def rows(self, n):
        assert all(self.d[(i, n)][0] == 1 for i in range(3))
        return jnp.concatenate([self.d[(i, n)][1] for i in range(3)], axis=0)


def _row_sigs():
    xs, ms = [], []
    for alg, dts, _ in BLOCKS:
        for e in alg:
            x = tuple((r, dts[k], c) for r, k, c in _nz(e[0]))
            if len(x) > 1 and x not in xs:
                xs.append(x)
            if e[3] is not None:
                m = tuple((dts[k], c) for k, c in enumerate(e[3][0]) if c)
                if len(m) > 1 and m not in ms:
                    ms.append(m)
    return xs, ms


XSIG, MSIG = _row_sigs()
OEXT = 240
PROFILE = False


def _scope(name):
    return jax.named_scope(name) if PROFILE else contextlib.nullcontext()


def _ln(x, toks=None):
    m = jnp.mean(x, axis=-1, keepdims=True)
    c = x - m
    v = jnp.mean(c * c, axis=-1, keepdims=True)
    r = lax.rsqrt(v + 1e-5)
    if toks is not None:
        toks.append(jnp.minimum(r, 0.0))
    return c * r


def _r(x):
    return x.astype(BF16).astype(F32)


def _split(x):
    hi = pltpu.bitcast(pltpu.bitcast(x, U32) & jnp.uint32(0xFFFF0000), F32)
    return hi, x - hi


def _pk(x):
    return pltpu.bitcast(x.astype(BF16), U32)


def _upk(w):
    return pltpu.bitcast(w, BF16)


def _basis(r, t):
    b = r & 63
    f = jnp.where(b < 32, 2 * b, 2 * b - 63)
    n = ((2 * f + 1) * t - jnp.where(r >= 64, TB, 0)) & (4 * TB - 1)
    n = jnp.where(n >= 2 * TB, n - 4 * TB, n)
    return jnp.cos(n.astype(F32) * (2.0 * math.pi / (4 * TB)))


def _halves(x):
    w = pltpu.bitcast(x, U32)
    return (pltpu.bitcast(w << 16, F32),
            pltpu.bitcast(w & jnp.uint32(0xFFFF0000), F32))


def _kernel(x_hbm, mem0_hbm, wq_hbm, wk_hbm, wv_hbm, wo_hbm,
            k_hbm, v_hbm, shk_hbm, ssmk_hbm, ssmd_hbm,
            out_hbm,
            x_s, wt_q, wt_kv, wo_s, wo_t,
            perm_s, fu_s, inv_s, u_s, kf_s, c_s, y_s,
            obuf, x2_s, out_s, qh_s, hbuf, sbuf, mem0_ref,
            sem):
    X0, XH = LAG * SEG, (LAG + NA) * SEG
    SW = HB + HB // 2
    hb = TB // 2
    wo_copy = pltpu.make_async_copy(wo_hbm, wo_s, sem.at[SW + 3])
    xb_copy = pltpu.make_async_copy(x_hbm.at[XH + SEG:, :], x_s.at[XH + SEG:, :], sem.at[SW + 7])

    def mac_units(row, half):
        rs = pl.ds(row, 8)
        state = {}

        def unit(p, avals, final, tok=None):
            acc = state.setdefault(p, dict(state.get(0, {})))
            for a in avals:
                u = u_s[a, 0, rs] + u_s[a, 1, rs] if p == 0 else u_s[a, p - 1, rs]
                if tok is not None:
                    u = u + tok
                for i in range(max(a, half * HB), half * HB + HB):
                    t = u * kf_s[i - a, p, rs]
                    acc[i] = t if i not in acc else (acc[i] - t if p == 2 else acc[i] + t)
            if final and p:
                for i, v in acc.items():
                    c_s[i + 1, 2 - p, rs] = v

        subs = UCUT if half else (range(HB),)
        return [functools.partial(unit, p, avals, n == len(subs) - 1)
                for p in range(3) for n, avals in enumerate(subs)]

    def inv_stage(i, units=None):
        q = TB // 4
        for g in range(NLB):
            re, im = [], []
            for b in range(4):
                rows = slice(g * TB + b * q, g * TB + (b + 1) * q)
                cr, ci_ = c_s[i + 1, 0, rows], c_s[i + 1, 1, rows]
                pr, pi = c_s[i, 0, rows], c_s[i, 1, rows]
                re.append(cr + pi if b in (0, 3) else cr - pi)
                im.append(ci_ - pr if b in (0, 3) else ci_ + pr)
            pe = jnp.concatenate([re[0] + re[2], re[1] + re[3], im[0] - im[2], im[1] - im[3]], axis=0)
            po = jnp.concatenate([re[0] - re[2], re[1] - re[3], im[0] + im[2], im[1] + im[3]], axis=0)
            for par, pp in enumerate((pe, po)):
                ph, plo = _split(pp)
                gh_, gl_ = (inv_s[n, par * q:(par + 1) * q] for n in range(2))
                y = jnp.dot(_upk(jnp.concatenate([gh_, gl_, gh_], axis=1)),
                            jnp.concatenate([ph, ph, plo], axis=0).astype(BF16),
                            preferred_element_type=F32)
                y_s[g, pl.ds(i * TB + par, hb, stride=2), :] = y
                if units:
                    tok = pltpu.bitcast(jnp.minimum(jnp.abs(y[0:16]), 0.0), U32)
                    for _ in range(3):
                        if units:
                            units.pop(0)(tok)

    def wslab(t, h):
        s0 = (max(t - 1, 0) * H + (h % 2) * 16 + h // 2) * WP
        return pltpu.bitcast((wt_kv if t else wt_q)[s0:s0 + D // 2, :], BF16)

    def loop(n, fn):
        def body(j, _):
            fn(j)
            return 0
        lax.fori_loop(0, n, body, 0)

    def phase0(k_s, v_s, ssmk_s, wraw, kpad, hl_s, shk_ref, ssmd_ref):

        def pair_rows(jp):
            r0 = jp * 2 * TB
            return pl.ds(r0 if isinstance(jp, int) else pl.multiple_of(r0, 2 * TB), 2 * TB)

        def ssmk_copy(jp):
            return pltpu.make_async_copy(ssmk_hbm.at[:, pair_rows(jp)], ssmk_s.at[jp], sem.at[jp])

        def kv_copies(rows, sm):
            return [pltpu.make_async_copy(k_hbm.at[rows, :], k_s.at[rows, :], sm),
                    pltpu.make_async_copy(v_hbm.at[rows, :], v_s.at[rows, :], sm)]
        DQ = 192
        wq_early = [pltpu.make_async_copy(wq_hbm.at[n * DQ:(n + 1) * DQ], wraw.at[0, n * DQ:(n + 1) * DQ],
                                          sem.at[SW + 10 + n]) for n in range(2)]
        w_copies = [pltpu.make_async_copy(wq_hbm.at[2 * DQ:], wraw.at[0, 2 * DQ:], sem.at[SW])]
        w_copies += [pltpu.make_async_copy(w.at[n * (D // 2):(n + 1) * (D // 2)],
                                           wraw.at[t, n * (D // 2):(n + 1) * (D // 2)],
                                           sem.at[SW + 11 * n + t])
                     for t, w in ((1, wk_hbm), (2, wv_hbm)) for n in range(2)]
        late_copies = kv_copies(pl.ds(S // 2, S // 2), sem.at[SW + 4])
        small_copies = [pltpu.make_async_copy(src, dst, sem.at[SW + 5])
                        for src, dst in ((shk_hbm, shk_ref), (ssmd_hbm, ssmd_ref), (mem0_hbm, mem0_ref.at[0:M]))]
        XM = XH - 2 * TB
        xa_copy = pltpu.make_async_copy(x_hbm.at[X0:XM, :], x_s.at[X0:XM, :], sem.at[SW + 6])
        late_copies += [pltpu.make_async_copy(x_hbm.at[a:b, :], x_s.at[a:b, :], sem.at[SW + 4])
                        for a, b in ((0, X0), (XM, XH + SEG))]
        for c in (small_copies + [ssmk_copy(jp) for jp in range(HB)]
                  + [c for jp in range(HB // 2) for c in kv_copies(pair_rows(jp), sem.at[HB + jp])]
                  + [xa_copy] + wq_early + [w_copies[0]] + late_copies + w_copies[1:] + [wo_copy]):
            c.start()

        ri = lax.broadcasted_iota(jnp.int32, (TB, TB), 0)
        ci = lax.broadcasted_iota(jnp.int32, (TB, TB), 1)
        perm_s[...] = _pk(jnp.where(ci == 2 * (ri & 63) + (ri >> 6), 1.0, 0.0))
        tab = _basis(ri, 2 * (ci & 63) + (ci >> 6))
        hi, lo = _split(tab)
        fu_s[0] = _pk(jnp.where(ci < hb, hi, pltpu.roll(lo, hb, 1)))
        fu_s[1] = _pk(jnp.where(ci < hb, pltpu.roll(hi, hb, 1), lo))
        gh, gl = _split(tab.T * (1.0 / TB))
        inv_s[0] = _pk(gh)
        inv_s[1] = _pk(gl)

        for c in small_copies:
            c.wait()
        shk_t = shk_ref[...].astype(F32)
        taps = [[shk_t[j:j + 1, g * 128:(g + 1) * 128] for g in range(NLB)] for j in range(KS)]
        dvec = ssmd_ref[...].astype(F32).reshape(1, D)
        for g in range(NLB):
            kpad[0, g, 0:8, :] = jnp.zeros((8, 128), F32)
            kpad[1, g, 0:8, :] = jnp.zeros((8, 128), F32)
        c_s[0] = jnp.zeros(c_s.shape[1:], F32)
        hbuf[0:16, :] = jnp.concatenate([mem0_ref[0:M, :].astype(F32)] * 2, axis=0).astype(BF16)
        obuf[...] = jnp.zeros((2 * SEG, D), F32)
        x2_s[...] = jnp.zeros(x2_s.shape, F32)

        def spectrum(e, o):
            fe = jnp.dot(_upk(fu_s[0]), jnp.concatenate([e, e], axis=0).astype(BF16), preferred_element_type=F32)
            fo = jnp.dot(_upk(fu_s[1]), jnp.concatenate([o, o], axis=0).astype(BF16), preferred_element_type=F32)
            return ((fe[:hb] + fo[:hb], fe[hb:] + fo[hb:]), (fe[:hb] - fo[:hb], fo[hb:] - fe[hb:]))

        def freq_rows(g):
            return slice(g * TB, g * TB + hb), slice(g * TB + hb, (g + 1) * TB)

        def fwd_k(jq):
            def transposed(n):
                if n % 2 == 0:
                    ssmk_copy(2 * jq + n // 2).wait()
                blk = ssmk_s[2 * jq + n // 2, :, (n % 2) * TB:(n % 2 + 1) * TB]
                return lax.dot_general(_upk(perm_s[...]), blk, (((1,), (1,)), ((), ())),
                                       preferred_element_type=F32)
            nxt = transposed(0)
            for n in range(4):
                kt = nxt
                if n < 3:
                    nxt = transposed(n + 1)
                j = 4 * jq + n
                for g in range(NLB):
                    lb = slice(g * 128, (g + 1) * 128)
                    for rows, (kr, ki) in zip(freq_rows(g), spectrum(kt[:hb, lb], kt[hb:, lb])):
                        if n == 0:
                            kr = kr + jnp.where(j == 0, dvec[:, lb], 0.0)
                        kf_s[j, 0, rows] = kr
                        kf_s[j, 1, rows] = ki - kr
                        kf_s[j, 2, rows] = kr + ki

        def fwd_u(jq, first):
            if first:
                for jp in (2 * jq, 2 * jq + 1):
                    for c in kv_copies(pair_rows(jp), sem.at[HB + jp]):
                        c.wait()
            for j in [4 * jq + n for n in range(4)]:
                r0 = pl.multiple_of(j * TB, TB)
                q0 = pl.multiple_of(j * hb, hb) + 8
                for g in range(NLB):
                    lb = slice(g * 128, (g + 1) * 128)
                    ke, ko = _halves(k_s[pl.ds(r0, TB), lb])
                    ve, vo = _halves(v_s[pl.ds(r0, TB), lb])
                    kpad[0, g, pl.ds(q0, hb), :] = ke
                    kpad[1, g, pl.ds(q0, hb), :] = ko
                    ke1 = kpad[0, g, pl.ds(q0 - 1, hb), :]
                    ko1 = kpad[1, g, pl.ds(q0 - 1, hb), :]
                    ko2 = kpad[1, g, pl.ds(q0 - 2, hb), :]
                    t0, t1, t2, t3 = (taps[t][g] for t in range(KS))
                    e = (ke * t0 + ko1 * t1 + ke1 * t2 + ko2 * t3) * ve
                    o = (ko * t0 + ke * t1 + ko1 * t2 + ke1 * t3) * vo
                    for rows, (ur, ui) in zip(freq_rows(g), spectrum(e, o)):
                        u_s[j, 0, rows] = ur
                        u_s[j, 1, rows] = ui

        def relayout_rows(t, dst, base, dp, tok=None):
            a = pltpu.bitcast(wraw[t, 2 * dp], U32)
            b = pltpu.bitcast(wraw[t, 2 * dp + 1], U32)
            if tok is not None:
                a = a | tok
            dst[pl.ds(base + dp, 16, stride=WP), :] = (a & jnp.uint32(0xFFFF)) | (b << 16)
            dst[pl.ds(base + 16 * WP + dp, 16, stride=WP), :] = (
                (a >> 16) | (b & jnp.uint32(0xFFFF0000)))

        def norm_rows(r0, nr):
            r0 = pl.multiple_of(r0, 16)
            for r in range(0, nr, 16):
                hl_s[pl.ds(r0 + r, 16), :] = _ln(
                    x_s[pl.ds(r0 + r + LAG * SEG, 16), :].astype(F32)).astype(BF16)

        def pre_queries(c, t=None):
            per = -(-(D // 4) // NQH)
            for sub in range(2):
                if t is not None:
                    half = wraw.at[t, sub * (D // 2):(sub + 1) * (D // 2)]
                    pltpu.make_async_copy(half, half, sem.at[SW + 11 * sub + t]).wait()
                    base = (t - 1) * (H * WP)
                    dp = sub * (D // 4)
                r0 = pl.multiple_of((2 * c + sub) * QR, QR)
                hl = hl_s[pl.ds(r0, QR), :]
                for hd in range(NQH):
                    r = jnp.dot(hl, wslab(0, hd), preferred_element_type=F32)
                    qh_s[hd, pl.ds(r0, QR), :] = r.astype(BF16)
                    if t is not None:
                        tok = pltpu.bitcast(jnp.minimum(jnp.abs(r[0:16]), 0.0), U32)
                        for _ in range(per):
                            if dp < (sub + 1) * (D // 4):
                                relayout_rows(t, wt_kv, base, dp, tok)
                                dp += 1

        nch = NA * SEG // TB
        QR = TB // 2
        with _scope("conv_k"):
            loop(HB // 2, fwd_k)
        with _scope("conv_u"):
            loop(HB // 4, lambda j: fwd_u(j, True))
        with _scope("conv_b"):
            loop(NPOS // 10, lambda j: [u() for n in range(10)
                                        for u in mac_units(pl.multiple_of(80 * j, 16) + 8 * n, 0)])
            xa_copy.wait()

            def inv_first(j):
                part = wraw.at[0, pl.ds(j * DQ, DQ)]
                pltpu.make_async_copy(part, part, sem.at[SW + 10 + j]).wait()
                units = [functools.partial(relayout_rows, 0, wt_q, 0, j * (DQ // 2) + dd)
                         for dd in range(DQ // 2)]
                for u in range(UI):
                    inv_stage(UI * j + u, units)
                assert not units
                norm_rows(j * ((XM - X0) // 2), (XM - X0) // 2)
            loop(HB // UI, inv_first)
        with _scope("rel0"):
            w_copies[0].wait()
            loop((D - 2 * DQ) // 64,
                 lambda i: [relayout_rows(0, wt_q, 0, DQ + i * 32 + dd) for dd in range(32)])
        with _scope("preq"):
            loop(nch - 2, pre_queries)
        with _scope("conv_c"):
            for c in late_copies:
                c.wait()

            def fwd_u_late(j):
                r0 = pl.multiple_of(j * 16, 16)
                hbuf[pl.ds(16 + r0, 16), :] = _ln(x_s[pl.ds(r0, 16), :].astype(F32)).astype(BF16)
                norm_rows(XM - X0 + j * TB, TB)
                fwd_u(HB // 4 + j, False)
            loop(HB // 4, fwd_u_late)
        with _scope("preq_rel"):
            loop(2, lambda i: pre_queries(i + nch - 2, i + 1))

    pl.run_scoped(
        phase0,
        pltpu.VMEM((S, D), BF16),
        pltpu.VMEM((S, D), BF16),
        pltpu.VMEM((HB, D, 2 * TB), BF16),
        pltpu.VMEM((3, D, H, DH), BF16),
        pltpu.VMEM((2, NLB, S // 2 + 32, 128), F32),
        pltpu.VMEM((NA * SEG, D), BF16),
        pltpu.VMEM((KS, D), BF16),
        pltpu.VMEM((D,), BF16),
    )

    def phase1(cq, ckv, co):
        scale = DH ** -0.5

        def masks(mode, q0=0):
            rows = ROWS if mode == 0 else ROWS - SEG
            qi = lax.broadcasted_iota(jnp.int32, (rows - q0, 128), 0) + q0
            kj = lax.broadcasted_iota(jnp.int32, (rows - q0, 128), 1)

            def layer_of(i):
                xl = (i - 2 * M) // SEG if mode == 0 else mode - 1
                return jnp.where(i < 2 * M, i // M, xl)
            same = (layer_of(qi) == layer_of(kj)) & (kj < rows)
            vis = same & ((qi < 2 * M) | (qi >= kj))
            fill = jnp.where(same, -1e9 / scale, -jnp.inf).astype(F32)
            return vis, fill

        mem0 = mem0_ref[0:M, :].astype(F32)

        def seg_row(seg):
            if isinstance(seg, int):
                return min(max(seg, 0), NSEG - 1) * SEG
            return pl.multiple_of(jnp.clip(seg, 0, NSEG - 1) * SEG, SEG)

        def gate(xa, r0, toks=None):
            y = jnp.concatenate([y_s[g, pl.ds(r0, xa.shape[0]), :] for g in range(NLB)], axis=1)
            return xa + _ln(xa, toks) * y

        def mm(a, b):
            return jnp.dot(a, b, preferred_element_type=F32)

        def cat(vs, axis=0):
            return vs[0] if len(vs) == 1 else jnp.concatenate(vs, axis=axis)

        def plain_tile(t, dt, hd, r0=0, nr=64):
            if t == 3:
                return wo_t[dt, pl.ds(hd * 64 + r0, nr), :]
            s0 = (max(t - 1, 0) * H + (hd % 2) * 16 + hd // 2) * WP
            return (wt_kv if t else wt_q)[pl.ds(s0 + dt * 64 + r0, nr), :]

        def sum_ref(t):
            return (cq, ckv, ckv, co)[t], (NSUM * 64 if t == 2 else 0)

        def wtile(t, b, p):
            alg, dts, hds = BLOCKS[b]
            if _slot(b, p) is None:
                (k, n, _), = _nz(alg[p][1])
                return plain_tile(t, dts[n], hds[k]) if t == 3 else plain_tile(t, dts[k], hds[n])
            ref, r0 = sum_ref(t)
            r0 += _slot(b, p) * 64
            return ref[r0:r0 + 64, :]

        def sum_unit(t, alg, dts, hds, slot0, r0, tok):
            src = {}
            for k in range(len(dts)):
                for n in range(len(dts)):
                    w = (plain_tile(t, dts[n], hds[k], r0, 8) if t == 3
                         else plain_tile(t, dts[k], hds[n], r0, 8))
                    if (n - k) % len(dts) == len(dts) - 2:
                        w = w | pltpu.bitcast(tok[0:8], U32)
                    src[k, n] = _upk(w).astype(F32)
            ref, base = sum_ref(t)
            sums = _pk(jnp.concatenate([_lin([(c, src[k, n]) for k, n, c in _nz(alg[p][1])])
                                        for p in _summed(alg)], axis=1))
            for i in range(len(_summed(alg))):
                ref[pl.ds(base + (slot0 + i) * 64 + r0, 8), :] = sums[:, i * 128:(i + 1) * 128]

        def sum_units(t):
            jobs = [(b, r0) for b in range(len(BLOCKS)) for r0 in range(0, 64, 8)]
            jobs.sort(key=lambda j: (j[0] * 64 + j[1]) / 640 if j[0] < 10
                      else ((j[0] - 10) * 64 + j[1]) / (17 * 64))
            return [functools.partial(sum_unit, t, *BLOCKS[b], _slot(b, _summed(BLOCKS[b][0])[0]), r0)
                    for b, r0 in jobs]

        def attention(h, vis, fill, chained, before_oproj=None, early=None, due=(), fast=False,
                      units=()):
            q0 = h.shape[0] - vis.shape[0]
            r = 2 * M
            units, due = list(units), list(due)
            nprod = sum(len(b[0]) for b in BLOCKS) + 2
            ncall = (3 * H if before_oproj else 4 * H - 4) if not fast else (3 * nprod if early is None else 2 * nprod + 5 * H)
            nunit, state = len(units), [0]
            if early is not None:
                hrest = jnp.concatenate([h[:r], h[r + SEG:]], axis=0)
                qrow = pl.multiple_of(early * SEG, SEG)
            if fast:
                sb = sbuf[0:16 * len(XSIG) + 8 * len(MSIG), :]

            def feed(x, weight=1):
                state[0] += weight
                n = -(-nunit * state[0] // (ncall + OEXT * fast)) - (nunit - len(units))
                if n > 0:
                    tok = jnp.minimum(jnp.abs(x[0:16]), 0.0)
                    for u in units[:n]:
                        u(tok)
                    del units[:n]

            @functools.cache
            def left(e, dts):
                x = tuple((row, dts[k], c) for row, k, c in _nz(e[0]))
                if len(x) > 1:
                    parts = [_upk(sb[16 * XSIG.index(x):16 * XSIG.index(x) + 16])]
                else:
                    row, dt, _ = x[0]
                    parts = [h[r + row * SEG:r + (row + 1) * SEG, dt * 128:(dt + 1) * 128]]
                if e[3] is not None:
                    m = tuple((dts[k], c) for k, c in enumerate(e[3][0]) if c)
                    if len(m) > 1:
                        m0 = 16 * len(XSIG) + 8 * MSIG.index(m)
                        parts.insert(0, _upk(sb[m0:m0 + 8]))
                    else:
                        parts.insert(0, h[:r, m[0][0] * 128:(m[0][0] + 1) * 128])
                return cat(parts)

            def proj(g, hooks=()):
                hds = GROUPS[g]
                hooks = list(hooks)

                def tick(done, total):
                    if hooks and done * 3 >= total * (3 - len(hooks)):
                        hooks.pop(0)()
                res = [{} for _ in range(3)]
                first = g == 0 and chained
                kc = D - 128

                def plain(t, hd, part=None):
                    pre = early is not None and t == 0
                    x = hrest if pre else (h if t else h[q0:])
                    if part is None:
                        y = mm(x, wslab(t, hd))
                    else:
                        y = mm(x[:, kc:], wslab(t, hd)[kc:]) + part
                    feed(y, 5 if fast else 1)
                    if t == 0:
                        y = y.astype(BF16)
                    if pre:
                        y = jnp.concatenate([y[:r], qh_s[hd, pl.ds(qrow, SEG), :], y[r:]], axis=0)
                    res[t][hd] = y

                if not fast:
                    order = [(t, hd) for hd in hds for t in range(2)] + [(2, hd) for hd in hds]
                    parts = [mm((h if t else h[q0:])[:, :kc], wslab(t, hd)[:kc])
                             for t, hd in order[:4 if first else 0]]
                    for n, (t, hd) in enumerate(order):
                        tick(n, len(order))
                        plain(t, hd, parts[n] if n < len(parts) else None)
                    return res

                blocks = sorted((b for b in range(len(BLOCKS)) if BLOCKS[b][2][0] in hds),
                                key=lambda b: (min(BLOCKS[b][2]) + 2.5 * (b < 10), b))
                accs = [_Acc() for _ in range(3)]
                ts = [t for t in range(3) if t or early is None]

                def run(t, b, sel):
                    alg, dts, bh = BLOCKS[b]
                    for p, e in enumerate(alg):
                        if sel(e):
                            y = mm(left(e, dts), _upk(wtile(t, b, p)))
                            feed(y)
                            accs[t].route(e, bh, y)

                lead = [(t, b) for t in ts[:2] for b in blocks] if first else []
                for t, b in lead:
                    run(t, b, lambda e: e[3] is None)
                todo = list(hds) if early is not None else []
                start = state[0]
                total = ncall * len(hds) // H
                for t in ts:
                    for b in blocks:
                        tick(state[0] - start, total)
                        run(t, b, (lambda e: e[3] is not None) if (t, b) in lead else (lambda e: True))
                        for _ in range(2):
                            if todo and t == 1:
                                plain(0, todo.pop(0))
                    for hd in hds:
                        y = accs[t].rows(hd)
                        if hd >= 30:
                            y = mm(h[:, 256:384], _upk(plain_tile(t, 2, hd))) + y
                            feed(y)
                        res[t][hd] = y.astype(BF16) if t == 0 else y
                assert not todo and not hooks
                return res

            def pad(kv):
                return jnp.concatenate([kv, jnp.zeros((128 - kv.shape[0], DH), F32)],
                                       axis=0).astype(BF16)

            def probs(qkv, hds):
                scs = [lax.dot_general(qkv[0][hd], pad(qkv[1][hd]), (((1,), (1,)), ((), ())),
                                       preferred_element_type=F32) for hd in hds]
                ps = []
                for n, sc in enumerate(scs):
                    sc = jnp.where(vis, sc, fill)
                    e = jnp.exp2((sc - jnp.max(sc, axis=-1, keepdims=True))
                                 * (scale * math.log2(math.e)))
                    den = jnp.sum(e, axis=-1, keepdims=True)
                    if due and n == 0 and hds[0] >= 6:
                        e = jnp.concatenate([e[:16] + due.pop(0), e[16:]], axis=0)
                    rc = pl.reciprocal(den, approx=True)
                    rc = rc * (2.0 - den * rc)
                    ps.append((e * rc).astype(BF16))
                return ps

            @functools.cache
            def head_rows(hd):
                return heads[hd][:r], heads[hd][r:r + SEG], heads[hd][r + SEG:]

            def oproj(h0, h1, acc, mid=()):
                mid = list(mid)

                def put(key, y):
                    acc[key] = y + acc[key] if key in acc else y

                if not fast:
                    cuts = list(range(h0, h1, 5)) + [h1] if units else [h0, h1]
                    for n in range(NLB):
                        for a, b in zip(cuts, cuts[1:]):
                            if before_oproj is not None:
                                w = wo_s[a * DH:b * DH, n * 128:(n + 1) * 128]
                                wo_t[n, a * 64:b * 64, :] = pltpu.bitcast(w, U32)
                            else:
                                w = _upk(wo_t[n, a * 64:b * 64, :])
                            put(n, mm(jnp.concatenate(heads[a:b], axis=1).astype(BF16), w))
                            feed(acc[n])
                        if mid and n in (0, 2, 3):
                            mid.pop(0)()
                    return
                for dts in ((0, 1, 2), (3, 4), (0, 1)):
                    bs = [b for b in range(len(BLOCKS))
                          if BLOCKS[b][1] == dts and h0 <= BLOCKS[b][2][0] < h1]
                    for p, e in enumerate(BLOCKS[bs[0]][0]) if bs else ():
                        if mid and (len(dts), p) in ((3, 3), (3, 11), (2, 1)):
                            mid.pop(0)()
                        ls = []
                        for b in bs:
                            o = [head_rows(hd) for hd in BLOCKS[b][2]]
                            parts = [_lin([(c, o[k][row + 1]) for row, k, c in _nz(e[0])])]
                            if e[3] is not None:
                                parts.insert(0, _lin([(c, o[k][0])
                                                      for k, c in enumerate(e[3][0]) if c]))
                            ls.append(cat(parts))
                        put((dts, p), mm(cat(ls, 1).astype(BF16),
                                         _upk(cat([wtile(3, b, p) for b in bs]))))
                        feed(acc[dts, p], len(bs))
                if h1 == H:
                    put(2, mm(jnp.concatenate(heads[30:], axis=1).astype(BF16),
                              _upk(wo_t[2, 30 * 64:, :])))

            heads, acc = [], {}
            qkv = proj(0)
            for g, hds in enumerate(GROUPS):
                ha, hb_ = hds[:len(hds) // 2], hds[len(hds) // 2:]
                cur, ps = qkv, probs(qkv, ha)

                def weigh(sub):
                    heads.extend(mm(ps[hd - hds[0]], pad(cur[2][hd])) for hd in sub)
                hooks = [lambda: ps.extend(probs(cur, hb_)), lambda: weigh(ha)]
                if g + 1 < len(GROUPS):
                    qkv = proj(g + 1, hooks)
                    weigh(hb_)
                else:
                    if before_oproj is not None:
                        before_oproj()
                    oproj(0, 18, acc, hooks + [lambda: weigh(hb_)])
            oproj(18, H, acc)
            assert not units and not due
            if not fast:
                return jnp.concatenate([acc[n] for n in range(NLB)], axis=1)
            out = _Acc()
            for key, y in acc.items():
                if key != 2:
                    out.route((HOPKERR if len(key[0]) == 3 else STRASSEN)[key[1]], key[0], y)
            return jnp.concatenate([out.rows(n) + acc[2] if n == 2 else out.rows(n)
                                    for n in range(NLB)], axis=1)

        def post2(s, toks=None):
            r3 = seg_row(s - 1 - LAG)
            for r in (0, 16):
                xc = _r(x2_s[(s + 4 - 1 - LAG) % 4, r:r + 16] + obuf[SEG + r:SEG + r + 16, :])
                out_s[pl.ds(r3 + r, 16), :] = gate(xc, r3 + r, toks).astype(BF16)

        def step(s, mode, vis, fill, chained=False, before_oproj=None, early=None, units=()):
            if mode == 0:
                h = hbuf[0:ROWS, :]
            elif mode == 1:
                h = hbuf[0:48, :]
            else:
                live = lax.broadcasted_iota(jnp.int32, (2 * M, D), 0) >= M
                mem = jnp.where(live, hbuf[0:16, :].astype(F32), 0.0).astype(BF16)
                h = jnp.concatenate([mem, hbuf[48:80, :]], axis=0)
            toks = []
            if mode != 1:
                post2(s, toks)
            if isinstance(s, int) and s == NSEG + LAG - 1:
                obuf[SEG:2 * SEG, :] = attention(h, vis, fill, chained, due=toks)
                return
            r1 = seg_row(s - 1)
            rn = seg_row(s + 1)
            h1n, h2n = [], []
            for r in (0, 16):
                xa = _r(x_s[pl.ds(r1 + r, 16), :].astype(F32) + obuf[r:r + 16, :])
                xb2 = _r(gate(xa, r1 + r))
                h2n.append(_ln(xb2, toks))
                x2_s[(s + 4 - 1) % 4, r:r + 16] = xb2
            if mode != 2:
                for r in (0, 16):
                    h1n.append(_ln(x_s[pl.ds(rn + r, 16), :].astype(F32), toks))

            if early is not None:
                mrow = pl.multiple_of(early * (8 * PPS), 8 * PPS)
                units = [functools.partial(lambda u, tok: u(tok[0:8]), u)
                         for n in range(PPS) for u in mac_units(mrow + 8 * n, 1)]
                tb = early // 2
                units += [functools.partial(sum_unit, 0, HOPKERR, (0, 1, 2),
                                            (3 * tb, 3 * tb + 1, 3 * tb + 2), 9 * tb,
                                            (early % 2) * 32 + r0) for r0 in range(0, 32, 8)]
                pb = jnp.minimum(early, 16)
                k0, h0 = jnp.where(pb < 16, 3, 0), 2 * jnp.minimum(pb, 15)
                units += [functools.partial(sum_unit, 0, STRASSEN, (k0, k0 + 1), (h0, h0 + 1),
                                            90 + 5 * pb, r0) for r0 in range(0, 64, 8)]

            o = attention(h, vis, fill, chained, before_oproj, early, toks, mode == 0, units)

            mem2 = mem0 if mode == 1 else o[M:2 * M]
            mem = jnp.concatenate([o[0:M], mem2], axis=0)
            hbuf[0:16, :] = mem.astype(BF16)
            for n, v in enumerate(h1n):
                hbuf[16 + 16 * n:32 + 16 * n, :] = v.astype(BF16)
            for n, v in enumerate(h2n):
                hbuf[48 + 16 * n:64 + 16 * n, :] = v.astype(BF16)
            if mode != 2:
                tile = lambda v, dt: v[:, dt * 128:(dt + 1) * 128]
                for i, sig in enumerate(MSIG):
                    m0 = 16 * len(XSIG) + 8 * i
                    sbuf[m0:m0 + 8, :] = _pk(_lin([(c, tile(mem, dt)) for dt, c in sig]))
                for n, xy in enumerate(zip(h1n, h2n)):
                    for i, sig in enumerate(XSIG):
                        sbuf[16 * i + 8 * n:16 * i + 8 * n + 8, :] = _pk(
                            _lin([(c, tile(xy[row], dt)) for row, dt, c in sig]))
            if mode == 0:
                obuf[...] = o[2 * M:]
            elif mode == 1:
                obuf[0:SEG, :] = o[2 * M:]
            else:
                obuf[SEG:2 * SEG, :] = o[2 * M:]

        with _scope("pro"):
            vis, fill = masks(1)
            kv_units = sum_units(1) + sum_units(2)
            cut = len(kv_units) * 2 // 3
            step(0, 1, vis, fill, False, wo_copy.wait, units=kv_units[:cut])
            step(1, 1, vis, fill, True, units=kv_units[cut:] + sum_units(3))
        xb_copy.start()
        vis, fill = masks(0)
        with _scope("main_a"):
            loop(NA // UA, lambda i: [step(UA * i + u + LAG, 0, vis, fill, u > 0, early=UA * i + u)
                                      for u in range(UA)])
        xb_copy.wait()
        with _scope("conv_e"):
            loop(HB // UI, lambda j: [inv_stage(HB + UI * j + u) for u in range(UI)])
        with _scope("main_b"):
            loop((NSEG - LAG - NA) // UB, lambda i: [step(UB * i + u + LAG + NA, 0, vis, fill, u > 0)
                                                     for u in range(UB)])
        done = (NSEG - 1 - LAG) * SEG
        out_a = pltpu.make_async_copy(out_s.at[0:done, :], out_hbm.at[0:done, :], sem.at[SW + 8])
        out_a.start()
        with _scope("epi"):
            vis, fill = masks(2)
            step(NSEG, 2, vis, fill)
            step(NSEG + 1, 2, *masks(2, 2 * M), True)
        post2(NSEG + LAG)
        out_b = pltpu.make_async_copy(out_s.at[done:S, :], out_hbm.at[done:S, :], sem.at[SW + 9])
        out_b.start()
        out_a.wait()
        out_b.wait()

    pl.run_scoped(
        phase1,
        pltpu.VMEM((NSUM * 64, 128), U32),
        pltpu.VMEM((2 * NSUM * 64, 128), U32),
        pltpu.VMEM((NSUM * 64, 128), U32),
    )


@jax.jit
def pallas_interleave_layers__memory_aug_recurrent_mem_tr__ssm_conv_h3__prompt_kernel(
    A_x, A_mem0, A_Wq, A_Wk, A_Wv, A_Wo, A_seg_len,
    B_q, B_k, B_v, B_shift_k, B_ssm_k, B_ssm_D,
):
    del A_seg_len, B_q
    assert A_x.shape == (1, S, D) and A_Wq.shape == (D, H, DH)
    hbm = pl.BlockSpec(memory_space=pl.ANY)
    out = pl.pallas_call(
        _kernel,
        out_shape=jax.ShapeDtypeStruct((S, D), BF16),
        in_specs=[hbm] * 11,
        out_specs=hbm,
        scratch_shapes=[
            pltpu.VMEM((S, D), BF16),
            pltpu.VMEM((H * WP + 352, 128), U32),
            pltpu.VMEM((2 * H * WP + 352, 128), U32),
            pltpu.VMEM((H * DH, D), BF16),
            pltpu.VMEM((NLB, H * DH // 2, 128), U32),
            pltpu.VMEM((TB // 2, TB), U32),
            pltpu.VMEM((2, TB // 2, TB), U32),
            pltpu.VMEM((2, TB // 2, TB), U32),
            pltpu.VMEM((NB, 2, NLB * TB, 128), F32),
            pltpu.VMEM((NB, 3, NLB * TB, 128), F32),
            pltpu.VMEM((NB + 1, 2, NLB * TB, 128), F32),
            pltpu.VMEM((NLB, S + 32, 128), F32),
            pltpu.VMEM((2 * SEG, D), F32),
            pltpu.VMEM((4, SEG, D), F32),
            pltpu.VMEM((S, D), BF16),
            pltpu.VMEM((NQH, NA * SEG, DH), BF16),
            pltpu.VMEM((128, D), BF16),
            pltpu.VMEM((320, 128), U32),
            pltpu.VMEM((64, D), BF16),
            pltpu.SemaphoreType.DMA((HB + HB // 2 + 14,)),
        ],
        compiler_params=pltpu.CompilerParams(vmem_limit_bytes=120 * 1024 * 1024),
    )(A_x.reshape(S, D), A_mem0.reshape(M, D), A_Wq, A_Wk, A_Wv,
      A_Wo.reshape(H * DH, D), B_k.reshape(S, D), B_v.reshape(S, D),
      B_shift_k.T, B_ssm_k, B_ssm_D)
    return out.reshape(1, S, D)
```
